```python
import jax
import jax.numpy as jnp

def _softmax(x, axis=-1):
    return jax.nn.softmax(x, axis=axis)
def _gelu(x):
    return jax.nn.gelu(x, approximate=True)
def _silu(x):
    return jax.nn.silu(x)
def _sigmoid(x):
    return jax.nn.sigmoid(x)
def _layernorm(x, axis=-1, eps=1e-5):
    m = jnp.mean(x, axis=axis, keepdims=True)
    v = jnp.var(x, axis=axis, keepdims=True)
    return (x - m) / jnp.sqrt(v + eps)
def _scatter_add(tgt, idx, src, axis=0):
    return tgt.at[idx].add(src)
def _segment_sum(src, seg, n):
    return jax.ops.segment_sum(src, seg, n)
class _Rng:
    def __init__(self, key):
        self._k = key
    def _next(self):
        self._k, sub = jax.random.split(self._k)
        return sub
    def normal(self, shape):
        return jax.random.normal(self._next(), shape, dtype=jnp.bfloat16)
    def randint(self, lo, hi, shape):
        return jax.random.randint(self._next(), shape, lo, hi, dtype=jnp.int32)
    def uniform(self, shape, lo=0.0, hi=1.0):
        return jax.random.uniform(self._next(), shape, jnp.bfloat16, lo, hi)
    def permutation(self, n):
        return jax.random.permutation(self._next(), n)


kernel_name = 'sequential_preLN__linear_kernel_hedgehog__moe_arch_mod__prompt'

def setup_inputs():
    _rng = _Rng(jax.random.key(int.from_bytes(__import__("os").urandom(4), "little")))
    _w = (lambda a: (lambda t: t.astype(jnp.bfloat16) if jnp.issubdtype(t.dtype, jnp.floating) else t)(jnp.asarray(a)))
    def _A_setup():
        B, S, D, H = 1, 2048, 1024, 32
        Dh = D // H
        return {
            "x": _w((lambda *s: _rng.normal(s) * 0.05)(B, S, D)),
            "wqkv": _w((lambda *s: _rng.normal(s) * 0.05)(D, 3 * D)),
            "w_phi": _w((lambda *s: _rng.normal(s) * 0.05)(H, Dh, Dh) * (Dh ** -0.5)),
            "wo": _w((lambda *s: _rng.normal(s) * 0.05)(D, D)),
        }
    _A_in = _A_setup()

    def _B_setup():
        B, S, D, F, C = 1, 2048, 1024, 3584, 1
        return {
            "x": _w((lambda *s: _rng.normal(s) * 0.05)(B, S, D)),
            "w_r": _w((lambda *s: _rng.normal(s) * 0.05)(D)),
            "w_gate": _w((lambda *s: _rng.normal(s) * 0.05)(D, F)),
            "w_up": _w((lambda *s: _rng.normal(s) * 0.05)(D, F)),
            "w_down": _w((lambda *s: _rng.normal(s) * 0.05)(F, D)),
        }
    _B_in = _B_setup()

    return {
        "A_x": _A_in["x"],
        "A_wqkv": _A_in["wqkv"],
        "A_w_phi": _A_in["w_phi"],
        "A_wo": _A_in["wo"],
        "B_x": _B_in["x"],
        "B_w_r": _B_in["w_r"],
        "B_w_gate": _B_in["w_gate"],
        "B_w_up": _B_in["w_up"],
        "B_w_down": _B_in["w_down"],
    }

def reference(A_x, A_wqkv, A_w_phi, A_wo, B_x, B_w_r, B_w_gate, B_w_up, B_w_down):
    def _A_ref(x, wqkv, w_phi, wo):
        B, S, D = x.shape
        H = 32; Dh = D // H
        qkv = (lambda x, *d: x.transpose(*d))((x @ wqkv).reshape(B, S, 3, H, Dh), 2, 0, 3, 1, 4)
        q, k, v = qkv[0], qkv[1], qkv[2]
        pq = jnp.einsum("bhsd,hdf->bhsf", q, w_phi)
        pk = jnp.einsum("bhsd,hdf->bhsf", k, w_phi)
        phi_q = jnp.concatenate([_softmax(pq, axis=-1), _softmax(-pq, axis=-1)], axis=-1)
        phi_k = jnp.concatenate([_softmax(pk, axis=-1), _softmax(-pk, axis=-1)], axis=-1)
        kv = jnp.einsum("bhsf,bhsd->bhfd", phi_k, v)
        z  = jnp.einsum("bhsf->bhf", phi_k)
        num = jnp.einsum("bhqf,bhfd->bhqd", phi_q, kv)
        den = jnp.einsum("bhqf,bhf->bhq", phi_q, z)[..., None] + 1e-6
        o = num / den
        return (lambda x, *d: x.transpose(*d))(o, 0, 2, 1, 3).reshape(B, S, D) @ wo

    def _B_ref(x, w_r, w_gate, w_up, w_down):
        B, S, D = x.shape
        C = 1
        r = x @ w_r
        idx = jnp.argsort(-r, axis=-1)[:, :C]
        idx_e = jnp.repeat(idx.reshape(B, C, 1), D, axis=2)
        x_sel = jnp.take_along_axis(x, idx_e, axis=1)
        g = _silu(x_sel @ w_gate)
        u = x_sel @ w_up
        y = (g * u) @ w_down
        r_sel = _sigmoid(jnp.take_along_axis(r, idx, axis=1))
        y = y * r_sel.reshape(B, C, 1)
        b_off = (jnp.arange(B) * S).reshape(B, 1)
        flat_idx = (idx + b_off).reshape(B * C)
        zero = (x * 0.0).reshape(B * S, D)
        upd = _scatter_add(zero, flat_idx, y.reshape(B * C, D), axis=0)
        return x + upd.reshape(B, S, D)

    x = A_x
    h = x + _A_ref(_layernorm(x, axis=-1), A_wqkv, A_w_phi, A_wo)
    h2 = h + _B_ref(_layernorm(h, axis=-1), B_w_r, B_w_gate, B_w_up, B_w_down)
    return h2
```

```python
import functools

import jax
import jax.numpy as jnp
from jax import lax
import jax.experimental.pallas as pl
import jax.experimental.pallas.tpu as pltpu

S = 2048
D = 1024
H = 32
DH = 32
F = 3584
T = 256
NT = S // T
NP = H // 2
LOG2E = 1.4426950408889634
LN_EPS = 1e-5
DEN_EPS = 1e-6

_NT_DIMS = (((1,), (1,)), ((), ()))
_TN_DIMS = (((0,), (0,)), ((), ()))

bf16 = jnp.bfloat16
f32 = jnp.float32


def _dot_nt(a, b):
    return lax.dot_general(a, b, _NT_DIMS, preferred_element_type=f32)


def _dot_nn(a, b):
    return jnp.dot(a, b, preferred_element_type=f32)


def _layernorm(x):
    m = jnp.mean(x, axis=-1, keepdims=True)
    xc = x - m
    v = jnp.mean(xc * xc, axis=-1, keepdims=True)
    return xc * lax.rsqrt(v + LN_EPS)


def _allreduce8(x, op):
    x = op(x, pltpu.roll(x, 4, 1))
    x = op(x, pltpu.roll(x, 2, 1))
    x = op(x, pltpu.roll(x, 1, 1))
    return x


def _hedgehog_t(p):
    t = p.shape[-1]
    p4 = p.reshape(2, 4, 8, t)
    mx = _allreduce8(jnp.max(p4, axis=1), jnp.maximum)
    mn = _allreduce8(jnp.min(p4, axis=1), jnp.minimum)
    ep = jnp.exp2(p4 - mx[:, None])
    en = jnp.exp2(mn[:, None] - p4)
    sp = _allreduce8(jnp.sum(ep, axis=1), jnp.add)
    sn = _allreduce8(jnp.sum(en, axis=1), jnp.add)
    fp = (ep * (1.0 / sp)[:, None]).reshape(64, t)
    fn = (en * (1.0 / sn)[:, None]).reshape(64, t)
    return jnp.concatenate([fp, fn], axis=0).astype(bf16)


def _kernel(x_hbm, wqkv_hbm, wphi_hbm, wo_hbm, wr_hbm, wg_hbm, wu_hbm, wd_hbm,
            out_hbm,
            x_v, wqkv_v, wphi_v, wo_v, wr_v, wg_v, wu_v, wd_v,
            wt_v, xn_v, phiq_v, kvacc_v, kvz_v, ot_v, attn_v, out_v, wrb_v,
            bestv_v, besti_v,
            sem_x, sem_w, sem_o):

    def cp_x(i):
        return pltpu.make_async_copy(x_hbm.at[pl.ds(i * T, T)], x_v.at[pl.ds(i * T, T)], sem_x.at[i])

    def cp_wqkv(c):
        return pltpu.make_async_copy(wqkv_hbm.at[:, pl.ds(c * D, D)], wqkv_v.at[:, pl.ds(c * D, D)], sem_w.at[c])

    cp_wphi = pltpu.make_async_copy(wphi_hbm, wphi_v, sem_w.at[3])
    cp_wo = pltpu.make_async_copy(wo_hbm, wo_v, sem_w.at[4])
    cp_wr = pltpu.make_async_copy(wr_hbm, wr_v, sem_w.at[5])
    cp_wg = pltpu.make_async_copy(wg_hbm, wg_v, sem_w.at[6])
    cp_wu = pltpu.make_async_copy(wu_hbm, wu_v, sem_w.at[7])
    cp_wd = pltpu.make_async_copy(wd_hbm, wd_v, sem_w.at[8])

    def cp_out(i):
        return pltpu.make_async_copy(out_v.at[pl.ds(i * T, T)], out_hbm.at[pl.ds(i * T, T)], sem_o.at[i])

    cp_wphi.start()
    cp_wr.start()
    cp_x(0).start()
    cp_wqkv(1).start()
    cp_wqkv(2).start()
    cp_wqkv(0).start()
    for i in range(1, NT):
        cp_x(i).start()
    cp_wo.start()
    cp_wg.start()
    cp_wu.start()
    cp_wd.start()

    def ln1(i, slot):
        xt = x_v[pl.ds(pl.multiple_of(i * T, T), T), :].astype(f32)
        xn_v[slot] = _layernorm(xt).astype(bf16)

    cp_wphi.wait()
    cp_wr.wait()
    r_i = lax.broadcasted_iota(jnp.int32, (128, DH), 0)
    c_i = lax.broadcasted_iota(jnp.int32, (128, DH), 1)
    expand = (r_i % DH == c_i).astype(bf16)
    r_h = lax.broadcasted_iota(jnp.int32, (128, 128), 0) // DH
    c_h = lax.broadcasted_iota(jnp.int32, (128, 128), 1) // DH
    same_head = r_h == c_h
    amats = []
    for g in range(8):
        a = _dot_nt(expand, wphi_v[g * 128:(g + 1) * 128, :])
        amats.append(jnp.where(same_head, a, 0.0).astype(bf16))

    wr = wr_v[...].astype(f32)
    wrb_v[...] = jnp.concatenate(
        [jnp.broadcast_to(wr[j:j + 1, :], (8, 128)) for j in range(8)], axis=1)

    cp_x(0).wait()
    ln1(0, 0)

    for c in (1, 2, 0):
        cp_wqkv(c).wait()
        if c == 2:
            wt_v[2 * D:3 * D, :] = wqkv_v[:, 2 * D:3 * D].T
        else:
            for g in range(8):
                w = wqkv_v[:, c * D + g * 128:c * D + (g + 1) * 128]
                wt_v[c * D + g * 128:c * D + (g + 1) * 128, :] = (
                    _dot_nt(amats[g], w) * LOG2E).astype(bf16)

    kvacc_v[...] = jnp.zeros(kvacc_v.shape, f32)

    ones16 = jnp.ones((16, T), bf16)

    def phase1(i, do_next):
        slot = i % 2
        xn = xn_v[slot]
        pk = _dot_nt(wt_v[D:2 * D, :], xn)
        phik = [_hedgehog_t(pk[j * 64:(j + 1) * 64]) for j in range(NP)]
        vt = _dot_nt(wt_v[2 * D:3 * D, :], xn).astype(bf16)
        pq = _dot_nt(wt_v[0:D, :], xn)
        for j in range(NP):
            phiq_v[i, j * 128:(j + 1) * 128, :] = _hedgehog_t(pq[j * 64:(j + 1) * 64])
        for j in range(NP):
            lhs = jnp.concatenate([vt[j * 64:(j + 1) * 64], ones16], axis=0)
            kvacc_v[j] += _dot_nt(lhs, phik[j])
        if do_next:
            ln1(i + 1, 1 - slot)

    def p1_body(i, c):
        cp_x(i + 1).wait()
        phase1(i, True)
        return c

    lax.fori_loop(0, NT - 1, p1_body, 0)
    phase1(NT - 1, False)

    rr = lax.broadcasted_iota(jnp.int32, (80, 128), 0)
    cc = lax.broadcasted_iota(jnp.int32, (80, 128), 1)
    row_head = jnp.where(rr < 64, rr // DH, (rr - 64) // 8)
    col_head = (cc // DH) % 2
    kv_mask = row_head == col_head
    for j in range(NP):
        kvz_v[j] = jnp.where(kv_mask, kvacc_v[j], 0.0).astype(bf16)

    def stage_g(i, slot):
        for j in range(NP):
            res = _dot_nn(kvz_v[j], phiq_v[i, j * 128:(j + 1) * 128, :])
            inv = 1.0 / (res[64:80] + DEN_EPS)
            o = res[0:64].reshape(2, 4, 8, T) * inv.reshape(2, 1, 8, T)
            ot_v[slot, j * 64:(j + 1) * 64, :] = o.reshape(64, T).astype(bf16)

    def stage_h(i, slot):
        attn_v[pl.ds(pl.multiple_of(i * T, T), T), :] = lax.dot_general(
            ot_v[slot], wo_v[...], _TN_DIMS, preferred_element_type=f32)

    def stage_i(i):
        rows = pl.ds(pl.multiple_of(i * T, T), T)
        h = x_v[rows, :].astype(f32) + attn_v[rows, :]
        hn = _layernorm(h)
        out_v[rows, :] = (h + hn).astype(bf16)
        r = jnp.sum(hn * wrb_v[0:1, :], axis=-1, keepdims=True)
        idx = lax.broadcasted_iota(jnp.int32, (T, 1), 0) + i * T
        better = r > bestv_v[...]
        bestv_v[...] = jnp.where(better, r, bestv_v[...])
        besti_v[...] = jnp.where(better, idx, besti_v[...])

    bestv_v[...] = jnp.full(bestv_v.shape, -jnp.inf, f32)
    besti_v[...] = lax.broadcasted_iota(jnp.int32, (T, 1), 0)

    cp_wo.wait()
    stage_g(0, 0)
    stage_h(0, 0)
    stage_g(1, 1)

    def p2_body(i, c):
        slot = i % 2
        stage_h(i, slot)
        stage_g(i + 1, 1 - slot)
        stage_i(i - 1)
        cp_out(i - 1).start()
        return c

    lax.fori_loop(1, NT - 1, p2_body, 0)
    stage_h(NT - 1, (NT - 1) % 2)
    stage_i(NT - 2)
    cp_out(NT - 2).start()
    stage_i(NT - 1)
    cp_out(NT - 1).start()

    bv = bestv_v[...]
    mval = jnp.max(bv, axis=0, keepdims=True)
    sel = jnp.min(jnp.where(bv == mval, besti_v[...], S), axis=0, keepdims=True)
    sel = jnp.minimum(sel, S - 1)
    idx = sel[0, 0]
    base = pl.multiple_of((idx // 16) * 16, 16)
    rows = pl.ds(base, 16)
    h = x_v[rows, :].astype(f32) + attn_v[rows, :]
    hn = _layernorm(h)
    xs = hn.astype(bf16)
    cp_wg.wait()
    cp_wu.wait()
    cp_wd.wait()
    g = _dot_nn(xs, wg_v[...])
    u = _dot_nn(xs, wu_v[...])
    a = (g * jax.nn.sigmoid(g) * u).astype(bf16)
    y = _dot_nn(a, wd_v[...]) * jax.nn.sigmoid(mval)
    rid = lax.broadcasted_iota(jnp.int32, (16, 1), 0) + base
    res = h + hn + jnp.where(rid == sel, y, 0.0)
    for i in range(NT):
        cp_out(i).wait()
    out_v[rows, :] = res.astype(bf16)
    fix = pltpu.make_async_copy(out_v.at[rows], out_hbm.at[rows], sem_o.at[0])
    fix.start()
    fix.wait()


@jax.jit
def pallas_sequential_preLN__linear_kernel_hedgehog__moe_arch_mod__prompt_kernel(
    A_x: jax.Array,
    A_wqkv: jax.Array,
    A_w_phi: jax.Array,
    A_wo: jax.Array,
    B_x: jax.Array,
    B_w_r: jax.Array,
    B_w_gate: jax.Array,
    B_w_up: jax.Array,
    B_w_down: jax.Array,
):
    del B_x
    x = A_x.reshape(S, D)
    wphi = A_w_phi.reshape(H * DH, DH)
    wr = B_w_r.reshape(8, 128)
    any_spec = pl.BlockSpec(memory_space=pl.ANY)
    out = pl.pallas_call(
        _kernel,
        out_shape=jax.ShapeDtypeStruct((S, D), bf16),
        in_specs=[any_spec] * 8,
        out_specs=any_spec,
        scratch_shapes=[
            pltpu.VMEM((S, D), bf16),
            pltpu.VMEM((D, 3 * D), bf16),
            pltpu.VMEM((H * DH, DH), bf16),
            pltpu.VMEM((D, D), bf16),
            pltpu.VMEM((8, 128), bf16),
            pltpu.VMEM((D, F), bf16),
            pltpu.VMEM((D, F), bf16),
            pltpu.VMEM((F, D), bf16),
            pltpu.VMEM((3 * D, D), bf16),
            pltpu.VMEM((2, T, D), bf16),
            pltpu.VMEM((NT, 2 * D, T), bf16),
            pltpu.VMEM((NP, 80, 128), f32),
            pltpu.VMEM((NP, 80, 128), bf16),
            pltpu.VMEM((2, D, T), bf16),
            pltpu.VMEM((S, D), f32),
            pltpu.VMEM((S, D), bf16),
            pltpu.VMEM((8, D), f32),
            pltpu.VMEM((T, 1), f32),
            pltpu.VMEM((T, 1), jnp.int32),
            pltpu.SemaphoreType.DMA((NT,)),
            pltpu.SemaphoreType.DMA((9,)),
            pltpu.SemaphoreType.DMA((NT,)),
        ],
        compiler_params=pltpu.CompilerParams(vmem_limit_bytes=110 * 1024 * 1024),
        name="hedgehog_mod",
    )(x, A_wqkv, wphi, A_wo, wr, B_w_gate, B_w_up, B_w_down)
    return out.reshape(1, S, D)
```

```python
import functools

import jax
import jax.numpy as jnp
from jax import lax
import jax.experimental.pallas as pl
import jax.experimental.pallas.tpu as pltpu

S = 2048
D = 1024
H = 32
DH = 32
F = 3584
T = 256
NT = S // T
B = 128
NB = S // B
BPI = 4
NP = H // 2
FC = 512
LOG2E = 1.4426950408889634
LN_EPS = 1e-5
DEN_EPS = 1e-6

_NT_DIMS = (((1,), (1,)), ((), ()))
_TN_DIMS = (((0,), (0,)), ((), ()))

bf16 = jnp.bfloat16
f32 = jnp.float32


def _dot_nt(a, b):
    return lax.dot_general(a, b, _NT_DIMS, preferred_element_type=f32)


def _dot_nn(a, b):
    return jnp.dot(a, b, preferred_element_type=f32)


def _layernorm(x):
    m = jnp.mean(x, axis=-1, keepdims=True)
    xc = x - m
    v = jnp.mean(xc * xc, axis=-1, keepdims=True)
    return xc * lax.rsqrt(v + LN_EPS)


def _allreduce8(x, op):
    x = op(x, pltpu.roll(x, 4, 1))
    x = op(x, pltpu.roll(x, 2, 1))
    x = op(x, pltpu.roll(x, 1, 1))
    return x


def _hedgehog_t(p):
    t = p.shape[-1]
    p4 = p.reshape(2, 4, 8, t)
    mx = _allreduce8(jnp.max(p4, axis=1), jnp.maximum)
    mn = _allreduce8(jnp.min(p4, axis=1), jnp.minimum)
    ep = jnp.exp2(p4 - mx[:, None])
    en = jnp.exp2(mn[:, None] - p4)
    sp = _allreduce8(jnp.sum(ep, axis=1), jnp.add)
    sn = _allreduce8(jnp.sum(en, axis=1), jnp.add)
    fp = (ep * (1.0 / sp)[:, None]).reshape(64, t)
    fn = (en * (1.0 / sn)[:, None]).reshape(64, t)
    return jnp.concatenate([fp, fn], axis=0).astype(bf16)


_WCHUNKS = ((D, 256), (D + 256, 256), (D + 512, 512),
            (0, 512), (512, 512),
            (2 * D, 512), (2 * D + 512, 512))


def _kernel(x_hbm, wqkv_hbm, wphi_hbm, wo_hbm, wr_hbm, wg_hbm, wu_hbm, wd_hbm,
            out_hbm,
            x_v, wqkv_v, wphi_v, wo_v, wr_v, wg_v, wu_v, wd_v,
            wt_v, xn_v, phiq_v, kvacc_v, kvz_v, attn_v, out_v, wrb_v,
            bestv_v, besti_v,
            sem_i, sem_o):

    def cp_x(i):
        return pltpu.make_async_copy(x_hbm.at[pl.ds(i * T, T)], x_v.at[pl.ds(i * T, T)], sem_i.at[i])

    def cp_w(c):
        lo, w = _WCHUNKS[c]
        return pltpu.make_async_copy(wqkv_hbm.at[:, pl.ds(lo, w)], wqkv_v.at[:, pl.ds(lo, w)], sem_i.at[NT + c])

    cp_wphi = pltpu.make_async_copy(wphi_hbm, wphi_v, sem_i.at[NT + len(_WCHUNKS) + 0])
    cp_wr = pltpu.make_async_copy(wr_hbm, wr_v, sem_i.at[NT + len(_WCHUNKS) + 1])
    cp_wo = pltpu.make_async_copy(wo_hbm, wo_v, sem_i.at[NT + len(_WCHUNKS) + 2])
    cp_wg = pltpu.make_async_copy(wg_hbm, wg_v, sem_i.at[NT + len(_WCHUNKS) + 3])
    cp_wu = pltpu.make_async_copy(wu_hbm, wu_v, sem_i.at[NT + len(_WCHUNKS) + 4])
    cp_wd = pltpu.make_async_copy(wd_hbm, wd_v.at[:, pl.ds(0, D)], sem_i.at[NT + len(_WCHUNKS) + 5])

    def cp_out(k, lo, n):
        return pltpu.make_async_copy(out_v.at[pl.ds(lo, n)], out_hbm.at[pl.ds(lo, n)], sem_o.at[k])

    cp_wphi.start()
    cp_wr.start()
    cp_x(0).start()
    for c in range(len(_WCHUNKS)):
        cp_w(c).start()
    for i in range(1, NT):
        cp_x(i).start()
    cp_wo.start()
    cp_wg.start()
    cp_wu.start()
    cp_wd.start()

    def ln1(row0):
        xt = x_v[pl.ds(row0, T), :].astype(f32)
        return _layernorm(xt).astype(bf16)

    ones16 = jnp.ones((16, T), bf16)

    def feat(p):
        return [_hedgehog_t(p[j * 64:(j + 1) * 64]) for j in range(p.shape[0] // 64)]

    def store_phiq(i, j0, phis):
        for j, ph in enumerate(phis):
            for s in range(T // B):
                phiq_v[i * (T // B) + s, (j0 + j) * 128:(j0 + j + 1) * 128, :] = ph[:, s * B:(s + 1) * B]

    def kv_prod(vt, phik, j):
        return _dot_nt(jnp.concatenate([vt, ones16], axis=0), phik)

    cp_wphi.wait()
    cp_wr.wait()
    r_i = lax.broadcasted_iota(jnp.int32, (128, DH), 0)
    c_i = lax.broadcasted_iota(jnp.int32, (128, DH), 1)
    expand = (r_i % DH == c_i).astype(bf16)
    r_h = lax.broadcasted_iota(jnp.int32, (128, 128), 0) // DH
    c_h = lax.broadcasted_iota(jnp.int32, (128, 128), 1) // DH
    same_head = r_h == c_h
    amats = []
    for g in range(8):
        a = _dot_nt(expand, wphi_v[g * 128:(g + 1) * 128, :])
        amats.append(jnp.where(same_head, a, 0.0).astype(bf16))

    wr = wr_v[...].astype(f32)
    wrb_v[...] = jnp.concatenate(
        [jnp.broadcast_to(wr[j:j + 1, :], (8, 128)) for j in range(8)], axis=1)
    bestv_v[...] = jnp.full(bestv_v.shape, -jnp.inf, f32)
    besti_v[...] = lax.broadcasted_iota(jnp.int32, (B, 1), 0)

    cp_x(0).wait()
    xn0 = ln1(0)

    def fold(c):
        lo, w = _WCHUNKS[c]
        parts = []
        for g0 in range(lo, lo + w, 128):
            g = (g0 % D) // 128
            parts.append((_dot_nt(amats[g], wqkv_v[:, g0:g0 + 128]) * LOG2E).astype(bf16))
        wt = jnp.concatenate(parts, axis=0)
        wt_v[lo:lo + w, :] = wt
        return wt

    def transpose_v(c):
        lo, w = _WCHUNKS[c]
        wt = wqkv_v[:, lo:lo + w].T
        wt_v[lo:lo + w, :] = wt
        return wt

    phik0 = []
    for c in (0, 1, 2):
        cp_w(c).wait()
        phik0 += feat(_dot_nt(fold(c), xn0))
    cp_w(3).wait()
    store_phiq(0, 0, feat(_dot_nt(fold(3), xn0)))
    cp_w(4).wait()
    cp_w(5).wait()
    wtv = transpose_v(5)
    store_phiq(0, 8, feat(_dot_nt(fold(4), xn0)))
    vt_a = _dot_nt(wtv, xn0).astype(bf16)
    cp_w(6).wait()
    cp_x(1).wait()
    wtv = transpose_v(6)
    xn_v[...] = ln1(T)
    for j in range(8):
        kvacc_v[j] = kv_prod(vt_a[j * 64:(j + 1) * 64], phik0[j], j)
    vt_b = _dot_nt(wtv, xn0).astype(bf16)
    for j in range(8):
        kvacc_v[8 + j] = kv_prod(vt_b[j * 64:(j + 1) * 64], phik0[8 + j], 8 + j)
    for i in range(2, NT):
        cp_x(i).wait()

    def p1_body(i, c):
        xn = xn_v[...]
        nxt = jnp.minimum(i + 1, NT - 1)
        xn_v[...] = ln1(pl.multiple_of(nxt * T, T))
        phik = feat(_dot_nt(wt_v[D:2 * D, :], xn))
        vt = _dot_nt(wt_v[2 * D:3 * D, :], xn).astype(bf16)
        store_phiq(i, 0, feat(_dot_nt(wt_v[0:D, :], xn)))
        for j in range(NP):
            kvacc_v[j] += kv_prod(vt[j * 64:(j + 1) * 64], phik[j], j)
        return c

    lax.fori_loop(1, NT, p1_body, 0)

    cp_wo.wait()
    rr = lax.broadcasted_iota(jnp.int32, (80, 128), 0)
    cc = lax.broadcasted_iota(jnp.int32, (80, 128), 1)
    row_head = jnp.where(rr < 64, rr // DH, (rr - 64) // 8)
    col_head = (cc // DH) % 2
    kv_mask = row_head == col_head
    for j in range(NP):
        kvz_v[j] = jnp.where(kv_mask, kvacc_v[j], 0.0).astype(bf16)

    def rows_of(b):
        if isinstance(b, int):
            return pl.ds(b * B, B)
        return pl.ds(pl.multiple_of(b * B, B), B)

    def stage_g(b):
        parts = []
        for j in range(NP):
            res = _dot_nn(kvz_v[j], phiq_v[b, j * 128:(j + 1) * 128, :])
            inv = 1.0 / (res[64:80] + DEN_EPS)
            o = res[0:64].reshape(2, 4, 8, B) * inv.reshape(2, 1, 8, B)
            parts.append(o.reshape(64, B).astype(bf16))
        return jnp.concatenate(parts, axis=0)

    def stage_h(b, ot):
        attn = lax.dot_general(ot, wo_v[...], _TN_DIMS, preferred_element_type=f32)
        attn_v[rows_of(b), :] = attn
        return attn

    def stage_i(b, attn):
        rows = rows_of(b)
        h = x_v[rows, :].astype(f32) + attn
        hn = _layernorm(h)
        out_v[rows, :] = (h + hn).astype(bf16)
        r = jnp.sum(hn * wrb_v[0:1, :], axis=-1, keepdims=True)
        idx = lax.broadcasted_iota(jnp.int32, (B, 1), 0) + b * B
        better = r > bestv_v[...]
        bestv_v[...] = jnp.where(better, r, bestv_v[...])
        besti_v[...] = jnp.where(better, idx, besti_v[...])

    def p2_group(b0, first):
        if not first:
            stage_i(b0 - 1, attn_v[rows_of(b0 - 1), :])
        ot = [stage_g(b0), stage_g(b0 + 1)]
        for s in range(BPI):
            attn = stage_h(b0 + s, ot[s])
            if s + 2 < BPI:
                ot.append(stage_g(b0 + s + 2))
            if s + 1 < BPI:
                stage_i(b0 + s, attn)

    p2_group(0, True)
    cp_out(0, 0, (BPI - 1) * B).start()

    def p2_body(i, c):
        b0 = i * BPI
        p2_group(b0, False)
        cp_out(i, pl.multiple_of((b0 - 1) * B, B), BPI * B).start()
        return c

    NI = NB // BPI
    lax.fori_loop(1, NI, p2_body, 0)
    cp_wg.wait()
    cp_wu.wait()
    cp_wd.wait()
    stage_i(NB - 1, attn_v[rows_of(NB - 1), :])
    cp_out(NI, (NB - 1) * B, B).start()

    bv = bestv_v[...]
    mval = jnp.max(bv, axis=0, keepdims=True)
    sel = jnp.min(jnp.where(bv == mval, besti_v[...], S), axis=0, keepdims=True)
    sel = jnp.minimum(sel, S - 1)
    idx = sel[0, 0]
    base = pl.multiple_of((idx // 16) * 16, 16)
    rows = pl.ds(base, 16)
    h = x_v[rows, :].astype(f32) + attn_v[rows, :]
    hn = _layernorm(h)
    xs = hn.astype(bf16)
    acts = []
    y = None
    for k in range(F // FC + 1):
        if k < F // FC:
            g = _dot_nn(xs, wg_v[:, k * FC:(k + 1) * FC])
            u = _dot_nn(xs, wu_v[:, k * FC:(k + 1) * FC])
            acts.append((g * jax.nn.sigmoid(g) * u).astype(bf16))
        if k >= 1:
            t = _dot_nn(acts[k - 1], wd_v[(k - 1) * FC:k * FC, 0:D])
            y = t if y is None else y + t
    y = y * jax.nn.sigmoid(mval)
    rid = lax.broadcasted_iota(jnp.int32, (16, 1), 0) + base
    res = (h + hn + jnp.where(rid == sel, y, 0.0)).astype(bf16)
    cp_out(0, 0, (BPI - 1) * B).wait()
    for i in range(1, NI):
        cp_out(i, (i * BPI - 1) * B, BPI * B).wait()
    cp_out(NI, (NB - 1) * B, B).wait()
    out_v[rows, :] = res
    fix = pltpu.make_async_copy(out_v.at[rows], out_hbm.at[rows], sem_o.at[0])
    fix.start()
    fix.wait()


@jax.jit
def pallas_sequential_preLN__linear_kernel_hedgehog__moe_arch_mod__prompt_kernel(
    A_x: jax.Array,
    A_wqkv: jax.Array,
    A_w_phi: jax.Array,
    A_wo: jax.Array,
    B_x: jax.Array,
    B_w_r: jax.Array,
    B_w_gate: jax.Array,
    B_w_up: jax.Array,
    B_w_down: jax.Array,
):
    del B_x
    x = A_x.reshape(S, D)
    wphi = A_w_phi.reshape(H * DH, DH)
    wr = B_w_r.reshape(8, 128)
    any_spec = pl.BlockSpec(memory_space=pl.ANY)
    out = pl.pallas_call(
        _kernel,
        out_shape=jax.ShapeDtypeStruct((S, D), bf16),
        in_specs=[any_spec] * 8,
        out_specs=any_spec,
        scratch_shapes=[
            pltpu.VMEM((S, D), bf16),
            pltpu.VMEM((D, 3 * D), bf16),
            pltpu.VMEM((H * DH, DH), bf16),
            pltpu.VMEM((D, D), bf16),
            pltpu.VMEM((8, 128), bf16),
            pltpu.VMEM((D, F), bf16),
            pltpu.VMEM((D, F), bf16),
            pltpu.VMEM((F, D + 128), bf16),
            pltpu.VMEM((3 * D, D), bf16),
            pltpu.VMEM((T, D), bf16),
            pltpu.VMEM((NB, 2 * D, B), bf16),
            pltpu.VMEM((NP, 80, 128), f32),
            pltpu.VMEM((NP, 80, 128), bf16),
            pltpu.VMEM((S, D), f32),
            pltpu.VMEM((S, D), bf16),
            pltpu.VMEM((8, D), f32),
            pltpu.VMEM((B, 1), f32),
            pltpu.VMEM((B, 1), jnp.int32),
            pltpu.SemaphoreType.DMA((NT + len(_WCHUNKS) + 6,)),
            pltpu.SemaphoreType.DMA((NB // BPI + 1,)),
        ],
        compiler_params=pltpu.CompilerParams(vmem_limit_bytes=110 * 1024 * 1024),
        name="hedgehog_mod",
    )(x, A_wqkv, wphi, A_wo, wr, B_w_gate, B_w_up, B_w_down)
    return out.reshape(1, S, D)
```

```python
import os
import jax
import jax.numpy as jnp
from jax import lax
import jax.experimental.pallas as pl
import jax.experimental.pallas.tpu as pltpu

S = 2048
D = 1024
H = 32
DH = 32
F = 3584
T = 256
NT = S // T
B = 128
NB = S // B
BPI = 4
NI = NB // BPI
NP = H // 2
FC = 512
R = 16
LOG2E = 1.4426950408889634
LN_EPS = 1e-5
DEN_EPS = 1e-6

_NT_DIMS = (((1,), (1,)), ((), ()))
_TN_DIMS = (((0,), (0,)), ((), ()))

bf16 = jnp.bfloat16
f32 = jnp.float32
u32 = jnp.uint32


def _opt(name, default):
    return type(default)(os.environ.get(name, default))


def _dot_nt(a, b):
    return lax.dot_general(a, b, _NT_DIMS, preferred_element_type=f32)


def _dot_nn(a, b):
    return jnp.dot(a, b, preferred_element_type=f32)


def _pk(x):
    return pltpu.bitcast(x, u32)


def _upk(x):
    return pltpu.bitcast(x, bf16)


def _layernorm(x):
    m = jnp.mean(x, axis=-1, keepdims=True)
    xc = x - m
    v = jnp.mean(xc * xc, axis=-1, keepdims=True)
    return xc * lax.rsqrt(v + LN_EPS)


def _allreduce8(x, op):
    x = op(x, pltpu.roll(x, 4, 1))
    x = op(x, pltpu.roll(x, 2, 1))
    x = op(x, pltpu.roll(x, 1, 1))
    return x


def _hedgehog_t(p, z=None):
    t = p.shape[-1]
    p4 = p.reshape(2, 4, 8, t)
    mx = _allreduce8(jnp.max(p4, axis=1), jnp.maximum)
    mn = _allreduce8(jnp.min(p4, axis=1), jnp.minimum)
    ep = jnp.exp2(p4 - mx[:, None])
    en = jnp.exp2(mn[:, None] - p4)
    a = pl.reciprocal(_allreduce8(jnp.sum(ep, axis=1), jnp.add), approx=True)
    b = pl.reciprocal(_allreduce8(jnp.sum(en, axis=1), jnp.add), approx=True)
    if z is not None:
        dp = jnp.sum(ep * z[0:64].reshape(2, 4, 8, t), axis=1)
        dn = jnp.sum(en * z[64:128].reshape(2, 4, 8, t), axis=1)
        den = _allreduce8(dp * a + dn * b, jnp.add) + DEN_EPS
        inv = pl.reciprocal(den, approx=True)
        a = a * inv
        b = b * inv
    fp = (ep * a[:, None]).reshape(64, t)
    fn = (en * b[:, None]).reshape(64, t)
    return jnp.concatenate([fp, fn], axis=0)


def _tie(keep, w, ties):
    rows = sorted({r for r, _ in ties})
    out, pos = [], 0
    for r in rows:
        if r > pos:
            out.append(w[pos:r])
        cols = sorted(c for rr, c in ties if rr == r)
        parts, cpos = [], 0
        for c in cols:
            if c > cpos:
                parts.append(w[r:r + 8, cpos:c])
            parts.append(jnp.where(keep, w[r:r + 8, c:c + 128], ties[(r, c)]))
            cpos = c + 128
        if cpos < w.shape[1]:
            parts.append(w[r:r + 8, cpos:])
        out.append(jnp.concatenate(parts, axis=1) if len(parts) > 1 else parts[0])
        pos = r + 8
    if pos < w.shape[0]:
        out.append(w[pos:])
    return jnp.concatenate(out, axis=0)


def _vregs(x):
    if x.dtype != u32:
        x = pltpu.bitcast(x, u32)
    return [x[r:r + 8, c:c + 128] for r in range(0, x.shape[0], 8) for c in range(0, x.shape[1], 128)]


_WCHUNKS = ((D, 256), (D + 256, 512), (D + 768, 256),
            (2 * D, 512), (2 * D + 512, 512),
            (0, 1024))
_NSEM_IN = NT + len(_WCHUNKS) + 7
_PHI_A = 256


def _kernel(x_hbm, wqkv_hbm, wphi_hbm, wo_hbm, wr_hbm, wg_hbm, wu_hbm, wd_hbm,
            out_hbm,
            x_v, wqkv_v, wphi_v, wo_v, wr_v, wg_v, wu_v, wd_v,
            wt_v, wou_v, amat_v, xn_v, kvacc_v, zacc_v, kv_v, attn_v, out_v, wrb_v,
            bestv_v, besti_v, flag_s,
            sem_i, sem_o):

    def cp_x(i):
        return pltpu.make_async_copy(x_hbm.at[pl.ds(i * T, T)], x_v.at[pl.ds(i * T, T)], sem_i.at[i])

    def cp_w(c):
        lo, w = _WCHUNKS[c]
        return pltpu.make_async_copy(wqkv_hbm.at[:, pl.ds(lo, w)], wqkv_v.at[:, pl.ds(lo, w)],
                                     sem_i.at[NT + c])

    s0 = NT + len(_WCHUNKS)
    cp_pa = pltpu.make_async_copy(wphi_hbm.at[pl.ds(0, _PHI_A)], wphi_v.at[pl.ds(0, _PHI_A)], sem_i.at[s0])
    cp_pb = pltpu.make_async_copy(wphi_hbm.at[pl.ds(_PHI_A, D - _PHI_A)], wphi_v.at[pl.ds(_PHI_A, D - _PHI_A)],
                                  sem_i.at[s0 + 6])
    cp_wr = pltpu.make_async_copy(wr_hbm, wr_v, sem_i.at[s0 + 1])
    cp_wo = pltpu.make_async_copy(wo_hbm, wo_v, sem_i.at[s0 + 2])
    cp_wg = pltpu.make_async_copy(wg_hbm, wg_v, sem_i.at[s0 + 3])
    cp_wu = pltpu.make_async_copy(wu_hbm, wu_v, sem_i.at[s0 + 4])
    cp_wd = pltpu.make_async_copy(wd_hbm, wd_v.at[:, pl.ds(0, D)], sem_i.at[s0 + 5])

    def cp_out(k):
        lo = k * BPI * B
        if not isinstance(k, int):
            lo = pl.multiple_of(lo, B)
        return pltpu.make_async_copy(out_v.at[pl.ds(lo, BPI * B)], out_hbm.at[pl.ds(lo, BPI * B)], sem_o.at[k])

    cp_pa.start()
    cp_w(0).start()
    cp_x(0).start()
    cp_pb.start()
    for c in range(1, 5):
        cp_w(c).start()
    for i in range(1, NT):
        cp_x(i).start()
    cp_wr.start()
    cp_w(5).start()
    cp_wo.start()
    cp_wg.start()
    cp_wu.start()
    cp_wd.start()
    flag_s[0] = 1

    def ln1_pieces(row0):
        return [_pk(_layernorm(x_v[pl.ds(row0 + k * R, R), :].astype(f32)).astype(bf16))
                for k in range(T // R)]

    def store_xn(i, pieces):
        n = B // R
        for s in range(T // B):
            xn_v[i * (T // B) + s] = jnp.concatenate(pieces[s * n:(s + 1) * n], axis=0)

    def k_side(p, j0, first):
        res = []
        for j in range(p.shape[0] // 64):
            ph = _hedgehog_t(p[j * 64:(j + 1) * 64])
            rows = slice((j0 + j) * 128, (j0 + j + 1) * 128)
            for s in range(T // 128):
                part = ph[:, s * 128:(s + 1) * 128]
                if first and s == 0:
                    zacc_v[rows, :] = part
                else:
                    zacc_v[rows, :] += part
            res.append(ph.astype(bf16))
        return res

    def lhs_ties(pieces, nrows):
        ties = {}
        half = (len(pieces) + 1) // 2
        step = (nrows // half) // 8 * 8
        for k, p in enumerate(pieces):
            for q, val in enumerate(p):
                ties[((k % half) * step + (q // 4) * 8, (k // half) * 512 + (q % 4) * 128)] = val
        return ties

    r_i = lax.broadcasted_iota(jnp.int32, (128, DH), 0)
    c_i = lax.broadcasted_iota(jnp.int32, (128, DH), 1)
    expand = (r_i % DH == c_i).astype(bf16)
    r_h = lax.broadcasted_iota(jnp.int32, (128, 128), 0) // DH
    c_h = lax.broadcasted_iota(jnp.int32, (128, 128), 1) // DH
    same_head = r_h == c_h

    def make_amat(g):
        a = _dot_nt(expand, wphi_v[g * 128:(g + 1) * 128, :])
        amat_v[g] = _pk(jnp.where(same_head, a, 0.0).astype(bf16))

    def fold(c, keep=None, ties=None):
        lo, w = _WCHUNKS[c]
        parts = []
        for n, g0 in enumerate(range(lo, lo + w, 128)):
            am = amat_v[(g0 % D) // 128]
            if ties is not None and ties[n]:
                am = _tie(keep, am, ties[n])
            parts.append((_dot_nt(_upk(am), wqkv_v[:, g0:g0 + 128]) * LOG2E).astype(bf16))
        wt = jnp.concatenate(parts, axis=0)
        wt_v[lo // 2:(lo + w) // 2, :] = _pk(wt)
        return wt

    def transpose_v(c):
        lo, w = _WCHUNKS[c]
        wt = _pk(wqkv_v[:, lo:lo + w].T)
        wt_v[lo // 2:(lo + w) // 2, :] = wt
        return wt

    bestv_v[...] = jnp.full(bestv_v.shape, -jnp.inf, f32)
    besti_v[...] = lax.broadcasted_iota(jnp.int32, besti_v.shape, 0)
    attn_v[0:B, :] = jnp.zeros((B, D), f32)

    cp_pa.wait()
    for g in range(_PHI_A // 128):
        make_amat(g)

    cp_w(0).wait()
    cp_x(0).wait()
    wt = fold(0)
    pieces = ln1_pieces(0)
    store_xn(0, pieces)
    xn0 = _upk(jnp.concatenate(pieces, axis=0))
    phik0 = k_side(_dot_nt(wt, xn0), 0, True)

    cp_pb.wait()
    cp_w(1).wait()
    for g in range(_PHI_A // 128, 8):
        make_amat(g)
    phik0 += k_side(_dot_nt(fold(1), xn0), len(phik0), True)

    cp_w(2).wait()
    cp_w(3).wait()
    phik0 += k_side(_dot_nt(fold(2), xn0), len(phik0), True)
    vt_a = _dot_nt(_upk(transpose_v(3)), xn0).astype(bf16)

    cp_w(4).wait()
    cp_x(1).wait()
    keep = flag_s[0] > 0
    wtv = transpose_v(4)
    for j in range(8):
        kvacc_v[j] = _dot_nt(vt_a[j * 64:(j + 1) * 64], phik0[j])
    pieces = ln1_pieces(T)
    store_xn(1, pieces)
    vt_b = _dot_nt(_upk(wtv), xn0).astype(bf16)
    vt_b = _pk(vt_b)
    for j in range(8):
        lhs = _tie(keep, vt_b[j * 32:(j + 1) * 32],
                   {((q // 2) * 8, (q % 2) * 128): v for q, v in enumerate(_vregs(pieces[2 * j]))})
        rhs = _tie(keep, _pk(phik0[8 + j]),
                   {((q // 2) * 8, (q % 2) * 128): v for q, v in enumerate(_vregs(pieces[2 * j + 1]))})
        kvacc_v[8 + j] = _dot_nt(_upk(lhs), _upk(rhs))

    def p1_body(i, c):
        nxt = jnp.minimum(i + 1, NT - 1)

        @pl.when(i + 1 < NT)
        def _():
            cp_x(nxt).wait()

        keep = flag_s[0] > 0
        xn = _upk(jnp.concatenate([xn_v[i * (T // B) + s] for s in range(T // B)], axis=0))
        phik = k_side(_dot_nt(_upk(wt_v[D // 2:D, :]), xn), 0, False)
        pieces = ln1_pieces(pl.multiple_of(nxt * T, T))
        wv = _tie(keep, wt_v[D:3 * D // 2, :], lhs_ties([_vregs(p) for p in pieces], D // 2))
        vt = _dot_nt(_upk(wv), xn).astype(bf16)
        store_xn(i + 1, pieces)
        for j in range(NP):
            kvacc_v[j] += _dot_nt(vt[j * 64:(j + 1) * 64], phik[j])
        return c

    lax.fori_loop(1, NT, p1_body, 0)

    cp_wr.wait()
    cp_w(5).wait()
    cp_wo.wait()
    keep = flag_s[0] > 0
    kv_mask = (lax.broadcasted_iota(jnp.int32, (64, 128), 0) // DH
               == (lax.broadcasted_iota(jnp.int32, (64, 128), 1) // DH) % 2)
    ties = [{} for _ in range(8)]
    for j in range(NP):
        kvj = _pk(jnp.where(kv_mask, kvacc_v[j], 0.0).astype(bf16))
        kv_v[j] = kvj
        zj = jnp.broadcast_to(jnp.sum(zacc_v[j * 128:(j + 1) * 128, :], axis=-1, keepdims=True), (128, 128))
        zacc_v[j * 128:(j + 1) * 128, :] = zj
        woj = _pk(wo_v[j * 64:(j + 1) * 64, :])
        wou_v[j * 32:(j + 1) * 32, :] = woj
        if j < 14:
            dep = kvj | pltpu.bitcast(jnp.max(zj.reshape(4, 32, 128), axis=0), u32)
            for c in range(8):
                dep = dep | woj[:, c * 128:(c + 1) * 128]
            for q, v in enumerate(_vregs(dep)):
                ties[1 + j // 2][((j % 2) * 32 + q * 8, 0)] = v
    wr = wr_v[...].astype(f32)
    wrb_v[...] = jnp.concatenate(
        [jnp.broadcast_to(wr[j:j + 1, :], (8, 128)) for j in range(8)], axis=1)
    fold(5, keep, ties)

    def row_at(b):
        if isinstance(b, int):
            return b * B
        return pl.multiple_of(b * B, B)

    def stage_q(b):
        p = _dot_nt(_upk(wt_v[0:D // 2, :]), _upk(xn_v[b]))
        return [_hedgehog_t(p[j * 64:(j + 1) * 64], zacc_v[j * 128:(j + 1) * 128, :]).astype(bf16)
                for j in range(NP)]

    def stage_g(phi):
        parts = [_dot_nn(_upk(kv_v[j]), phi[j]) for j in range(NP)]
        return jnp.concatenate(parts, axis=0).astype(bf16)

    def stage_h(b, ot, keep, pieces):
        ties = {}
        for k, vals in enumerate(pieces):
            q = min(int(_opt('QS', 1.6) * k) + _opt('Q0', 4), 15)
            for m, val in enumerate(vals):
                ties[((q % 2) * 256 + m * 8, (q // 2) * 128)] = val
        wo = _tie(keep, wou_v[...], ties)
        attn = lax.dot_general(ot, _upk(wo), _TN_DIMS, preferred_element_type=f32)
        attn_v[pl.ds(row_at(b), B), :] = attn
        return attn

    def stage_i(b, attn, valid=None):
        rows = pl.ds(row_at(b), B)
        if attn is None:
            attn = attn_v[rows, :]
        xb = x_v[rows, :]
        bv = bestv_v[...]
        bi = besti_v[...]
        wrow = wrb_v[0:1, :]
        pieces, outs, nvs, nis = [], [], [], []
        for k in range(B // R):
            sl = slice(k * R, (k + 1) * R)
            h = xb[sl].astype(f32) + attn[sl]
            xc = h - jnp.mean(h, axis=-1, keepdims=True)
            v = jnp.mean(xc * xc, axis=-1, keepdims=True)
            rw = jnp.sum(xc * wrow, axis=-1, keepdims=True)
            rs = lax.rsqrt(v + LN_EPS)
            o = h + xc * rs
            outs.append(o.astype(bf16))
            r = jnp.broadcast_to(rw * rs, (R, 128))
            if valid is not None:
                r = jnp.where(valid, r, -jnp.inf)
            idx = lax.broadcasted_iota(jnp.int32, (R, 128), 0) + (b * B + k * R)
            better = r > bv[sl]
            nv = jnp.where(better, r, bv[sl])
            nvs.append(nv)
            nis.append(jnp.where(better, idx, bi[sl]))
            pieces.append(_vregs(o) + _vregs(nv))
        out_v[rows, :] = jnp.concatenate(outs, axis=0)
        bestv_v[...] = jnp.concatenate(nvs, axis=0)
        besti_v[...] = jnp.concatenate(nis, axis=0)
        return pieces

    def p2_body(i, c):
        b0 = i * BPI
        keep = flag_s[0] > 0
        pieces = stage_i(jnp.maximum(b0 - 1, 0), None, i > 0)
        phi = [stage_q(b0), stage_q(b0 + 1)]
        ot = [stage_g(phi[0])]
        phi.append(stage_q(b0 + 2))
        attn = stage_h(b0, ot[0], keep, pieces)
        ot.append(stage_g(phi[1]))
        pieces = stage_i(b0, attn)
        phi.append(stage_q(b0 + 3))
        attn = stage_h(b0 + 1, ot[1], keep, pieces)
        ot.append(stage_g(phi[2]))
        ot.append(stage_g(phi[3]))
        pieces = stage_i(b0 + 1, attn)
        attn = stage_h(b0 + 2, ot[2], keep, pieces)
        pieces = stage_i(b0 + 2, attn)
        stage_h(b0 + 3, ot[3], keep, pieces)

        @pl.when(i > 0)
        def _():
            cp_out(jnp.maximum(i - 1, 0)).start()

        return c

    lax.fori_loop(0, NI, p2_body, 0)
    cp_wg.wait()
    cp_wu.wait()
    cp_wd.wait()
    stage_i(NB - 1, None)
    cp_out(NI - 1).start()

    bv = bestv_v[...]
    mval = jnp.max(bv, axis=0, keepdims=True)
    sel = jnp.min(jnp.where(bv == mval, besti_v[...], S - 1), axis=0, keepdims=True)
    idx = sel[0, 0]
    base = pl.multiple_of((idx // 16) * 16, 16)
    rows = pl.ds(base, 16)
    h = x_v[rows, :].astype(f32) + attn_v[rows, :]
    hn = _layernorm(h)
    xs = hn.astype(bf16)
    acts = []
    y = None
    for k in range(F // FC + 1):
        if k < F // FC:
            g = _dot_nn(xs, wg_v[:, k * FC:(k + 1) * FC])
            u = _dot_nn(xs, wu_v[:, k * FC:(k + 1) * FC])
            acts.append((g * jax.nn.sigmoid(g) * u).astype(bf16))
        if k >= 1:
            t = _dot_nn(acts[k - 1], wd_v[(k - 1) * FC:k * FC, 0:D])
            y = t if y is None else y + t
    y = y * jax.nn.sigmoid(mval[:, 0:1])
    rid = lax.broadcasted_iota(jnp.int32, (16, 1), 0) + base
    res = (h + hn + jnp.where(rid == idx, y, 0.0)).astype(bf16)
    for i in range(NI):
        cp_out(i).wait()
    out_v[rows, :] = res
    fix = pltpu.make_async_copy(out_v.at[rows], out_hbm.at[rows], sem_o.at[0])
    fix.start()
    fix.wait()


@jax.jit
def pallas_sequential_preLN__linear_kernel_hedgehog__moe_arch_mod__prompt_kernel(
    A_x: jax.Array,
    A_wqkv: jax.Array,
    A_w_phi: jax.Array,
    A_wo: jax.Array,
    B_x: jax.Array,
    B_w_r: jax.Array,
    B_w_gate: jax.Array,
    B_w_up: jax.Array,
    B_w_down: jax.Array,
):
    del B_x
    x = A_x.reshape(S, D)
    wphi = A_w_phi.reshape(H * DH, DH)
    wr = B_w_r.reshape(8, 128)
    any_spec = pl.BlockSpec(memory_space=pl.ANY)
    out = pl.pallas_call(
        _kernel,
        out_shape=jax.ShapeDtypeStruct((S, D), bf16),
        in_specs=[any_spec] * 8,
        out_specs=any_spec,
        scratch_shapes=[
            pltpu.VMEM((S, D), bf16),
            pltpu.VMEM((D, 3 * D), bf16),
            pltpu.VMEM((H * DH, DH), bf16),
            pltpu.VMEM((D, D), bf16),
            pltpu.VMEM((8, 128), bf16),
            pltpu.VMEM((D, F), bf16),
            pltpu.VMEM((D, F), bf16),
            pltpu.VMEM((F, D + 128), bf16),
            pltpu.VMEM((3 * D // 2, D), u32),
            pltpu.VMEM((D // 2, D), u32),
            pltpu.VMEM((8, 64, 128), u32),
            pltpu.VMEM((NB + T // B, B // 2, D), u32),
            pltpu.VMEM((NP, 64, 128), f32),
            pltpu.VMEM((2 * D, 128), f32),
            pltpu.VMEM((NP, 32, 128), u32),
            pltpu.VMEM((S, D), f32),
            pltpu.VMEM((S, D), bf16),
            pltpu.VMEM((8, D), f32),
            pltpu.VMEM((B, 128), f32),
            pltpu.VMEM((B, 128), jnp.int32),
            pltpu.SMEM((1,), jnp.int32),
            pltpu.SemaphoreType.DMA((_NSEM_IN,)),
            pltpu.SemaphoreType.DMA((NI,)),
        ],
        compiler_params=pltpu.CompilerParams(vmem_limit_bytes=110 * 1024 * 1024),
        name="hedgehog_mod",
    )(x, A_wqkv, wphi, A_wo, wr, B_w_gate, B_w_up, B_w_down)
    return out.reshape(1, S, D)
```

```python
import os
import jax
import jax.numpy as jnp
from jax import lax
import jax.experimental.pallas as pl
import jax.experimental.pallas.tpu as pltpu

S = 2048
D = 1024
H = 32
DH = 32
F = 3584
T = 256
NT = S // T
B = 128
NB = S // B
BPI = 4
NI = NB // BPI
NP = H // 2
FC = 512
R = 16
NBV = 13
NCH = 4
LOG2E = 1.4426950408889634
LN_EPS = 1e-5
DEN_EPS = 1e-6

_NT_DIMS = (((1,), (1,)), ((), ()))
_TN_DIMS = (((0,), (0,)), ((), ()))

bf16 = jnp.bfloat16
f32 = jnp.float32
u32 = jnp.uint32


def _opt(name, default):
    return type(default)(os.environ.get(name, default))


def _dot_nt(a, b):
    return lax.dot_general(a, b, _NT_DIMS, preferred_element_type=f32)


def _dot_nn(a, b):
    return jnp.dot(a, b, preferred_element_type=f32)


def _pk(x):
    return pltpu.bitcast(x, u32)


def _upk(x):
    return pltpu.bitcast(x, bf16)


def _layernorm(x):
    m = jnp.mean(x, axis=-1, keepdims=True)
    xc = x - m
    v = jnp.mean(xc * xc, axis=-1, keepdims=True)
    return xc * lax.rsqrt(v + LN_EPS)


def _allreduce8(x, op):
    x = op(x, pltpu.roll(x, 4, 1))
    x = op(x, pltpu.roll(x, 2, 1))
    x = op(x, pltpu.roll(x, 1, 1))
    return x


def _hedgehog_t(p, z=None):
    t = p.shape[-1]
    p4 = p.reshape(2, 4, 8, t)
    mx = _allreduce8(jnp.max(p4, axis=1), jnp.maximum)
    mn = _allreduce8(jnp.min(p4, axis=1), jnp.minimum)
    ep = jnp.exp2(p4 - mx[:, None])
    en = jnp.exp2(mn[:, None] - p4)
    a = pl.reciprocal(_allreduce8(jnp.sum(ep, axis=1), jnp.add), approx=True)
    b = pl.reciprocal(_allreduce8(jnp.sum(en, axis=1), jnp.add), approx=True)
    if z is not None:
        dp = jnp.sum(ep * z[0:64].reshape(2, 4, 8, t), axis=1)
        dn = jnp.sum(en * z[64:128].reshape(2, 4, 8, t), axis=1)
        den = _allreduce8(dp * a + dn * b, jnp.add) + DEN_EPS
        inv = pl.reciprocal(den, approx=True)
        a = a * inv
        b = b * inv
    fp = (ep * a[:, None]).reshape(64, t)
    fn = (en * b[:, None]).reshape(64, t)
    return jnp.concatenate([fp, fn], axis=0)


def _tie(keep, w, ties):
    rows = sorted({r for r, _ in ties})
    out, pos = [], 0
    for r in rows:
        if r > pos:
            out.append(w[pos:r])
        cols = sorted(c for rr, c in ties if rr == r)
        parts, cpos = [], 0
        for c in cols:
            if c > cpos:
                parts.append(w[r:r + 8, cpos:c])
            parts.append(jnp.where(keep, w[r:r + 8, c:c + 128], ties[(r, c)]))
            cpos = c + 128
        if cpos < w.shape[1]:
            parts.append(w[r:r + 8, cpos:])
        out.append(jnp.concatenate(parts, axis=1) if len(parts) > 1 else parts[0])
        pos = r + 8
    if pos < w.shape[0]:
        out.append(w[pos:])
    return jnp.concatenate(out, axis=0)


def _vregs(x):
    if x.dtype != u32:
        x = pltpu.bitcast(x, u32)
    return [x[r:r + 8, c:c + 128] for r in range(0, x.shape[0], 8) for c in range(0, x.shape[1], 128)]


_WCHUNKS = ((D, 256, 2), (D + 256, 256, 3), (D + 512, 512, 4),
            (2 * D, 512, 5), (2 * D + 512, 512, 6),
            (0, 1024, 9))
_NSEM_IN = 10
_PHI_A = 256


def _kernel(x_hbm, wqkv_hbm, wphi_hbm, wo_hbm, wr_hbm, wg_hbm, wu_hbm, wd_hbm,
            out_hbm,
            x_v, wqkv_v, wphi_v, wo_v, wr_v, wg_v, wu_v, wd_v,
            wt_v, amat_v, xn_v, kvacc_v, zacc_v, kv_v, phi_v, d_v, st_v, pend_v, out_v, wrb_v,
            bestv_v, besti_v, flag_s,
            sem_i, sem_o):

    wqkv_u = wqkv_hbm.bitcast(u32)

    def cp_x(lo, n, sem):
        return pltpu.make_async_copy(x_hbm.at[pl.ds(lo, n)], x_v.at[pl.ds(lo, n)], sem_i.at[sem])

    def cp_w(c):
        lo, w, sem = _WCHUNKS[c]
        return pltpu.make_async_copy(wqkv_u.at[:, pl.ds(lo, w)], wqkv_v.at[:, pl.ds(lo, w)], sem_i.at[sem])

    cp_pa = pltpu.make_async_copy(wphi_hbm.at[pl.ds(0, _PHI_A)], wphi_v.at[pl.ds(0, _PHI_A)], sem_i.at[0])
    cp_x0 = cp_x(0, T, 1)
    cp_pb = pltpu.make_async_copy(wphi_hbm.at[pl.ds(_PHI_A, D - _PHI_A)], wphi_v.at[pl.ds(_PHI_A, D - _PHI_A)],
                                  sem_i.at[3])
    cp_x1 = cp_x(T, T, 6)
    cp_x2 = cp_x(2 * T, T, 7)
    cp_x3 = cp_x(3 * T, S - 3 * T, 8)
    cp_wr = pltpu.make_async_copy(wr_hbm, wr_v, sem_i.at[9])
    cp_wo = pltpu.make_async_copy(wo_hbm.bitcast(u32), wo_v, sem_i.at[9])
    cp_wg = pltpu.make_async_copy(wg_hbm.bitcast(u32), wg_v.at[:, pl.ds(0, F)], sem_i.at[9])
    cp_wu = pltpu.make_async_copy(wu_hbm.bitcast(u32), wu_v.at[:, pl.ds(0, F)], sem_i.at[9])
    cp_wd = pltpu.make_async_copy(wd_hbm.bitcast(u32), wd_v.at[:, pl.ds(0, D)], sem_i.at[9])

    def cp_out(k):
        lo = k * BPI * B
        if not isinstance(k, int):
            lo = pl.multiple_of(lo, B)
        return pltpu.make_async_copy(out_v.at[pl.ds(lo, BPI * B)], out_hbm.at[pl.ds(lo, BPI * B)], sem_o.at[0])

    cp_pa.start()
    cp_x0.start()
    cp_w(0).start()
    cp_pb.start()
    for c in range(1, 5):
        cp_w(c).start()
    cp_x1.start()
    cp_x2.start()
    cp_x3.start()
    cp_wr.start()
    cp_w(5).start()
    cp_wo.start()
    cp_wg.start()
    cp_wu.start()
    cp_wd.start()
    flag_s[0] = 1

    wt_b, amat_b, xn_b, kv_b = (r.bitcast(bf16) for r in (wt_v, amat_v, xn_v, kv_v))

    def ln1(i):
        if isinstance(i, int):
            src = dst = i * T
        else:
            src = pl.multiple_of(jnp.minimum(i, NT - 1) * T, T)
            dst = pl.multiple_of(i * T, T)
        pieces = []
        for k in range(T // R):
            p = _layernorm(x_v[pl.ds(src + k * R, R), :].astype(f32))
            xn_b[pl.ds(dst + k * R, R), :] = p.astype(bf16)
            pieces.append(p)
        return pieces

    def load_xn(i, n):
        lo = i * (n // 2)
        if not isinstance(i, int):
            lo = pl.multiple_of(lo, n // 2)
        return _upk(xn_v[pl.ds(lo, n // 2), :])

    def k_side(p, j0, first):
        res = []
        for j in range(p.shape[0] // 64):
            ph = _hedgehog_t(p[j * 64:(j + 1) * 64])
            rows = slice((j0 + j) * 128, (j0 + j + 1) * 128)
            for s in range(T // 128):
                part = ph[:, s * 128:(s + 1) * 128]
                if first and s == 0:
                    zacc_v[rows, :] = part
                else:
                    zacc_v[rows, :] += part
            res.append(ph.astype(bf16))
        return res

    def lhs_ties(pieces, nrows):
        ties = {}
        half = (len(pieces) + 1) // 2
        step = (nrows // half) // 8 * 8
        for k, p in enumerate(pieces):
            for q, val in enumerate(p):
                ties[((k % half) * step + (q // 4) * 8, (k // half) * 512 + (q % 4) * 128)] = val
        return ties

    r_i = lax.broadcasted_iota(jnp.int32, (128, DH), 0)
    c_i = lax.broadcasted_iota(jnp.int32, (128, DH), 1)
    expand = (r_i % DH == c_i).astype(bf16)
    r_h = lax.broadcasted_iota(jnp.int32, (128, 128), 0) // DH
    c_h = lax.broadcasted_iota(jnp.int32, (128, 128), 1) // DH
    same_head = r_h == c_h

    def make_amat(g):
        a = _dot_nt(expand, wphi_v[g * 128:(g + 1) * 128, :])
        amat_b[:, g * 128:(g + 1) * 128] = jnp.where(same_head, a, 0.0).astype(bf16)

    def fold(c, keep=None, ties=None):
        lo, w, _ = _WCHUNKS[c]
        for n, g0 in enumerate(range(lo, lo + w, 128)):
            am = amat_v[:, g0 % D:g0 % D + 128]
            if ties is not None and ties[n]:
                am = _tie(keep, am, ties[n])
            wt_b[g0:g0 + 128, :] = (_dot_nt(_upk(am), _upk(wqkv_v[:, g0:g0 + 128])) * LOG2E).astype(bf16)

    def transpose_v(c):
        lo, w, _ = _WCHUNKS[c]
        wt_b[lo:lo + w, :] = _upk(wqkv_v[:, lo:lo + w]).T

    def wt_rows(lo, w):
        return _upk(wt_v[lo // 2:(lo + w) // 2, :])

    def kv_prod(vt, j, phik):
        return _dot_nt(vt[j * 64:(j + 1) * 64].astype(bf16), phik)

    bestv_v[...] = jnp.full(bestv_v.shape, -jnp.inf, f32)
    besti_v[...] = lax.broadcasted_iota(jnp.int32, besti_v.shape, 0)
    d_v[0:B, :] = jnp.zeros((B, D), f32)
    pend_v[...] = jnp.zeros(pend_v.shape, f32)

    cp_pa.wait()
    for g in range(_PHI_A // 128):
        make_amat(g)

    cp_x0.wait()
    ln1(0)
    xn0 = load_xn(0, T)

    cp_w(0).wait()
    fold(0)
    phik0 = k_side(_dot_nt(wt_rows(D, 256), xn0), 0, True)

    cp_pb.wait()
    cp_w(1).wait()
    for g in range(_PHI_A // 128, 8):
        make_amat(g)
    fold(1)
    phik0 += k_side(_dot_nt(wt_rows(D + 256, 256), xn0), len(phik0), True)

    cp_w(2).wait()
    fold(2)
    phik0 += k_side(_dot_nt(wt_rows(D + 512, 256), xn0), len(phik0), True)

    cp_w(3).wait()
    phik0 += k_side(_dot_nt(wt_rows(D + 768, 256), xn0), len(phik0), True)
    transpose_v(3)
    vt_a = _dot_nt(wt_rows(2 * D, 512), xn0)

    cp_w(4).wait()
    cp_x1.wait()
    keep = flag_s[0] > 0
    transpose_v(4)
    for j in range(8):
        kvacc_v[j] = kv_prod(vt_a, j, phik0[j])
    pieces = ln1(1)
    wv = wt_v[(2 * D + 512) // 2:(3 * D) // 2, :]
    vt_b0 = _dot_nt(_upk(wv), xn0[0:B])
    vt_b1 = _dot_nt(_upk(_tie(keep, wv, lhs_ties([_vregs(p) for p in pieces], 256))), xn0[B:T])
    vt_b = jnp.concatenate([vt_b0, vt_b1], axis=1)
    for j in range(8):
        kvacc_v[8 + j] = kv_prod(vt_b, j, phik0[8 + j])
    cp_x2.wait()

    def p1_body(i, c):
        @pl.when(i == 2)
        def _():
            cp_x3.wait()

        keep = flag_s[0] > 0
        xn = load_xn(i, T)
        phik = k_side(_dot_nt(wt_rows(D, D), xn), 0, False)
        pieces = [_vregs(p) for p in ln1(i + 1)]
        wv = wt_v[D:3 * D // 2, :]
        if _opt('LNT', 1) == 0:
            vt = _dot_nt(_upk(_tie(keep, wv, lhs_ties(pieces, D // 2))), xn)
        else:
            ties = lhs_ties(pieces, D // 2)
            t0 = {(r, c + 512): v for (r, c), v in ties.items() if c < 512}
            t1 = {(r, c - 512): v for (r, c), v in ties.items() if c >= 512}
            vt = jnp.concatenate([_dot_nt(_upk(_tie(keep, wv, t0)), xn[0:B]),
                                  _dot_nt(_upk(_tie(keep, wv, t1)), xn[B:T])], axis=1)
        for j in range(NP):
            kvacc_v[j] += kv_prod(vt, j, phik[j])
        return c

    lax.fori_loop(1, NT, p1_body, 0)

    cp_wr.wait()
    cp_w(5).wait()
    cp_wo.wait()
    cp_wg.wait()
    cp_wu.wait()
    cp_wd.wait()
    keep = flag_s[0] > 0
    kv_mask = (lax.broadcasted_iota(jnp.int32, (64, 128), 0) // DH
               == (lax.broadcasted_iota(jnp.int32, (64, 128), 1) // DH) % 2)
    ties = [{} for _ in range(8)]
    for j in range(NP):
        kvj = jnp.where(kv_mask, kvacc_v[j], 0.0)
        kv_b[:, j * 128:(j + 1) * 128] = kvj.astype(bf16)
        zj = jnp.broadcast_to(jnp.sum(zacc_v[j * 128:(j + 1) * 128, :], axis=-1, keepdims=True), (128, 128))
        zacc_v[j * 128:(j + 1) * 128, :] = zj
        if j < 14:
            dep = jnp.max(jnp.concatenate([kvj, zj], axis=0).reshape(6, 32, 128), axis=0)
            for q, v in enumerate(_vregs(dep)):
                ties[1 + j // 2][((j % 2) * 32 + q * 8, 0)] = v
    wr = wr_v[...].astype(f32)
    wsum = jnp.sum(jnp.sum(wr, axis=0, keepdims=True), axis=1, keepdims=True)
    wrb_v[...] = jnp.concatenate(
        [jnp.broadcast_to(wr[j:j + 1, :], (8, 128)) for j in range(8)] + [jnp.broadcast_to(wsum, (8, 128))],
        axis=1)
    fold(5, keep, ties)

    def row_at(b):
        if isinstance(b, int):
            return b * B
        return pl.multiple_of(b * B, B)

    def stage_q(b, slot, keep=None, pieces=None):
        wq = wt_v[0:D // 2, :]
        if pieces is not None:
            ties = {}
            r0, r1 = _opt('TQ0', 128), _opt('TQ1', 512)
            step = (r1 - r0) // len(pieces) // 8 * 8
            for k, vals in enumerate(pieces):
                for m, val in enumerate(vals):
                    ties[(r0 + k * step + (m // 4) * 8, (m % 4) * 128)] = val
            wq = _tie(keep, wq, ties)
        p = _dot_nt(_upk(wq), load_xn(b, B))
        res = []
        for j in range(NP):
            ph = _hedgehog_t(p[j * 64:(j + 1) * 64], zacc_v[j * 128:(j + 1) * 128, :]).astype(bf16)
            if _opt('PHIV', 0):
                phi_v[slot, j * 64:(j + 1) * 64, :] = _pk(ph)
            res.append(ph)
        return res

    def stage_g(phi, slot):
        if _opt('PHIV', 0):
            phi = [_upk(phi_v[slot, j * 64:(j + 1) * 64, :]) for j in range(NP)]
        parts = [_dot_nn(_upk(kv_v[:, j * 128:(j + 1) * 128]), phi[j]) for j in range(NP)]
        return jnp.concatenate(parts, axis=0).astype(bf16)

    def lanes(x):
        return jnp.broadcast_to(x, (x.shape[0], 128))

    def stage_h(b, ot, keep, pieces):
        wo = wo_v[...]
        if pieces is not None:
            ties = {}
            for k, vals in enumerate(pieces):
                q = min(int(_opt('QS', 1.6) * k) + _opt('Q0', 4), 15)
                for m, val in enumerate(vals):
                    ties[((q % 2) * 256 + m * 8, (q // 2) * 128)] = val
            wo = _tie(keep, wo, ties)
        rows = pl.ds(row_at(b), B)
        h = x_v[rows, :].astype(f32) + lax.dot_general(ot, _upk(wo), _TN_DIMS, preferred_element_type=f32)
        c0 = lanes(jnp.mean(h[:, 0:128], axis=-1, keepdims=True))
        s1 = s2 = s3 = None
        ds = []
        for c in range(D // 128):
            d = h[:, c * 128:(c + 1) * 128] - c0
            ds.append(d)
            t2 = d * d
            t3 = (d.reshape(B // 8, 8, 128) * wrb_v[:, c * 128:(c + 1) * 128][None]).reshape(B, 128)
            s1, s2, s3 = (d, t2, t3) if c == 0 else (s1 + d, s2 + t2, s3 + t3)
        d_v[rows, :] = jnp.concatenate(ds, axis=1)
        return jnp.concatenate([s1, s2, s3, c0], axis=1)

    def stage_i(b, part, valid=None):
        rows = pl.ds(row_at(b), B)
        d = d_v[rows, :]
        bv = bestv_v[...]
        bi = besti_v[...]
        wsum = wrb_v[0:1, D:D + 128]
        pieces, outs, nvs, nis, sts = [], [], [], [], []
        for k in range(B // R):
            sl = slice(k * R, (k + 1) * R)
            red = [lanes(jnp.sum(part[sl, n * 128:(n + 1) * 128], axis=-1, keepdims=True)) for n in range(3)]
            c0 = part[sl, 384:512]
            mu = red[0] * (1.0 / D)
            var = jnp.maximum(red[1] * (1.0 / D) - mu * mu, 0.0)
            rs = lax.rsqrt(var + LN_EPS)
            murs = mu * rs
            r = red[2] * rs - murs * wsum
            a = 1.0 + rs
            off = c0 - murs
            o = jnp.concatenate([d[sl, c * 128:(c + 1) * 128] * a + off for c in range(D // 128)], axis=1)
            outs.append(o.astype(bf16))
            sts.append(jnp.concatenate([rs, murs, c0], axis=1))
            if valid is not None:
                r = jnp.where(valid, r, -jnp.inf)
            idx = lax.broadcasted_iota(jnp.int32, (R, 128), 0) + (b * B + k * R)
            better = r > bv[sl]
            nv = jnp.where(better, r, bv[sl])
            nvs.append(nv)
            nis.append(jnp.where(better, idx, bi[sl]))
            pieces.append(_vregs(o) + _vregs(nv))
        out_v[rows, :] = jnp.concatenate(outs, axis=0)
        st_v[rows, :] = jnp.concatenate(sts, axis=0)
        bestv_v[...] = jnp.concatenate(nvs, axis=0)
        besti_v[...] = jnp.concatenate(nis, axis=0)
        return pieces

    def p2_body(i, c):
        b0 = i * BPI
        keep = flag_s[0] > 0
        qt = _opt('QTIE', 1)
        pieces = stage_i(jnp.maximum(b0 - 1, 0), pend_v[...], i > 0)
        phi = [stage_q(b0, 0), stage_q(b0 + 1, 1, keep, pieces if qt else None)]
        ot = [stage_g(phi[0], 0)]
        phi.append(stage_q(b0 + 2, 2))
        part = stage_h(b0, ot[0], keep, None if qt else pieces)
        ot.append(stage_g(phi[1], 1))
        pieces = stage_i(b0, part)
        phi.append(stage_q(b0 + 3, 3, keep, pieces if qt == 2 else None))
        part = stage_h(b0 + 1, ot[1], keep, None if qt == 2 else pieces)
        ot.append(stage_g(phi[2], 2))
        ot.append(stage_g(phi[3], 3))
        pieces = stage_i(b0 + 1, part)
        part = stage_h(b0 + 2, ot[2], keep, pieces)
        pieces = stage_i(b0 + 2, part)
        pend_v[...] = stage_h(b0 + 3, ot[3], keep, pieces)

        @pl.when(i > 0)
        def _():
            cp_out(jnp.maximum(i - 1, 0)).start()

        return c

    lax.fori_loop(0, NI, p2_body, 0)
    stage_i(NB - 1, pend_v[...])
    cp_out(NI - 1).start()

    keep = flag_s[0] > 0
    bv = bestv_v[...]
    mval = jnp.max(bv, axis=0, keepdims=True)
    sel = jnp.min(jnp.where(bv == mval, besti_v[...], S - 1), axis=0, keepdims=True)
    idx = sel[0, 0]
    drow = d_v[pl.ds(idx, 1), :]
    strow = st_v[pl.ds(idx, 1), :]
    xrow = jnp.concatenate([drow[:, c * 128:(c + 1) * 128] * strow[:, 0:128] - strow[:, 128:256]
                            for c in range(D // 128)], axis=1).astype(bf16)
    xs = jnp.broadcast_to(xrow, (16, D))

    def act(g, u):
        a = g * pl.reciprocal(1.0 + jnp.exp(-g), approx=True) * u
        return jnp.concatenate([a, a], axis=0).astype(bf16)

    def down(a, lo, w):
        return _dot_nn(a, _upk(wd_v[lo // 2:(lo + w) // 2, 0:D]))[0:8]

    NM = F - NBV * 128
    xcol = jnp.broadcast_to(xrow.astype(f32), (128, D)).T
    jobs = [(which, b) for b in range(NBV) for which in (0, 1)]
    vres, prev = {}, None
    for j0 in range(0, len(jobs), NCH):
        grp = jobs[j0:j0 + NCH]
        accs = [None] * len(grp)
        for r in range(D // 16):
            for n, (which, b) in enumerate(grp):
                w = _upk((wg_v, wu_v)[which][r * 8:(r + 1) * 8, NM + b * 128:NM + (b + 1) * 128]).astype(f32)
                t0 = w[0:8] * xcol[r * 16:r * 16 + 8]
                t1 = w[8:16] * xcol[r * 16 + 8:r * 16 + 16]
                if accs[n] is None:
                    if prev is not None:
                        t0 = jnp.where(keep, t0, prev[n % len(prev)])
                    accs[n] = t0 + t1
                else:
                    accs[n] = (accs[n] + t0) + t1
        prev = accs
        for n, job in enumerate(grp):
            vres[job] = _allreduce8(accs[n][None], jnp.add)[0]

    chunks = [(lo, min(FC, NM - lo)) for lo in range(0, NM, FC)]
    acts, y = [], None
    for k, (lo, w) in enumerate(chunks):
        g = _dot_nn(xs, _upk(wg_v[:, lo:lo + w]))
        u = _dot_nn(xs, _upk(wu_v[:, lo:lo + w]))
        acts.append(act(g[0:8], u[0:8]))
        if k >= 1:
            t = down(acts[k - 1], *chunks[k - 1])
            y = t if y is None else y + t
    y = y + down(acts[-1], *chunks[-1])
    for b0, nb in ((0, 4), (4, 4), (8, 4), (12, 1)):
        g = jnp.concatenate([vres[(0, b)] for b in range(b0, b0 + nb)], axis=1)
        u = jnp.concatenate([vres[(1, b)] for b in range(b0, b0 + nb)], axis=1)
        y = y + down(act(g, u), NM + b0 * 128, nb * 128)

    gate = jnp.broadcast_to(jax.nn.sigmoid(mval), (8, 128))
    base = pl.multiple_of((idx >> 4) << 4, 16)
    rows = pl.ds(base, 16)
    d16 = d_v[rows, :]
    st16 = st_v[rows, :]
    a16 = 1.0 + st16[:, 0:128]
    off16 = st16[:, 256:384] - st16[:, 128:256]
    hit = (lax.broadcasted_iota(jnp.int32, (16, 128), 0) + base) == idx
    res = []
    for c in range(D // 128):
        yc = y[:, c * 128:(c + 1) * 128] * gate
        yc = jnp.concatenate([yc, yc], axis=0)
        res.append(d16[:, c * 128:(c + 1) * 128] * a16 + off16 + jnp.where(hit, yc, 0.0))
    res = jnp.concatenate(res, axis=1).astype(bf16)
    for i in range(NI):
        cp_out(i).wait()
    out_v[rows, :] = res
    fix = pltpu.make_async_copy(out_v.at[rows], out_hbm.at[rows], sem_o.at[0])
    fix.start()
    fix.wait()


@jax.jit
def pallas_sequential_preLN__linear_kernel_hedgehog__moe_arch_mod__prompt_kernel(
    A_x: jax.Array,
    A_wqkv: jax.Array,
    A_w_phi: jax.Array,
    A_wo: jax.Array,
    B_x: jax.Array,
    B_w_r: jax.Array,
    B_w_gate: jax.Array,
    B_w_up: jax.Array,
    B_w_down: jax.Array,
):
    del B_x
    x = A_x.reshape(S, D)
    wphi = A_w_phi.reshape(H * DH, DH)
    wr = B_w_r.reshape(8, 128)
    any_spec = pl.BlockSpec(memory_space=pl.ANY)
    out = pl.pallas_call(
        _kernel,
        out_shape=jax.ShapeDtypeStruct((S, D), bf16),
        in_specs=[any_spec] * 8,
        out_specs=any_spec,
        scratch_shapes=[
            pltpu.VMEM((S, D), bf16),
            pltpu.VMEM((D // 2, 3 * D), u32),
            pltpu.VMEM((H * DH, DH), bf16),
            pltpu.VMEM((D // 2, D), u32),
            pltpu.VMEM((8, 128), bf16),
            pltpu.VMEM((D // 2, F + 128), u32),
            pltpu.VMEM((D // 2, F + 128), u32),
            pltpu.VMEM((F // 2, D + 128), u32),
            pltpu.VMEM((3 * D // 2, D), u32),
            pltpu.VMEM((64, 8 * 128), u32),
            pltpu.VMEM(((S + T) // 2, D), u32),
            pltpu.VMEM((NP, 64, 128), f32),
            pltpu.VMEM((2 * D, 128), f32),
            pltpu.VMEM((32, NP * 128), u32),
            pltpu.VMEM((BPI, D, B), u32),
            pltpu.VMEM((S, D), f32),
            pltpu.VMEM((S, 384), f32),
            pltpu.VMEM((B, 512), f32),
            pltpu.VMEM((S, D), bf16),
            pltpu.VMEM((8, D + 128), f32),
            pltpu.VMEM((B, 128), f32),
            pltpu.VMEM((B, 128), jnp.int32),
            pltpu.SMEM((1,), jnp.int32),
            pltpu.SemaphoreType.DMA((_NSEM_IN,)),
            pltpu.SemaphoreType.DMA((1,)),
        ],
        compiler_params=pltpu.CompilerParams(vmem_limit_bytes=110 * 1024 * 1024),
        name="hedgehog_mod",
    )(x, A_wqkv, wphi, A_wo, wr, B_w_gate, B_w_up, B_w_down)
    return out.reshape(1, S, D)
```

```python
import os
import jax
import jax.numpy as jnp
from jax import lax
import jax.experimental.pallas as pl
import jax.experimental.pallas.tpu as pltpu

S = 2048
D = 1024
H = 32
DH = 32
F = 3584
T = 512
NT = S // T
T0 = 256
B = 128
NB = S // B
BPI = 4
NI = NB // BPI
NP = H // 2
FC = 512
R = 16
NBV = 13
NCH = 4
LOG2E = 1.4426950408889634
LN_EPS = 1e-5
DEN_EPS = 1e-6

_NT_DIMS = (((1,), (1,)), ((), ()))
_TN_DIMS = (((0,), (0,)), ((), ()))

bf16 = jnp.bfloat16
f32 = jnp.float32
u32 = jnp.uint32


def _opt(name, default):
    return type(default)(os.environ.get(name, default))


def _dot_nt(a, b):
    return lax.dot_general(a, b, _NT_DIMS, preferred_element_type=f32)


def _dot_nn(a, b):
    return jnp.dot(a, b, preferred_element_type=f32)


def _pk(x):
    return pltpu.bitcast(x, u32)


def _upk(x):
    return pltpu.bitcast(x, bf16)


def _layernorm(x):
    m = jnp.mean(x, axis=-1, keepdims=True)
    xc = x - m
    v = jnp.mean(xc * xc, axis=-1, keepdims=True)
    return xc * lax.rsqrt(v + LN_EPS)


def _allreduce8(x, op):
    x = op(x, pltpu.roll(x, 4, 1))
    x = op(x, pltpu.roll(x, 2, 1))
    x = op(x, pltpu.roll(x, 1, 1))
    return x


def _hedgehog_t(p, z=None):
    t = p.shape[-1]
    p4 = p.reshape(2, 4, 8, t)
    mx = _allreduce8(jnp.max(p4, axis=1), jnp.maximum)
    mn = _allreduce8(jnp.min(p4, axis=1), jnp.minimum)
    ep = jnp.exp2(p4 - mx[:, None])
    en = jnp.exp2(mn[:, None] - p4)
    a = pl.reciprocal(_allreduce8(jnp.sum(ep, axis=1), jnp.add), approx=True)
    b = pl.reciprocal(_allreduce8(jnp.sum(en, axis=1), jnp.add), approx=True)
    if z is not None:
        dp = jnp.sum(ep * z[0:64].reshape(2, 4, 8, t), axis=1)
        dn = jnp.sum(en * z[64:128].reshape(2, 4, 8, t), axis=1)
        den = _allreduce8(dp * a + dn * b, jnp.add) + DEN_EPS
        inv = pl.reciprocal(den, approx=True)
        a = a * inv
        b = b * inv
    fp = (ep * a[:, None]).reshape(64, t)
    fn = (en * b[:, None]).reshape(64, t)
    return jnp.concatenate([fp, fn], axis=0)


def _tie(keep, w, ties):
    rows = sorted({r for r, _ in ties})
    out, pos = [], 0
    for r in rows:
        if r > pos:
            out.append(w[pos:r])
        cols = sorted(c for rr, c in ties if rr == r)
        parts, cpos = [], 0
        for c in cols:
            if c > cpos:
                parts.append(w[r:r + 8, cpos:c])
            parts.append(jnp.where(keep, w[r:r + 8, c:c + 128], ties[(r, c)]))
            cpos = c + 128
        if cpos < w.shape[1]:
            parts.append(w[r:r + 8, cpos:])
        out.append(jnp.concatenate(parts, axis=1) if len(parts) > 1 else parts[0])
        pos = r + 8
    if pos < w.shape[0]:
        out.append(w[pos:])
    return jnp.concatenate(out, axis=0)


def _vregs(x):
    if x.dtype != u32:
        x = pltpu.bitcast(x, u32)
    return [x[r:r + 8, c:c + 128] for r in range(0, x.shape[0], 8) for c in range(0, x.shape[1], 128)]


_WCHUNKS = ((D, 256, 2), (D + 256, 384, 3), (D + 640, 384, 4),
            (2 * D, 1024, 5),
            (0, 1024, 7))
_NSEM_IN = 8
_PHI_A = 256


def _kernel(x_hbm, wqkv_hbm, wphi_hbm, wo_hbm, wr_hbm, wg_hbm, wu_hbm, wd_hbm,
            out_hbm,
            x_v, wqkv_v, wphi_v, wo_v, wr_v, wg_v, wu_v, wd_v,
            wt_v, amat_v, xn_v, kvacc_v, zacc_v, kv_v, phi_v, vt_v, pq0_v, pq1_v, pq2_v, pq3_v, d_v, st_v, pend_v, out_v, wrb_v,
            bestv_v, besti_v, flag_s,
            sem_i, sem_o):

    wqkv_u = wqkv_hbm.bitcast(u32)

    def cp_x(lo, n, sem):
        return pltpu.make_async_copy(x_hbm.at[pl.ds(lo, n)], x_v.at[pl.ds(lo, n)], sem_i.at[sem])

    def cp_w(c):
        lo, w, sem = _WCHUNKS[c]
        return pltpu.make_async_copy(wqkv_u.at[:, pl.ds(lo, w)], wqkv_v.at[:, pl.ds(lo, w)], sem_i.at[sem])

    cp_pa = pltpu.make_async_copy(wphi_hbm.at[pl.ds(0, _PHI_A)], wphi_v.at[pl.ds(0, _PHI_A)], sem_i.at[0])
    cp_x0 = cp_x(0, T0, 1)
    cp_pb = pltpu.make_async_copy(wphi_hbm.at[pl.ds(_PHI_A, D - _PHI_A)], wphi_v.at[pl.ds(_PHI_A, D - _PHI_A)],
                                  sem_i.at[3])
    cp_x1 = cp_x(T0, T0, 4)
    cp_x2 = cp_x(T, T, 5)
    cp_x3 = cp_x(2 * T, S - 2 * T, 6)
    cp_wr = pltpu.make_async_copy(wr_hbm, wr_v, sem_i.at[7])
    cp_wo = pltpu.make_async_copy(wo_hbm.bitcast(u32), wo_v, sem_i.at[7])
    cp_wg = pltpu.make_async_copy(wg_hbm.bitcast(u32), wg_v.at[:, pl.ds(0, F)], sem_i.at[7])
    cp_wu = pltpu.make_async_copy(wu_hbm.bitcast(u32), wu_v.at[:, pl.ds(0, F)], sem_i.at[7])
    cp_wd = pltpu.make_async_copy(wd_hbm.bitcast(u32), wd_v.at[:, pl.ds(0, D)], sem_i.at[7])

    def cp_out(b, n):
        lo = b * B
        if not isinstance(b, int):
            lo = pl.multiple_of(lo, B)
        return pltpu.make_async_copy(out_v.at[pl.ds(lo, n * B)], out_hbm.at[pl.ds(lo, n * B)], sem_o.at[0])

    cp_pa.start()
    cp_x0.start()
    cp_w(0).start()
    cp_pb.start()
    cp_w(1).start()
    cp_w(2).start()
    cp_x1.start()
    cp_w(3).start()
    cp_x2.start()
    cp_x3.start()
    cp_wr.start()
    cp_w(4).start()
    cp_wo.start()
    cp_wg.start()
    cp_wu.start()
    cp_wd.start()
    flag_s[0] = 1
    flag_s[1] = 0

    wt_b, amat_b, xn_b, kv_b, phi_b, vt_b = (r.bitcast(bf16) for r in (wt_v, amat_v, xn_v, kv_v, phi_v, vt_v))

    def ln1(src, dst, n):
        pieces = []
        for k in range(n // R):
            p = _layernorm(x_v[pl.ds(src + k * R, R), :].astype(f32))
            xn_b[pl.ds(dst + k * R, R), :] = p.astype(bf16)
            pieces.append(_vregs(p))
        return pieces

    def load_xn(i, n):
        lo = i * (n // 2)
        if not isinstance(i, int):
            lo = pl.multiple_of(lo, n // 2)
        return _upk(xn_v[pl.ds(lo, n // 2), :])

    def k_side(p, j0, first, s, pk):
        res = []
        for j in range(p.shape[0] // 64):
            ph = _hedgehog_t(p[j * 64:(j + 1) * 64])
            rows = slice((j0 + j) * 128, (j0 + j + 1) * 128)
            if first:
                zacc_v[rows, :] = ph
            else:
                zacc_v[rows, :] += ph
            if pk:
                phi_b[rows, s * B:(s + 1) * B] = ph.astype(bf16)
            res.append(ph)
        return res

    def proj(lo, w, xb, keep=None, early=(), late=()):
        lhs = wt_v[lo // 2:(lo + w) // 2, :]
        ties = {}
        for col, pieces in ((0, early), (512, late)):
            if pieces:
                step = (w // 2) // len(pieces) // 8 * 8
                for k, p in enumerate(pieces):
                    for q, val in enumerate(p):
                        ties[(k * step + (q // 4) * 8, col + (q % 4) * 128)] = val
        if ties:
            lhs = _tie(keep, lhs, ties)
        return _dot_nt(_upk(lhs), xb)

    def kv_prod(vts, phis, j, pk):
        zero = flag_s[1]
        if _opt('VK', 0):
            vt = _upk(vt_v[pl.ds(pl.multiple_of(zero + j * 32, 8), 32), :])
        else:
            vt = jnp.concatenate([v[j * 64:(j + 1) * 64] for v in vts], axis=1).astype(bf16)
        if pk:
            ph = _upk(phi_v.at[pl.ds(pl.multiple_of(zero, D), D)][j * 64:(j + 1) * 64, :])
        else:
            ph = jnp.concatenate([p[j] for p in phis], axis=1).astype(bf16)
        return _dot_nt(vt, ph)

    def v_side(xbs, keep, pieces):
        nb = len(xbs)
        slots = 2 * nb - 2
        per = [pieces[k * len(pieces) // slots:(k + 1) * len(pieces) // slots] for k in range(slots)]
        per = [()] + per + [()]
        res = [proj(2 * D, D, xb, keep, per[2 * s], per[2 * s + 1]) for s, xb in enumerate(xbs)]
        if _opt('VK', 0):
            for s, v in enumerate(res):
                vt_b[:, s * B:(s + 1) * B] = v.astype(bf16)
        return res

    r_i = lax.broadcasted_iota(jnp.int32, (128, DH), 0)
    c_i = lax.broadcasted_iota(jnp.int32, (128, DH), 1)
    expand = (r_i % DH == c_i).astype(bf16)
    r_h = lax.broadcasted_iota(jnp.int32, (128, 128), 0) // DH
    c_h = lax.broadcasted_iota(jnp.int32, (128, 128), 1) // DH
    same_head = r_h == c_h

    def make_amat(g):
        a = _dot_nt(expand, wphi_v[g * 128:(g + 1) * 128, :])
        amat_b[:, g * 128:(g + 1) * 128] = jnp.where(same_head, a, 0.0).astype(bf16)

    def fold(c, keep=None, ties=None):
        lo, w, _ = _WCHUNKS[c]
        for n, g0 in enumerate(range(lo, lo + w, 128)):
            am = amat_v[:, g0 % D:g0 % D + 128]
            if ties is not None and ties[n]:
                am = _tie(keep, am, ties[n])
            wt_b[g0:g0 + 128, :] = (_dot_nt(_upk(am), _upk(wqkv_v[:, g0:g0 + 128])) * LOG2E).astype(bf16)

    def transpose_v(c):
        lo, w, _ = _WCHUNKS[c]
        wt_b[lo:lo + w, :] = _upk(wqkv_v[:, lo:lo + w]).T

    bestv_v[...] = jnp.full(bestv_v.shape, -jnp.inf, f32)
    besti_v[...] = lax.broadcasted_iota(jnp.int32, besti_v.shape, 0)
    d_v[(BPI - 1) * B:BPI * B, :] = jnp.zeros((B, D), f32)
    pend_v[...] = jnp.zeros(pend_v.shape, f32)

    cp_pa.wait()
    for g in range(_PHI_A // 128):
        make_amat(g)

    cp_x0.wait()
    ln1(0, 0, T0)
    xb = [load_xn(s, B) for s in range(2)]
    phik = [[], [], [], []]

    def k_chunk(s, lo, w, keep=None, early=(), late=()):
        phik[s] += k_side(proj(D + lo, w, xb[s], keep, early, late), lo // 64, s == 0, s, True)

    cp_w(0).wait()
    fold(0)
    k_chunk(0, 0, 256)
    k_chunk(1, 0, 256)

    cp_pb.wait()
    cp_w(1).wait()
    for g in range(_PHI_A // 128, 8):
        make_amat(g)
    fold(1)
    k_chunk(0, 256, 384)
    k_chunk(1, 256, 384)

    cp_w(2).wait()
    cp_x1.wait()
    keep = flag_s[0] > 0
    fold(2)
    pieces = ln1(T0, T0, T0)
    k_chunk(0, 640, 384, keep, pieces[0:4], pieces[4:8])
    k_chunk(1, 640, 384, keep, pieces[8:12], pieces[12:16])
    xb += [load_xn(s, B) for s in range(2, 4)]
    k_chunk(2, 0, D)
    KS = _opt('KS', 640)
    k_chunk(3, 0, KS)

    cp_w(3).wait()
    cp_x2.wait()
    keep = flag_s[0] > 0
    k_chunk(3, KS, D - KS)
    transpose_v(3)
    vts = v_side(xb, keep, ln1(T, T, T))
    for j in range(NP):
        kvacc_v[j] = kv_prod(vts, phik, j, True)
    cp_x3.wait()

    def p1_body(i, c):
        keep = flag_s[0] > 0
        xb = [load_xn(i * (T // B) + s, B) for s in range(T // B)]
        phik = [k_side(proj(D, D, x), 0, False, s, _opt('PK', 0)) for s, x in enumerate(xb)]
        src = pl.multiple_of(jnp.minimum(i + 1, NT - 1) * T, T)
        vts = v_side(xb, keep, ln1(src, pl.multiple_of((i + 1) * T, T), T))
        for j in range(NP):
            kvacc_v[j] += kv_prod(vts, phik, j, _opt('PK', 0))
        return c

    lax.fori_loop(1, NT, p1_body, 0)

    cp_wr.wait()
    cp_w(4).wait()
    cp_wo.wait()
    cp_wg.wait()
    cp_wu.wait()
    cp_wd.wait()
    keep = flag_s[0] > 0
    kv_mask = (lax.broadcasted_iota(jnp.int32, (64, 128), 0) // DH
               == (lax.broadcasted_iota(jnp.int32, (64, 128), 1) // DH) % 2)
    ties = [{} for _ in range(8)]
    for j in range(NP):
        kvj = jnp.where(kv_mask, kvacc_v[j], 0.0)
        kv_b[:, j * 128:(j + 1) * 128] = kvj.astype(bf16)
        zj = jnp.broadcast_to(jnp.sum(zacc_v[j * 128:(j + 1) * 128, :], axis=-1, keepdims=True), (128, 128))
        zacc_v[j * 128:(j + 1) * 128, :] = zj
        if j < 14:
            dep = jnp.max(jnp.concatenate([kvj, zj], axis=0).reshape(6, 32, 128), axis=0)
            for q, v in enumerate(_vregs(dep)):
                ties[1 + j // 2][((j % 2) * 32 + q * 8, 0)] = v
    wr = wr_v[...].astype(f32)
    wl = jnp.sum(wr, axis=0, keepdims=True)
    wsum = jnp.sum(wl, axis=1, keepdims=True)
    wrb_v[...] = jnp.concatenate(
        [jnp.broadcast_to(wr[j:j + 1, :], (8, 128)) for j in range(8)]
        + [jnp.broadcast_to(wsum, (8, 128)), jnp.broadcast_to(wl, (8, 128))], axis=1)
    fold(4, keep, ties)

    def group(ref, g):
        lo = g * (BPI * B)
        if not isinstance(g, int):
            lo = pl.multiple_of(lo, BPI * B)
        return ref.at[pl.ds(lo, BPI * B)]

    pq_v = (pq0_v, pq1_v, pq2_v, pq3_v)

    def stage_q(b, slot, keep=None, pieces=None):
        wq = wt_v[0:D // 2, :]
        if pieces is not None:
            ties = {}
            r0, r1 = _opt('TQ0', 128), _opt('TQ1', 512)
            step = (r1 - r0) // len(pieces) // 8 * 8
            for k, vals in enumerate(pieces):
                for m, val in enumerate(vals):
                    ties[(r0 + k * step + (m // 4) * 8, (m % 4) * 128)] = val
            wq = _tie(keep, wq, ties)
        p = _dot_nt(_upk(wq), load_xn(b, B))
        res = []
        for j in range(NP):
            ph = _hedgehog_t(p[j * 64:(j + 1) * 64], zacc_v[j * 128:(j + 1) * 128, :]).astype(bf16)
            if _opt('PHIV', 1):
                pq_v[slot].bitcast(bf16)[(j // 2) * 128:(j // 2 + 1) * 128, (j % 2) * B:(j % 2 + 1) * B] = ph
            res.append(ph)
        return res

    def stage_g(phi, slot):
        if _opt('PHIV', 1):
            pq = pq_v[slot].at[pl.ds(pl.multiple_of(flag_s[1], D // 2), D // 2)]
            phi = [_upk(pq[(j // 2) * 64:(j // 2 + 1) * 64, (j % 2) * B:(j % 2 + 1) * B]) for j in range(NP)]
        parts = [_dot_nn(_upk(kv_v[:, j * 128:(j + 1) * 128]), phi[j]) for j in range(NP)]
        return jnp.concatenate(parts, axis=0).astype(bf16)

    def lanes(x):
        return jnp.broadcast_to(x, (x.shape[0], 128))

    def stage_h(views, s, ot, keep, pieces):
        wo = wo_v[...]
        if pieces is not None and _opt('HT', 1):
            ties = {}
            for k, vals in enumerate(pieces):
                q = min(int(_opt('QS', 1.6) * k) + _opt('Q0', 4), 15)
                for m, val in enumerate(vals):
                    ties[((q % 2) * 256 + m * 8, (q // 2) * 128)] = val
            wo = _tie(keep, wo, ties)
        rows = slice(s * B, (s + 1) * B)
        x_g, h_g = views[0], views[1]
        h = x_g[rows, :].astype(f32) + lax.dot_general(ot, _upk(wo), _TN_DIMS, preferred_element_type=f32)
        h_g[rows, :] = h

        def wmul(d, lo):
            return (d.reshape(B // 8, 8, 128) * wrb_v[:, lo:lo + 128][None]).reshape(B, 128)

        h0 = h[:, 0:128]
        s1 = s2 = s3 = None
        for c in range(1, D // 128):
            d = h[:, c * 128:(c + 1) * 128] - h0
            t2 = d * d
            t3 = wmul(d, c * 128)
            s1, s2, s3 = (d, t2, t3) if c == 1 else (s1 + d, s2 + t2, s3 + t3)
        c0 = lanes(jnp.mean(h0, axis=-1, keepdims=True))
        g0 = h0 - c0
        t1 = s1 + 8.0 * g0
        t2 = s2 + g0 * (s1 + t1)
        t3 = s3 + wmul(g0, D + 128)
        return jnp.concatenate([t1, t2, t3, c0], axis=1)

    def stage_i(views, s, part, valid=None):
        _, h_g, out_g, st_g, g = views
        b = g * BPI + s
        rows = slice(s * B, (s + 1) * B)
        d = h_g[rows, :]
        bv = bestv_v[...]
        bi = besti_v[...]
        wsum = wrb_v[0:1, D:D + 128]
        pieces, outs, nvs, nis, sts = [], [], [], [], []
        for k in range(B // R):
            sl = slice(k * R, (k + 1) * R)
            red = [lanes(jnp.sum(part[sl, n * 128:(n + 1) * 128], axis=-1, keepdims=True)) for n in range(3)]
            c0 = part[sl, 384:512]
            mu = red[0] * (1.0 / D)
            var = jnp.maximum(red[1] * (1.0 / D) - mu * mu, 0.0)
            rs = lax.rsqrt(var + LN_EPS)
            r = (red[2] - mu * wsum) * rs
            murs = (mu + c0) * rs
            a = 1.0 + rs
            o = jnp.concatenate([d[sl, c * 128:(c + 1) * 128] * a - murs for c in range(D // 128)], axis=1)
            outs.append(o.astype(bf16))
            sts.append(jnp.concatenate([rs, murs], axis=1))
            if valid is not None:
                r = jnp.where(valid, r, -jnp.inf)
            idx = lax.broadcasted_iota(jnp.int32, (R, 128), 0) + (b * B + k * R)
            better = r > bv[sl]
            nv = jnp.where(better, r, bv[sl])
            nvs.append(nv)
            nis.append(jnp.where(better, idx, bi[sl]))
            pieces.append(_vregs(o) + _vregs(nv))
        out_g[rows, :] = jnp.concatenate(outs, axis=0)
        st_g[rows, :] = jnp.concatenate(sts, axis=0)
        bestv_v[...] = jnp.concatenate(nvs, axis=0)
        besti_v[...] = jnp.concatenate(nis, axis=0)
        return pieces

    def views_of(g):
        return (group(x_v, g), group(d_v, g), group(out_v, g), group(st_v, g), g)

    def p2_body(i, c):
        b0 = i * BPI
        keep = flag_s[0] > 0
        cur = views_of(i)
        pieces = stage_i(views_of(jnp.maximum(i - 1, 0)), BPI - 1, pend_v[...], i > 0)
        if _opt('ORD', 3) == 3:
            phi = [stage_q(b0, 0), stage_q(b0 + 1, 1, keep, pieces), stage_q(b0 + 2, 2), stage_q(b0 + 3, 3)]
            ot = [stage_g(phi[s], s) for s in range(BPI)]
            part = stage_h(cur, 0, ot[0], keep, None)
            pieces = stage_i(cur, 0, part)
            part = stage_h(cur, 1, ot[1], keep, pieces)
        else:
            phi = [stage_q(b0, 0), stage_q(b0 + 1, 1, keep, pieces), stage_q(b0 + 2, 2)]
            ot = [stage_g(phi[0], 0), stage_g(phi[1], 1)]
            part = stage_h(cur, 0, ot[0], keep, None)
            pieces = stage_i(cur, 0, part)
            phi.append(stage_q(b0 + 3, 3, keep, pieces))
            part = stage_h(cur, 1, ot[1], keep, None)
            ot.append(stage_g(phi[2], 2))
            ot.append(stage_g(phi[3], 3))
        pieces = stage_i(cur, 1, part)
        part = stage_h(cur, 2, ot[2], keep, pieces)
        pieces = stage_i(cur, 2, part)
        pend_v[...] = stage_h(cur, 3, ot[3], keep, pieces)

        @pl.when(i > 0)
        def _():
            cp_out(jnp.maximum(b0 - 1, 0), 1).start()

        cp_out(b0, BPI - 1).start()

        return c

    lax.fori_loop(0, NI, p2_body, 0)
    stage_i(views_of(NI - 1), BPI - 1, pend_v[...])
    cp_out(NB - 1, 1).start()

    keep = flag_s[0] > 0
    bv = bestv_v[...]
    mval = jnp.max(bv, axis=0, keepdims=True)
    sel = jnp.min(jnp.where(bv == mval, besti_v[...], S - 1), axis=0, keepdims=True)
    idx = sel[0, 0]
    drow = d_v[pl.ds(idx, 1), :]
    strow = st_v[pl.ds(idx, 1), :]
    xrow = jnp.concatenate([drow[:, c * 128:(c + 1) * 128] * strow[:, 0:128] - strow[:, 128:256]
                            for c in range(D // 128)], axis=1).astype(bf16)
    xs = jnp.broadcast_to(xrow, (16, D))

    def act(g, u):
        a = g * pl.reciprocal(1.0 + jnp.exp(-g), approx=True) * u
        return jnp.concatenate([a, a], axis=0).astype(bf16)

    def down(a, lo, w):
        return _dot_nn(a, _upk(wd_v[lo // 2:(lo + w) // 2, 0:D]))[0:8]

    NM = F - NBV * 128
    xcol = jnp.broadcast_to(xrow.astype(f32), (128, D)).T
    jobs = [(which, b) for b in range(NBV) for which in (0, 1)]
    vres, prev = {}, None
    for j0 in range(0, len(jobs), NCH):
        grp = jobs[j0:j0 + NCH]
        accs = [None] * len(grp)
        for r in range(D // 16):
            for n, (which, b) in enumerate(grp):
                w = _upk((wg_v, wu_v)[which][r * 8:(r + 1) * 8, NM + b * 128:NM + (b + 1) * 128]).astype(f32)
                t0 = w[0:8] * xcol[r * 16:r * 16 + 8]
                t1 = w[8:16] * xcol[r * 16 + 8:r * 16 + 16]
                if accs[n] is None:
                    if prev is not None:
                        t0 = jnp.where(keep, t0, prev[n % len(prev)])
                    accs[n] = t0 + t1
                else:
                    accs[n] = (accs[n] + t0) + t1
        prev = accs
        for n, job in enumerate(grp):
            vres[job] = _allreduce8(accs[n][None], jnp.add)[0]

    chunks = [(lo, min(FC, NM - lo)) for lo in range(0, NM, FC)]
    acts, y = [], None
    for k, (lo, w) in enumerate(chunks):
        g = _dot_nn(xs, _upk(wg_v[:, lo:lo + w]))
        u = _dot_nn(xs, _upk(wu_v[:, lo:lo + w]))
        acts.append(act(g[0:8], u[0:8]))
        if k >= 1:
            t = down(acts[k - 1], *chunks[k - 1])
            y = t if y is None else y + t
    y = y + down(acts[-1], *chunks[-1])
    for b0, nb in ((0, 4), (4, 4), (8, 4), (12, 1)):
        g = jnp.concatenate([vres[(0, b)] for b in range(b0, b0 + nb)], axis=1)
        u = jnp.concatenate([vres[(1, b)] for b in range(b0, b0 + nb)], axis=1)
        y = y + down(act(g, u), NM + b0 * 128, nb * 128)

    gate = jnp.broadcast_to(jax.nn.sigmoid(mval), (8, 128))
    base = pl.multiple_of((idx >> 4) << 4, 16)
    rows = pl.ds(base, 16)
    d16 = d_v[rows, :]
    st16 = st_v[rows, :]
    a16 = 1.0 + st16[:, 0:128]
    off16 = st16[:, 128:256]
    hit = (lax.broadcasted_iota(jnp.int32, (16, 128), 0) + base) == idx
    res = []
    for c in range(D // 128):
        yc = y[:, c * 128:(c + 1) * 128] * gate
        yc = jnp.concatenate([yc, yc], axis=0)
        res.append(d16[:, c * 128:(c + 1) * 128] * a16 - off16 + jnp.where(hit, yc, 0.0))
    res = jnp.concatenate(res, axis=1).astype(bf16)
    for i in range(NI):
        cp_out(i * BPI, BPI - 1).wait()
        cp_out(i * BPI + BPI - 1, 1).wait()
    out_v[rows, :] = res
    fix = pltpu.make_async_copy(out_v.at[rows], out_hbm.at[rows], sem_o.at[0])
    fix.start()
    fix.wait()


@jax.jit
def pallas_sequential_preLN__linear_kernel_hedgehog__moe_arch_mod__prompt_kernel(
    A_x: jax.Array,
    A_wqkv: jax.Array,
    A_w_phi: jax.Array,
    A_wo: jax.Array,
    B_x: jax.Array,
    B_w_r: jax.Array,
    B_w_gate: jax.Array,
    B_w_up: jax.Array,
    B_w_down: jax.Array,
):
    del B_x
    x = A_x.reshape(S, D)
    wphi = A_w_phi.reshape(H * DH, DH)
    wr = B_w_r.reshape(8, 128)
    any_spec = pl.BlockSpec(memory_space=pl.ANY)
    out = pl.pallas_call(
        _kernel,
        out_shape=jax.ShapeDtypeStruct((S, D), bf16),
        in_specs=[any_spec] * 8,
        out_specs=any_spec,
        scratch_shapes=[
            pltpu.VMEM((S, D), bf16),
            pltpu.VMEM((D // 2, 3 * D), u32),
            pltpu.VMEM((H * DH, DH), bf16),
            pltpu.VMEM((D // 2, D), u32),
            pltpu.VMEM((8, 128), bf16),
            pltpu.VMEM((D // 2, F + 128), u32),
            pltpu.VMEM((D // 2, F + 128), u32),
            pltpu.VMEM((F // 2, D + 128), u32),
            pltpu.VMEM((3 * D // 2, D), u32),
            pltpu.VMEM((64, 8 * 128), u32),
            pltpu.VMEM(((S + T) // 2, D), u32),
            pltpu.VMEM((NP, 64, 128), f32),
            pltpu.VMEM((2 * D, 128), f32),
            pltpu.VMEM((32, NP * 128), u32),
            pltpu.VMEM((D, T), u32),
            pltpu.VMEM((D // 2, T), u32),
            pltpu.VMEM((D // 2, 256), u32),
            pltpu.VMEM((D // 2, 256), u32),
            pltpu.VMEM((D // 2, 256), u32),
            pltpu.VMEM((D // 2, 256), u32),
            pltpu.VMEM((S, D), f32),
            pltpu.VMEM((S, 256), f32),
            pltpu.VMEM((B, 512), f32),
            pltpu.VMEM((S, D), bf16),
            pltpu.VMEM((8, D + 256), f32),
            pltpu.VMEM((B, 128), f32),
            pltpu.VMEM((B, 128), jnp.int32),
            pltpu.SMEM((2,), jnp.int32),
            pltpu.SemaphoreType.DMA((_NSEM_IN,)),
            pltpu.SemaphoreType.DMA((1,)),
        ],
        compiler_params=pltpu.CompilerParams(vmem_limit_bytes=110 * 1024 * 1024),
        name="hedgehog_mod",
    )(x, A_wqkv, wphi, A_wo, wr, B_w_gate, B_w_up, B_w_down)
    return out.reshape(1, S, D)
```

```python
import jax
import jax.numpy as jnp
from jax import lax
import jax.experimental.pallas as pl
import jax.experimental.pallas.tpu as pltpu

S = 2048
D = 1024
H = 32
DH = 32
F = 3584
T = 512
NT = S // T
T0 = 256
B = 128
NB = S // B
BPI = 4
NI = NB // BPI
NP = H // 2
FC = 512
R = 16
NBV = 12
NCH = 4
DCH = 1200
LOG2E = 1.4426950408889634
LN_EPS = 1e-5
DEN_EPS = 1e-6

_NT_DIMS = (((1,), (1,)), ((), ()))
_TN_DIMS = (((0,), (0,)), ((), ()))

bf16 = jnp.bfloat16
f32 = jnp.float32
u32 = jnp.uint32


def _dot_nt(a, b):
    return lax.dot_general(a, b, _NT_DIMS, preferred_element_type=f32)


def _dot_nn(a, b):
    return jnp.dot(a, b, preferred_element_type=f32)


def _pk(x):
    return pltpu.bitcast(x, u32)


def _upk(x):
    return pltpu.bitcast(x, bf16)


def _lanes(x):
    return jnp.broadcast_to(x, (x.shape[0], 128))


def _layernorm(x):
    m = jnp.mean(x, axis=-1, keepdims=True)
    xc = x - m
    v = jnp.mean(xc * xc, axis=-1, keepdims=True)
    return xc * lax.rsqrt(v + LN_EPS)


def _allreduce8(x, op):
    x = op(x, pltpu.roll(x, 4, 1))
    x = op(x, pltpu.roll(x, 2, 1))
    x = op(x, pltpu.roll(x, 1, 1))
    return x


def _hedgehog_t(p, z=None):
    t = p.shape[-1]
    p4 = p.reshape(2, 4, 8, t)
    mx = _allreduce8(jnp.max(p4, axis=1), jnp.maximum)
    mn = _allreduce8(jnp.min(p4, axis=1), jnp.minimum)
    ep = jnp.exp2(p4 - mx[:, None])
    en = jnp.exp2(mn[:, None] - p4)
    a = pl.reciprocal(_allreduce8(jnp.sum(ep, axis=1), jnp.add), approx=True)
    b = pl.reciprocal(_allreduce8(jnp.sum(en, axis=1), jnp.add), approx=True)
    if z is not None:
        dp = jnp.sum(ep * z[0:64].reshape(2, 4, 8, t), axis=1)
        dn = jnp.sum(en * z[64:128].reshape(2, 4, 8, t), axis=1)
        den = _allreduce8(dp * a + dn * b, jnp.add) + DEN_EPS
        inv = pl.reciprocal(den, approx=True)
        a = a * inv
        b = b * inv
    fp = (ep * a[:, None]).reshape(64, t)
    fn = (en * b[:, None]).reshape(64, t)
    return jnp.concatenate([fp, fn], axis=0)


def _tie(keep, w, ties):
    rows = sorted({r for r, _ in ties})
    out, pos = [], 0
    for r in rows:
        if r > pos:
            out.append(w[pos:r])
        cols = sorted(c for rr, c in ties if rr == r)
        parts, cpos = [], 0
        for c in cols:
            if c > cpos:
                parts.append(w[r:r + 8, cpos:c])
            parts.append(jnp.where(keep, w[r:r + 8, c:c + 128], ties[(r, c)]))
            cpos = c + 128
        if cpos < w.shape[1]:
            parts.append(w[r:r + 8, cpos:])
        out.append(jnp.concatenate(parts, axis=1) if len(parts) > 1 else parts[0])
        pos = r + 8
    if pos < w.shape[0]:
        out.append(w[pos:])
    return jnp.concatenate(out, axis=0)


def _vregs(x):
    if x.dtype != u32:
        x = pltpu.bitcast(x, u32)
    return [x[r:r + 8, c:c + 128] for r in range(0, x.shape[0], 8) for c in range(0, x.shape[1], 128)]


def _or_all(vals):
    acc = vals[0]
    for v in vals[1:]:
        acc = acc | v
    return acc


_WCHUNKS = ((D, 256, 2), (D + 256, 384, 3), (D + 640, 384, 4),
            (2 * D, 1024, 5),
            (0, 1024, 7))
_NSEM_IN = 10
_PHI_A = 256


def _kernel(x_hbm, wqkv_hbm, wphi_hbm, wo_hbm, wr_hbm, wg_hbm, wu_hbm, wd_hbm,
            out_hbm,
            x_v, wqkv_v, wphi_v, wo_v, wr_v, wg_v, wu_v, wd_v,
            wt_v, wop_v, wdp_v, amat_v, xn_v, kvacc_v, zacc_v, kv_v, phi_v,
            pq0_v, pq1_v, pq2_v, pq3_v, h_v, st_v, pend_v, out_v, wrb_v,
            bestv_v, besti_v, flag_s,
            sem_i, sem_o):

    def cp_x(lo, n, sem):
        return pltpu.make_async_copy(x_hbm.at[pl.ds(lo, n)], x_v.at[pl.ds(lo, n)], sem_i.at[sem])

    def cp_w(c):
        lo, w, sem = _WCHUNKS[c]
        return pltpu.make_async_copy(wqkv_hbm.at[:, pl.ds(lo, w)], wqkv_v.at[:, pl.ds(lo, w)], sem_i.at[sem])

    def cp_wd(k):
        lo, n = k * DCH, min(DCH, F - k * DCH)
        return pltpu.make_async_copy(wd_hbm.at[pl.ds(lo, n)], wd_v.at[pl.ds(lo, n)], sem_i.at[(6, 8, 9)[k]])

    cp_pa = pltpu.make_async_copy(wphi_hbm.at[pl.ds(0, _PHI_A)], wphi_v.at[pl.ds(0, _PHI_A)], sem_i.at[0])
    cp_pb = pltpu.make_async_copy(wphi_hbm.at[pl.ds(_PHI_A, D - _PHI_A)], wphi_v.at[pl.ds(_PHI_A, D - _PHI_A)],
                                  sem_i.at[3])
    cp_x0 = cp_x(0, T0, 1)
    cp_x1 = cp_x(T0, T0, 4)
    cp_x2 = cp_x(T, T, 5)
    cp_x3 = cp_x(2 * T, T, 6)
    cp_x4 = cp_x(3 * T, T, 8)
    cp_wr = pltpu.make_async_copy(wr_hbm, wr_v, sem_i.at[7])
    cp_wo = pltpu.make_async_copy(wo_hbm, wo_v, sem_i.at[7])
    cp_wg = pltpu.make_async_copy(wg_hbm, wg_v.at[:, pl.ds(0, F)], sem_i.at[7])
    cp_wu = pltpu.make_async_copy(wu_hbm, wu_v.at[:, pl.ds(0, F)], sem_i.at[7])

    def cp_out(b, n):
        lo = b * B
        if not isinstance(b, int):
            lo = pl.multiple_of(lo, B)
        return pltpu.make_async_copy(out_v.at[pl.ds(lo, n * B)], out_hbm.at[pl.ds(lo, n * B)], sem_o.at[0])

    for cp in (cp_pa, cp_x0, cp_w(0), cp_pb, cp_w(1), cp_w(2), cp_x1, cp_w(3), cp_x2,
               cp_x3, cp_wd(0), cp_x4, cp_wd(1), cp_wd(2), cp_wr, cp_w(4), cp_wo, cp_wg, cp_wu):
        cp.start()
    flag_s[0] = 1
    flag_s[1] = 0

    def ln1(src, dst, n):
        pieces = []
        for k in range(n // R):
            p = _layernorm(x_v[pl.ds(src + k * R, R), :].astype(f32))
            lo = (dst + k * R) // 2
            if not isinstance(lo, int):
                lo = pl.multiple_of(lo, R // 2)
            xn_v[pl.ds(lo, R // 2), :] = _pk(p.astype(bf16))
            pieces.append(_vregs(p))
        return pieces

    def load_xn(b):
        lo = b * (B // 2)
        if not isinstance(b, int):
            lo = pl.multiple_of(lo, B // 2)
        return _upk(xn_v[pl.ds(lo, B // 2), :])

    def k_side(p, j0, first, slot=None):
        res = []
        for j in range(j0, j0 + p.shape[0] // 64):
            ph = _hedgehog_t(p[(j - j0) * 64:(j - j0 + 1) * 64])
            if first:
                zacc_v[j * 128:(j + 1) * 128, :] = ph
            else:
                zacc_v[j * 128:(j + 1) * 128, :] += ph
            if slot is not None:
                phi_v[j * 64:(j + 1) * 64, slot * B:(slot + 1) * B] = _pk(ph.astype(bf16))
            res.append(ph)
        return res

    def proj(lo, w, xb, keep=None, early=(), late=(), deps=(), row0=0):
        lhs = wt_v[lo // 2:(lo + w) // 2, :]
        ties = {}
        for col, pieces in ((0, early), (512, late)):
            if pieces:
                step = (w // 2 - row0) // len(pieces) // 8 * 8
                for k, p in enumerate(pieces):
                    for q, val in enumerate(p):
                        ties[(row0 + k * step + (q // 4) * 8, col + (q % 4) * 128)] = val
        if deps:
            free = [(r, c) for r in range(32, w // 2, 8) for c in range(0, 512, 128)]
            for k, val in enumerate(deps):
                ties[free[k * len(free) // len(deps)]] = val
        if ties:
            lhs = _tie(keep, lhs, ties)
        return _dot_nt(_upk(lhs), xb)

    def kv_prod(vts, ph, j):
        vt = jnp.concatenate([v[j * 64:(j + 1) * 64] for v in vts], axis=1).astype(bf16)
        return _dot_nt(vt, ph)

    def v_side(xbs, keep, pieces):
        slots = 2 * len(xbs) - 2
        per = [pieces[k * len(pieces) // slots:(k + 1) * len(pieces) // slots] for k in range(slots)]
        per = [()] + per + [()]
        return [proj(2 * D, D, xb, keep, per[2 * s], per[2 * s + 1]) for s, xb in enumerate(xbs)]

    r_i = lax.broadcasted_iota(jnp.int32, (128, DH), 0)
    c_i = lax.broadcasted_iota(jnp.int32, (128, DH), 1)
    expand = (r_i % DH == c_i).astype(bf16)
    r_h = lax.broadcasted_iota(jnp.int32, (128, 128), 0) // DH
    c_h = lax.broadcasted_iota(jnp.int32, (128, 128), 1) // DH
    same_head = r_h == c_h

    def make_amat(g):
        a = _dot_nt(expand, wphi_v[g * 128:(g + 1) * 128, :])
        amat_v[:, g * 128:(g + 1) * 128] = _pk(jnp.where(same_head, a, 0.0).astype(bf16))

    def fold(c, keep=None, ties=None):
        lo, w, _ = _WCHUNKS[c]
        for n, g0 in enumerate(range(lo, lo + w, 128)):
            am = amat_v[:, g0 % D:g0 % D + 128]
            if ties is not None and ties[n]:
                am = _tie(keep, am, ties[n])
            wt = _dot_nt(_upk(am), wqkv_v[:, g0:g0 + 128]) * LOG2E
            wt_v[g0 // 2:(g0 + 128) // 2, :] = _pk(wt.astype(bf16))

    bestv_v[...] = jnp.full(bestv_v.shape, -jnp.inf, f32)
    besti_v[...] = lax.broadcasted_iota(jnp.int32, besti_v.shape, 0)
    h_v[(BPI - 1) * B:BPI * B, :] = jnp.zeros((B, D), f32)
    pend_v[...] = jnp.zeros(pend_v.shape, f32)

    cp_pa.wait()
    for g in range(_PHI_A // 128):
        make_amat(g)

    cp_x0.wait()
    ln1(0, 0, T0)
    xb = [load_xn(s) for s in range(2)]
    held = []

    def k_chunk(s, lo, w, keep=None, early=(), late=(), hold=0):
        p = proj(D + lo, w, xb[s], keep, early, late)
        n = w - hold * 64
        k_side(p[0:n], lo // 64, s == 0, s)
        if hold:
            held.append((p[n:w], (lo + n) // 64, s == 0, s))

    def flush():
        while held:
            k_side(*held.pop())

    cp_w(0).wait()
    fold(0)
    k_chunk(0, 0, 256)
    k_chunk(1, 0, 256, hold=2)

    cp_pb.wait()
    cp_w(1).wait()
    flush()
    for g in range(_PHI_A // 128, 8):
        make_amat(g)
    fold(1)
    k_chunk(0, 256, 384)
    k_chunk(1, 256, 384, hold=2)

    cp_w(2).wait()
    cp_x1.wait()
    flush()
    keep = flag_s[0] > 0
    fold(2)
    pieces = ln1(T0, T0, T0)
    k_chunk(0, 640, 384, keep, pieces[0:4], pieces[4:5])
    k_chunk(1, 640, 384, keep, pieces[5:8])
    xb += [load_xn(s) for s in range(2, 4)]
    k_chunk(2, 0, D, keep, pieces[8:16])
    k_chunk(3, 0, 768, hold=2)

    cp_w(3).wait()
    cp_x2.wait()
    flush()
    keep = flag_s[0] > 0
    k_chunk(3, 768, D - 768)
    wt_v[D:3 * D // 2, :] = _pk(wqkv_v[:, 2 * D:3 * D].T)
    vts = v_side(xb, keep, ln1(T, T, T))
    phi_m = phi_v.at[pl.ds(pl.multiple_of(flag_s[1], D), D)]
    for j in range(NP):
        kvacc_v[j] = kv_prod(vts, _upk(phi_m[j * 64:(j + 1) * 64, :]), j)
    cp_x3.wait()
    cp_wd(0).wait()

    def p1_body(i, c):
        @pl.when(i == 2)
        def _():
            cp_x4.wait()
            cp_wd(1).wait()

        @pl.when(i == 3)
        def _():
            cp_wd(2).wait()

        keep = flag_s[0] > 0
        lo = jnp.minimum((i - 1) * DCH, F - DCH)
        sv = wd_v.at[pl.ds(pl.multiple_of(lo, 16), DCH)]
        dv = wdp_v.at[pl.ds(pl.multiple_of(lo // 2, 8), DCH // 2)]
        deps = []
        for r in range(0, DCH, 16):
            val = _pk(sv[r:r + 16, :])
            dv[r // 2:r // 2 + 8, 0:D] = val
            deps.append(_or_all(_vregs(val)))
        nd = len(deps)

        xb = [load_xn(i * (T // B) + s) for s in range(T // B)]
        phik = [k_side(proj(D, D, x, keep, deps=deps[s * nd // 4:(s + 1) * nd // 4]), 0, False)
                for s, x in enumerate(xb)]
        src = pl.multiple_of(jnp.minimum(i + 1, NT - 1) * T, T)
        vts = v_side(xb, keep, ln1(src, (i + 1) * T, T))
        for j in range(NP):
            ph = jnp.concatenate([p[j] for p in phik], axis=1).astype(bf16)
            kvacc_v[j] += kv_prod(vts, ph, j)
        return c

    lax.fori_loop(1, NT, p1_body, 0)

    cp_wr.wait()
    cp_w(4).wait()
    cp_wo.wait()
    cp_wg.wait()
    cp_wu.wait()
    keep = flag_s[0] > 0
    kv_mask = (lax.broadcasted_iota(jnp.int32, (64, 128), 0) // DH
               == (lax.broadcasted_iota(jnp.int32, (64, 128), 1) // DH) % 2)
    ties = [{} for _ in range(8)]
    for j in range(NP):
        kvj = jnp.where(kv_mask, kvacc_v[j], 0.0)
        kv_v[:, j * 128:(j + 1) * 128] = _pk(kvj.astype(bf16))
        zj = _lanes(jnp.sum(zacc_v[j * 128:(j + 1) * 128, :], axis=-1, keepdims=True))
        zacc_v[j * 128:(j + 1) * 128, :] = zj
        woj = _pk(wo_v[j * 64:(j + 1) * 64, :])
        wop_v[j * 32:(j + 1) * 32, :] = woj
        if j < 14:
            dep = jnp.max(jnp.concatenate([kvj, zj], axis=0).reshape(6, 32, 128), axis=0)
            dep = _or_all([pltpu.bitcast(dep, u32)] + [woj[:, c * 128:(c + 1) * 128] for c in range(8)])
            for q, v in enumerate(_vregs(dep)):
                ties[1 + j // 2][((j % 2) * 32 + q * 8, 0)] = v
    wr = wr_v[...].astype(f32)
    wl = jnp.sum(wr, axis=0, keepdims=True)
    wsum = jnp.sum(wl, axis=1, keepdims=True)
    wrb_v[...] = jnp.concatenate(
        [jnp.broadcast_to(wr[j:j + 1, :], (8, 128)) for j in range(8)]
        + [jnp.broadcast_to(wsum, (8, 128)), jnp.broadcast_to(wl, (8, 128))], axis=1)
    fold(4, keep, ties)

    pq_v = (pq0_v, pq1_v, pq2_v, pq3_v)

    def views_of(g):
        lo = g * (BPI * B)
        if not isinstance(g, int):
            lo = pl.multiple_of(lo, BPI * B)
        return tuple(ref.at[pl.ds(lo, BPI * B)] for ref in (x_v, h_v, out_v, st_v)) + (g,)

    def stage_q(b, slot, keep=None, pieces=()):
        p = proj(0, D, load_xn(b), keep, pieces, row0=128)
        for j in range(NP):
            ph = _hedgehog_t(p[j * 64:(j + 1) * 64], zacc_v[j * 128:(j + 1) * 128, :])
            pq_v[slot][(j // 2) * 64:(j // 2 + 1) * 64, (j % 2) * B:(j % 2 + 1) * B] = _pk(ph.astype(bf16))

    def stage_g(slot):
        pq = pq_v[slot].at[pl.ds(pl.multiple_of(flag_s[1], D // 2), D // 2)]
        parts = [_dot_nn(_upk(kv_v[:, j * 128:(j + 1) * 128]),
                         _upk(pq[(j // 2) * 64:(j // 2 + 1) * 64, (j % 2) * B:(j % 2 + 1) * B]))
                 for j in range(NP)]
        return jnp.concatenate(parts, axis=0).astype(bf16)

    def stage_h(views, s, ot, keep, pieces):
        wo = wop_v[...]
        if pieces:
            ties = {}
            for k, vals in enumerate(pieces):
                q = min(int(1.6 * k) + 4, 15)
                for m, val in enumerate(vals):
                    ties[((q % 2) * 256 + m * 8, (q // 2) * 128)] = val
            wo = _tie(keep, wo, ties)
        rows = slice(s * B, (s + 1) * B)
        x_g, h_g = views[0], views[1]
        h = x_g[rows, :].astype(f32) + lax.dot_general(ot, _upk(wo), _TN_DIMS, preferred_element_type=f32)
        h_g[rows, :] = h

        def wmul(d, lo):
            return (d.reshape(B // 8, 8, 128) * wrb_v[:, lo:lo + 128][None]).reshape(B, 128)

        h0 = h[:, 0:128]
        s1 = s2 = s3 = None
        for c in range(1, D // 128):
            d = h[:, c * 128:(c + 1) * 128] - h0
            t2 = d * d
            t3 = wmul(d, c * 128)
            s1, s2, s3 = (d, t2, t3) if c == 1 else (s1 + d, s2 + t2, s3 + t3)
        c0 = _lanes(jnp.mean(h0, axis=-1, keepdims=True))
        g0 = h0 - c0
        t1 = s1 + 8.0 * g0
        t2 = s2 + g0 * (s1 + t1)
        t3 = s3 + wmul(g0, D + 128)
        return jnp.concatenate([t1, t2, t3, c0], axis=1)

    def stage_i(views, s, part, valid=None):
        _, h_g, out_g, st_g, g = views
        b = g * BPI + s
        rows = slice(s * B, (s + 1) * B)
        h = h_g[rows, :]
        bv = bestv_v[...]
        bi = besti_v[...]
        wsum = wrb_v[0:1, D:D + 128]
        pieces, outs, nvs, nis, sts = [], [], [], [], []
        for k in range(B // R):
            sl = slice(k * R, (k + 1) * R)
            red = [_lanes(jnp.sum(part[sl, n * 128:(n + 1) * 128], axis=-1, keepdims=True)) for n in range(3)]
            c0 = part[sl, 384:512]
            mu = red[0] * (1.0 / D)
            var = jnp.maximum(red[1] * (1.0 / D) - mu * mu, 0.0)
            rs = lax.rsqrt(var + LN_EPS)
            r = (red[2] - mu * wsum) * rs
            murs = (mu + c0) * rs
            a = 1.0 + rs
            o = jnp.concatenate([h[sl, c * 128:(c + 1) * 128] * a - murs for c in range(D // 128)], axis=1)
            outs.append(o.astype(bf16))
            sts.append(jnp.concatenate([rs, murs], axis=1))
            if valid is not None:
                r = jnp.where(valid, r, -jnp.inf)
            idx = lax.broadcasted_iota(jnp.int32, (R, 128), 0) + (b * B + k * R)
            better = r > bv[sl]
            nv = jnp.where(better, r, bv[sl])
            nvs.append(nv)
            nis.append(jnp.where(better, idx, bi[sl]))
            pieces.append(_vregs(o) + _vregs(nv))
        out_g[rows, :] = jnp.concatenate(outs, axis=0)
        st_g[rows, :] = jnp.concatenate(sts, axis=0)
        bestv_v[...] = jnp.concatenate(nvs, axis=0)
        besti_v[...] = jnp.concatenate(nis, axis=0)
        return pieces

    def p2_body(i, c):
        b0 = i * BPI
        keep = flag_s[0] > 0
        cur = views_of(i)
        pieces = stage_i(views_of(jnp.maximum(i - 1, 0)), BPI - 1, pend_v[...], i > 0)
        for s in range(BPI):
            stage_q(b0 + s, s, keep, pieces if s == 1 else ())
        ot = [stage_g(s) for s in range(BPI)]
        part = stage_h(cur, 0, ot[0], keep, ())
        for s in range(1, BPI):
            pieces = stage_i(cur, s - 1, part)
            part = stage_h(cur, s, ot[s], keep, pieces)
        pend_v[...] = part

        @pl.when(i > 0)
        def _():
            cp_out(jnp.maximum(b0 - 1, 0), 1).start()

        cp_out(b0, BPI - 1).start()
        return c

    lax.fori_loop(0, NI, p2_body, 0)
    stage_i(views_of(NI - 1), BPI - 1, pend_v[...])
    cp_out(NB - 1, 1).start()

    keep = flag_s[0] > 0
    bv = bestv_v[...]
    mval = jnp.max(bv, axis=0, keepdims=True)
    sel = jnp.min(jnp.where(bv == mval, besti_v[...], S - 1), axis=0, keepdims=True)
    idx = sel[0, 0]
    hrow = h_v[pl.ds(idx, 1), :]
    strow = st_v[pl.ds(idx, 1), :]
    xrow = jnp.concatenate([hrow[:, c * 128:(c + 1) * 128] * strow[:, 0:128] - strow[:, 128:256]
                            for c in range(D // 128)], axis=1).astype(bf16)
    xs = jnp.broadcast_to(xrow, (16, D))

    def act(g, u):
        a = g * pl.reciprocal(1.0 + jnp.exp(-g), approx=True) * u
        return jnp.concatenate([a, a], axis=0).astype(bf16)

    def down(a, lo, w):
        return _dot_nn(a, _upk(wdp_v[lo // 2:(lo + w) // 2, 0:D]))[0:8]

    NM = F - NBV * 128
    xcol = jnp.broadcast_to(xrow.astype(f32), (128, D)).T
    jobs = [(which, b) for b in range(NBV) for which in (0, 1)]
    vres, prev = {}, None
    for j0 in range(0, len(jobs), NCH):
        grp = jobs[j0:j0 + NCH]
        accs = [None] * len(grp)
        for r in range(D // 16):
            for n, (which, b) in enumerate(grp):
                w = (wg_v, wu_v)[which][r * 16:(r + 1) * 16, NM + b * 128:NM + (b + 1) * 128].astype(f32)
                t0 = w[0:8] * xcol[r * 16:r * 16 + 8]
                t1 = w[8:16] * xcol[r * 16 + 8:r * 16 + 16]
                if accs[n] is None:
                    if prev is not None:
                        t0 = jnp.where(keep, t0, prev[n % len(prev)])
                    accs[n] = t0 + t1
                else:
                    accs[n] = (accs[n] + t0) + t1
        prev = accs
        for n, job in enumerate(grp):
            vres[job] = _allreduce8(accs[n][None], jnp.add)[0]

    chunks = [(lo, min(FC, NM - lo)) for lo in range(0, NM, FC)]
    acts, y = [], None
    for k, (lo, w) in enumerate(chunks):
        g = _dot_nn(xs, wg_v[:, lo:lo + w])
        u = _dot_nn(xs, wu_v[:, lo:lo + w])
        acts.append(act(g[0:8], u[0:8]))
        if k >= 1:
            t = down(acts[k - 1], *chunks[k - 1])
            y = t if y is None else y + t
    y = y + down(acts[-1], *chunks[-1])
    for b0, nb in ((0, 4), (4, 4), (8, 3), (11, 1)):
        g = jnp.concatenate([vres[(0, b)] for b in range(b0, b0 + nb)], axis=1)
        u = jnp.concatenate([vres[(1, b)] for b in range(b0, b0 + nb)], axis=1)
        y = y + down(act(g, u), NM + b0 * 128, nb * 128)

    gate = jnp.broadcast_to(jax.nn.sigmoid(mval), (8, 128))
    base = pl.multiple_of((idx >> 4) << 4, 16)
    rows = pl.ds(base, 16)
    h16 = h_v[rows, :]
    st16 = st_v[rows, :]
    a16 = 1.0 + st16[:, 0:128]
    m16 = st16[:, 128:256]
    hit = (lax.broadcasted_iota(jnp.int32, (16, 128), 0) + base) == idx
    res = []
    for c in range(D // 128):
        yc = y[:, c * 128:(c + 1) * 128] * gate
        yc = jnp.concatenate([yc, yc], axis=0)
        res.append(h16[:, c * 128:(c + 1) * 128] * a16 - m16 + jnp.where(hit, yc, 0.0))
    res = jnp.concatenate(res, axis=1).astype(bf16)
    for i in range(NI):
        cp_out(i * BPI, BPI - 1).wait()
        cp_out(i * BPI + BPI - 1, 1).wait()
    out_v[rows, :] = res
    fix = pltpu.make_async_copy(out_v.at[rows], out_hbm.at[rows], sem_o.at[0])
    fix.start()
    fix.wait()


@jax.jit
def pallas_sequential_preLN__linear_kernel_hedgehog__moe_arch_mod__prompt_kernel(
    A_x: jax.Array,
    A_wqkv: jax.Array,
    A_w_phi: jax.Array,
    A_wo: jax.Array,
    B_x: jax.Array,
    B_w_r: jax.Array,
    B_w_gate: jax.Array,
    B_w_up: jax.Array,
    B_w_down: jax.Array,
):
    del B_x
    x = A_x.reshape(S, D)
    wphi = A_w_phi.reshape(H * DH, DH)
    wr = B_w_r.reshape(8, 128)
    any_spec = pl.BlockSpec(memory_space=pl.ANY)
    out = pl.pallas_call(
        _kernel,
        out_shape=jax.ShapeDtypeStruct((S, D), bf16),
        in_specs=[any_spec] * 8,
        out_specs=any_spec,
        scratch_shapes=[
            pltpu.VMEM((S, D), bf16),
            pltpu.VMEM((D, 3 * D), bf16),
            pltpu.VMEM((H * DH, DH), bf16),
            pltpu.VMEM((D, D), bf16),
            pltpu.VMEM((8, 128), bf16),
            pltpu.VMEM((D, F + 128), bf16),
            pltpu.VMEM((D, F + 128), bf16),
            pltpu.VMEM((F, D), bf16),
            pltpu.VMEM((3 * D // 2, D), u32),
            pltpu.VMEM((D // 2, D), u32),
            pltpu.VMEM((F // 2, D + 128), u32),
            pltpu.VMEM((64, 8 * 128), u32),
            pltpu.VMEM(((S + T) // 2, D), u32),
            pltpu.VMEM((NP, 64, 128), f32),
            pltpu.VMEM((2 * D, 128), f32),
            pltpu.VMEM((32, NP * 128), u32),
            pltpu.VMEM((D, T), u32),
            pltpu.VMEM((D // 2, 2 * B), u32),
            pltpu.VMEM((D // 2, 2 * B), u32),
            pltpu.VMEM((D // 2, 2 * B), u32),
            pltpu.VMEM((D // 2, 2 * B), u32),
            pltpu.VMEM((S, D), f32),
            pltpu.VMEM((S, 256), f32),
            pltpu.VMEM((B, 512), f32),
            pltpu.VMEM((S, D), bf16),
            pltpu.VMEM((8, D + 256), f32),
            pltpu.VMEM((B, 128), f32),
            pltpu.VMEM((B, 128), jnp.int32),
            pltpu.SMEM((2,), jnp.int32),
            pltpu.SemaphoreType.DMA((_NSEM_IN,)),
            pltpu.SemaphoreType.DMA((1,)),
        ],
        compiler_params=pltpu.CompilerParams(vmem_limit_bytes=110 * 1024 * 1024,
                                             disable_bounds_checks=True,
                                             disable_semaphore_checks=True),
        name="hedgehog_mod",
    )(x, A_wqkv, wphi, A_wo, wr, B_w_gate, B_w_up, B_w_down)
    return out.reshape(1, S, D)
```

```python
import jax
import jax.numpy as jnp
from jax import lax
import jax.experimental.pallas as pl
import jax.experimental.pallas.tpu as pltpu

S = 2048
D = 1024
H = 32
DH = 32
F = 3584
T = 512
NT = S // T
T0 = 256
B = 128
NB = S // B
BPI = 4
NI = NB // BPI
NP = H // 2
FC = 512
R = 16
NBV = 12
NCH = 4
DCH = 1200
LOG2E = 1.4426950408889634
LN_EPS = 1e-5
DEN_EPS = 1e-6

_NT_DIMS = (((1,), (1,)), ((), ()))
_TN_DIMS = (((0,), (0,)), ((), ()))

bf16 = jnp.bfloat16
f32 = jnp.float32
u32 = jnp.uint32


def _dot_nt(a, b):
    return lax.dot_general(a, b, _NT_DIMS, preferred_element_type=f32)


def _dot_nn(a, b):
    return jnp.dot(a, b, preferred_element_type=f32)


def _pk(x):
    return pltpu.bitcast(x, u32)


def _upk(x):
    return pltpu.bitcast(x, bf16)


def _lanes(x):
    return jnp.broadcast_to(x, (x.shape[0], 128))


def _layernorm(x):
    m = jnp.mean(x, axis=-1, keepdims=True)
    xc = x - m
    v = jnp.mean(xc * xc, axis=-1, keepdims=True)
    return xc * lax.rsqrt(v + LN_EPS)


def _allreduce8(x, op):
    x = op(x, pltpu.roll(x, 4, 1))
    x = op(x, pltpu.roll(x, 2, 1))
    x = op(x, pltpu.roll(x, 1, 1))
    return x


def _hedgehog_t(p, z=None):
    t = p.shape[-1]
    p4 = p.reshape(2, 4, 8, t)
    mx = _allreduce8(jnp.max(p4, axis=1), jnp.maximum)
    mn = _allreduce8(jnp.min(p4, axis=1), jnp.minimum)
    ep = jnp.exp2(p4 - mx[:, None])
    en = jnp.exp2(mn[:, None] - p4)
    a = pl.reciprocal(_allreduce8(jnp.sum(ep, axis=1), jnp.add), approx=True)
    b = pl.reciprocal(_allreduce8(jnp.sum(en, axis=1), jnp.add), approx=True)
    if z is not None:
        dp = jnp.sum(ep * z[0:64].reshape(2, 4, 8, t), axis=1)
        dn = jnp.sum(en * z[64:128].reshape(2, 4, 8, t), axis=1)
        den = _allreduce8(dp * a + dn * b, jnp.add) + DEN_EPS
        inv = pl.reciprocal(den, approx=True)
        a = a * inv
        b = b * inv
    fp = (ep * a[:, None]).reshape(64, t)
    fn = (en * b[:, None]).reshape(64, t)
    return jnp.concatenate([fp, fn], axis=0)


def _tie(keep, w, ties):
    rows = sorted({r for r, _ in ties})
    out, pos = [], 0
    for r in rows:
        if r > pos:
            out.append(w[pos:r])
        cols = sorted(c for rr, c in ties if rr == r)
        parts, cpos = [], 0
        for c in cols:
            if c > cpos:
                parts.append(w[r:r + 8, cpos:c])
            parts.append(jnp.where(keep, w[r:r + 8, c:c + 128], ties[(r, c)]))
            cpos = c + 128
        if cpos < w.shape[1]:
            parts.append(w[r:r + 8, cpos:])
        out.append(jnp.concatenate(parts, axis=1) if len(parts) > 1 else parts[0])
        pos = r + 8
    if pos < w.shape[0]:
        out.append(w[pos:])
    return jnp.concatenate(out, axis=0)


def _vregs(x):
    if x.dtype != u32:
        x = pltpu.bitcast(x, u32)
    return [x[r:r + 8, c:c + 128] for r in range(0, x.shape[0], 8) for c in range(0, x.shape[1], 128)]


def _or_all(vals):
    acc = vals[0]
    for v in vals[1:]:
        acc = acc | v
    return acc


_WCHUNKS = ((D, 256, 2), (D + 256, 384, 3), (D + 640, 384, 4),
            (2 * D, 1024, 5),
            (0, 1024, 7))
_NSEM_IN = 10
_PHI_A = 256


def _kernel(x_hbm, wqkv_hbm, wphi_hbm, wo_hbm, wr_hbm, wg_hbm, wu_hbm, wd_hbm,
            out_hbm,
            x_v, wqkv_v, wphi_v, wo_v, wr_v, wg_v, wu_v, wd_v,
            wt_v, wop_v, wdp_v, amat_v, xn_v, kvacc_v, zacc_v, kv_v, phi_v,
            pq0_v, pq1_v, pq2_v, pq3_v, h_v, st_v, pend_v, out_v, wrb_v,
            bestv_v, besti_v, flag_s,
            sem_i, sem_o):

    def cp_x(lo, n, sem):
        return pltpu.make_async_copy(x_hbm.at[pl.ds(lo, n)], x_v.at[pl.ds(lo, n)], sem_i.at[sem])

    def cp_w(c):
        lo, w, sem = _WCHUNKS[c]
        return pltpu.make_async_copy(wqkv_hbm.at[:, pl.ds(lo, w)], wqkv_v.at[:, pl.ds(lo, w)], sem_i.at[sem])

    def cp_wd(k):
        lo, n = k * DCH, min(DCH, F - k * DCH)
        return pltpu.make_async_copy(wd_hbm.at[pl.ds(lo, n)], wd_v.at[pl.ds(lo, n)], sem_i.at[(6, 8, 9)[k]])

    cp_pa = pltpu.make_async_copy(wphi_hbm.at[pl.ds(0, _PHI_A)], wphi_v.at[pl.ds(0, _PHI_A)], sem_i.at[0])
    cp_pb = pltpu.make_async_copy(wphi_hbm.at[pl.ds(_PHI_A, D - _PHI_A)], wphi_v.at[pl.ds(_PHI_A, D - _PHI_A)],
                                  sem_i.at[3])
    cp_x0 = cp_x(0, T0, 1)
    cp_x1 = cp_x(T0, T0, 4)
    cp_x2 = cp_x(T, T, 5)
    cp_x3 = cp_x(2 * T, T, 6)
    cp_x4 = cp_x(3 * T, T, 8)
    cp_wr = pltpu.make_async_copy(wr_hbm, wr_v, sem_i.at[7])
    cp_wo = pltpu.make_async_copy(wo_hbm, wo_v, sem_i.at[7])
    cp_wg = pltpu.make_async_copy(wg_hbm, wg_v.at[:, pl.ds(0, F)], sem_i.at[7])
    cp_wu = pltpu.make_async_copy(wu_hbm, wu_v.at[:, pl.ds(0, F)], sem_i.at[7])

    def cp_out(b, n):
        lo = b * B
        if not isinstance(b, int):
            lo = pl.multiple_of(lo, B)
        return pltpu.make_async_copy(out_v.at[pl.ds(lo, n * B)], out_hbm.at[pl.ds(lo, n * B)], sem_o.at[0])

    for cp in (cp_pa, cp_x0, cp_w(0), cp_pb, cp_w(1), cp_w(2), cp_x1, cp_w(3), cp_x2,
               cp_x3, cp_wd(0), cp_x4, cp_wd(1), cp_wd(2), cp_wr, cp_w(4), cp_wo, cp_wg, cp_wu):
        cp.start()
    flag_s[0] = 1
    flag_s[1] = 0

    def ln1(src, dst, n):
        pieces = []
        for k in range(n // R):
            p = _layernorm(x_v[pl.ds(src + k * R, R), :].astype(f32))
            lo = (dst + k * R) // 2
            if not isinstance(lo, int):
                lo = pl.multiple_of(lo, R // 2)
            xn_v[pl.ds(lo, R // 2), :] = _pk(p.astype(bf16))
            pieces.append(_vregs(p))
        return pieces

    def load_xn(b):
        lo = b * (B // 2)
        if not isinstance(b, int):
            lo = pl.multiple_of(lo, B // 2)
        return _upk(xn_v[pl.ds(lo, B // 2), :])

    def k_side(p, j0, first, slot=None):
        res = []
        for j in range(j0, j0 + p.shape[0] // 64):
            ph = _hedgehog_t(p[(j - j0) * 64:(j - j0 + 1) * 64])
            if first:
                zacc_v[j * 128:(j + 1) * 128, :] = ph
            else:
                zacc_v[j * 128:(j + 1) * 128, :] += ph
            if slot is not None:
                phi_v[j * 64:(j + 1) * 64, slot * B:(slot + 1) * B] = _pk(ph.astype(bf16))
            res.append(ph)
        return res

    def proj(lo, w, xb, keep=None, early=(), late=(), deps=(), row0=0):
        lhs = wt_v[lo // 2:(lo + w) // 2, :]
        ties = {}
        for col, pieces in ((0, early), (512, late)):
            if pieces:
                step = (w // 2 - row0) // len(pieces) // 8 * 8
                for k, p in enumerate(pieces):
                    for q, val in enumerate(p):
                        ties[(row0 + k * step + (q // 4) * 8, col + (q % 4) * 128)] = val
        if deps:
            free = [(r, c) for r in range(32, w // 2, 8) for c in range(0, 512, 128)]
            for k, val in enumerate(deps):
                ties[free[k * len(free) // len(deps)]] = val
        if ties:
            lhs = _tie(keep, lhs, ties)
        return _dot_nt(_upk(lhs), xb)

    def kv_prod(vts, ph, j):
        vt = jnp.concatenate([v[j * 64:(j + 1) * 64] for v in vts], axis=1).astype(bf16)
        return _dot_nt(vt, ph)

    def v_side(xbs, keep, pieces):
        slots = 2 * len(xbs) - 2
        per = [pieces[k * len(pieces) // slots:(k + 1) * len(pieces) // slots] for k in range(slots)]
        per = [()] + per + [()]
        return [proj(2 * D, D, xb, keep, per[2 * s], per[2 * s + 1]) for s, xb in enumerate(xbs)]

    r_i = lax.broadcasted_iota(jnp.int32, (128, DH), 0)
    c_i = lax.broadcasted_iota(jnp.int32, (128, DH), 1)
    expand = (r_i % DH == c_i).astype(bf16)
    r_h = lax.broadcasted_iota(jnp.int32, (128, 128), 0) // DH
    c_h = lax.broadcasted_iota(jnp.int32, (128, 128), 1) // DH
    same_head = r_h == c_h

    def make_amat(g):
        a = _dot_nt(expand, wphi_v[g * 128:(g + 1) * 128, :])
        amat_v[:, g * 128:(g + 1) * 128] = _pk(jnp.where(same_head, a, 0.0).astype(bf16))

    def fold(c, keep=None, ties=None):
        lo, w, _ = _WCHUNKS[c]
        for n, g0 in enumerate(range(lo, lo + w, 128)):
            am = amat_v[:, g0 % D:g0 % D + 128]
            if ties is not None and ties[n]:
                am = _tie(keep, am, ties[n])
            wt = _dot_nt(_upk(am), wqkv_v[:, g0:g0 + 128]) * LOG2E
            wt_v[g0 // 2:(g0 + 128) // 2, :] = _pk(wt.astype(bf16))

    bestv_v[...] = jnp.full(bestv_v.shape, -jnp.inf, f32)
    besti_v[...] = lax.broadcasted_iota(jnp.int32, besti_v.shape, 0)
    h_v[(BPI - 1) * B:BPI * B, :] = jnp.zeros((B, D), f32)
    pend_v[...] = jnp.zeros(pend_v.shape, f32)

    cp_pa.wait()
    for g in range(_PHI_A // 128):
        make_amat(g)

    cp_x0.wait()
    ln1(0, 0, T0)
    xb = [load_xn(s) for s in range(2)]
    held = []

    def k_chunk(s, lo, w, keep=None, early=(), late=(), hold=0):
        p = proj(D + lo, w, xb[s], keep, early, late)
        n = w - hold * 64
        k_side(p[0:n], lo // 64, s == 0, s)
        if hold:
            held.append((p[n:w], (lo + n) // 64, s == 0, s))

    def flush():
        while held:
            k_side(*held.pop())

    cp_w(0).wait()
    fold(0)
    k_chunk(0, 0, 256)
    k_chunk(1, 0, 256, hold=2)

    cp_pb.wait()
    cp_w(1).wait()
    flush()
    for g in range(_PHI_A // 128, 8):
        make_amat(g)
    fold(1)
    k_chunk(0, 256, 384)
    k_chunk(1, 256, 384, hold=2)

    cp_w(2).wait()
    cp_x1.wait()
    flush()
    keep = flag_s[0] > 0
    fold(2)
    pieces = ln1(T0, T0, T0)
    k_chunk(0, 640, 384, keep, pieces[0:4], pieces[4:5])
    k_chunk(1, 640, 384, keep, pieces[5:8])
    xb += [load_xn(s) for s in range(2, 4)]
    k_chunk(2, 0, D, keep, pieces[8:16])
    k_chunk(3, 0, 768, hold=2)

    cp_w(3).wait()
    cp_x2.wait()
    flush()
    keep = flag_s[0] > 0
    k_chunk(3, 768, D - 768)
    wt_v[D:3 * D // 2, :] = _pk(wqkv_v[:, 2 * D:3 * D].T)
    vts = v_side(xb, keep, ln1(T, T, T))
    phi_m = phi_v.at[pl.ds(pl.multiple_of(flag_s[1], D), D)]
    for j in range(NP):
        kvacc_v[j] = kv_prod(vts, _upk(phi_m[j * 64:(j + 1) * 64, :]), j)
    cp_x3.wait()
    cp_wd(0).wait()

    def p1_body(i, c):
        @pl.when(i == 2)
        def _():
            cp_x4.wait()
            cp_wd(1).wait()

        @pl.when(i == 3)
        def _():
            cp_wd(2).wait()

        keep = flag_s[0] > 0
        lo = jnp.minimum((i - 1) * DCH, F - DCH)
        sv = wd_v.at[pl.ds(pl.multiple_of(lo, 16), DCH)]
        dv = wdp_v.at[pl.ds(pl.multiple_of(lo // 2, 8), DCH // 2)]
        deps = []
        for r in range(0, DCH, 16):
            val = _pk(sv[r:r + 16, :])
            dv[r // 2:r // 2 + 8, 0:D] = val
            deps.append(_or_all(_vregs(val)))
        nd = len(deps)

        xb = [load_xn(i * (T // B) + s) for s in range(T // B)]
        phik = [k_side(proj(D, D, x, keep, deps=deps[s * nd // 4:(s + 1) * nd // 4]), 0, False)
                for s, x in enumerate(xb)]
        src = pl.multiple_of(jnp.minimum(i + 1, NT - 1) * T, T)
        vts = v_side(xb, keep, ln1(src, (i + 1) * T, T))
        for j in range(NP):
            ph = jnp.concatenate([p[j] for p in phik], axis=1).astype(bf16)
            kvacc_v[j] += kv_prod(vts, ph, j)
        return c

    lax.fori_loop(1, NT, p1_body, 0)

    cp_wr.wait()
    cp_w(4).wait()
    cp_wo.wait()
    cp_wg.wait()
    cp_wu.wait()
    keep = flag_s[0] > 0
    kv_mask = (lax.broadcasted_iota(jnp.int32, (64, 128), 0) // DH
               == (lax.broadcasted_iota(jnp.int32, (64, 128), 1) // DH) % 2)
    ties = [{} for _ in range(8)]
    for j in range(NP):
        kvj = jnp.where(kv_mask, kvacc_v[j], 0.0)
        kv_v[:, j * 128:(j + 1) * 128] = _pk(kvj.astype(bf16))
        zj = _lanes(jnp.sum(zacc_v[j * 128:(j + 1) * 128, :], axis=-1, keepdims=True))
        zacc_v[j * 128:(j + 1) * 128, :] = zj
        woj = _pk(wo_v[j * 64:(j + 1) * 64, :])
        wop_v[j * 32:(j + 1) * 32, :] = woj
        if j < 14:
            dep = jnp.max(jnp.concatenate([kvj, zj], axis=0).reshape(6, 32, 128), axis=0)
            dep = _or_all([pltpu.bitcast(dep, u32)] + [woj[:, c * 128:(c + 1) * 128] for c in range(8)])
            for q, v in enumerate(_vregs(dep)):
                ties[1 + j // 2][((j % 2) * 32 + q * 8, 0)] = v
    wr = wr_v[...].astype(f32)
    wl = jnp.sum(wr, axis=0, keepdims=True)
    wsum = jnp.sum(wl, axis=1, keepdims=True)
    wrb_v[...] = jnp.concatenate(
        [jnp.broadcast_to(wr[j:j + 1, :], (8, 128)) for j in range(8)]
        + [jnp.broadcast_to(wsum, (8, 128)), jnp.broadcast_to(wl, (8, 128))], axis=1)
    fold(4, keep, ties)

    pq_v = (pq0_v, pq1_v, pq2_v, pq3_v)

    def views_of(g):
        lo = g * (BPI * B)
        if not isinstance(g, int):
            lo = pl.multiple_of(lo, BPI * B)
        return tuple(ref.at[pl.ds(lo, BPI * B)] for ref in (x_v, h_v, out_v, st_v)) + (g,)

    def stage_q(b, slot, keep=None, pieces=()):
        p = proj(0, D, load_xn(b), keep, pieces, row0=128)
        for j in range(NP):
            ph = _hedgehog_t(p[j * 64:(j + 1) * 64], zacc_v[j * 128:(j + 1) * 128, :])
            pq_v[slot][(j // 2) * 64:(j // 2 + 1) * 64, (j % 2) * B:(j % 2 + 1) * B] = _pk(ph.astype(bf16))

    def stage_g(slot):
        pq = pq_v[slot].at[pl.ds(pl.multiple_of(flag_s[1], D // 2), D // 2)]
        parts = [_dot_nn(_upk(kv_v[:, j * 128:(j + 1) * 128]),
                         _upk(pq[(j // 2) * 64:(j // 2 + 1) * 64, (j % 2) * B:(j % 2 + 1) * B]))
                 for j in range(NP)]
        return jnp.concatenate(parts, axis=0).astype(bf16)

    def stage_h(views, s, ot, keep, pieces):
        wo = wop_v[...]
        if pieces:
            ties = {}
            for k, vals in enumerate(pieces):
                q = min(int(1.72 * k) + 3, 15)
                for m, val in enumerate(vals):
                    ties[((q % 2) * 256 + m * 8, (q // 2) * 128)] = val
            wo = _tie(keep, wo, ties)
        rows = slice(s * B, (s + 1) * B)
        x_g, h_g = views[0], views[1]
        h = x_g[rows, :].astype(f32) + lax.dot_general(ot, _upk(wo), _TN_DIMS, preferred_element_type=f32)
        h_g[rows, :] = h

        def wmul(d, lo):
            return (d.reshape(B // 8, 8, 128) * wrb_v[:, lo:lo + 128][None]).reshape(B, 128)

        h0 = h[:, 0:128]
        s1 = s2 = s3 = None
        for c in range(1, D // 128):
            d = h[:, c * 128:(c + 1) * 128] - h0
            t2 = d * d
            t3 = wmul(d, c * 128)
            s1, s2, s3 = (d, t2, t3) if c == 1 else (s1 + d, s2 + t2, s3 + t3)
        c0 = _lanes(jnp.mean(h0, axis=-1, keepdims=True))
        g0 = h0 - c0
        t1 = s1 + 8.0 * g0
        t2 = s2 + g0 * (s1 + t1)
        t3 = s3 + wmul(g0, D + 128)
        return jnp.concatenate([t1, t2, t3, c0], axis=1), h

    def stage_i(views, s, part, h=None, valid=None):
        _, h_g, out_g, st_g, g = views
        b = g * BPI + s
        rows = slice(s * B, (s + 1) * B)
        if h is None:
            h = h_g[rows, :]
        bv = bestv_v[...]
        bi = besti_v[...]
        wsum = wrb_v[0:1, D:D + 128]
        pieces, outs, nvs, nis, sts = [], [], [], [], []
        for k in range(B // R):
            sl = slice(k * R, (k + 1) * R)
            red = [_lanes(jnp.sum(part[sl, n * 128:(n + 1) * 128], axis=-1, keepdims=True)) for n in range(3)]
            c0 = part[sl, 384:512]
            mu = red[0] * (1.0 / D)
            var = jnp.maximum(red[1] * (1.0 / D) - mu * mu, 0.0)
            rs = lax.rsqrt(var + LN_EPS)
            r = (red[2] - mu * wsum) * rs
            murs = (mu + c0) * rs
            a = 1.0 + rs
            o = jnp.concatenate([h[sl, c * 128:(c + 1) * 128] * a - murs for c in range(D // 128)], axis=1)
            outs.append(o.astype(bf16))
            sts.append(jnp.concatenate([rs, murs], axis=1))
            if valid is not None:
                r = jnp.where(valid, r, -jnp.inf)
            idx = lax.broadcasted_iota(jnp.int32, (R, 128), 0) + (b * B + k * R)
            better = r > bv[sl]
            nv = jnp.where(better, r, bv[sl])
            nvs.append(nv)
            nis.append(jnp.where(better, idx, bi[sl]))
            pieces.append(_vregs(o) + _vregs(nv))
        out_g[rows, :] = jnp.concatenate(outs, axis=0)
        st_g[rows, :] = jnp.concatenate(sts, axis=0)
        bestv_v[...] = jnp.concatenate(nvs, axis=0)
        besti_v[...] = jnp.concatenate(nis, axis=0)
        return pieces

    def p2_body(i, c):
        b0 = i * BPI
        keep = flag_s[0] > 0
        cur = views_of(i)
        pieces = stage_i(views_of(jnp.maximum(i - 1, 0)), BPI - 1, pend_v[...], valid=i > 0)
        for s in range(BPI):
            stage_q(b0 + s, s, keep, pieces if s == 0 else ())
        ot = [stage_g(s) for s in range(BPI)]
        part, h = stage_h(cur, 0, ot[0], keep, ())
        for s in range(1, BPI):
            pieces = stage_i(cur, s - 1, part, h)
            part, h = stage_h(cur, s, ot[s], keep, pieces)
        pend_v[...] = part

        @pl.when(i > 0)
        def _():
            cp_out(jnp.maximum(b0 - 1, 0), 1).start()

        cp_out(b0, BPI - 1).start()
        return c

    lax.fori_loop(0, NI, p2_body, 0)
    stage_i(views_of(NI - 1), BPI - 1, pend_v[...])
    cp_out(NB - 1, 1).start()

    keep = flag_s[0] > 0
    bv = bestv_v[...]
    mval = jnp.max(bv, axis=0, keepdims=True)
    sel = jnp.min(jnp.where(bv == mval, besti_v[...], S - 1), axis=0, keepdims=True)
    idx = sel[0, 0]
    hrow = h_v[pl.ds(idx, 1), :]
    strow = st_v[pl.ds(idx, 1), :]
    xrow = jnp.concatenate([hrow[:, c * 128:(c + 1) * 128] * strow[:, 0:128] - strow[:, 128:256]
                            for c in range(D // 128)], axis=1).astype(bf16)
    xs = jnp.broadcast_to(xrow, (16, D))

    def act(g, u):
        a = g * pl.reciprocal(1.0 + jnp.exp(-g), approx=True) * u
        return jnp.concatenate([a, a], axis=0).astype(bf16)

    def down(a, lo, w):
        return _dot_nn(a, _upk(wdp_v[lo // 2:(lo + w) // 2, 0:D]))[0:8]

    NM = F - NBV * 128
    xcol = jnp.broadcast_to(xrow.astype(f32), (128, D)).T
    jobs = [(which, b) for b in range(NBV) for which in (0, 1)]
    vres, prev = {}, None
    for j0 in range(0, len(jobs), NCH):
        grp = jobs[j0:j0 + NCH]
        accs = [None] * len(grp)
        for r in range(D // 16):
            for n, (which, b) in enumerate(grp):
                w = (wg_v, wu_v)[which][r * 16:(r + 1) * 16, NM + b * 128:NM + (b + 1) * 128].astype(f32)
                t0 = w[0:8] * xcol[r * 16:r * 16 + 8]
                t1 = w[8:16] * xcol[r * 16 + 8:r * 16 + 16]
                if accs[n] is None:
                    if prev is not None:
                        t0 = jnp.where(keep, t0, prev[n % len(prev)])
                    accs[n] = t0 + t1
                else:
                    accs[n] = (accs[n] + t0) + t1
        prev = accs
        for n, job in enumerate(grp):
            vres[job] = _allreduce8(accs[n][None], jnp.add)[0]

    chunks = [(lo, min(FC, NM - lo)) for lo in range(0, NM, FC)]
    acts, y = [], None
    for k, (lo, w) in enumerate(chunks):
        g = _dot_nn(xs, wg_v[:, lo:lo + w])
        u = _dot_nn(xs, wu_v[:, lo:lo + w])
        acts.append(act(g[0:8], u[0:8]))
        if k >= 1:
            t = down(acts[k - 1], *chunks[k - 1])
            y = t if y is None else y + t
    y = y + down(acts[-1], *chunks[-1])
    for b0, nb in ((0, 4), (4, 4), (8, 3), (11, 1)):
        g = jnp.concatenate([vres[(0, b)] for b in range(b0, b0 + nb)], axis=1)
        u = jnp.concatenate([vres[(1, b)] for b in range(b0, b0 + nb)], axis=1)
        y = y + down(act(g, u), NM + b0 * 128, nb * 128)

    gate = jnp.broadcast_to(jax.nn.sigmoid(mval), (8, 128))
    base = pl.multiple_of((idx >> 4) << 4, 16)
    rows = pl.ds(base, 16)
    h16 = h_v[rows, :]
    st16 = st_v[rows, :]
    a16 = 1.0 + st16[:, 0:128]
    m16 = st16[:, 128:256]
    hit = (lax.broadcasted_iota(jnp.int32, (16, 128), 0) + base) == idx
    res = []
    for c in range(D // 128):
        yc = y[:, c * 128:(c + 1) * 128] * gate
        yc = jnp.concatenate([yc, yc], axis=0)
        res.append(h16[:, c * 128:(c + 1) * 128] * a16 - m16 + jnp.where(hit, yc, 0.0))
    res = jnp.concatenate(res, axis=1).astype(bf16)
    for i in range(NI):
        cp_out(i * BPI, BPI - 1).wait()
        cp_out(i * BPI + BPI - 1, 1).wait()
    out_v[rows, :] = res
    fix = pltpu.make_async_copy(out_v.at[rows], out_hbm.at[rows], sem_o.at[0])
    fix.start()
    fix.wait()


@jax.jit
def pallas_sequential_preLN__linear_kernel_hedgehog__moe_arch_mod__prompt_kernel(
    A_x: jax.Array,
    A_wqkv: jax.Array,
    A_w_phi: jax.Array,
    A_wo: jax.Array,
    B_x: jax.Array,
    B_w_r: jax.Array,
    B_w_gate: jax.Array,
    B_w_up: jax.Array,
    B_w_down: jax.Array,
):
    del B_x
    x = A_x.reshape(S, D)
    wphi = A_w_phi.reshape(H * DH, DH)
    wr = B_w_r.reshape(8, 128)
    any_spec = pl.BlockSpec(memory_space=pl.ANY)
    out = pl.pallas_call(
        _kernel,
        out_shape=jax.ShapeDtypeStruct((S, D), bf16),
        in_specs=[any_spec] * 8,
        out_specs=any_spec,
        scratch_shapes=[
            pltpu.VMEM((S, D), bf16),
            pltpu.VMEM((D, 3 * D), bf16),
            pltpu.VMEM((H * DH, DH), bf16),
            pltpu.VMEM((D, D), bf16),
            pltpu.VMEM((8, 128), bf16),
            pltpu.VMEM((D, F + 128), bf16),
            pltpu.VMEM((D, F + 128), bf16),
            pltpu.VMEM((F, D), bf16),
            pltpu.VMEM((3 * D // 2, D), u32),
            pltpu.VMEM((D // 2, D), u32),
            pltpu.VMEM((F // 2, D + 128), u32),
            pltpu.VMEM((64, 8 * 128), u32),
            pltpu.VMEM(((S + T) // 2, D), u32),
            pltpu.VMEM((NP, 64, 128), f32),
            pltpu.VMEM((2 * D, 128), f32),
            pltpu.VMEM((32, NP * 128), u32),
            pltpu.VMEM((D, T), u32),
            pltpu.VMEM((D // 2, 2 * B), u32),
            pltpu.VMEM((D // 2, 2 * B), u32),
            pltpu.VMEM((D // 2, 2 * B), u32),
            pltpu.VMEM((D // 2, 2 * B), u32),
            pltpu.VMEM((S, D), f32),
            pltpu.VMEM((S, 256), f32),
            pltpu.VMEM((B, 512), f32),
            pltpu.VMEM((S, D), bf16),
            pltpu.VMEM((8, D + 256), f32),
            pltpu.VMEM((B, 128), f32),
            pltpu.VMEM((B, 128), jnp.int32),
            pltpu.SMEM((2,), jnp.int32),
            pltpu.SemaphoreType.DMA((_NSEM_IN,)),
            pltpu.SemaphoreType.DMA((1,)),
        ],
        compiler_params=pltpu.CompilerParams(vmem_limit_bytes=110 * 1024 * 1024,
                                             disable_bounds_checks=True,
                                             disable_semaphore_checks=True),
        name="hedgehog_mod",
    )(x, A_wqkv, wphi, A_wo, wr, B_w_gate, B_w_up, B_w_down)
    return out.reshape(1, S, D)
```

```python
import os
import jax
import jax.numpy as jnp
from jax import lax
import jax.experimental.pallas as pl
import jax.experimental.pallas.tpu as pltpu

S = 2048
D = 1024
H = 32
DH = 32
F = 3584
T = 512
NT = S // T
T0 = 256
B = 128
NB = S // B
BPI = 4
NI = NB // BPI
NP = H // 2
FC = 512
R = 16
NBV = 12
NCH = 4
DCH = 1200
NV = 124
PR = NV * 4
Q0, K0, V0 = 0, PR, 2 * PR
LOG2E = 1.4426950408889634
LN_EPS = 1e-5
DEN_EPS = 1e-6

_NT_DIMS = (((1,), (1,)), ((), ()))
_TN_DIMS = (((0,), (0,)), ((), ()))

bf16 = jnp.bfloat16
f32 = jnp.float32
u32 = jnp.uint32


def _opt(name, default):
    return type(default)(os.environ.get(name, default))


def _dot_nt(a, b):
    return lax.dot_general(a, b, _NT_DIMS, preferred_element_type=f32)


def _dot_nn(a, b):
    return jnp.dot(a, b, preferred_element_type=f32)


def _pk(x):
    return pltpu.bitcast(x, u32)


def _upk(x):
    return pltpu.bitcast(x, bf16)


def _lanes(x):
    return jnp.broadcast_to(x, (x.shape[0], 128))


def _layernorm(x):
    m = jnp.mean(x, axis=-1, keepdims=True)
    xc = x - m
    v = jnp.mean(xc * xc, axis=-1, keepdims=True)
    return xc * lax.rsqrt(v + LN_EPS)


def _allreduce8(x, op):
    x = op(x, pltpu.roll(x, 4, 1))
    x = op(x, pltpu.roll(x, 2, 1))
    x = op(x, pltpu.roll(x, 1, 1))
    return x


def _hedgehog_t(p, z=None):
    t = p.shape[-1]
    p4 = p.reshape(2, 4, 8, t)
    mx = _allreduce8(jnp.max(p4, axis=1), jnp.maximum)
    mn = _allreduce8(jnp.min(p4, axis=1), jnp.minimum)
    ep = jnp.exp2(p4 - mx[:, None])
    en = jnp.exp2(mn[:, None] - p4)
    a = pl.reciprocal(_allreduce8(jnp.sum(ep, axis=1), jnp.add), approx=True)
    b = pl.reciprocal(_allreduce8(jnp.sum(en, axis=1), jnp.add), approx=True)
    if z is not None:
        dp = jnp.sum(ep * z[0:64].reshape(2, 4, 8, t), axis=1)
        dn = jnp.sum(en * z[64:128].reshape(2, 4, 8, t), axis=1)
        den = _allreduce8(dp * a + dn * b, jnp.add) + DEN_EPS
        inv = pl.reciprocal(den, approx=True)
        a = a * inv
        b = b * inv
    fp = (ep * a[:, None]).reshape(64, t)
    fn = (en * b[:, None]).reshape(64, t)
    return jnp.concatenate([fp, fn], axis=0)


def _head_groups(h):
    base, k = (NV // 4) * (h // 8), h % 8
    return ([base + 4 * k + i for i in range(3)],
            base + 4 * k - 1 if k > 0 else None,
            base + 4 * k + 3 if k < 7 else None,
            8 - k)


def _pair_logits(group, j):
    parts = []
    for h in (2 * j, 2 * j + 1):
        full, below, above, a = _head_groups(h)
        ref = group(full[0])
        sub = lax.broadcasted_iota(jnp.int32, ref.shape, 0)
        if above is None:
            m = jnp.where(sub >= a, group(below), 0.0)
        else:
            m = jnp.where(sub == a - 1, 0.0, group(above))
            if below is not None:
                m = jnp.where(sub >= a, group(below), m)
        parts += [m] + [group(q) for q in full]
    return jnp.concatenate(parts, axis=0)


def _pair_need(j):
    full, _, above, _ = _head_groups(2 * j + 1)
    return full[2] if above is None else above


def _tie(keep, w, ties):
    rows = sorted({r for r, _ in ties})
    out, pos = [], 0
    for r in rows:
        if r > pos:
            out.append(w[pos:r])
        cols = sorted(c for rr, c in ties if rr == r)
        parts, cpos = [], 0
        for c in cols:
            if c > cpos:
                parts.append(w[r:r + 8, cpos:c])
            parts.append(jnp.where(keep, w[r:r + 8, c:c + 128], ties[(r, c)]))
            cpos = c + 128
        if cpos < w.shape[1]:
            parts.append(w[r:r + 8, cpos:])
        out.append(jnp.concatenate(parts, axis=1) if len(parts) > 1 else parts[0])
        pos = r + 8
    if pos < w.shape[0]:
        out.append(w[pos:])
    return jnp.concatenate(out, axis=0)


def _vregs(x):
    if x.dtype != u32:
        x = pltpu.bitcast(x, u32)
    return [x[r:r + 8, c:c + 128] for r in range(0, x.shape[0], 8) for c in range(0, x.shape[1], 128)]


def _or_all(vals):
    acc = vals[0]
    for v in vals[1:]:
        acc = acc | v
    return acc


_WCHUNKS = ((D, 256, 2), (D + 256, 384, 3), (D + 640, 384, 4),
            (2 * D, 1024, 5),
            (0, 1024, 7))
_NSEM_IN = 10
_PHI_A = 256


def _kernel(x_hbm, wqkv_hbm, wphi_hbm, wo_hbm, wr_hbm, wg_hbm, wu_hbm, wd_hbm,
            out_hbm,
            x_v, wqkv_v, wphi_v, wo_v, wr_v, wg_v, wu_v, wd_v,
            wt_v, wop_v, wdp_v, amat_v, xn_v, kvacc_v, zacc_v, kv_v, phi_v,
            pq0_v, pq1_v, pq2_v, pq3_v, h_v, st_v, pend_v, out_v, wrb_v,
            bestv_v, besti_v, flag_s,
            sem_i, sem_o):

    def cp_x(lo, n, sem):
        return pltpu.make_async_copy(x_hbm.at[pl.ds(lo, n)], x_v.at[pl.ds(lo, n)], sem_i.at[sem])

    def cp_w(c):
        lo, w, sem = _WCHUNKS[c]
        return pltpu.make_async_copy(wqkv_hbm.at[:, pl.ds(lo, w)], wqkv_v.at[:, pl.ds(lo, w)], sem_i.at[sem])

    def cp_wd(k):
        lo, n = k * DCH, min(DCH, F - k * DCH)
        return pltpu.make_async_copy(wd_hbm.at[pl.ds(lo, n)], wd_v.at[pl.ds(lo, n)], sem_i.at[(6, 8, 9)[k]])

    cp_pa = pltpu.make_async_copy(wphi_hbm.at[pl.ds(0, _PHI_A)], wphi_v.at[pl.ds(0, _PHI_A)], sem_i.at[0])
    cp_pb = pltpu.make_async_copy(wphi_hbm.at[pl.ds(_PHI_A, D - _PHI_A)], wphi_v.at[pl.ds(_PHI_A, D - _PHI_A)],
                                  sem_i.at[3])
    cp_x0 = cp_x(0, T0, 1)
    cp_x1 = cp_x(T0, T0, 4)
    cp_x2 = cp_x(T, T, 5)
    cp_x3 = cp_x(2 * T, T, 6)
    cp_x4 = cp_x(3 * T, T, 8)
    cp_wr = pltpu.make_async_copy(wr_hbm, wr_v, sem_i.at[7])
    cp_wo = pltpu.make_async_copy(wo_hbm, wo_v, sem_i.at[7])
    cp_wg = pltpu.make_async_copy(wg_hbm, wg_v.at[:, pl.ds(0, F)], sem_i.at[7])
    cp_wu = pltpu.make_async_copy(wu_hbm, wu_v.at[:, pl.ds(0, F)], sem_i.at[7])

    def cp_out(b, n):
        lo = b * B
        if not isinstance(b, int):
            lo = pl.multiple_of(lo, B)
        return pltpu.make_async_copy(out_v.at[pl.ds(lo, n * B)], out_hbm.at[pl.ds(lo, n * B)], sem_o.at[0])

    for cp in (cp_pa, cp_x0, cp_w(0), cp_pb, cp_w(1), cp_w(2), cp_x1, cp_w(3), cp_x2,
               cp_x3, cp_wd(0), cp_x4, cp_wd(1), cp_wd(2), cp_wr, cp_w(4), cp_wo, cp_wg, cp_wu):
        cp.start()
    flag_s[0] = 1
    flag_s[1] = 0

    def ln1(src, dst, n):
        pieces = []
        for k in range(n // R):
            p = _layernorm(x_v[pl.ds(src + k * R, R), :].astype(f32))
            lo = (dst + k * R) // 2
            if not isinstance(lo, int):
                lo = pl.multiple_of(lo, R // 2)
            xn_v[pl.ds(lo, R // 2), :] = _pk(p.astype(bf16))
            pieces.append(_vregs(p))
        return pieces

    def load_xn(b):
        lo = b * (B // 2)
        if not isinstance(b, int):
            lo = pl.multiple_of(lo, B // 2)
        return _upk(xn_v[pl.ds(lo, B // 2), :])

    def k_side(group, pairs, first, slot=None):
        res = []
        for j in pairs:
            ph = _hedgehog_t(_pair_logits(group, j))
            if first:
                zacc_v[j * 128:(j + 1) * 128, :] = ph
            else:
                zacc_v[j * 128:(j + 1) * 128, :] += ph
            if slot is not None:
                phi_v[j * 64:(j + 1) * 64, slot * B:(slot + 1) * B] = _pk(ph.astype(bf16))
            res.append(ph)
        return res

    def proj(lo, n, xb, keep=None, early=(), late=(), deps=(), row0=0):
        lhs = wt_v[lo:lo + n, :]
        ties = {}
        for col, pieces in ((0, early), (512, late)):
            if pieces:
                step = (n - row0) // len(pieces) // 8 * 8
                for k, p in enumerate(pieces):
                    for q, val in enumerate(p):
                        ties[(row0 + k * step + (q // 4) * 8, col + (q % 4) * 128)] = val
        if deps:
            free = [(r, c) for r in range(32, n, 8) for c in range(0, 512, 128)]
            for k, val in enumerate(deps):
                ties[free[k * len(free) // len(deps)]] = val
        if ties:
            lhs = _tie(keep, lhs, ties)
        return _dot_nt(_upk(lhs), xb)

    def groups_of(p):
        return lambda pos: p[pos * 8:(pos + 1) * 8]

    def kv_prod(vts, ph, j):
        vt = jnp.concatenate([v[j * 64:(j + 1) * 64] for v in vts], axis=1).astype(bf16)
        return _dot_nt(vt, ph)

    def v_side(xbs, keep, pieces):
        slots = 2 * len(xbs) - 2
        per = [pieces[k * len(pieces) // slots:(k + 1) * len(pieces) // slots] for k in range(slots)]
        per = [()] + per + [()]
        return [proj(V0, D // 2, xb, keep, per[2 * s], per[2 * s + 1]) for s, xb in enumerate(xbs)]

    r_i = lax.broadcasted_iota(jnp.int32, (128, DH), 0)
    c_i = lax.broadcasted_iota(jnp.int32, (128, DH), 1)
    expand = (r_i % DH == c_i).astype(bf16)
    r_h = lax.broadcasted_iota(jnp.int32, (128, 128), 0) // DH
    c_h = lax.broadcasted_iota(jnp.int32, (128, 128), 1) // DH
    same_head = r_h == c_h

    def make_amat(g):
        a = _dot_nt(expand, wphi_v[g * 128:(g + 1) * 128, :])
        amat_v[:, g * 128:(g + 1) * 128] = _pk(jnp.where(same_head, a, 0.0).astype(bf16))

    class Folder:
        def __init__(self, dst):
            self.dst, self.rows, self.mprev, self.done = dst, {}, None, 0

        def fold(self, c, keep=None, ties=None):
            lo, w, _ = _WCHUNKS[c]
            sub = lax.broadcasted_iota(jnp.int32, (8, D), 0)
            for n, g0 in enumerate(range(lo, lo + w, 128)):
                g = (g0 % D) // 128
                am = amat_v[:, g * 128:(g + 1) * 128]
                if ties is not None and ties[n]:
                    am = _tie(keep, am, ties[n])
                wt = _dot_nt(_upk(am), wqkv_v[:, g0:g0 + 128])
                for hh in range(4):
                    full, below, _, a = _head_groups(4 * g + hh)
                    r0 = hh * DH
                    ref = jnp.broadcast_to(wt[r0 + a - 1:r0 + a, :], (8, D))
                    part = [(wt[r0 + 8 * i:r0 + 8 * (i + 1)] - ref) * LOG2E for i in range(4)]
                    if below is not None:
                        self.rows[below] = jnp.where(sub >= a, part[0], self.mprev)
                    self.mprev = part[0]
                    for q, v in zip(full, part[1:]):
                        self.rows[q] = v
                while self.done in self.rows and self.done + 1 in self.rows:
                    pair = jnp.concatenate([self.rows.pop(self.done), self.rows.pop(self.done + 1)], axis=0)
                    r = self.dst + self.done * 4
                    wt_v[r:r + 8, :] = _pk(pair.astype(bf16))
                    self.done += 2
            return self.done

    bestv_v[...] = jnp.full(bestv_v.shape, -jnp.inf, f32)
    besti_v[...] = lax.broadcasted_iota(jnp.int32, besti_v.shape, 0)
    h_v[(BPI - 1) * B:BPI * B, :] = jnp.zeros((B, D), f32)
    pend_v[...] = jnp.zeros(pend_v.shape, f32)

    cp_pa.wait()
    for g in range(_PHI_A // 128):
        make_amat(g)

    cp_x0.wait()
    ln1(0, 0, T0)
    xb = [load_xn(s) for s in range(2)]
    logits = [{} for _ in range(4)]
    npairs = [0] * 4

    def k_finish(s, hold=0):
        ready = [j for j in range(npairs[s], NP) if _pair_need(j) < len(logits[s])]
        ready = ready[:len(ready) - hold]
        k_side(logits[s].__getitem__, ready, s == 0, s)
        npairs[s] += len(ready)

    def k_chunk(s, hi, keep=None, early=(), late=(), hold=0):
        lo = len(logits[s])
        p = proj(K0 + lo * 4, (hi - lo) * 4, xb[s], keep, early, late)
        for q in range(lo, hi):
            logits[s][q] = p[(q - lo) * 8:(q - lo + 1) * 8]
        k_finish(s, hold)

    fk = Folder(K0)
    HOLD = _opt('HOLD', 1)
    cp_w(0).wait()
    n = fk.fold(0)
    k_chunk(0, n)
    k_chunk(1, n, hold=HOLD)

    cp_pb.wait()
    cp_w(1).wait()
    k_finish(1)
    for g in range(_PHI_A // 128, 8):
        make_amat(g)
    n = fk.fold(1)
    k_chunk(0, n)
    k_chunk(1, n, hold=HOLD)

    cp_w(2).wait()
    cp_x1.wait()
    k_finish(1)
    keep = flag_s[0] > 0
    n = fk.fold(2)
    pieces = ln1(T0, T0, T0)
    k_chunk(0, n, keep, pieces[0:4], pieces[4:5])
    k_chunk(1, n, keep, pieces[5:8])
    xb += [load_xn(s) for s in range(2, 4)]
    k_chunk(2, NV, keep, pieces[8:16])
    k_chunk(3, _opt('KS', 96), hold=2)

    cp_w(3).wait()
    cp_x2.wait()
    k_finish(3)
    keep = flag_s[0] > 0
    k_chunk(3, NV)
    wt_v[V0:V0 + D // 2, :] = _pk(wqkv_v[:, 2 * D:3 * D].T)
    vts = v_side(xb, keep, ln1(T, T, T))
    phi_m = phi_v.at[pl.ds(pl.multiple_of(flag_s[1], D), D)]
    for j in range(NP):
        kvacc_v[j] = kv_prod(vts, _upk(phi_m[j * 64:(j + 1) * 64, :]), j)
    cp_x3.wait()
    cp_wd(0).wait()

    def p1_body(i, c):
        @pl.when(i == 2)
        def _():
            cp_x4.wait()
            cp_wd(1).wait()

        @pl.when(i == 3)
        def _():
            cp_wd(2).wait()

        keep = flag_s[0] > 0
        lo = jnp.minimum((i - 1) * DCH, F - DCH)
        sv = wd_v.at[pl.ds(pl.multiple_of(lo, 16), DCH)]
        dv = wdp_v.at[pl.ds(pl.multiple_of(lo // 2, 8), DCH // 2)]
        deps = []
        for r in range(0, DCH, 16):
            val = _pk(sv[r:r + 16, :])
            dv[r // 2:r // 2 + 8, 0:D] = val
            deps.append(_or_all(_vregs(val)))
        nd = len(deps)

        xb = [load_xn(i * (T // B) + s) for s in range(T // B)]
        phik = [k_side(groups_of(proj(K0, PR, x, keep, deps=deps[s * nd // 4:(s + 1) * nd // 4])), range(NP), False)
                for s, x in enumerate(xb)]
        src = pl.multiple_of(jnp.minimum(i + 1, NT - 1) * T, T)
        vts = v_side(xb, keep, ln1(src, (i + 1) * T, T))
        for j in range(NP):
            ph = jnp.concatenate([p[j] for p in phik], axis=1).astype(bf16)
            kvacc_v[j] += kv_prod(vts, ph, j)
        return c

    lax.fori_loop(1, NT, p1_body, 0)

    cp_wr.wait()
    cp_w(4).wait()
    cp_wo.wait()
    cp_wg.wait()
    cp_wu.wait()
    keep = flag_s[0] > 0
    kv_mask = (lax.broadcasted_iota(jnp.int32, (64, 128), 0) // DH
               == (lax.broadcasted_iota(jnp.int32, (64, 128), 1) // DH) % 2)
    ties = [{} for _ in range(8)]
    for j in range(NP):
        kvj = jnp.where(kv_mask, kvacc_v[j], 0.0)
        kv_v[:, j * 128:(j + 1) * 128] = _pk(kvj.astype(bf16))
        zj = _lanes(jnp.sum(zacc_v[j * 128:(j + 1) * 128, :], axis=-1, keepdims=True))
        zacc_v[j * 128:(j + 1) * 128, :] = zj
        woj = _pk(wo_v[j * 64:(j + 1) * 64, :])
        wop_v[j * 32:(j + 1) * 32, :] = woj
        if j < 14:
            dep = jnp.max(jnp.concatenate([kvj, zj], axis=0).reshape(6, 32, 128), axis=0)
            dep = _or_all([pltpu.bitcast(dep, u32)] + [woj[:, c * 128:(c + 1) * 128] for c in range(8)])
            for q, v in enumerate(_vregs(dep)):
                ties[1 + j // 2][((j % 2) * 32 + q * 8, 0)] = v
    wr = wr_v[...].astype(f32)
    wl = jnp.sum(wr, axis=0, keepdims=True)
    wsum = jnp.sum(wl, axis=1, keepdims=True)
    wrb_v[...] = jnp.concatenate(
        [jnp.broadcast_to(wr[j:j + 1, :], (8, 128)) for j in range(8)]
        + [jnp.broadcast_to(wsum, (8, 128)), jnp.broadcast_to(wl, (8, 128))], axis=1)
    Folder(Q0).fold(4, keep, ties)

    pq_v = (pq0_v, pq1_v, pq2_v, pq3_v)

    def views_of(g):
        lo = g * (BPI * B)
        if not isinstance(g, int):
            lo = pl.multiple_of(lo, BPI * B)
        return tuple(ref.at[pl.ds(lo, BPI * B)] for ref in (x_v, h_v, out_v, st_v)) + (g,)

    def stage_q(b, slot, keep=None, pieces=()):
        group = groups_of(proj(Q0, PR, load_xn(b), keep, pieces, row0=128))
        for j in range(NP):
            ph = _hedgehog_t(_pair_logits(group, j), zacc_v[j * 128:(j + 1) * 128, :])
            pq_v[slot][(j // 2) * 64:(j // 2 + 1) * 64, (j % 2) * B:(j % 2 + 1) * B] = _pk(ph.astype(bf16))

    def stage_g(slot):
        pq = pq_v[slot].at[pl.ds(pl.multiple_of(flag_s[1], D // 2), D // 2)]
        parts = [_dot_nn(_upk(kv_v[:, j * 128:(j + 1) * 128]),
                         _upk(pq[(j // 2) * 64:(j // 2 + 1) * 64, (j % 2) * B:(j % 2 + 1) * B]))
                 for j in range(NP)]
        return jnp.concatenate(parts, axis=0).astype(bf16)

    def stage_h(views, s, ot, keep, pieces):
        wo = wop_v[...]
        if pieces:
            ties = {}
            for k, vals in enumerate(pieces):
                q = min(int(1.72 * k) + 3, 15)
                for m, val in enumerate(vals):
                    ties[((q % 2) * 256 + m * 8, (q // 2) * 128)] = val
            wo = _tie(keep, wo, ties)
        rows = slice(s * B, (s + 1) * B)
        x_g, h_g = views[0], views[1]
        h = x_g[rows, :].astype(f32) + lax.dot_general(ot, _upk(wo), _TN_DIMS, preferred_element_type=f32)
        h_g[rows, :] = h

        def wmul(d, lo):
            return (d.reshape(B // 8, 8, 128) * wrb_v[:, lo:lo + 128][None]).reshape(B, 128)

        h0 = h[:, 0:128]
        s1 = s2 = s3 = None
        for c in range(1, D // 128):
            d = h[:, c * 128:(c + 1) * 128] - h0
            t2 = d * d
            t3 = wmul(d, c * 128)
            s1, s2, s3 = (d, t2, t3) if c == 1 else (s1 + d, s2 + t2, s3 + t3)
        c0 = _lanes(jnp.mean(h0, axis=-1, keepdims=True))
        g0 = h0 - c0
        t1 = s1 + 8.0 * g0
        t2 = s2 + g0 * (s1 + t1)
        t3 = s3 + wmul(g0, D + 128)
        return jnp.concatenate([t1, t2, t3, c0], axis=1), h

    def stage_i(views, s, part, h=None, valid=None):
        _, h_g, out_g, st_g, g = views
        b = g * BPI + s
        rows = slice(s * B, (s + 1) * B)
        if h is None:
            h = h_g[rows, :]
        bv = bestv_v[...]
        bi = besti_v[...]
        wsum = wrb_v[0:1, D:D + 128]
        pieces, outs, nvs, nis, sts = [], [], [], [], []
        for k in range(B // R):
            sl = slice(k * R, (k + 1) * R)
            red = [_lanes(jnp.sum(part[sl, n * 128:(n + 1) * 128], axis=-1, keepdims=True)) for n in range(3)]
            c0 = part[sl, 384:512]
            mu = red[0] * (1.0 / D)
            var = jnp.maximum(red[1] * (1.0 / D) - mu * mu, 0.0)
            rs = lax.rsqrt(var + LN_EPS)
            r = (red[2] - mu * wsum) * rs
            murs = (mu + c0) * rs
            a = 1.0 + rs
            o = jnp.concatenate([h[sl, c * 128:(c + 1) * 128] * a - murs for c in range(D // 128)], axis=1)
            outs.append(o.astype(bf16))
            sts.append(jnp.concatenate([rs, murs], axis=1))
            if valid is not None:
                r = jnp.where(valid, r, -jnp.inf)
            idx = lax.broadcasted_iota(jnp.int32, (R, 128), 0) + (b * B + k * R)
            better = r > bv[sl]
            nv = jnp.where(better, r, bv[sl])
            nvs.append(nv)
            nis.append(jnp.where(better, idx, bi[sl]))
            pieces.append(_vregs(o) + _vregs(nv))
        out_g[rows, :] = jnp.concatenate(outs, axis=0)
        st_g[rows, :] = jnp.concatenate(sts, axis=0)
        bestv_v[...] = jnp.concatenate(nvs, axis=0)
        besti_v[...] = jnp.concatenate(nis, axis=0)
        return pieces

    def p2_body(i, c):
        b0 = i * BPI
        keep = flag_s[0] > 0
        cur = views_of(i)
        pieces = stage_i(views_of(jnp.maximum(i - 1, 0)), BPI - 1, pend_v[...], valid=i > 0)
        for s in range(BPI):
            stage_q(b0 + s, s, keep, pieces if s == 0 else ())
        ot = [stage_g(s) for s in range(BPI)]
        part, h = stage_h(cur, 0, ot[0], keep, ())
        for s in range(1, BPI):
            pieces = stage_i(cur, s - 1, part, h)
            part, h = stage_h(cur, s, ot[s], keep, pieces)
        pend_v[...] = part

        @pl.when(i > 0)
        def _():
            cp_out(jnp.maximum(b0 - 1, 0), 1).start()

        cp_out(b0, BPI - 1).start()
        return c

    lax.fori_loop(0, NI, p2_body, 0)
    stage_i(views_of(NI - 1), BPI - 1, pend_v[...])
    cp_out(NB - 1, 1).start()

    keep = flag_s[0] > 0
    bv = bestv_v[...]
    mval = jnp.max(bv, axis=0, keepdims=True)
    sel = jnp.min(jnp.where(bv == mval, besti_v[...], S - 1), axis=0, keepdims=True)
    idx = sel[0, 0]
    hrow = h_v[pl.ds(idx, 1), :]
    strow = st_v[pl.ds(idx, 1), :]
    xrow = jnp.concatenate([hrow[:, c * 128:(c + 1) * 128] * strow[:, 0:128] - strow[:, 128:256]
                            for c in range(D // 128)], axis=1).astype(bf16)
    xs = jnp.broadcast_to(xrow, (16, D))

    def act(g, u):
        a = g * pl.reciprocal(1.0 + jnp.exp(-g), approx=True) * u
        return jnp.concatenate([a, a], axis=0).astype(bf16)

    def down(a, lo, w):
        return _dot_nn(a, _upk(wdp_v[lo // 2:(lo + w) // 2, 0:D]))[0:8]

    NM = F - NBV * 128
    xcol = jnp.broadcast_to(xrow.astype(f32), (128, D)).T
    jobs = [(which, b) for b in range(NBV) for which in (0, 1)]
    vres, prev = {}, None
    for j0 in range(0, len(jobs), NCH):
        grp = jobs[j0:j0 + NCH]
        accs = [None] * len(grp)
        for r in range(D // 16):
            for n, (which, b) in enumerate(grp):
                w = (wg_v, wu_v)[which][r * 16:(r + 1) * 16, NM + b * 128:NM + (b + 1) * 128].astype(f32)
                t0 = w[0:8] * xcol[r * 16:r * 16 + 8]
                t1 = w[8:16] * xcol[r * 16 + 8:r * 16 + 16]
                if accs[n] is None:
                    if prev is not None:
                        t0 = jnp.where(keep, t0, prev[n % len(prev)])
                    accs[n] = t0 + t1
                else:
                    accs[n] = (accs[n] + t0) + t1
        prev = accs
        for n, job in enumerate(grp):
            vres[job] = _allreduce8(accs[n][None], jnp.add)[0]

    chunks = [(lo, min(FC, NM - lo)) for lo in range(0, NM, FC)]
    acts, y = [], None
    for k, (lo, w) in enumerate(chunks):
        g = _dot_nn(xs, wg_v[:, lo:lo + w])
        u = _dot_nn(xs, wu_v[:, lo:lo + w])
        acts.append(act(g[0:8], u[0:8]))
        if k >= 1:
            t = down(acts[k - 1], *chunks[k - 1])
            y = t if y is None else y + t
    y = y + down(acts[-1], *chunks[-1])
    for b0, nb in ((0, 4), (4, 4), (8, 3), (11, 1)):
        g = jnp.concatenate([vres[(0, b)] for b in range(b0, b0 + nb)], axis=1)
        u = jnp.concatenate([vres[(1, b)] for b in range(b0, b0 + nb)], axis=1)
        y = y + down(act(g, u), NM + b0 * 128, nb * 128)

    gate = jnp.broadcast_to(jax.nn.sigmoid(mval), (8, 128))
    base = pl.multiple_of((idx >> 4) << 4, 16)
    rows = pl.ds(base, 16)
    h16 = h_v[rows, :]
    st16 = st_v[rows, :]
    a16 = 1.0 + st16[:, 0:128]
    m16 = st16[:, 128:256]
    hit = (lax.broadcasted_iota(jnp.int32, (16, 128), 0) + base) == idx
    res = []
    for c in range(D // 128):
        yc = y[:, c * 128:(c + 1) * 128] * gate
        yc = jnp.concatenate([yc, yc], axis=0)
        res.append(h16[:, c * 128:(c + 1) * 128] * a16 - m16 + jnp.where(hit, yc, 0.0))
    res = jnp.concatenate(res, axis=1).astype(bf16)
    for i in range(NI):
        cp_out(i * BPI, BPI - 1).wait()
        cp_out(i * BPI + BPI - 1, 1).wait()
    out_v[rows, :] = res
    fix = pltpu.make_async_copy(out_v.at[rows], out_hbm.at[rows], sem_o.at[0])
    fix.start()
    fix.wait()


@jax.jit
def pallas_sequential_preLN__linear_kernel_hedgehog__moe_arch_mod__prompt_kernel(
    A_x: jax.Array,
    A_wqkv: jax.Array,
    A_w_phi: jax.Array,
    A_wo: jax.Array,
    B_x: jax.Array,
    B_w_r: jax.Array,
    B_w_gate: jax.Array,
    B_w_up: jax.Array,
    B_w_down: jax.Array,
):
    del B_x
    x = A_x.reshape(S, D)
    wphi = A_w_phi.reshape(H * DH, DH)
    wr = B_w_r.reshape(8, 128)
    any_spec = pl.BlockSpec(memory_space=pl.ANY)
    out = pl.pallas_call(
        _kernel,
        out_shape=jax.ShapeDtypeStruct((S, D), bf16),
        in_specs=[any_spec] * 8,
        out_specs=any_spec,
        scratch_shapes=[
            pltpu.VMEM((S, D), bf16),
            pltpu.VMEM((D, 3 * D), bf16),
            pltpu.VMEM((H * DH, DH), bf16),
            pltpu.VMEM((D, D), bf16),
            pltpu.VMEM((8, 128), bf16),
            pltpu.VMEM((D, F + 128), bf16),
            pltpu.VMEM((D, F + 128), bf16),
            pltpu.VMEM((F, D), bf16),
            pltpu.VMEM((2 * PR + D // 2, D), u32),
            pltpu.VMEM((D // 2, D), u32),
            pltpu.VMEM((F // 2, D + 128), u32),
            pltpu.VMEM((64, 8 * 128), u32),
            pltpu.VMEM(((S + T) // 2, D), u32),
            pltpu.VMEM((NP, 64, 128), f32),
            pltpu.VMEM((2 * D, 128), f32),
            pltpu.VMEM((32, NP * 128), u32),
            pltpu.VMEM((D, T), u32),
            pltpu.VMEM((D // 2, 2 * B), u32),
            pltpu.VMEM((D // 2, 2 * B), u32),
            pltpu.VMEM((D // 2, 2 * B), u32),
            pltpu.VMEM((D // 2, 2 * B), u32),
            pltpu.VMEM((S, D), f32),
            pltpu.VMEM((S, 256), f32),
            pltpu.VMEM((B, 512), f32),
            pltpu.VMEM((S, D), bf16),
            pltpu.VMEM((8, D + 256), f32),
            pltpu.VMEM((B, 128), f32),
            pltpu.VMEM((B, 128), jnp.int32),
            pltpu.SMEM((2,), jnp.int32),
            pltpu.SemaphoreType.DMA((_NSEM_IN,)),
            pltpu.SemaphoreType.DMA((1,)),
        ],
        compiler_params=pltpu.CompilerParams(vmem_limit_bytes=110 * 1024 * 1024,
                                             disable_bounds_checks=True,
                                             disable_semaphore_checks=True),
        name="hedgehog_mod",
    )(x, A_wqkv, wphi, A_wo, wr, B_w_gate, B_w_up, B_w_down)
    return out.reshape(1, S, D)
```

```python
import os
import jax
import jax.numpy as jnp
from jax import lax
import jax.experimental.pallas as pl
import jax.experimental.pallas.tpu as pltpu

S = 2048
D = 1024
H = 32
DH = 32
F = 3584
T = 512
NT = S // T
T0 = 256
B = 128
NB = S // B
BPI = 4
NI = NB // BPI
NP = H // 2
FC = 512
R = 16
NBV = 12
NCH = 4
OCH = 176
DCH = 1200
NV = 124
PR = NV * 4
HK = D // 2
P2 = 2 * B
LOG2E = 1.4426950408889634
LN_EPS = 1e-5
DEN_EPS = 1e-6

_NT_DIMS = (((1,), (1,)), ((), ()))
_TN_DIMS = (((0,), (0,)), ((), ()))

bf16 = jnp.bfloat16
f32 = jnp.float32
u32 = jnp.uint32


def _opt(name, default):
    return type(default)(os.environ.get(name, default))


def _dot_nt(a, b):
    return lax.dot_general(a, b, _NT_DIMS, preferred_element_type=f32)


def _dot_nn(a, b):
    return jnp.dot(a, b, preferred_element_type=f32)


def _pk(x):
    return pltpu.bitcast(x, u32)


def _upk(x):
    return pltpu.bitcast(x, bf16)


def _lanes(x):
    return jnp.broadcast_to(x, (x.shape[0], 128))


def _layernorm(x):
    m = jnp.mean(x, axis=-1, keepdims=True)
    xc = x - m
    v = jnp.mean(xc * xc, axis=-1, keepdims=True)
    return xc * lax.rsqrt(v + LN_EPS)


def _allreduce8(x, op):
    x = op(x, pltpu.roll(x, 4, 1))
    x = op(x, pltpu.roll(x, 2, 1))
    x = op(x, pltpu.roll(x, 1, 1))
    return x


def _hedgehog_t(p, z=None):
    t = p.shape[-1]
    p4 = p.reshape(2, 4, 8, t)
    mx = _allreduce8(jnp.max(p4, axis=1), jnp.maximum)
    mn = _allreduce8(jnp.min(p4, axis=1), jnp.minimum)
    ep = jnp.exp2(p4 - mx[:, None])
    en = jnp.exp2(mn[:, None] - p4)
    a = pl.reciprocal(_allreduce8(jnp.sum(ep, axis=1), jnp.add), approx=True)
    b = pl.reciprocal(_allreduce8(jnp.sum(en, axis=1), jnp.add), approx=True)
    if z is not None:
        dp = jnp.sum(ep * z[0:64].reshape(2, 4, 8, t), axis=1)
        dn = jnp.sum(en * z[64:128].reshape(2, 4, 8, t), axis=1)
        den = _allreduce8(dp * a + dn * b, jnp.add) + DEN_EPS
        inv = pl.reciprocal(den, approx=True)
        a = a * inv
        b = b * inv
    fp = (ep * a[:, None]).reshape(64, t)
    fn = (en * b[:, None]).reshape(64, t)
    return jnp.concatenate([fp, fn], axis=0)


_SA = ((3, None, 0), (2, 3, 1), (0, 1, 1), (0, None, 0), (0, 3, 1), (1, 3, -1), (2, 0, -1))
_SB = ((2, 0, -1), (0, None, 0), (3, None, 0), (1, 3, -1), (0, 3, 1), (2, 3, 1), (0, 1, 1))


def _combo(blocks, spec):
    a, b, sign = spec
    if b is None:
        return blocks[a]
    return blocks[a] + blocks[b] if sign > 0 else blocks[a] - blocks[b]


def _strassen(product, emit):
    m4 = product(0)
    m2 = product(1)
    emit(2, m4 + m2)
    m5 = product(2)
    u = m4 - m5
    m3 = product(3)
    emit(1, m5 + m3)
    v = m3 - m2
    m1 = product(4)
    u = u + m1
    v = v + m1
    emit(0, u + product(5))
    emit(3, v + product(6))


def _head_groups(h):
    base, k = (NV // 4) * (h // 8), h % 8
    return ([base + 4 * k + i for i in range(3)],
            base + 4 * k - 1 if k > 0 else None,
            base + 4 * k + 3 if k < 7 else None,
            8 - k)


def _pair_logits(group, j):
    parts = []
    for h in (2 * j, 2 * j + 1):
        full, below, above, a = _head_groups(h)
        ref = group(full[0])
        sub = lax.broadcasted_iota(jnp.int32, ref.shape, 0)
        if above is None:
            m = jnp.where(sub >= a, group(below), 0.0)
        else:
            m = jnp.where(sub == a - 1, 0.0, group(above))
            if below is not None:
                m = jnp.where(sub >= a, group(below), m)
        parts += [m] + [group(q) for q in full]
    return jnp.concatenate(parts, axis=0)


def _pair_need(j):
    full, _, above, _ = _head_groups(2 * j + 1)
    return full[2] if above is None else above


def _tie(keep, w, ties):
    rows = sorted({r for r, _ in ties})
    out, pos = [], 0
    for r in rows:
        if r > pos:
            out.append(w[pos:r])
        cols = sorted(c for rr, c in ties if rr == r)
        parts, cpos = [], 0
        for c in cols:
            if c > cpos:
                parts.append(w[r:r + 8, cpos:c])
            parts.append(jnp.where(keep, w[r:r + 8, c:c + 128], ties[(r, c)]))
            cpos = c + 128
        if cpos < w.shape[1]:
            parts.append(w[r:r + 8, cpos:])
        out.append(jnp.concatenate(parts, axis=1) if len(parts) > 1 else parts[0])
        pos = r + 8
    if pos < w.shape[0]:
        out.append(w[pos:])
    return jnp.concatenate(out, axis=0)


def _vregs(x):
    if x.dtype != u32:
        x = pltpu.bitcast(x, u32)
    return [x[r:r + 8, c:c + 128] for r in range(0, x.shape[0], 8) for c in range(0, x.shape[1], 128)]


def _or_all(vals):
    acc = vals[0]
    for v in vals[1:]:
        acc = acc | v
    return acc


_WCHUNKS = ((D, 256, 2), (D + 256, 384, 3), (D + 640, 384, 4),
            (2 * D, 1024, 5),
            (0, 1024, 7))
_NSEM_IN = 11
_PHI_A = 256


def _kernel(x_hbm, wqkv_hbm, wphi_hbm, wo_hbm, wr_hbm, wg_hbm, wu_hbm, wd_hbm,
            out_hbm,
            x_v, wqkv_v, wphi_v, wo_v, wr_v, wg_v, wu_v, wd_v,
            wtk_v, wtv_v, wsq_v, wsk_v, wsv_v, wso_v, wdp_v, amat_v, xn_v, xs_v, kvacc_v, zacc_v, kv_v, phi_v,
            pq0_v, pq1_v, pq2_v, pq3_v, oc0_v, oc1_v, h_v, st_v, pend_v, out_v, wrb_v,
            bestv_v, besti_v, flag_s,
            sem_i, sem_o):

    def cp_x(lo, n, sem):
        return pltpu.make_async_copy(x_hbm.at[pl.ds(lo, n)], x_v.at[pl.ds(lo, n)], sem_i.at[sem])

    def cp_w(c):
        lo, w, sem = _WCHUNKS[c]
        return pltpu.make_async_copy(wqkv_hbm.at[:, pl.ds(lo, w)], wqkv_v.at[:, pl.ds(lo, w)], sem_i.at[sem])

    def cp_wd(k):
        lo, n = k * DCH, min(DCH, F - k * DCH)
        return pltpu.make_async_copy(wd_hbm.at[pl.ds(lo, n)], wd_v.at[pl.ds(lo, n)], sem_i.at[(6, 8, 9)[k]])

    cp_pa = pltpu.make_async_copy(wphi_hbm.at[pl.ds(0, _PHI_A)], wphi_v.at[pl.ds(0, _PHI_A)], sem_i.at[0])
    cp_pb = pltpu.make_async_copy(wphi_hbm.at[pl.ds(_PHI_A, D - _PHI_A)], wphi_v.at[pl.ds(_PHI_A, D - _PHI_A)],
                                  sem_i.at[3])
    cp_x0 = cp_x(0, T0, 1)
    cp_x1 = cp_x(T0, T0, 4)
    cp_x2 = cp_x(T, T, 5)
    cp_x3 = cp_x(2 * T, T, 6)
    cp_x4 = cp_x(3 * T, T, 8)
    cp_wr = pltpu.make_async_copy(wr_hbm, wr_v, sem_i.at[7])

    def cp_wo(k, half):
        lo, n = k * OCH, min(OCH, HK - k * OCH)
        rows = pl.ds(half * HK + lo, n)
        return pltpu.make_async_copy(wo_hbm.at[rows], wo_v.at[rows], sem_i.at[(6, 8, 9)[k]])

    def wait_bg(k):
        cp_wo(k, 0).wait()
        cp_wo(k, 1).wait()
        cp_wd(k).wait()

    cp_wg = pltpu.make_async_copy(wg_hbm, wg_v.at[:, pl.ds(0, F)], sem_i.at[10])
    cp_wu = pltpu.make_async_copy(wu_hbm, wu_v.at[:, pl.ds(0, F)], sem_i.at[10])

    def cp_out(b, n):
        lo = b * B
        if not isinstance(b, int):
            lo = pl.multiple_of(lo, B)
        return pltpu.make_async_copy(out_v.at[pl.ds(P2 + lo, n * B)], out_hbm.at[pl.ds(lo, n * B)], sem_o.at[0])

    for cp in (cp_pa, cp_x0, cp_w(0), cp_pb, cp_w(1), cp_w(2), cp_x1, cp_w(3), cp_x2,
               cp_x3, cp_wo(0, 0), cp_wo(0, 1), cp_wd(0), cp_x4, cp_wo(1, 0), cp_wo(1, 1), cp_wd(1),
               cp_wo(2, 0), cp_wo(2, 1), cp_wd(2), cp_wr, cp_w(4), cp_wg, cp_wu):
        cp.start()
    flag_s[0] = 1
    flag_s[1] = 0

    def ln1(xg, src, xd, dst, n, which=None, keep=None, anchors=None):
        pieces = []
        for pr in range(n // P2):
            for k in range(B // R):
                off = pr * P2 + k * R
                if which is not None and pr * (B // R) + k not in which:
                    continue
                x0 = xg[src + off:src + off + R, :].astype(f32)
                x1 = xg[src + off + B:src + off + B + R, :].astype(f32)
                if anchors is not None:
                    a = anchors[len(pieces)]
                    x0 = jnp.concatenate([jnp.where(keep, x0[:, :128], a), x0[:, 128:]], axis=1)
                    x1 = jnp.concatenate([jnp.where(keep, x1[:, :128], a), x1[:, 128:]], axis=1)
                p0 = _layernorm(x0)
                p1 = _layernorm(x1)
                lo = (dst + pr * P2) // 4 + k * (R // 2)
                if _opt('LNM', 0):
                    top = jnp.concatenate([p0[:, :HK], p1[:, :HK]], axis=1)
                    bot = jnp.concatenate([p0[:, HK:], p1[:, HK:]], axis=1)
                    pieces.append([store_combos(xd, lo, top, bot, _SB)])
                    continue
                blocks = (p0[:, :HK], p1[:, :HK], p0[:, HK:], p1[:, HK:])
                vs = []
                for m, spec in enumerate(_SB):
                    t = _combo(blocks, spec)
                    xd[lo:lo + R // 2, m * HK:(m + 1) * HK] = _pk(t.astype(bf16))
                    if spec[1] is not None:
                        vs.append(_vregs(t))
                pieces.append([_or_all(list(col)) for col in zip(*vs)])
        return pieces

    def ln_plain(lo, n):
        pieces = []
        for r in range(lo, lo + n, R):
            p = _layernorm(x_v[r:r + R, :].astype(f32))
            xn_v[r // 2:(r + R) // 2, :] = _pk(p.astype(bf16))
            pieces.append(_vregs(p))
        return pieces

    def load_xn(b):
        return _upk(xn_v[b * (B // 2):(b + 1) * (B // 2), :])

    def piece_ties(pieces, n, row0=0, col=0):
        ties = {}
        if pieces:
            step = (n - row0) // len(pieces) // 8 * 8
            for k, p in enumerate(pieces):
                for q, val in enumerate(p):
                    ties[(row0 + k * step + (q // 4) * 8, col + (q % 4) * 128)] = val
        return ties

    def xs_view(i, tiles):
        return xs_v.at[pl.ds(pl.multiple_of(i * (T // 4), T // 4), tiles * (T // 4))]

    def sproj(ws, xd, pr, emit, keep=None, work=None):
        lo = pr * (B // 2)

        def product(m):
            lhs = ws[:, m * HK:(m + 1) * HK]
            if work and work.get(m):
                lhs = _tie(keep, lhs, piece_ties(work[m], lhs.shape[0], 32))
            return _dot_nt(_upk(lhs), _upk(xd[lo:lo + B // 2, m * HK:(m + 1) * HK]))

        _strassen(product, lambda k, val: emit(k // 2, k % 2, val))

    def spread(pieces, slots):
        res = {}
        for k, (pr, m) in enumerate(slots):
            res.setdefault(pr, {})[m] = pieces[k * len(pieces) // len(slots):(k + 1) * len(pieces) // len(slots)]
        return res

    def fence(ref, row, col):
        return ref[pl.ds(pl.multiple_of(flag_s[1] + row, 8), 8), col:col + 128]

    def store_combos(ws, row, top, bot, table=_SA, keep=None, dep=None, every=1):
        for n, c in enumerate(range(0, HK, 128)):
            raw = [top[:, c:c + 128], top[:, HK + c:HK + c + 128], bot[:, c:c + 128], bot[:, HK + c:HK + c + 128]]
            if keep is not None and dep is not None:
                for q in (0, 3):
                    d = dep if raw[q].dtype == u32 else pltpu.bitcast(jnp.concatenate([dep, dep], axis=0), f32)
                    raw[q] = jnp.where(keep, raw[q], d)
            blocks = [_upk(b).astype(f32) if b.dtype == u32 else b for b in raw]
            for m, spec in enumerate(table):
                t = raw[spec[0]] if spec[1] is None else _combo(blocks, spec)
                ws[row:row + 8, m * HK + c:m * HK + c + 128] = t if t.dtype == u32 else _pk(t.astype(bf16))
            if keep is not None and (n + 1) % every == 0:
                dep = fence(ws, row, c)
        return dep if keep is not None else fence(ws, row, 0)

    def k_side(group, pairs, first, slot=None):
        res = []
        for j in pairs:
            ph = _hedgehog_t(_pair_logits(group, j))
            if first:
                zacc_v[j * 128:(j + 1) * 128, :] = ph
            else:
                zacc_v[j * 128:(j + 1) * 128, :] += ph
            if slot is not None:
                phi_v[j * 64:(j + 1) * 64, slot * B:(slot + 1) * B] = _pk(ph.astype(bf16))
            res.append(ph)
        return res

    def proj(wt, lo, n, xb, keep=None, early=(), late=()):
        lhs = wt[lo:lo + n, :]
        ties = piece_ties(early, n)
        ties.update(piece_ties(late, n, col=HK))
        if ties:
            lhs = _tie(keep, lhs, ties)
        return _dot_nt(_upk(lhs), xb)

    def half_groups(p, half):
        return lambda pos: p[(pos - half * (NV // 2)) * 8:(pos - half * (NV // 2) + 1) * 8]

    def half_pairs(half):
        return range(half * (NP // 2), (half + 1) * (NP // 2))

    def kv_prod(vt, ph, j):
        half, r = j // (NP // 2), (j % (NP // 2)) * 64
        v = jnp.concatenate([vt[(s, half)][r:r + 64] for s in range(T // B)], axis=1).astype(bf16)
        return _dot_nt(v, ph)

    def v_side(xd, keep, pieces, chain):
        work = spread(pieces, [(0, m) for m in range(1, 7)] + [(1, m) for m in range(6)])
        vt = {}
        for q in range(T // P2):
            sproj(wsv_v, xd, q, lambda half, blk, val, q=q: vt.__setitem__((2 * q + blk, half), val),
                  keep, work.get(q))
            if q == 0:
                m = _opt('OM', 2)
                work[1][m] = list(work[1].get(m, [])) + [[chain(pltpu.bitcast(vt[(0, 1)][0:8], u32))]]
        return vt

    r_i = lax.broadcasted_iota(jnp.int32, (128, DH), 0)
    c_i = lax.broadcasted_iota(jnp.int32, (128, DH), 1)
    expand = (r_i % DH == c_i).astype(bf16)
    r_h = lax.broadcasted_iota(jnp.int32, (128, 128), 0) // DH
    c_h = lax.broadcasted_iota(jnp.int32, (128, 128), 1) // DH
    same_head = r_h == c_h

    def make_amat(g):
        a = _dot_nt(expand, wphi_v[g * 128:(g + 1) * 128, :])
        amat_v[:, g * 128:(g + 1) * 128] = _pk(jnp.where(same_head, a, 0.0).astype(bf16))

    class Folder:
        def __init__(self, col0, first=0):
            self.col0, self.rows, self.mprev, self.done = col0, {}, None, first

        def fold(self, g, keep=None, ties=None):
            sub = lax.broadcasted_iota(jnp.int32, (8, D), 0)
            am = amat_v[:, g * 128:(g + 1) * 128]
            if ties:
                am = _tie(keep, am, ties)
            wt = _dot_nt(_upk(am), wqkv_v[:, self.col0 + g * 128:self.col0 + (g + 1) * 128])
            for hh in range(4):
                full, below, _, a = _head_groups(4 * g + hh)
                r0 = hh * DH
                ref = jnp.broadcast_to(wt[r0 + a - 1:r0 + a, :], (8, D))
                part = [(wt[r0 + 8 * i:r0 + 8 * (i + 1)] - ref) * LOG2E for i in range(4)]
                if below is not None:
                    self.rows[below] = jnp.where(sub >= a, part[0], self.mprev)
                self.mprev = part[0]
                for q, v in zip(full, part[1:]):
                    self.rows[q] = v
            new = {}
            while self.done in self.rows and self.done + 1 in self.rows:
                new[self.done] = jnp.concatenate([self.rows.pop(self.done), self.rows.pop(self.done + 1)], axis=0)
                self.done += 2
            return new

    bestv_v[...] = jnp.full(bestv_v.shape, -jnp.inf, f32)
    besti_v[...] = lax.broadcasted_iota(jnp.int32, besti_v.shape, 0)
    h_v[0:P2, :] = jnp.zeros((P2, D), f32)
    st_v[0:B, :] = jnp.zeros((B, 256), f32)
    pend_v[...] = jnp.zeros(pend_v.shape, f32)

    cp_pa.wait()
    for g in range(_PHI_A // 128):
        make_amat(g)

    cp_x0.wait()
    ln_plain(0, T0)
    xb = [load_xn(s) for s in range(2)]
    logits = [{} for _ in range(4)]
    npairs = [0] * 4

    def k_finish(s, hold=0):
        ready = [j for j in range(npairs[s], NP) if _pair_need(j) < len(logits[s])]
        ready = ready[:len(ready) - hold]
        k_side(logits[s].__getitem__, ready, s == 0, s)
        npairs[s] += len(ready)

    def k_chunk(s, hi, keep=None, early=(), late=(), hold=0):
        lo = len(logits[s])
        p = proj(wtk_v, lo * 4, (hi - lo) * 4, xb[s], keep, early, late)
        for q in range(lo, hi):
            logits[s][q] = p[(q - lo) * 8:(q - lo + 1) * 8]
        k_finish(s, hold)

    def weight_combos(wt, ws, keep, dep, lo=0, hi=None):
        n = wt.shape[0] // 2
        deps = []
        for r in range(lo * 8, n if hi is None else hi * 8, 8):
            dep = store_combos(ws, r, wt[r:r + 8, :], wt[n + r:n + r + 8, :], _SA, keep, dep, _opt('EV', 1))
            deps.append([dep])
        return deps

    fk = Folder(D)

    def fold_k(c):
        lo, w, _ = _WCHUNKS[c]
        for g in range((lo - D) // 128, (lo - D + w) // 128):
            for pos, slab in fk.fold(g).items():
                wtk_v[pos * 4:pos * 4 + 8, :] = _pk(slab.astype(bf16))
        return fk.done

    HOLD = _opt('HOLD', 1)
    cp_w(0).wait()
    n = fold_k(0)
    k_chunk(0, n)
    k_chunk(1, n, hold=HOLD)

    cp_pb.wait()
    cp_w(1).wait()
    k_finish(1)
    for g in range(_PHI_A // 128, 8):
        make_amat(g)
    n = fold_k(1)
    k_chunk(0, n)
    k_chunk(1, n, hold=HOLD)

    cp_w(2).wait()
    cp_x1.wait()
    k_finish(1)
    keep = flag_s[0] > 0
    n = fold_k(2)
    pieces = ln_plain(T0, T0)
    c = [int(v) for v in _opt('LS', '0,3,6,8').split(',')]
    k_chunk(0, n, keep, pieces[0:c[0]], pieces[c[0]:c[1]])
    k_chunk(1, n, keep, pieces[c[1]:c[2]], pieces[c[2]:c[3]])
    xb += [load_xn(s) for s in range(2, 4)]
    k_chunk(2, NV, keep, pieces[c[3]:16])
    KB = _opt('KB', 0)
    wtk_m = wtk_v.at[pl.ds(pl.multiple_of(flag_s[1], PR), PR)]
    kd3 = weight_combos(wtk_m, wsk_v, keep, pieces[_opt('D3', 15)][0], 0, KB)
    k_chunk(3, _opt('KS', 96), keep, (), [[], [], kd3[-1]] if KB else (), hold=2)

    cp_w(3).wait()
    cp_x2.wait()
    k_finish(3)
    keep = flag_s[0] > 0
    k_chunk(3, NV)
    wtv_v[...] = _pk(wqkv_v[:, 2 * D:3 * D].T)

    vt = {}
    l0, l1 = [int(v) for v in _opt('B4L', '1,7').split(',')]
    AP, AR = _opt('AP', 0), _opt('AR', 512)
    pending, final, acc = [], [], None
    for ps in range(8):
        s, half = ps // 2, ps % 2
        wt = wtv_v if s == 0 else wtv_v.at[pl.ds(pl.multiple_of(flag_s[1] * s, D // 2), D // 2)]
        lhs = wt[:, half * HK:(half + 1) * HK]
        work = list(pending)
        if ps == 7:
            work = work + [[]] * (4 - len(work)) + final
        if work:
            lhs = _tie(keep, lhs, piece_ties(work, D // 2))
        part = _dot_nt(_upk(lhs), xb[s][:, half * HK:(half + 1) * HK])
        acc = part if half == 0 else acc + part
        if half == 1:
            vt[(s, 0)], vt[(s, 1)] = acc[:HK], acc[HK:]
        pending = []
        if l0 <= ps < l1:
            which = list(range((ps - l0) * 16 // (l1 - l0), (ps - l0 + 1) * 16 // (l1 - l0)))
            rows = [n * D // len(which) // 16 * 16 for n in range(len(which))]
            pending = ln1(x_v, T, xs_v, T, T, which, keep, [part[r:r + R] for r in rows])
        if ps == AP:
            dep0 = pltpu.bitcast(part[AR:AR + 8], u32)
            kdeps = weight_combos(wtk_m, wsk_v, keep, dep0, KB) or [[dep0]]
            vdeps = weight_combos(wtv_v.at[pl.ds(pl.multiple_of(flag_s[1], D // 2), D // 2)], wsv_v, keep,
                                  kdeps[-1][0] if _opt('CH', 1) else dep0)
            final = [vdeps[-1] + kdeps[-1]]
    phi_m = phi_v.at[pl.ds(pl.multiple_of(flag_s[1], D), D)]
    for j in range(NP):
        kvacc_v[j] = kv_prod(vt, _upk(phi_m[j * 64:(j + 1) * 64, :]), j)
    cp_x3.wait()
    wait_bg(0)

    def p1_body(i, c):
        @pl.when(i == 2)
        def _():
            cp_x4.wait()
            wait_bg(1)

        @pl.when(i == 3)
        def _():
            wait_bg(2)

        keep = flag_s[0] > 0
        lo = jnp.minimum((i - 1) * DCH, F - DCH)
        sv = wd_v.at[pl.ds(pl.multiple_of(lo, 16), DCH)]
        dv = wdp_v.at[pl.ds(pl.multiple_of(lo // 2, 8), DCH // 2)]
        deps = []
        for r in range(0, DCH, 16):
            val = _pk(sv[r:r + 16, :])
            dv[r // 2:r // 2 + 8, 0:D] = val
            deps.append([_or_all(_vregs(val))])
        lo = jnp.minimum((i - 1) * OCH, HK - OCH)
        ov = wo_v.at[pl.ds(pl.multiple_of(lo, 16), HK + OCH)]
        od = wso_v.at[pl.ds(pl.multiple_of(lo // 2, 8), OCH // 2)]
        work = spread(deps, [(q, m) for q in range(2) for m in (0, 2, 4)])

        phik = {}
        PK = _opt('PK', 1)

        def k_emit(q):
            def emit(half, blk, val):
                for j, ph in zip(half_pairs(half), k_side(half_groups(val, half), half_pairs(half), False, 2 * q + blk if PK else None)):
                    phik[(2 * q + blk, j)] = ph
            return emit

        xd = xs_view(i, 2)
        for q in range(T // P2):
            sproj(wsk_v, xd, q, k_emit(q), keep, work[q])
        xg = x_v.at[pl.ds(pl.multiple_of(((i + 1) % NT) * T, T), T)]
        pieces = ln1(xg, 0, xd, T, T)

        def wo_chain(dep):
            for r in range(0, OCH, 16):
                dep = store_combos(od, r // 2, ov[r:r + 16, :].astype(f32), ov[HK + r:HK + r + 16, :].astype(f32),
                                   _SB, keep, dep)
            return dep

        vt = v_side(xd, keep, pieces, wo_chain)
        phi_m = phi_v.at[pl.ds(pl.multiple_of(flag_s[1], D), D)]
        for j in range(NP):
            if PK:
                ph = _upk(phi_m[j * 64:(j + 1) * 64, :])
            else:
                ph = jnp.concatenate([phik[(s, j)] for s in range(T // B)], axis=1).astype(bf16)
            kvacc_v[j] += kv_prod(vt, ph, j)
        return c

    lax.fori_loop(1, NT, p1_body, 0)

    cp_wr.wait()
    cp_w(4).wait()
    keep = flag_s[0] > 0
    kv_mask = (lax.broadcasted_iota(jnp.int32, (64, 128), 0) // DH
               == (lax.broadcasted_iota(jnp.int32, (64, 128), 1) // DH) % 2)
    ties = [{} for _ in range(8)]
    for j in range(NP):
        kvj = jnp.where(kv_mask, kvacc_v[j], 0.0)
        kv_v[:, j * 128:(j + 1) * 128] = _pk(kvj.astype(bf16))
        zj = _lanes(jnp.sum(zacc_v[j * 128:(j + 1) * 128, :], axis=-1, keepdims=True))
        zacc_v[j * 128:(j + 1) * 128, :] = zj
        vals = _vregs(kvj) + _vregs(zj)
        if j < 14:
            for q in range(4):
                ties[1 + j // 2][((j % 2) * 32 + q * 8, 0)] = _or_all(vals[q::4])
    wr = wr_v[...].astype(f32)
    wl = jnp.sum(wr, axis=0, keepdims=True)
    wsum = jnp.sum(wl, axis=1, keepdims=True)
    wrb_v[...] = jnp.concatenate(
        [jnp.broadcast_to(wr[j:j + 1, :], (8, 128)) for j in range(8)]
        + [jnp.broadcast_to(wsum, (8, 128)), jnp.broadcast_to(wl, (8, 128))], axis=1)
    fq = (Folder(0), Folder(0, NV // 2))
    tops = {}
    for n in range(8):
        half, g = n % 2, n // 2 + 4 * (n % 2)
        new = fq[half].fold(g, keep, ties[n])
        if half == 0:
            tops = new
        else:
            for pos, slab in new.items():
                store_combos(wsq_v, (pos - NV // 2) * 4, tops[pos - NV // 2], slab)

    pq_v = (pq0_v, pq1_v, pq2_v, pq3_v)

    def views_of(g):
        lo = g * (BPI * B)
        if not isinstance(g, int):
            lo = pl.multiple_of(lo, BPI * B)
        return ((x_v.at[pl.ds(lo, BPI * B)],)
                + tuple(ref.at[pl.ds(lo, P2 + BPI * B)] for ref in (h_v, out_v, st_v)) + (g,))

    def stage_q(xd, q, keep, work):
        def emit(half, blk, val):
            group = half_groups(val, half)
            for j in half_pairs(half):
                ph = _hedgehog_t(_pair_logits(group, j), zacc_v[j * 128:(j + 1) * 128, :])
                pq_v[2 * q + blk][(j // 2) * 64:(j // 2 + 1) * 64, (j % 2) * B:(j % 2 + 1) * B] = _pk(ph.astype(bf16))

        sproj(wsq_v, xd, q, emit, keep, work)

    oc_v = (oc0_v, oc1_v)

    def stage_g(q):
        pq = [pq_v[2 * q + blk].at[pl.ds(pl.multiple_of(flag_s[1], D // 2), D // 2)] for blk in range(2)]
        for jj in range(NP // 2):
            blocks = [_dot_nn(_upk(kv_v[:, j * 128:(j + 1) * 128]),
                              _upk(pq[blk][(j // 2) * 64:(j // 2 + 1) * 64, (j % 2) * B:(j % 2 + 1) * B]))
                      for blk in range(2) for j in (jj, jj + NP // 2)]
            for m, spec in enumerate(_SA):
                oc_v[q][jj * 32:(jj + 1) * 32, m * B:(m + 1) * B] = _pk(_combo(blocks, spec).astype(bf16))

    def stage_h(views, q, keep, pieces):
        x_g, h_g = views[0], views[1]
        oc = oc_v[q].at[pl.ds(pl.multiple_of(flag_s[1], HK // 2), HK // 2)]
        first, last = _opt('H0', 3), _opt('H1', 22)
        ties = [{} for _ in range(7)]
        for k, vals in enumerate(pieces):
            t = first + k * (last - first) // max(len(pieces) - 1, 1)
            for m, val in enumerate(vals):
                ties[t // 4][(m * 8, (t % 4) * 128)] = val
        state = {}
        done = [0]

        def product(m):
            w = wso_v[:, m * HK:(m + 1) * HK]
            if ties[m]:
                w = _tie(keep, w, ties[m])
            done[0] = m
            return lax.dot_general(_upk(oc[:, m * B:(m + 1) * B]), _upk(w), _TN_DIMS,
                                   preferred_element_type=f32)

        def wmul(d, lo):
            return (d.reshape(B // 8, 8, 128) * wrb_v[:, lo:lo + 128][None]).reshape(B, 128)

        def emit(k, val):
            blk, half = k // 2, k % 2
            s = 2 * q + blk
            cols = slice(half * HK, (half + 1) * HK)
            h = x_g[s * B:(s + 1) * B, cols].astype(f32) + val
            h_g[(s + 2) * B:(s + 3) * B, cols] = h
            st = state.setdefault(blk, {'h': {}})
            st['h'][half] = h
            for c in range(0, HK, 128):
                ht = h[:, c:c + 128]
                if 'h0' not in st:
                    st['h0'] = ht
                    continue
                d = ht - st['h0']
                new = (d, d * d, wmul(d, half * HK + c))
                st['s'] = new if 's' not in st else tuple(a + b for a, b in zip(st['s'], new))
            lag = _opt('SL', 2)
            if lag and len(st['h']) == 1:
                vals = [_or_all(list(v)) for v in zip(*[_vregs(a) for a in st['s']])]
                m = done[0] + lag
                for n, val in enumerate(vals):
                    ties[m][(248 - (n % 4) * 8, (n // 4) * 128)] = val

        _strassen(product, emit)

        res = []
        for blk in range(2):
            st = state[blk]
            s1, s2, s3 = st['s']
            c0 = _lanes(jnp.mean(st['h0'], axis=-1, keepdims=True))
            g0 = st['h0'] - c0
            t1 = s1 + 8.0 * g0
            t2 = s2 + g0 * (s1 + t1)
            t3 = s3 + wmul(g0, D + 128)
            res.append((jnp.concatenate([t1, t2, t3, c0], axis=1),
                        jnp.concatenate([st['h'][0], st['h'][1]], axis=1)))
        return res

    def stage_stats(views, s, part, valid=None):
        st_g, g = views[3], views[4]
        b = g * BPI + s
        bv = bestv_v[...]
        bi = besti_v[...]
        wsum = wrb_v[0:1, D:D + 128]
        nvs, nis, sts = [], [], []
        for k in range(B // R):
            sl = slice(k * R, (k + 1) * R)
            red = [_lanes(jnp.sum(part[sl, n * 128:(n + 1) * 128], axis=-1, keepdims=True)) for n in range(3)]
            mu = red[0] * (1.0 / D)
            var = jnp.maximum(red[1] * (1.0 / D) - mu * mu, 0.0)
            rs = lax.rsqrt(var + LN_EPS)
            r = (red[2] - mu * wsum) * rs
            sts.append(jnp.concatenate([rs, (mu + part[sl, 384:512]) * rs], axis=1))
            if valid is not None:
                r = jnp.where(valid, r, -jnp.inf)
            idx = lax.broadcasted_iota(jnp.int32, (R, 128), 0) + (b * B + k * R)
            better = r > bv[sl]
            nvs.append(jnp.where(better, r, bv[sl]))
            nis.append(jnp.where(better, idx, bi[sl]))
        st = jnp.concatenate(sts, axis=0)
        st_g[(s + 2) * B:(s + 3) * B, :] = st
        bestv_v[...] = jnp.concatenate(nvs, axis=0)
        besti_v[...] = jnp.concatenate(nis, axis=0)
        return st, nvs

    def stage_out(views, s, st=None, h=None):
        h_g, out_g, st_g = views[1], views[2], views[3]
        rows = slice((s + 2) * B, (s + 3) * B)
        h = h_g[rows, :] if h is None else h
        st = st_g[rows, :] if st is None else st
        outs = []
        for k in range(B // R):
            sl = slice(k * R, (k + 1) * R)
            a = 1.0 + st[sl, 0:128]
            outs.append(jnp.concatenate([h[sl, c * 128:(c + 1) * 128] * a - st[sl, 128:256]
                                         for c in range(D // 128)], axis=1))
        out_g[rows, :] = jnp.concatenate([o.astype(bf16) for o in outs], axis=0)
        return [_vregs(o) for o in outs]

    def stage_i(views, s, part, h=None, valid=None):
        st, nvs = stage_stats(views, s, part, valid)
        return [o + _vregs(nv) for o, nv in zip(stage_out(views, s, st, h), nvs)]

    def p2_body(i, c):
        b0 = i * BPI
        keep = flag_s[0] > 0
        cur = views_of(i)
        pieces = stage_out(cur, -2) + stage_i(cur, -1, pend_v[...], valid=i > 0)
        for q in range(2):
            stage_q(xs_view((i + NT - 1) % NT + 1, 1), q, keep, None)
        stage_g(0)
        stage_g(1)
        res = stage_h(cur, 0, keep, pieces)
        pieces = stage_i(cur, 0, *res[0]) + stage_i(cur, 1, *res[1])
        res = stage_h(cur, 1, keep, pieces)
        stage_stats(cur, BPI - 2, res[0][0])
        pend_v[...] = res[1][0]

        @pl.when(i > 0)
        def _():
            cp_out(jnp.maximum(b0 - 2, 0), 2).start()

        cp_out(b0, 2).start()
        return c

    lax.fori_loop(0, NI, p2_body, 0)
    cp_wg.wait()
    cp_wu.wait()
    stage_out(views_of(NI - 1), BPI - 2)
    stage_i(views_of(NI - 1), BPI - 1, pend_v[...])
    cp_out(NB - 2, 2).start()

    keep = flag_s[0] > 0
    bv = bestv_v[...]
    mval = jnp.max(bv, axis=0, keepdims=True)
    sel = jnp.min(jnp.where(bv == mval, besti_v[...], S - 1), axis=0, keepdims=True)
    idx = sel[0, 0]
    hrow = h_v[pl.ds(P2 + idx, 1), :]
    strow = st_v[pl.ds(P2 + idx, 1), :]
    xrow = jnp.concatenate([hrow[:, c * 128:(c + 1) * 128] * strow[:, 0:128] - strow[:, 128:256]
                            for c in range(D // 128)], axis=1).astype(bf16)
    xs = jnp.broadcast_to(xrow, (16, D))

    def act(g, u):
        a = g * pl.reciprocal(1.0 + jnp.exp(-g), approx=True) * u
        return jnp.concatenate([a, a], axis=0).astype(bf16)

    def down(a, lo, w):
        return _dot_nn(a, _upk(wdp_v[lo // 2:(lo + w) // 2, 0:D]))[0:8]

    NM = F - NBV * 128
    xcol = jnp.broadcast_to(xrow.astype(f32), (128, D)).T
    jobs = [(which, b) for b in range(NBV) for which in (0, 1)]
    vres, prev = {}, None
    for j0 in range(0, len(jobs), NCH):
        grp = jobs[j0:j0 + NCH]
        accs = [None] * len(grp)
        for r in range(D // 16):
            for n, (which, b) in enumerate(grp):
                w = (wg_v, wu_v)[which][r * 16:(r + 1) * 16, NM + b * 128:NM + (b + 1) * 128].astype(f32)
                t0 = w[0:8] * xcol[r * 16:r * 16 + 8]
                t1 = w[8:16] * xcol[r * 16 + 8:r * 16 + 16]
                if accs[n] is None:
                    if prev is not None:
                        t0 = jnp.where(keep, t0, prev[n % len(prev)])
                    accs[n] = t0 + t1
                else:
                    accs[n] = (accs[n] + t0) + t1
        prev = accs
        for n, job in enumerate(grp):
            vres[job] = _allreduce8(accs[n][None], jnp.add)[0]

    chunks = [(lo, min(FC, NM - lo)) for lo in range(0, NM, FC)]
    acts, y = [], None
    for k, (lo, w) in enumerate(chunks):
        g = _dot_nn(xs, wg_v[:, lo:lo + w])
        u = _dot_nn(xs, wu_v[:, lo:lo + w])
        acts.append(act(g[0:8], u[0:8]))
        if k >= 1:
            t = down(acts[k - 1], *chunks[k - 1])
            y = t if y is None else y + t
    y = y + down(acts[-1], *chunks[-1])
    for b0, nb in ((0, 4), (4, 4), (8, 3), (11, 1)):
        g = jnp.concatenate([vres[(0, b)] for b in range(b0, b0 + nb)], axis=1)
        u = jnp.concatenate([vres[(1, b)] for b in range(b0, b0 + nb)], axis=1)
        y = y + down(act(g, u), NM + b0 * 128, nb * 128)

    gate = jnp.broadcast_to(jax.nn.sigmoid(mval), (8, 128))
    base = pl.multiple_of((idx >> 4) << 4, 16)
    rows = pl.ds(pl.multiple_of(P2 + base, 16), 16)
    h16 = h_v[rows, :]
    st16 = st_v[rows, :]
    a16 = 1.0 + st16[:, 0:128]
    m16 = st16[:, 128:256]
    hit = (lax.broadcasted_iota(jnp.int32, (16, 128), 0) + base) == idx
    res = []
    for c in range(D // 128):
        yc = y[:, c * 128:(c + 1) * 128] * gate
        yc = jnp.concatenate([yc, yc], axis=0)
        res.append(h16[:, c * 128:(c + 1) * 128] * a16 - m16 + jnp.where(hit, yc, 0.0))
    res = jnp.concatenate(res, axis=1).astype(bf16)
    for i in range(NI):
        cp_out(i * BPI, 2).wait()
        cp_out(i * BPI + 2, 2).wait()
    out_v[rows, :] = res
    fix = pltpu.make_async_copy(out_v.at[rows], out_hbm.at[pl.ds(base, 16)], sem_o.at[0])
    fix.start()
    fix.wait()


@jax.jit
def pallas_sequential_preLN__linear_kernel_hedgehog__moe_arch_mod__prompt_kernel(
    A_x: jax.Array,
    A_wqkv: jax.Array,
    A_w_phi: jax.Array,
    A_wo: jax.Array,
    B_x: jax.Array,
    B_w_r: jax.Array,
    B_w_gate: jax.Array,
    B_w_up: jax.Array,
    B_w_down: jax.Array,
):
    del B_x
    x = A_x.reshape(S, D)
    wphi = A_w_phi.reshape(H * DH, DH)
    wr = B_w_r.reshape(8, 128)
    any_spec = pl.BlockSpec(memory_space=pl.ANY)
    out = pl.pallas_call(
        _kernel,
        out_shape=jax.ShapeDtypeStruct((S, D), bf16),
        in_specs=[any_spec] * 8,
        out_specs=any_spec,
        scratch_shapes=[
            pltpu.VMEM((S, D), bf16),
            pltpu.VMEM((D, 3 * D), bf16),
            pltpu.VMEM((H * DH, DH), bf16),
            pltpu.VMEM((D, D), bf16),
            pltpu.VMEM((8, 128), bf16),
            pltpu.VMEM((D, F + 128), bf16),
            pltpu.VMEM((D, F + 128), bf16),
            pltpu.VMEM((F, D), bf16),
            pltpu.VMEM((PR, D), u32),
            pltpu.VMEM((D // 2, D), u32),
            pltpu.VMEM((PR // 2, 7 * HK), u32),
            pltpu.VMEM((PR // 2, 7 * HK), u32),
            pltpu.VMEM((D // 4, 7 * HK), u32),
            pltpu.VMEM((D // 4, 7 * HK), u32),
            pltpu.VMEM((F // 2, D + 128), u32),
            pltpu.VMEM((64, 8 * 128), u32),
            pltpu.VMEM((T // 2, D), u32),
            pltpu.VMEM(((S + T) // 4, 7 * HK), u32),
            pltpu.VMEM((NP, 64, 128), f32),
            pltpu.VMEM((2 * D, 128), f32),
            pltpu.VMEM((32, NP * 128), u32),
            pltpu.VMEM((D, T), u32),
            pltpu.VMEM((D // 2, 2 * B), u32),
            pltpu.VMEM((D // 2, 2 * B), u32),
            pltpu.VMEM((D // 2, 2 * B), u32),
            pltpu.VMEM((D // 2, 2 * B), u32),
            pltpu.VMEM((HK // 2, 7 * B), u32),
            pltpu.VMEM((HK // 2, 7 * B), u32),
            pltpu.VMEM((P2 + S, D), f32),
            pltpu.VMEM((P2 + S, 256), f32),
            pltpu.VMEM((B, 512), f32),
            pltpu.VMEM((P2 + S, D), bf16),
            pltpu.VMEM((8, D + 256), f32),
            pltpu.VMEM((B, 128), f32),
            pltpu.VMEM((B, 128), jnp.int32),
            pltpu.SMEM((2,), jnp.int32),
            pltpu.SemaphoreType.DMA((_NSEM_IN,)),
            pltpu.SemaphoreType.DMA((1,)),
        ],
        compiler_params=pltpu.CompilerParams(vmem_limit_bytes=110 * 1024 * 1024,
                                             disable_bounds_checks=True,
                                             disable_semaphore_checks=True),
        name="hedgehog_mod",
    )(x, A_wqkv, wphi, A_wo, wr, B_w_gate, B_w_up, B_w_down)
    return out.reshape(1, S, D)
```

```python
import os
import jax
import jax.numpy as jnp
from jax import lax
import jax.experimental.pallas as pl
import jax.experimental.pallas.tpu as pltpu

S = 2048
D = 1024
H = 32
DH = 32
F = 3584
T = 512
NT = S // T
T0 = 256
B = 128
NB = S // B
BPI = 4
NI = NB // BPI
NP = H // 2
FC = 512
R = 16
NBV = 12
NCH = 4
OCH = 176
DCH = 1200
NV = 124
PR = NV * 4
HK = D // 2
P2 = 2 * B
LOG2E = 1.4426950408889634
LN_EPS = 1e-5
DEN_EPS = 1e-6

_NT_DIMS = (((1,), (1,)), ((), ()))
_TN_DIMS = (((0,), (0,)), ((), ()))

bf16 = jnp.bfloat16
f32 = jnp.float32
u32 = jnp.uint32


def _opt(name, default):
    return type(default)(os.environ.get(name, default))


def _dot_nt(a, b):
    return lax.dot_general(a, b, _NT_DIMS, preferred_element_type=f32)


def _dot_nn(a, b):
    return jnp.dot(a, b, preferred_element_type=f32)


def _pk(x):
    return pltpu.bitcast(x, u32)


def _upk(x):
    return pltpu.bitcast(x, bf16)


def _lanes(x):
    return jnp.broadcast_to(x, (x.shape[0], 128))


def _layernorm(x):
    m = jnp.mean(x, axis=-1, keepdims=True)
    xc = x - m
    v = jnp.mean(xc * xc, axis=-1, keepdims=True)
    return xc * lax.rsqrt(v + LN_EPS)


def _allreduce8(x, op):
    x = op(x, pltpu.roll(x, 4, 1))
    x = op(x, pltpu.roll(x, 2, 1))
    x = op(x, pltpu.roll(x, 1, 1))
    return x


def _hedgehog_t(p, z=None):
    t = p.shape[-1]
    p4 = p.reshape(2, 4, 8, t)
    mx = _allreduce8(jnp.max(p4, axis=1), jnp.maximum)
    mn = _allreduce8(jnp.min(p4, axis=1), jnp.minimum)
    ep = jnp.exp2(p4 - mx[:, None])
    en = jnp.exp2(mn[:, None] - p4)
    a = pl.reciprocal(_allreduce8(jnp.sum(ep, axis=1), jnp.add), approx=True)
    b = pl.reciprocal(_allreduce8(jnp.sum(en, axis=1), jnp.add), approx=True)
    if z is not None:
        dp = jnp.sum(ep * z[0:64].reshape(2, 4, 8, t), axis=1)
        dn = jnp.sum(en * z[64:128].reshape(2, 4, 8, t), axis=1)
        den = _allreduce8(dp * a + dn * b, jnp.add) + DEN_EPS
        inv = pl.reciprocal(den, approx=True)
        a = a * inv
        b = b * inv
    fp = (ep * a[:, None]).reshape(64, t)
    fn = (en * b[:, None]).reshape(64, t)
    return jnp.concatenate([fp, fn], axis=0)


_SA = ((3, None, 0), (2, 3, 1), (0, 1, 1), (0, None, 0), (0, 3, 1), (1, 3, -1), (2, 0, -1))
_SB = ((2, 0, -1), (0, None, 0), (3, None, 0), (1, 3, -1), (0, 3, 1), (2, 3, 1), (0, 1, 1))


def _combo(blocks, spec):
    a, b, sign = spec
    if b is None:
        return blocks[a]
    return blocks[a] + blocks[b] if sign > 0 else blocks[a] - blocks[b]


def _strassen(product, emit):
    m4 = product(0)
    m2 = product(1)
    emit(2, m4 + m2)
    m5 = product(2)
    u = m4 - m5
    m3 = product(3)
    emit(1, m5 + m3)
    v = m3 - m2
    m1 = product(4)
    u = u + m1
    v = v + m1
    emit(0, u + product(5))
    emit(3, v + product(6))


def _head_groups(h):
    base, k = (NV // 4) * (h // 8), h % 8
    return ([base + 4 * k + i for i in range(3)],
            base + 4 * k - 1 if k > 0 else None,
            base + 4 * k + 3 if k < 7 else None,
            8 - k)


def _pair_logits(group, j):
    parts = []
    for h in (2 * j, 2 * j + 1):
        full, below, above, a = _head_groups(h)
        ref = group(full[0])
        sub = lax.broadcasted_iota(jnp.int32, ref.shape, 0)
        if above is None:
            m = jnp.where(sub >= a, group(below), 0.0)
        else:
            m = jnp.where(sub == a - 1, 0.0, group(above))
            if below is not None:
                m = jnp.where(sub >= a, group(below), m)
        parts += [m] + [group(q) for q in full]
    return jnp.concatenate(parts, axis=0)


def _pair_need(j):
    full, _, above, _ = _head_groups(2 * j + 1)
    return full[2] if above is None else above


def _tie(keep, w, ties):
    rows = sorted({r for r, _ in ties})
    out, pos = [], 0
    for r in rows:
        if r > pos:
            out.append(w[pos:r])
        cols = sorted(c for rr, c in ties if rr == r)
        parts, cpos = [], 0
        for c in cols:
            if c > cpos:
                parts.append(w[r:r + 8, cpos:c])
            parts.append(jnp.where(keep, w[r:r + 8, c:c + 128], ties[(r, c)]))
            cpos = c + 128
        if cpos < w.shape[1]:
            parts.append(w[r:r + 8, cpos:])
        out.append(jnp.concatenate(parts, axis=1) if len(parts) > 1 else parts[0])
        pos = r + 8
    if pos < w.shape[0]:
        out.append(w[pos:])
    return jnp.concatenate(out, axis=0)


def _vregs(x):
    if x.dtype != u32:
        x = pltpu.bitcast(x, u32)
    return [x[r:r + 8, c:c + 128] for r in range(0, x.shape[0], 8) for c in range(0, x.shape[1], 128)]


def _or_all(vals):
    acc = vals[0]
    for v in vals[1:]:
        acc = acc | v
    return acc


_KSTAGES = (((0, 1), (4, 1)), ((1, 2), (5, 1)), ((3, 1), (6, 2)))
_PSTAGES = (((0, 1), (4, 1)), ((1, 3), (5, 3)))
_NSEM_IN = 12


def _kernel(x_hbm, wqkv_hbm, wphi_hbm, wo_hbm, wr_hbm, wg_hbm, wu_hbm, wd_hbm,
            out_hbm,
            x_v, wqkv_v, wphi_v, wo_v, wr_v, wg_v, wu_v, wd_v,
            wtk_v, wsq_v, wsk_v, wsv_v, wso_v, wdp_v, amat_v, xn_v, xs_v, kvacc_v, zacc_v, kv_v, phi_v,
            pq0_v, pq1_v, pq2_v, pq3_v, oc0_v, oc1_v, h_v, st_v, pend_v, out_v, wrb_v,
            bestv_v, besti_v, flag_s,
            sem_i, sem_o):

    def cp_x(lo, n, sem):
        return pltpu.make_async_copy(x_hbm.at[pl.ds(lo, n)], x_v.at[pl.ds(lo, n)], sem_i.at[sem])

    def cp_w(lo, w, sem):
        return pltpu.make_async_copy(wqkv_hbm.at[:, pl.ds(lo, w)], wqkv_v.at[:, pl.ds(lo, w)], sem_i.at[sem])

    cp_k = [[cp_w(D + g * 128, n * 128, 2 + c) for g, n in st] for c, st in enumerate(_KSTAGES)]
    cp_p = [[pltpu.make_async_copy(wphi_hbm.at[pl.ds(g * 128, n * 128)], wphi_v.at[pl.ds(g * 128, n * 128)],
                                   sem_i.at[3 * c]) for g, n in st] for c, st in enumerate(_PSTAGES)]
    cp_wv = cp_w(2 * D, D, 5)
    cp_wq = cp_w(0, D, 7)

    def cp_wd(k):
        lo, n = k * DCH, min(DCH, F - k * DCH)
        return pltpu.make_async_copy(wd_hbm.at[pl.ds(lo, n)], wd_v.at[pl.ds(lo, n)], sem_i.at[(6, 8, 9)[k]])

    cp_x0 = cp_x(0, T0, 1)
    cp_x1 = cp_x(T0, T0, 4)
    cp_x2 = cp_x(T, T, 11)
    cp_x3 = cp_x(2 * T, T, 6)
    cp_x4 = cp_x(3 * T, T, 8)
    cp_wr = pltpu.make_async_copy(wr_hbm, wr_v, sem_i.at[7])

    def cp_wo(k, half):
        lo, n = k * OCH, min(OCH, HK - k * OCH)
        rows = pl.ds(half * HK + lo, n)
        return pltpu.make_async_copy(wo_hbm.at[rows], wo_v.at[rows], sem_i.at[(6, 8, 9)[k]])

    def wait_bg(k):
        cp_wo(k, 0).wait()
        cp_wo(k, 1).wait()
        cp_wd(k).wait()

    cp_wg = pltpu.make_async_copy(wg_hbm, wg_v.at[:, pl.ds(0, F)], sem_i.at[10])
    cp_wu = pltpu.make_async_copy(wu_hbm, wu_v.at[:, pl.ds(0, F)], sem_i.at[10])

    def cp_out(b, n):
        lo = b * B
        if not isinstance(b, int):
            lo = pl.multiple_of(lo, B)
        return pltpu.make_async_copy(out_v.at[pl.ds(P2 + lo, n * B)], out_hbm.at[pl.ds(lo, n * B)], sem_o.at[0])

    for cp in (*cp_p[0], cp_x0, *cp_k[0], *cp_p[1], *cp_k[1], *cp_k[2], cp_x1, cp_wv, cp_x2,
               cp_x3, cp_wo(0, 0), cp_wo(0, 1), cp_wd(0), cp_x4, cp_wo(1, 0), cp_wo(1, 1), cp_wd(1),
               cp_wo(2, 0), cp_wo(2, 1), cp_wd(2), cp_wr, cp_wq, cp_wg, cp_wu):
        cp.start()
    flag_s[0] = 1
    flag_s[1] = 0

    def ln1(xg, src, xd, dst, n, which=None, keep=None, anchors=None, plain=False, split=False):
        pieces = []
        for pr in range(n // P2):
            for k in range(B // R):
                off = pr * P2 + k * R
                if which is not None and pr * (B // R) + k not in which:
                    continue
                x0 = xg[src + off:src + off + R, :].astype(f32)
                x1 = xg[src + off + B:src + off + B + R, :].astype(f32)
                if anchors is not None:
                    a = anchors[len(pieces)]
                    x0 = jnp.concatenate([jnp.where(keep, x0[:, :128], a), x0[:, 128:]], axis=1)
                    x1 = jnp.concatenate([jnp.where(keep, x1[:, :128], a), x1[:, 128:]], axis=1)
                p0 = _layernorm(x0)
                p1 = _layernorm(x1)
                if plain:
                    xn_v[off // 2:(off + R) // 2, :] = _pk(p0.astype(bf16))
                    xn_v[(off + B) // 2:(off + B + R) // 2, :] = _pk(p1.astype(bf16))
                lo = (dst + pr * P2) // 4 + k * (R // 2)
                blocks = (p0[:, :HK], p1[:, :HK], p0[:, HK:], p1[:, HK:])
                vs = []
                for m, spec in enumerate(_SB):
                    t = _combo(blocks, spec)
                    xd[lo:lo + R // 2, m * HK:(m + 1) * HK] = _pk(t.astype(bf16))
                    if spec[1] is not None:
                        vs.append(_vregs(t))
                if split:
                    pieces.append((vs[0], vs[1], [_or_all(list(col)) for col in zip(*vs[2:])]))
                else:
                    pieces.append([_or_all(list(col)) for col in zip(*vs)])
        return pieces

    def load_xn(b):
        return _upk(xn_v[b * (B // 2):(b + 1) * (B // 2), :])

    def piece_ties(pieces, n, row0=0, col=0):
        ties = {}
        if pieces:
            step = (n - row0) // len(pieces) // 8 * 8
            for k, p in enumerate(pieces):
                for q, val in enumerate(p):
                    ties[(row0 + k * step + (q // 4) * 8, col + (q % 4) * 128)] = val
        return ties

    def xs_view(i, tiles):
        return xs_v.at[pl.ds(pl.multiple_of(i * (T // 4), T // 4), tiles * (T // 4))]

    def sproj(ws, xd, pr, emit, keep=None, work=None, before=None, after=None):
        lo = pr * (B // 2)

        def product(m):
            if before:
                before(m)
            lhs = ws[:, m * HK:(m + 1) * HK]
            if work and work.get(m):
                lhs = _tie(keep, lhs, piece_ties(work[m], lhs.shape[0], 32))
            res = _dot_nt(_upk(lhs), _upk(xd[lo:lo + B // 2, m * HK:(m + 1) * HK]))
            if after:
                after(m, res)
            return res

        _strassen(product, lambda k, val: emit(k // 2, k % 2, val))

    def spread(pieces, slots):
        res = {}
        for k, (pr, m) in enumerate(slots):
            res.setdefault(pr, {})[m] = pieces[k * len(pieces) // len(slots):(k + 1) * len(pieces) // len(slots)]
        return res

    def fence(ref, row, col):
        return ref[pl.ds(pl.multiple_of(flag_s[1] + row, 8), 8), col:col + 128]

    def store_combos(ws, row, top, bot, table=_SA, keep=None, dep=None, every=1):
        for n, c in enumerate(range(0, HK, 128)):
            raw = [top[:, c:c + 128], top[:, HK + c:HK + c + 128], bot[:, c:c + 128], bot[:, HK + c:HK + c + 128]]
            if keep is not None and dep is not None:
                for q in (0, 3):
                    d = dep if raw[q].dtype == u32 else pltpu.bitcast(jnp.concatenate([dep, dep], axis=0), f32)
                    raw[q] = jnp.where(keep, raw[q], d)
            blocks = [_upk(b).astype(f32) if b.dtype == u32 else b for b in raw]
            for m, spec in enumerate(table):
                t = raw[spec[0]] if spec[1] is None else _combo(blocks, spec)
                ws[row:row + 8, m * HK + c:m * HK + c + 128] = t if t.dtype == u32 else _pk(t.astype(bf16))
            if keep is not None and (n + 1) % every == 0:
                dep = fence(ws, row, c)
        return dep if keep is not None else fence(ws, row, 0)

    def k_side(group, pairs, first, slot=None, keep=None, anchor=None):
        res = []
        for j in pairs:
            p = _pair_logits(group, j)
            if anchor is not None:
                p = jnp.concatenate([jnp.where(keep, p[0:8], anchor), p[8:32],
                                     jnp.where(keep, p[32:40], anchor), p[40:64]], axis=0)
            ph = _hedgehog_t(p)
            if first:
                zacc_v[j * 128:(j + 1) * 128, :] = ph
            else:
                zacc_v[j * 128:(j + 1) * 128, :] += ph
            if slot is not None:
                phi_v[j * 64:(j + 1) * 64, slot * B:(slot + 1) * B] = _pk(ph.astype(bf16))
            res.append(ph)
        return res

    def half_groups(p, half):
        return lambda pos: p[(pos - half * (NV // 2)) * 8:(pos - half * (NV // 2) + 1) * 8]

    def half_pairs(half):
        return range(half * (NP // 2), (half + 1) * (NP // 2))

    def kv_prod(vt, ph, j):
        half, r = j // (NP // 2), (j % (NP // 2)) * 64
        v = jnp.concatenate([vt[(s, half)][r:r + 64] for s in range(T // B)], axis=1).astype(bf16)
        return _dot_nt(v, ph)

    def v_side(xd, keep, pieces, chain):
        work = spread(pieces, [(0, m) for m in range(1, 7)] + [(1, m) for m in range(6)])
        vt = {}
        for q in range(T // P2):
            sproj(wsv_v, xd, q, lambda half, blk, val, q=q: vt.__setitem__((2 * q + blk, half), val),
                  keep, work.get(q))
            if q == 0:
                m = _opt('OM', 2)
                work[1][m] = list(work[1].get(m, [])) + [[chain(pltpu.bitcast(vt[(0, 1)][0:8], u32))]]
        return vt

    r_i = lax.broadcasted_iota(jnp.int32, (128, DH), 0)
    c_i = lax.broadcasted_iota(jnp.int32, (128, DH), 1)
    expand = (r_i % DH == c_i).astype(bf16)
    r_h = lax.broadcasted_iota(jnp.int32, (128, 128), 0) // DH
    c_h = lax.broadcasted_iota(jnp.int32, (128, 128), 1) // DH
    same_head = r_h == c_h

    def make_amat(g):
        a = _dot_nt(expand, wphi_v[g * 128:(g + 1) * 128, :])
        amat_v[:, g * 128:(g + 1) * 128] = _pk(jnp.where(same_head, a, 0.0).astype(bf16))

    class Folder:
        def __init__(self, col0, first=0):
            self.col0, self.rows, self.mprev, self.done = col0, {}, None, first

        def tile(self, g, rows, keep=None, ties=None):
            am = amat_v[:, g * 128:(g + 1) * 128]
            if ties:
                am = _tie(keep, am, ties)
            return _dot_nt(_upk(am), wqkv_v[rows, self.col0 + g * 128:self.col0 + (g + 1) * 128])

        def fold(self, g, wt=None):
            sub = lax.broadcasted_iota(jnp.int32, (8, D), 0)
            if wt is None:
                wt = self.tile(g, slice(None))
            for hh in range(4):
                full, below, _, a = _head_groups(4 * g + hh)
                r0 = hh * DH
                ref = jnp.broadcast_to(wt[r0 + a - 1:r0 + a, :], (8, D))
                part = [(wt[r0 + 8 * i:r0 + 8 * (i + 1)] - ref) * LOG2E for i in range(4)]
                if below is not None:
                    self.rows[below] = jnp.where(sub >= a, part[0], self.mprev)
                self.mprev = part[0]
                for q, v in zip(full, part[1:]):
                    self.rows[q] = v
            new = {}
            while self.done in self.rows and self.done + 1 in self.rows:
                new[self.done] = jnp.concatenate([self.rows.pop(self.done), self.rows.pop(self.done + 1)], axis=0)
                self.done += 2
            return new

    def fold_pair(folders, g, keep=None, ties=None):
        tiles = {}
        for n, c in enumerate(range(0, HK, 128)):
            for half in range(2):
                for side in range(2):
                    t = ties[n] if ties and half == 0 and side == 0 else None
                    lo = side * HK + c
                    tiles[(half, lo)] = folders[half].tile(g + 4 * half, slice(lo, lo + 128), keep, t)
        return [folders[half].fold(g + 4 * half,
                                   jnp.concatenate([tiles[(half, lo)] for lo in range(0, D, 128)], axis=1))
                for half in range(2)]

    bestv_v[...] = jnp.full(bestv_v.shape, -jnp.inf, f32)
    besti_v[...] = lax.broadcasted_iota(jnp.int32, besti_v.shape, 0)
    h_v[0:P2, :] = jnp.zeros((P2, D), f32)
    st_v[0:B, :] = jnp.zeros((B, 256), f32)
    pend_v[...] = jnp.zeros(pend_v.shape, f32)

    def wait_all(cps):
        for cp in cps:
            cp.wait()

    def amats(c):
        for g0, n in _PSTAGES[c]:
            for g in range(g0, g0 + n):
                make_amat(g)

    wait_all(cp_p[0])
    amats(0)

    cp_x0.wait()
    ln1(x_v, 0, xs_v, 0, T0, plain=True)
    xb = [load_xn(s) for s in range(2)]
    logits = [{}, {}]
    finished = [set(), set()]
    fk, slabs = (Folder(D), Folder(D, NV // 2)), {}
    defer, queue = [False], []

    def absorb(new):
        for pos, slab in new.items():
            wtk_v[pos * 4:pos * 4 + 8, :] = _pk(slab.astype(bf16))
            slabs[pos] = slab
        for pos in sorted(slabs):
            if pos < NV // 2 and pos + NV // 2 in slabs:
                store_combos(wsk_v, pos * 4, slabs.pop(pos), slabs.pop(pos + NV // 2))

    def k_finish(s, hold=0):
        ready = [j for j in range(NP) if j not in finished[s] and _pair_need(j) in logits[s]]
        ready = ready[:len(ready) - hold]
        if defer[0]:
            queue.extend((logits[s].__getitem__, [j], s == 0, s) for j in ready)
        else:
            k_side(logits[s].__getitem__, ready, s == 0, s)
        finished[s].update(ready)

    def k_chunk(s, keep=None, early=(), late=(), hold=0):
        todo = [q for half in range(2) for q in range(half * (NV // 2), fk[half].done) if q not in logits[s]]
        runs = [[q for q in todo if q < NV // 2], [q for q in todo if q >= NV // 2]]
        lhs = jnp.concatenate([wtk_v[r[0] * 4:(r[-1] + 1) * 4, :] for r in runs if r], axis=0)
        ties = piece_ties(early, lhs.shape[0])
        ties.update(piece_ties(late, lhs.shape[0], col=HK))
        if ties:
            lhs = _tie(keep, lhs, ties)
        p = _dot_nt(_upk(lhs), xb[s])
        for n, q in enumerate(todo):
            logits[s][q] = p[n * 8:(n + 1) * 8]
        k_finish(s, hold)
        return p

    HOLD = _opt('HOLD', 1)
    wait_all(cp_k[0])
    for new in fold_pair(fk, 0):
        absorb(new)
    k_chunk(0)
    k_chunk(1, hold=HOLD)

    wait_all(cp_p[1] + cp_k[1])
    k_finish(1)
    amats(1)
    for new in fold_pair(fk, 1):
        absorb(new)
    absorb(fk[0].fold(2))
    k_chunk(0)
    k_chunk(1, hold=HOLD)

    wait_all(cp_k[2] + [cp_x1])
    defer[0] = True
    keep = flag_s[0] > 0
    w6 = fk[1].tile(6, slice(None))
    absorb(fk[1].fold(6, w6))
    new = fold_pair(fk, 3)
    top = list(new[0].values())
    for n in new:
        absorb(n)
    anc = [None, w6[0:R, 0:128], w6[64:64 + R, 512:640], top[0][:, 128:256], top[-1][:, 384:512]]
    A0 = [int(v) for v in _opt('A0', '0,4,4').split(',')]
    n0 = len(A0)
    pieces = [ln1(x_v, T0, xs_v, T0, T0, [k], keep, None if anc[a] is None else [anc[a]])[0] for k, a in enumerate(A0)]
    t0 = _opt('T0A', 2)
    p = k_chunk(0, keep, (), pieces[:t0])
    rows = [k * p.shape[0] // (8 - n0) // 16 * 16 for k in range(8 - n0)]
    pieces += ln1(x_v, T0, xs_v, T0, T0, list(range(n0, 8)), keep, [p[r:r + R] for r in rows])
    k_chunk(1, keep, pieces[t0:n0], pieces[n0:])
    NOW = _opt('NOW', 3)

    def k_emit1(half, blk, val):
        order = {(1, 0): 0, (0, 1): 1, (0, 0): 2, (1, 1): 3}[(half, blk)]
        queue.extend((half_groups(val, half), [j], False, 2 + blk) for j in half_pairs(half))

    def run_queue(n, res):
        for k in range(min(n, len(queue))):
            r = k * res.shape[0] // n // 8 * 8
            k_side(*queue.pop(0), keep=flag_s[0] > 0, anchor=res[r:r + 8])

    def k_after(m, res):
        if m < NOW:
            run_queue(_opt('NQ', 6), res)

    def v_prep():
        VL = _opt('VL', 0)
        fences = []
        for rb in range(0, HK, 128):
            for c in range(0, HK, 128):
                raw = [wqkv_v[side * HK + c:side * HK + c + 128, 2 * D + half * HK + rb:2 * D + half * HK + rb + 128]
                       for half in range(2) for side in range(2)]
                if VL and len(fences) >= VL:
                    d = fences[len(fences) - VL]
                    raw = [_upk(_tie(keep, _pk(t), {(0, 0): d})) for t in raw]
                raw = [t.T for t in raw]
                blocks = [t.astype(f32) for t in raw]
                for m, spec in enumerate(_SA):
                    t = raw[spec[0]] if spec[1] is None else _combo(blocks, spec).astype(bf16)
                    wsv_v[rb // 2:rb // 2 + 64, m * HK + c:m * HK + c + 128] = _pk(t)
                if VL:
                    fences.append(fence(wsv_v, rb // 2, c))

    def k_before(m):
        if m == 4:
            cp_wv.wait()
            v_prep()

    sproj(wsk_v.at[pl.ds(pl.multiple_of(flag_s[1], 8), PR // 2)] if _opt('KO', 0) else wsk_v, xs_v, 1, k_emit1, keep, None, k_before, k_after)

    vt = {}
    wsv = wsv_v.at[pl.ds(pl.multiple_of(flag_s[1], D // 4), D // 4)] if _opt('VO', 1) else wsv_v
    XW = _opt('XW', 5)
    work = {0: {}, 1: {}}
    slots = [(0, m) for m in range(XW, 7)] + [(1, m) for m in range(6)]

    def v_before(m):
        if m == XW:
            cp_x2.wait()

    def v_after(q):
        def after(m, res):
            left = _opt('QE', 4) - (7 * q + m)
            if left > 0 and not (q == 0 and m == XW - 1):
                run_queue(-(-len(queue) // left), res)
            if (q, m) in slots:
                k = slots.index((q, m))
                which = list(range(k * 16 // len(slots), (k + 1) * 16 // len(slots)))
                rows = [n * HK // len(which) // 16 * 16 for n in range(len(which))]
                nq, nm = (q, m + 1) if m < 6 else (q + 1, 0)
                pcs = ln1(x_v, T, xs_v, T, T, which, flag_s[0] > 0, [res[r:r + R] for r in rows])
                work[nq][nm] = [[]] * (2 - len(pcs) + 1) + pcs if _opt('LD', 1) else pcs
        return after

    for q in range(2):
        sproj(wsv, xs_v, q, lambda half, blk, val, q=q: vt.__setitem__((2 * q + blk, half), val),
              keep, work[q], v_before if q == 0 else None, v_after(q))
    assert not queue
    phi_m = phi_v.at[pl.ds(pl.multiple_of(flag_s[1], D), D)]
    for j in range(NP):
        kvacc_v[j] = kv_prod(vt, _upk(phi_m[j * 64:(j + 1) * 64, :]), j)
    cp_x3.wait()
    wait_bg(0)

    def p1_body(i, c):
        @pl.when(i == 2)
        def _():
            cp_x4.wait()
            wait_bg(1)

        @pl.when(i == 3)
        def _():
            wait_bg(2)

        keep = flag_s[0] > 0
        lo = jnp.minimum((i - 1) * DCH, F - DCH)
        sv = wd_v.at[pl.ds(pl.multiple_of(lo, 16), DCH)]
        dv = wdp_v.at[pl.ds(pl.multiple_of(lo // 2, 8), DCH // 2)]
        deps = []
        for r in range(0, DCH, 16):
            val = _pk(sv[r:r + 16, :])
            dv[r // 2:r // 2 + 8, 0:D] = val
            deps.append([_or_all(_vregs(val))])
        lo = jnp.minimum((i - 1) * OCH, HK - OCH)
        ov = wo_v.at[pl.ds(pl.multiple_of(lo, 16), HK + OCH)]
        od = wso_v.at[pl.ds(pl.multiple_of(lo // 2, 8), OCH // 2)]
        work = spread(deps, [(q, m) for q in range(2) for m in (0, 2, 4)])

        phik = {}
        PK = _opt('PK', 1)

        def k_emit(q):
            def emit(half, blk, val):
                for j, ph in zip(half_pairs(half), k_side(half_groups(val, half), half_pairs(half), False, 2 * q + blk if PK else None)):
                    phik[(2 * q + blk, j)] = ph
            return emit

        xd = xs_view(i, 2)
        for q in range(T // P2):
            sproj(wsk_v, xd, q, k_emit(q), keep, work[q])
        xg = x_v.at[pl.ds(pl.multiple_of(jnp.minimum(i + 1, NT - 1) * T, T), T)]
        pieces = ln1(xg, 0, xd, T, T)

        def wo_chain(dep):
            for r in range(0, OCH, 16):
                dep = store_combos(od, r // 2, ov[r:r + 16, :].astype(f32), ov[HK + r:HK + r + 16, :].astype(f32),
                                   _SB, keep, dep)
            return dep

        vt = v_side(xd, keep, pieces, wo_chain)
        phi_m = phi_v.at[pl.ds(pl.multiple_of(flag_s[1], D), D)]
        for j in range(NP):
            if PK:
                ph = _upk(phi_m[j * 64:(j + 1) * 64, :])
            else:
                ph = jnp.concatenate([phik[(s, j)] for s in range(T // B)], axis=1).astype(bf16)
            kvacc_v[j] += kv_prod(vt, ph, j)
        return c

    lax.fori_loop(1, NT, p1_body, 0)

    cp_wr.wait()
    cp_wq.wait()
    keep = flag_s[0] > 0
    kv_mask = (lax.broadcasted_iota(jnp.int32, (64, 128), 0) // DH
               == (lax.broadcasted_iota(jnp.int32, (64, 128), 1) // DH) % 2)
    ties = [{} for _ in range(16)]
    for j in range(NP):
        kvj = jnp.where(kv_mask, kvacc_v[j], 0.0)
        kv_v[:, j * 128:(j + 1) * 128] = _pk(kvj.astype(bf16))
        zj = _lanes(jnp.sum(zacc_v[j * 128:(j + 1) * 128, :], axis=-1, keepdims=True))
        zacc_v[j * 128:(j + 1) * 128, :] = zj
        vals = _vregs(kvj) + _vregs(zj)
        b0 = _opt('BT', 1)
        if j + b0 < 16:
            for q in range(4):
                ties[j + b0][(32 + q * 8, 0)] = _or_all(vals[q::4])
    wr = wr_v[...].astype(f32)
    wl = jnp.sum(wr, axis=0, keepdims=True)
    wsum = jnp.sum(wl, axis=1, keepdims=True)
    wrb_v[...] = jnp.concatenate(
        [jnp.broadcast_to(wr[j:j + 1, :], (8, 128)) for j in range(8)]
        + [jnp.broadcast_to(wsum, (8, 128)), jnp.broadcast_to(wl, (8, 128))], axis=1)
    fq = (Folder(0), Folder(0, NV // 2))
    for g in range(4):
        new = fold_pair(fq, g, keep, ties[4 * g:4 * g + 4])
        for pos, slab in new[0].items():
            store_combos(wsq_v, pos * 4, slab, new[1][pos + NV // 2])

    pq_v = (pq0_v, pq1_v, pq2_v, pq3_v)

    def views_of(g):
        lo = g * (BPI * B)
        if not isinstance(g, int):
            lo = pl.multiple_of(lo, BPI * B)
        return ((x_v.at[pl.ds(lo, BPI * B)],)
                + tuple(ref.at[pl.ds(lo, P2 + BPI * B)] for ref in (h_v, out_v, st_v)) + (g,))

    def stage_q(xd, q, keep, work):
        def emit(half, blk, val):
            group = half_groups(val, half)
            for j in half_pairs(half):
                ph = _hedgehog_t(_pair_logits(group, j), zacc_v[j * 128:(j + 1) * 128, :])
                pq_v[2 * q + blk][(j // 2) * 64:(j // 2 + 1) * 64, (j % 2) * B:(j % 2 + 1) * B] = _pk(ph.astype(bf16))

        sproj(wsq_v, xd, q, emit, keep, work)

    oc_v = (oc0_v, oc1_v)

    def stage_g(q):
        pq = [pq_v[2 * q + blk].at[pl.ds(pl.multiple_of(flag_s[1], D // 2), D // 2)] for blk in range(2)]
        for jj in range(NP // 2):
            blocks = [_dot_nn(_upk(kv_v[:, j * 128:(j + 1) * 128]),
                              _upk(pq[blk][(j // 2) * 64:(j // 2 + 1) * 64, (j % 2) * B:(j % 2 + 1) * B]))
                      for blk in range(2) for j in (jj, jj + NP // 2)]
            for m, spec in enumerate(_SA):
                oc_v[q][jj * 32:(jj + 1) * 32, m * B:(m + 1) * B] = _pk(_combo(blocks, spec).astype(bf16))

    def stage_h(views, q, keep, pieces):
        x_g, h_g = views[0], views[1]
        oc = oc_v[q].at[pl.ds(pl.multiple_of(flag_s[1], HK // 2), HK // 2)]
        first, last = _opt('H0', 3), _opt('H1', 22)
        ties = [{} for _ in range(7)]
        for k, vals in enumerate(pieces):
            t = first + k * (last - first) // max(len(pieces) - 1, 1)
            for m, val in enumerate(vals):
                ties[t // 4][(m * 8, (t % 4) * 128)] = val
        state = {}
        done = [0]

        def product(m):
            w = wso_v[:, m * HK:(m + 1) * HK]
            if ties[m]:
                w = _tie(keep, w, ties[m])
            done[0] = m
            return lax.dot_general(_upk(oc[:, m * B:(m + 1) * B]), _upk(w), _TN_DIMS,
                                   preferred_element_type=f32)

        def wmul(d, lo):
            return (d.reshape(B // 8, 8, 128) * wrb_v[:, lo:lo + 128][None]).reshape(B, 128)

        def emit(k, val):
            blk, half = k // 2, k % 2
            s = 2 * q + blk
            cols = slice(half * HK, (half + 1) * HK)
            h = x_g[s * B:(s + 1) * B, cols].astype(f32) + val
            h_g[(s + 2) * B:(s + 3) * B, cols] = h
            st = state.setdefault(blk, {'h': {}})
            st['h'][half] = h
            for c in range(0, HK, 128):
                ht = h[:, c:c + 128]
                if 'h0' not in st:
                    st['h0'] = ht
                    continue
                d = ht - st['h0']
                new = (d, d * d, wmul(d, half * HK + c))
                st['s'] = new if 's' not in st else tuple(a + b for a, b in zip(st['s'], new))
            lag = _opt('SL', 2)
            if lag and len(st['h']) == 1:
                vals = [_or_all(list(v)) for v in zip(*[_vregs(a) for a in st['s']])]
                m = done[0] + lag
                for n, val in enumerate(vals):
                    ties[m][(248 - (n % 4) * 8, (n // 4) * 128)] = val

        _strassen(product, emit)

        res = []
        for blk in range(2):
            st = state[blk]
            s1, s2, s3 = st['s']
            c0 = _lanes(jnp.mean(st['h0'], axis=-1, keepdims=True))
            g0 = st['h0'] - c0
            t1 = s1 + 8.0 * g0
            t2 = s2 + g0 * (s1 + t1)
            t3 = s3 + wmul(g0, D + 128)
            res.append((jnp.concatenate([t1, t2, t3, c0], axis=1),
                        jnp.concatenate([st['h'][0], st['h'][1]], axis=1)))
        return res

    def stage_stats(views, s, part, valid=None, keep=None, after=None):
        st_g, g = views[3], views[4]
        b = g * BPI + s
        bv = bestv_v[...]
        bi = besti_v[...]
        if after is not None:
            bv = jnp.concatenate([bv[:B - R], jnp.where(keep, bv[B - R:], after)], axis=0)
        wsum = wrb_v[0:1, D:D + 128]
        nvs, nis, sts = [], [], []
        for k in range(B // R):
            sl = slice(k * R, (k + 1) * R)
            red = [_lanes(jnp.sum(part[sl, n * 128:(n + 1) * 128], axis=-1, keepdims=True)) for n in range(3)]
            mu = red[0] * (1.0 / D)
            var = jnp.maximum(red[1] * (1.0 / D) - mu * mu, 0.0)
            rs = lax.rsqrt(var + LN_EPS)
            r = (red[2] - mu * wsum) * rs
            sts.append(jnp.concatenate([rs, (mu + part[sl, 384:512]) * rs], axis=1))
            if valid is not None:
                r = jnp.where(valid, r, -jnp.inf)
            idx = lax.broadcasted_iota(jnp.int32, (R, 128), 0) + (b * B + k * R)
            better = r > bv[sl]
            nvs.append(jnp.where(better, r, bv[sl]))
            nis.append(jnp.where(better, idx, bi[sl]))
        st = jnp.concatenate(sts, axis=0)
        st_g[(s + 2) * B:(s + 3) * B, :] = st
        bestv_v[...] = jnp.concatenate(nvs, axis=0)
        besti_v[...] = jnp.concatenate(nis, axis=0)
        return st, nvs

    def stage_out(views, s, st=None, h=None):
        h_g, out_g, st_g = views[1], views[2], views[3]
        rows = slice((s + 2) * B, (s + 3) * B)
        h = h_g[rows, :] if h is None else h
        st = st_g[rows, :] if st is None else st
        outs = []
        for k in range(B // R):
            sl = slice(k * R, (k + 1) * R)
            a = 1.0 + st[sl, 0:128]
            outs.append(jnp.concatenate([h[sl, c * 128:(c + 1) * 128] * a - st[sl, 128:256]
                                         for c in range(D // 128)], axis=1))
        out_g[rows, :] = jnp.concatenate([o.astype(bf16) for o in outs], axis=0)
        return [_vregs(o) for o in outs]

    def stage_i(views, s, part, h=None, valid=None, keep=None, after=None):
        st, nvs = stage_stats(views, s, part, valid, keep, after)
        return [o + _vregs(nv) for o, nv in zip(stage_out(views, s, st, h), nvs)]

    def p2_body(i, c):
        b0 = i * BPI
        keep = flag_s[0] > 0
        cur = views_of(i)
        pieces = stage_out(cur, -2) + stage_i(cur, -1, pend_v[...], valid=i > 0)
        for q in range(2):
            stage_q(xs_view(i, 1), q, keep, None)
        stage_g(0)
        stage_g(1)
        res = stage_h(cur, 0, keep, pieces)
        pieces = stage_i(cur, 0, *res[0]) + stage_i(cur, 1, *res[1])
        res = stage_h(cur, 1, keep, pieces)
        stage_stats(cur, BPI - 2, res[0][0])
        pend_v[...] = res[1][0]

        @pl.when(i > 0)
        def _():
            cp_out(jnp.maximum(b0 - 2, 0), 2).start()

        cp_out(b0, 2).start()
        return c

    lax.fori_loop(0, NI, p2_body, 0)
    cp_wg.wait()
    cp_wu.wait()
    keep = flag_s[0] > 0
    last = views_of(NI - 1)

    def out_fence():
        return out_v[pl.ds(pl.multiple_of(flag_s[1] + S, R), R), 0:128].astype(f32)

    TM = _opt('TM', 1)
    if TM == 0:
        stage_out(last, BPI - 2)
        st, _ = stage_stats(last, BPI - 1, pend_v[...], keep=keep, after=out_fence())
    else:
        st, _ = stage_stats(last, BPI - 1, pend_v[...])

    bv = bestv_v[...]
    mval = jnp.max(bv, axis=0, keepdims=True)
    sel = jnp.min(jnp.where(bv == mval, besti_v[...], S - 1), axis=0, keepdims=True)
    idx = sel[0, 0]
    sel_f = jnp.broadcast_to(pltpu.bitcast(sel, f32), (B, 128))
    if TM == 1:
        st2 = last[3][BPI * B:(BPI + 1) * B, :]
        stage_out(last, BPI - 2, jnp.concatenate([jnp.where(keep, st2[:, 0:128], sel_f), st2[:, 128:256]], axis=1))
    stage_out(last, BPI - 1, jnp.concatenate([jnp.where(keep, st[:, 0:128], sel_f), st[:, 128:256]], axis=1))
    ofence = out_fence()
    cp_out(NB - 2, 2).start()
    hrow = h_v[pl.ds(P2 + idx, 1), :]
    strow = st_v[pl.ds(P2 + idx, 1), :]
    xrow = jnp.concatenate([hrow[:, c * 128:(c + 1) * 128] * strow[:, 0:128] - strow[:, 128:256]
                            for c in range(D // 128)], axis=1).astype(bf16)
    xs = jnp.broadcast_to(xrow, (16, D))

    def act(g, u):
        a = g * pl.reciprocal(1.0 + jnp.exp(-g), approx=True) * u
        return jnp.concatenate([a, a], axis=0).astype(bf16)

    def down(a, lo, w):
        return _dot_nn(a, _upk(wdp_v[lo // 2:(lo + w) // 2, 0:D]))[0:8]

    NM = F - NBV * 128
    xcol = jnp.broadcast_to(xrow.astype(f32), (128, D)).T
    jobs = [(which, b) for b in range(NBV) for which in (0, 1)]
    vres, prev = {}, None
    OF = _opt('OF', 40)
    for j0 in range(0, len(jobs), NCH):
        grp = jobs[j0:j0 + NCH]
        accs = [None] * len(grp)
        for r in range(D // 16):
            for n, (which, b) in enumerate(grp):
                w = (wg_v, wu_v)[which][r * 16:(r + 1) * 16, NM + b * 128:NM + (b + 1) * 128].astype(f32)
                t0 = w[0:8] * xcol[r * 16:r * 16 + 8]
                t1 = w[8:16] * xcol[r * 16 + 8:r * 16 + 16]
                if accs[n] is None:
                    if prev is not None:
                        t0 = jnp.where(keep, t0, prev[n % len(prev)])
                    accs[n] = t0 + t1
                else:
                    if j0 == 0 and n == 0 and r == OF:
                        t0 = jnp.where(keep, t0, ofence[0:8])
                    accs[n] = (accs[n] + t0) + t1
        prev = accs
        for n, job in enumerate(grp):
            vres[job] = _allreduce8(accs[n][None], jnp.add)[0]

    chunks = [(lo, min(FC, NM - lo)) for lo in range(0, NM, FC)]
    acts, y = [], None
    for k, (lo, w) in enumerate(chunks):
        g = _dot_nn(xs, wg_v[:, lo:lo + w])
        u = _dot_nn(xs, wu_v[:, lo:lo + w])
        acts.append(act(g[0:8], u[0:8]))
        if k >= 1:
            t = down(acts[k - 1], *chunks[k - 1])
            y = t if y is None else y + t
    y = y + down(acts[-1], *chunks[-1])
    for b0, nb in ((0, 4), (4, 4), (8, 3), (11, 1)):
        g = jnp.concatenate([vres[(0, b)] for b in range(b0, b0 + nb)], axis=1)
        u = jnp.concatenate([vres[(1, b)] for b in range(b0, b0 + nb)], axis=1)
        y = y + down(act(g, u), NM + b0 * 128, nb * 128)

    gate = jnp.broadcast_to(jax.nn.sigmoid(mval), (8, 128))
    base = pl.multiple_of((idx >> 4) << 4, 16)
    rows = pl.ds(pl.multiple_of(P2 + base, 16), 16)
    h16 = h_v[rows, :]
    st16 = st_v[rows, :]
    a16 = 1.0 + st16[:, 0:128]
    m16 = st16[:, 128:256]
    hit = (lax.broadcasted_iota(jnp.int32, (16, 128), 0) + base) == idx
    res = []
    for c in range(D // 128):
        yc = y[:, c * 128:(c + 1) * 128] * gate
        yc = jnp.concatenate([yc, yc], axis=0)
        res.append(h16[:, c * 128:(c + 1) * 128] * a16 - m16 + jnp.where(hit, yc, 0.0))
    res = jnp.concatenate(res, axis=1).astype(bf16)
    for i in range(NI):
        cp_out(i * BPI, 2).wait()
        cp_out(i * BPI + 2, 2).wait()
    out_v[rows, :] = res
    fix = pltpu.make_async_copy(out_v.at[rows], out_hbm.at[pl.ds(base, 16)], sem_o.at[0])
    fix.start()
    fix.wait()


@jax.jit
def pallas_sequential_preLN__linear_kernel_hedgehog__moe_arch_mod__prompt_kernel(
    A_x: jax.Array,
    A_wqkv: jax.Array,
    A_w_phi: jax.Array,
    A_wo: jax.Array,
    B_x: jax.Array,
    B_w_r: jax.Array,
    B_w_gate: jax.Array,
    B_w_up: jax.Array,
    B_w_down: jax.Array,
):
    del B_x
    x = A_x.reshape(S, D)
    wphi = A_w_phi.reshape(H * DH, DH)
    wr = B_w_r.reshape(8, 128)
    any_spec = pl.BlockSpec(memory_space=pl.ANY)
    out = pl.pallas_call(
        _kernel,
        out_shape=jax.ShapeDtypeStruct((S, D), bf16),
        in_specs=[any_spec] * 8,
        out_specs=any_spec,
        scratch_shapes=[
            pltpu.VMEM((S, D), bf16),
            pltpu.VMEM((D, 3 * D), bf16),
            pltpu.VMEM((H * DH, DH), bf16),
            pltpu.VMEM((D, D), bf16),
            pltpu.VMEM((8, 128), bf16),
            pltpu.VMEM((D, F + 128), bf16),
            pltpu.VMEM((D, F + 128), bf16),
            pltpu.VMEM((F, D), bf16),
            pltpu.VMEM((PR, D), u32),
            pltpu.VMEM((PR // 2, 7 * HK), u32),
            pltpu.VMEM((PR // 2, 7 * HK), u32),
            pltpu.VMEM((D // 4, 7 * HK), u32),
            pltpu.VMEM((D // 4, 7 * HK), u32),
            pltpu.VMEM((F // 2, D + 128), u32),
            pltpu.VMEM((64, 8 * 128), u32),
            pltpu.VMEM((T0 // 2, D), u32),
            pltpu.VMEM(((S + T) // 4, 7 * HK), u32),
            pltpu.VMEM((NP, 64, 128), f32),
            pltpu.VMEM((2 * D, 128), f32),
            pltpu.VMEM((32, NP * 128), u32),
            pltpu.VMEM((D, T), u32),
            pltpu.VMEM((D // 2, 2 * B), u32),
            pltpu.VMEM((D // 2, 2 * B), u32),
            pltpu.VMEM((D // 2, 2 * B), u32),
            pltpu.VMEM((D // 2, 2 * B), u32),
            pltpu.VMEM((HK // 2, 7 * B), u32),
            pltpu.VMEM((HK // 2, 7 * B), u32),
            pltpu.VMEM((P2 + S, D), f32),
            pltpu.VMEM((P2 + S, 256), f32),
            pltpu.VMEM((B, 512), f32),
            pltpu.VMEM((P2 + S, D), bf16),
            pltpu.VMEM((8, D + 256), f32),
            pltpu.VMEM((B, 128), f32),
            pltpu.VMEM((B, 128), jnp.int32),
            pltpu.SMEM((2,), jnp.int32),
            pltpu.SemaphoreType.DMA((_NSEM_IN,)),
            pltpu.SemaphoreType.DMA((1,)),
        ],
        compiler_params=pltpu.CompilerParams(vmem_limit_bytes=110 * 1024 * 1024,
                                             disable_bounds_checks=True,
                                             disable_semaphore_checks=True),
        name="hedgehog_mod",
    )(x, A_wqkv, wphi, A_wo, wr, B_w_gate, B_w_up, B_w_down)
    return out.reshape(1, S, D)
```

```python
import os
import jax
import jax.numpy as jnp
from jax import lax
import jax.experimental.pallas as pl
import jax.experimental.pallas.tpu as pltpu

S = 2048
D = 1024
H = 32
DH = 32
F = 3584
T = 512
NT = S // T
T0 = 256
B = 128
NB = S // B
BPI = 4
NI = NB // BPI
NP = H // 2
FC = 512
R = 16
NBV = 12
NCH = 4
OCH = 176
DCH = int(os.environ.get('DCH', 1216))
NV = 124
PR = NV * 4
HK = D // 2
P2 = 2 * B
LOG2E = 1.4426950408889634
LN_EPS = 1e-5
DEN_EPS = 1e-6

_NT_DIMS = (((1,), (1,)), ((), ()))
_TN_DIMS = (((0,), (0,)), ((), ()))

bf16 = jnp.bfloat16
f32 = jnp.float32
u32 = jnp.uint32


def _opt(name, default):
    return type(default)(os.environ.get(name, default))


def _dot_nt(a, b):
    return lax.dot_general(a, b, _NT_DIMS, preferred_element_type=f32)


def _dot_nn(a, b):
    return jnp.dot(a, b, preferred_element_type=f32)


def _pk(x):
    return pltpu.bitcast(x, u32)


def _upk(x):
    return pltpu.bitcast(x, bf16)


def _lanes(x):
    return jnp.broadcast_to(x, (x.shape[0], 128))


def _layernorm(x):
    m = jnp.mean(x, axis=-1, keepdims=True)
    xc = x - m
    v = jnp.mean(xc * xc, axis=-1, keepdims=True)
    return xc * lax.rsqrt(v + LN_EPS)


def _allreduce8(x, op):
    x = op(x, pltpu.roll(x, 4, 1))
    x = op(x, pltpu.roll(x, 2, 1))
    x = op(x, pltpu.roll(x, 1, 1))
    return x


def _hedgehog_t(p, z=None):
    t = p.shape[-1]
    p4 = p.reshape(2, 4, 8, t)
    mx = _allreduce8(jnp.max(p4, axis=1), jnp.maximum)
    mn = _allreduce8(jnp.min(p4, axis=1), jnp.minimum)
    ep = jnp.exp2(p4 - mx[:, None])
    en = jnp.exp2(mn[:, None] - p4)
    a = pl.reciprocal(_allreduce8(jnp.sum(ep, axis=1), jnp.add), approx=True)
    b = pl.reciprocal(_allreduce8(jnp.sum(en, axis=1), jnp.add), approx=True)
    if z is not None:
        dp = jnp.sum(ep * z[0:64].reshape(2, 4, 8, t), axis=1)
        dn = jnp.sum(en * z[64:128].reshape(2, 4, 8, t), axis=1)
        den = _allreduce8(dp * a + dn * b, jnp.add) + DEN_EPS
        inv = pl.reciprocal(den, approx=True)
        a = a * inv
        b = b * inv
    fp = (ep * a[:, None]).reshape(64, t)
    fn = (en * b[:, None]).reshape(64, t)
    return jnp.concatenate([fp, fn], axis=0)


_SA = ((3, None, 0), (2, 3, 1), (0, 1, 1), (0, None, 0), (0, 3, 1), (1, 3, -1), (2, 0, -1))
_SB = ((2, 0, -1), (0, None, 0), (3, None, 0), (1, 3, -1), (0, 3, 1), (2, 3, 1), (0, 1, 1))


def _combo(blocks, spec):
    a, b, sign = spec
    if b is None:
        return blocks[a]
    return blocks[a] + blocks[b] if sign > 0 else blocks[a] - blocks[b]


def _strassen(product, emit):
    m4 = product(0)
    m2 = product(1)
    emit(2, m4 + m2)
    m5 = product(2)
    u = m4 - m5
    m3 = product(3)
    emit(1, m5 + m3)
    v = m3 - m2
    m1 = product(4)
    u = u + m1
    v = v + m1
    emit(0, u + product(5))
    emit(3, v + product(6))


def _head_groups(h):
    base, k = (NV // 4) * (h // 8), h % 8
    return ([base + 4 * k + i for i in range(3)],
            base + 4 * k - 1 if k > 0 else None,
            base + 4 * k + 3 if k < 7 else None,
            8 - k)


def _pair_logits(group, j):
    parts = []
    for h in (2 * j, 2 * j + 1):
        full, below, above, a = _head_groups(h)
        ref = group(full[0])
        sub = lax.broadcasted_iota(jnp.int32, ref.shape, 0)
        if above is None:
            m = jnp.where(sub >= a, group(below), 0.0)
        else:
            m = jnp.where(sub == a - 1, 0.0, group(above))
            if below is not None:
                m = jnp.where(sub >= a, group(below), m)
        parts += [m] + [group(q) for q in full]
    return jnp.concatenate(parts, axis=0)


def _pair_need(j):
    full, _, above, _ = _head_groups(2 * j + 1)
    return full[2] if above is None else above


def _tie(keep, w, ties):
    rows = sorted({r for r, _ in ties})
    out, pos = [], 0
    for r in rows:
        if r > pos:
            out.append(w[pos:r])
        cols = sorted(c for rr, c in ties if rr == r)
        parts, cpos = [], 0
        for c in cols:
            if c > cpos:
                parts.append(w[r:r + 8, cpos:c])
            parts.append(jnp.where(keep, w[r:r + 8, c:c + 128], ties[(r, c)]))
            cpos = c + 128
        if cpos < w.shape[1]:
            parts.append(w[r:r + 8, cpos:])
        out.append(jnp.concatenate(parts, axis=1) if len(parts) > 1 else parts[0])
        pos = r + 8
    if pos < w.shape[0]:
        out.append(w[pos:])
    return jnp.concatenate(out, axis=0)


def _vregs(x):
    if x.dtype != u32:
        x = pltpu.bitcast(x, u32)
    return [x[r:r + 8, c:c + 128] for r in range(0, x.shape[0], 8) for c in range(0, x.shape[1], 128)]


def _or_all(vals):
    acc = vals[0]
    for v in vals[1:]:
        acc = acc | v
    return acc


_KSTAGES = (((0, 1), (4, 1)), ((1, 2), (5, 1)), ((3, 1), (6, 2)))
_PSTAGES = (((0, 1), (4, 1)), ((1, 3), (5, 3)))
_NSEM_IN = 12


def _kernel(x_hbm, wqkv_hbm, wphi_hbm, wo_hbm, wr_hbm, wg_hbm, wu_hbm, wd_hbm,
            out_hbm,
            x_v, wqkv_v, wphi_v, wo_v, wr_v, wg_v, wu_v, wd_v,
            wtk_v, wsq_v, wsk_v, wsv_v, wso_v, wdp_v, amat_v, xn_v, xs_v, kvacc_v, zacc_v, kv_v, phi_v,
            pq0_v, pq1_v, pq2_v, pq3_v, oc0_v, oc1_v, h_v, st_v, pend_v, out_v, wrb_v,
            bestv_v, besti_v, flag_s,
            sem_i, sem_o):

    def cp_x(lo, n, sem):
        return pltpu.make_async_copy(x_hbm.at[pl.ds(lo, n)], x_v.at[pl.ds(lo, n)], sem_i.at[sem])

    def cp_w(lo, w, sem):
        return pltpu.make_async_copy(wqkv_hbm.at[:, pl.ds(lo, w)], wqkv_v.at[:, pl.ds(lo, w)], sem_i.at[sem])

    cp_k = [[cp_w(D + g * 128, n * 128, 2 + c) for g, n in st] for c, st in enumerate(_KSTAGES)]
    cp_p = [[pltpu.make_async_copy(wphi_hbm.at[pl.ds(g * 128, n * 128)], wphi_v.at[pl.ds(g * 128, n * 128)],
                                   sem_i.at[3 * c]) for g, n in st] for c, st in enumerate(_PSTAGES)]
    cp_wv = cp_w(2 * D, D, 5)
    cp_wq = cp_w(0, D, 7)

    def cp_wd(k):
        lo, n = k * DCH, min(DCH, F - k * DCH)
        return pltpu.make_async_copy(wd_hbm.at[pl.ds(lo, n)], wd_v.at[pl.ds(lo, n)], sem_i.at[(6, 8, 9)[k]])

    cp_x0 = cp_x(0, T0, 1)
    cp_x1 = cp_x(T0, T0, 4)
    cp_x2 = cp_x(T, T, 11)
    cp_x3 = cp_x(2 * T, T, 6)
    cp_x4 = cp_x(3 * T, T, 8)
    cp_wr = pltpu.make_async_copy(wr_hbm, wr_v.at[pl.ds(0, 8)], sem_i.at[7])

    def cp_wo(k, half):
        lo, n = k * OCH, min(OCH, HK - k * OCH)
        rows = pl.ds(half * HK + lo, n)
        return pltpu.make_async_copy(wo_hbm.at[rows], wo_v.at[rows], sem_i.at[(6, 8, 9)[k]])

    def wait_bg(k):
        cp_wo(k, 0).wait()
        cp_wo(k, 1).wait()
        cp_wd(k).wait()

    cp_wg = pltpu.make_async_copy(wg_hbm, wg_v.at[:, pl.ds(0, F)], sem_i.at[10])
    cp_wu = pltpu.make_async_copy(wu_hbm, wu_v.at[:, pl.ds(0, F)], sem_i.at[10])

    def cp_out(b, n):
        lo = b * B
        if not isinstance(b, int):
            lo = pl.multiple_of(lo, B)
        return pltpu.make_async_copy(out_v.at[pl.ds(P2 + lo, n * B)], out_hbm.at[pl.ds(lo, n * B)], sem_o.at[0])

    for cp in (*cp_p[0], cp_x0, *cp_k[0], *cp_p[1], *cp_k[1], *cp_k[2], cp_x1, cp_wv, cp_x2,
               cp_x3, cp_wo(0, 0), cp_wo(0, 1), cp_wd(0), cp_x4, cp_wo(1, 0), cp_wo(1, 1), cp_wd(1),
               cp_wo(2, 0), cp_wo(2, 1), cp_wd(2), cp_wr, cp_wq, cp_wg, cp_wu):
        cp.start()
    flag_s[0] = 1
    flag_s[1] = 0

    def ln1(xg, src, xd, dst, n, which=None, keep=None, anchors=None, plain=False, split=False):
        pieces = []
        for pr in range(n // P2):
            for k in range(B // R):
                off = pr * P2 + k * R
                if which is not None and pr * (B // R) + k not in which:
                    continue
                x0 = xg[src + off:src + off + R, :].astype(f32)
                x1 = xg[src + off + B:src + off + B + R, :].astype(f32)
                if anchors is not None:
                    a = anchors[len(pieces)]
                    x0 = jnp.concatenate([jnp.where(keep, x0[:, :128], a), x0[:, 128:]], axis=1)
                    x1 = jnp.concatenate([jnp.where(keep, x1[:, :128], a), x1[:, 128:]], axis=1)
                p0 = _layernorm(x0)
                p1 = _layernorm(x1)
                if plain:
                    xn_v[off // 2:(off + R) // 2, :] = _pk(p0.astype(bf16))
                    xn_v[(off + B) // 2:(off + B + R) // 2, :] = _pk(p1.astype(bf16))
                lo = (dst + pr * P2) // 4 + k * (R // 2)
                blocks = (p0[:, :HK], p1[:, :HK], p0[:, HK:], p1[:, HK:])
                vs = []
                for m, spec in enumerate(_SB):
                    t = _combo(blocks, spec)
                    xd[lo:lo + R // 2, m * HK:(m + 1) * HK] = _pk(t.astype(bf16))
                    if spec[1] is not None:
                        vs.append(_vregs(t))
                if split:
                    pieces.append((vs[0], vs[1], [_or_all(list(col)) for col in zip(*vs[2:])]))
                else:
                    pieces.append([_or_all(list(col)) for col in zip(*vs)])
        return pieces

    def load_xn(b):
        return _upk(xn_v[b * (B // 2):(b + 1) * (B // 2), :])

    def piece_ties(pieces, n, row0=0, col=0):
        ties = {}
        if pieces:
            step = (n - row0) // len(pieces) // 8 * 8
            for k, p in enumerate(pieces):
                for q, val in enumerate(p):
                    ties[(row0 + k * step + (q // 4) * 8, col + (q % 4) * 128)] = val
        return ties

    def xs_view(i, tiles):
        return xs_v.at[pl.ds(pl.multiple_of(i * (T // 4), T // 4), tiles * (T // 4))]

    def sproj(ws, xd, pr, emit, keep=None, work=None, before=None, after=None):
        lo = pr * (B // 2)

        def product(m):
            if before:
                before(m)
            lhs = ws[:, m * HK:(m + 1) * HK]
            if work is not None and work.get(m):
                lhs = _tie(keep, lhs, piece_ties(work[m], lhs.shape[0], 32))
            res = _dot_nt(_upk(lhs), _upk(xd[lo:lo + B // 2, m * HK:(m + 1) * HK]))
            if after:
                after(m, res)
            return res

        _strassen(product, lambda k, val: emit(k // 2, k % 2, val))

    def spread(pieces, slots):
        res = {}
        for k, (pr, m) in enumerate(slots):
            res.setdefault(pr, {})[m] = pieces[k * len(pieces) // len(slots):(k + 1) * len(pieces) // len(slots)]
        return res

    def sealed(ref):
        n = ref.shape[0] - 8
        if _opt('SEAL', 1):
            ref[pl.ds(pl.multiple_of(flag_s[1] + n, 8), 8), 0:128] = jnp.zeros((8, 128), u32)
            return ref
        return ref.at[pl.ds(pl.multiple_of(flag_s[1], 8), n)]

    def fence(ref, row, col):
        return ref[pl.ds(pl.multiple_of(flag_s[1] + row, 8), 8), col:col + 128]

    def store_combos(ws, row, top, bot, table=_SA, keep=None, dep=None, every=1):
        for n, c in enumerate(range(0, HK, 128)):
            raw = [top[:, c:c + 128], top[:, HK + c:HK + c + 128], bot[:, c:c + 128], bot[:, HK + c:HK + c + 128]]
            if keep is not None and dep is not None:
                for q in (0, 3):
                    d = dep if raw[q].dtype == u32 else pltpu.bitcast(jnp.concatenate([dep, dep], axis=0), f32)
                    raw[q] = jnp.where(keep, raw[q], d)
            blocks = [_upk(b).astype(f32) if b.dtype == u32 else b for b in raw]
            for m, spec in enumerate(table):
                t = raw[spec[0]] if spec[1] is None else _combo(blocks, spec)
                ws[row:row + 8, m * HK + c:m * HK + c + 128] = t if t.dtype == u32 else _pk(t.astype(bf16))
            if keep is not None and (n + 1) % every == 0:
                dep = fence(ws, row, c)
        return dep if keep is not None else fence(ws, row, 0)

    zinit = set()

    def k_side(group, pairs, first, slot=None, keep=None, anchor=None):
        res = []
        for j in pairs:
            p = _pair_logits(group, j)
            if anchor is not None:
                p = jnp.concatenate([jnp.where(keep, p[0:8], anchor), p[8:32],
                                     jnp.where(keep, p[32:40], anchor), p[40:64]], axis=0)
            ph = _hedgehog_t(p)
            if j not in zinit:
                zinit.add(j)
                zacc_v[j * 128:(j + 1) * 128, :] = ph
            else:
                zacc_v[j * 128:(j + 1) * 128, :] += ph
            if slot is not None:
                phi_v[j * 64:(j + 1) * 64, slot * B:(slot + 1) * B] = _pk(ph.astype(bf16))
            res.append(ph)
        return res

    def half_groups(p, half):
        return lambda pos: p[(pos - half * (NV // 2)) * 8:(pos - half * (NV // 2) + 1) * 8]

    def half_pairs(half):
        return range(half * (NP // 2), (half + 1) * (NP // 2))

    def kv_prod(vt, ph, j):
        half, r = j // (NP // 2), (j % (NP // 2)) * 64
        v = jnp.concatenate([vt[(s, half)][r:r + 64] for s in range(T // B)], axis=1).astype(bf16)
        return _dot_nt(v, ph)

    def v_side(xd, keep, pieces, chain):
        work = spread(pieces, [(0, m) for m in range(1, 7)] + [(1, m) for m in range(6)])
        vt = {}
        for q in range(T // P2):
            sproj(wsv_v, xd, q, lambda half, blk, val, q=q: vt.__setitem__((2 * q + blk, half), val),
                  keep, work.get(q))
            if q == 0:
                m = _opt('OM', 2)
                work[1][m] = list(work[1].get(m, [])) + [[chain(pltpu.bitcast(vt[(0, 1)][0:8], u32))]]
        return vt

    r_i = lax.broadcasted_iota(jnp.int32, (128, DH), 0)
    c_i = lax.broadcasted_iota(jnp.int32, (128, DH), 1)
    expand = (r_i % DH == c_i).astype(bf16)
    r_h = lax.broadcasted_iota(jnp.int32, (128, 128), 0) // DH
    c_h = lax.broadcasted_iota(jnp.int32, (128, 128), 1) // DH
    same_head = r_h == c_h

    def make_amat(g):
        a = _dot_nt(expand, wphi_v[g * 128:(g + 1) * 128, :])
        amat_v[:, g * 128:(g + 1) * 128] = _pk(jnp.where(same_head, a, 0.0).astype(bf16))

    class Folder:
        def __init__(self, col0, first=0):
            self.col0, self.rows, self.mprev, self.done = col0, {}, None, first

        def tile(self, g, rows, keep=None, ties=None):
            am = amat_v[:, g * 128:(g + 1) * 128]
            if ties:
                am = _tie(keep, am, ties)
            return _dot_nt(_upk(am), wqkv_v[rows, self.col0 + g * 128:self.col0 + (g + 1) * 128])

        def fold(self, g, wt=None):
            sub = lax.broadcasted_iota(jnp.int32, (8, D), 0)
            if wt is None:
                wt = self.tile(g, slice(None))
            for hh in range(4):
                full, below, _, a = _head_groups(4 * g + hh)
                r0 = hh * DH
                ref = jnp.broadcast_to(wt[r0 + a - 1:r0 + a, :], (8, D))
                part = [(wt[r0 + 8 * i:r0 + 8 * (i + 1)] - ref) * LOG2E for i in range(4)]
                if below is not None:
                    self.rows[below] = jnp.where(sub >= a, part[0], self.mprev)
                self.mprev = part[0]
                for q, v in zip(full, part[1:]):
                    self.rows[q] = v
            new = {}
            while self.done in self.rows and self.done + 1 in self.rows:
                new[self.done] = jnp.concatenate([self.rows.pop(self.done), self.rows.pop(self.done + 1)], axis=0)
                self.done += 2
            return new

    def fold_pair(folders, g, keep=None, ties=None):
        tiles = {}
        for n, c in enumerate(range(0, HK, 128)):
            for half in range(2):
                for side in range(2):
                    t = ties[n] if ties and half == 0 and side == 0 else None
                    lo = side * HK + c
                    tiles[(half, lo)] = folders[half].tile(g + 4 * half, slice(lo, lo + 128), keep, t)
        return [folders[half].fold(g + 4 * half,
                                   jnp.concatenate([tiles[(half, lo)] for lo in range(0, D, 128)], axis=1))
                for half in range(2)]

    bestv_v[...] = jnp.full(bestv_v.shape, -jnp.inf, f32)
    besti_v[...] = lax.broadcasted_iota(jnp.int32, besti_v.shape, 0)
    h_v[0:P2, :] = jnp.zeros((P2, D), f32)
    st_v[0:B, :] = jnp.zeros((B, 256), f32)
    pend_v[...] = jnp.zeros(pend_v.shape, f32)

    def wait_all(cps):
        for cp in cps:
            cp.wait()

    def amats(c):
        for g0, n in _PSTAGES[c]:
            for g in range(g0, g0 + n):
                make_amat(g)

    wait_all(cp_p[0])
    amats(0)

    cp_x0.wait()
    ln1(x_v, 0, xs_v, 0, T0, plain=True)
    xb = [load_xn(s) for s in range(2)]
    logits = [{}, {}]
    finished = [set(), set()]
    fk, slabs = (Folder(D), Folder(D, NV // 2)), {}
    defer, queue = [False], []

    def absorb(new):
        for pos, slab in new.items():
            wtk_v[pos * 4:pos * 4 + 8, :] = _pk(slab.astype(bf16))
            slabs[pos] = slab
        for pos in sorted(slabs):
            if pos < NV // 2 and pos + NV // 2 in slabs:
                store_combos(wsk_v, pos * 4, slabs.pop(pos), slabs.pop(pos + NV // 2))

    def k_finish(s, hold=0):
        ready = [j for j in range(NP) if j not in finished[s] and _pair_need(j) in logits[s]]
        ready = ready[:len(ready) - hold]
        if defer[0]:
            queue.extend((logits[s].__getitem__, [j], s == 0, s) for j in ready)
        else:
            k_side(logits[s].__getitem__, ready, s == 0, s)
        finished[s].update(ready)

    def k_chunk(s, keep=None, early=(), late=(), hold=0):
        todo = [q for half in range(2) for q in range(half * (NV // 2), fk[half].done) if q not in logits[s]]
        runs = [[q for q in todo if q < NV // 2], [q for q in todo if q >= NV // 2]]
        lhs = jnp.concatenate([wtk_v[r[0] * 4:(r[-1] + 1) * 4, :] for r in runs if r], axis=0)
        ties = piece_ties(early, lhs.shape[0])
        ties.update(piece_ties(late, lhs.shape[0], col=HK))
        if ties:
            lhs = _tie(keep, lhs, ties)
        p = _dot_nt(_upk(lhs), xb[s])
        for n, q in enumerate(todo):
            logits[s][q] = p[n * 8:(n + 1) * 8]
        k_finish(s, hold)
        return p

    HOLD = _opt('HOLD', 1)
    wait_all(cp_k[0])
    for new in fold_pair(fk, 0):
        absorb(new)
    k_chunk(0)
    k_chunk(1, hold=HOLD)

    wait_all(cp_p[1] + cp_k[1])
    k_finish(1)
    amats(1)
    for new in fold_pair(fk, 1):
        absorb(new)
    absorb(fk[0].fold(2))
    k_chunk(0)
    k_chunk(1, hold=HOLD)

    wait_all(cp_k[2] + [cp_x1])
    defer[0] = True
    keep = flag_s[0] > 0
    w6 = fk[1].tile(6, slice(None))
    absorb(fk[1].fold(6, w6))
    new = fold_pair(fk, 3)
    top = list(new[0].values())
    for n in new:
        absorb(n)
    anc = [None, w6[0:R, 0:128], w6[64:64 + R, 512:640], top[0][:, 128:256], top[-1][:, 384:512]]
    A0 = [int(v) for v in _opt('A0', '0,4,4').split(',')]
    n0 = len(A0)
    pieces = [ln1(x_v, T0, xs_v, T0, T0, [k], keep, None if anc[a] is None else [anc[a]])[0] for k, a in enumerate(A0)]
    t0 = _opt('T0A', 2)
    p = k_chunk(0, keep, (), pieces[:t0])
    rows = [k * p.shape[0] // (8 - n0) // 16 * 16 for k in range(8 - n0)]
    pieces += ln1(x_v, T0, xs_v, T0, T0, list(range(n0, 8)), keep, [p[r:r + R] for r in rows])
    k_chunk(1, keep, pieces[t0:n0], pieces[n0:])
    NOW = _opt('NOW', 3)

    def k_emit1(half, blk, val):
        order = {(1, 0): 0, (0, 1): 1, (0, 0): 2, (1, 1): 3}[(half, blk)]
        pairs = list(half_pairs(half))
        nat = [int(v) for v in _opt('NAT', '8,6,0,0').split(',')][order]
        k_side(half_groups(val, half), pairs[:nat], False, 2 + blk)
        queue.extend((half_groups(val, half), [j], False, 2 + blk) for j in pairs[nat:])

    def run_queue(n, res):
        deps = []
        mode = _opt('QM', 3)
        for k in range(min(n, len(queue))):
            r = k * res.shape[0] // n // 8 * 8
            if mode == 2:
                r = 0
            ph = k_side(*queue.pop(0), keep=flag_s[0] > 0, anchor=None if mode == 1 else res[r:r + 8])
            v = _vregs(ph[0])
            deps.append([_or_all(v[q::4]) for q in range(4)])
        return deps if mode else []

    kwork = {}

    def k_after(m, res):
        if str(m) in _opt('KM', '02'):
            kwork[m + 1] = run_queue(_opt('NQ', 4), res)

    def v_prep():
        VL = _opt('VL', 0)
        fences = []
        for rb in range(0, HK, 128):
            for c in range(0, HK, 128):
                raw = [wqkv_v[side * HK + c:side * HK + c + 128, 2 * D + half * HK + rb:2 * D + half * HK + rb + 128]
                       for half in range(2) for side in range(2)]
                if VL and len(fences) >= VL:
                    d = fences[len(fences) - VL]
                    raw = [_upk(_tie(keep, _pk(t), {(0, 0): d})) for t in raw]
                raw = [t.T for t in raw]
                blocks = [t.astype(f32) for t in raw]
                for m, spec in enumerate(_SA):
                    t = raw[spec[0]] if spec[1] is None else _combo(blocks, spec).astype(bf16)
                    wsv_v[rb // 2:rb // 2 + 64, m * HK + c:m * HK + c + 128] = _pk(t)
                if VL:
                    fences.append(fence(wsv_v, rb // 2, c))

    def k_before(m):
        if m == 4:
            cp_wv.wait()
            v_prep()

    sproj(wsk_v.at[pl.ds(pl.multiple_of(flag_s[1], 8), PR // 2)] if _opt('KO', 0) else wsk_v, xs_v, 1, k_emit1, keep, kwork, k_before, k_after)

    vt = {}
    wsv = wsv_v.at[pl.ds(pl.multiple_of(flag_s[1], D // 4), D // 4)] if _opt('VO', 1) else wsv_v
    XW = _opt('XW', 5)
    work = {0: {}, 1: {}}
    slots = [(0, m) for m in range(XW, 7)] + [(1, m) for m in range(6)]

    def v_before(m):
        if m == XW:
            cp_x2.wait()

    def v_after(q):
        def after(m, res):
            left = _opt('QE', 4) - (7 * q + m)
            if left > 0 and not (q == 0 and m == XW - 1):
                work[q][m + 1] = run_queue(-(-len(queue) // left), res)
            if (q, m) in slots:
                k = slots.index((q, m))
                which = list(range(k * 16 // len(slots), (k + 1) * 16 // len(slots)))
                rows = [n * HK // len(which) // 16 * 16 for n in range(len(which))]
                nq, nm = (q, m + 1) if m < 6 else (q + 1, 0)
                pcs = ln1(x_v, T, xs_v, T, T, which, flag_s[0] > 0, [res[r:r + R] for r in rows])
                work[nq][nm] = [[]] * (2 - len(pcs) + 1) + pcs if _opt('LD', 1) else pcs
        return after

    for q in range(2):
        sproj(wsv, xs_v, q, lambda half, blk, val, q=q: vt.__setitem__((2 * q + blk, half), val),
              keep, work[q], v_before if q == 0 else None, v_after(q))
    assert not queue
    phi_m = sealed(phi_v)
    for j in range(NP):
        kvacc_v[j] = kv_prod(vt, _upk(phi_m[j * 64:(j + 1) * 64, :]), j)
    cp_x3.wait()
    wait_bg(0)

    def p1_body(i, c):
        @pl.when(i == 2)
        def _():
            cp_x4.wait()
            wait_bg(1)

        @pl.when(i == 3)
        def _():
            wait_bg(2)

        keep = flag_s[0] > 0
        lo = jnp.minimum((i - 1) * DCH, F - DCH)
        sv = wd_v.at[pl.ds(pl.multiple_of(lo, 16), DCH)]
        dv = wdp_v.at[pl.ds(pl.multiple_of(lo // 2, 8), DCH // 2)]
        deps = []
        for r in range(0, DCH, 16):
            val = _pk(sv[r:r + 16, :])
            dv[r // 2:r // 2 + 8, 0:D] = val
            deps.append([_or_all(_vregs(val))])
        lo = jnp.minimum((i - 1) * OCH, HK - OCH)
        ov = wo_v.at[pl.ds(pl.multiple_of(lo, 16), HK + OCH)]
        od = wso_v.at[pl.ds(pl.multiple_of(lo // 2, 8), OCH // 2)]
        work = spread(deps, [(q, m) for q in range(2) for m in (0, 2, 4)])

        phik = {}
        PK = _opt('PK', 1)

        def k_emit(q):
            def emit(half, blk, val):
                for j, ph in zip(half_pairs(half), k_side(half_groups(val, half), half_pairs(half), False, 2 * q + blk if PK else None)):
                    phik[(2 * q + blk, j)] = ph
            return emit

        xd = xs_view(i, 2)
        for q in range(T // P2):
            sproj(wsk_v, xd, q, k_emit(q), keep, work[q])
        xg = x_v.at[pl.ds(pl.multiple_of(jnp.minimum(i + 1, NT - 1) * T, T), T)]
        pieces = ln1(xg, 0, xd, T, T)

        def wo_chain(dep):
            for r in range(0, OCH, 16):
                dep = store_combos(od, r // 2, ov[r:r + 16, :].astype(f32), ov[HK + r:HK + r + 16, :].astype(f32),
                                   _SB, keep, dep)
            return dep

        vt = v_side(xd, keep, pieces, wo_chain)
        phi_m = sealed(phi_v)
        for j in range(NP):
            if PK:
                ph = _upk(phi_m[j * 64:(j + 1) * 64, :])
            else:
                ph = jnp.concatenate([phik[(s, j)] for s in range(T // B)], axis=1).astype(bf16)
            kvacc_v[j] += kv_prod(vt, ph, j)
        return c

    lax.fori_loop(1, NT, p1_body, 0)

    cp_wr.wait()
    cp_wq.wait()
    keep = flag_s[0] > 0
    kv_mask = (lax.broadcasted_iota(jnp.int32, (64, 128), 0) // DH
               == (lax.broadcasted_iota(jnp.int32, (64, 128), 1) // DH) % 2)
    ties = [{} for _ in range(16)]
    for j in range(NP):
        kvj = jnp.where(kv_mask, kvacc_v[j], 0.0)
        kv_v[:, j * 128:(j + 1) * 128] = _pk(kvj.astype(bf16))
        zj = _lanes(jnp.sum(zacc_v[j * 128:(j + 1) * 128, :], axis=-1, keepdims=True))
        zacc_v[j * 128:(j + 1) * 128, :] = zj
        vals = _vregs(kvj) + _vregs(zj)
        b0 = _opt('BT', 1)
        if j + b0 < 16:
            for q in range(4):
                ties[j + b0][(32 + q * 8, 0)] = _or_all(vals[q::4])
    wr = wr_v[0:8, :].astype(f32)
    wl = jnp.sum(wr, axis=0, keepdims=True)
    wsum = jnp.sum(wl, axis=1, keepdims=True)
    wrb_v[:, 0:D + 256] = jnp.concatenate(
        [jnp.broadcast_to(wr[j:j + 1, :], (8, 128)) for j in range(8)]
        + [jnp.broadcast_to(wsum, (8, 128)), jnp.broadcast_to(wl, (8, 128))], axis=1)
    fq = (Folder(0), Folder(0, NV // 2))
    for g in range(4):
        new = fold_pair(fq, g, keep, ties[4 * g:4 * g + 4])
        for pos, slab in new[0].items():
            store_combos(wsq_v, pos * 4, slab, new[1][pos + NV // 2])

    pq_v = (pq0_v, pq1_v, pq2_v, pq3_v)

    def views_of(g):
        lo = g * (BPI * B)
        if not isinstance(g, int):
            lo = pl.multiple_of(lo, BPI * B)
        return ((x_v.at[pl.ds(lo, BPI * B)],)
                + tuple(ref.at[pl.ds(lo, P2 + BPI * B)] for ref in (h_v, out_v, st_v)) + (g,))

    def stage_q(xd, q, keep, work):
        def emit(half, blk, val):
            group = half_groups(val, half)
            for j in half_pairs(half):
                ph = _hedgehog_t(_pair_logits(group, j), zacc_v[j * 128:(j + 1) * 128, :])
                pq_v[2 * q + blk][(j // 2) * 64:(j // 2 + 1) * 64, (j % 2) * B:(j % 2 + 1) * B] = _pk(ph.astype(bf16))

        sproj(wsq_v, xd, q, emit, keep, work)

    oc_v = (oc0_v, oc1_v)

    def stage_g(q):
        pq = [sealed(pq_v[2 * q + blk]) for blk in range(2)]
        for jj in range(NP // 2):
            blocks = [_dot_nn(_upk(kv_v[:, j * 128:(j + 1) * 128]),
                              _upk(pq[blk][(j // 2) * 64:(j // 2 + 1) * 64, (j % 2) * B:(j % 2 + 1) * B]))
                      for blk in range(2) for j in (jj, jj + NP // 2)]
            for m, spec in enumerate(_SA):
                oc_v[q][jj * 32:(jj + 1) * 32, m * B:(m + 1) * B] = _pk(_combo(blocks, spec).astype(bf16))

    def stage_h(views, q, keep, pieces):
        x_g, h_g = views[0], views[1]
        oc = sealed(oc_v[q])
        first, last = _opt('H0', 3), _opt('H1', 22)
        ties = [{} for _ in range(7)]
        for k, vals in enumerate(pieces):
            t = first + k * (last - first) // max(len(pieces) - 1, 1)
            for m, val in enumerate(vals):
                ties[t // 4][(m * 8, (t % 4) * 128)] = val
        state = {}
        done = [0]

        def product(m):
            w = wso_v[:, m * HK:(m + 1) * HK]
            if ties[m]:
                w = _tie(keep, w, ties[m])
            done[0] = m
            return lax.dot_general(_upk(oc[0:HK // 2, m * B:(m + 1) * B]), _upk(w), _TN_DIMS,
                                   preferred_element_type=f32)

        def wmul(d, lo):
            return (d.reshape(B // 8, 8, 128) * wrb_v[:, lo:lo + 128][None]).reshape(B, 128)

        def emit(k, val):
            blk, half = k // 2, k % 2
            s = 2 * q + blk
            cols = slice(half * HK, (half + 1) * HK)
            h = x_g[s * B:(s + 1) * B, cols].astype(f32) + val
            h_g[(s + 2) * B:(s + 3) * B, cols] = h
            st = state.setdefault(blk, {'h': {}})
            st['h'][half] = h
            for c in range(0, HK, 128):
                ht = h[:, c:c + 128]
                if 'h0' not in st:
                    st['h0'] = ht
                    continue
                d = ht - st['h0']
                new = (d, d * d, wmul(d, half * HK + c))
                st['s'] = new if 's' not in st else tuple(a + b for a, b in zip(st['s'], new))
            lag = _opt('SL', 2)
            if lag and len(st['h']) == 1:
                vals = [_or_all(list(v)) for v in zip(*[_vregs(a) for a in st['s']])]
                m = done[0] + lag
                for n, val in enumerate(vals):
                    ties[m][(248 - (n % 4) * 8, (n // 4) * 128)] = val

        _strassen(product, emit)

        res = []
        for blk in range(2):
            st = state[blk]
            s1, s2, s3 = st['s']
            c0 = _lanes(jnp.mean(st['h0'], axis=-1, keepdims=True))
            g0 = st['h0'] - c0
            t1 = s1 + 8.0 * g0
            t2 = s2 + g0 * (s1 + t1)
            t3 = s3 + wmul(g0, D + 128)
            res.append((jnp.concatenate([t1, t2, t3, c0], axis=1),
                        jnp.concatenate([st['h'][0], st['h'][1]], axis=1)))
        return res

    def stage_stats(views, s, part, valid=None, keep=None, after=None):
        st_g, g = views[3], views[4]
        b = g * BPI + s
        bv = bestv_v[...]
        bi = besti_v[...]
        if after is not None:
            bv = jnp.concatenate([bv[:B - R], jnp.where(keep, bv[B - R:], after)], axis=0)
        wsum = wrb_v[0:1, D:D + 128]
        nvs, nis, sts = [], [], []
        for k in range(B // R):
            sl = slice(k * R, (k + 1) * R)
            red = [_lanes(jnp.sum(part[sl, n * 128:(n + 1) * 128], axis=-1, keepdims=True)) for n in range(3)]
            mu = red[0] * (1.0 / D)
            var = jnp.maximum(red[1] * (1.0 / D) - mu * mu, 0.0)
            rs = lax.rsqrt(var + LN_EPS)
            r = (red[2] - mu * wsum) * rs
            sts.append(jnp.concatenate([rs, (mu + part[sl, 384:512]) * rs], axis=1))
            if valid is not None:
                r = jnp.where(valid, r, -jnp.inf)
            idx = lax.broadcasted_iota(jnp.int32, (R, 128), 0) + (b * B + k * R)
            better = r > bv[sl]
            nvs.append(jnp.where(better, r, bv[sl]))
            nis.append(jnp.where(better, idx, bi[sl]))
        st = jnp.concatenate(sts, axis=0)
        st_g[(s + 2) * B:(s + 3) * B, :] = st
        bestv_v[...] = jnp.concatenate(nvs, axis=0)
        besti_v[...] = jnp.concatenate(nis, axis=0)
        return st, nvs

    def stage_out(views, s, st=None, h=None):
        h_g, out_g, st_g = views[1], views[2], views[3]
        rows = slice((s + 2) * B, (s + 3) * B)
        h = h_g[rows, :] if h is None else h
        st = st_g[rows, :] if st is None else st
        outs = []
        for k in range(B // R):
            sl = slice(k * R, (k + 1) * R)
            a = 1.0 + st[sl, 0:128]
            outs.append(jnp.concatenate([h[sl, c * 128:(c + 1) * 128] * a - st[sl, 128:256]
                                         for c in range(D // 128)], axis=1))
        out_g[rows, :] = jnp.concatenate([o.astype(bf16) for o in outs], axis=0)
        return [_vregs(o) for o in outs]

    def stage_i(views, s, part, h=None, valid=None, keep=None, after=None):
        st, nvs = stage_stats(views, s, part, valid, keep, after)
        return [o + _vregs(nv) for o, nv in zip(stage_out(views, s, st, h), nvs)]

    def p2_body(i, c):
        b0 = i * BPI
        keep = flag_s[0] > 0
        cur = views_of(i)
        pieces = stage_out(cur, -2) + stage_i(cur, -1, pend_v[...], valid=i > 0)
        for q in range(2):
            stage_q(xs_view(i, 1), q, keep, None)
        stage_g(0)
        stage_g(1)
        res = stage_h(cur, 0, keep, pieces)
        pieces = stage_i(cur, 0, *res[0]) + stage_i(cur, 1, *res[1])
        res = stage_h(cur, 1, keep, pieces)
        stage_stats(cur, BPI - 2, res[0][0])
        pend_v[...] = res[1][0]

        @pl.when(i > 0)
        def _():
            cp_out(jnp.maximum(b0 - 2, 0), 2).start()

        cp_out(b0, 2).start()
        return c

    lax.fori_loop(0, NI, p2_body, 0)
    cp_wg.wait()
    cp_wu.wait()
    keep = flag_s[0] > 0
    last = views_of(NI - 1)

    def out_fence():
        return out_v[pl.ds(pl.multiple_of(flag_s[1] + S, R), R), 0:128].astype(f32)

    TM = _opt('TM', 1)
    if TM == 0:
        stage_out(last, BPI - 2)
        st, _ = stage_stats(last, BPI - 1, pend_v[...], keep=keep, after=out_fence())
    else:
        st, _ = stage_stats(last, BPI - 1, pend_v[...])

    bv = bestv_v[...]
    mval = jnp.max(bv, axis=0, keepdims=True)
    sel = jnp.min(jnp.where(bv == mval, besti_v[...], S - 1), axis=0, keepdims=True)
    idx = sel[0, 0]
    sel_f = jnp.broadcast_to(pltpu.bitcast(sel, f32), (B, 128))
    if TM == 1:
        st2 = last[3][BPI * B:(BPI + 1) * B, :]
        stage_out(last, BPI - 2, jnp.concatenate([jnp.where(keep, st2[:, 0:128], sel_f), st2[:, 128:256]], axis=1))
    stage_out(last, BPI - 1, jnp.concatenate([jnp.where(keep, st[:, 0:128], sel_f), st[:, 128:256]], axis=1))
    ofence = out_fence()
    cp_out(NB - 2, 2).start()
    hrow = h_v[pl.ds(P2 + idx, 1), :]
    strow = st_v[pl.ds(P2 + idx, 1), :]
    xrow = jnp.concatenate([hrow[:, c * 128:(c + 1) * 128] * strow[:, 0:128] - strow[:, 128:256]
                            for c in range(D // 128)], axis=1).astype(bf16)
    xs = jnp.broadcast_to(xrow, (16, D))

    def act(g, u):
        a = g * pl.reciprocal(1.0 + jnp.exp(-g), approx=True) * u
        return jnp.concatenate([a, a], axis=0).astype(bf16)

    def down(a, lo, w):
        return _dot_nn(a, _upk(wdp_v[lo // 2:(lo + w) // 2, 0:D]))[0:8]

    NM = F - NBV * 128
    xcol = jnp.broadcast_to(xrow.astype(f32), (128, D)).T
    jobs = [(which, b) for b in range(NBV) for which in (0, 1)]
    vres, prev = {}, None
    OF = _opt('OF', 40)
    for j0 in range(0, len(jobs), NCH):
        grp = jobs[j0:j0 + NCH]
        accs = [None] * len(grp)
        for r in range(D // 16):
            for n, (which, b) in enumerate(grp):
                w = (wg_v, wu_v)[which][r * 16:(r + 1) * 16, NM + b * 128:NM + (b + 1) * 128].astype(f32)
                t0 = w[0:8] * xcol[r * 16:r * 16 + 8]
                t1 = w[8:16] * xcol[r * 16 + 8:r * 16 + 16]
                if accs[n] is None:
                    if prev is not None:
                        t0 = jnp.where(keep, t0, prev[n % len(prev)])
                    accs[n] = t0 + t1
                else:
                    if j0 == 0 and n == 0 and r == OF:
                        t0 = jnp.where(keep, t0, ofence[0:8])
                    accs[n] = (accs[n] + t0) + t1
        prev = accs
        for n, job in enumerate(grp):
            vres[job] = _allreduce8(accs[n][None], jnp.add)[0]

    chunks = [(lo, min(FC, NM - lo)) for lo in range(0, NM, FC)]
    acts, y = [], None
    for k, (lo, w) in enumerate(chunks):
        g = _dot_nn(xs, wg_v[:, lo:lo + w])
        u = _dot_nn(xs, wu_v[:, lo:lo + w])
        acts.append(act(g[0:8], u[0:8]))
        if k >= 1:
            t = down(acts[k - 1], *chunks[k - 1])
            y = t if y is None else y + t
    y = y + down(acts[-1], *chunks[-1])
    for b0, nb in ((0, 4), (4, 4), (8, 3), (11, 1)):
        g = jnp.concatenate([vres[(0, b)] for b in range(b0, b0 + nb)], axis=1)
        u = jnp.concatenate([vres[(1, b)] for b in range(b0, b0 + nb)], axis=1)
        y = y + down(act(g, u), NM + b0 * 128, nb * 128)

    gate = jnp.broadcast_to(jax.nn.sigmoid(mval), (8, 128))
    base = pl.multiple_of((idx >> 4) << 4, 16)
    rows = pl.ds(pl.multiple_of(P2 + base, 16), 16)
    h16 = h_v[rows, :]
    st16 = st_v[rows, :]
    a16 = 1.0 + st16[:, 0:128]
    m16 = st16[:, 128:256]
    hit = (lax.broadcasted_iota(jnp.int32, (16, 128), 0) + base) == idx
    res = []
    for c in range(D // 128):
        yc = y[:, c * 128:(c + 1) * 128] * gate
        yc = jnp.concatenate([yc, yc], axis=0)
        res.append(h16[:, c * 128:(c + 1) * 128] * a16 - m16 + jnp.where(hit, yc, 0.0))
    res = jnp.concatenate(res, axis=1).astype(bf16)
    for i in range(NI):
        cp_out(i * BPI, 2).wait()
        cp_out(i * BPI + 2, 2).wait()
    out_v[rows, :] = res
    fix = pltpu.make_async_copy(out_v.at[rows], out_hbm.at[pl.ds(base, 16)], sem_o.at[0])
    fix.start()
    fix.wait()


@jax.jit
def pallas_sequential_preLN__linear_kernel_hedgehog__moe_arch_mod__prompt_kernel(
    A_x: jax.Array,
    A_wqkv: jax.Array,
    A_w_phi: jax.Array,
    A_wo: jax.Array,
    B_x: jax.Array,
    B_w_r: jax.Array,
    B_w_gate: jax.Array,
    B_w_up: jax.Array,
    B_w_down: jax.Array,
):
    del B_x
    x = A_x.reshape(S, D)
    wphi = A_w_phi.reshape(H * DH, DH)
    wr = B_w_r.reshape(8, 128)
    any_spec = pl.BlockSpec(memory_space=pl.ANY)
    out = pl.pallas_call(
        _kernel,
        out_shape=jax.ShapeDtypeStruct((S, D), bf16),
        in_specs=[any_spec] * 8,
        out_specs=any_spec,
        scratch_shapes=[
            pltpu.VMEM((S, D), bf16),
            pltpu.VMEM((D, 3 * D), bf16),
            pltpu.VMEM((H * DH, DH), bf16),
            pltpu.VMEM((D, D), bf16),
            pltpu.VMEM((_opt('WRP', 64), 128), bf16),
            pltpu.VMEM((D, F + 128), bf16),
            pltpu.VMEM((D, F + 128), bf16),
            pltpu.VMEM((F, D), bf16),
            pltpu.VMEM((PR, D), u32),
            pltpu.VMEM((PR // 2, 7 * HK), u32),
            pltpu.VMEM((PR // 2, 7 * HK), u32),
            pltpu.VMEM((D // 4, 7 * HK), u32),
            pltpu.VMEM((D // 4, 7 * HK), u32),
            pltpu.VMEM((F // 2, D + 128), u32),
            pltpu.VMEM((64, 8 * 128), u32),
            pltpu.VMEM((T0 // 2, D), u32),
            pltpu.VMEM(((S + T) // 4, 7 * HK), u32),
            pltpu.VMEM((NP, 64, 128), f32),
            pltpu.VMEM((2 * D, 128), f32),
            pltpu.VMEM((32, NP * 128), u32),
            pltpu.VMEM((D + 8, T), u32),
            pltpu.VMEM((D // 2 + 16, 2 * B), u32),
            pltpu.VMEM((D // 2 + 16, 2 * B), u32),
            pltpu.VMEM((D // 2 + 16, 2 * B), u32),
            pltpu.VMEM((D // 2 + 16, 2 * B), u32),
            pltpu.VMEM((HK // 2 + 32, 7 * B), u32),
            pltpu.VMEM((HK // 2 + 32, 7 * B), u32),
            pltpu.VMEM((P2 + S, D), f32),
            pltpu.VMEM((P2 + S, 256), f32),
            pltpu.VMEM((B, 512), f32),
            pltpu.VMEM((P2 + S, D), bf16),
            pltpu.VMEM((8, D + 512), f32),
            pltpu.VMEM((B, 128), f32),
            pltpu.VMEM((B, 128), jnp.int32),
            pltpu.SMEM((2,), jnp.int32),
            pltpu.SemaphoreType.DMA((_NSEM_IN,)),
            pltpu.SemaphoreType.DMA((1,)),
        ],
        compiler_params=pltpu.CompilerParams(vmem_limit_bytes=110 * 1024 * 1024,
                                             disable_bounds_checks=True,
                                             disable_semaphore_checks=True),
        name="hedgehog_mod",
    )(x, A_wqkv, wphi, A_wo, wr, B_w_gate, B_w_up, B_w_down)
    return out.reshape(1, S, D)
```

```python
import jax
import jax.numpy as jnp
from jax import lax
import jax.experimental.pallas as pl
import jax.experimental.pallas.tpu as pltpu

S = 2048
D = 1024
H = 32
DH = 32
F = 3584
T = 512
NT = S // T
T0 = 256
B = 128
NB = S // B
BPI = 4
NI = NB // BPI
NP = H // 2
FC = 512
R = 16
NBV = 12
NCH = 4
OCH = 176
DCH = 1216
NV = 124
PR = NV * 4
HK = D // 2
P2 = 2 * B
LOG2E = 1.4426950408889634
LN_EPS = 1e-5
DEN_EPS = 1e-6

_NT_DIMS = (((1,), (1,)), ((), ()))
_TN_DIMS = (((0,), (0,)), ((), ()))

bf16 = jnp.bfloat16
f32 = jnp.float32
u32 = jnp.uint32


def _dot_nt(a, b):
    return lax.dot_general(a, b, _NT_DIMS, preferred_element_type=f32)


def _dot_nn(a, b):
    return jnp.dot(a, b, preferred_element_type=f32)


def _pk(x):
    return pltpu.bitcast(x, u32)


def _upk(x):
    return pltpu.bitcast(x, bf16)


def _lanes(x):
    return jnp.broadcast_to(x, (x.shape[0], 128))


def _layernorm(x):
    m = jnp.mean(x, axis=-1, keepdims=True)
    xc = x - m
    v = jnp.mean(xc * xc, axis=-1, keepdims=True)
    return xc * lax.rsqrt(v + LN_EPS)


def _allreduce8(x, op):
    x = op(x, pltpu.roll(x, 4, 1))
    x = op(x, pltpu.roll(x, 2, 1))
    x = op(x, pltpu.roll(x, 1, 1))
    return x


def _hedgehog_t(p, z=None):
    t = p.shape[-1]
    p4 = p.reshape(2, 4, 8, t)
    mx = _allreduce8(jnp.max(p4, axis=1), jnp.maximum)
    mn = _allreduce8(jnp.min(p4, axis=1), jnp.minimum)
    ep = jnp.exp2(p4 - mx[:, None])
    en = jnp.exp2(mn[:, None] - p4)
    a = pl.reciprocal(_allreduce8(jnp.sum(ep, axis=1), jnp.add), approx=True)
    b = pl.reciprocal(_allreduce8(jnp.sum(en, axis=1), jnp.add), approx=True)
    if z is not None:
        dp = jnp.sum(ep * z[0:64].reshape(2, 4, 8, t), axis=1)
        dn = jnp.sum(en * z[64:128].reshape(2, 4, 8, t), axis=1)
        den = _allreduce8(dp * a + dn * b, jnp.add) + DEN_EPS
        inv = pl.reciprocal(den, approx=True)
        a = a * inv
        b = b * inv
    fp = (ep * a[:, None]).reshape(64, t)
    fn = (en * b[:, None]).reshape(64, t)
    return jnp.concatenate([fp, fn], axis=0)


_SA = ((3, None, 0), (2, 3, 1), (0, 1, 1), (0, None, 0), (0, 3, 1), (1, 3, -1), (2, 0, -1))
_SB = ((2, 0, -1), (0, None, 0), (3, None, 0), (1, 3, -1), (0, 3, 1), (2, 3, 1), (0, 1, 1))


def _combo(blocks, spec):
    a, b, sign = spec
    if b is None:
        return blocks[a]
    return blocks[a] + blocks[b] if sign > 0 else blocks[a] - blocks[b]


def _strassen(product, emit):
    m4 = product(0)
    m2 = product(1)
    emit(2, m4 + m2)
    m5 = product(2)
    u = m4 - m5
    m3 = product(3)
    emit(1, m5 + m3)
    v = m3 - m2
    m1 = product(4)
    u = u + m1
    v = v + m1
    emit(0, u + product(5))
    emit(3, v + product(6))


def _head_groups(h):
    base, k = (NV // 4) * (h // 8), h % 8
    return ([base + 4 * k + i for i in range(3)],
            base + 4 * k - 1 if k > 0 else None,
            base + 4 * k + 3 if k < 7 else None,
            8 - k)


def _pair_logits(group, j):
    parts = []
    for h in (2 * j, 2 * j + 1):
        full, below, above, a = _head_groups(h)
        ref = group(full[0])
        sub = lax.broadcasted_iota(jnp.int32, ref.shape, 0)
        if above is None:
            m = jnp.where(sub >= a, group(below), 0.0)
        else:
            m = jnp.where(sub == a - 1, 0.0, group(above))
            if below is not None:
                m = jnp.where(sub >= a, group(below), m)
        parts += [m] + [group(q) for q in full]
    return jnp.concatenate(parts, axis=0)


def _pair_need(j):
    full, _, above, _ = _head_groups(2 * j + 1)
    return full[2] if above is None else above


def _tie(keep, w, ties):
    rows = sorted({r for r, _ in ties})
    out, pos = [], 0
    for r in rows:
        if r > pos:
            out.append(w[pos:r])
        cols = sorted(c for rr, c in ties if rr == r)
        parts, cpos = [], 0
        for c in cols:
            if c > cpos:
                parts.append(w[r:r + 8, cpos:c])
            parts.append(jnp.where(keep, w[r:r + 8, c:c + 128], ties[(r, c)]))
            cpos = c + 128
        if cpos < w.shape[1]:
            parts.append(w[r:r + 8, cpos:])
        out.append(jnp.concatenate(parts, axis=1) if len(parts) > 1 else parts[0])
        pos = r + 8
    if pos < w.shape[0]:
        out.append(w[pos:])
    return jnp.concatenate(out, axis=0)


def _vregs(x):
    if x.dtype != u32:
        x = pltpu.bitcast(x, u32)
    return [x[r:r + 8, c:c + 128] for r in range(0, x.shape[0], 8) for c in range(0, x.shape[1], 128)]


def _or_all(vals):
    acc = vals[0]
    for v in vals[1:]:
        acc = acc | v
    return acc


_KSTAGES = (((0, 1), (4, 1)), ((1, 2), (5, 1)), ((3, 1), (6, 2)))
_PSTAGES = (((0, 1), (4, 1)), ((1, 3), (5, 3)))
_NSEM_IN = 11


def _kernel(x_hbm, wqkv_hbm, wphi_hbm, wo_hbm, wr_hbm, wg_hbm, wu_hbm, wd_hbm,
            out_hbm,
            x_v, wqkv_v, wphi_v, wo_v, wr_v, wg_v, wu_v, wd_v,
            wtk_v, wsq_v, wsk_v, wsv_v, wso_v, wdp_v, amat_v, xn_v, xs_v, kvacc_v, zacc_v, kv_v, phi_v,
            pq0_v, pq1_v, pq2_v, pq3_v, oc0_v, oc1_v, h_v, st_v, pend_v, out_v, wrb_v,
            bestv_v, besti_v, flag_s,
            sem_i, sem_o):

    def cp_x(lo, n, sem):
        return pltpu.make_async_copy(x_hbm.at[pl.ds(lo, n)], x_v.at[pl.ds(lo, n)], sem_i.at[sem])

    def cp_w(lo, w, sem):
        return pltpu.make_async_copy(wqkv_hbm.at[:, pl.ds(lo, w)], wqkv_v.at[:, pl.ds(lo, w)], sem_i.at[sem])

    cp_k = [[cp_w(D + g * 128, n * 128, 2 + c) for g, n in st] for c, st in enumerate(_KSTAGES)]
    cp_p = [[pltpu.make_async_copy(wphi_hbm.at[pl.ds(g * 128, n * 128)], wphi_v.at[pl.ds(g * 128, n * 128)],
                                   sem_i.at[3 * c]) for g, n in st] for c, st in enumerate(_PSTAGES)]
    cp_wv = cp_w(2 * D, D, 5)
    cp_wq = cp_w(0, D, 7)

    def cp_wd(k):
        lo, n = k * DCH, min(DCH, F - k * DCH)
        return pltpu.make_async_copy(wd_hbm.at[pl.ds(lo, n)], wd_v.at[pl.ds(lo, n)], sem_i.at[(6, 8, 9)[k]])

    cp_x0 = cp_x(0, T0, 1)
    cp_x1 = cp_x(T0, T0, 4)
    cp_x2 = cp_x(T, P2, 5)
    cp_x3 = cp_x(T + P2, T, 6)
    cp_x4 = cp_x(2 * T + P2, S - 2 * T - P2, 8)
    cp_wr = pltpu.make_async_copy(wr_hbm, wr_v.at[pl.ds(0, 8)], sem_i.at[7])

    def cp_wo(k, half):
        lo, n = k * OCH, min(OCH, HK - k * OCH)
        rows = pl.ds(half * HK + lo, n)
        return pltpu.make_async_copy(wo_hbm.at[rows], wo_v.at[rows], sem_i.at[(6, 8, 9)[k]])

    def wait_bg(k):
        cp_wo(k, 0).wait()
        cp_wo(k, 1).wait()
        cp_wd(k).wait()

    cp_wg = pltpu.make_async_copy(wg_hbm, wg_v.at[:, pl.ds(0, F)], sem_i.at[10])
    cp_wu = pltpu.make_async_copy(wu_hbm, wu_v.at[:, pl.ds(0, F)], sem_i.at[10])

    def cp_out(b, n):
        lo = b * B
        if not isinstance(b, int):
            lo = pl.multiple_of(lo, B)
        return pltpu.make_async_copy(out_v.at[pl.ds(P2 + lo, n * B)], out_hbm.at[pl.ds(lo, n * B)], sem_o.at[0])

    for cp in (*cp_p[0], cp_x0, *cp_k[0], *cp_p[1], *cp_k[1], *cp_k[2], cp_x1, cp_wv, cp_x2,
               cp_x3, cp_wo(0, 0), cp_wo(0, 1), cp_wd(0), cp_x4, cp_wo(1, 0), cp_wo(1, 1), cp_wd(1),
               cp_wo(2, 0), cp_wo(2, 1), cp_wd(2), cp_wr, cp_wq, cp_wg, cp_wu):
        cp.start()
    flag_s[0] = 1
    flag_s[1] = 0

    def ln1(xg, src, xd, dst, n, which=None, keep=None, anchors=None, plain=False):
        pieces = []
        for pr in range(n // P2):
            for k in range(B // R):
                off = pr * P2 + k * R
                if which is not None and pr * (B // R) + k not in which:
                    continue
                x0 = xg[src + off:src + off + R, :].astype(f32)
                x1 = xg[src + off + B:src + off + B + R, :].astype(f32)
                if anchors is not None:
                    a = anchors[len(pieces)]
                    x0 = jnp.concatenate([jnp.where(keep, x0[:, :128], a), x0[:, 128:]], axis=1)
                    x1 = jnp.concatenate([jnp.where(keep, x1[:, :128], a), x1[:, 128:]], axis=1)
                p0 = _layernorm(x0)
                p1 = _layernorm(x1)
                if plain:
                    xn_v[off // 2:(off + R) // 2, :] = _pk(p0.astype(bf16))
                    xn_v[(off + B) // 2:(off + B + R) // 2, :] = _pk(p1.astype(bf16))
                lo = (dst + pr * P2) // 4 + k * (R // 2)
                blocks = (p0[:, :HK], p1[:, :HK], p0[:, HK:], p1[:, HK:])
                vs = []
                for m, spec in enumerate(_SB):
                    t = _combo(blocks, spec)
                    xd[lo:lo + R // 2, m * HK:(m + 1) * HK] = _pk(t.astype(bf16))
                    if spec[1] is not None:
                        vs.append(_vregs(t))
                pieces.append([_or_all(list(col)) for col in zip(*vs)])
        return pieces

    def load_xn(b):
        return _upk(xn_v[b * (B // 2):(b + 1) * (B // 2), :])

    def piece_ties(pieces, n, row0=0, col=0):
        ties = {}
        if pieces:
            step = (n - row0) // len(pieces) // 8 * 8
            for k, p in enumerate(pieces):
                for q, val in enumerate(p):
                    ties[(row0 + k * step + (q // 4) * 8, col + (q % 4) * 128)] = val
        return ties

    def xs_view(i, tiles):
        return xs_v.at[pl.ds(pl.multiple_of(i * (T // 4), T // 4), tiles * (T // 4))]

    def sproj(ws, xd, pr, emit, keep=None, work=None, before=None, after=None):
        lo = pr * (B // 2)

        def product(m):
            if before:
                before(m)
            lhs = ws[:, m * HK:(m + 1) * HK]
            if work is not None and work.get(m):
                lhs = _tie(keep, lhs, piece_ties(work[m], lhs.shape[0], 32))
            res = _dot_nt(_upk(lhs), _upk(xd[lo:lo + B // 2, m * HK:(m + 1) * HK]))
            if after:
                after(m, res)
            return res

        _strassen(product, lambda k, val: emit(k // 2, k % 2, val))

    def spread(pieces, slots):
        res = {}
        for k, (pr, m) in enumerate(slots):
            res.setdefault(pr, {})[m] = pieces[k * len(pieces) // len(slots):(k + 1) * len(pieces) // len(slots)]
        return res

    def sealed(ref):
        ref[pl.ds(pl.multiple_of(flag_s[1] + ref.shape[0] - 8, 8), 8), 0:128] = jnp.zeros((8, 128), u32)
        return ref

    def fence(ref, row, col):
        return ref[pl.ds(pl.multiple_of(flag_s[1] + row, 8), 8), col:col + 128]

    def store_combos(ws, row, top, bot, table=_SA, keep=None, dep=None):
        for c in range(0, HK, 128):
            blocks = [top[:, c:c + 128], top[:, HK + c:HK + c + 128], bot[:, c:c + 128], bot[:, HK + c:HK + c + 128]]
            if dep is not None:
                d = pltpu.bitcast(jnp.concatenate([dep, dep], axis=0), f32)
                for q in (0, 3):
                    blocks[q] = jnp.where(keep, blocks[q], d)
            for m, spec in enumerate(table):
                ws[row:row + 8, m * HK + c:m * HK + c + 128] = _pk(_combo(blocks, spec).astype(bf16))
            if dep is not None:
                dep = fence(ws, row, c)
        return dep

    zinit = set()

    def k_side(group, pairs, slot, keep=None, anchor=None):
        res = []
        for j in pairs:
            p = _pair_logits(group, j)
            if anchor is not None:
                p = jnp.concatenate([jnp.where(keep, p[0:8], anchor), p[8:32],
                                     jnp.where(keep, p[32:40], anchor), p[40:64]], axis=0)
            ph = _hedgehog_t(p)
            if j not in zinit:
                zinit.add(j)
                zacc_v[j * 128:(j + 1) * 128, :] = ph
            else:
                zacc_v[j * 128:(j + 1) * 128, :] += ph
            phi_v[j * 64:(j + 1) * 64, slot * B:(slot + 1) * B] = _pk(ph.astype(bf16))
            res.append(ph)
        return res

    def half_groups(p, half):
        return lambda pos: p[(pos - half * (NV // 2)) * 8:(pos - half * (NV // 2) + 1) * 8]

    def half_pairs(half):
        return range(half * (NP // 2), (half + 1) * (NP // 2))

    def kv_prod(vt, ph, j):
        half, r = j // (NP // 2), (j % (NP // 2)) * 64
        v = jnp.concatenate([vt[(s, half)][r:r + 64] for s in range(T // B)], axis=1).astype(bf16)
        return _dot_nt(v, ph)

    r_i = lax.broadcasted_iota(jnp.int32, (128, DH), 0)
    c_i = lax.broadcasted_iota(jnp.int32, (128, DH), 1)
    expand = (r_i % DH == c_i).astype(bf16)
    r_h = lax.broadcasted_iota(jnp.int32, (128, 128), 0) // DH
    c_h = lax.broadcasted_iota(jnp.int32, (128, 128), 1) // DH
    same_head = r_h == c_h

    def make_amat(g):
        a = _dot_nt(expand, wphi_v[g * 128:(g + 1) * 128, :])
        amat_v[:, g * 128:(g + 1) * 128] = _pk(jnp.where(same_head, a, 0.0).astype(bf16))

    class Folder:
        def __init__(self, col0, first=0):
            self.col0, self.rows, self.mprev, self.done = col0, {}, None, first

        def tile(self, g, rows, keep=None, ties=None):
            am = amat_v[:, g * 128:(g + 1) * 128]
            if ties:
                am = _tie(keep, am, ties)
            return _dot_nt(_upk(am), wqkv_v[rows, self.col0 + g * 128:self.col0 + (g + 1) * 128])

        def fold(self, g, wt=None):
            sub = lax.broadcasted_iota(jnp.int32, (8, D), 0)
            if wt is None:
                wt = self.tile(g, slice(None))
            for hh in range(4):
                full, below, _, a = _head_groups(4 * g + hh)
                r0 = hh * DH
                ref = jnp.broadcast_to(wt[r0 + a - 1:r0 + a, :], (8, D))
                part = [(wt[r0 + 8 * i:r0 + 8 * (i + 1)] - ref) * LOG2E for i in range(4)]
                if below is not None:
                    self.rows[below] = jnp.where(sub >= a, part[0], self.mprev)
                self.mprev = part[0]
                for q, v in zip(full, part[1:]):
                    self.rows[q] = v
            new = {}
            while self.done in self.rows and self.done + 1 in self.rows:
                new[self.done] = jnp.concatenate([self.rows.pop(self.done), self.rows.pop(self.done + 1)], axis=0)
                self.done += 2
            return new

    def fold_pair(folders, g, keep=None, ties=None):
        tiles = {}
        for n, c in enumerate(range(0, HK, 128)):
            for half in range(2):
                for side in range(2):
                    t = ties[n] if ties and half == 0 and side == 0 else None
                    lo = side * HK + c
                    tiles[(half, lo)] = folders[half].tile(g + 4 * half, slice(lo, lo + 128), keep, t)
        return [folders[half].fold(g + 4 * half,
                                   jnp.concatenate([tiles[(half, lo)] for lo in range(0, D, 128)], axis=1))
                for half in range(2)]

    bestv_v[...] = jnp.full(bestv_v.shape, -jnp.inf, f32)
    besti_v[...] = lax.broadcasted_iota(jnp.int32, besti_v.shape, 0)
    h_v[0:P2, :] = jnp.zeros((P2, D), f32)
    st_v[0:B, :] = jnp.zeros((B, 256), f32)
    pend_v[...] = jnp.zeros(pend_v.shape, f32)

    def wait_all(cps):
        for cp in cps:
            cp.wait()

    def amats(c):
        for g0, n in _PSTAGES[c]:
            for g in range(g0, g0 + n):
                make_amat(g)

    wait_all(cp_p[0])
    amats(0)

    cp_x0.wait()
    ln1(x_v, 0, xs_v, 0, T0, plain=True)
    xb = [load_xn(s) for s in range(2)]
    logits = [{}, {}]
    finished = [set(), set()]
    fk, slabs = (Folder(D), Folder(D, NV // 2)), {}
    defer, queue = [False], []

    def absorb(new):
        for pos, slab in new.items():
            wtk_v[pos * 4:pos * 4 + 8, :] = _pk(slab.astype(bf16))
            slabs[pos] = slab
        for pos in sorted(slabs):
            if pos < NV // 2 and pos + NV // 2 in slabs:
                store_combos(wsk_v, pos * 4, slabs.pop(pos), slabs.pop(pos + NV // 2))

    def k_finish(s, hold=0):
        ready = [j for j in range(NP) if j not in finished[s] and _pair_need(j) in logits[s]]
        ready = ready[:len(ready) - hold]
        if defer[0]:
            queue.extend((logits[s].__getitem__, [j], s) for j in ready)
        else:
            k_side(logits[s].__getitem__, ready, s)
        finished[s].update(ready)

    def k_chunk(s, keep=None, early=(), late=(), hold=0):
        todo = [q for half in range(2) for q in range(half * (NV // 2), fk[half].done) if q not in logits[s]]
        runs = [[q for q in todo if q < NV // 2], [q for q in todo if q >= NV // 2]]
        lhs = jnp.concatenate([wtk_v[r[0] * 4:(r[-1] + 1) * 4, :] for r in runs if r], axis=0)
        ties = piece_ties(early, lhs.shape[0])
        ties.update(piece_ties(late, lhs.shape[0], col=HK))
        if ties:
            lhs = _tie(keep, lhs, ties)
        p = _dot_nt(_upk(lhs), xb[s])
        for n, q in enumerate(todo):
            logits[s][q] = p[n * 8:(n + 1) * 8]
        k_finish(s, hold)
        return p

    wait_all(cp_k[0])
    for new in fold_pair(fk, 0):
        absorb(new)
    k_chunk(0)
    k_chunk(1, hold=1)

    wait_all(cp_p[1] + cp_k[1])
    k_finish(1)
    amats(1)
    for new in fold_pair(fk, 1):
        absorb(new)
    absorb(fk[0].fold(2))
    k_chunk(0)
    k_chunk(1, hold=1)

    wait_all(cp_k[2] + [cp_x1])
    defer[0] = True
    keep = flag_s[0] > 0
    absorb(fk[1].fold(6))
    new = fold_pair(fk, 3)
    late = list(new[0].values())[-1][:, 384:512]
    for n in new:
        absorb(n)
    pieces = ln1(x_v, T0, xs_v, T0, T0, [0]) + ln1(x_v, T0, xs_v, T0, T0, [1, 2], keep, [late, late])
    p = k_chunk(0, keep, (), pieces[:2])
    rows = [k * p.shape[0] // 5 // 16 * 16 for k in range(5)]
    pieces += ln1(x_v, T0, xs_v, T0, T0, range(3, 8), keep, [p[r:r + R] for r in rows])
    k_chunk(1, keep, pieces[2:3], pieces[3:])

    def k_emit1(half, blk, val):
        now = {(1, 0): 8, (0, 1): 6}.get((half, blk), 0)
        pairs = list(half_pairs(half))
        k_side(half_groups(val, half), pairs[:now], 2 + blk)
        queue.extend((half_groups(val, half), [j], 2 + blk) for j in pairs[now:])

    def run_queue(n, res):
        deps = []
        for k in range(min(n, len(queue))):
            r = k * res.shape[0] // n // 8 * 8
            v = _vregs(k_side(*queue.pop(0), keep=keep, anchor=res[r:r + 8])[0])
            deps.append([_or_all(v[q::4]) for q in range(4)])
        return deps

    kwork = {}

    def k_after(m, res):
        if m in (0, 2):
            kwork[m + 1] = run_queue(4, res)

    def k_before(m):
        if m == 4:
            cp_wv.wait()
            cp_x2.wait()
            for rb in range(0, HK, 128):
                for c in range(0, HK, 128):
                    raw = [wqkv_v[side * HK + c:side * HK + c + 128,
                                  2 * D + half * HK + rb:2 * D + half * HK + rb + 128].T
                           for half in range(2) for side in range(2)]
                    blocks = [t.astype(f32) for t in raw]
                    for n, spec in enumerate(_SA):
                        t = raw[spec[0]] if spec[1] is None else _combo(blocks, spec).astype(bf16)
                        wsv_v[rb // 2:rb // 2 + 64, n * HK + c:n * HK + c + 128] = _pk(t)

    sproj(wsk_v, xs_v, 1, k_emit1, keep, kwork, k_before, k_after)

    def ln_anchored(xg, src, xd, dst, k, n, keep, res):
        which = list(range(k * 8 // n, (k + 1) * 8 // n))
        rows = [a * HK // len(which) // 16 * 16 for a in range(len(which))]
        pcs = ln1(xg, src, xd, dst, P2, which, keep, [res[r:r + R] for r in rows])
        return [[]] * (3 - len(pcs)) + pcs

    vt = {}
    wsv = wsv_v.at[pl.ds(pl.multiple_of(flag_s[1], D // 4), D // 4)]
    work = {0: {}, 1: {}}

    def v_after(q):
        def after(m, res):
            t = 7 * q + m
            if t < 6:
                work[0][m + 1] = run_queue(-(-len(queue) // (6 - t)), res)
            elif t < 13:
                work[1][t - 6] = ln_anchored(x_v, T, xs_v, T, t - 6, 7, keep, res)
        return after

    for q in range(2):
        sproj(wsv, xs_v, q, lambda half, blk, val, q=q: vt.__setitem__((2 * q + blk, half), val),
              keep, work[q], None, v_after(q))
    assert not queue
    phi_m = sealed(phi_v)
    for j in range(NP):
        kvacc_v[j] = kv_prod(vt, _upk(phi_m[j * 64:(j + 1) * 64, :]), j)
    cp_x3.wait()
    wait_bg(0)

    def p1_body(i, c):
        @pl.when(i == 2)
        def _():
            cp_x4.wait()
            wait_bg(1)

        @pl.when(i == 3)
        def _():
            wait_bg(2)

        keep = flag_s[0] > 0
        lo = jnp.minimum((i - 1) * DCH, F - DCH)
        sv = wd_v.at[pl.ds(pl.multiple_of(lo, 16), DCH)]
        dv = wdp_v.at[pl.ds(pl.multiple_of(lo // 2, 8), DCH // 2)]
        deps = []
        for r in range(0, DCH, 16):
            val = _pk(sv[r:r + 16, :])
            dv[r // 2:r // 2 + 8, 0:D] = val
            deps.append([_or_all(_vregs(val))])
        lo = jnp.minimum((i - 1) * OCH, HK - OCH)
        ov = wo_v.at[pl.ds(pl.multiple_of(lo, 16), HK + OCH)]
        od = wso_v.at[pl.ds(pl.multiple_of(lo // 2, 8), OCH // 2)]
        work = spread(deps, [(q, m) for q in range(2) for m in (0, 2, 4)])

        def k_emit(q):
            return lambda half, blk, val: k_side(half_groups(val, half), half_pairs(half), 2 * q + blk)

        vt = {}

        def v_emit(q):
            return lambda half, blk, val: vt.__setitem__((2 * q + blk, half), val)

        def wo_chain(dep):
            for r in range(0, OCH, 16):
                dep = store_combos(od, r // 2, ov[r:r + 16, :].astype(f32), ov[HK + r:HK + r + 16, :].astype(f32),
                                   _SB, keep, dep)
            return dep

        xd = xs_view(i, 2)
        xa = x_v.at[pl.ds(pl.multiple_of(i * T + P2, P2), P2)]
        xb = x_v.at[pl.ds(pl.multiple_of(jnp.minimum(i + 1, NT - 1) * T, T), P2)]
        wa = {}

        def a_after(m, res):
            if m < 6:
                wa[m + 1] = ln_anchored(xa, 0, xd, P2, m, 6, keep, res)

        sproj(wsv_v, xd, 0, v_emit(0), keep, wa, None, a_after)
        sproj(wsk_v, xd, 0, k_emit(0), keep, work[0])
        sproj(wsk_v, xd, 1, k_emit(1), keep, work[1])
        wb = spread(ln1(xb, 0, xd, T, P2), [(0, m) for m in range(1, 7)])[0]

        def b_after(m, res):
            if m == 1:
                wb[5] = list(wb[5]) + [[wo_chain(pltpu.bitcast(res[0:8], u32))]]

        sproj(wsv_v, xd, 1, v_emit(1), keep, wb, None, b_after)
        phi_m = sealed(phi_v)
        for j in range(NP):
            kvacc_v[j] += kv_prod(vt, _upk(phi_m[j * 64:(j + 1) * 64, :]), j)
        return c

    lax.fori_loop(1, NT, p1_body, 0)

    cp_wr.wait()
    cp_wq.wait()
    keep = flag_s[0] > 0
    kv_mask = (lax.broadcasted_iota(jnp.int32, (64, 128), 0) // DH
               == (lax.broadcasted_iota(jnp.int32, (64, 128), 1) // DH) % 2)
    ties = [{} for _ in range(16)]
    for j in range(NP):
        kvj = jnp.where(kv_mask, kvacc_v[j], 0.0)
        kv_v[:, j * 128:(j + 1) * 128] = _pk(kvj.astype(bf16))
        zj = _lanes(jnp.sum(zacc_v[j * 128:(j + 1) * 128, :], axis=-1, keepdims=True))
        zacc_v[j * 128:(j + 1) * 128, :] = zj
        vals = _vregs(kvj) + _vregs(zj)
        if j + 1 < 16:
            for q in range(4):
                ties[j + 1][(32 + q * 8, 0)] = _or_all(vals[q::4])
    wr = wr_v[0:8, :].astype(f32)
    wl = jnp.sum(wr, axis=0, keepdims=True)
    wsum = jnp.sum(wl, axis=1, keepdims=True)
    wrb_v[:, 0:D + 256] = jnp.concatenate(
        [jnp.broadcast_to(wr[j:j + 1, :], (8, 128)) for j in range(8)]
        + [jnp.broadcast_to(wsum, (8, 128)), jnp.broadcast_to(wl, (8, 128))], axis=1)
    fq = (Folder(0), Folder(0, NV // 2))
    for g in range(4):
        new = fold_pair(fq, g, keep, ties[4 * g:4 * g + 4])
        for pos, slab in new[0].items():
            store_combos(wsq_v, pos * 4, slab, new[1][pos + NV // 2])

    pq_v = (pq0_v, pq1_v, pq2_v, pq3_v)

    def views_of(g):
        lo = g * (BPI * B)
        if not isinstance(g, int):
            lo = pl.multiple_of(lo, BPI * B)
        return ((x_v.at[pl.ds(lo, BPI * B)],)
                + tuple(ref.at[pl.ds(lo, P2 + BPI * B)] for ref in (h_v, out_v, st_v)) + (g,))

    def stage_q(xd, q):
        def emit(half, blk, val):
            group = half_groups(val, half)
            for j in half_pairs(half):
                ph = _hedgehog_t(_pair_logits(group, j), zacc_v[j * 128:(j + 1) * 128, :])
                pq_v[2 * q + blk][(j // 2) * 64:(j // 2 + 1) * 64, (j % 2) * B:(j % 2 + 1) * B] = _pk(ph.astype(bf16))

        sproj(wsq_v, xd, q, emit)

    oc_v = (oc0_v, oc1_v)

    def stage_g(q):
        pq = [sealed(pq_v[2 * q + blk]) for blk in range(2)]
        for jj in range(NP // 2):
            blocks = [_dot_nn(_upk(kv_v[:, j * 128:(j + 1) * 128]),
                              _upk(pq[blk][(j // 2) * 64:(j // 2 + 1) * 64, (j % 2) * B:(j % 2 + 1) * B]))
                      for blk in range(2) for j in (jj, jj + NP // 2)]
            for m, spec in enumerate(_SA):
                oc_v[q][jj * 32:(jj + 1) * 32, m * B:(m + 1) * B] = _pk(_combo(blocks, spec).astype(bf16))

    def stage_h(views, q, keep, pieces):
        x_g, h_g = views[0], views[1]
        oc = sealed(oc_v[q])
        first, last = 3, 22
        ties = [{} for _ in range(7)]
        for k, vals in enumerate(pieces):
            t = first + k * (last - first) // max(len(pieces) - 1, 1)
            for m, val in enumerate(vals):
                ties[t // 4][(m * 8, (t % 4) * 128)] = val
        state = {}
        done = [0]

        def product(m):
            w = wso_v[:, m * HK:(m + 1) * HK]
            if ties[m]:
                w = _tie(keep, w, ties[m])
            done[0] = m
            return lax.dot_general(_upk(oc[0:HK // 2, m * B:(m + 1) * B]), _upk(w), _TN_DIMS,
                                   preferred_element_type=f32)

        def wmul(d, lo):
            return (d.reshape(B // 8, 8, 128) * wrb_v[:, lo:lo + 128][None]).reshape(B, 128)

        def emit(k, val):
            blk, half = k // 2, k % 2
            s = 2 * q + blk
            cols = slice(half * HK, (half + 1) * HK)
            h = x_g[s * B:(s + 1) * B, cols].astype(f32) + val
            h_g[(s + 2) * B:(s + 3) * B, cols] = h
            st = state.setdefault(blk, {'h': {}})
            st['h'][half] = h
            for c in range(0, HK, 128):
                ht = h[:, c:c + 128]
                if 'h0' not in st:
                    st['h0'] = ht
                    continue
                d = ht - st['h0']
                new = (d, d * d, wmul(d, half * HK + c))
                st['s'] = new if 's' not in st else tuple(a + b for a, b in zip(st['s'], new))
            if len(st['h']) == 1:
                vals = [_or_all(list(v)) for v in zip(*[_vregs(a) for a in st['s']])]
                m = done[0] + 2
                for n, val in enumerate(vals):
                    ties[m][(248 - (n % 4) * 8, (n // 4) * 128)] = val

        _strassen(product, emit)

        res = []
        for blk in range(2):
            st = state[blk]
            s1, s2, s3 = st['s']
            c0 = _lanes(jnp.mean(st['h0'], axis=-1, keepdims=True))
            g0 = st['h0'] - c0
            t1 = s1 + 8.0 * g0
            t2 = s2 + g0 * (s1 + t1)
            t3 = s3 + wmul(g0, D + 128)
            res.append((jnp.concatenate([t1, t2, t3, c0], axis=1),
                        jnp.concatenate([st['h'][0], st['h'][1]], axis=1)))
        return res

    def stage_stats(views, s, part, valid=None):
        st_g, g = views[3], views[4]
        b = g * BPI + s
        bv = bestv_v[...]
        bi = besti_v[...]
        wsum = wrb_v[0:1, D:D + 128]
        nvs, nis, sts = [], [], []
        for k in range(B // R):
            sl = slice(k * R, (k + 1) * R)
            red = [_lanes(jnp.sum(part[sl, n * 128:(n + 1) * 128], axis=-1, keepdims=True)) for n in range(3)]
            mu = red[0] * (1.0 / D)
            var = jnp.maximum(red[1] * (1.0 / D) - mu * mu, 0.0)
            rs = lax.rsqrt(var + LN_EPS)
            r = (red[2] - mu * wsum) * rs
            sts.append(jnp.concatenate([rs, (mu + part[sl, 384:512]) * rs], axis=1))
            if valid is not None:
                r = jnp.where(valid, r, -jnp.inf)
            idx = lax.broadcasted_iota(jnp.int32, (R, 128), 0) + (b * B + k * R)
            better = r > bv[sl]
            nvs.append(jnp.where(better, r, bv[sl]))
            nis.append(jnp.where(better, idx, bi[sl]))
        st = jnp.concatenate(sts, axis=0)
        st_g[(s + 2) * B:(s + 3) * B, :] = st
        bestv_v[...] = jnp.concatenate(nvs, axis=0)
        besti_v[...] = jnp.concatenate(nis, axis=0)
        return st, nvs

    def stage_out(views, s, st=None, h=None):
        h_g, out_g, st_g = views[1], views[2], views[3]
        rows = slice((s + 2) * B, (s + 3) * B)
        h = h_g[rows, :] if h is None else h
        st = st_g[rows, :] if st is None else st
        outs = []
        for k in range(B // R):
            sl = slice(k * R, (k + 1) * R)
            a = 1.0 + st[sl, 0:128]
            outs.append(jnp.concatenate([h[sl, c * 128:(c + 1) * 128] * a - st[sl, 128:256]
                                         for c in range(D // 128)], axis=1))
        out_g[rows, :] = jnp.concatenate([o.astype(bf16) for o in outs], axis=0)
        return [_vregs(o) for o in outs]

    def stage_i(views, s, part, h=None, valid=None):
        st, nvs = stage_stats(views, s, part, valid)
        return [o + _vregs(nv) for o, nv in zip(stage_out(views, s, st, h), nvs)]

    def p2_body(i, c):
        b0 = i * BPI
        keep = flag_s[0] > 0
        cur = views_of(i)
        pieces = stage_out(cur, -2) + stage_i(cur, -1, pend_v[...], valid=i > 0)
        for q in range(2):
            stage_q(xs_view(i, 1), q)
        stage_g(0)
        stage_g(1)
        res = stage_h(cur, 0, keep, pieces)
        pieces = stage_i(cur, 0, *res[0]) + stage_i(cur, 1, *res[1])
        res = stage_h(cur, 1, keep, pieces)
        stage_stats(cur, BPI - 2, res[0][0])
        pend_v[...] = res[1][0]

        @pl.when(i > 0)
        def _():
            cp_out(jnp.maximum(b0 - 2, 0), 2).start()

        cp_out(b0, 2).start()
        return c

    lax.fori_loop(0, NI, p2_body, 0)
    cp_wg.wait()
    cp_wu.wait()
    keep = flag_s[0] > 0
    last = views_of(NI - 1)

    st, _ = stage_stats(last, BPI - 1, pend_v[...])

    bv = bestv_v[...]
    mval = jnp.max(bv, axis=0, keepdims=True)
    sel = jnp.min(jnp.where(bv == mval, besti_v[...], S - 1), axis=0, keepdims=True)
    idx = sel[0, 0]
    sel_f = jnp.broadcast_to(pltpu.bitcast(sel, f32), (B, 128))
    for s, stv in ((BPI - 2, last[3][BPI * B:(BPI + 1) * B, :]), (BPI - 1, st)):
        stage_out(last, s, jnp.concatenate([jnp.where(keep, stv[:, 0:128], sel_f), stv[:, 128:256]], axis=1))
    ofence = out_v[pl.ds(pl.multiple_of(flag_s[1] + S, R), R), 0:128].astype(f32)
    cp_out(NB - 2, 2).start()
    hrow = h_v[pl.ds(P2 + idx, 1), :]
    strow = st_v[pl.ds(P2 + idx, 1), :]
    xrow = jnp.concatenate([hrow[:, c * 128:(c + 1) * 128] * strow[:, 0:128] - strow[:, 128:256]
                            for c in range(D // 128)], axis=1).astype(bf16)
    xs = jnp.broadcast_to(xrow, (16, D))

    def act(g, u):
        a = g * pl.reciprocal(1.0 + jnp.exp(-g), approx=True) * u
        return jnp.concatenate([a, a], axis=0).astype(bf16)

    def down(a, lo, w):
        return _dot_nn(a, _upk(wdp_v[lo // 2:(lo + w) // 2, 0:D]))[0:8]

    NM = F - NBV * 128
    xcol = jnp.broadcast_to(xrow.astype(f32), (128, D)).T
    jobs = [(which, b) for b in range(NBV) for which in (0, 1)]
    vres, prev = {}, None
    for j0 in range(0, len(jobs), NCH):
        grp = jobs[j0:j0 + NCH]
        accs = [None] * len(grp)
        for r in range(D // 16):
            for n, (which, b) in enumerate(grp):
                w = (wg_v, wu_v)[which][r * 16:(r + 1) * 16, NM + b * 128:NM + (b + 1) * 128].astype(f32)
                t0 = w[0:8] * xcol[r * 16:r * 16 + 8]
                t1 = w[8:16] * xcol[r * 16 + 8:r * 16 + 16]
                if accs[n] is None:
                    if prev is not None:
                        t0 = jnp.where(keep, t0, prev[n % len(prev)])
                    accs[n] = t0 + t1
                else:
                    if j0 == 0 and n == 0 and r == 40:
                        t0 = jnp.where(keep, t0, ofence[0:8])
                    accs[n] = (accs[n] + t0) + t1
        prev = accs
        for n, job in enumerate(grp):
            vres[job] = _allreduce8(accs[n][None], jnp.add)[0]

    chunks = [(lo, min(FC, NM - lo)) for lo in range(0, NM, FC)]
    acts, y = [], None
    for k, (lo, w) in enumerate(chunks):
        g = _dot_nn(xs, wg_v[:, lo:lo + w])
        u = _dot_nn(xs, wu_v[:, lo:lo + w])
        acts.append(act(g[0:8], u[0:8]))
        if k >= 1:
            t = down(acts[k - 1], *chunks[k - 1])
            y = t if y is None else y + t
    y = y + down(acts[-1], *chunks[-1])
    for b0, nb in ((0, 4), (4, 4), (8, 3), (11, 1)):
        g = jnp.concatenate([vres[(0, b)] for b in range(b0, b0 + nb)], axis=1)
        u = jnp.concatenate([vres[(1, b)] for b in range(b0, b0 + nb)], axis=1)
        y = y + down(act(g, u), NM + b0 * 128, nb * 128)

    gate = jnp.broadcast_to(jax.nn.sigmoid(mval), (8, 128))
    base = pl.multiple_of((idx >> 4) << 4, 16)
    rows = pl.ds(pl.multiple_of(P2 + base, 16), 16)
    h16 = h_v[rows, :]
    st16 = st_v[rows, :]
    a16 = 1.0 + st16[:, 0:128]
    m16 = st16[:, 128:256]
    hit = (lax.broadcasted_iota(jnp.int32, (16, 128), 0) + base) == idx
    res = []
    for c in range(D // 128):
        yc = y[:, c * 128:(c + 1) * 128] * gate
        yc = jnp.concatenate([yc, yc], axis=0)
        res.append(h16[:, c * 128:(c + 1) * 128] * a16 - m16 + jnp.where(hit, yc, 0.0))
    res = jnp.concatenate(res, axis=1).astype(bf16)
    for i in range(NI):
        cp_out(i * BPI, 2).wait()
        cp_out(i * BPI + 2, 2).wait()
    out_v[rows, :] = res
    fix = pltpu.make_async_copy(out_v.at[rows], out_hbm.at[pl.ds(base, 16)], sem_o.at[0])
    fix.start()
    fix.wait()


@jax.jit
def pallas_sequential_preLN__linear_kernel_hedgehog__moe_arch_mod__prompt_kernel(
    A_x: jax.Array,
    A_wqkv: jax.Array,
    A_w_phi: jax.Array,
    A_wo: jax.Array,
    B_x: jax.Array,
    B_w_r: jax.Array,
    B_w_gate: jax.Array,
    B_w_up: jax.Array,
    B_w_down: jax.Array,
):
    del B_x
    x = A_x.reshape(S, D)
    wphi = A_w_phi.reshape(H * DH, DH)
    wr = B_w_r.reshape(8, 128)
    any_spec = pl.BlockSpec(memory_space=pl.ANY)
    out = pl.pallas_call(
        _kernel,
        out_shape=jax.ShapeDtypeStruct((S, D), bf16),
        in_specs=[any_spec] * 8,
        out_specs=any_spec,
        scratch_shapes=[
            pltpu.VMEM((S, D), bf16),
            pltpu.VMEM((D, 3 * D), bf16),
            pltpu.VMEM((H * DH, DH), bf16),
            pltpu.VMEM((D, D), bf16),
            pltpu.VMEM((64, 128), bf16),
            pltpu.VMEM((D, F + 128), bf16),
            pltpu.VMEM((D, F + 128), bf16),
            pltpu.VMEM((F, D), bf16),
            pltpu.VMEM((PR, D), u32),
            pltpu.VMEM((PR // 2, 7 * HK), u32),
            pltpu.VMEM((PR // 2, 7 * HK), u32),
            pltpu.VMEM((D // 4, 7 * HK), u32),
            pltpu.VMEM((D // 4, 7 * HK), u32),
            pltpu.VMEM((F // 2, D + 128), u32),
            pltpu.VMEM((64, 8 * 128), u32),
            pltpu.VMEM((T0 // 2, D), u32),
            pltpu.VMEM(((S + T) // 4, 7 * HK), u32),
            pltpu.VMEM((NP, 64, 128), f32),
            pltpu.VMEM((2 * D, 128), f32),
            pltpu.VMEM((32, NP * 128), u32),
            pltpu.VMEM((D + 8, T), u32),
            pltpu.VMEM((D // 2 + 16, 2 * B), u32),
            pltpu.VMEM((D // 2 + 16, 2 * B), u32),
            pltpu.VMEM((D // 2 + 16, 2 * B), u32),
            pltpu.VMEM((D // 2 + 16, 2 * B), u32),
            pltpu.VMEM((HK // 2 + 32, 7 * B), u32),
            pltpu.VMEM((HK // 2 + 32, 7 * B), u32),
            pltpu.VMEM((P2 + S, D), f32),
            pltpu.VMEM((P2 + S, 256), f32),
            pltpu.VMEM((B, 512), f32),
            pltpu.VMEM((P2 + S, D), bf16),
            pltpu.VMEM((8, D + 512), f32),
            pltpu.VMEM((B, 128), f32),
            pltpu.VMEM((B, 128), jnp.int32),
            pltpu.SMEM((2,), jnp.int32),
            pltpu.SemaphoreType.DMA((_NSEM_IN,)),
            pltpu.SemaphoreType.DMA((1,)),
        ],
        compiler_params=pltpu.CompilerParams(vmem_limit_bytes=110 * 1024 * 1024,
                                             disable_bounds_checks=True,
                                             disable_semaphore_checks=True),
        name="hedgehog_mod",
    )(x, A_wqkv, wphi, A_wo, wr, B_w_gate, B_w_up, B_w_down)
    return out.reshape(1, S, D)
```

```python
import jax
import jax.numpy as jnp
from jax import lax
import jax.experimental.pallas as pl
import jax.experimental.pallas.tpu as pltpu

S = 2048
D = 1024
H = 32
DH = 32
F = 3584
T = 512
NT = S // T
T0 = 256
B = 128
NB = S // B
BPI = 4
NI = NB // BPI
NP = H // 2
FC = 1024
R = 16
NBV = 12
NCH = 4
OCH = 176
DCH = 1216
NV = 124
PR = NV * 4
HK = D // 2
P2 = 2 * B
LOG2E = 1.4426950408889634
LN_EPS = 1e-5
DEN_EPS = 1e-6

_NT_DIMS = (((1,), (1,)), ((), ()))
_TN_DIMS = (((0,), (0,)), ((), ()))

bf16 = jnp.bfloat16
f32 = jnp.float32
u32 = jnp.uint32


def _dot_nt(a, b):
    return lax.dot_general(a, b, _NT_DIMS, preferred_element_type=f32)


def _dot_nn(a, b):
    return jnp.dot(a, b, preferred_element_type=f32)


def _pk(x):
    return pltpu.bitcast(x, u32)


def _upk(x):
    return pltpu.bitcast(x, bf16)


def _lanes(x):
    return jnp.broadcast_to(x, (x.shape[0], 128))


def _layernorm(x):
    m = jnp.mean(x, axis=-1, keepdims=True)
    xc = x - m
    v = jnp.mean(xc * xc, axis=-1, keepdims=True)
    return xc * lax.rsqrt(v + LN_EPS)


def _allreduce8(x, op):
    x = op(x, pltpu.roll(x, 4, 1))
    x = op(x, pltpu.roll(x, 2, 1))
    x = op(x, pltpu.roll(x, 1, 1))
    return x


def _hedgehog_t(p, z=None):
    t = p.shape[-1]
    p4 = p.reshape(2, 4, 8, t)
    mx = _allreduce8(jnp.max(p4, axis=1), jnp.maximum)
    mn = _allreduce8(jnp.min(p4, axis=1), jnp.minimum)
    ep = jnp.exp2(p4 - mx[:, None])
    en = jnp.exp2(mn[:, None] - p4)
    a = pl.reciprocal(_allreduce8(jnp.sum(ep, axis=1), jnp.add), approx=True)
    b = pl.reciprocal(_allreduce8(jnp.sum(en, axis=1), jnp.add), approx=True)
    if z is not None:
        dp = jnp.sum(ep * z[0:64].reshape(2, 4, 8, t), axis=1)
        dn = jnp.sum(en * z[64:128].reshape(2, 4, 8, t), axis=1)
        den = _allreduce8(dp * a + dn * b, jnp.add) + DEN_EPS
        inv = pl.reciprocal(den, approx=True)
        a = a * inv
        b = b * inv
    fp = (ep * a[:, None]).reshape(64, t)
    fn = (en * b[:, None]).reshape(64, t)
    return jnp.concatenate([fp, fn], axis=0)


_SA = ((3, None, 0), (2, 3, 1), (0, 1, 1), (0, None, 0), (0, 3, 1), (1, 3, -1), (2, 0, -1))
_SB = ((2, 0, -1), (0, None, 0), (3, None, 0), (1, 3, -1), (0, 3, 1), (2, 3, 1), (0, 1, 1))


def _combo(blocks, spec):
    a, b, sign = spec
    if b is None:
        return blocks[a]
    return blocks[a] + blocks[b] if sign > 0 else blocks[a] - blocks[b]


def _strassen(product, emit):
    m4 = product(0)
    m2 = product(1)
    emit(2, m4 + m2)
    m5 = product(2)
    u = m4 - m5
    m3 = product(3)
    emit(1, m5 + m3)
    v = m3 - m2
    m1 = product(4)
    u = u + m1
    v = v + m1
    emit(0, u + product(5))
    emit(3, v + product(6))


def _head_groups(h):
    base, k = (NV // 4) * (h // 8), h % 8
    return ([base + 4 * k + i for i in range(3)],
            base + 4 * k - 1 if k > 0 else None,
            base + 4 * k + 3 if k < 7 else None,
            8 - k)


def _pair_logits(group, j):
    parts = []
    for h in (2 * j, 2 * j + 1):
        full, below, above, a = _head_groups(h)
        ref = group(full[0])
        sub = lax.broadcasted_iota(jnp.int32, ref.shape, 0)
        if above is None:
            m = jnp.where(sub >= a, group(below), 0.0)
        else:
            m = jnp.where(sub == a - 1, 0.0, group(above))
            if below is not None:
                m = jnp.where(sub >= a, group(below), m)
        parts += [m] + [group(q) for q in full]
    return jnp.concatenate(parts, axis=0)


def _pair_need(j):
    full, _, above, _ = _head_groups(2 * j + 1)
    return full[2] if above is None else above


def _tie(keep, w, ties):
    rows = sorted({r for r, _ in ties})
    out, pos = [], 0
    for r in rows:
        if r > pos:
            out.append(w[pos:r])
        cols = sorted(c for rr, c in ties if rr == r)
        parts, cpos = [], 0
        for c in cols:
            if c > cpos:
                parts.append(w[r:r + 8, cpos:c])
            parts.append(jnp.where(keep, w[r:r + 8, c:c + 128], ties[(r, c)]))
            cpos = c + 128
        if cpos < w.shape[1]:
            parts.append(w[r:r + 8, cpos:])
        out.append(jnp.concatenate(parts, axis=1) if len(parts) > 1 else parts[0])
        pos = r + 8
    if pos < w.shape[0]:
        out.append(w[pos:])
    return jnp.concatenate(out, axis=0)


def _vregs(x):
    if x.dtype != u32:
        x = pltpu.bitcast(x, u32)
    return [x[r:r + 8, c:c + 128] for r in range(0, x.shape[0], 8) for c in range(0, x.shape[1], 128)]


def _or_all(vals):
    acc = vals[0]
    for v in vals[1:]:
        acc = acc | v
    return acc


_KSTAGES = (((0, 1), (4, 1)), ((1, 2), (5, 1)), ((3, 1), (6, 2)))
_PSTAGES = (((0, 1), (4, 1)), ((1, 3), (5, 3)))
_NSEM_IN = 11


def _kernel(x_hbm, wqkv_hbm, wphi_hbm, wo_hbm, wr_hbm, wg_hbm, wu_hbm, wd_hbm,
            out_hbm,
            x_v, wqkv_v, wphi_v, wo_v, wr_v, wg_v, wu_v, wd_v,
            wtk_v, wsq_v, wsk_v, wsv_v, wso_v, wdp_v, amat_v, xn_v, xs_v, xt_v, kvacc_v, zacc_v, kv_v, phi_v,
            pq0_v, pq1_v, pq2_v, pq3_v, oc0_v, oc1_v, h_v, st_v, pend_v, out_v, wrb_v,
            bestv_v, besti_v, flag_s,
            sem_i, sem_o):

    def cp_x(lo, n, sem):
        return pltpu.make_async_copy(x_hbm.at[pl.ds(lo, n)], x_v.at[pl.ds(lo, n)], sem_i.at[sem])

    def cp_w(lo, w, sem):
        return pltpu.make_async_copy(wqkv_hbm.at[:, pl.ds(lo, w)], wqkv_v.at[:, pl.ds(lo, w)], sem_i.at[sem])

    cp_k = [[cp_w(D + g * 128, n * 128, 2 + c) for g, n in st] for c, st in enumerate(_KSTAGES)]
    cp_p = [[pltpu.make_async_copy(wphi_hbm.at[pl.ds(g * 128, n * 128)], wphi_v.at[pl.ds(g * 128, n * 128)],
                                   sem_i.at[3 * c]) for g, n in st] for c, st in enumerate(_PSTAGES)]
    cp_wv = cp_w(2 * D, D, 5)
    cp_wq = cp_w(0, D, 7)

    def cp_wd(k):
        lo, n = k * DCH, min(DCH, F - k * DCH)
        return pltpu.make_async_copy(wd_hbm.at[pl.ds(lo, n)], wd_v.at[pl.ds(lo, n)], sem_i.at[(6, 8, 9)[k]])

    cp_x0 = cp_x(0, T0, 1)
    cp_x1 = cp_x(T0, T0, 4)
    cp_x2 = cp_x(T, P2, 5)
    cp_x3 = cp_x(T + P2, T, 6)
    cp_x4 = cp_x(2 * T + P2, S - 2 * T - P2, 8)
    cp_wr = pltpu.make_async_copy(wr_hbm, wr_v.at[pl.ds(0, 8)], sem_i.at[7])

    def cp_wo(k, half):
        lo, n = k * OCH, min(OCH, HK - k * OCH)
        rows = pl.ds(half * HK + lo, n)
        return pltpu.make_async_copy(wo_hbm.at[rows], wo_v.at[rows], sem_i.at[(6, 8, 9)[k]])

    def wait_bg(k):
        cp_wo(k, 0).wait()
        cp_wo(k, 1).wait()
        cp_wd(k).wait()

    cp_wg = pltpu.make_async_copy(wg_hbm, wg_v.at[:, pl.ds(0, F)], sem_i.at[10])
    cp_wu = pltpu.make_async_copy(wu_hbm, wu_v.at[:, pl.ds(0, F)], sem_i.at[10])

    def cp_out(b, n):
        lo = b * B
        if not isinstance(b, int):
            lo = pl.multiple_of(lo, B)
        return pltpu.make_async_copy(out_v.at[pl.ds(P2 + lo, n * B)], out_hbm.at[pl.ds(lo, n * B)], sem_o.at[0])

    for cp in (*cp_p[0], cp_x0, *cp_k[0], *cp_p[1], *cp_k[1], *cp_k[2], cp_x1, cp_wv, cp_x2,
               cp_x3, cp_wo(0, 0), cp_wo(0, 1), cp_wd(0), cp_x4, cp_wo(1, 0), cp_wo(1, 1), cp_wd(1),
               cp_wo(2, 0), cp_wo(2, 1), cp_wd(2), cp_wr, cp_wq, cp_wg, cp_wu):
        cp.start()
    flag_s[0] = 1
    flag_s[1] = 0

    def ln1(xg, src, xd, dst, n, which=None, keep=None, anchors=None, plain=False):
        pieces = []
        for pr in range(n // P2):
            for k in range(B // R):
                off = pr * P2 + k * R
                if which is not None and pr * (B // R) + k not in which:
                    continue
                x0 = xg[src + off:src + off + R, :].astype(f32)
                x1 = xg[src + off + B:src + off + B + R, :].astype(f32)
                if anchors is not None:
                    a = anchors[len(pieces)]
                    x0 = jnp.concatenate([jnp.where(keep, x0[:, :128], a), x0[:, 128:]], axis=1)
                    x1 = jnp.concatenate([jnp.where(keep, x1[:, :128], a), x1[:, 128:]], axis=1)
                p0 = _layernorm(x0)
                p1 = _layernorm(x1)
                if plain:
                    xn_v[off // 2:(off + R) // 2, :] = _pk(p0.astype(bf16))
                    xn_v[(off + B) // 2:(off + B + R) // 2, :] = _pk(p1.astype(bf16))
                lo = (dst + pr * P2) // 4 + k * (R // 2)
                blocks = (p0[:, :HK], p1[:, :HK], p0[:, HK:], p1[:, HK:])
                vs = []
                for m, spec in enumerate(_SB):
                    t = _combo(blocks, spec)
                    xd[lo:lo + R // 2, m * HK:(m + 1) * HK] = _pk(t.astype(bf16))
                    if spec[1] is not None:
                        vs.append(_vregs(t))
                pieces.append([_or_all(list(col)) for col in zip(*vs)])
        return pieces

    def load_xn(b):
        return _upk(xn_v[b * (B // 2):(b + 1) * (B // 2), :])

    def piece_ties(pieces, n, row0=0, col=0):
        ties = {}
        if pieces:
            step = (n - row0) // len(pieces) // 8 * 8
            for k, p in enumerate(pieces):
                for q, val in enumerate(p):
                    ties[(row0 + k * step + (q // 4) * 8, col + (q % 4) * 128)] = val
        return ties

    def xs_view(i, tiles):
        return xs_v.at[pl.ds(pl.multiple_of(i * (T // 4), T // 4), tiles * (T // 4))]

    def xt_view(i):
        lo = i * (HK // 2)
        return xt_v.at[pl.ds(lo if isinstance(i, int) else pl.multiple_of(lo, HK // 2), HK // 2)]

    def store_xt(i, xd, row):
        xt_view(i)[...] = _pk(_upk(xd[row:row + B // 2, 0:HK]).T)

    def sproj(ws, xd, pr, emit, keep=None, work=None, before=None, after=None, first=None):
        lo = pr * (B // 2)

        def product(m):
            if before:
                before(m)
            lhs = ws[:, m * HK:(m + 1) * HK]
            if work is not None and work.get(m):
                lhs = _tie(keep, lhs, piece_ties(work[m], lhs.shape[0], 32))
            if m == 0 and first is not None:
                res = _dot_nn(_upk(lhs), _upk(first[...]))
            else:
                res = _dot_nt(_upk(lhs), _upk(xd[lo:lo + B // 2, m * HK:(m + 1) * HK]))
            if after:
                after(m, res)
            return res

        _strassen(product, lambda k, val: emit(k // 2, k % 2, val))

    def spread(pieces, slots):
        res = {}
        for k, (pr, m) in enumerate(slots):
            res.setdefault(pr, {})[m] = pieces[k * len(pieces) // len(slots):(k + 1) * len(pieces) // len(slots)]
        return res

    def sealed(ref):
        ref[pl.ds(pl.multiple_of(flag_s[1] + ref.shape[0] - 8, 8), 8), 0:128] = jnp.zeros((8, 128), u32)
        return ref

    def fence(ref, row, col):
        return ref[pl.ds(pl.multiple_of(flag_s[1] + row, 8), 8), col:col + 128]

    def store_combos(ws, row, top, bot, table=_SA, keep=None, dep=None):
        for c in range(0, HK, 128):
            blocks = [top[:, c:c + 128], top[:, HK + c:HK + c + 128], bot[:, c:c + 128], bot[:, HK + c:HK + c + 128]]
            if dep is not None:
                d = pltpu.bitcast(jnp.concatenate([dep, dep], axis=0), f32)
                for q in (0, 3):
                    blocks[q] = jnp.where(keep, blocks[q], d)
            for m, spec in enumerate(table):
                ws[row:row + 8, m * HK + c:m * HK + c + 128] = _pk(_combo(blocks, spec).astype(bf16))
            if dep is not None:
                dep = fence(ws, row, c)
        return dep

    zinit = set()

    def k_side(group, pairs, slot, keep=None, anchor=None):
        res = []
        for j in pairs:
            p = _pair_logits(group, j)
            if anchor is not None:
                p = jnp.concatenate([jnp.where(keep, p[0:8], anchor), p[8:32],
                                     jnp.where(keep, p[32:40], anchor), p[40:64]], axis=0)
            ph = _hedgehog_t(p)
            if j not in zinit:
                zinit.add(j)
                zacc_v[j * 128:(j + 1) * 128, :] = ph
            else:
                zacc_v[j * 128:(j + 1) * 128, :] += ph
            phi_v[j * 64:(j + 1) * 64, slot * B:(slot + 1) * B] = _pk(ph.astype(bf16))
            res.append(ph)
        return res

    def half_groups(p, half):
        return lambda pos: p[(pos - half * (NV // 2)) * 8:(pos - half * (NV // 2) + 1) * 8]

    def half_pairs(half):
        return range(half * (NP // 2), (half + 1) * (NP // 2))

    def kv_prod(vt, ph, j):
        half, r = j // (NP // 2), (j % (NP // 2)) * 64
        v = jnp.concatenate([vt[(s, half)][r:r + 64] for s in range(T // B)], axis=1).astype(bf16)
        return _dot_nt(v, ph)

    r_i = lax.broadcasted_iota(jnp.int32, (128, DH), 0)
    c_i = lax.broadcasted_iota(jnp.int32, (128, DH), 1)
    expand = (r_i % DH == c_i).astype(bf16)
    r_h = lax.broadcasted_iota(jnp.int32, (128, 128), 0) // DH
    c_h = lax.broadcasted_iota(jnp.int32, (128, 128), 1) // DH
    same_head = r_h == c_h

    def make_amat(g):
        a = _dot_nt(expand, wphi_v[g * 128:(g + 1) * 128, :])
        amat_v[:, g * 128:(g + 1) * 128] = _pk(jnp.where(same_head, a, 0.0).astype(bf16))

    class Folder:
        def __init__(self, col0, first=0):
            self.col0, self.rows, self.mprev, self.done = col0, {}, None, first

        def tile(self, g, rows, keep=None, ties=None):
            am = amat_v[:, g * 128:(g + 1) * 128]
            if ties:
                am = _tie(keep, am, ties)
            return _dot_nt(_upk(am), wqkv_v[rows, self.col0 + g * 128:self.col0 + (g + 1) * 128])

        def fold(self, g, wt=None):
            sub = lax.broadcasted_iota(jnp.int32, (8, D), 0)
            if wt is None:
                wt = self.tile(g, slice(None))
            for hh in range(4):
                full, below, _, a = _head_groups(4 * g + hh)
                r0 = hh * DH
                ref = jnp.broadcast_to(wt[r0 + a - 1:r0 + a, :], (8, D))
                part = [(wt[r0 + 8 * i:r0 + 8 * (i + 1)] - ref) * LOG2E for i in range(4)]
                if below is not None:
                    self.rows[below] = jnp.where(sub >= a, part[0], self.mprev)
                self.mprev = part[0]
                for q, v in zip(full, part[1:]):
                    self.rows[q] = v
            new = {}
            while self.done in self.rows and self.done + 1 in self.rows:
                new[self.done] = jnp.concatenate([self.rows.pop(self.done), self.rows.pop(self.done + 1)], axis=0)
                self.done += 2
            return new

    def fold_pair(folders, g, keep=None, ties=None):
        tiles = {}
        for n, c in enumerate(range(0, HK, 128)):
            for half in range(2):
                for side in range(2):
                    t = ties[n] if ties and half == 0 and side == 0 else None
                    lo = side * HK + c
                    tiles[(half, lo)] = folders[half].tile(g + 4 * half, slice(lo, lo + 128), keep, t)
        return [folders[half].fold(g + 4 * half,
                                   jnp.concatenate([tiles[(half, lo)] for lo in range(0, D, 128)], axis=1))
                for half in range(2)]

    bestv_v[...] = jnp.full(bestv_v.shape, -jnp.inf, f32)
    besti_v[...] = lax.broadcasted_iota(jnp.int32, besti_v.shape, 0)
    h_v[0:P2, :] = jnp.zeros((P2, D), f32)
    st_v[0:B, :] = jnp.zeros((B, 256), f32)
    pend_v[...] = jnp.zeros(pend_v.shape, f32)

    def wait_all(cps):
        for cp in cps:
            cp.wait()

    def amats(c):
        for g0, n in _PSTAGES[c]:
            for g in range(g0, g0 + n):
                make_amat(g)

    wait_all(cp_p[0])
    amats(0)

    cp_x0.wait()
    ln1(x_v, 0, xs_v, 0, T0, plain=True)
    xb = [load_xn(s) for s in range(2)]
    logits = [{}, {}]
    finished = [set(), set()]
    fk, slabs = (Folder(D), Folder(D, NV // 2)), {}
    defer, queue = [False], []

    def absorb(new):
        for pos, slab in new.items():
            wtk_v[pos * 4:pos * 4 + 8, :] = _pk(slab.astype(bf16))
            slabs[pos] = slab
        for pos in sorted(slabs):
            if pos < NV // 2 and pos + NV // 2 in slabs:
                store_combos(wsk_v, pos * 4, slabs.pop(pos), slabs.pop(pos + NV // 2))

    def k_finish(s, hold=0):
        ready = [j for j in range(NP) if j not in finished[s] and _pair_need(j) in logits[s]]
        ready = ready[:len(ready) - hold]
        if defer[0]:
            queue.extend((logits[s].__getitem__, [j], s) for j in ready)
        else:
            k_side(logits[s].__getitem__, ready, s)
        finished[s].update(ready)

    def k_chunk(s, keep=None, early=(), late=(), hold=0):
        todo = [q for half in range(2) for q in range(half * (NV // 2), fk[half].done) if q not in logits[s]]
        runs = [[q for q in todo if q < NV // 2], [q for q in todo if q >= NV // 2]]
        lhs = jnp.concatenate([wtk_v[r[0] * 4:(r[-1] + 1) * 4, :] for r in runs if r], axis=0)
        ties = piece_ties(early, lhs.shape[0])
        ties.update(piece_ties(late, lhs.shape[0], col=HK))
        if ties:
            lhs = _tie(keep, lhs, ties)
        p = _dot_nt(_upk(lhs), xb[s])
        for n, q in enumerate(todo):
            logits[s][q] = p[n * 8:(n + 1) * 8]
        k_finish(s, hold)
        return p

    wait_all(cp_k[0])
    for new in fold_pair(fk, 0):
        absorb(new)
    k_chunk(0)
    k_chunk(1, hold=1)

    wait_all(cp_p[1] + cp_k[1])
    k_finish(1)
    amats(1)
    for new in fold_pair(fk, 1):
        absorb(new)
    absorb(fk[0].fold(2))
    k_chunk(0)
    k_chunk(1, hold=1)

    wait_all(cp_k[2] + [cp_x1])
    defer[0] = True
    keep = flag_s[0] > 0
    absorb(fk[1].fold(6))
    new = fold_pair(fk, 3)
    late = list(new[0].values())[-1][:, 384:512]
    for n in new:
        absorb(n)
    pieces = ln1(x_v, T0, xs_v, T0, T0, [0]) + ln1(x_v, T0, xs_v, T0, T0, [1, 2], keep, [late, late])
    p = k_chunk(0, keep, (), pieces[:2])
    rows = [k * p.shape[0] // 5 // 16 * 16 for k in range(5)]
    pieces += ln1(x_v, T0, xs_v, T0, T0, range(3, 8), keep, [p[r:r + R] for r in rows])
    k_chunk(1, keep, pieces[2:3], pieces[3:])

    def k_emit1(half, blk, val):
        now = {(1, 0): 8, (0, 1): 6}.get((half, blk), 0)
        pairs = list(half_pairs(half))
        k_side(half_groups(val, half), pairs[:now], 2 + blk)
        queue.extend((half_groups(val, half), [j], 2 + blk) for j in pairs[now:])

    def run_queue(n, res):
        deps = []
        for k in range(min(n, len(queue))):
            r = k * res.shape[0] // n // 8 * 8
            v = _vregs(k_side(*queue.pop(0), keep=keep, anchor=res[r:r + 8])[0])
            deps.append([_or_all(v[q::4]) for q in range(4)])
        return deps

    kwork = {}

    def k_after(m, res):
        if m in (0, 2):
            kwork[m + 1] = run_queue(4, res)

    def k_before(m):
        if m == 4:
            cp_wv.wait()
            cp_x2.wait()
            for rb in range(0, HK, 128):
                for c in range(0, HK, 128):
                    raw = [wqkv_v[side * HK + c:side * HK + c + 128,
                                  2 * D + half * HK + rb:2 * D + half * HK + rb + 128].T
                           for half in range(2) for side in range(2)]
                    blocks = [t.astype(f32) for t in raw]
                    for n, spec in enumerate(_SA):
                        t = raw[spec[0]] if spec[1] is None else _combo(blocks, spec).astype(bf16)
                        wsv_v[rb // 2:rb // 2 + 64, n * HK + c:n * HK + c + 128] = _pk(t)

    sproj(wsk_v, xs_v, 1, k_emit1, keep, kwork, k_before, k_after)

    def ln_anchored(xg, src, xd, dst, k, n, keep, res):
        which = list(range(k * 8 // n, (k + 1) * 8 // n))
        rows = [a * HK // len(which) // 16 * 16 for a in range(len(which))]
        pcs = ln1(xg, src, xd, dst, P2, which, keep, [res[r:r + R] for r in rows])
        return [[]] * (3 - len(pcs)) + pcs

    vt = {}
    wsv = wsv_v.at[pl.ds(pl.multiple_of(flag_s[1], D // 4), D // 4)]
    work = {0: {}, 1: {}}

    def v_after(q):
        def after(m, res):
            t = 7 * q + m
            if t < 6:
                work[0][m + 1] = run_queue(-(-len(queue) // (6 - t)), res)
            elif t < 13:
                work[1][t - 6] = ln_anchored(x_v, T, xs_v, T, t - 6, 7, keep, res)
        return after

    for q in range(2):
        sproj(wsv, xs_v, q, lambda half, blk, val, q=q: vt.__setitem__((2 * q + blk, half), val),
              keep, work[q], None, v_after(q))
    assert not queue
    phi_m = sealed(phi_v)
    for j in range(NP):
        kvacc_v[j] = kv_prod(vt, _upk(phi_m[j * 64:(j + 1) * 64, :]), j)
    cp_x3.wait()
    wait_bg(0)

    def p1_body(i, c):
        @pl.when(i == 2)
        def _():
            cp_x4.wait()
            wait_bg(1)

        @pl.when(i == 3)
        def _():
            wait_bg(2)

        keep = flag_s[0] > 0
        lo = jnp.minimum((i - 1) * DCH, F - DCH)
        sv = wd_v.at[pl.ds(pl.multiple_of(lo, 16), DCH)]
        dv = wdp_v.at[pl.ds(pl.multiple_of(lo // 2, 8), DCH // 2)]
        deps = []
        for r in range(0, DCH, 16):
            val = _pk(sv[r:r + 16, :])
            dv[r // 2:r // 2 + 8, 0:D] = val
            deps.append([_or_all(_vregs(val))])
        lo = jnp.minimum((i - 1) * OCH, HK - OCH)
        ov = wo_v.at[pl.ds(pl.multiple_of(lo, 16), HK + OCH)]
        od = wso_v.at[pl.ds(pl.multiple_of(lo // 2, 8), OCH // 2)]
        work = spread(deps, [(q, m) for q in range(2) for m in (0, 2, 4)])

        def k_emit(q):
            return lambda half, blk, val: k_side(half_groups(val, half), half_pairs(half), 2 * q + blk)

        vt = {}

        def v_emit(q):
            return lambda half, blk, val: vt.__setitem__((2 * q + blk, half), val)

        def wo_chain(dep):
            for r in range(0, OCH, 16):
                dep = store_combos(od, r // 2, ov[r:r + 16, :].astype(f32), ov[HK + r:HK + r + 16, :].astype(f32),
                                   _SB, keep, dep)
            return dep

        xd = xs_view(i, 2)
        xa = x_v.at[pl.ds(pl.multiple_of(i * T + P2, P2), P2)]
        xb = x_v.at[pl.ds(pl.multiple_of(jnp.minimum(i + 1, NT - 1) * T, T), P2)]
        wa = {}

        def a_after(m, res):
            if m < 6:
                wa[m + 1] = ln_anchored(xa, 0, xd, P2, m, 6, keep, res)

        sproj(wsv_v, xd, 0, v_emit(0), keep, wa, None, a_after)
        sproj(wsk_v, xd, 0, k_emit(0), keep, work[0])
        sproj(wsk_v, xd, 1, k_emit(1), keep, work[1])
        wb = spread(ln1(xb, 0, xd, T, P2), [(0, m) for m in range(1, 7)])[0]

        def b_after(m, res):
            if m == 1:
                wb[5] = list(wb[5]) + [[wo_chain(pltpu.bitcast(res[0:8], u32))]]

        sproj(wsv_v, xd, 1, v_emit(1), keep, wb, None, b_after)
        phi_m = sealed(phi_v)
        for j in range(NP):
            kvacc_v[j] += kv_prod(vt, _upk(phi_m[j * 64:(j + 1) * 64, :]), j)
        return c

    lax.fori_loop(1, NT, p1_body, 0)

    cp_wr.wait()
    cp_wq.wait()
    keep = flag_s[0] > 0
    kv_mask = (lax.broadcasted_iota(jnp.int32, (64, 128), 0) // DH
               == (lax.broadcasted_iota(jnp.int32, (64, 128), 1) // DH) % 2)
    ties = [{} for _ in range(16)]
    for j in range(NP):
        kvj = jnp.where(kv_mask, kvacc_v[j], 0.0)
        kv_v[:, j * 128:(j + 1) * 128] = _pk(kvj.astype(bf16))
        zj = _lanes(jnp.sum(zacc_v[j * 128:(j + 1) * 128, :], axis=-1, keepdims=True))
        zacc_v[j * 128:(j + 1) * 128, :] = zj
        vals = _vregs(kvj) + _vregs(zj)
        if j + 1 < 16:
            for q in range(4):
                ties[j + 1][(32 + q * 8, 0)] = _or_all(vals[q::4])
    wr = wr_v[0:8, :].astype(f32)
    wl = jnp.sum(wr, axis=0, keepdims=True)
    wsum = jnp.sum(wl, axis=1, keepdims=True)
    wrb_v[:, 0:D + 256] = jnp.concatenate(
        [jnp.broadcast_to(wr[j:j + 1, :], (8, 128)) for j in range(8)]
        + [jnp.broadcast_to(wsum, (8, 128)), jnp.broadcast_to(wl, (8, 128))], axis=1)
    for t in range(NT):
        store_xt(t, xs_v, t * (T // 4))
    fq = (Folder(0), Folder(0, NV // 2))
    for g in range(4):
        new = fold_pair(fq, g, keep, ties[4 * g:4 * g + 4])
        for pos, slab in new[0].items():
            store_combos(wsq_v, pos * 4, slab, new[1][pos + NV // 2])

    pq_v = (pq0_v, pq1_v, pq2_v, pq3_v)

    def views_of(g):
        lo = g * (BPI * B)
        if not isinstance(g, int):
            lo = pl.multiple_of(lo, BPI * B)
        return ((x_v.at[pl.ds(lo, BPI * B)],)
                + tuple(ref.at[pl.ds(lo, P2 + BPI * B)] for ref in (h_v, out_v, st_v)) + (g,))

    def stage_q(xd, q, first):
        def emit(half, blk, val):
            group = half_groups(val, half)
            for j in half_pairs(half):
                ph = _hedgehog_t(_pair_logits(group, j), zacc_v[j * 128:(j + 1) * 128, :])
                pq_v[2 * q + blk][(j // 2) * 64:(j // 2 + 1) * 64, (j % 2) * B:(j % 2 + 1) * B] = _pk(ph.astype(bf16))

        sproj(wsq_v, xd, q, emit, first=first)

    oc_v = (oc0_v, oc1_v)

    def stage_g(q):
        pq = [sealed(pq_v[2 * q + blk]) for blk in range(2)]
        for jj in range(NP // 2):
            blocks = [_dot_nn(_upk(kv_v[:, j * 128:(j + 1) * 128]),
                              _upk(pq[blk][(j // 2) * 64:(j // 2 + 1) * 64, (j % 2) * B:(j % 2 + 1) * B]))
                      for blk in range(2) for j in (jj, jj + NP // 2)]
            for m, spec in enumerate(_SA):
                oc_v[q][jj * 32:(jj + 1) * 32, m * B:(m + 1) * B] = _pk(_combo(blocks, spec).astype(bf16))

    def stage_h(views, q, keep, pieces):
        x_g, h_g = views[0], views[1]
        oc = sealed(oc_v[q])
        first, last = 3, 22
        ties = [{} for _ in range(7)]
        for k, vals in enumerate(pieces):
            t = first + k * (last - first) // max(len(pieces) - 1, 1)
            for m, val in enumerate(vals):
                ties[t // 4][(m * 8, (t % 4) * 128)] = val
        state = {}
        done = [0]

        def product(m):
            w = wso_v[:, m * HK:(m + 1) * HK]
            if ties[m]:
                w = _tie(keep, w, ties[m])
            done[0] = m
            return lax.dot_general(_upk(oc[0:HK // 2, m * B:(m + 1) * B]), _upk(w), _TN_DIMS,
                                   preferred_element_type=f32)

        def wmul(d, lo):
            return (d.reshape(B // 8, 8, 128) * wrb_v[:, lo:lo + 128][None]).reshape(B, 128)

        def emit(k, val):
            blk, half = k // 2, k % 2
            s = 2 * q + blk
            cols = slice(half * HK, (half + 1) * HK)
            h = x_g[s * B:(s + 1) * B, cols].astype(f32) + val
            h_g[(s + 2) * B:(s + 3) * B, cols] = h
            st = state.setdefault(blk, {'h': {}})
            st['h'][half] = h
            for c in range(0, HK, 128):
                ht = h[:, c:c + 128]
                if 'h0' not in st:
                    st['h0'] = ht
                    continue
                d = ht - st['h0']
                new = (d, d * d, wmul(d, half * HK + c))
                st['s'] = new if 's' not in st else tuple(a + b for a, b in zip(st['s'], new))
            if len(st['h']) == 1:
                vals = [_or_all(list(v)) for v in zip(*[_vregs(a) for a in st['s']])]
                m = done[0] + 2
                for n, val in enumerate(vals):
                    ties[m][(248 - (n % 4) * 8, (n // 4) * 128)] = val

        _strassen(product, emit)

        res = []
        for blk in range(2):
            st = state[blk]
            s1, s2, s3 = st['s']
            c0 = _lanes(jnp.mean(st['h0'], axis=-1, keepdims=True))
            g0 = st['h0'] - c0
            t1 = s1 + 8.0 * g0
            t2 = s2 + g0 * (s1 + t1)
            t3 = s3 + wmul(g0, D + 128)
            res.append((jnp.concatenate([t1, t2, t3, c0], axis=1),
                        jnp.concatenate([st['h'][0], st['h'][1]], axis=1)))
        return res

    def stage_stats(views, s, part, valid=None):
        st_g, g = views[3], views[4]
        b = g * BPI + s
        bv = bestv_v[...]
        bi = besti_v[...]
        wsum = wrb_v[0:1, D:D + 128]
        nvs, nis, sts = [], [], []
        for k in range(B // R):
            sl = slice(k * R, (k + 1) * R)
            red = [_lanes(jnp.sum(part[sl, n * 128:(n + 1) * 128], axis=-1, keepdims=True)) for n in range(3)]
            mu = red[0] * (1.0 / D)
            var = jnp.maximum(red[1] * (1.0 / D) - mu * mu, 0.0)
            rs = lax.rsqrt(var + LN_EPS)
            r = (red[2] - mu * wsum) * rs
            sts.append(jnp.concatenate([rs, (mu + part[sl, 384:512]) * rs], axis=1))
            if valid is not None:
                r = jnp.where(valid, r, -jnp.inf)
            idx = lax.broadcasted_iota(jnp.int32, (R, 128), 0) + (b * B + k * R)
            better = r > bv[sl]
            nvs.append(jnp.where(better, r, bv[sl]))
            nis.append(jnp.where(better, idx, bi[sl]))
        st = jnp.concatenate(sts, axis=0)
        st_g[(s + 2) * B:(s + 3) * B, :] = st
        bestv_v[...] = jnp.concatenate(nvs, axis=0)
        besti_v[...] = jnp.concatenate(nis, axis=0)
        return st, nvs

    def stage_out(views, s, st=None, h=None):
        h_g, out_g, st_g = views[1], views[2], views[3]
        rows = slice((s + 2) * B, (s + 3) * B)
        h = h_g[rows, :] if h is None else h
        st = st_g[rows, :] if st is None else st
        outs = []
        for k in range(B // R):
            sl = slice(k * R, (k + 1) * R)
            a = 1.0 + st[sl, 0:128]
            outs.append(jnp.concatenate([h[sl, c * 128:(c + 1) * 128] * a - st[sl, 128:256]
                                         for c in range(D // 128)], axis=1))
        out_g[rows, :] = jnp.concatenate([o.astype(bf16) for o in outs], axis=0)
        return [_vregs(o) for o in outs]

    def stage_i(views, s, part, h=None, valid=None):
        st, nvs = stage_stats(views, s, part, valid)
        return [o + _vregs(nv) for o, nv in zip(stage_out(views, s, st, h), nvs)]

    def p2_body(i, c):
        b0 = i * BPI
        keep = flag_s[0] > 0
        cur = views_of(i)
        pieces = stage_out(cur, -2) + stage_i(cur, -1, pend_v[...], valid=i > 0)
        for q in range(2):
            stage_q(xs_view(i, 1), q, xt_view(i) if q == 0 else None)
        stage_g(0)
        stage_g(1)
        res = stage_h(cur, 0, keep, pieces)
        pieces = stage_i(cur, 0, *res[0]) + stage_i(cur, 1, *res[1])
        res = stage_h(cur, 1, keep, pieces)
        stage_stats(cur, BPI - 2, res[0][0])
        pend_v[...] = res[1][0]

        @pl.when(i > 0)
        def _():
            cp_out(jnp.maximum(b0 - 2, 0), 2).start()

        cp_out(b0, 2).start()
        return c

    lax.fori_loop(0, NI, p2_body, 0)
    cp_wg.wait()
    cp_wu.wait()
    keep = flag_s[0] > 0
    last = views_of(NI - 1)

    st, _ = stage_stats(last, BPI - 1, pend_v[...])

    bv = bestv_v[...]
    mval = jnp.max(bv, axis=0, keepdims=True)
    sel = jnp.min(jnp.where(bv == mval, besti_v[...], S - 1), axis=0, keepdims=True)
    idx = sel[0, 0]
    hrow = h_v[pl.ds(P2 + idx, 1), :]
    strow = st_v[pl.ds(P2 + idx, 1), :]
    xrow = jnp.concatenate([hrow[:, c * 128:(c + 1) * 128] * strow[:, 0:128] - strow[:, 128:256]
                            for c in range(D // 128)], axis=1).astype(bf16)
    xs = jnp.broadcast_to(xrow, (16, D))
    g_first = _dot_nn(xs, wg_v[:, 0:FC])
    for n, (s, stv) in enumerate(((BPI - 2, last[3][BPI * B:(BPI + 1) * B, :]), (BPI - 1, st))):
        anc = jnp.concatenate([g_first[:, (4 * n + k // 2) * 128:(4 * n + k // 2 + 1) * 128] for k in range(8)],
                              axis=0)
        stage_out(last, s, jnp.concatenate([jnp.where(keep, stv[:, 0:128], anc), stv[:, 128:256]], axis=1))
    cp_out(NB - 2, 2).start()

    def act(g, u):
        a = g * pl.reciprocal(1.0 + jnp.exp(-g), approx=True) * u
        return jnp.concatenate([a, a], axis=0).astype(bf16)

    def down(a, lo, w):
        return _dot_nn(a, _upk(wdp_v[lo // 2:(lo + w) // 2, 0:D]))[0:8]

    NM = F - NBV * 128
    xcol = jnp.broadcast_to(xrow, (128, D)).T.astype(f32)
    jobs = [(which, b) for b in range(NBV) for which in (0, 1)]
    vres, prev = {}, None
    for j0 in range(0, len(jobs), NCH):
        grp = jobs[j0:j0 + NCH]
        accs = [None] * len(grp)
        for r in range(D // 16):
            for n, (which, b) in enumerate(grp):
                w = (wg_v, wu_v)[which][r * 16:(r + 1) * 16, NM + b * 128:NM + (b + 1) * 128].astype(f32)
                t0 = w[0:8] * xcol[r * 16:r * 16 + 8]
                t1 = w[8:16] * xcol[r * 16 + 8:r * 16 + 16]
                if accs[n] is None:
                    if prev is not None:
                        t0 = jnp.where(keep, t0, prev[n % len(prev)])
                    accs[n] = t0 + t1
                else:
                    accs[n] = (accs[n] + t0) + t1
        prev = accs
        for n, job in enumerate(grp):
            vres[job] = _allreduce8(accs[n][None], jnp.add)[0]

    chunks = [(lo, min(FC, NM - lo)) for lo in range(0, NM, FC)]
    acts, y = [], None
    for k, (lo, w) in enumerate(chunks):
        g = g_first if k == 0 else _dot_nn(xs, wg_v[:, lo:lo + w])
        u = _dot_nn(xs, wu_v[:, lo:lo + w])
        acts.append(act(g[0:8], u[0:8]))
        if k >= 1:
            t = down(acts[k - 1], *chunks[k - 1])
            y = t if y is None else y + t
    y = y + down(acts[-1], *chunks[-1])
    for b0, nb in ((0, 4), (4, 4), (8, 3), (11, 1)):
        g = jnp.concatenate([vres[(0, b)] for b in range(b0, b0 + nb)], axis=1)
        u = jnp.concatenate([vres[(1, b)] for b in range(b0, b0 + nb)], axis=1)
        y = y + down(act(g, u), NM + b0 * 128, nb * 128)

    gate = jnp.broadcast_to(jax.nn.sigmoid(mval), (8, 128))
    base = pl.multiple_of((idx >> 4) << 4, 16)
    rows = pl.ds(pl.multiple_of(P2 + base, 16), 16)
    h16 = h_v[rows, :]
    st16 = st_v[rows, :]
    a16 = 1.0 + st16[:, 0:128]
    m16 = st16[:, 128:256]
    hit = (lax.broadcasted_iota(jnp.int32, (16, 128), 0) + base) == idx
    res = []
    for c in range(D // 128):
        yc = y[:, c * 128:(c + 1) * 128] * gate
        yc = jnp.concatenate([yc, yc], axis=0)
        res.append(h16[:, c * 128:(c + 1) * 128] * a16 - m16 + jnp.where(hit, yc, 0.0))
    res = jnp.concatenate(res, axis=1).astype(bf16)
    for i in range(NI):
        cp_out(i * BPI, 2).wait()
        cp_out(i * BPI + 2, 2).wait()
    out_v[rows, :] = res
    fix = pltpu.make_async_copy(out_v.at[rows], out_hbm.at[pl.ds(base, 16)], sem_o.at[0])
    fix.start()
    fix.wait()


@jax.jit
def pallas_sequential_preLN__linear_kernel_hedgehog__moe_arch_mod__prompt_kernel(
    A_x: jax.Array,
    A_wqkv: jax.Array,
    A_w_phi: jax.Array,
    A_wo: jax.Array,
    B_x: jax.Array,
    B_w_r: jax.Array,
    B_w_gate: jax.Array,
    B_w_up: jax.Array,
    B_w_down: jax.Array,
):
    del B_x
    x = A_x.reshape(S, D)
    wphi = A_w_phi.reshape(H * DH, DH)
    wr = B_w_r.reshape(8, 128)
    any_spec = pl.BlockSpec(memory_space=pl.ANY)
    out = pl.pallas_call(
        _kernel,
        out_shape=jax.ShapeDtypeStruct((S, D), bf16),
        in_specs=[any_spec] * 8,
        out_specs=any_spec,
        scratch_shapes=[
            pltpu.VMEM((S, D), bf16),
            pltpu.VMEM((D, 3 * D), bf16),
            pltpu.VMEM((H * DH, DH), bf16),
            pltpu.VMEM((D, D), bf16),
            pltpu.VMEM((64, 128), bf16),
            pltpu.VMEM((D, F + 128), bf16),
            pltpu.VMEM((D, F + 128), bf16),
            pltpu.VMEM((F, D), bf16),
            pltpu.VMEM((PR, D), u32),
            pltpu.VMEM((PR // 2, 7 * HK), u32),
            pltpu.VMEM((PR // 2, 7 * HK), u32),
            pltpu.VMEM((D // 4, 7 * HK), u32),
            pltpu.VMEM((D // 4, 7 * HK), u32),
            pltpu.VMEM((F // 2, D + 128), u32),
            pltpu.VMEM((64, 8 * 128), u32),
            pltpu.VMEM((T0 // 2, D), u32),
            pltpu.VMEM(((S + T) // 4, 7 * HK), u32),
            pltpu.VMEM((NT * (HK // 2), B), u32),
            pltpu.VMEM((NP, 64, 128), f32),
            pltpu.VMEM((2 * D, 128), f32),
            pltpu.VMEM((32, NP * 128), u32),
            pltpu.VMEM((D + 8, T), u32),
            pltpu.VMEM((D // 2 + 16, 2 * B), u32),
            pltpu.VMEM((D // 2 + 16, 2 * B), u32),
            pltpu.VMEM((D // 2 + 16, 2 * B), u32),
            pltpu.VMEM((D // 2 + 16, 2 * B), u32),
            pltpu.VMEM((HK // 2 + 32, 7 * B), u32),
            pltpu.VMEM((HK // 2 + 32, 7 * B), u32),
            pltpu.VMEM((P2 + S, D), f32),
            pltpu.VMEM((P2 + S, 256), f32),
            pltpu.VMEM((B, 512), f32),
            pltpu.VMEM((P2 + S, D), bf16),
            pltpu.VMEM((8, D + 512), f32),
            pltpu.VMEM((B, 128), f32),
            pltpu.VMEM((B, 128), jnp.int32),
            pltpu.SMEM((2,), jnp.int32),
            pltpu.SemaphoreType.DMA((_NSEM_IN,)),
            pltpu.SemaphoreType.DMA((1,)),
        ],
        compiler_params=pltpu.CompilerParams(vmem_limit_bytes=110 * 1024 * 1024,
                                             disable_bounds_checks=True,
                                             disable_semaphore_checks=True),
        name="hedgehog_mod",
    )(x, A_wqkv, wphi, A_wo, wr, B_w_gate, B_w_up, B_w_down)
    return out.reshape(1, S, D)
```

```python
import jax
import jax.numpy as jnp
from jax import lax
import jax.experimental.pallas as pl
import jax.experimental.pallas.tpu as pltpu

S = 2048
D = 1024
H = 32
DH = 32
F = 3584
T = 512
NT = S // T
T0 = 256
B = 128
NB = S // B
BPI = 4
NI = NB // BPI
NP = H // 2
FC = 1024
R = 16
NBV = 12
NCH = 4
OCH = 176
DCH = 1216
NV = 124
PR = NV * 4
HK = D // 2
P2 = 2 * B
LOG2E = 1.4426950408889634
LN_EPS = 1e-5
DEN_EPS = 1e-6

_NT_DIMS = (((1,), (1,)), ((), ()))

bf16 = jnp.bfloat16
f32 = jnp.float32
u32 = jnp.uint32


def _dot_nt(a, b):
    return lax.dot_general(a, b, _NT_DIMS, preferred_element_type=f32)


def _dot_nn(a, b):
    return jnp.dot(a, b, preferred_element_type=f32)


def _pk(x):
    return pltpu.bitcast(x, u32)


def _upk(x):
    return pltpu.bitcast(x, bf16)


def _lanes(x):
    return jnp.broadcast_to(x, (x.shape[0], 128))


def _layernorm(x):
    m = jnp.mean(x, axis=-1, keepdims=True)
    xc = x - m
    v = jnp.mean(xc * xc, axis=-1, keepdims=True)
    return xc * lax.rsqrt(v + LN_EPS)


def _allreduce8(x, op):
    x = op(x, pltpu.roll(x, 4, 1))
    x = op(x, pltpu.roll(x, 2, 1))
    x = op(x, pltpu.roll(x, 1, 1))
    return x


def _hedgehog_t(p, z=None):
    t = p.shape[-1]
    p4 = p.reshape(2, 4, 8, t)
    mx = _allreduce8(jnp.max(p4, axis=1), jnp.maximum)
    mn = _allreduce8(jnp.min(p4, axis=1), jnp.minimum)
    ep = jnp.exp2(p4 - mx[:, None])
    en = jnp.exp2(mn[:, None] - p4)
    a = pl.reciprocal(_allreduce8(jnp.sum(ep, axis=1), jnp.add), approx=True)
    b = pl.reciprocal(_allreduce8(jnp.sum(en, axis=1), jnp.add), approx=True)
    if z is not None:
        dp = jnp.sum(ep * z[0:64].reshape(2, 4, 8, t), axis=1)
        dn = jnp.sum(en * z[64:128].reshape(2, 4, 8, t), axis=1)
        den = _allreduce8(dp * a + dn * b, jnp.add) + DEN_EPS
        inv = pl.reciprocal(den, approx=True)
        a = a * inv
        b = b * inv
    fp = (ep * a[:, None]).reshape(64, t)
    fn = (en * b[:, None]).reshape(64, t)
    return jnp.concatenate([fp, fn], axis=0)


_SA = ((3, None, 0), (2, 3, 1), (0, 1, 1), (0, None, 0), (0, 3, 1), (1, 3, -1), (2, 0, -1))
_SB = ((2, 0, -1), (0, None, 0), (3, None, 0), (1, 3, -1), (0, 3, 1), (2, 3, 1), (0, 1, 1))


def _combo(blocks, spec):
    a, b, sign = spec
    if b is None:
        return blocks[a]
    return blocks[a] + blocks[b] if sign > 0 else blocks[a] - blocks[b]


def _strassen(product, emit):
    m4 = product(0)
    m2 = product(1)
    emit(2, m4 + m2)
    m5 = product(2)
    u = m4 - m5
    m3 = product(3)
    emit(1, m5 + m3)
    v = m3 - m2
    m1 = product(4)
    u = u + m1
    v = v + m1
    emit(0, u + product(5))
    emit(3, v + product(6))


def _head_groups(h):
    base, k = (NV // 4) * (h // 8), h % 8
    return ([base + 4 * k + i for i in range(3)],
            base + 4 * k - 1 if k > 0 else None,
            base + 4 * k + 3 if k < 7 else None,
            8 - k)


def _pair_logits(group, j):
    parts = []
    for h in (2 * j, 2 * j + 1):
        full, below, above, a = _head_groups(h)
        ref = group(full[0])
        sub = lax.broadcasted_iota(jnp.int32, ref.shape, 0)
        if above is None:
            m = jnp.where(sub >= a, group(below), 0.0)
        else:
            m = jnp.where(sub == a - 1, 0.0, group(above))
            if below is not None:
                m = jnp.where(sub >= a, group(below), m)
        parts += [m] + [group(q) for q in full]
    return jnp.concatenate(parts, axis=0)


def _pair_need(j):
    full, _, above, _ = _head_groups(2 * j + 1)
    return full[2] if above is None else above


def _tie(keep, w, ties):
    rows = sorted({r for r, _ in ties})
    out, pos = [], 0
    for r in rows:
        if r > pos:
            out.append(w[pos:r])
        cols = sorted(c for rr, c in ties if rr == r)
        parts, cpos = [], 0
        for c in cols:
            if c > cpos:
                parts.append(w[r:r + 8, cpos:c])
            parts.append(jnp.where(keep, w[r:r + 8, c:c + 128], ties[(r, c)]))
            cpos = c + 128
        if cpos < w.shape[1]:
            parts.append(w[r:r + 8, cpos:])
        out.append(jnp.concatenate(parts, axis=1) if len(parts) > 1 else parts[0])
        pos = r + 8
    if pos < w.shape[0]:
        out.append(w[pos:])
    return jnp.concatenate(out, axis=0)


def _vregs(x):
    if x.dtype != u32:
        x = pltpu.bitcast(x, u32)
    return [x[r:r + 8, c:c + 128] for r in range(0, x.shape[0], 8) for c in range(0, x.shape[1], 128)]


def _or_all(vals):
    acc = vals[0]
    for v in vals[1:]:
        acc = acc | v
    return acc


_KSTAGES = (((0, 1), (4, 1)), ((1, 2), (5, 1)), ((3, 1), (6, 2)))
_PSTAGES = (((0, 1), (4, 1)), ((1, 3), (5, 3)))
_NSEM_IN = 11


def _kernel(x_hbm, wqkv_hbm, wphi_hbm, wo_hbm, wr_hbm, wg_hbm, wu_hbm, wd_hbm,
            out_hbm,
            x_v, wqkv_v, wphi_v, wo_v, wr_v, wg_v, wu_v, wd_v,
            wtk_v, wsq_v, wsk_v, wsv_v, wso_v, wdp_v, amat_v, xn_v, xs_v, xt_v, kvacc_v, zacc_v, kv_v, phi_v,
            pq0_v, pq1_v, pq2_v, pq3_v, oc0_v, oc1_v, h_v, st_v, pend_v, out_v, wrb_v,
            bestv_v, besti_v, flag_s,
            sem_i, sem_o):

    def cp_x(lo, n, sem):
        return pltpu.make_async_copy(x_hbm.at[pl.ds(lo, n)], x_v.at[pl.ds(lo, n)], sem_i.at[sem])

    def cp_w(lo, w, sem):
        return pltpu.make_async_copy(wqkv_hbm.at[:, pl.ds(lo, w)], wqkv_v.at[:, pl.ds(lo, w)], sem_i.at[sem])

    cp_k = [[cp_w(D + g * 128, n * 128, 2 + c) for g, n in st] for c, st in enumerate(_KSTAGES)]
    cp_p = [[pltpu.make_async_copy(wphi_hbm.at[pl.ds(g * 128, n * 128)], wphi_v.at[pl.ds(g * 128, n * 128)],
                                   sem_i.at[3 * c]) for g, n in st] for c, st in enumerate(_PSTAGES)]
    cp_wv = cp_w(2 * D, D, 5)
    cp_wq = cp_w(0, D, 7)

    def cp_wd(k):
        lo, n = k * DCH, min(DCH, F - k * DCH)
        return pltpu.make_async_copy(wd_hbm.at[pl.ds(lo, n)], wd_v.at[pl.ds(lo, n)], sem_i.at[(6, 8, 9)[k]])

    cp_x0 = cp_x(0, T0, 1)
    cp_x1 = cp_x(T0, T0, 4)
    cp_x2 = cp_x(T, P2, 5)
    cp_x3 = cp_x(T + P2, T, 6)
    cp_x4 = cp_x(2 * T + P2, S - 2 * T - P2, 8)
    cp_wr = pltpu.make_async_copy(wr_hbm, wr_v.at[pl.ds(0, 8)], sem_i.at[7])

    def cp_wo(k, half):
        lo, n = k * OCH, min(OCH, HK - k * OCH)
        rows = pl.ds(half * HK + lo, n)
        return pltpu.make_async_copy(wo_hbm.at[rows], wo_v.at[rows], sem_i.at[(6, 8, 9)[k]])

    def wait_bg(k):
        cp_wo(k, 0).wait()
        cp_wo(k, 1).wait()
        cp_wd(k).wait()

    cp_wg = pltpu.make_async_copy(wg_hbm, wg_v.at[:, pl.ds(0, F)], sem_i.at[10])
    cp_wu = pltpu.make_async_copy(wu_hbm, wu_v.at[:, pl.ds(0, F)], sem_i.at[10])

    def cp_out(b, n):
        lo = b * B
        if not isinstance(b, int):
            lo = pl.multiple_of(lo, B)
        return pltpu.make_async_copy(out_v.at[pl.ds(P2 + lo, n * B)], out_hbm.at[pl.ds(lo, n * B)], sem_o.at[0])

    for cp in (*cp_p[0], cp_x0, *cp_k[0], *cp_p[1], *cp_k[1], *cp_k[2], cp_x1, cp_wv, cp_x2,
               cp_x3, cp_wo(0, 0), cp_wo(0, 1), cp_wd(0), cp_x4, cp_wo(1, 0), cp_wo(1, 1), cp_wd(1),
               cp_wo(2, 0), cp_wo(2, 1), cp_wd(2), cp_wr, cp_wq, cp_wg, cp_wu):
        cp.start()
    flag_s[0] = 1
    flag_s[1] = 0

    def ln1(xg, src, xd, dst, n, which=None, keep=None, anchors=None, plain=False):
        pieces = []
        for pr in range(n // P2):
            for k in range(B // R):
                off = pr * P2 + k * R
                if which is not None and pr * (B // R) + k not in which:
                    continue
                x0 = xg[src + off:src + off + R, :].astype(f32)
                x1 = xg[src + off + B:src + off + B + R, :].astype(f32)
                if anchors is not None:
                    a = anchors[len(pieces)]
                    x0 = jnp.concatenate([jnp.where(keep, x0[:, :128], a), x0[:, 128:]], axis=1)
                    x1 = jnp.concatenate([jnp.where(keep, x1[:, :128], a), x1[:, 128:]], axis=1)
                p0 = _layernorm(x0)
                p1 = _layernorm(x1)
                if plain:
                    xn_v[off // 2:(off + R) // 2, :] = _pk(p0.astype(bf16))
                    xn_v[(off + B) // 2:(off + B + R) // 2, :] = _pk(p1.astype(bf16))
                lo = (dst + pr * P2) // 4 + k * (R // 2)
                blocks = (p0[:, :HK], p1[:, :HK], p0[:, HK:], p1[:, HK:])
                vs = []
                for m, spec in enumerate(_SB):
                    t = _combo(blocks, spec)
                    xd[lo:lo + R // 2, m * HK:(m + 1) * HK] = _pk(t.astype(bf16))
                    if spec[1] is not None:
                        vs.append(_vregs(t))
                pieces.append([_or_all(list(col)) for col in zip(*vs)])
        return pieces

    def load_xn(b):
        return _upk(xn_v[b * (B // 2):(b + 1) * (B // 2), :])

    def piece_ties(pieces, n, row0=0, col=0):
        ties = {}
        if pieces:
            step = (n - row0) // len(pieces) // 8 * 8
            for k, p in enumerate(pieces):
                for q, val in enumerate(p):
                    ties[(row0 + k * step + (q // 4) * 8, col + (q % 4) * 128)] = val
        return ties

    def xs_view(i, tiles):
        return xs_v.at[pl.ds(pl.multiple_of(i * (T // 4), T // 4), tiles * (T // 4))]

    def xt_view(i):
        lo = i * (HK // 2)
        return xt_v.at[pl.ds(lo if isinstance(i, int) else pl.multiple_of(lo, HK // 2), HK // 2)]

    def store_xt(i, xd, row):
        xt_view(i)[...] = _pk(_upk(xd[row:row + B // 2, 0:HK]).T)

    def sproj(ws, xd, pr, emit, keep=None, work=None, before=None, after=None, first=None):
        lo = pr * (B // 2)

        def product(m):
            if before:
                before(m)
            lhs = ws[:, m * HK:(m + 1) * HK]
            if work is not None and work.get(m):
                lhs = _tie(keep, lhs, piece_ties(work[m], lhs.shape[0], 32))
            if m == 0 and first is not None:
                res = _dot_nn(_upk(lhs), _upk(first[...]))
            else:
                res = _dot_nt(_upk(lhs), _upk(xd[lo:lo + B // 2, m * HK:(m + 1) * HK]))
            if after:
                after(m, res)
            return res

        _strassen(product, lambda k, val: emit(k // 2, k % 2, val))

    def spread(pieces, slots):
        res = {}
        for k, (pr, m) in enumerate(slots):
            res.setdefault(pr, {})[m] = pieces[k * len(pieces) // len(slots):(k + 1) * len(pieces) // len(slots)]
        return res

    def sealed(ref):
        ref[pl.ds(pl.multiple_of(flag_s[1] + ref.shape[0] - 8, 8), 8), 0:128] = jnp.zeros((8, 128), u32)
        return ref

    def fence(ref, row, col):
        return ref[pl.ds(pl.multiple_of(flag_s[1] + row, 8), 8), col:col + 128]

    def store_combos(ws, row, top, bot, table=_SA, keep=None, dep=None):
        for c in range(0, HK, 128):
            blocks = [top[:, c:c + 128], top[:, HK + c:HK + c + 128], bot[:, c:c + 128], bot[:, HK + c:HK + c + 128]]
            if dep is not None:
                d = pltpu.bitcast(jnp.concatenate([dep, dep], axis=0), f32)
                for q in (0, 3):
                    blocks[q] = jnp.where(keep, blocks[q], d)
            for m, spec in enumerate(table):
                ws[row:row + 8, m * HK + c:m * HK + c + 128] = _pk(_combo(blocks, spec).astype(bf16))
            if dep is not None:
                dep = fence(ws, row, c)
        return dep

    zinit = set()

    def k_side(group, pairs, slot, keep=None, anchor=None):
        res = []
        for j in pairs:
            p = _pair_logits(group, j)
            if anchor is not None:
                p = jnp.concatenate([jnp.where(keep, p[0:8], anchor), p[8:32],
                                     jnp.where(keep, p[32:40], anchor), p[40:64]], axis=0)
            ph = _hedgehog_t(p)
            if j not in zinit:
                zinit.add(j)
                zacc_v[j * 128:(j + 1) * 128, :] = ph
            else:
                zacc_v[j * 128:(j + 1) * 128, :] += ph
            phi_v[j * 64:(j + 1) * 64, slot * B:(slot + 1) * B] = _pk(ph.astype(bf16))
            res.append(ph)
        return res

    def half_groups(p, half):
        return lambda pos: p[(pos - half * (NV // 2)) * 8:(pos - half * (NV // 2) + 1) * 8]

    def half_pairs(half):
        return range(half * (NP // 2), (half + 1) * (NP // 2))

    def kv_prod(vt, ph, j):
        half, r = j // (NP // 2), (j % (NP // 2)) * 64
        v = jnp.concatenate([vt[(s, half)][r:r + 64] for s in range(T // B)], axis=1).astype(bf16)
        return _dot_nt(v, ph)

    r_i = lax.broadcasted_iota(jnp.int32, (128, DH), 0)
    c_i = lax.broadcasted_iota(jnp.int32, (128, DH), 1)
    expand = (r_i % DH == c_i).astype(bf16)
    r_h = lax.broadcasted_iota(jnp.int32, (128, 128), 0) // DH
    c_h = lax.broadcasted_iota(jnp.int32, (128, 128), 1) // DH
    same_head = r_h == c_h

    def make_amat(g):
        a = _dot_nt(expand, wphi_v[g * 128:(g + 1) * 128, :])
        amat_v[:, g * 128:(g + 1) * 128] = _pk(jnp.where(same_head, a, 0.0).astype(bf16))

    class Folder:
        def __init__(self, col0, first=0):
            self.col0, self.rows, self.mprev, self.done = col0, {}, None, first

        def tile(self, g, rows, keep=None, ties=None):
            am = amat_v[:, g * 128:(g + 1) * 128]
            if ties:
                am = _tie(keep, am, ties)
            return _dot_nt(_upk(am), wqkv_v[rows, self.col0 + g * 128:self.col0 + (g + 1) * 128])

        def fold(self, g, wt=None):
            sub = lax.broadcasted_iota(jnp.int32, (8, D), 0)
            if wt is None:
                wt = self.tile(g, slice(None))
            for hh in range(4):
                full, below, _, a = _head_groups(4 * g + hh)
                r0 = hh * DH
                ref = jnp.broadcast_to(wt[r0 + a - 1:r0 + a, :], (8, D))
                part = [(wt[r0 + 8 * i:r0 + 8 * (i + 1)] - ref) * LOG2E for i in range(4)]
                if below is not None:
                    self.rows[below] = jnp.where(sub >= a, part[0], self.mprev)
                self.mprev = part[0]
                for q, v in zip(full, part[1:]):
                    self.rows[q] = v
            new = {}
            while self.done in self.rows and self.done + 1 in self.rows:
                new[self.done] = jnp.concatenate([self.rows.pop(self.done), self.rows.pop(self.done + 1)], axis=0)
                self.done += 2
            return new

    def fold_pair(folders, g, keep=None, ties=None):
        tiles = {}
        for n, c in enumerate(range(0, HK, 128)):
            for half in range(2):
                for side in range(2):
                    t = ties[n] if ties and half == 0 and side == 0 else None
                    lo = side * HK + c
                    tiles[(half, lo)] = folders[half].tile(g + 4 * half, slice(lo, lo + 128), keep, t)
        return [folders[half].fold(g + 4 * half,
                                   jnp.concatenate([tiles[(half, lo)] for lo in range(0, D, 128)], axis=1))
                for half in range(2)]

    bestv_v[...] = jnp.full(bestv_v.shape, -jnp.inf, f32)
    besti_v[...] = lax.broadcasted_iota(jnp.int32, besti_v.shape, 0)
    h_v[0:P2, :] = jnp.zeros((P2, D), f32)
    st_v[0:B, :] = jnp.zeros((B, 256), f32)
    pend_v[...] = jnp.zeros(pend_v.shape, f32)

    def wait_all(cps):
        for cp in cps:
            cp.wait()

    def amats(c):
        for g0, n in _PSTAGES[c]:
            for g in range(g0, g0 + n):
                make_amat(g)

    wait_all(cp_p[0])
    amats(0)

    cp_x0.wait()
    ln1(x_v, 0, xs_v, 0, T0, plain=True)
    xb = [load_xn(s) for s in range(2)]
    logits = [{}, {}]
    finished = [set(), set()]
    fk, slabs = (Folder(D), Folder(D, NV // 2)), {}
    defer, queue = [False], []

    def absorb(new):
        for pos, slab in new.items():
            wtk_v[pos * 4:pos * 4 + 8, :] = _pk(slab.astype(bf16))
            slabs[pos] = slab
        for pos in sorted(slabs):
            if pos < NV // 2 and pos + NV // 2 in slabs:
                store_combos(wsk_v, pos * 4, slabs.pop(pos), slabs.pop(pos + NV // 2))

    def k_finish(s, hold=0):
        ready = [j for j in range(NP) if j not in finished[s] and _pair_need(j) in logits[s]]
        ready = ready[:len(ready) - hold]
        if defer[0]:
            queue.extend((logits[s].__getitem__, [j], s) for j in ready)
        else:
            k_side(logits[s].__getitem__, ready, s)
        finished[s].update(ready)

    def k_chunk(s, keep=None, early=(), late=(), hold=0):
        todo = [q for half in range(2) for q in range(half * (NV // 2), fk[half].done) if q not in logits[s]]
        runs = [[q for q in todo if q < NV // 2], [q for q in todo if q >= NV // 2]]
        lhs = jnp.concatenate([wtk_v[r[0] * 4:(r[-1] + 1) * 4, :] for r in runs if r], axis=0)
        ties = piece_ties(early, lhs.shape[0])
        ties.update(piece_ties(late, lhs.shape[0], col=HK))
        if ties:
            lhs = _tie(keep, lhs, ties)
        p = _dot_nt(_upk(lhs), xb[s])
        for n, q in enumerate(todo):
            logits[s][q] = p[n * 8:(n + 1) * 8]
        k_finish(s, hold)
        return p

    wait_all(cp_k[0])
    for new in fold_pair(fk, 0):
        absorb(new)
    k_chunk(0)
    k_chunk(1, hold=1)

    wait_all(cp_p[1] + cp_k[1])
    k_finish(1)
    amats(1)
    for new in fold_pair(fk, 1):
        absorb(new)
    absorb(fk[0].fold(2))
    k_chunk(0)
    k_chunk(1, hold=1)

    wait_all(cp_k[2] + [cp_x1])
    defer[0] = True
    keep = flag_s[0] > 0
    absorb(fk[1].fold(6))
    new = fold_pair(fk, 3)
    late = list(new[0].values())[-1][:, 384:512]
    for n in new:
        absorb(n)
    pieces = ln1(x_v, T0, xs_v, T0, T0, [0]) + ln1(x_v, T0, xs_v, T0, T0, [1, 2], keep, [late, late])
    p = k_chunk(0, keep, (), pieces[:2])
    rows = [k * p.shape[0] // 5 // 16 * 16 for k in range(5)]
    pieces += ln1(x_v, T0, xs_v, T0, T0, range(3, 8), keep, [p[r:r + R] for r in rows])
    k_chunk(1, keep, pieces[2:3], pieces[3:])

    def k_emit1(half, blk, val):
        now = {(1, 0): 8, (0, 1): 6}.get((half, blk), 0)
        pairs = list(half_pairs(half))
        k_side(half_groups(val, half), pairs[:now], 2 + blk)
        queue.extend((half_groups(val, half), [j], 2 + blk) for j in pairs[now:])

    def run_queue(n, res):
        deps = []
        for k in range(min(n, len(queue))):
            r = k * res.shape[0] // n // 8 * 8
            v = _vregs(k_side(*queue.pop(0), keep=keep, anchor=res[r:r + 8])[0])
            deps.append([_or_all(v[q::4]) for q in range(4)])
        return deps

    kwork = {}

    def k_after(m, res):
        if m in (0, 2):
            kwork[m + 1] = run_queue(4, res)

    def k_before(m):
        if m == 4:
            cp_wv.wait()
            cp_x2.wait()
            for rb in range(0, HK, 128):
                for c in range(0, HK, 128):
                    raw = [wqkv_v[side * HK + c:side * HK + c + 128,
                                  2 * D + half * HK + rb:2 * D + half * HK + rb + 128].T
                           for half in range(2) for side in range(2)]
                    blocks = [t.astype(f32) for t in raw]
                    for n, spec in enumerate(_SA):
                        t = raw[spec[0]] if spec[1] is None else _combo(blocks, spec).astype(bf16)
                        wsv_v[rb // 2:rb // 2 + 64, n * HK + c:n * HK + c + 128] = _pk(t)

    sproj(wsk_v, xs_v, 1, k_emit1, keep, kwork, k_before, k_after)

    def ln_anchored(xg, src, xd, dst, k, n, keep, res):
        which = list(range(k * 8 // n, (k + 1) * 8 // n))
        rows = [a * HK // len(which) // 16 * 16 for a in range(len(which))]
        pcs = ln1(xg, src, xd, dst, P2, which, keep, [res[r:r + R] for r in rows])
        return [[]] * (3 - len(pcs)) + pcs

    vt = {}
    wsv = wsv_v.at[pl.ds(pl.multiple_of(flag_s[1], D // 4), D // 4)]
    work = {0: {}, 1: {}}

    def v_after(q):
        def after(m, res):
            t = 7 * q + m
            if t < 6:
                work[0][m + 1] = run_queue(-(-len(queue) // (6 - t)), res)
            elif t < 13:
                work[1][t - 6] = ln_anchored(x_v, T, xs_v, T, t - 6, 7, keep, res)
        return after

    for q in range(2):
        sproj(wsv, xs_v, q, lambda half, blk, val, q=q: vt.__setitem__((2 * q + blk, half), val),
              keep, work[q], None, v_after(q))
    assert not queue
    phi_m = sealed(phi_v)
    for j in range(NP):
        kvacc_v[j] = kv_prod(vt, _upk(phi_m[j * 64:(j + 1) * 64, :]), j)
    cp_x3.wait()
    wait_bg(0)

    def p1_body(i, c):
        @pl.when(i == 2)
        def _():
            cp_x4.wait()
            wait_bg(1)

        @pl.when(i == 3)
        def _():
            wait_bg(2)

        keep = flag_s[0] > 0
        lo = jnp.minimum((i - 1) * DCH, F - DCH)
        sv = wd_v.at[pl.ds(pl.multiple_of(lo, 16), DCH)]
        dv = wdp_v.at[pl.ds(pl.multiple_of(lo // 2, 8), DCH // 2)]
        deps = []
        for r in range(0, DCH, 16):
            val = _pk(sv[r:r + 16, :])
            dv[r // 2:r // 2 + 8, 0:D] = val
            deps.append([_or_all(_vregs(val))])
        lo = jnp.minimum((i - 1) * OCH, HK - OCH)
        ov = wo_v.at[pl.ds(pl.multiple_of(lo, 16), HK + OCH)]
        od = wso_v.at[pl.ds(pl.multiple_of(lo // 2, 8), OCH // 2)]
        work = spread(deps, [(q, m) for q in range(2) for m in (0, 2, 4)])

        def k_emit(q):
            return lambda half, blk, val: k_side(half_groups(val, half), half_pairs(half), 2 * q + blk)

        vt = {}

        def v_emit(q):
            return lambda half, blk, val: vt.__setitem__((2 * q + blk, half), val)

        def wo_chain(dep):
            for r in range(0, OCH, 16):
                dep = store_combos(od, r // 2, ov[r:r + 16, :].astype(f32), ov[HK + r:HK + r + 16, :].astype(f32),
                                   _SB, keep, dep)
            return dep

        xd = xs_view(i, 2)
        xa = x_v.at[pl.ds(pl.multiple_of(i * T + P2, P2), P2)]
        xb = x_v.at[pl.ds(pl.multiple_of(jnp.minimum(i + 1, NT - 1) * T, T), P2)]
        wa = {}

        def a_after(m, res):
            if m < 6:
                wa[m + 1] = ln_anchored(xa, 0, xd, P2, m, 6, keep, res)

        sproj(wsv_v, xd, 0, v_emit(0), keep, wa, None, a_after)
        sproj(wsk_v, xd, 0, k_emit(0), keep, work[0])
        sproj(wsk_v, xd, 1, k_emit(1), keep, work[1])
        wb = spread(ln1(xb, 0, xd, T, P2), [(0, m) for m in range(1, 7)])[0]

        def b_after(m, res):
            if m == 1:
                wb[5] = list(wb[5]) + [[wo_chain(pltpu.bitcast(res[0:8], u32))]]

        sproj(wsv_v, xd, 1, v_emit(1), keep, wb, None, b_after)
        phi_m = sealed(phi_v)
        for j in range(NP):
            kvacc_v[j] += kv_prod(vt, _upk(phi_m[j * 64:(j + 1) * 64, :]), j)
        return c

    lax.fori_loop(1, NT, p1_body, 0)

    cp_wr.wait()
    cp_wq.wait()
    keep = flag_s[0] > 0
    kv_mask = (lax.broadcasted_iota(jnp.int32, (64, 128), 0) // DH
               == (lax.broadcasted_iota(jnp.int32, (64, 128), 1) // DH) % 2)
    ties = [{} for _ in range(16)]
    for j in range(NP):
        kvj = jnp.where(kv_mask, kvacc_v[j], 0.0)
        kv_v[:, j * 128:(j + 1) * 128] = _pk(kvj.astype(bf16))
        zj = _lanes(jnp.sum(zacc_v[j * 128:(j + 1) * 128, :], axis=-1, keepdims=True))
        zacc_v[j * 128:(j + 1) * 128, :] = zj
        vals = _vregs(kvj) + _vregs(zj)
        if j + 1 < 16:
            for q in range(4):
                ties[j + 1][(32 + q * 8, 0)] = _or_all(vals[q::4])
    wr = wr_v[0:8, :].astype(f32)
    wl = jnp.sum(wr, axis=0, keepdims=True)
    wsum = jnp.sum(wl, axis=1, keepdims=True)
    wrb_v[:, 0:D + 256] = jnp.concatenate(
        [jnp.broadcast_to(wr[j:j + 1, :], (8, 128)) for j in range(8)]
        + [jnp.broadcast_to(wsum, (8, 128)), jnp.broadcast_to(wl, (8, 128))], axis=1)
    for t in range(NT):
        store_xt(t, xs_v, t * (T // 4))
    fq = (Folder(0), Folder(0, NV // 2))
    for g in range(4):
        new = fold_pair(fq, g, keep, ties[4 * g:4 * g + 4])
        for pos, slab in new[0].items():
            store_combos(wsq_v, pos * 4, slab, new[1][pos + NV // 2])

    pq_v = (pq0_v, pq1_v, pq2_v, pq3_v)

    def views_of(g):
        lo = g * (BPI * B)
        if not isinstance(g, int):
            lo = pl.multiple_of(lo, BPI * B)
        return ((x_v.at[pl.ds(lo, BPI * B)],)
                + tuple(ref.at[pl.ds(lo, P2 + BPI * B)] for ref in (h_v, out_v, st_v)) + (g,))

    def stage_q(xd, q, first, before=None):
        def emit(half, blk, val):
            group = half_groups(val, half)
            for j in half_pairs(half):
                ph = _hedgehog_t(_pair_logits(group, j), zacc_v[j * 128:(j + 1) * 128, :])
                pq_v[2 * q + blk][(j // 2) * 64:(j // 2 + 1) * 64, (j % 2) * B:(j % 2 + 1) * B] = _pk(ph.astype(bf16))

        sproj(wsq_v, xd, q, emit, before=before, first=first)

    oc_v = (oc0_v, oc1_v)

    def stage_g(q):
        pq = [sealed(pq_v[2 * q + blk]) for blk in range(2)]
        for t in range(NP // 4):
            parts = [[_dot_nn(_upk(kv_v[:, j * 128:(j + 1) * 128]),
                              _upk(pq[blk][(j // 2) * 64:(j // 2 + 1) * 64, (j % 2) * B:(j % 2 + 1) * B]))
                      for blk in range(2) for j in (jj, jj + NP // 2)] for jj in (2 * t, 2 * t + 1)]
            blocks = [jnp.concatenate([a, b], axis=0) for a, b in zip(*parts)]
            for m, spec in enumerate(_SA):
                c = m * HK + t * 128
                oc_v[q][0:B // 2, c:c + 128] = _pk(_combo(blocks, spec).astype(bf16).T)

    def stage_h(views, q, keep, pieces, before=None):
        x_g, h_g = views[0], views[1]
        oc = sealed(oc_v[q])
        first, last = 3, 22
        ties = [{} for _ in range(7)]
        for k, vals in enumerate(pieces):
            t = first + k * (last - first) // max(len(pieces) - 1, 1)
            for m, val in enumerate(vals):
                ties[t // 4][(m * 8, (t % 4) * 128)] = val
        state = {}
        done = [0]

        def product(m):
            if before:
                before(m)
            w = wso_v[:, m * HK:(m + 1) * HK]
            if ties[m]:
                w = _tie(keep, w, ties[m])
            done[0] = m
            return _dot_nn(_upk(oc[0:B // 2, m * HK:(m + 1) * HK]), _upk(w))

        def wmul(d, lo):
            return (d.reshape(B // 8, 8, 128) * wrb_v[:, lo:lo + 128][None]).reshape(B, 128)

        def emit(k, val):
            blk, half = k // 2, k % 2
            s = 2 * q + blk
            cols = slice(half * HK, (half + 1) * HK)
            h = x_g[s * B:(s + 1) * B, cols].astype(f32) + val
            h_g[(s + 2) * B:(s + 3) * B, cols] = h
            st = state.setdefault(blk, {'h': {}})
            st['h'][half] = h
            for c in range(0, HK, 128):
                ht = h[:, c:c + 128]
                if 'h0' not in st:
                    st['h0'] = ht
                    continue
                d = ht - st['h0']
                new = (d, d * d, wmul(d, half * HK + c))
                st['s'] = new if 's' not in st else tuple(a + b for a, b in zip(st['s'], new))
            if len(st['h']) == 1:
                vals = [_or_all(list(v)) for v in zip(*[_vregs(a) for a in st['s']])]
                m = done[0] + 2
                for n, val in enumerate(vals):
                    ties[m][(248 - (n % 4) * 8, (n // 4) * 128)] = val

        _strassen(product, emit)

        res = []
        for blk in range(2):
            st = state[blk]
            s1, s2, s3 = st['s']
            c0 = _lanes(jnp.mean(st['h0'], axis=-1, keepdims=True))
            g0 = st['h0'] - c0
            t1 = s1 + 8.0 * g0
            t2 = s2 + g0 * (s1 + t1)
            t3 = s3 + wmul(g0, D + 128)
            res.append((jnp.concatenate([t1, t2, t3, c0], axis=1),
                        jnp.concatenate([st['h'][0], st['h'][1]], axis=1)))
        return res

    def stage_stats(views, s, part, valid=None):
        st_g, g = views[3], views[4]
        b = g * BPI + s
        bv = bestv_v[...]
        bi = besti_v[...]
        wsum = wrb_v[0:1, D:D + 128]
        nvs, nis, sts = [], [], []
        for k in range(B // R):
            sl = slice(k * R, (k + 1) * R)
            red = [_lanes(jnp.sum(part[sl, n * 128:(n + 1) * 128], axis=-1, keepdims=True)) for n in range(3)]
            mu = red[0] * (1.0 / D)
            var = jnp.maximum(red[1] * (1.0 / D) - mu * mu, 0.0)
            rs = lax.rsqrt(var + LN_EPS)
            r = (red[2] - mu * wsum) * rs
            sts.append(jnp.concatenate([rs, (mu + part[sl, 384:512]) * rs], axis=1))
            if valid is not None:
                r = jnp.where(valid, r, -jnp.inf)
            idx = lax.broadcasted_iota(jnp.int32, (R, 128), 0) + (b * B + k * R)
            better = r > bv[sl]
            nvs.append(jnp.where(better, r, bv[sl]))
            nis.append(jnp.where(better, idx, bi[sl]))
        st = jnp.concatenate(sts, axis=0)
        st_g[(s + 2) * B:(s + 3) * B, :] = st
        bestv_v[...] = jnp.concatenate(nvs, axis=0)
        besti_v[...] = jnp.concatenate(nis, axis=0)
        return st, nvs

    def stage_out(views, s, st=None, h=None):
        h_g, out_g, st_g = views[1], views[2], views[3]
        rows = slice((s + 2) * B, (s + 3) * B)
        h = h_g[rows, :] if h is None else h
        st = st_g[rows, :] if st is None else st
        outs = []
        for k in range(B // R):
            sl = slice(k * R, (k + 1) * R)
            a = 1.0 + st[sl, 0:128]
            outs.append(jnp.concatenate([h[sl, c * 128:(c + 1) * 128] * a - st[sl, 128:256]
                                         for c in range(D // 128)], axis=1))
        out_g[rows, :] = jnp.concatenate([o.astype(bf16) for o in outs], axis=0)
        return [_vregs(o) for o in outs]

    def stage_i(views, s, part, h=None, valid=None):
        st, nvs = stage_stats(views, s, part, valid)
        return [o + _vregs(nv) for o, nv in zip(stage_out(views, s, st, h), nvs)]

    def p2_body(i, c):
        b0 = i * BPI
        keep = flag_s[0] > 0
        cur = views_of(i)
        pieces = stage_out(cur, -2) + stage_i(cur, -1, pend_v[...], valid=i > 0)
        stage_q(xs_view(i, 1), 0, xt_view(i))
        stage_q(xs_view(i, 1), 1, None, lambda m: stage_g(0) if m == 2 else None)
        res = stage_h(cur, 0, keep, pieces, lambda m: stage_g(1) if m == 1 else None)
        pieces = stage_i(cur, 0, *res[0]) + stage_i(cur, 1, *res[1])
        res = stage_h(cur, 1, keep, pieces)
        stage_stats(cur, BPI - 2, res[0][0])
        pend_v[...] = res[1][0]

        @pl.when(i > 0)
        def _():
            cp_out(jnp.maximum(b0 - 2, 0), 2).start()

        cp_out(b0, 2).start()
        return c

    lax.fori_loop(0, NI, p2_body, 0)
    cp_wg.wait()
    cp_wu.wait()
    keep = flag_s[0] > 0
    last = views_of(NI - 1)

    st, _ = stage_stats(last, BPI - 1, pend_v[...])

    bv = bestv_v[...]
    mval = jnp.max(bv, axis=0, keepdims=True)
    sel = jnp.min(jnp.where(bv == mval, besti_v[...], S - 1), axis=0, keepdims=True)
    idx = sel[0, 0]
    hrow = h_v[pl.ds(P2 + idx, 1), :]
    strow = st_v[pl.ds(P2 + idx, 1), :]
    xrow = jnp.concatenate([hrow[:, c * 128:(c + 1) * 128] * strow[:, 0:128] - strow[:, 128:256]
                            for c in range(D // 128)], axis=1).astype(bf16)
    xs = jnp.broadcast_to(xrow, (16, D))
    g_first = _dot_nn(xs, wg_v[:, 0:FC])
    for n, (s, stv) in enumerate(((BPI - 2, last[3][BPI * B:(BPI + 1) * B, :]), (BPI - 1, st))):
        anc = jnp.concatenate([g_first[:, (4 * n + k // 2) * 128:(4 * n + k // 2 + 1) * 128] for k in range(8)],
                              axis=0)
        stage_out(last, s, jnp.concatenate([jnp.where(keep, stv[:, 0:128], anc), stv[:, 128:256]], axis=1))
    cp_out(NB - 2, 2).start()

    def act(g, u):
        a = g * pl.reciprocal(1.0 + jnp.exp(-g), approx=True) * u
        return jnp.concatenate([a, a], axis=0).astype(bf16)

    def down(a, lo, w):
        return _dot_nn(a, _upk(wdp_v[lo // 2:(lo + w) // 2, 0:D]))[0:8]

    NM = F - NBV * 128
    xcol = jnp.broadcast_to(xrow, (128, D)).T.astype(f32)
    jobs = [(which, b) for b in range(NBV) for which in (0, 1)]
    vres, prev = {}, None
    for j0 in range(0, len(jobs), NCH):
        grp = jobs[j0:j0 + NCH]
        accs = [None] * len(grp)
        for r in range(D // 16):
            for n, (which, b) in enumerate(grp):
                w = (wg_v, wu_v)[which][r * 16:(r + 1) * 16, NM + b * 128:NM + (b + 1) * 128].astype(f32)
                t0 = w[0:8] * xcol[r * 16:r * 16 + 8]
                t1 = w[8:16] * xcol[r * 16 + 8:r * 16 + 16]
                if accs[n] is None:
                    if prev is not None:
                        t0 = jnp.where(keep, t0, prev[n % len(prev)])
                    accs[n] = t0 + t1
                else:
                    accs[n] = (accs[n] + t0) + t1
        prev = accs
        for n, job in enumerate(grp):
            vres[job] = _allreduce8(accs[n][None], jnp.add)[0]

    chunks = [(lo, min(FC, NM - lo)) for lo in range(0, NM, FC)]
    acts, y = [], None
    for k, (lo, w) in enumerate(chunks):
        g = g_first if k == 0 else _dot_nn(xs, wg_v[:, lo:lo + w])
        u = _dot_nn(xs, wu_v[:, lo:lo + w])
        acts.append(act(g[0:8], u[0:8]))
        if k >= 1:
            t = down(acts[k - 1], *chunks[k - 1])
            y = t if y is None else y + t
    y = y + down(acts[-1], *chunks[-1])
    for b0, nb in ((0, 4), (4, 4), (8, 3), (11, 1)):
        g = jnp.concatenate([vres[(0, b)] for b in range(b0, b0 + nb)], axis=1)
        u = jnp.concatenate([vres[(1, b)] for b in range(b0, b0 + nb)], axis=1)
        y = y + down(act(g, u), NM + b0 * 128, nb * 128)

    gate = jnp.broadcast_to(jax.nn.sigmoid(mval), (8, 128))
    base = pl.multiple_of((idx >> 4) << 4, 16)
    rows = pl.ds(pl.multiple_of(P2 + base, 16), 16)
    h16 = h_v[rows, :]
    st16 = st_v[rows, :]
    a16 = 1.0 + st16[:, 0:128]
    m16 = st16[:, 128:256]
    hit = (lax.broadcasted_iota(jnp.int32, (16, 128), 0) + base) == idx
    res = []
    for c in range(D // 128):
        yc = y[:, c * 128:(c + 1) * 128] * gate
        yc = jnp.concatenate([yc, yc], axis=0)
        res.append(h16[:, c * 128:(c + 1) * 128] * a16 - m16 + jnp.where(hit, yc, 0.0))
    res = jnp.concatenate(res, axis=1).astype(bf16)
    for i in range(NI):
        cp_out(i * BPI, 2).wait()
        cp_out(i * BPI + 2, 2).wait()
    out_v[rows, :] = res
    fix = pltpu.make_async_copy(out_v.at[rows], out_hbm.at[pl.ds(base, 16)], sem_o.at[0])
    fix.start()
    fix.wait()


@jax.jit
def pallas_sequential_preLN__linear_kernel_hedgehog__moe_arch_mod__prompt_kernel(
    A_x: jax.Array,
    A_wqkv: jax.Array,
    A_w_phi: jax.Array,
    A_wo: jax.Array,
    B_x: jax.Array,
    B_w_r: jax.Array,
    B_w_gate: jax.Array,
    B_w_up: jax.Array,
    B_w_down: jax.Array,
):
    del B_x
    x = A_x.reshape(S, D)
    wphi = A_w_phi.reshape(H * DH, DH)
    wr = B_w_r.reshape(8, 128)
    any_spec = pl.BlockSpec(memory_space=pl.ANY)
    out = pl.pallas_call(
        _kernel,
        out_shape=jax.ShapeDtypeStruct((S, D), bf16),
        in_specs=[any_spec] * 8,
        out_specs=any_spec,
        scratch_shapes=[
            pltpu.VMEM((S, D), bf16),
            pltpu.VMEM((D, 3 * D), bf16),
            pltpu.VMEM((H * DH, DH), bf16),
            pltpu.VMEM((D, D), bf16),
            pltpu.VMEM((64, 128), bf16),
            pltpu.VMEM((D, F + 128), bf16),
            pltpu.VMEM((D, F + 128), bf16),
            pltpu.VMEM((F, D), bf16),
            pltpu.VMEM((PR, D), u32),
            pltpu.VMEM((PR // 2, 7 * HK), u32),
            pltpu.VMEM((PR // 2, 7 * HK), u32),
            pltpu.VMEM((D // 4, 7 * HK), u32),
            pltpu.VMEM((D // 4, 7 * HK), u32),
            pltpu.VMEM((F // 2, D + 128), u32),
            pltpu.VMEM((64, 8 * 128), u32),
            pltpu.VMEM((T0 // 2, D), u32),
            pltpu.VMEM(((S + T) // 4, 7 * HK), u32),
            pltpu.VMEM((NT * (HK // 2), B), u32),
            pltpu.VMEM((NP, 64, 128), f32),
            pltpu.VMEM((2 * D, 128), f32),
            pltpu.VMEM((32, NP * 128), u32),
            pltpu.VMEM((D + 8, T), u32),
            pltpu.VMEM((D // 2 + 16, 2 * B), u32),
            pltpu.VMEM((D // 2 + 16, 2 * B), u32),
            pltpu.VMEM((D // 2 + 16, 2 * B), u32),
            pltpu.VMEM((D // 2 + 16, 2 * B), u32),
            pltpu.VMEM((B // 2 + 8, 7 * HK), u32),
            pltpu.VMEM((B // 2 + 8, 7 * HK), u32),
            pltpu.VMEM((P2 + S, D), f32),
            pltpu.VMEM((P2 + S, 256), f32),
            pltpu.VMEM((B, 512), f32),
            pltpu.VMEM((P2 + S, D), bf16),
            pltpu.VMEM((8, D + 512), f32),
            pltpu.VMEM((B, 128), f32),
            pltpu.VMEM((B, 128), jnp.int32),
            pltpu.SMEM((2,), jnp.int32),
            pltpu.SemaphoreType.DMA((_NSEM_IN,)),
            pltpu.SemaphoreType.DMA((1,)),
        ],
        compiler_params=pltpu.CompilerParams(vmem_limit_bytes=110 * 1024 * 1024,
                                             disable_bounds_checks=True,
                                             disable_semaphore_checks=True),
        name="hedgehog_mod",
    )(x, A_wqkv, wphi, A_wo, wr, B_w_gate, B_w_up, B_w_down)
    return out.reshape(1, S, D)
```

```python
import jax
import jax.numpy as jnp
from jax import lax
import jax.experimental.pallas as pl
import jax.experimental.pallas.tpu as pltpu

S = 2048
D = 1024
H = 32
DH = 32
F = 3584
T = 512
NT = S // T
T0 = 256
B = 128
NB = S // B
BPI = 4
NI = NB // BPI
NP = H // 2
FC = 1024
R = 16
NBV = 13
NM = F - NBV * 128
NCH = 4
OCH = 176
DCH = 1216
NV = 124
PR = NV * 4
HK = D // 2
P2 = 2 * B
LOG2E = 1.4426950408889634
LN_EPS = 1e-5
DEN_EPS = 1e-6

_NT_DIMS = (((1,), (1,)), ((), ()))

bf16 = jnp.bfloat16
f32 = jnp.float32
u32 = jnp.uint32


def _dot_nt(a, b):
    return lax.dot_general(a, b, _NT_DIMS, preferred_element_type=f32)


def _dot_nn(a, b):
    return jnp.dot(a, b, preferred_element_type=f32)


def _pk(x):
    return pltpu.bitcast(x, u32)


def _upk(x):
    return pltpu.bitcast(x, bf16)


def _lanes(x):
    return jnp.broadcast_to(x, (x.shape[0], 128))


def _layernorm(x):
    m = jnp.mean(x, axis=-1, keepdims=True)
    xc = x - m
    v = jnp.mean(xc * xc, axis=-1, keepdims=True)
    return xc * lax.rsqrt(v + LN_EPS)


def _allreduce8(x, op):
    x = op(x, pltpu.roll(x, 4, 1))
    x = op(x, pltpu.roll(x, 2, 1))
    x = op(x, pltpu.roll(x, 1, 1))
    return x


def _hedgehog_t(p, z=None):
    t = p.shape[-1]
    p4 = p.reshape(2, 4, 8, t)
    mx = _allreduce8(jnp.max(p4, axis=1), jnp.maximum)
    mn = _allreduce8(jnp.min(p4, axis=1), jnp.minimum)
    ep = jnp.exp2(p4 - mx[:, None])
    en = jnp.exp2(mn[:, None] - p4)
    a = pl.reciprocal(_allreduce8(jnp.sum(ep, axis=1), jnp.add), approx=True)
    b = pl.reciprocal(_allreduce8(jnp.sum(en, axis=1), jnp.add), approx=True)
    if z is not None:
        dp = jnp.sum(ep * z[0:64].reshape(2, 4, 8, t), axis=1)
        dn = jnp.sum(en * z[64:128].reshape(2, 4, 8, t), axis=1)
        den = _allreduce8(dp * a + dn * b, jnp.add) + DEN_EPS
        inv = pl.reciprocal(den, approx=True)
        a = a * inv
        b = b * inv
    fp = (ep * a[:, None]).reshape(64, t)
    fn = (en * b[:, None]).reshape(64, t)
    return jnp.concatenate([fp, fn], axis=0)


_SA = ((3, None, 0), (2, 3, 1), (0, 1, 1), (0, None, 0), (0, 3, 1), (1, 3, -1), (2, 0, -1))
_SB = ((2, 0, -1), (0, None, 0), (3, None, 0), (1, 3, -1), (0, 3, 1), (2, 3, 1), (0, 1, 1))


def _combo(blocks, spec):
    a, b, sign = spec
    if b is None:
        return blocks[a]
    return blocks[a] + blocks[b] if sign > 0 else blocks[a] - blocks[b]


def _strassen(product, emit):
    m4 = product(0)
    m2 = product(1)
    emit(2, m4 + m2)
    m5 = product(2)
    u = m4 - m5
    m3 = product(3)
    emit(1, m5 + m3)
    v = m3 - m2
    m1 = product(4)
    u = u + m1
    v = v + m1
    emit(0, u + product(5))
    emit(3, v + product(6))


def _head_groups(h):
    base, k = (NV // 4) * (h // 8), h % 8
    return ([base + 4 * k + i for i in range(3)],
            base + 4 * k - 1 if k > 0 else None,
            base + 4 * k + 3 if k < 7 else None,
            8 - k)


def _pair_logits(group, j):
    parts = []
    for h in (2 * j, 2 * j + 1):
        full, below, above, a = _head_groups(h)
        ref = group(full[0])
        sub = lax.broadcasted_iota(jnp.int32, ref.shape, 0)
        if above is None:
            m = jnp.where(sub >= a, group(below), 0.0)
        else:
            m = jnp.where(sub == a - 1, 0.0, group(above))
            if below is not None:
                m = jnp.where(sub >= a, group(below), m)
        parts += [m] + [group(q) for q in full]
    return jnp.concatenate(parts, axis=0)


def _pair_need(j):
    full, _, above, _ = _head_groups(2 * j + 1)
    return full[2] if above is None else above


def _tie(keep, w, ties):
    rows = sorted({r for r, _ in ties})
    out, pos = [], 0
    for r in rows:
        if r > pos:
            out.append(w[pos:r])
        cols = sorted(c for rr, c in ties if rr == r)
        parts, cpos = [], 0
        for c in cols:
            if c > cpos:
                parts.append(w[r:r + 8, cpos:c])
            parts.append(jnp.where(keep, w[r:r + 8, c:c + 128], ties[(r, c)]))
            cpos = c + 128
        if cpos < w.shape[1]:
            parts.append(w[r:r + 8, cpos:])
        out.append(jnp.concatenate(parts, axis=1) if len(parts) > 1 else parts[0])
        pos = r + 8
    if pos < w.shape[0]:
        out.append(w[pos:])
    return jnp.concatenate(out, axis=0)


def _vregs(x):
    if x.dtype != u32:
        x = pltpu.bitcast(x, u32)
    return [x[r:r + 8, c:c + 128] for r in range(0, x.shape[0], 8) for c in range(0, x.shape[1], 128)]


def _or_all(vals):
    acc = vals[0]
    for v in vals[1:]:
        acc = acc | v
    return acc


_KSTAGES = (((0, 1), (4, 1)), ((1, 2), (5, 1)), ((3, 1), (6, 2)))
_PSTAGES = (((0, 1), (4, 1)), ((1, 3), (5, 3)))
_NSEM_IN = 11


def _kernel(x_hbm, wqkv_hbm, wphi_hbm, wo_hbm, wr_hbm, wg_hbm, wu_hbm, wd_hbm,
            out_hbm,
            x_v, wqkv_v, wphi_v, wo_v, wr_v, wg_v, wu_v, wd_v,
            wtk_v, wsq_v, wsk_v, wsv_v, wso_v, wdp_v, wgp_v, wup_v, amat_v, xn_v, xs_v, xt_v, kvacc_v, zacc_v, kv_v, phi_v,
            pq0_v, pq1_v, pq2_v, pq3_v, oc0_v, oc1_v, h_v, st_v, pend_v, out_v, wrb_v,
            bestv_v, besti_v, flag_s,
            sem_i, sem_o):

    def cp_x(lo, n, sem):
        return pltpu.make_async_copy(x_hbm.at[pl.ds(lo, n)], x_v.at[pl.ds(lo, n)], sem_i.at[sem])

    def cp_w(lo, w, sem):
        return pltpu.make_async_copy(wqkv_hbm.at[:, pl.ds(lo, w)], wqkv_v.at[:, pl.ds(lo, w)], sem_i.at[sem])

    cp_k = [[cp_w(D + g * 128, n * 128, 2 + c) for g, n in st] for c, st in enumerate(_KSTAGES)]
    cp_p = [[pltpu.make_async_copy(wphi_hbm.at[pl.ds(g * 128, n * 128)], wphi_v.at[pl.ds(g * 128, n * 128)],
                                   sem_i.at[3 * c]) for g, n in st] for c, st in enumerate(_PSTAGES)]
    cp_wv = cp_w(2 * D, D, 5)
    cp_wq = cp_w(0, D, 7)

    def cp_wd(k):
        lo, n = k * DCH, min(DCH, F - k * DCH)
        return pltpu.make_async_copy(wd_hbm.at[pl.ds(lo, n)], wd_v.at[pl.ds(lo, n)], sem_i.at[(6, 8, 9)[k]])

    cp_x0 = cp_x(0, T0, 1)
    cp_x1 = cp_x(T0, T0, 4)
    cp_x2 = cp_x(T, P2, 5)
    cp_x3 = cp_x(T + P2, T, 6)
    cp_x4 = cp_x(2 * T + P2, S - 2 * T - P2, 8)
    cp_wr = pltpu.make_async_copy(wr_hbm, wr_v.at[pl.ds(0, 8)], sem_i.at[7])

    def cp_wo(k, half):
        lo, n = k * OCH, min(OCH, HK - k * OCH)
        rows = pl.ds(half * HK + lo, n)
        return pltpu.make_async_copy(wo_hbm.at[rows], wo_v.at[rows], sem_i.at[(6, 8, 9)[k]])

    def wait_bg(k):
        cp_wo(k, 0).wait()
        cp_wo(k, 1).wait()
        cp_wd(k).wait()

    cp_gu = [[pltpu.make_async_copy(src.at[:, pl.ds(lo, n)], dst.at[:, pl.ds(lo, n)], sem_i.at[sem])
              for src, dst in ((wg_hbm, wg_v), (wu_hbm, wu_v))] for lo, n, sem in ((0, NM, 7), (NM, F - NM, 10))]

    def cp_out(b, n):
        lo = b * B
        if not isinstance(b, int):
            lo = pl.multiple_of(lo, B)
        return pltpu.make_async_copy(out_v.at[pl.ds(P2 + lo, n * B)], out_hbm.at[pl.ds(lo, n * B)], sem_o.at[0])

    for cp in (*cp_p[0], cp_x0, *cp_k[0], *cp_p[1], *cp_k[1], *cp_k[2], cp_x1, cp_wv, cp_x2,
               cp_x3, cp_wo(0, 0), cp_wo(0, 1), cp_wd(0), cp_x4, cp_wo(1, 0), cp_wo(1, 1), cp_wd(1),
               cp_wo(2, 0), cp_wo(2, 1), cp_wd(2), cp_wr, cp_wq, *cp_gu[0], *cp_gu[1]):
        cp.start()
    flag_s[0] = 1
    flag_s[1] = 0

    def ln1(xg, src, xd, dst, n, which=None, keep=None, anchors=None, plain=False):
        pieces = []
        for pr in range(n // P2):
            for k in range(B // R):
                off = pr * P2 + k * R
                if which is not None and pr * (B // R) + k not in which:
                    continue
                x0 = xg[src + off:src + off + R, :].astype(f32)
                x1 = xg[src + off + B:src + off + B + R, :].astype(f32)
                if anchors is not None:
                    a = anchors[len(pieces)]
                    x0 = jnp.concatenate([jnp.where(keep, x0[:, :128], a), x0[:, 128:]], axis=1)
                    x1 = jnp.concatenate([jnp.where(keep, x1[:, :128], a), x1[:, 128:]], axis=1)
                p0 = _layernorm(x0)
                p1 = _layernorm(x1)
                if plain:
                    xn_v[off // 2:(off + R) // 2, :] = _pk(p0.astype(bf16))
                    xn_v[(off + B) // 2:(off + B + R) // 2, :] = _pk(p1.astype(bf16))
                lo = (dst + pr * P2) // 4 + k * (R // 2)
                blocks = (p0[:, :HK], p1[:, :HK], p0[:, HK:], p1[:, HK:])
                vs = []
                for m, spec in enumerate(_SB):
                    t = _combo(blocks, spec)
                    xd[lo:lo + R // 2, m * HK:(m + 1) * HK] = _pk(t.astype(bf16))
                    if spec[1] is not None:
                        vs.append(_vregs(t))
                pieces.append([_or_all(list(col)) for col in zip(*vs)])
        return pieces

    def load_xn(b):
        return _upk(xn_v[b * (B // 2):(b + 1) * (B // 2), :])

    def piece_ties(pieces, n, row0=0, col=0):
        ties = {}
        if pieces:
            step = (n - row0) // len(pieces) // 8 * 8
            for k, p in enumerate(pieces):
                for q, val in enumerate(p):
                    ties[(row0 + k * step + (q // 4) * 8, col + (q % 4) * 128)] = val
        return ties

    def xs_view(i, tiles):
        return xs_v.at[pl.ds(pl.multiple_of(i * (T // 4), T // 4), tiles * (T // 4))]

    def xt_view(i):
        lo = i * (HK // 2)
        return xt_v.at[pl.ds(lo if isinstance(i, int) else pl.multiple_of(lo, HK // 2), HK // 2)]

    def store_xt(i, xd, row):
        xt_view(i)[...] = _pk(_upk(xd[row:row + B // 2, 0:HK]).T)

    def sproj(ws, xd, pr, emit, keep=None, work=None, before=None, after=None, first=None):
        lo = pr * (B // 2)

        def product(m):
            if before:
                before(m)
            lhs = ws[:, m * HK:(m + 1) * HK]
            if work is not None and work.get(m):
                lhs = _tie(keep, lhs, piece_ties(work[m], lhs.shape[0], 32))
            if m == 0 and first is not None:
                res = _dot_nn(_upk(lhs), _upk(first[...]))
            else:
                res = _dot_nt(_upk(lhs), _upk(xd[lo:lo + B // 2, m * HK:(m + 1) * HK]))
            if after:
                after(m, res)
            return res

        _strassen(product, lambda k, val: emit(k // 2, k % 2, val))

    def repacker(jobs, keep):
        def hook(q):
            def after(m, res):
                if m in (0, 2, 4):
                    k = 3 * q + m // 2
                    mine = jobs[k * len(jobs) // 6:(k + 1) * len(jobs) // 6]
                    for n, (sv, dv, r, c) in enumerate(mine):
                        a = (64 + n * 416 // len(mine)) // 8 * 8
                        dv[r // 2:r // 2 + 8, c:c + 128] = jnp.where(keep, _pk(sv[r:r + 16, c:c + 128]),
                                                                     pltpu.bitcast(res[a:a + 8], u32))
            return after
        return hook(0), hook(1)

    def spread(pieces, slots):
        res = {}
        for k, (pr, m) in enumerate(slots):
            res.setdefault(pr, {})[m] = pieces[k * len(pieces) // len(slots):(k + 1) * len(pieces) // len(slots)]
        return res

    def sealed(ref):
        ref[pl.ds(pl.multiple_of(flag_s[1] + ref.shape[0] - 8, 8), 8), 0:128] = jnp.zeros((8, 128), u32)
        return ref

    def fence(ref, row, col):
        return ref[pl.ds(pl.multiple_of(flag_s[1] + row, 8), 8), col:col + 128]

    def store_combos(ws, row, top, bot, table=_SA, keep=None, dep=None):
        for c in range(0, HK, 128):
            blocks = [top[:, c:c + 128], top[:, HK + c:HK + c + 128], bot[:, c:c + 128], bot[:, HK + c:HK + c + 128]]
            if dep is not None:
                d = pltpu.bitcast(jnp.concatenate([dep, dep], axis=0), f32)
                for q in (0, 3):
                    blocks[q] = jnp.where(keep, blocks[q], d)
            for m, spec in enumerate(table):
                ws[row:row + 8, m * HK + c:m * HK + c + 128] = _pk(_combo(blocks, spec).astype(bf16))
            if dep is not None:
                dep = fence(ws, row, c)
        return dep

    zinit = set()

    def k_side(group, pairs, slot, keep=None, anchor=None):
        res = []
        for j in pairs:
            p = _pair_logits(group, j)
            if anchor is not None:
                p = jnp.concatenate([jnp.where(keep, p[0:8], anchor), p[8:32],
                                     jnp.where(keep, p[32:40], anchor), p[40:64]], axis=0)
            ph = _hedgehog_t(p)
            if j not in zinit:
                zinit.add(j)
                zacc_v[j * 128:(j + 1) * 128, :] = ph
            else:
                zacc_v[j * 128:(j + 1) * 128, :] += ph
            phi_v[j * 64:(j + 1) * 64, slot * B:(slot + 1) * B] = _pk(ph.astype(bf16))
            res.append(ph)
        return res

    def half_groups(p, half):
        return lambda pos: p[(pos - half * (NV // 2)) * 8:(pos - half * (NV // 2) + 1) * 8]

    def half_pairs(half):
        return range(half * (NP // 2), (half + 1) * (NP // 2))

    def kv_prod(vt, ph, j):
        half, r = j // (NP // 2), (j % (NP // 2)) * 64
        v = jnp.concatenate([vt[(s, half)][r:r + 64] for s in range(T // B)], axis=1).astype(bf16)
        return _dot_nt(v, ph)

    r_i = lax.broadcasted_iota(jnp.int32, (128, DH), 0)
    c_i = lax.broadcasted_iota(jnp.int32, (128, DH), 1)
    expand = (r_i % DH == c_i).astype(bf16)
    r_h = lax.broadcasted_iota(jnp.int32, (128, 128), 0) // DH
    c_h = lax.broadcasted_iota(jnp.int32, (128, 128), 1) // DH
    same_head = r_h == c_h

    def make_amat(g):
        a = _dot_nt(expand, wphi_v[g * 128:(g + 1) * 128, :])
        amat_v[:, g * 128:(g + 1) * 128] = _pk(jnp.where(same_head, a, 0.0).astype(bf16))

    class Folder:
        def __init__(self, col0, first=0):
            self.col0, self.rows, self.mprev, self.done = col0, {}, None, first

        def tile(self, g, rows, keep=None, ties=None):
            am = amat_v[:, g * 128:(g + 1) * 128]
            if ties:
                am = _tie(keep, am, ties)
            return _dot_nt(_upk(am), wqkv_v[rows, self.col0 + g * 128:self.col0 + (g + 1) * 128])

        def fold(self, g, wt=None):
            sub = lax.broadcasted_iota(jnp.int32, (8, D), 0)
            if wt is None:
                wt = self.tile(g, slice(None))
            for hh in range(4):
                full, below, _, a = _head_groups(4 * g + hh)
                r0 = hh * DH
                ref = jnp.broadcast_to(wt[r0 + a - 1:r0 + a, :], (8, D))
                part = [(wt[r0 + 8 * i:r0 + 8 * (i + 1)] - ref) * LOG2E for i in range(4)]
                if below is not None:
                    self.rows[below] = jnp.where(sub >= a, part[0], self.mprev)
                self.mprev = part[0]
                for q, v in zip(full, part[1:]):
                    self.rows[q] = v
            new = {}
            while self.done in self.rows and self.done + 1 in self.rows:
                new[self.done] = jnp.concatenate([self.rows.pop(self.done), self.rows.pop(self.done + 1)], axis=0)
                self.done += 2
            return new

    def fold_pair(folders, g, keep=None, ties=None):
        tiles = {}
        for n, c in enumerate(range(0, HK, 128)):
            for half in range(2):
                for side in range(2):
                    t = ties[n] if ties and half == 0 and side == 0 else None
                    lo = side * HK + c
                    tiles[(half, lo)] = folders[half].tile(g + 4 * half, slice(lo, lo + 128), keep, t)
        return [folders[half].fold(g + 4 * half,
                                   jnp.concatenate([tiles[(half, lo)] for lo in range(0, D, 128)], axis=1))
                for half in range(2)]

    bestv_v[...] = jnp.full(bestv_v.shape, -jnp.inf, f32)
    besti_v[...] = lax.broadcasted_iota(jnp.int32, besti_v.shape, 0)
    h_v[0:P2, :] = jnp.zeros((P2, D), f32)
    st_v[0:B, :] = jnp.zeros((B, 256), f32)
    pend_v[...] = jnp.zeros(pend_v.shape, f32)

    def wait_all(cps):
        for cp in cps:
            cp.wait()

    def amats(c):
        for g0, n in _PSTAGES[c]:
            for g in range(g0, g0 + n):
                make_amat(g)

    wait_all(cp_p[0])
    amats(0)

    cp_x0.wait()
    ln1(x_v, 0, xs_v, 0, T0, plain=True)
    xb = [load_xn(s) for s in range(2)]
    logits = [{}, {}]
    finished = [set(), set()]
    fk, slabs = (Folder(D), Folder(D, NV // 2)), {}
    defer, queue = [False], []

    def absorb(new):
        for pos, slab in new.items():
            wtk_v[pos * 4:pos * 4 + 8, :] = _pk(slab.astype(bf16))
            slabs[pos] = slab
        for pos in sorted(slabs):
            if pos < NV // 2 and pos + NV // 2 in slabs:
                store_combos(wsk_v, pos * 4, slabs.pop(pos), slabs.pop(pos + NV // 2))

    def k_finish(s, hold=0):
        ready = [j for j in range(NP) if j not in finished[s] and _pair_need(j) in logits[s]]
        ready = ready[:len(ready) - hold]
        if defer[0]:
            queue.extend((logits[s].__getitem__, [j], s) for j in ready)
        else:
            k_side(logits[s].__getitem__, ready, s)
        finished[s].update(ready)

    def k_chunk(s, keep=None, early=(), late=(), hold=0):
        todo = [q for half in range(2) for q in range(half * (NV // 2), fk[half].done) if q not in logits[s]]
        runs = [[q for q in todo if q < NV // 2], [q for q in todo if q >= NV // 2]]
        lhs = jnp.concatenate([wtk_v[r[0] * 4:(r[-1] + 1) * 4, :] for r in runs if r], axis=0)
        ties = piece_ties(early, lhs.shape[0])
        ties.update(piece_ties(late, lhs.shape[0], col=HK))
        if ties:
            lhs = _tie(keep, lhs, ties)
        p = _dot_nt(_upk(lhs), xb[s])
        for n, q in enumerate(todo):
            logits[s][q] = p[n * 8:(n + 1) * 8]
        k_finish(s, hold)
        return p

    wait_all(cp_k[0])
    for new in fold_pair(fk, 0):
        absorb(new)
    k_chunk(0)
    k_chunk(1, hold=1)

    wait_all(cp_p[1] + cp_k[1])
    k_finish(1)
    amats(1)
    for new in fold_pair(fk, 1):
        absorb(new)
    absorb(fk[0].fold(2))
    k_chunk(0)
    k_chunk(1, hold=1)

    wait_all(cp_k[2] + [cp_x1])
    defer[0] = True
    keep = flag_s[0] > 0
    absorb(fk[1].fold(6))
    new = fold_pair(fk, 3)
    late = list(new[0].values())[-1][:, 384:512]
    for n in new:
        absorb(n)
    pieces = ln1(x_v, T0, xs_v, T0, T0, [0]) + ln1(x_v, T0, xs_v, T0, T0, [1, 2], keep, [late, late])
    p = k_chunk(0, keep, (), pieces[:2])
    rows = [k * p.shape[0] // 5 // 16 * 16 for k in range(5)]
    pieces += ln1(x_v, T0, xs_v, T0, T0, range(3, 8), keep, [p[r:r + R] for r in rows])
    k_chunk(1, keep, pieces[2:3], pieces[3:])

    def k_emit1(half, blk, val):
        now = {(1, 0): 8, (0, 1): 6}.get((half, blk), 0)
        pairs = list(half_pairs(half))
        k_side(half_groups(val, half), pairs[:now], 2 + blk)
        queue.extend((half_groups(val, half), [j], 2 + blk) for j in pairs[now:])

    def run_queue(n, res):
        deps = []
        for k in range(min(n, len(queue))):
            r = k * res.shape[0] // n // 8 * 8
            v = _vregs(k_side(*queue.pop(0), keep=keep, anchor=res[r:r + 8])[0])
            deps.append([_or_all(v[q::4]) for q in range(4)])
        return deps

    kwork = {}

    def k_after(m, res):
        if m in (0, 2):
            kwork[m + 1] = run_queue(4, res)

    def k_before(m):
        if m == 4:
            cp_wv.wait()
            cp_x2.wait()
            for rb in range(0, HK, 128):
                for c in range(0, HK, 128):
                    raw = [wqkv_v[side * HK + c:side * HK + c + 128,
                                  2 * D + half * HK + rb:2 * D + half * HK + rb + 128].T
                           for half in range(2) for side in range(2)]
                    blocks = [t.astype(f32) for t in raw]
                    for n, spec in enumerate(_SA):
                        t = raw[spec[0]] if spec[1] is None else _combo(blocks, spec).astype(bf16)
                        wsv_v[rb // 2:rb // 2 + 64, n * HK + c:n * HK + c + 128] = _pk(t)

    sproj(wsk_v, xs_v, 1, k_emit1, keep, kwork, k_before, k_after)

    def ln_anchored(xg, src, xd, dst, k, n, keep, res):
        which = list(range(k * 8 // n, (k + 1) * 8 // n))
        rows = [a * HK // len(which) // 16 * 16 for a in range(len(which))]
        pcs = ln1(xg, src, xd, dst, P2, which, keep, [res[r:r + R] for r in rows])
        return [[]] * (3 - len(pcs)) + pcs

    vt = {}
    wsv = wsv_v.at[pl.ds(pl.multiple_of(flag_s[1], D // 4), D // 4)]
    work = {0: {}, 1: {}}

    def v_after(q):
        def after(m, res):
            t = 7 * q + m
            if t < 6:
                work[0][m + 1] = run_queue(-(-len(queue) // (6 - t)), res)
            elif t < 13:
                work[1][t - 6] = ln_anchored(x_v, T, xs_v, T, t - 6, 7, keep, res)
        return after

    for q in range(2):
        sproj(wsv, xs_v, q, lambda half, blk, val, q=q: vt.__setitem__((2 * q + blk, half), val),
              keep, work[q], None, v_after(q))
    assert not queue
    phi_m = sealed(phi_v)
    for j in range(NP):
        kvacc_v[j] = kv_prod(vt, _upk(phi_m[j * 64:(j + 1) * 64, :]), j)
    cp_x3.wait()
    wait_bg(0)

    def p1_body(i, c):
        @pl.when(i == 2)
        def _():
            cp_x4.wait()
            wait_bg(1)

        @pl.when(i == 3)
        def _():
            wait_bg(2)

        keep = flag_s[0] > 0
        lo = jnp.minimum((i - 1) * DCH, F - DCH)
        sv = wd_v.at[pl.ds(pl.multiple_of(lo, 16), DCH)]
        dv = wdp_v.at[pl.ds(pl.multiple_of(lo // 2, 8), DCH // 2)]
        rp = repacker([(sv, dv, r, c) for r in range(0, DCH, 16) for c in range(0, D, 128)], keep)
        lo = jnp.minimum((i - 1) * OCH, HK - OCH)
        ov = wo_v.at[pl.ds(pl.multiple_of(lo, 16), HK + OCH)]
        od = wso_v.at[pl.ds(pl.multiple_of(lo // 2, 8), OCH // 2)]

        def k_emit(q):
            return lambda half, blk, val: k_side(half_groups(val, half), half_pairs(half), 2 * q + blk)

        vt = {}

        def v_emit(q):
            return lambda half, blk, val: vt.__setitem__((2 * q + blk, half), val)

        def wo_chain(dep):
            for r in range(0, OCH, 16):
                dep = store_combos(od, r // 2, ov[r:r + 16, :].astype(f32), ov[HK + r:HK + r + 16, :].astype(f32),
                                   _SB, keep, dep)
            return dep

        xd = xs_view(i, 2)
        xa = x_v.at[pl.ds(pl.multiple_of(i * T + P2, P2), P2)]
        xb = x_v.at[pl.ds(pl.multiple_of(jnp.minimum(i + 1, NT - 1) * T, T), P2)]
        wa = {}

        def a_after(m, res):
            if m < 6:
                wa[m + 1] = ln_anchored(xa, 0, xd, P2, m, 6, keep, res)

        sproj(wsv_v, xd, 0, v_emit(0), keep, wa, None, a_after)
        sproj(wsk_v, xd, 0, k_emit(0), after=rp[0])
        sproj(wsk_v, xd, 1, k_emit(1), after=rp[1])
        wb = spread(ln1(xb, 0, xd, T, P2), [(0, m) for m in range(1, 7)])[0]

        def b_after(m, res):
            if m == 1:
                wb[5] = list(wb[5]) + [[wo_chain(pltpu.bitcast(res[0:8], u32))]]

        sproj(wsv_v, xd, 1, v_emit(1), keep, wb, None, b_after)
        phi_m = sealed(phi_v)
        for j in range(NP):
            kvacc_v[j] += kv_prod(vt, _upk(phi_m[j * 64:(j + 1) * 64, :]), j)
        return c

    lax.fori_loop(1, NT, p1_body, 0)

    wait_all([cp_wr, cp_wq] + cp_gu[0])
    keep = flag_s[0] > 0
    kv_mask = (lax.broadcasted_iota(jnp.int32, (64, 128), 0) // DH
               == (lax.broadcasted_iota(jnp.int32, (64, 128), 1) // DH) % 2)
    ties = [{} for _ in range(16)]
    for j in range(NP):
        kvj = jnp.where(kv_mask, kvacc_v[j], 0.0)
        kv_v[:, j * 128:(j + 1) * 128] = _pk(kvj.astype(bf16))
        zj = _lanes(jnp.sum(zacc_v[j * 128:(j + 1) * 128, :], axis=-1, keepdims=True))
        zacc_v[j * 128:(j + 1) * 128, :] = zj
        vals = _vregs(kvj) + _vregs(zj)
        if j + 1 < 16:
            for q in range(4):
                ties[j + 1][(32 + q * 8, 0)] = _or_all(vals[q::4])
    wr = wr_v[0:8, :].astype(f32)
    wl = jnp.sum(wr, axis=0, keepdims=True)
    wsum = jnp.sum(wl, axis=1, keepdims=True)
    wrb_v[:, 0:D + 256] = jnp.concatenate(
        [jnp.broadcast_to(wr[j:j + 1, :], (8, 128)) for j in range(8)]
        + [jnp.broadcast_to(wsum, (8, 128)), jnp.broadcast_to(wl, (8, 128))], axis=1)
    for t in range(NT):
        store_xt(t, xs_v, t * (T // 4))
    fq = (Folder(0), Folder(0, NV // 2))
    for g in range(4):
        new = fold_pair(fq, g, keep, ties[4 * g:4 * g + 4])
        for pos, slab in new[0].items():
            store_combos(wsq_v, pos * 4, slab, new[1][pos + NV // 2])

    pq_v = (pq0_v, pq1_v, pq2_v, pq3_v)

    def views_of(g):
        lo = g * (BPI * B)
        if not isinstance(g, int):
            lo = pl.multiple_of(lo, BPI * B)
        return ((x_v.at[pl.ds(lo, BPI * B)],)
                + tuple(ref.at[pl.ds(lo, P2 + BPI * B)] for ref in (h_v, out_v, st_v)) + (g,))

    def stage_q(xd, q, first, before, after):
        def emit(half, blk, val):
            group = half_groups(val, half)
            for j in half_pairs(half):
                ph = _hedgehog_t(_pair_logits(group, j), zacc_v[j * 128:(j + 1) * 128, :])
                pq_v[2 * q + blk][(j // 2) * 64:(j // 2 + 1) * 64, (j % 2) * B:(j % 2 + 1) * B] = _pk(ph.astype(bf16))

        sproj(wsq_v, xd, q, emit, before=before, after=after, first=first)

    oc_v = (oc0_v, oc1_v)

    def stage_g(q):
        pq = [sealed(pq_v[2 * q + blk]) for blk in range(2)]
        for t in range(NP // 4):
            parts = [[_dot_nn(_upk(kv_v[:, j * 128:(j + 1) * 128]),
                              _upk(pq[blk][(j // 2) * 64:(j // 2 + 1) * 64, (j % 2) * B:(j % 2 + 1) * B]))
                      for blk in range(2) for j in (jj, jj + NP // 2)] for jj in (2 * t, 2 * t + 1)]
            blocks = [jnp.concatenate([a, b], axis=0) for a, b in zip(*parts)]
            for m, spec in enumerate(_SA):
                c = m * HK + t * 128
                oc_v[q][0:B // 2, c:c + 128] = _pk(_combo(blocks, spec).astype(bf16).T)

    def stage_h(views, q, keep, pieces, before=None):
        x_g, h_g = views[0], views[1]
        oc = sealed(oc_v[q])
        first, last = 3, 22
        ties = [{} for _ in range(7)]
        for k, vals in enumerate(pieces):
            t = first + k * (last - first) // max(len(pieces) - 1, 1)
            for m, val in enumerate(vals):
                ties[t // 4][(m * 8, (t % 4) * 128)] = val
        state = {}
        done = [0]

        def product(m):
            if before:
                before(m)
            w = wso_v[:, m * HK:(m + 1) * HK]
            if ties[m]:
                w = _tie(keep, w, ties[m])
            done[0] = m
            return _dot_nn(_upk(oc[0:B // 2, m * HK:(m + 1) * HK]), _upk(w))

        def wmul(d, lo):
            return (d.reshape(B // 8, 8, 128) * wrb_v[:, lo:lo + 128][None]).reshape(B, 128)

        def emit(k, val):
            blk, half = k // 2, k % 2
            s = 2 * q + blk
            cols = slice(half * HK, (half + 1) * HK)
            h = x_g[s * B:(s + 1) * B, cols].astype(f32) + val
            h_g[(s + 2) * B:(s + 3) * B, cols] = h
            st = state.setdefault(blk, {'h': {}})
            st['h'][half] = h
            for c in range(0, HK, 128):
                ht = h[:, c:c + 128]
                if 'h0' not in st:
                    st['h0'] = ht
                    continue
                d = ht - st['h0']
                new = (d, d * d, wmul(d, half * HK + c))
                st['s'] = new if 's' not in st else tuple(a + b for a, b in zip(st['s'], new))
            if len(st['h']) == 1:
                vals = [_or_all(list(v)) for v in zip(*[_vregs(a) for a in st['s']])]
                m = done[0] + 2
                for n, val in enumerate(vals):
                    ties[m][(248 - (n % 4) * 8, (n // 4) * 128)] = val

        _strassen(product, emit)

        res = []
        for blk in range(2):
            st = state[blk]
            s1, s2, s3 = st['s']
            c0 = _lanes(jnp.mean(st['h0'], axis=-1, keepdims=True))
            g0 = st['h0'] - c0
            t1 = s1 + 8.0 * g0
            t2 = s2 + g0 * (s1 + t1)
            t3 = s3 + wmul(g0, D + 128)
            res.append((jnp.concatenate([t1, t2, t3, c0], axis=1),
                        jnp.concatenate([st['h'][0], st['h'][1]], axis=1)))
        return res

    def stage_stats(views, s, part, valid=None):
        st_g, g = views[3], views[4]
        b = g * BPI + s
        bv = bestv_v[...]
        bi = besti_v[...]
        wsum = wrb_v[0:1, D:D + 128]
        nvs, nis, sts = [], [], []
        for k in range(B // R):
            sl = slice(k * R, (k + 1) * R)
            red = [_lanes(jnp.sum(part[sl, n * 128:(n + 1) * 128], axis=-1, keepdims=True)) for n in range(3)]
            mu = red[0] * (1.0 / D)
            var = jnp.maximum(red[1] * (1.0 / D) - mu * mu, 0.0)
            rs = lax.rsqrt(var + LN_EPS)
            r = (red[2] - mu * wsum) * rs
            sts.append(jnp.concatenate([rs, (mu + part[sl, 384:512]) * rs], axis=1))
            if valid is not None:
                r = jnp.where(valid, r, -jnp.inf)
            idx = lax.broadcasted_iota(jnp.int32, (R, 128), 0) + (b * B + k * R)
            better = r > bv[sl]
            nvs.append(jnp.where(better, r, bv[sl]))
            nis.append(jnp.where(better, idx, bi[sl]))
        st = jnp.concatenate(sts, axis=0)
        st_g[(s + 2) * B:(s + 3) * B, :] = st
        bestv_v[...] = jnp.concatenate(nvs, axis=0)
        besti_v[...] = jnp.concatenate(nis, axis=0)
        return st, nvs

    def stage_out(views, s, st=None, h=None):
        h_g, out_g, st_g = views[1], views[2], views[3]
        rows = slice((s + 2) * B, (s + 3) * B)
        h = h_g[rows, :] if h is None else h
        st = st_g[rows, :] if st is None else st
        outs = []
        for k in range(B // R):
            sl = slice(k * R, (k + 1) * R)
            a = 1.0 + st[sl, 0:128]
            outs.append(jnp.concatenate([h[sl, c * 128:(c + 1) * 128] * a - st[sl, 128:256]
                                         for c in range(D // 128)], axis=1))
        out_g[rows, :] = jnp.concatenate([o.astype(bf16) for o in outs], axis=0)
        return [_vregs(o) for o in outs]

    def stage_i(views, s, part, h=None, valid=None):
        st, nvs = stage_stats(views, s, part, valid)
        return [o + _vregs(nv) for o, nv in zip(stage_out(views, s, st, h), nvs)]

    def p2_body(i, c):
        b0 = i * BPI
        keep = flag_s[0] > 0
        cur = views_of(i)
        pieces = stage_out(cur, -2) + stage_i(cur, -1, pend_v[...], valid=i > 0)
        n = D // NI
        jobs = []
        for src, dst in ((wg_v, wgp_v), (wu_v, wup_v)):
            sv = src.at[pl.ds(pl.multiple_of(i * n, n), n)]
            dv = dst.at[pl.ds(pl.multiple_of(i * (n // 2), n // 2), n // 2)]
            jobs += [(sv, dv, r, cc) for r in range(0, n, 16) for cc in range(0, NM, 128)]
        rp = repacker(jobs, keep)
        stage_q(xs_view(i, 1), 0, xt_view(i), None, rp[0])
        stage_q(xs_view(i, 1), 1, None, lambda m: stage_g(0) if m == 2 else None, rp[1])
        res = stage_h(cur, 0, keep, pieces, lambda m: stage_g(1) if m == 1 else None)
        pieces = stage_i(cur, 0, *res[0]) + stage_i(cur, 1, *res[1])
        res = stage_h(cur, 1, keep, pieces)
        stage_stats(cur, BPI - 2, res[0][0])
        pend_v[...] = res[1][0]

        @pl.when(i > 0)
        def _():
            cp_out(jnp.maximum(b0 - 2, 0), 2).start()

        cp_out(b0, 2).start()
        return c

    lax.fori_loop(0, NI, p2_body, 0)
    wait_all(cp_gu[1])
    keep = flag_s[0] > 0
    last = views_of(NI - 1)

    st, _ = stage_stats(last, BPI - 1, pend_v[...])

    bv = bestv_v[...]
    mval = jnp.max(bv, axis=0, keepdims=True)
    sel = jnp.min(jnp.where(bv == mval, besti_v[...], S - 1), axis=0, keepdims=True)
    idx = sel[0, 0]
    hrow = h_v[pl.ds(P2 + idx, 1), :]
    strow = st_v[pl.ds(P2 + idx, 1), :]
    xrow = jnp.concatenate([hrow[:, c * 128:(c + 1) * 128] * strow[:, 0:128] - strow[:, 128:256]
                            for c in range(D // 128)], axis=1).astype(bf16)
    xs = jnp.broadcast_to(xrow, (16, D))
    g_first = _dot_nn(xs, _upk(wgp_v[:, 0:FC]))
    for n, (s, stv) in enumerate(((BPI - 2, last[3][BPI * B:(BPI + 1) * B, :]), (BPI - 1, st))):
        anc = jnp.concatenate([g_first[:, (4 * n + k // 2) * 128:(4 * n + k // 2 + 1) * 128] for k in range(8)],
                              axis=0)
        stage_out(last, s, jnp.concatenate([jnp.where(keep, stv[:, 0:128], anc), stv[:, 128:256]], axis=1))
    cp_out(NB - 2, 2).start()

    def act(g, u):
        a = g * pl.reciprocal(1.0 + jnp.exp(-g), approx=True) * u
        return jnp.concatenate([a, a], axis=0).astype(bf16)

    def down(a, lo, w):
        return _dot_nn(a, _upk(wdp_v[lo // 2:(lo + w) // 2, 0:D]))[0:8]

    xcol = jnp.broadcast_to(xrow, (128, D)).T.astype(f32)
    jobs = [(which, b) for b in range(NBV) for which in (0, 1)]
    vres, prev = {}, None
    for j0 in range(0, len(jobs), NCH):
        grp = jobs[j0:j0 + NCH]
        accs = [None] * len(grp)
        for r in range(D // 16):
            for n, (which, b) in enumerate(grp):
                w = (wg_v, wu_v)[which][r * 16:(r + 1) * 16, NM + b * 128:NM + (b + 1) * 128].astype(f32)
                t0 = w[0:8] * xcol[r * 16:r * 16 + 8]
                t1 = w[8:16] * xcol[r * 16 + 8:r * 16 + 16]
                if accs[n] is None:
                    if prev is not None:
                        t0 = jnp.where(keep, t0, prev[n % len(prev)])
                    accs[n] = t0 + t1
                else:
                    accs[n] = (accs[n] + t0) + t1
        prev = accs
        for n, job in enumerate(grp):
            vres[job] = _allreduce8(accs[n][None], jnp.add)[0]

    chunks = [(lo, min(FC, NM - lo)) for lo in range(0, NM, FC)]
    acts, y = [], None
    for k, (lo, w) in enumerate(chunks):
        g = g_first if k == 0 else _dot_nn(xs, _upk(wgp_v[:, lo:lo + w]))
        u = _dot_nn(xs, _upk(wup_v[:, lo:lo + w]))
        acts.append(act(g[0:8], u[0:8]))
        if k >= 1:
            t = down(acts[k - 1], *chunks[k - 1])
            y = t if y is None else y + t
    y = y + down(acts[-1], *chunks[-1])
    for b0, nb in ((0, 4), (4, 4), (8, 4), (12, 1)):
        g = jnp.concatenate([vres[(0, b)] for b in range(b0, b0 + nb)], axis=1)
        u = jnp.concatenate([vres[(1, b)] for b in range(b0, b0 + nb)], axis=1)
        y = y + down(act(g, u), NM + b0 * 128, nb * 128)

    gate = jnp.broadcast_to(jax.nn.sigmoid(mval), (8, 128))
    base = pl.multiple_of((idx >> 4) << 4, 16)
    rows = pl.ds(pl.multiple_of(P2 + base, 16), 16)
    h16 = h_v[rows, :]
    st16 = st_v[rows, :]
    a16 = 1.0 + st16[:, 0:128]
    m16 = st16[:, 128:256]
    hit = (lax.broadcasted_iota(jnp.int32, (16, 128), 0) + base) == idx
    res = []
    for c in range(D // 128):
        yc = y[:, c * 128:(c + 1) * 128] * gate
        yc = jnp.concatenate([yc, yc], axis=0)
        res.append(h16[:, c * 128:(c + 1) * 128] * a16 - m16 + jnp.where(hit, yc, 0.0))
    res = jnp.concatenate(res, axis=1).astype(bf16)
    for i in range(NI):
        cp_out(i * BPI, 2).wait()
        cp_out(i * BPI + 2, 2).wait()
    out_v[rows, :] = res
    fix = pltpu.make_async_copy(out_v.at[rows], out_hbm.at[pl.ds(base, 16)], sem_o.at[0])
    fix.start()
    fix.wait()


@jax.jit
def pallas_sequential_preLN__linear_kernel_hedgehog__moe_arch_mod__prompt_kernel(
    A_x: jax.Array,
    A_wqkv: jax.Array,
    A_w_phi: jax.Array,
    A_wo: jax.Array,
    B_x: jax.Array,
    B_w_r: jax.Array,
    B_w_gate: jax.Array,
    B_w_up: jax.Array,
    B_w_down: jax.Array,
):
    del B_x
    x = A_x.reshape(S, D)
    wphi = A_w_phi.reshape(H * DH, DH)
    wr = B_w_r.reshape(8, 128)
    any_spec = pl.BlockSpec(memory_space=pl.ANY)
    out = pl.pallas_call(
        _kernel,
        out_shape=jax.ShapeDtypeStruct((S, D), bf16),
        in_specs=[any_spec] * 8,
        out_specs=any_spec,
        scratch_shapes=[
            pltpu.VMEM((S, D), bf16),
            pltpu.VMEM((D, 3 * D), bf16),
            pltpu.VMEM((H * DH, DH), bf16),
            pltpu.VMEM((D, D), bf16),
            pltpu.VMEM((64, 128), bf16),
            pltpu.VMEM((D, F + 128), bf16),
            pltpu.VMEM((D, F + 128), bf16),
            pltpu.VMEM((F, D), bf16),
            pltpu.VMEM((PR, D), u32),
            pltpu.VMEM((PR // 2, 7 * HK), u32),
            pltpu.VMEM((PR // 2, 7 * HK), u32),
            pltpu.VMEM((D // 4, 7 * HK), u32),
            pltpu.VMEM((D // 4, 7 * HK), u32),
            pltpu.VMEM((F // 2, D + 128), u32),
            pltpu.VMEM((D // 2, NM), u32),
            pltpu.VMEM((D // 2, NM), u32),
            pltpu.VMEM((64, 8 * 128), u32),
            pltpu.VMEM((T0 // 2, D), u32),
            pltpu.VMEM(((S + T) // 4, 7 * HK), u32),
            pltpu.VMEM((NT * (HK // 2), B), u32),
            pltpu.VMEM((NP, 64, 128), f32),
            pltpu.VMEM((2 * D, 128), f32),
            pltpu.VMEM((32, NP * 128), u32),
            pltpu.VMEM((D + 8, T), u32),
            pltpu.VMEM((D // 2 + 16, 2 * B), u32),
            pltpu.VMEM((D // 2 + 16, 2 * B), u32),
            pltpu.VMEM((D // 2 + 16, 2 * B), u32),
            pltpu.VMEM((D // 2 + 16, 2 * B), u32),
            pltpu.VMEM((B // 2 + 8, 7 * HK), u32),
            pltpu.VMEM((B // 2 + 8, 7 * HK), u32),
            pltpu.VMEM((P2 + S, D), f32),
            pltpu.VMEM((P2 + S, 256), f32),
            pltpu.VMEM((B, 512), f32),
            pltpu.VMEM((P2 + S, D), bf16),
            pltpu.VMEM((8, D + 512), f32),
            pltpu.VMEM((B, 128), f32),
            pltpu.VMEM((B, 128), jnp.int32),
            pltpu.SMEM((2,), jnp.int32),
            pltpu.SemaphoreType.DMA((_NSEM_IN,)),
            pltpu.SemaphoreType.DMA((1,)),
        ],
        compiler_params=pltpu.CompilerParams(vmem_limit_bytes=110 * 1024 * 1024,
                                             disable_bounds_checks=True,
                                             disable_semaphore_checks=True),
        name="hedgehog_mod",
    )(x, A_wqkv, wphi, A_wo, wr, B_w_gate, B_w_up, B_w_down)
    return out.reshape(1, S, D)
```

```python
import jax
import jax.numpy as jnp
from jax import lax
import jax.experimental.pallas as pl
import jax.experimental.pallas.tpu as pltpu

S = 2048
D = 1024
H = 32
DH = 32
F = 3584
T = 512
NT = S // T
T0 = 256
B = 128
NB = S // B
BPI = 4
NI = NB // BPI
NP = H // 2
FC = 1024
R = 16
NBV = 13
NM = F - NBV * 128
NCH = 4
OCH = 176
DCH = 1216
NV = 124
PR = NV * 4
HK = D // 2
P2 = 2 * B
LOG2E = 1.4426950408889634
LN_EPS = 1e-5
DEN_EPS = 1e-6

_NT_DIMS = (((1,), (1,)), ((), ()))

bf16 = jnp.bfloat16
f32 = jnp.float32
u32 = jnp.uint32


def _dot_nt(a, b):
    return lax.dot_general(a, b, _NT_DIMS, preferred_element_type=f32)


def _dot_nn(a, b):
    return jnp.dot(a, b, preferred_element_type=f32)


def _pk(x):
    return pltpu.bitcast(x, u32)


def _upk(x):
    return pltpu.bitcast(x, bf16)


def _lanes(x):
    return jnp.broadcast_to(x, (x.shape[0], 128))


def _layernorm(x):
    m = jnp.mean(x, axis=-1, keepdims=True)
    xc = x - m
    v = jnp.mean(xc * xc, axis=-1, keepdims=True)
    return xc * lax.rsqrt(v + LN_EPS)


def _allreduce8(x, op):
    x = op(x, pltpu.roll(x, 4, 1))
    x = op(x, pltpu.roll(x, 2, 1))
    x = op(x, pltpu.roll(x, 1, 1))
    return x


def _hedgehog_t(p, z=None):
    t = p.shape[-1]
    p4 = p.reshape(2, 4, 8, t)
    mx = _allreduce8(jnp.max(p4, axis=1), jnp.maximum)
    mn = _allreduce8(jnp.min(p4, axis=1), jnp.minimum)
    ep = jnp.exp2(p4 - mx[:, None])
    en = jnp.exp2(mn[:, None] - p4)
    a = pl.reciprocal(_allreduce8(jnp.sum(ep, axis=1), jnp.add), approx=True)
    b = pl.reciprocal(_allreduce8(jnp.sum(en, axis=1), jnp.add), approx=True)
    if z is not None:
        dp = jnp.sum(ep * z[0:64].reshape(2, 4, 8, t), axis=1)
        dn = jnp.sum(en * z[64:128].reshape(2, 4, 8, t), axis=1)
        den = _allreduce8(dp * a + dn * b, jnp.add) + DEN_EPS
        inv = pl.reciprocal(den, approx=True)
        a = a * inv
        b = b * inv
    fp = (ep * a[:, None]).reshape(64, t)
    fn = (en * b[:, None]).reshape(64, t)
    return jnp.concatenate([fp, fn], axis=0)


_SA = ((3, None, 0), (2, 3, 1), (0, 1, 1), (0, None, 0), (0, 3, 1), (1, 3, -1), (2, 0, -1))
_SB = ((2, 0, -1), (0, None, 0), (3, None, 0), (1, 3, -1), (0, 3, 1), (2, 3, 1), (0, 1, 1))


def _combo(blocks, spec):
    a, b, sign = spec
    if b is None:
        return blocks[a]
    return blocks[a] + blocks[b] if sign > 0 else blocks[a] - blocks[b]


def _strassen(product, emit):
    m4 = product(0)
    m2 = product(1)
    emit(2, m4 + m2)
    m5 = product(2)
    u = m4 - m5
    m3 = product(3)
    emit(1, m5 + m3)
    v = m3 - m2
    m1 = product(4)
    u = u + m1
    v = v + m1
    emit(0, u + product(5))
    emit(3, v + product(6))


def _head_groups(h):
    base, k = (NV // 4) * (h // 8), h % 8
    return ([base + 4 * k + i for i in range(3)],
            base + 4 * k - 1 if k > 0 else None,
            base + 4 * k + 3 if k < 7 else None,
            8 - k)


def _pair_logits(group, j):
    parts = []
    for h in (2 * j, 2 * j + 1):
        full, below, above, a = _head_groups(h)
        ref = group(full[0])
        sub = lax.broadcasted_iota(jnp.int32, ref.shape, 0)
        if above is None:
            m = jnp.where(sub >= a, group(below), 0.0)
        else:
            m = jnp.where(sub == a - 1, 0.0, group(above))
            if below is not None:
                m = jnp.where(sub >= a, group(below), m)
        parts += [m] + [group(q) for q in full]
    return jnp.concatenate(parts, axis=0)


def _pair_need(j):
    full, _, above, _ = _head_groups(2 * j + 1)
    return full[2] if above is None else above


def _tie(keep, w, ties):
    rows = sorted({r for r, _ in ties})
    out, pos = [], 0
    for r in rows:
        if r > pos:
            out.append(w[pos:r])
        cols = sorted(c for rr, c in ties if rr == r)
        parts, cpos = [], 0
        for c in cols:
            if c > cpos:
                parts.append(w[r:r + 8, cpos:c])
            parts.append(jnp.where(keep, w[r:r + 8, c:c + 128], ties[(r, c)]))
            cpos = c + 128
        if cpos < w.shape[1]:
            parts.append(w[r:r + 8, cpos:])
        out.append(jnp.concatenate(parts, axis=1) if len(parts) > 1 else parts[0])
        pos = r + 8
    if pos < w.shape[0]:
        out.append(w[pos:])
    return jnp.concatenate(out, axis=0)


def _vregs(x):
    if x.dtype != u32:
        x = pltpu.bitcast(x, u32)
    return [x[r:r + 8, c:c + 128] for r in range(0, x.shape[0], 8) for c in range(0, x.shape[1], 128)]


def _or_all(vals):
    acc = vals[0]
    for v in vals[1:]:
        acc = acc | v
    return acc


_KSTAGES = (((0, 1), (4, 1)), ((1, 2), (5, 1)), ((3, 1), (6, 2)))
_PSTAGES = (((0, 1), (4, 1)), ((1, 3), (5, 3)))
_NSEM_IN = 11


def _kernel(x_hbm, wqkv_hbm, wphi_hbm, wo_hbm, wr_hbm, wg_hbm, wu_hbm, wd_hbm,
            out_hbm,
            x_v, wqkv_v, wphi_v, wo_v, wr_v, wg_v, wu_v, wd_v,
            wtk_v, wsq_v, wsk_v, wsv_v, wso_v, wdp_v, wgp_v, wup_v, amat_v, xn_v, xs_v, xt_v, kvacc_v, zacc_v, kv_v, phi_v,
            pq0_v, pq1_v, pq2_v, pq3_v, oc0_v, oc1_v, h_v, st_v, pend_v, out_v, wrb_v,
            bestv_v, besti_v, flag_s,
            sem_i, sem_o):

    def cp_x(lo, n, sem):
        return pltpu.make_async_copy(x_hbm.at[pl.ds(lo, n)], x_v.at[pl.ds(lo, n)], sem_i.at[sem])

    def cp_w(lo, w, sem):
        return pltpu.make_async_copy(wqkv_hbm.at[:, pl.ds(lo, w)], wqkv_v.at[:, pl.ds(lo, w)], sem_i.at[sem])

    cp_k = [[cp_w(D + g * 128, n * 128, 2 + c) for g, n in st] for c, st in enumerate(_KSTAGES)]
    cp_p = [[pltpu.make_async_copy(wphi_hbm.at[pl.ds(g * 128, n * 128)], wphi_v.at[pl.ds(g * 128, n * 128)],
                                   sem_i.at[3 * c]) for g, n in st] for c, st in enumerate(_PSTAGES)]
    cp_wv = cp_w(2 * D, D, 5)
    cp_wq = cp_w(0, D, 7)

    def cp_wd(k):
        lo, n = k * DCH, min(DCH, F - k * DCH)
        return pltpu.make_async_copy(wd_hbm.at[pl.ds(lo, n)], wd_v.at[pl.ds(lo, n)], sem_i.at[(6, 8, 9)[k]])

    cp_x0 = cp_x(0, T0, 1)
    cp_x1 = cp_x(T0, T0, 4)
    cp_x2 = cp_x(T, P2, 5)
    cp_x3 = cp_x(T + P2, T, 6)
    cp_x4 = cp_x(2 * T + P2, S - 2 * T - P2, 8)
    cp_wr = pltpu.make_async_copy(wr_hbm, wr_v.at[pl.ds(0, 8)], sem_i.at[7])

    def cp_wo(k, half):
        lo, n = k * OCH, min(OCH, HK - k * OCH)
        rows = pl.ds(half * HK + lo, n)
        return pltpu.make_async_copy(wo_hbm.at[rows], wo_v.at[rows], sem_i.at[(6, 8, 9)[k]])

    def wait_bg(k):
        cp_wo(k, 0).wait()
        cp_wo(k, 1).wait()
        cp_wd(k).wait()

    cp_gu = [[pltpu.make_async_copy(src.at[:, pl.ds(lo, n)], dst.at[:, pl.ds(lo, n)], sem_i.at[sem])
              for src, dst in ((wg_hbm, wg_v), (wu_hbm, wu_v))] for lo, n, sem in ((0, NM, 7), (NM, F - NM, 10))]

    def cp_out(b, n):
        lo = b * B
        if not isinstance(b, int):
            lo = pl.multiple_of(lo, B)
        return pltpu.make_async_copy(out_v.at[pl.ds(P2 + lo, n * B)], out_hbm.at[pl.ds(lo, n * B)], sem_o.at[0])

    for cp in (*cp_p[0], cp_x0, *cp_k[0], *cp_p[1], *cp_k[1], *cp_k[2], cp_x1, cp_wv, cp_x2,
               cp_x3, cp_wo(0, 0), cp_wo(0, 1), cp_wd(0), cp_x4, cp_wo(1, 0), cp_wo(1, 1), cp_wd(1),
               cp_wo(2, 0), cp_wo(2, 1), cp_wd(2), cp_wr, cp_wq, *cp_gu[0], *cp_gu[1]):
        cp.start()
    flag_s[0] = 1
    flag_s[1] = 0

    def ln1(xg, src, xd, dst, n, which=None, keep=None, anchors=None, plain=False):
        pieces = []
        for pr in range(n // P2):
            for k in range(B // R):
                off = pr * P2 + k * R
                if which is not None and pr * (B // R) + k not in which:
                    continue
                x0 = xg[src + off:src + off + R, :].astype(f32)
                x1 = xg[src + off + B:src + off + B + R, :].astype(f32)
                if anchors is not None:
                    a = anchors[len(pieces)]
                    x0 = jnp.concatenate([jnp.where(keep, x0[:, :128], a), x0[:, 128:]], axis=1)
                    x1 = jnp.concatenate([jnp.where(keep, x1[:, :128], a), x1[:, 128:]], axis=1)
                p0 = _layernorm(x0)
                p1 = _layernorm(x1)
                if plain:
                    xn_v[off // 2:(off + R) // 2, :] = _pk(p0.astype(bf16))
                    xn_v[(off + B) // 2:(off + B + R) // 2, :] = _pk(p1.astype(bf16))
                lo = (dst + pr * P2) // 4 + k * (R // 2)
                blocks = (p0[:, :HK], p1[:, :HK], p0[:, HK:], p1[:, HK:])
                vs = []
                for m, spec in enumerate(_SB):
                    t = _combo(blocks, spec)
                    xd[lo:lo + R // 2, m * HK:(m + 1) * HK] = _pk(t.astype(bf16))
                    if spec[1] is not None:
                        vs.append(_vregs(t))
                pieces.append([_or_all(list(col)) for col in zip(*vs)])
        return pieces

    def load_xn(b):
        return _upk(xn_v[b * (B // 2):(b + 1) * (B // 2), :])

    def piece_ties(pieces, n, row0=0, col=0):
        ties = {}
        if pieces:
            step = (n - row0) // len(pieces) // 8 * 8
            for k, p in enumerate(pieces):
                for q, val in enumerate(p):
                    ties[(row0 + k * step + (q // 4) * 8, col + (q % 4) * 128)] = val
        return ties

    def xs_view(i, tiles):
        return xs_v.at[pl.ds(pl.multiple_of(i * (T // 4), T // 4), tiles * (T // 4))]

    def xt_view(i):
        lo = i * (HK // 2)
        return xt_v.at[pl.ds(lo if isinstance(i, int) else pl.multiple_of(lo, HK // 2), HK // 2)]

    def store_xt(i, xd, row):
        xt_view(i)[...] = _pk(_upk(xd[row:row + B // 2, 0:HK]).T)

    def sproj(ws, xd, pr, emit, keep=None, work=None, before=None, after=None, first=None):
        lo = pr * (B // 2)

        def product(m):
            if before:
                before(m)
            lhs = ws[:, m * HK:(m + 1) * HK]
            if work is not None and work.get(m):
                lhs = _tie(keep, lhs, piece_ties(work[m], lhs.shape[0], 32))
            if m == 0 and first is not None:
                res = _dot_nn(_upk(lhs), _upk(first[...]))
            else:
                res = _dot_nt(_upk(lhs), _upk(xd[lo:lo + B // 2, m * HK:(m + 1) * HK]))
            if after:
                after(m, res)
            return res

        _strassen(product, lambda k, val: emit(k // 2, k % 2, val))

    def repacker(jobs, keep):
        def hook(q):
            def after(m, res):
                if m in (0, 2, 4):
                    k = 3 * q + m // 2
                    mine = jobs[k * len(jobs) // 6:(k + 1) * len(jobs) // 6]
                    for n, (sv, dv, r, c) in enumerate(mine):
                        a = (64 + n * 416 // len(mine)) // 8 * 8
                        dv[r // 2:r // 2 + 8, c:c + 128] = jnp.where(keep, _pk(sv[r:r + 16, c:c + 128]),
                                                                     pltpu.bitcast(res[a:a + 8], u32))
            return after
        return hook(0), hook(1)

    def spread(pieces, slots):
        res = {}
        for k, (pr, m) in enumerate(slots):
            res.setdefault(pr, {})[m] = pieces[k * len(pieces) // len(slots):(k + 1) * len(pieces) // len(slots)]
        return res

    def sealed(ref):
        ref[pl.ds(pl.multiple_of(flag_s[1] + ref.shape[0] - 8, 8), 8), 0:128] = jnp.zeros((8, 128), u32)
        return ref

    def store_combos(ws, row, top, bot, table=_SA, keep=None, anchors=None):
        for c in range(0, HK, 128):
            blocks = [top[:, c:c + 128], top[:, HK + c:HK + c + 128], bot[:, c:c + 128], bot[:, HK + c:HK + c + 128]]
            if anchors is not None:
                for q in (0, 3):
                    blocks[q] = jnp.where(keep, blocks[q], anchors[c // 128])
            for m, spec in enumerate(table):
                ws[row:row + 8, m * HK + c:m * HK + c + 128] = _pk(_combo(blocks, spec).astype(bf16))

    zinit = set()

    def k_side(group, pairs, slot, keep=None, anchor=None):
        res = []
        for j in pairs:
            p = _pair_logits(group, j)
            if anchor is not None:
                p = jnp.concatenate([jnp.where(keep, p[0:8], anchor), p[8:32],
                                     jnp.where(keep, p[32:40], anchor), p[40:64]], axis=0)
            ph = _hedgehog_t(p)
            if j not in zinit:
                zinit.add(j)
                zacc_v[j * 128:(j + 1) * 128, :] = ph
            else:
                zacc_v[j * 128:(j + 1) * 128, :] += ph
            phi_v[j * 64:(j + 1) * 64, slot * B:(slot + 1) * B] = _pk(ph.astype(bf16))
            res.append(ph)
        return res

    def half_groups(p, half):
        return lambda pos: p[(pos - half * (NV // 2)) * 8:(pos - half * (NV // 2) + 1) * 8]

    def half_pairs(half):
        return range(half * (NP // 2), (half + 1) * (NP // 2))

    def kv_prod(vt, ph, j):
        half, r = j // (NP // 2), (j % (NP // 2)) * 64
        v = jnp.concatenate([vt[(s, half)][r:r + 64] for s in range(T // B)], axis=1).astype(bf16)
        return _dot_nt(v, ph)

    r_i = lax.broadcasted_iota(jnp.int32, (128, DH), 0)
    c_i = lax.broadcasted_iota(jnp.int32, (128, DH), 1)
    expand = (r_i % DH == c_i).astype(bf16)
    r_h = lax.broadcasted_iota(jnp.int32, (128, 128), 0) // DH
    c_h = lax.broadcasted_iota(jnp.int32, (128, 128), 1) // DH
    same_head = r_h == c_h

    def make_amat(g):
        a = _dot_nt(expand, wphi_v[g * 128:(g + 1) * 128, :])
        amat_v[:, g * 128:(g + 1) * 128] = _pk(jnp.where(same_head, a, 0.0).astype(bf16))

    class Folder:
        def __init__(self, col0, first=0):
            self.col0, self.rows, self.mprev, self.done = col0, {}, None, first

        def tile(self, g, rows, keep=None, ties=None):
            am = amat_v[:, g * 128:(g + 1) * 128]
            if ties:
                am = _tie(keep, am, ties)
            return _dot_nt(_upk(am), wqkv_v[rows, self.col0 + g * 128:self.col0 + (g + 1) * 128])

        def fold(self, g, wt=None):
            sub = lax.broadcasted_iota(jnp.int32, (8, D), 0)
            if wt is None:
                wt = self.tile(g, slice(None))
            for hh in range(4):
                full, below, _, a = _head_groups(4 * g + hh)
                r0 = hh * DH
                ref = jnp.broadcast_to(wt[r0 + a - 1:r0 + a, :], (8, D))
                part = [(wt[r0 + 8 * i:r0 + 8 * (i + 1)] - ref) * LOG2E for i in range(4)]
                if below is not None:
                    self.rows[below] = jnp.where(sub >= a, part[0], self.mprev)
                self.mprev = part[0]
                for q, v in zip(full, part[1:]):
                    self.rows[q] = v
            new = {}
            while self.done in self.rows and self.done + 1 in self.rows:
                new[self.done] = jnp.concatenate([self.rows.pop(self.done), self.rows.pop(self.done + 1)], axis=0)
                self.done += 2
            return new

    def fold_pair(folders, g, keep=None, ties=None):
        tiles = {}
        for n, c in enumerate(range(0, HK, 128)):
            for half in range(2):
                for side in range(2):
                    t = ties[n] if ties and half == 0 and side == 0 else None
                    lo = side * HK + c
                    tiles[(half, lo)] = folders[half].tile(g + 4 * half, slice(lo, lo + 128), keep, t)
        return [folders[half].fold(g + 4 * half,
                                   jnp.concatenate([tiles[(half, lo)] for lo in range(0, D, 128)], axis=1))
                for half in range(2)]

    bestv_v[...] = jnp.full(bestv_v.shape, -jnp.inf, f32)
    besti_v[...] = lax.broadcasted_iota(jnp.int32, besti_v.shape, 0)
    h_v[0:P2, :] = jnp.zeros((P2, D), f32)
    st_v[0:B, :] = jnp.zeros((B, 256), f32)
    pend_v[...] = jnp.zeros(pend_v.shape, f32)

    def wait_all(cps):
        for cp in cps:
            cp.wait()

    def amats(c):
        for g0, n in _PSTAGES[c]:
            for g in range(g0, g0 + n):
                make_amat(g)

    wait_all(cp_p[0])
    amats(0)

    cp_x0.wait()
    ln1(x_v, 0, xs_v, 0, T0, plain=True)
    xb = [load_xn(s) for s in range(2)]
    logits = [{}, {}]
    finished = [set(), set()]
    fk, slabs = (Folder(D), Folder(D, NV // 2)), {}
    defer, queue = [False], []

    def absorb(new):
        for pos, slab in new.items():
            wtk_v[pos * 4:pos * 4 + 8, :] = _pk(slab.astype(bf16))
            slabs[pos] = slab
        for pos in sorted(slabs):
            if pos < NV // 2 and pos + NV // 2 in slabs:
                store_combos(wsk_v, pos * 4, slabs.pop(pos), slabs.pop(pos + NV // 2))

    def k_finish(s, hold=0):
        ready = [j for j in range(NP) if j not in finished[s] and _pair_need(j) in logits[s]]
        ready = ready[:len(ready) - hold]
        if defer[0]:
            queue.extend((logits[s].__getitem__, [j], s) for j in ready)
        else:
            k_side(logits[s].__getitem__, ready, s)
        finished[s].update(ready)

    def k_chunk(s, keep=None, early=(), late=(), hold=0):
        todo = [q for half in range(2) for q in range(half * (NV // 2), fk[half].done) if q not in logits[s]]
        runs = [[q for q in todo if q < NV // 2], [q for q in todo if q >= NV // 2]]
        lhs = jnp.concatenate([wtk_v[r[0] * 4:(r[-1] + 1) * 4, :] for r in runs if r], axis=0)
        ties = piece_ties(early, lhs.shape[0])
        ties.update(piece_ties(late, lhs.shape[0], col=HK))
        if ties:
            lhs = _tie(keep, lhs, ties)
        p = _dot_nt(_upk(lhs), xb[s])
        for n, q in enumerate(todo):
            logits[s][q] = p[n * 8:(n + 1) * 8]
        k_finish(s, hold)
        return p

    wait_all(cp_k[0])
    for new in fold_pair(fk, 0):
        absorb(new)
    k_chunk(0)
    k_chunk(1, hold=1)

    wait_all(cp_p[1] + cp_k[1])
    k_finish(1)
    amats(1)
    for new in fold_pair(fk, 1):
        absorb(new)
    absorb(fk[0].fold(2))
    k_chunk(0)
    k_chunk(1, hold=1)

    wait_all(cp_k[2] + [cp_x1])
    defer[0] = True
    keep = flag_s[0] > 0
    absorb(fk[1].fold(6))
    new = fold_pair(fk, 3)
    late = list(new[0].values())[-1][:, 384:512]
    for n in new:
        absorb(n)
    pieces = ln1(x_v, T0, xs_v, T0, T0, [0]) + ln1(x_v, T0, xs_v, T0, T0, [1, 2], keep, [late, late])
    p = k_chunk(0, keep, (), pieces[:2])
    rows = [k * p.shape[0] // 5 // 16 * 16 for k in range(5)]
    pieces += ln1(x_v, T0, xs_v, T0, T0, range(3, 8), keep, [p[r:r + R] for r in rows])
    k_chunk(1, keep, pieces[2:3], pieces[3:])

    def k_emit1(half, blk, val):
        now = {(1, 0): 8, (0, 1): 6}.get((half, blk), 0)
        pairs = list(half_pairs(half))
        k_side(half_groups(val, half), pairs[:now], 2 + blk)
        queue.extend((half_groups(val, half), [j], 2 + blk) for j in pairs[now:])

    def run_queue(n, res):
        deps = []
        for k in range(min(n, len(queue))):
            r = k * res.shape[0] // n // 8 * 8
            v = _vregs(k_side(*queue.pop(0), keep=keep, anchor=res[r:r + 8])[0])
            deps.append([_or_all(v[q::4]) for q in range(4)])
        return deps

    kwork = {}

    def k_after(m, res):
        if m in (0, 2):
            kwork[m + 1] = run_queue(4, res)

    def k_before(m):
        if m == 4:
            cp_wv.wait()
            cp_x2.wait()
            for rb in range(0, HK, 128):
                for c in range(0, HK, 128):
                    raw = [wqkv_v[side * HK + c:side * HK + c + 128,
                                  2 * D + half * HK + rb:2 * D + half * HK + rb + 128].T
                           for half in range(2) for side in range(2)]
                    blocks = [t.astype(f32) for t in raw]
                    for n, spec in enumerate(_SA):
                        t = raw[spec[0]] if spec[1] is None else _combo(blocks, spec).astype(bf16)
                        wsv_v[rb // 2:rb // 2 + 64, n * HK + c:n * HK + c + 128] = _pk(t)

    sproj(wsk_v, xs_v, 1, k_emit1, keep, kwork, k_before, k_after)

    def ln_anchored(xg, src, xd, dst, k, n, keep, res):
        which = list(range(k * 8 // n, (k + 1) * 8 // n))
        rows = [a * HK // len(which) // 16 * 16 for a in range(len(which))]
        pcs = ln1(xg, src, xd, dst, P2, which, keep, [res[r:r + R] for r in rows])
        return [[]] * (3 - len(pcs)) + pcs

    vt = {}
    wsv = wsv_v.at[pl.ds(pl.multiple_of(flag_s[1], D // 4), D // 4)]
    work = {0: {}, 1: {}}

    def v_after(q):
        def after(m, res):
            t = 7 * q + m
            if t < 6:
                work[0][m + 1] = run_queue(-(-len(queue) // (6 - t)), res)
            elif t < 13:
                work[1][t - 6] = ln_anchored(x_v, T, xs_v, T, t - 6, 7, keep, res)
        return after

    for q in range(2):
        sproj(wsv, xs_v, q, lambda half, blk, val, q=q: vt.__setitem__((2 * q + blk, half), val),
              keep, work[q], None, v_after(q))
    assert not queue
    phi_m = sealed(phi_v)
    for j in range(NP):
        kvacc_v[j] = kv_prod(vt, _upk(phi_m[j * 64:(j + 1) * 64, :]), j)
    cp_x3.wait()
    wait_bg(0)

    def p1_body(i, c):
        @pl.when(i == 2)
        def _():
            cp_x4.wait()
            wait_bg(1)

        @pl.when(i == 3)
        def _():
            wait_bg(2)

        keep = flag_s[0] > 0
        lo = jnp.minimum((i - 1) * DCH, F - DCH)
        sv = wd_v.at[pl.ds(pl.multiple_of(lo, 16), DCH)]
        dv = wdp_v.at[pl.ds(pl.multiple_of(lo // 2, 8), DCH // 2)]
        rp = repacker([(sv, dv, r, c) for r in range(0, DCH, 16) for c in range(0, D, 128)], keep)
        lo = jnp.minimum((i - 1) * OCH, HK - OCH)
        ov = wo_v.at[pl.ds(pl.multiple_of(lo, 16), HK + OCH)]
        od = wso_v.at[pl.ds(pl.multiple_of(lo // 2, 8), OCH // 2)]

        def k_emit(q):
            return lambda half, blk, val: k_side(half_groups(val, half), half_pairs(half), 2 * q + blk)

        vt = {}

        def v_emit(q):
            return lambda half, blk, val: vt.__setitem__((2 * q + blk, half), val)

        xd = xs_view(i, 2)
        xa = x_v.at[pl.ds(pl.multiple_of(i * T + P2, P2), P2)]
        xb = x_v.at[pl.ds(pl.multiple_of(jnp.minimum(i + 1, NT - 1) * T, T), P2)]
        wa = {}

        def a_after(m, res):
            if m < 6:
                wa[m + 1] = ln_anchored(xa, 0, xd, P2, m, 6, keep, res)

        sproj(wsv_v, xd, 0, v_emit(0), keep, wa, None, a_after)
        sproj(wsk_v, xd, 0, k_emit(0), after=rp[0])
        sproj(wsk_v, xd, 1, k_emit(1), after=rp[1])
        wb = spread(ln1(xb, 0, xd, T, P2), [(0, m) for m in range(1, 7)])[0]

        def b_after(m, res):
            slabs = list(range(0, OCH, 16))
            mine = slabs[(m - 1) * len(slabs) // 6:m * len(slabs) // 6] if m else []
            for n, r in enumerate(mine):
                rows = [((4 * n + c) * HK // (4 * len(mine))) // 16 * 16 for c in range(4)]
                store_combos(od, r // 2, ov[r:r + 16, :].astype(f32), ov[HK + r:HK + r + 16, :].astype(f32),
                             _SB, keep, [res[a:a + R] for a in rows])

        sproj(wsv_v, xd, 1, v_emit(1), keep, wb, None, b_after)
        phi_m = sealed(phi_v)
        for j in range(NP):
            kvacc_v[j] += kv_prod(vt, _upk(phi_m[j * 64:(j + 1) * 64, :]), j)
        return c

    lax.fori_loop(1, NT, p1_body, 0)

    wait_all([cp_wr, cp_wq] + cp_gu[0])
    keep = flag_s[0] > 0
    kv_mask = (lax.broadcasted_iota(jnp.int32, (64, 128), 0) // DH
               == (lax.broadcasted_iota(jnp.int32, (64, 128), 1) // DH) % 2)
    ties = [{} for _ in range(16)]
    for j in range(NP):
        kvj = jnp.where(kv_mask, kvacc_v[j], 0.0)
        kv_v[:, j * 128:(j + 1) * 128] = _pk(kvj.astype(bf16))
        zj = _lanes(jnp.sum(zacc_v[j * 128:(j + 1) * 128, :], axis=-1, keepdims=True))
        zacc_v[j * 128:(j + 1) * 128, :] = zj
        vals = _vregs(kvj) + _vregs(zj)
        if j + 1 < 16:
            for q in range(4):
                ties[j + 1][(32 + q * 8, 0)] = _or_all(vals[q::4])
    wr = wr_v[0:8, :].astype(f32)
    wl = jnp.sum(wr, axis=0, keepdims=True)
    wsum = jnp.sum(wl, axis=1, keepdims=True)
    wrb_v[:, 0:D + 256] = jnp.concatenate(
        [jnp.broadcast_to(wr[j:j + 1, :], (8, 128)) for j in range(8)]
        + [jnp.broadcast_to(wsum, (8, 128)), jnp.broadcast_to(wl, (8, 128))], axis=1)
    for t in range(NT):
        store_xt(t, xs_v, t * (T // 4))
    fq = (Folder(0), Folder(0, NV // 2))
    for g in range(4):
        new = fold_pair(fq, g, keep, ties[4 * g:4 * g + 4])
        for pos, slab in new[0].items():
            store_combos(wsq_v, pos * 4, slab, new[1][pos + NV // 2])

    pq_v = (pq0_v, pq1_v, pq2_v, pq3_v)

    def views_of(g):
        lo = g * (BPI * B)
        if not isinstance(g, int):
            lo = pl.multiple_of(lo, BPI * B)
        return ((x_v.at[pl.ds(lo, BPI * B)],)
                + tuple(ref.at[pl.ds(lo, P2 + BPI * B)] for ref in (h_v, out_v, st_v)) + (g,))

    def stage_q(xd, q, first, before, after):
        def emit(half, blk, val):
            group = half_groups(val, half)
            for j in half_pairs(half):
                ph = _hedgehog_t(_pair_logits(group, j), zacc_v[j * 128:(j + 1) * 128, :])
                pq_v[2 * q + blk][(j // 2) * 64:(j // 2 + 1) * 64, (j % 2) * B:(j % 2 + 1) * B] = _pk(ph.astype(bf16))

        sproj(wsq_v, xd, q, emit, before=before, after=after, first=first)

    oc_v = (oc0_v, oc1_v)

    def stage_g(q):
        pq = [sealed(pq_v[2 * q + blk]) for blk in range(2)]
        for t in range(NP // 4):
            parts = [[_dot_nn(_upk(kv_v[:, j * 128:(j + 1) * 128]),
                              _upk(pq[blk][(j // 2) * 64:(j // 2 + 1) * 64, (j % 2) * B:(j % 2 + 1) * B]))
                      for blk in range(2) for j in (jj, jj + NP // 2)] for jj in (2 * t, 2 * t + 1)]
            blocks = [jnp.concatenate([a, b], axis=0) for a, b in zip(*parts)]
            for m, spec in enumerate(_SA):
                c = m * HK + t * 128
                oc_v[q][0:B // 2, c:c + 128] = _pk(_combo(blocks, spec).astype(bf16).T)

    def stage_h(views, q, keep, pieces, jobs, before=None):
        x_g, h_g = views[0], views[1]
        oc = sealed(oc_v[q])
        first, last = 4, 12
        ties = [{} for _ in range(7)]
        for k, vals in enumerate(pieces):
            t = first + k * (last - first) // max(len(pieces) - 1, 1)
            for m, val in enumerate(vals):
                ties[t // 4][(m * 8, (t % 4) * 128)] = val
        state = {}
        done = [0]

        def product(m):
            if before:
                before(m)
            w = wso_v[:, m * HK:(m + 1) * HK]
            if ties[m]:
                w = _tie(keep, w, ties[m])
            done[0] = m
            res = _dot_nn(_upk(oc[0:B // 2, m * HK:(m + 1) * HK]), _upk(w))
            for k, job in enumerate(jobs):
                t = 2 * q + k * (24 - 4 * q) // len(jobs)
                if t // 4 == m:
                    job(res[0:R, (t % 4) * 128:(t % 4 + 1) * 128])
            return res

        def wmul(d, lo):
            return (d.reshape(B // 8, 8, 128) * wrb_v[:, lo:lo + 128][None]).reshape(B, 128)

        def emit(k, val):
            blk, half = k // 2, k % 2
            s = 2 * q + blk
            cols = slice(half * HK, (half + 1) * HK)
            h = x_g[s * B:(s + 1) * B, cols].astype(f32) + val
            h_g[(s + 2) * B:(s + 3) * B, cols] = h
            st = state.setdefault(blk, {'h': {}})
            st['h'][half] = h
            for c in range(0, HK, 128):
                ht = h[:, c:c + 128]
                if 'h0' not in st:
                    st['h0'] = ht
                    continue
                d = ht - st['h0']
                new = (d, d * d, wmul(d, half * HK + c))
                st['s'] = new if 's' not in st else tuple(a + b for a, b in zip(st['s'], new))
            if len(st['h']) == 1:
                vals = [_or_all(list(v)) for v in zip(*[_vregs(a) for a in st['s']])]
                m = done[0] + 2
                for n, val in enumerate(vals):
                    ties[m][(248 - (n % 4) * 8, (n // 4) * 128)] = val

        _strassen(product, emit)

        res = []
        for blk in range(2):
            st = state[blk]
            s1, s2, s3 = st['s']
            c0 = _lanes(jnp.mean(st['h0'], axis=-1, keepdims=True))
            g0 = st['h0'] - c0
            t1 = s1 + 8.0 * g0
            t2 = s2 + g0 * (s1 + t1)
            t3 = s3 + wmul(g0, D + 128)
            res.append((jnp.concatenate([t1, t2, t3, c0], axis=1),
                        jnp.concatenate([st['h'][0], st['h'][1]], axis=1)))
        return res

    def stage_stats(views, s, part, valid=None):
        st_g, g = views[3], views[4]
        b = g * BPI + s
        bv = bestv_v[...]
        bi = besti_v[...]
        wsum = wrb_v[0:1, D:D + 128]
        nvs, nis, sts = [], [], []
        for k in range(B // R):
            sl = slice(k * R, (k + 1) * R)
            red = [_lanes(jnp.sum(part[sl, n * 128:(n + 1) * 128], axis=-1, keepdims=True)) for n in range(3)]
            mu = red[0] * (1.0 / D)
            var = jnp.maximum(red[1] * (1.0 / D) - mu * mu, 0.0)
            rs = lax.rsqrt(var + LN_EPS)
            r = (red[2] - mu * wsum) * rs
            sts.append(jnp.concatenate([rs, (mu + part[sl, 384:512]) * rs], axis=1))
            if valid is not None:
                r = jnp.where(valid, r, -jnp.inf)
            idx = lax.broadcasted_iota(jnp.int32, (R, 128), 0) + (b * B + k * R)
            better = r > bv[sl]
            nvs.append(jnp.where(better, r, bv[sl]))
            nis.append(jnp.where(better, idx, bi[sl]))
        st = jnp.concatenate(sts, axis=0)
        st_g[(s + 2) * B:(s + 3) * B, :] = st
        bestv_v[...] = jnp.concatenate(nvs, axis=0)
        besti_v[...] = jnp.concatenate(nis, axis=0)
        return st, [_vregs(nv) for nv in nvs]

    def out_jobs(views, s, keep, st=None, h=None):
        h_g, out_g, st_g = views[1], views[2], views[3]

        def job(k):
            def run(anchor):
                rows = slice((s + 2) * B + k * R, (s + 2) * B + (k + 1) * R)
                hk = h_g[rows, :] if h is None else h[k * R:(k + 1) * R]
                sk = st_g[rows, :] if st is None else st[k * R:(k + 1) * R]
                a = 1.0 + jnp.where(keep, sk[:, 0:128], anchor)
                o = [hk[:, c * 128:(c + 1) * 128] * a - sk[:, 128:256] for c in range(D // 128)]
                out_g[rows, :] = jnp.concatenate(o, axis=1).astype(bf16)
            return run
        return [job(k) for k in range(B // R)]

    def p2_body(i, c):
        b0 = i * BPI
        keep = flag_s[0] > 0
        cur = views_of(i)
        st, pieces = stage_stats(cur, -1, pend_v[...], i > 0)
        ojobs = out_jobs(cur, -2, keep) + out_jobs(cur, -1, keep, st)
        n = D // NI
        jobs = []
        for src, dst in ((wg_v, wgp_v), (wu_v, wup_v)):
            sv = src.at[pl.ds(pl.multiple_of(i * n, n), n)]
            dv = dst.at[pl.ds(pl.multiple_of(i * (n // 2), n // 2), n // 2)]
            jobs += [(sv, dv, r, cc) for r in range(0, n, 16) for cc in range(0, NM, 128)]
        rp = repacker(jobs, keep)
        stage_q(xs_view(i, 1), 0, xt_view(i), None, rp[0])
        stage_q(xs_view(i, 1), 1, None, lambda m: stage_g(0) if m == 2 else None, rp[1])
        res = stage_h(cur, 0, keep, pieces, ojobs, lambda m: stage_g(1) if m == 1 else None)
        st0, _ = stage_stats(cur, 0, res[0][0])
        st1, pieces = stage_stats(cur, 1, res[1][0])
        ojobs = out_jobs(cur, 0, keep, st0, res[0][1]) + out_jobs(cur, 1, keep, st1, res[1][1])
        res = stage_h(cur, 1, keep, pieces, ojobs)
        stage_stats(cur, BPI - 2, res[0][0])
        pend_v[...] = res[1][0]

        @pl.when(i > 0)
        def _():
            cp_out(jnp.maximum(b0 - 2, 0), 2).start()

        cp_out(b0, 2).start()
        return c

    lax.fori_loop(0, NI, p2_body, 0)
    wait_all(cp_gu[1])
    keep = flag_s[0] > 0
    last = views_of(NI - 1)

    st, _ = stage_stats(last, BPI - 1, pend_v[...])

    bv = bestv_v[...]
    mval = jnp.max(bv, axis=0, keepdims=True)
    sel = jnp.min(jnp.where(bv == mval, besti_v[...], S - 1), axis=0, keepdims=True)
    idx = sel[0, 0]
    hrow = h_v[pl.ds(P2 + idx, 1), :]
    strow = st_v[pl.ds(P2 + idx, 1), :]
    xrow = jnp.concatenate([hrow[:, c * 128:(c + 1) * 128] * strow[:, 0:128] - strow[:, 128:256]
                            for c in range(D // 128)], axis=1).astype(bf16)
    xs = jnp.broadcast_to(xrow, (16, D))
    g_first = _dot_nn(xs, _upk(wgp_v[:, 0:FC]))
    for k, job in enumerate(out_jobs(last, BPI - 2, keep) + out_jobs(last, BPI - 1, keep, st)):
        job(g_first[:, (k // 2) * 128:(k // 2 + 1) * 128])
    cp_out(NB - 2, 2).start()

    def act(g, u):
        a = g * pl.reciprocal(1.0 + jnp.exp(-g), approx=True) * u
        return jnp.concatenate([a, a], axis=0).astype(bf16)

    def down(a, lo, w):
        return _dot_nn(a, _upk(wdp_v[lo // 2:(lo + w) // 2, 0:D]))[0:8]

    xcol = jnp.broadcast_to(xrow, (128, D)).T.astype(f32)
    jobs = [(which, b) for b in range(NBV) for which in (0, 1)]
    vres, prev = {}, None
    for j0 in range(0, len(jobs), NCH):
        grp = jobs[j0:j0 + NCH]
        accs = [None] * len(grp)
        for r in range(D // 16):
            for n, (which, b) in enumerate(grp):
                w = (wg_v, wu_v)[which][r * 16:(r + 1) * 16, NM + b * 128:NM + (b + 1) * 128].astype(f32)
                t0 = w[0:8] * xcol[r * 16:r * 16 + 8]
                t1 = w[8:16] * xcol[r * 16 + 8:r * 16 + 16]
                if accs[n] is None:
                    if prev is not None:
                        t0 = jnp.where(keep, t0, prev[n % len(prev)])
                    accs[n] = t0 + t1
                else:
                    accs[n] = (accs[n] + t0) + t1
        prev = accs
        for n, job in enumerate(grp):
            vres[job] = _allreduce8(accs[n][None], jnp.add)[0]

    chunks = [(lo, min(FC, NM - lo)) for lo in range(0, NM, FC)]
    acts, y = [], None
    for k, (lo, w) in enumerate(chunks):
        g = g_first if k == 0 else _dot_nn(xs, _upk(wgp_v[:, lo:lo + w]))
        u = _dot_nn(xs, _upk(wup_v[:, lo:lo + w]))
        acts.append(act(g[0:8], u[0:8]))
        if k >= 1:
            t = down(acts[k - 1], *chunks[k - 1])
            y = t if y is None else y + t
    y = y + down(acts[-1], *chunks[-1])
    for b0, nb in ((0, 4), (4, 4), (8, 4), (12, 1)):
        g = jnp.concatenate([vres[(0, b)] for b in range(b0, b0 + nb)], axis=1)
        u = jnp.concatenate([vres[(1, b)] for b in range(b0, b0 + nb)], axis=1)
        y = y + down(act(g, u), NM + b0 * 128, nb * 128)

    gate = jnp.broadcast_to(jax.nn.sigmoid(mval), (8, 128))
    base = pl.multiple_of((idx >> 4) << 4, 16)
    rows = pl.ds(pl.multiple_of(P2 + base, 16), 16)
    h16 = h_v[rows, :]
    st16 = st_v[rows, :]
    a16 = 1.0 + st16[:, 0:128]
    m16 = st16[:, 128:256]
    hit = (lax.broadcasted_iota(jnp.int32, (16, 128), 0) + base) == idx
    res = []
    for c in range(D // 128):
        yc = y[:, c * 128:(c + 1) * 128] * gate
        yc = jnp.concatenate([yc, yc], axis=0)
        res.append(h16[:, c * 128:(c + 1) * 128] * a16 - m16 + jnp.where(hit, yc, 0.0))
    res = jnp.concatenate(res, axis=1).astype(bf16)
    for i in range(NI):
        cp_out(i * BPI, 2).wait()
        cp_out(i * BPI + 2, 2).wait()
    out_v[rows, :] = res
    fix = pltpu.make_async_copy(out_v.at[rows], out_hbm.at[pl.ds(base, 16)], sem_o.at[0])
    fix.start()
    fix.wait()


@jax.jit
def pallas_sequential_preLN__linear_kernel_hedgehog__moe_arch_mod__prompt_kernel(
    A_x: jax.Array,
    A_wqkv: jax.Array,
    A_w_phi: jax.Array,
    A_wo: jax.Array,
    B_x: jax.Array,
    B_w_r: jax.Array,
    B_w_gate: jax.Array,
    B_w_up: jax.Array,
    B_w_down: jax.Array,
):
    del B_x
    x = A_x.reshape(S, D)
    wphi = A_w_phi.reshape(H * DH, DH)
    wr = B_w_r.reshape(8, 128)
    any_spec = pl.BlockSpec(memory_space=pl.ANY)
    out = pl.pallas_call(
        _kernel,
        out_shape=jax.ShapeDtypeStruct((S, D), bf16),
        in_specs=[any_spec] * 8,
        out_specs=any_spec,
        scratch_shapes=[
            pltpu.VMEM((S, D), bf16),
            pltpu.VMEM((D, 3 * D), bf16),
            pltpu.VMEM((H * DH, DH), bf16),
            pltpu.VMEM((D, D), bf16),
            pltpu.VMEM((64, 128), bf16),
            pltpu.VMEM((D, F + 128), bf16),
            pltpu.VMEM((D, F + 128), bf16),
            pltpu.VMEM((F, D), bf16),
            pltpu.VMEM((PR, D), u32),
            pltpu.VMEM((PR // 2, 7 * HK), u32),
            pltpu.VMEM((PR // 2, 7 * HK), u32),
            pltpu.VMEM((D // 4, 7 * HK), u32),
            pltpu.VMEM((D // 4, 7 * HK), u32),
            pltpu.VMEM((F // 2, D + 128), u32),
            pltpu.VMEM((D // 2, NM), u32),
            pltpu.VMEM((D // 2, NM), u32),
            pltpu.VMEM((64, 8 * 128), u32),
            pltpu.VMEM((T0 // 2, D), u32),
            pltpu.VMEM(((S + T) // 4, 7 * HK), u32),
            pltpu.VMEM((NT * (HK // 2), B), u32),
            pltpu.VMEM((NP, 64, 128), f32),
            pltpu.VMEM((2 * D, 128), f32),
            pltpu.VMEM((32, NP * 128), u32),
            pltpu.VMEM((D + 8, T), u32),
            pltpu.VMEM((D // 2 + 16, 2 * B), u32),
            pltpu.VMEM((D // 2 + 16, 2 * B), u32),
            pltpu.VMEM((D // 2 + 16, 2 * B), u32),
            pltpu.VMEM((D // 2 + 16, 2 * B), u32),
            pltpu.VMEM((B // 2 + 8, 7 * HK), u32),
            pltpu.VMEM((B // 2 + 8, 7 * HK), u32),
            pltpu.VMEM((P2 + S, D), f32),
            pltpu.VMEM((P2 + S, 256), f32),
            pltpu.VMEM((B, 512), f32),
            pltpu.VMEM((P2 + S, D), bf16),
            pltpu.VMEM((8, D + 512), f32),
            pltpu.VMEM((B, 128), f32),
            pltpu.VMEM((B, 128), jnp.int32),
            pltpu.SMEM((2,), jnp.int32),
            pltpu.SemaphoreType.DMA((_NSEM_IN,)),
            pltpu.SemaphoreType.DMA((1,)),
        ],
        compiler_params=pltpu.CompilerParams(vmem_limit_bytes=110 * 1024 * 1024,
                                             disable_bounds_checks=True,
                                             disable_semaphore_checks=True),
        name="hedgehog_mod",
    )(x, A_wqkv, wphi, A_wo, wr, B_w_gate, B_w_up, B_w_down)
    return out.reshape(1, S, D)
```

```python
import jax
import jax.numpy as jnp
from jax import lax
import jax.experimental.pallas as pl
import jax.experimental.pallas.tpu as pltpu

S = 2048
D = 1024
H = 32
DH = 32
F = 3584
T = 512
NT = S // T
T0 = 256
B = 128
NB = S // B
BPI = 4
NI = NB // BPI
NP = H // 2
FC = 1024
R = 16
NBV = 13
NM = F - NBV * 128
NCH = 4
OCH = 176
DCH = 1216
NV = 124
PR = NV * 4
HK = D // 2
P2 = 2 * B
LOG2E = 1.4426950408889634
LN_EPS = 1e-5
DEN_EPS = 1e-6

_NT_DIMS = (((1,), (1,)), ((), ()))

bf16 = jnp.bfloat16
f32 = jnp.float32
u32 = jnp.uint32


def _dot_nt(a, b):
    return lax.dot_general(a, b, _NT_DIMS, preferred_element_type=f32)


def _dot_nn(a, b):
    return jnp.dot(a, b, preferred_element_type=f32)


def _pk(x):
    return pltpu.bitcast(x, u32)


def _upk(x):
    return pltpu.bitcast(x, bf16)


def _lanes(x):
    return jnp.broadcast_to(x, (x.shape[0], 128))


def _layernorm(x):
    m = jnp.mean(x, axis=-1, keepdims=True)
    xc = x - m
    v = jnp.mean(xc * xc, axis=-1, keepdims=True)
    return xc * lax.rsqrt(v + LN_EPS)


def _allreduce8(x, op):
    x = op(x, pltpu.roll(x, 4, 1))
    x = op(x, pltpu.roll(x, 2, 1))
    x = op(x, pltpu.roll(x, 1, 1))
    return x


def _hedgehog_t(p, z=None):
    t = p.shape[-1]
    p4 = p.reshape(2, 4, 8, t)
    mx = _allreduce8(jnp.max(p4, axis=1), jnp.maximum)
    mn = _allreduce8(jnp.min(p4, axis=1), jnp.minimum)
    ep = jnp.exp2(p4 - mx[:, None])
    en = jnp.exp2(mn[:, None] - p4)
    a = pl.reciprocal(_allreduce8(jnp.sum(ep, axis=1), jnp.add), approx=True)
    b = pl.reciprocal(_allreduce8(jnp.sum(en, axis=1), jnp.add), approx=True)
    if z is not None:
        dp = jnp.sum(ep * z[0:64].reshape(2, 4, 8, t), axis=1)
        dn = jnp.sum(en * z[64:128].reshape(2, 4, 8, t), axis=1)
        den = _allreduce8(dp * a + dn * b, jnp.add) + DEN_EPS
        inv = pl.reciprocal(den, approx=True)
        a = a * inv
        b = b * inv
    fp = (ep * a[:, None]).reshape(64, t)
    fn = (en * b[:, None]).reshape(64, t)
    return jnp.concatenate([fp, fn], axis=0)


_SA = ((3, None, 0), (2, 3, 1), (0, 1, 1), (0, None, 0), (0, 3, 1), (1, 3, -1), (2, 0, -1))
_SB = ((2, 0, -1), (0, None, 0), (3, None, 0), (1, 3, -1), (0, 3, 1), (2, 3, 1), (0, 1, 1))


def _combo(blocks, spec):
    a, b, sign = spec
    if b is None:
        return blocks[a]
    return blocks[a] + blocks[b] if sign > 0 else blocks[a] - blocks[b]


def _strassen(product, emit):
    m4 = product(0)
    m2 = product(1)
    emit(2, m4 + m2)
    m5 = product(2)
    u = m4 - m5
    m3 = product(3)
    emit(1, m5 + m3)
    v = m3 - m2
    m1 = product(4)
    u = u + m1
    v = v + m1
    emit(0, u + product(5))
    emit(3, v + product(6))


def _head_groups(h):
    base, k = (NV // 4) * (h // 8), h % 8
    return ([base + 4 * k + i for i in range(3)],
            base + 4 * k - 1 if k > 0 else None,
            base + 4 * k + 3 if k < 7 else None,
            8 - k)


def _pair_logits(group, j):
    parts = []
    for h in (2 * j, 2 * j + 1):
        full, below, above, a = _head_groups(h)
        ref = group(full[0])
        sub = lax.broadcasted_iota(jnp.int32, ref.shape, 0)
        if above is None:
            m = jnp.where(sub >= a, group(below), 0.0)
        else:
            m = jnp.where(sub == a - 1, 0.0, group(above))
            if below is not None:
                m = jnp.where(sub >= a, group(below), m)
        parts += [m] + [group(q) for q in full]
    return jnp.concatenate(parts, axis=0)


def _pair_need(j):
    full, _, above, _ = _head_groups(2 * j + 1)
    return full[2] if above is None else above


def _tie(keep, w, ties):
    rows = sorted({r for r, _ in ties})
    out, pos = [], 0
    for r in rows:
        if r > pos:
            out.append(w[pos:r])
        cols = sorted(c for rr, c in ties if rr == r)
        parts, cpos = [], 0
        for c in cols:
            if c > cpos:
                parts.append(w[r:r + 8, cpos:c])
            parts.append(jnp.where(keep, w[r:r + 8, c:c + 128], ties[(r, c)]))
            cpos = c + 128
        if cpos < w.shape[1]:
            parts.append(w[r:r + 8, cpos:])
        out.append(jnp.concatenate(parts, axis=1) if len(parts) > 1 else parts[0])
        pos = r + 8
    if pos < w.shape[0]:
        out.append(w[pos:])
    return jnp.concatenate(out, axis=0)


def _vregs(x):
    if x.dtype != u32:
        x = pltpu.bitcast(x, u32)
    return [x[r:r + 8, c:c + 128] for r in range(0, x.shape[0], 8) for c in range(0, x.shape[1], 128)]


def _or_all(vals):
    acc = vals[0]
    for v in vals[1:]:
        acc = acc | v
    return acc


_KSTAGES = (((0, 1), (4, 1)), ((1, 2), (5, 1)), ((3, 1), (6, 2)))
_PSTAGES = (((0, 1), (4, 1)), ((1, 3), (5, 3)))
_NSEM_IN = 11


def _kernel(x_hbm, wqkv_hbm, wphi_hbm, wo_hbm, wr_hbm, wg_hbm, wu_hbm, wd_hbm,
            out_hbm,
            x_v, wqkv_v, wphi_v, wo_v, wr_v, wg_v, wu_v, wd_v,
            wtk_v, wsq_v, wsk_v, wsv_v, wso_v, wdp_v, wgp_v, wup_v, amat_v, xn_v, xs_v, xt_v, kvacc_v, zacc_v, kv_v, phi_v,
            pq0_v, pq1_v, pq2_v, pq3_v, oc0_v, oc1_v, h_v, st_v, pend_v, out_v, wrb_v,
            bestv_v, besti_v, flag_s,
            sem_i, sem_o):

    def cp_x(lo, n, sem):
        return pltpu.make_async_copy(x_hbm.at[pl.ds(lo, n)], x_v.at[pl.ds(lo, n)], sem_i.at[sem])

    def cp_w(lo, w, sem):
        return pltpu.make_async_copy(wqkv_hbm.at[:, pl.ds(lo, w)], wqkv_v.at[:, pl.ds(lo, w)], sem_i.at[sem])

    cp_k = [[cp_w(D + g * 128, n * 128, 2 + c) for g, n in st] for c, st in enumerate(_KSTAGES)]
    cp_p = [[pltpu.make_async_copy(wphi_hbm.at[pl.ds(g * 128, n * 128)], wphi_v.at[pl.ds(g * 128, n * 128)],
                                   sem_i.at[3 * c]) for g, n in st] for c, st in enumerate(_PSTAGES)]
    cp_wv = cp_w(2 * D, D, 5)
    cp_wq = cp_w(0, D, 7)

    def cp_wd(k):
        lo, n = k * DCH, min(DCH, F - k * DCH)
        return pltpu.make_async_copy(wd_hbm.at[pl.ds(lo, n)], wd_v.at[pl.ds(lo, n)], sem_i.at[(6, 8, 9)[k]])

    cp_x0 = cp_x(0, T0, 1)
    cp_x1 = cp_x(T0, T0, 4)
    cp_x2 = cp_x(T, P2, 5)
    cp_x3 = cp_x(T + P2, T, 6)
    cp_x4 = cp_x(2 * T + P2, S - 2 * T - P2, 8)
    cp_wr = pltpu.make_async_copy(wr_hbm, wr_v.at[pl.ds(0, 8)], sem_i.at[7])

    def cp_wo(k, half):
        lo, n = k * OCH, min(OCH, HK - k * OCH)
        rows = pl.ds(half * HK + lo, n)
        return pltpu.make_async_copy(wo_hbm.at[rows], wo_v.at[rows], sem_i.at[(6, 8, 9)[k]])

    def wait_bg(k):
        cp_wo(k, 0).wait()
        cp_wo(k, 1).wait()
        cp_wd(k).wait()

    cp_gu = [[pltpu.make_async_copy(src.at[:, pl.ds(lo, n)], dst.at[:, pl.ds(lo, n)], sem_i.at[sem])
              for src, dst in ((wg_hbm, wg_v), (wu_hbm, wu_v))] for lo, n, sem in ((0, NM, 7), (NM, F - NM, 10))]

    def cp_out(b, n):
        lo = b * B
        if not isinstance(b, int):
            lo = pl.multiple_of(lo, B)
        return pltpu.make_async_copy(out_v.at[pl.ds(P2 + lo, n * B)], out_hbm.at[pl.ds(lo, n * B)], sem_o.at[0])

    for cp in (*cp_p[0], cp_x0, *cp_k[0], *cp_p[1], *cp_k[1], *cp_k[2], cp_x1, cp_wv, cp_x2,
               cp_x3, cp_wo(0, 0), cp_wo(0, 1), cp_wd(0), cp_x4, cp_wo(1, 0), cp_wo(1, 1), cp_wd(1),
               cp_wo(2, 0), cp_wo(2, 1), cp_wd(2), cp_wr, cp_wq, *cp_gu[0], *cp_gu[1]):
        cp.start()
    flag_s[0] = 1
    flag_s[1] = 0

    def ln1(xg, src, xd, dst, n, which=None, keep=None, anchors=None, plain=False):
        pieces = []
        for pr in range(n // P2):
            for k in range(B // R):
                off = pr * P2 + k * R
                if which is not None and pr * (B // R) + k not in which:
                    continue
                x0 = xg[src + off:src + off + R, :].astype(f32)
                x1 = xg[src + off + B:src + off + B + R, :].astype(f32)
                if anchors is not None:
                    a = anchors[len(pieces)]
                    x0 = jnp.concatenate([jnp.where(keep, x0[:, :128], a), x0[:, 128:]], axis=1)
                    x1 = jnp.concatenate([jnp.where(keep, x1[:, :128], a), x1[:, 128:]], axis=1)
                p0 = _layernorm(x0)
                p1 = _layernorm(x1)
                if plain:
                    xn_v[off // 2:(off + R) // 2, :] = _pk(p0.astype(bf16))
                    xn_v[(off + B) // 2:(off + B + R) // 2, :] = _pk(p1.astype(bf16))
                lo = (dst + pr * P2) // 4 + k * (R // 2)
                blocks = (p0[:, :HK], p1[:, :HK], p0[:, HK:], p1[:, HK:])
                vs = []
                for m, spec in enumerate(_SB):
                    t = _combo(blocks, spec)
                    xd[lo:lo + R // 2, m * HK:(m + 1) * HK] = _pk(t.astype(bf16))
                    if spec[1] is not None:
                        vs.append(_vregs(t))
                pieces.append([_or_all(list(col)) for col in zip(*vs)])
        return pieces

    def load_xn(b):
        return _upk(xn_v[b * (B // 2):(b + 1) * (B // 2), :])

    def piece_ties(pieces, n, row0=0, col=0):
        ties = {}
        if pieces:
            step = (n - row0) // len(pieces) // 8 * 8
            for k, p in enumerate(pieces):
                for q, val in enumerate(p):
                    ties[(row0 + k * step + (q // 4) * 8, col + (q % 4) * 128)] = val
        return ties

    def xs_view(i, tiles):
        return xs_v.at[pl.ds(pl.multiple_of(i * (T // 4), T // 4), tiles * (T // 4))]

    def xt_view(i):
        lo = i * (HK // 2)
        return xt_v.at[pl.ds(lo if isinstance(i, int) else pl.multiple_of(lo, HK // 2), HK // 2)]

    def store_xt(i, xd, row):
        xt_view(i)[...] = _pk(_upk(xd[row:row + B // 2, 0:HK]).T)

    def sproj(ws, xd, pr, emit, keep=None, work=None, before=None, after=None, first=None):
        lo = pr * (B // 2)

        def product(m):
            if before:
                before(m)
            lhs = ws[:, m * HK:(m + 1) * HK]
            if work is not None and work.get(m):
                lhs = _tie(keep, lhs, piece_ties(work[m], lhs.shape[0], 32))
            if m == 0 and first is not None:
                res = _dot_nn(_upk(lhs), _upk(first[...]))
            else:
                res = _dot_nt(_upk(lhs), _upk(xd[lo:lo + B // 2, m * HK:(m + 1) * HK]))
            if after:
                after(m, res)
            return res

        _strassen(product, lambda k, val: emit(k // 2, k % 2, val))

    def repacker(jobs, keep):
        def hook(q):
            def after(m, res):
                if m in (0, 2, 4):
                    k = 3 * q + m // 2
                    mine = jobs[k * len(jobs) // 6:(k + 1) * len(jobs) // 6]
                    for n, (sv, dv, r, c) in enumerate(mine):
                        a = (64 + n * 416 // len(mine)) // 8 * 8
                        dv[r // 2:r // 2 + 8, c:c + 128] = jnp.where(keep, _pk(sv[r:r + 16, c:c + 128]),
                                                                     pltpu.bitcast(res[a:a + 8], u32))
            return after
        return hook(0), hook(1)

    def spread(pieces, slots):
        res = {}
        for k, (pr, m) in enumerate(slots):
            res.setdefault(pr, {})[m] = pieces[k * len(pieces) // len(slots):(k + 1) * len(pieces) // len(slots)]
        return res

    def sealed(ref):
        ref[pl.ds(pl.multiple_of(flag_s[1] + ref.shape[0] - 8, 8), 8), 0:128] = jnp.zeros((8, 128), u32)
        return ref

    def store_combos(ws, row, top, bot, table=_SA, keep=None, anchors=None):
        for c in range(0, HK, 128):
            blocks = [top[:, c:c + 128], top[:, HK + c:HK + c + 128], bot[:, c:c + 128], bot[:, HK + c:HK + c + 128]]
            if anchors is not None:
                for q in (0, 3):
                    blocks[q] = jnp.where(keep, blocks[q], anchors[c // 128])
            for m, spec in enumerate(table):
                ws[row:row + 8, m * HK + c:m * HK + c + 128] = _pk(_combo(blocks, spec).astype(bf16))

    zinit = set()

    def k_side(group, pairs, slot, keep=None, anchor=None):
        res = []
        for j in pairs:
            p = _pair_logits(group, j)
            if anchor is not None:
                p = jnp.concatenate([jnp.where(keep, p[0:8], anchor), p[8:32],
                                     jnp.where(keep, p[32:40], anchor), p[40:64]], axis=0)
            ph = _hedgehog_t(p)
            if j not in zinit:
                zinit.add(j)
                zacc_v[j * 128:(j + 1) * 128, :] = ph
            else:
                zacc_v[j * 128:(j + 1) * 128, :] += ph
            phi_v[j * 64:(j + 1) * 64, slot * B:(slot + 1) * B] = _pk(ph.astype(bf16))
            res.append(ph)
        return res

    def half_groups(p, half):
        return lambda pos: p[(pos - half * (NV // 2)) * 8:(pos - half * (NV // 2) + 1) * 8]

    def half_pairs(half):
        return range(half * (NP // 2), (half + 1) * (NP // 2))

    def kv_prod(vt, ph, j):
        half, r = j // (NP // 2), (j % (NP // 2)) * 64
        v = jnp.concatenate([vt[(s, half)][r:r + 64] for s in range(T // B)], axis=1).astype(bf16)
        return _dot_nt(v, ph)

    r_i = lax.broadcasted_iota(jnp.int32, (128, DH), 0)
    c_i = lax.broadcasted_iota(jnp.int32, (128, DH), 1)
    expand = (r_i % DH == c_i).astype(bf16)
    r_h = lax.broadcasted_iota(jnp.int32, (128, 128), 0) // DH
    c_h = lax.broadcasted_iota(jnp.int32, (128, 128), 1) // DH
    same_head = r_h == c_h

    def make_amat(g):
        a = _dot_nt(expand, wphi_v[g * 128:(g + 1) * 128, :])
        amat_v[:, g * 128:(g + 1) * 128] = _pk(jnp.where(same_head, a, 0.0).astype(bf16))

    class Folder:
        def __init__(self, col0, first=0):
            self.col0, self.rows, self.mprev, self.done = col0, {}, None, first

        def tile(self, g, rows, keep=None, ties=None):
            am = amat_v[:, g * 128:(g + 1) * 128]
            if ties:
                am = _tie(keep, am, ties)
            return _dot_nt(_upk(am), wqkv_v[rows, self.col0 + g * 128:self.col0 + (g + 1) * 128])

        def fold(self, g, wt=None):
            sub = lax.broadcasted_iota(jnp.int32, (8, D), 0)
            if wt is None:
                wt = self.tile(g, slice(None))
            for hh in range(4):
                full, below, _, a = _head_groups(4 * g + hh)
                r0 = hh * DH
                ref = jnp.broadcast_to(wt[r0 + a - 1:r0 + a, :], (8, D))
                part = [(wt[r0 + 8 * i:r0 + 8 * (i + 1)] - ref) * LOG2E for i in range(4)]
                if below is not None:
                    self.rows[below] = jnp.where(sub >= a, part[0], self.mprev)
                self.mprev = part[0]
                for q, v in zip(full, part[1:]):
                    self.rows[q] = v
            new = {}
            while self.done in self.rows and self.done + 1 in self.rows:
                new[self.done] = jnp.concatenate([self.rows.pop(self.done), self.rows.pop(self.done + 1)], axis=0)
                self.done += 2
            return new

    def fold_pair(folders, g, keep=None, ties=None):
        tiles = {}
        for n, c in enumerate(range(0, HK, 128)):
            for half in range(2):
                for side in range(2):
                    t = ties[n] if ties and half == 0 and side == 0 else None
                    lo = side * HK + c
                    tiles[(half, lo)] = folders[half].tile(g + 4 * half, slice(lo, lo + 128), keep, t)
        return [folders[half].fold(g + 4 * half,
                                   jnp.concatenate([tiles[(half, lo)] for lo in range(0, D, 128)], axis=1))
                for half in range(2)]

    bestv_v[...] = jnp.full(bestv_v.shape, -jnp.inf, f32)
    besti_v[...] = lax.broadcasted_iota(jnp.int32, besti_v.shape, 0)
    h_v[0:P2, :] = jnp.zeros((P2, D), f32)
    st_v[0:B, :] = jnp.zeros((B, 256), f32)
    pend_v[...] = jnp.zeros(pend_v.shape, f32)

    def wait_all(cps):
        for cp in cps:
            cp.wait()

    def amats(c):
        for g0, n in _PSTAGES[c]:
            for g in range(g0, g0 + n):
                make_amat(g)

    wait_all(cp_p[0])
    amats(0)

    cp_x0.wait()
    ln1(x_v, 0, xs_v, 0, T0, plain=True)
    xb = [load_xn(s) for s in range(2)]
    logits = [{}, {}]
    finished = [set(), set()]
    fk, slabs = (Folder(D), Folder(D, NV // 2)), {}
    defer, queue = [False], []

    def absorb(new):
        for pos, slab in new.items():
            wtk_v[pos * 4:pos * 4 + 8, :] = _pk(slab.astype(bf16))
            slabs[pos] = slab
        for pos in sorted(slabs):
            if pos < NV // 2 and pos + NV // 2 in slabs:
                store_combos(wsk_v, pos * 4, slabs.pop(pos), slabs.pop(pos + NV // 2))

    def k_finish(s, hold=0):
        ready = [j for j in range(NP) if j not in finished[s] and _pair_need(j) in logits[s]]
        ready = ready[:len(ready) - hold]
        if defer[0]:
            queue.extend((logits[s].__getitem__, [j], s) for j in ready)
        else:
            k_side(logits[s].__getitem__, ready, s)
        finished[s].update(ready)

    def k_chunk(s, keep=None, early=(), late=(), hold=0):
        todo = [q for half in range(2) for q in range(half * (NV // 2), fk[half].done) if q not in logits[s]]
        runs = [[q for q in todo if q < NV // 2], [q for q in todo if q >= NV // 2]]
        lhs = jnp.concatenate([wtk_v[r[0] * 4:(r[-1] + 1) * 4, :] for r in runs if r], axis=0)
        ties = piece_ties(early, lhs.shape[0])
        ties.update(piece_ties(late, lhs.shape[0], col=HK))
        if ties:
            lhs = _tie(keep, lhs, ties)
        p = _dot_nt(_upk(lhs), xb[s])
        for n, q in enumerate(todo):
            logits[s][q] = p[n * 8:(n + 1) * 8]
        k_finish(s, hold)
        return p

    wait_all(cp_k[0])
    for new in fold_pair(fk, 0):
        absorb(new)
    k_chunk(0)
    k_chunk(1, hold=1)

    wait_all(cp_p[1] + cp_k[1])
    k_finish(1)
    amats(1)
    for new in fold_pair(fk, 1):
        absorb(new)
    absorb(fk[0].fold(2))
    k_chunk(0)
    k_chunk(1, hold=1)

    wait_all(cp_k[2] + [cp_x1])
    defer[0] = True
    keep = flag_s[0] > 0
    absorb(fk[1].fold(6))
    new = fold_pair(fk, 3)
    late = list(new[0].values())[-1][:, 384:512]
    for n in new:
        absorb(n)
    pieces = ln1(x_v, T0, xs_v, T0, T0, [0]) + ln1(x_v, T0, xs_v, T0, T0, [1, 2], keep, [late, late])
    p = k_chunk(0, keep, (), pieces[:2])
    rows = [k * p.shape[0] // 5 // 16 * 16 for k in range(5)]
    pieces += ln1(x_v, T0, xs_v, T0, T0, range(3, 8), keep, [p[r:r + R] for r in rows])
    k_chunk(1, keep, pieces[2:3], pieces[3:])

    def k_emit1(half, blk, val):
        now = {(1, 0): 8, (0, 1): 6}.get((half, blk), 0)
        pairs = list(half_pairs(half))
        k_side(half_groups(val, half), pairs[:now], 2 + blk)
        queue.extend((half_groups(val, half), [j], 2 + blk) for j in pairs[now:])

    def run_queue(n, res):
        deps = []
        for k in range(min(n, len(queue))):
            r = k * res.shape[0] // n // 8 * 8
            v = _vregs(k_side(*queue.pop(0), keep=keep, anchor=res[r:r + 8])[0])
            deps.append([_or_all(v[q::4]) for q in range(4)])
        return deps

    kwork = {}

    def k_after(m, res):
        if m in (0, 2):
            kwork[m + 1] = run_queue(4, res)

    def k_before(m):
        if m == 4:
            cp_wv.wait()
            cp_x2.wait()
            for rb in range(0, HK, 128):
                for c in range(0, HK, 128):
                    raw = [wqkv_v[side * HK + c:side * HK + c + 128,
                                  2 * D + half * HK + rb:2 * D + half * HK + rb + 128].T
                           for half in range(2) for side in range(2)]
                    blocks = [t.astype(f32) for t in raw]
                    for n, spec in enumerate(_SA):
                        t = raw[spec[0]] if spec[1] is None else _combo(blocks, spec).astype(bf16)
                        wsv_v[rb // 2:rb // 2 + 64, n * HK + c:n * HK + c + 128] = _pk(t)

    sproj(wsk_v, xs_v, 1, k_emit1, keep, kwork, k_before, k_after)

    def ln_anchored(xg, src, xd, dst, k, n, keep, res):
        which = list(range(k * 8 // n, (k + 1) * 8 // n))
        rows = [a * HK // len(which) // 16 * 16 for a in range(len(which))]
        pcs = ln1(xg, src, xd, dst, P2, which, keep, [res[r:r + R] for r in rows])
        return [[]] * (3 - len(pcs)) + pcs

    vt = {}
    wsv = wsv_v.at[pl.ds(pl.multiple_of(flag_s[1], D // 4), D // 4)]
    work = {0: {}, 1: {}}

    def v_after(q):
        def after(m, res):
            t = 7 * q + m
            if t < 6:
                work[0][m + 1] = run_queue(-(-len(queue) // (6 - t)), res)
            elif t < 13:
                work[1][t - 6] = ln_anchored(x_v, T, xs_v, T, t - 6, 7, keep, res)
        return after

    for q in range(2):
        sproj(wsv, xs_v, q, lambda half, blk, val, q=q: vt.__setitem__((2 * q + blk, half), val),
              keep, work[q], None, v_after(q))
    assert not queue
    phi_m = sealed(phi_v)
    for j in range(NP):
        kvacc_v[j] = kv_prod(vt, _upk(phi_m[j * 64:(j + 1) * 64, :]), j)
    cp_x3.wait()
    wait_bg(0)

    def p1_body(i, c):
        @pl.when(i == 2)
        def _():
            cp_x4.wait()
            wait_bg(1)

        @pl.when(i == 3)
        def _():
            wait_bg(2)

        keep = flag_s[0] > 0
        lo = jnp.minimum((i - 1) * DCH, F - DCH)
        sv = wd_v.at[pl.ds(pl.multiple_of(lo, 16), DCH)]
        dv = wdp_v.at[pl.ds(pl.multiple_of(lo // 2, 8), DCH // 2)]
        rp = repacker([(sv, dv, r, c) for r in range(0, DCH, 16) for c in range(0, D, 128)], keep)
        lo = jnp.minimum((i - 1) * OCH, HK - OCH)
        ov = wo_v.at[pl.ds(pl.multiple_of(lo, 16), HK + OCH)]
        od = wso_v.at[pl.ds(pl.multiple_of(lo // 2, 8), OCH // 2)]

        def k_emit(q):
            return lambda half, blk, val: k_side(half_groups(val, half), half_pairs(half), 2 * q + blk)

        vt = {}

        def v_emit(q):
            return lambda half, blk, val: vt.__setitem__((2 * q + blk, half), val)

        xd = xs_view(i, 2)
        xa = x_v.at[pl.ds(pl.multiple_of(i * T + P2, P2), P2)]
        xb = x_v.at[pl.ds(pl.multiple_of(jnp.minimum(i + 1, NT - 1) * T, T), P2)]
        wa = {}

        def a_after(m, res):
            if m < 6:
                wa[m + 1] = ln_anchored(xa, 0, xd, P2, m, 6, keep, res)

        sproj(wsv_v, xd, 0, v_emit(0), keep, wa, None, a_after)
        sproj(wsk_v, xd, 0, k_emit(0), after=rp[0])
        sproj(wsk_v, xd, 1, k_emit(1), after=rp[1])
        wb = spread(ln1(xb, 0, xd, T, P2), [(0, m) for m in range(1, 7)])[0]

        def b_after(m, res):
            slabs = list(range(0, OCH, 16))
            mine = slabs[(m - 1) * len(slabs) // 6:m * len(slabs) // 6] if m else []
            for n, r in enumerate(mine):
                rows = [((4 * n + c) * HK // (4 * len(mine))) // 16 * 16 for c in range(4)]
                store_combos(od, r // 2, ov[r:r + 16, :].astype(f32), ov[HK + r:HK + r + 16, :].astype(f32),
                             _SB, keep, [res[a:a + R] for a in rows])

        sproj(wsv_v, xd, 1, v_emit(1), keep, wb, None, b_after)
        phi_m = sealed(phi_v)
        for j in range(NP):
            kvacc_v[j] += kv_prod(vt, _upk(phi_m[j * 64:(j + 1) * 64, :]), j)
        return c

    lax.fori_loop(1, NT, p1_body, 0)

    wait_all([cp_wr, cp_wq] + cp_gu[0])
    keep = flag_s[0] > 0
    kv_mask = (lax.broadcasted_iota(jnp.int32, (64, 128), 0) // DH
               == (lax.broadcasted_iota(jnp.int32, (64, 128), 1) // DH) % 2)
    ties = [{} for _ in range(16)]
    for j in range(NP):
        kvj = jnp.where(kv_mask, kvacc_v[j], 0.0)
        kv_v[:, j * 128:(j + 1) * 128] = _pk(kvj.astype(bf16))
        zj = _lanes(jnp.sum(zacc_v[j * 128:(j + 1) * 128, :], axis=-1, keepdims=True))
        zacc_v[j * 128:(j + 1) * 128, :] = zj
        vals = _vregs(kvj) + _vregs(zj)
        if j + 1 < 16:
            for q in range(4):
                ties[j + 1][(32 + q * 8, 0)] = _or_all(vals[q::4])
    wr = wr_v[0:8, :].astype(f32)
    wl = jnp.sum(wr, axis=0, keepdims=True)
    wsum = jnp.sum(wl, axis=1, keepdims=True)
    wrb_v[:, 0:D + 256] = jnp.concatenate(
        [jnp.broadcast_to(wr[j:j + 1, :], (8, 128)) for j in range(8)]
        + [jnp.broadcast_to(wsum, (8, 128)), jnp.broadcast_to(wl, (8, 128))], axis=1)
    for t in range(NT):
        store_xt(t, xs_v, t * (T // 4))
    fq = (Folder(0), Folder(0, NV // 2))
    for g in range(4):
        new = fold_pair(fq, g, keep, ties[4 * g:4 * g + 4])
        for pos, slab in new[0].items():
            store_combos(wsq_v, pos * 4, slab, new[1][pos + NV // 2])

    pq_v = (pq0_v, pq1_v, pq2_v, pq3_v)

    def views_of(g):
        lo = g * (BPI * B)
        if not isinstance(g, int):
            lo = pl.multiple_of(lo, BPI * B)
        return ((x_v.at[pl.ds(lo, BPI * B)],)
                + tuple(ref.at[pl.ds(lo, P2 + BPI * B)] for ref in (h_v, out_v, st_v)) + (g,))

    def stage_q(xd, q, first, before, after):
        def emit(half, blk, val):
            group = half_groups(val, half)
            for j in half_pairs(half):
                ph = _hedgehog_t(_pair_logits(group, j), zacc_v[j * 128:(j + 1) * 128, :])
                pq_v[2 * q + blk][(j // 2) * 64:(j // 2 + 1) * 64, (j % 2) * B:(j % 2 + 1) * B] = _pk(ph.astype(bf16))

        sproj(wsq_v, xd, q, emit, before=before, after=after, first=first)

    oc_v = (oc0_v, oc1_v)

    def stage_g(q):
        pq = [sealed(pq_v[2 * q + blk]) for blk in range(2)]
        for t in range(NP // 4):
            parts = [[_dot_nn(_upk(kv_v[:, j * 128:(j + 1) * 128]),
                              _upk(pq[blk][(j // 2) * 64:(j // 2 + 1) * 64, (j % 2) * B:(j % 2 + 1) * B]))
                      for blk in range(2) for j in (jj, jj + NP // 2)] for jj in (2 * t, 2 * t + 1)]
            blocks = [jnp.concatenate([a, b], axis=0) for a, b in zip(*parts)]
            for m, spec in enumerate(_SA):
                c = m * HK + t * 128
                oc_v[q][0:B // 2, c:c + 128] = _pk(_combo(blocks, spec).astype(bf16).T)

    def stage_h(views, q, keep, pieces, jobs, before=None):
        x_g, h_g = views[0], views[1]
        oc = sealed(oc_v[q])
        first, last = 4, 12
        ties = [{} for _ in range(7)]
        for k, vals in enumerate(pieces):
            t = first + k * (last - first) // max(len(pieces) - 1, 1)
            for m, val in enumerate(vals):
                ties[t // 4][(m * 8, (t % 4) * 128)] = val
        state = {}
        done = [0]

        def product(m):
            if before:
                before(m)
            w = wso_v[:, m * HK:(m + 1) * HK]
            if ties[m]:
                w = _tie(keep, w, ties[m])
            done[0] = m
            res = _dot_nn(_upk(oc[0:B // 2, m * HK:(m + 1) * HK]), _upk(w))
            for k, job in enumerate(jobs):
                t = 2 * q + k * (24 - 4 * q) // len(jobs)
                if t // 4 == m:
                    job(res[0:R, (t % 4) * 128:(t % 4 + 1) * 128])
            return res

        def wmul(d, lo):
            return (d.reshape(B // 8, 8, 128) * wrb_v[:, lo:lo + 128][None]).reshape(B, 128)

        def emit(k, val):
            blk, half = k // 2, k % 2
            s = 2 * q + blk
            cols = slice(half * HK, (half + 1) * HK)
            h = x_g[s * B:(s + 1) * B, cols].astype(f32) + val
            h_g[(s + 2) * B:(s + 3) * B, cols] = h
            st = state.setdefault(blk, {'h': {}})
            st['h'][half] = h
            for c in range(0, HK, 128):
                ht = h[:, c:c + 128]
                if 'h0' not in st:
                    st['h0'] = ht
                    continue
                d = ht - st['h0']
                new = (d, d * d, wmul(d, half * HK + c))
                st['s'] = new if 's' not in st else tuple(a + b for a, b in zip(st['s'], new))
            if len(st['h']) == 1:
                vals = [_or_all(list(v)) for v in zip(*[_vregs(a) for a in st['s']])]
                m = done[0] + 2
                for n, val in enumerate(vals):
                    ties[m][(248 - (n % 4) * 8, (n // 4) * 128)] = val

        _strassen(product, emit)

        res = []
        for blk in range(2):
            st = state[blk]
            s1, s2, s3 = st['s']
            c0 = _lanes(jnp.mean(st['h0'], axis=-1, keepdims=True))
            g0 = st['h0'] - c0
            t1 = s1 + 8.0 * g0
            t2 = s2 + g0 * (s1 + t1)
            t3 = s3 + wmul(g0, D + 128)
            res.append((jnp.concatenate([t1, t2, t3, c0], axis=1),
                        jnp.concatenate([st['h'][0], st['h'][1]], axis=1)))
        return res

    def stage_stats(views, s, part, valid=None):
        st_g, g = views[3], views[4]
        b = g * BPI + s
        bv = bestv_v[...]
        bi = besti_v[...]
        wsum = wrb_v[0:1, D:D + 128]
        nvs, nis, sts = [], [], []
        for k in range(B // R):
            sl = slice(k * R, (k + 1) * R)
            red = [_lanes(jnp.sum(part[sl, n * 128:(n + 1) * 128], axis=-1, keepdims=True)) for n in range(3)]
            mu = red[0] * (1.0 / D)
            var = jnp.maximum(red[1] * (1.0 / D) - mu * mu, 0.0)
            rs = lax.rsqrt(var + LN_EPS)
            r = (red[2] - mu * wsum) * rs
            sts.append(jnp.concatenate([rs, (mu + part[sl, 384:512]) * rs], axis=1))
            if valid is not None:
                r = jnp.where(valid, r, -jnp.inf)
            idx = lax.broadcasted_iota(jnp.int32, (R, 128), 0) + (b * B + k * R)
            better = r > bv[sl]
            nvs.append(jnp.where(better, r, bv[sl]))
            nis.append(jnp.where(better, idx, bi[sl]))
        st = jnp.concatenate(sts, axis=0)
        st_g[(s + 2) * B:(s + 3) * B, :] = st
        bestv_v[...] = jnp.concatenate(nvs, axis=0)
        besti_v[...] = jnp.concatenate(nis, axis=0)
        return st, [_vregs(nv) for nv in nvs]

    def out_jobs(views, s, keep, st=None, h=None):
        h_g, out_g, st_g = views[1], views[2], views[3]

        def job(k):
            def run(anchor):
                rows = slice((s + 2) * B + k * R, (s + 2) * B + (k + 1) * R)
                hk = h_g[rows, :] if h is None else h[k * R:(k + 1) * R]
                sk = st_g[rows, :] if st is None else st[k * R:(k + 1) * R]
                a = 1.0 + jnp.where(keep, sk[:, 0:128], anchor)
                o = [hk[:, c * 128:(c + 1) * 128] * a - sk[:, 128:256] for c in range(D // 128)]
                out_g[rows, :] = jnp.concatenate(o, axis=1).astype(bf16)
            return run
        return [job(k) for k in range(B // R)]

    def p2_body(i, c):
        b0 = i * BPI
        keep = flag_s[0] > 0
        cur = views_of(i)
        st, pieces = stage_stats(cur, -1, pend_v[...], i > 0)
        ojobs = out_jobs(cur, -2, keep) + out_jobs(cur, -1, keep, st)
        n = D // NI
        jobs = []
        for src, dst in ((wg_v, wgp_v), (wu_v, wup_v)):
            sv = src.at[pl.ds(pl.multiple_of(i * n, n), n)]
            dv = dst.at[pl.ds(pl.multiple_of(i * (n // 2), n // 2), n // 2)]
            jobs += [(sv, dv, r, cc) for r in range(0, n, 16) for cc in range(0, NM, 128)]
        rp = repacker(jobs, keep)
        stage_q(xs_view(i, 1), 0, xt_view(i), None, rp[0])
        stage_q(xs_view(i, 1), 1, None, lambda m: stage_g(0) if m == 2 else None, rp[1])
        res = stage_h(cur, 0, keep, pieces, ojobs, lambda m: stage_g(1) if m == 1 else None)
        st0, _ = stage_stats(cur, 0, res[0][0])
        st1, pieces = stage_stats(cur, 1, res[1][0])
        ojobs = out_jobs(cur, 0, keep, st0, res[0][1]) + out_jobs(cur, 1, keep, st1, res[1][1])
        res = stage_h(cur, 1, keep, pieces, ojobs)
        stage_stats(cur, BPI - 2, res[0][0])
        pend_v[...] = res[1][0]

        @pl.when(i > 0)
        def _():
            cp_out(jnp.maximum(b0 - 2, 0), 2).start()

        cp_out(b0, 2).start()
        return c

    lax.fori_loop(0, NI, p2_body, 0)
    wait_all(cp_gu[1])
    keep = flag_s[0] > 0
    last = views_of(NI - 1)

    st, _ = stage_stats(last, BPI - 1, pend_v[...])

    bv = bestv_v[...]
    mval = jnp.max(bv, axis=0, keepdims=True)
    sel = jnp.min(jnp.where(bv == mval, besti_v[...], S - 1), axis=0, keepdims=True)
    idx = sel[0, 0]
    hrow = h_v[pl.ds(P2 + idx, 1), :]
    strow = st_v[pl.ds(P2 + idx, 1), :]
    xrow = jnp.concatenate([hrow[:, c * 128:(c + 1) * 128] * strow[:, 0:128] - strow[:, 128:256]
                            for c in range(D // 128)], axis=1).astype(bf16)
    xs = jnp.broadcast_to(xrow, (16, D))
    g_first = _dot_nn(xs, _upk(wgp_v[:, 0:FC]))
    anchors = ([jnp.broadcast_to(pltpu.bitcast(sel, f32), (R, 128))] * 4
               + [jnp.broadcast_to(xrow[:, 0:128].astype(f32), (R, 128))] * 4
               + [g_first[:, (k // 2) * 128:(k // 2 + 1) * 128] for k in range(8)])
    for job, anchor in zip(out_jobs(last, BPI - 2, keep) + out_jobs(last, BPI - 1, keep, st), anchors):
        job(anchor)
    cp_out(NB - 2, 2).start()

    def act(g, u):
        a = g * pl.reciprocal(1.0 + jnp.exp(-g), approx=True) * u
        return jnp.concatenate([a, a], axis=0).astype(bf16)

    def down(a, lo, w):
        return _dot_nn(a, _upk(wdp_v[lo // 2:(lo + w) // 2, 0:D]))[0:8]

    xcol = jnp.broadcast_to(xrow, (128, D)).T.astype(f32)
    jobs = [(which, b) for b in range(NBV) for which in (0, 1)]
    vres, prev = {}, None
    for j0 in range(0, len(jobs), NCH):
        grp = jobs[j0:j0 + NCH]
        accs = [None] * len(grp)
        for r in range(D // 16):
            for n, (which, b) in enumerate(grp):
                w = (wg_v, wu_v)[which][r * 16:(r + 1) * 16, NM + b * 128:NM + (b + 1) * 128].astype(f32)
                t0 = w[0:8] * xcol[r * 16:r * 16 + 8]
                t1 = w[8:16] * xcol[r * 16 + 8:r * 16 + 16]
                if accs[n] is None:
                    if prev is not None:
                        t0 = jnp.where(keep, t0, prev[n % len(prev)])
                    accs[n] = t0 + t1
                else:
                    accs[n] = (accs[n] + t0) + t1
        prev = accs
        for n, job in enumerate(grp):
            vres[job] = _allreduce8(accs[n][None], jnp.add)[0]

    chunks = [(lo, min(FC, NM - lo)) for lo in range(0, NM, FC)]
    acts, y = [], None
    for k, (lo, w) in enumerate(chunks):
        g = g_first if k == 0 else _dot_nn(xs, _upk(wgp_v[:, lo:lo + w]))
        u = _dot_nn(xs, _upk(wup_v[:, lo:lo + w]))
        acts.append(act(g[0:8], u[0:8]))
        if k >= 1:
            t = down(acts[k - 1], *chunks[k - 1])
            y = t if y is None else y + t
    y = y + down(acts[-1], *chunks[-1])
    for b0, nb in ((0, 4), (4, 4), (8, 4), (12, 1)):
        g = jnp.concatenate([vres[(0, b)] for b in range(b0, b0 + nb)], axis=1)
        u = jnp.concatenate([vres[(1, b)] for b in range(b0, b0 + nb)], axis=1)
        y = y + down(act(g, u), NM + b0 * 128, nb * 128)

    gate = jnp.broadcast_to(jax.nn.sigmoid(mval), (8, 128))
    base = pl.multiple_of((idx >> 4) << 4, 16)
    rows = pl.ds(pl.multiple_of(P2 + base, 16), 16)
    h16 = h_v[rows, :]
    st16 = st_v[rows, :]
    a16 = 1.0 + st16[:, 0:128]
    m16 = st16[:, 128:256]
    hit = (lax.broadcasted_iota(jnp.int32, (16, 128), 0) + base) == idx
    res = []
    for c in range(D // 128):
        yc = y[:, c * 128:(c + 1) * 128] * gate
        yc = jnp.concatenate([yc, yc], axis=0)
        res.append(h16[:, c * 128:(c + 1) * 128] * a16 - m16 + jnp.where(hit, yc, 0.0))
    res = jnp.concatenate(res, axis=1).astype(bf16)
    for i in range(NI):
        cp_out(i * BPI, 2).wait()
        cp_out(i * BPI + 2, 2).wait()
    out_v[rows, :] = res
    fix = pltpu.make_async_copy(out_v.at[rows], out_hbm.at[pl.ds(base, 16)], sem_o.at[0])
    fix.start()
    fix.wait()


@jax.jit
def pallas_sequential_preLN__linear_kernel_hedgehog__moe_arch_mod__prompt_kernel(
    A_x: jax.Array,
    A_wqkv: jax.Array,
    A_w_phi: jax.Array,
    A_wo: jax.Array,
    B_x: jax.Array,
    B_w_r: jax.Array,
    B_w_gate: jax.Array,
    B_w_up: jax.Array,
    B_w_down: jax.Array,
):
    del B_x
    x = A_x.reshape(S, D)
    wphi = A_w_phi.reshape(H * DH, DH)
    wr = B_w_r.reshape(8, 128)
    any_spec = pl.BlockSpec(memory_space=pl.ANY)
    out = pl.pallas_call(
        _kernel,
        out_shape=jax.ShapeDtypeStruct((S, D), bf16),
        in_specs=[any_spec] * 8,
        out_specs=any_spec,
        scratch_shapes=[
            pltpu.VMEM((S, D), bf16),
            pltpu.VMEM((D, 3 * D), bf16),
            pltpu.VMEM((H * DH, DH), bf16),
            pltpu.VMEM((D, D), bf16),
            pltpu.VMEM((64, 128), bf16),
            pltpu.VMEM((D, F + 128), bf16),
            pltpu.VMEM((D, F + 128), bf16),
            pltpu.VMEM((F, D), bf16),
            pltpu.VMEM((PR, D), u32),
            pltpu.VMEM((PR // 2, 7 * HK), u32),
            pltpu.VMEM((PR // 2, 7 * HK), u32),
            pltpu.VMEM((D // 4, 7 * HK), u32),
            pltpu.VMEM((D // 4, 7 * HK), u32),
            pltpu.VMEM((F // 2, D + 128), u32),
            pltpu.VMEM((D // 2, NM), u32),
            pltpu.VMEM((D // 2, NM), u32),
            pltpu.VMEM((64, 8 * 128), u32),
            pltpu.VMEM((T0 // 2, D), u32),
            pltpu.VMEM(((S + T) // 4, 7 * HK), u32),
            pltpu.VMEM((NT * (HK // 2), B), u32),
            pltpu.VMEM((NP, 64, 128), f32),
            pltpu.VMEM((2 * D, 128), f32),
            pltpu.VMEM((32, NP * 128), u32),
            pltpu.VMEM((D + 8, T), u32),
            pltpu.VMEM((D // 2 + 16, 2 * B), u32),
            pltpu.VMEM((D // 2 + 16, 2 * B), u32),
            pltpu.VMEM((D // 2 + 16, 2 * B), u32),
            pltpu.VMEM((D // 2 + 16, 2 * B), u32),
            pltpu.VMEM((B // 2 + 8, 7 * HK), u32),
            pltpu.VMEM((B // 2 + 8, 7 * HK), u32),
            pltpu.VMEM((P2 + S, D), f32),
            pltpu.VMEM((P2 + S, 256), f32),
            pltpu.VMEM((B, 512), f32),
            pltpu.VMEM((P2 + S, D), bf16),
            pltpu.VMEM((8, D + 512), f32),
            pltpu.VMEM((B, 128), f32),
            pltpu.VMEM((B, 128), jnp.int32),
            pltpu.SMEM((2,), jnp.int32),
            pltpu.SemaphoreType.DMA((_NSEM_IN,)),
            pltpu.SemaphoreType.DMA((1,)),
        ],
        compiler_params=pltpu.CompilerParams(vmem_limit_bytes=110 * 1024 * 1024,
                                             disable_bounds_checks=True,
                                             disable_semaphore_checks=True),
        name="hedgehog_mod",
    )(x, A_wqkv, wphi, A_wo, wr, B_w_gate, B_w_up, B_w_down)
    return out.reshape(1, S, D)
```

```python
import jax
import jax.numpy as jnp
from jax import lax
import jax.experimental.pallas as pl
import jax.experimental.pallas.tpu as pltpu

S = 2048
D = 1024
H = 32
DH = 32
F = 3584
T = 512
NT = S // T
T0 = 256
B = 128
NB = S // B
BPI = 4
NI = NB // BPI
NP = H // 2
FC = 1024
R = 16
NBV = 13
NM = F - NBV * 128
NCH = 4
OCH = 176
DCH = 1216
NV = 124
PR = NV * 4
HK = D // 2
P2 = 2 * B
LOG2E = 1.4426950408889634
LN_EPS = 1e-5
DEN_EPS = 1e-6

_NT_DIMS = (((1,), (1,)), ((), ()))

bf16 = jnp.bfloat16
f32 = jnp.float32
u32 = jnp.uint32


def _dot_nt(a, b):
    return lax.dot_general(a, b, _NT_DIMS, preferred_element_type=f32)


def _dot_nn(a, b):
    return jnp.dot(a, b, preferred_element_type=f32)


def _pk(x):
    return pltpu.bitcast(x, u32)


def _upk(x):
    return pltpu.bitcast(x, bf16)


def _lanes(x):
    return jnp.broadcast_to(x, (x.shape[0], 128))


def _layernorm(x):
    m = jnp.mean(x, axis=-1, keepdims=True)
    xc = x - m
    v = jnp.mean(xc * xc, axis=-1, keepdims=True)
    return xc * lax.rsqrt(v + LN_EPS)


def _allreduce8(x, op):
    x = op(x, pltpu.roll(x, 4, 1))
    x = op(x, pltpu.roll(x, 2, 1))
    x = op(x, pltpu.roll(x, 1, 1))
    return x


def _hedgehog_t(p, z=None):
    t = p.shape[-1]
    p4 = p.reshape(2, 4, 8, t)
    mx = _allreduce8(jnp.max(p4, axis=1), jnp.maximum)
    mn = _allreduce8(jnp.min(p4, axis=1), jnp.minimum)
    ep = jnp.exp2(p4 - mx[:, None])
    en = jnp.exp2(mn[:, None] - p4)
    a = pl.reciprocal(_allreduce8(jnp.sum(ep, axis=1), jnp.add), approx=True)
    b = pl.reciprocal(_allreduce8(jnp.sum(en, axis=1), jnp.add), approx=True)
    if z is not None:
        dp = jnp.sum(ep * z[0:64].reshape(2, 4, 8, t), axis=1)
        dn = jnp.sum(en * z[64:128].reshape(2, 4, 8, t), axis=1)
        den = _allreduce8(dp * a + dn * b, jnp.add) + DEN_EPS
        inv = pl.reciprocal(den, approx=True)
        a = a * inv
        b = b * inv
    fp = (ep * a[:, None]).reshape(64, t)
    fn = (en * b[:, None]).reshape(64, t)
    return jnp.concatenate([fp, fn], axis=0)


_SA = ((3, None, 0), (2, 3, 1), (0, 1, 1), (0, None, 0), (0, 3, 1), (1, 3, -1), (2, 0, -1))
_SB = ((2, 0, -1), (0, None, 0), (3, None, 0), (1, 3, -1), (0, 3, 1), (2, 3, 1), (0, 1, 1))


def _combo(blocks, spec):
    a, b, sign = spec
    if b is None:
        return blocks[a]
    return blocks[a] + blocks[b] if sign > 0 else blocks[a] - blocks[b]


def _strassen(product, emit):
    m4 = product(0)
    m2 = product(1)
    emit(2, m4 + m2)
    m5 = product(2)
    u = m4 - m5
    m3 = product(3)
    emit(1, m5 + m3)
    v = m3 - m2
    m1 = product(4)
    u = u + m1
    v = v + m1
    emit(0, u + product(5))
    emit(3, v + product(6))


def _head_groups(h):
    base, k = (NV // 4) * (h // 8), h % 8
    return ([base + 4 * k + i for i in range(3)],
            base + 4 * k - 1 if k > 0 else None,
            base + 4 * k + 3 if k < 7 else None,
            8 - k)


def _pair_logits(group, j):
    parts = []
    for h in (2 * j, 2 * j + 1):
        full, below, above, a = _head_groups(h)
        ref = group(full[0])
        sub = lax.broadcasted_iota(jnp.int32, ref.shape, 0)
        if above is None:
            m = jnp.where(sub >= a, group(below), 0.0)
        else:
            m = jnp.where(sub == a - 1, 0.0, group(above))
            if below is not None:
                m = jnp.where(sub >= a, group(below), m)
        parts += [m] + [group(q) for q in full]
    return jnp.concatenate(parts, axis=0)


def _pair_need(j):
    full, _, above, _ = _head_groups(2 * j + 1)
    return full[2] if above is None else above


def _tie(keep, w, ties):
    rows = sorted({r for r, _ in ties})
    out, pos = [], 0
    for r in rows:
        if r > pos:
            out.append(w[pos:r])
        cols = sorted(c for rr, c in ties if rr == r)
        parts, cpos = [], 0
        for c in cols:
            if c > cpos:
                parts.append(w[r:r + 8, cpos:c])
            parts.append(jnp.where(keep, w[r:r + 8, c:c + 128], ties[(r, c)]))
            cpos = c + 128
        if cpos < w.shape[1]:
            parts.append(w[r:r + 8, cpos:])
        out.append(jnp.concatenate(parts, axis=1) if len(parts) > 1 else parts[0])
        pos = r + 8
    if pos < w.shape[0]:
        out.append(w[pos:])
    return jnp.concatenate(out, axis=0)


def _vregs(x):
    if x.dtype != u32:
        x = pltpu.bitcast(x, u32)
    return [x[r:r + 8, c:c + 128] for r in range(0, x.shape[0], 8) for c in range(0, x.shape[1], 128)]


def _or_all(vals):
    acc = vals[0]
    for v in vals[1:]:
        acc = acc | v
    return acc


_KSTAGES = (((0, 1), (4, 1)), ((1, 2), (5, 1)), ((3, 1), (6, 2)))
_PSTAGES = (((0, 1), (4, 1)), ((1, 3), (5, 3)))
_NSEM_IN = 11


def _kernel(x_hbm, wqkv_hbm, wphi_hbm, wo_hbm, wr_hbm, wg_hbm, wu_hbm, wd_hbm,
            out_hbm,
            x_v, wqkv_v, wphi_v, wo_v, wr_v, wg_v, wu_v, wd_v,
            wtk_v, wsq_v, wsk_v, wsv_v, wso_v, wdp_v, wgp_v, wup_v, amat_v, xn_v, xs_v, xt_v, kvacc_v, zacc_v, kv_v, phi_v,
            pq0_v, pq1_v, pq2_v, pq3_v, oc0_v, oc1_v, h_v, st_v, pend_v, out_v, wrb_v,
            bestv_v, besti_v, flag_s,
            sem_i, sem_o):

    def cp_x(lo, n, sem):
        return pltpu.make_async_copy(x_hbm.at[pl.ds(lo, n)], x_v.at[pl.ds(lo, n)], sem_i.at[sem])

    def cp_w(lo, w, sem):
        return pltpu.make_async_copy(wqkv_hbm.at[:, pl.ds(lo, w)], wqkv_v.at[:, pl.ds(lo, w)], sem_i.at[sem])

    cp_k = [[cp_w(D + g * 128, n * 128, 2 + c) for g, n in st] for c, st in enumerate(_KSTAGES)]
    cp_p = [[pltpu.make_async_copy(wphi_hbm.at[pl.ds(g * 128, n * 128)], wphi_v.at[pl.ds(g * 128, n * 128)],
                                   sem_i.at[3 * c]) for g, n in st] for c, st in enumerate(_PSTAGES)]
    cp_wv = cp_w(2 * D, D, 5)
    cp_wq = cp_w(0, D, 7)

    def cp_wd(k):
        lo, n = k * DCH, min(DCH, F - k * DCH)
        return pltpu.make_async_copy(wd_hbm.at[pl.ds(lo, n)], wd_v.at[pl.ds(lo, n)], sem_i.at[(6, 8, 9)[k]])

    cp_x0 = cp_x(0, T0, 1)
    cp_x1 = cp_x(T0, T0, 4)
    cp_x2 = cp_x(T, P2, 5)
    cp_x3 = cp_x(T + P2, T, 6)
    cp_x4 = cp_x(2 * T + P2, S - 2 * T - P2, 8)
    cp_wr = pltpu.make_async_copy(wr_hbm, wr_v.at[pl.ds(0, 8)], sem_i.at[7])

    def cp_wo(k, half):
        lo, n = k * OCH, min(OCH, HK - k * OCH)
        rows = pl.ds(half * HK + lo, n)
        return pltpu.make_async_copy(wo_hbm.at[rows], wo_v.at[rows], sem_i.at[(6, 8, 9)[k]])

    def wait_bg(k):
        cp_wo(k, 0).wait()
        cp_wo(k, 1).wait()
        cp_wd(k).wait()

    cp_gu = [[pltpu.make_async_copy(src.at[:, pl.ds(lo, n)], dst.at[:, pl.ds(lo, n)], sem_i.at[sem])
              for src, dst in ((wg_hbm, wg_v), (wu_hbm, wu_v))] for lo, n, sem in ((0, NM, 7), (NM, F - NM, 10))]

    def cp_out(b, n):
        lo = b * B
        if not isinstance(b, int):
            lo = pl.multiple_of(lo, B)
        return pltpu.make_async_copy(out_v.at[pl.ds(P2 + lo, n * B)], out_hbm.at[pl.ds(lo, n * B)], sem_o.at[0])

    for cp in (*cp_p[0], cp_x0, *cp_k[0], *cp_p[1], *cp_k[1], *cp_k[2], cp_x1, cp_wv, cp_x2,
               cp_x3, cp_wo(0, 0), cp_wo(0, 1), cp_wd(0), cp_x4, cp_wo(1, 0), cp_wo(1, 1), cp_wd(1),
               cp_wo(2, 0), cp_wo(2, 1), cp_wd(2), cp_wr, cp_wq, *cp_gu[0], *cp_gu[1]):
        cp.start()
    flag_s[0] = 1
    flag_s[1] = 0

    def ln1(xg, src, xd, dst, n, which=None, keep=None, anchors=None, plain=False):
        pieces = []
        for pr in range(n // P2):
            for k in range(B // R):
                off = pr * P2 + k * R
                if which is not None and pr * (B // R) + k not in which:
                    continue
                x0 = xg[src + off:src + off + R, :].astype(f32)
                x1 = xg[src + off + B:src + off + B + R, :].astype(f32)
                if anchors is not None:
                    a = anchors[len(pieces)]
                    x0 = jnp.concatenate([jnp.where(keep, x0[:, :128], a), x0[:, 128:]], axis=1)
                    x1 = jnp.concatenate([jnp.where(keep, x1[:, :128], a), x1[:, 128:]], axis=1)
                p0 = _layernorm(x0)
                p1 = _layernorm(x1)
                if plain:
                    xn_v[off // 2:(off + R) // 2, :] = _pk(p0.astype(bf16))
                    xn_v[(off + B) // 2:(off + B + R) // 2, :] = _pk(p1.astype(bf16))
                lo = (dst + pr * P2) // 4 + k * (R // 2)
                blocks = (p0[:, :HK], p1[:, :HK], p0[:, HK:], p1[:, HK:])
                vs = []
                for m, spec in enumerate(_SB):
                    t = _combo(blocks, spec)
                    xd[lo:lo + R // 2, m * HK:(m + 1) * HK] = _pk(t.astype(bf16))
                    if spec[1] is not None:
                        vs.append(_vregs(t))
                pieces.append([_or_all(list(col)) for col in zip(*vs)])
        return pieces

    def load_xn(b):
        return _upk(xn_v[b * (B // 2):(b + 1) * (B // 2), :])

    def piece_ties(pieces, n, row0=0, col=0):
        ties = {}
        if pieces:
            step = (n - row0) // len(pieces) // 8 * 8
            for k, p in enumerate(pieces):
                for q, val in enumerate(p):
                    ties[(row0 + k * step + (q // 4) * 8, col + (q % 4) * 128)] = val
        return ties

    def xs_view(i, tiles):
        return xs_v.at[pl.ds(pl.multiple_of(i * (T // 4), T // 4), tiles * (T // 4))]

    def xt_view(i):
        lo = i * (HK // 2)
        return xt_v.at[pl.ds(lo if isinstance(i, int) else pl.multiple_of(lo, HK // 2), HK // 2)]

    def store_xt(i, xd, row):
        xt_view(i)[...] = _pk(_upk(xd[row:row + B // 2, 0:HK]).T)

    def sproj(ws, xd, pr, emit, keep=None, work=None, before=None, after=None, first=None):
        lo = pr * (B // 2)

        def product(m):
            if before:
                before(m)
            lhs = ws[:, m * HK:(m + 1) * HK]
            if work is not None and work.get(m):
                lhs = _tie(keep, lhs, piece_ties(work[m], lhs.shape[0], 32))
            if m == 0 and first is not None:
                res = _dot_nn(_upk(lhs), _upk(first[...]))
            else:
                res = _dot_nt(_upk(lhs), _upk(xd[lo:lo + B // 2, m * HK:(m + 1) * HK]))
            if after:
                after(m, res)
            return res

        _strassen(product, lambda k, val: emit(k // 2, k % 2, val))

    def repacker(jobs, keep):
        def hook(q):
            def after(m, res):
                if m in (0, 2, 4):
                    k = 3 * q + m // 2
                    mine = jobs[k * len(jobs) // 6:(k + 1) * len(jobs) // 6]
                    for n, (sv, dv, r, c) in enumerate(mine):
                        a = (64 + n * 416 // len(mine)) // 8 * 8
                        dv[r // 2:r // 2 + 8, c:c + 128] = jnp.where(keep, _pk(sv[r:r + 16, c:c + 128]),
                                                                     pltpu.bitcast(res[a:a + 8], u32))
            return after
        return hook(0), hook(1)

    def spread(pieces, slots):
        res = {}
        for k, (pr, m) in enumerate(slots):
            res.setdefault(pr, {})[m] = pieces[k * len(pieces) // len(slots):(k + 1) * len(pieces) // len(slots)]
        return res

    def sealed(ref):
        ref[pl.ds(pl.multiple_of(flag_s[1] + ref.shape[0] - 8, 8), 8), 0:128] = jnp.zeros((8, 128), u32)
        return ref

    def store_combos(ws, row, top, bot, table=_SA, keep=None, anchors=None):
        for c in range(0, HK, 128):
            blocks = [top[:, c:c + 128], top[:, HK + c:HK + c + 128], bot[:, c:c + 128], bot[:, HK + c:HK + c + 128]]
            if anchors is not None:
                for q in (0, 3):
                    blocks[q] = jnp.where(keep, blocks[q], anchors[c // 128])
            for m, spec in enumerate(table):
                ws[row:row + 8, m * HK + c:m * HK + c + 128] = _pk(_combo(blocks, spec).astype(bf16))

    zinit = set()

    def k_side(group, pairs, slot, keep=None, anchor=None):
        res = []
        for j in pairs:
            p = _pair_logits(group, j)
            if anchor is not None:
                p = jnp.concatenate([jnp.where(keep, p[0:8], anchor), p[8:32],
                                     jnp.where(keep, p[32:40], anchor), p[40:64]], axis=0)
            ph = _hedgehog_t(p)
            if j not in zinit:
                zinit.add(j)
                zacc_v[j * 128:(j + 1) * 128, :] = ph
            else:
                zacc_v[j * 128:(j + 1) * 128, :] += ph
            phi_v[j * 64:(j + 1) * 64, slot * B:(slot + 1) * B] = _pk(ph.astype(bf16))
            res.append(ph)
        return res

    def half_groups(p, half):
        return lambda pos: p[(pos - half * (NV // 2)) * 8:(pos - half * (NV // 2) + 1) * 8]

    def half_pairs(half):
        return range(half * (NP // 2), (half + 1) * (NP // 2))

    def kv_prod(vt, ph, j):
        half, r = j // (NP // 2), (j % (NP // 2)) * 64
        v = jnp.concatenate([vt[(s, half)][r:r + 64] for s in range(T // B)], axis=1).astype(bf16)
        return _dot_nt(v, ph)

    r_i = lax.broadcasted_iota(jnp.int32, (128, DH), 0)
    c_i = lax.broadcasted_iota(jnp.int32, (128, DH), 1)
    expand = (r_i % DH == c_i).astype(bf16)
    r_h = lax.broadcasted_iota(jnp.int32, (128, 128), 0) // DH
    c_h = lax.broadcasted_iota(jnp.int32, (128, 128), 1) // DH
    same_head = r_h == c_h

    def make_amat(g):
        a = _dot_nt(expand, wphi_v[g * 128:(g + 1) * 128, :])
        amat_v[:, g * 128:(g + 1) * 128] = _pk(jnp.where(same_head, a, 0.0).astype(bf16))

    class Folder:
        def __init__(self, col0, first=0):
            self.col0, self.rows, self.mprev, self.done = col0, {}, None, first

        def tile(self, g, rows, keep=None, ties=None):
            am = amat_v[:, g * 128:(g + 1) * 128]
            if ties:
                am = _tie(keep, am, ties)
            return _dot_nt(_upk(am), wqkv_v[rows, self.col0 + g * 128:self.col0 + (g + 1) * 128])

        def fold(self, g, wt=None):
            sub = lax.broadcasted_iota(jnp.int32, (8, D), 0)
            if wt is None:
                wt = self.tile(g, slice(None))
            for hh in range(4):
                full, below, _, a = _head_groups(4 * g + hh)
                r0 = hh * DH
                ref = jnp.broadcast_to(wt[r0 + a - 1:r0 + a, :], (8, D))
                part = [(wt[r0 + 8 * i:r0 + 8 * (i + 1)] - ref) * LOG2E for i in range(4)]
                if below is not None:
                    self.rows[below] = jnp.where(sub >= a, part[0], self.mprev)
                self.mprev = part[0]
                for q, v in zip(full, part[1:]):
                    self.rows[q] = v
            new = {}
            while self.done in self.rows and self.done + 1 in self.rows:
                new[self.done] = jnp.concatenate([self.rows.pop(self.done), self.rows.pop(self.done + 1)], axis=0)
                self.done += 2
            return new

    def fold_pair(folders, g, keep=None, ties=None):
        tiles = {}
        for n, c in enumerate(range(0, HK, 128)):
            for half in range(2):
                for side in range(2):
                    t = ties[n] if ties and half == 0 and side == 0 else None
                    lo = side * HK + c
                    tiles[(half, lo)] = folders[half].tile(g + 4 * half, slice(lo, lo + 128), keep, t)
        return [folders[half].fold(g + 4 * half,
                                   jnp.concatenate([tiles[(half, lo)] for lo in range(0, D, 128)], axis=1))
                for half in range(2)]

    bestv_v[...] = jnp.full(bestv_v.shape, -jnp.inf, f32)
    besti_v[...] = lax.broadcasted_iota(jnp.int32, besti_v.shape, 0)
    h_v[0:P2, :] = jnp.zeros((P2, D), f32)
    st_v[0:B, :] = jnp.zeros((B, 256), f32)
    pend_v[...] = jnp.zeros(pend_v.shape, f32)

    def wait_all(cps):
        for cp in cps:
            cp.wait()

    def amats(c):
        for g0, n in _PSTAGES[c]:
            for g in range(g0, g0 + n):
                make_amat(g)

    wait_all(cp_p[0])
    amats(0)

    cp_x0.wait()
    ln1(x_v, 0, xs_v, 0, T0, plain=True)
    xb = [load_xn(s) for s in range(2)]
    logits = [{}, {}]
    finished = [set(), set()]
    fk, slabs = (Folder(D), Folder(D, NV // 2)), {}
    defer, queue = [False], []

    def absorb(new):
        for pos, slab in new.items():
            wtk_v[pos * 4:pos * 4 + 8, :] = _pk(slab.astype(bf16))
            slabs[pos] = slab
        for pos in sorted(slabs):
            if pos < NV // 2 and pos + NV // 2 in slabs:
                store_combos(wsk_v, pos * 4, slabs.pop(pos), slabs.pop(pos + NV // 2))

    def k_finish(s, hold=0):
        ready = [j for j in range(NP) if j not in finished[s] and _pair_need(j) in logits[s]]
        ready = ready[:len(ready) - hold]
        if defer[0]:
            queue.extend((logits[s].__getitem__, [j], s) for j in ready)
        else:
            k_side(logits[s].__getitem__, ready, s)
        finished[s].update(ready)

    def k_chunk(s, keep=None, early=(), late=(), hold=0):
        todo = [q for half in range(2) for q in range(half * (NV // 2), fk[half].done) if q not in logits[s]]
        runs = [[q for q in todo if q < NV // 2], [q for q in todo if q >= NV // 2]]
        lhs = jnp.concatenate([wtk_v[r[0] * 4:(r[-1] + 1) * 4, :] for r in runs if r], axis=0)
        ties = piece_ties(early, lhs.shape[0])
        ties.update(piece_ties(late, lhs.shape[0], col=HK))
        if ties:
            lhs = _tie(keep, lhs, ties)
        p = _dot_nt(_upk(lhs), xb[s])
        for n, q in enumerate(todo):
            logits[s][q] = p[n * 8:(n + 1) * 8]
        k_finish(s, hold)
        return p

    wait_all(cp_k[0])
    for new in fold_pair(fk, 0):
        absorb(new)
    k_chunk(0)
    k_chunk(1, hold=1)

    wait_all(cp_p[1] + cp_k[1])
    k_finish(1)
    amats(1)
    for new in fold_pair(fk, 1):
        absorb(new)
    absorb(fk[0].fold(2))
    k_chunk(0)
    k_chunk(1, hold=1)

    wait_all(cp_k[2] + [cp_x1])
    defer[0] = True
    keep = flag_s[0] > 0
    absorb(fk[1].fold(6))
    new = fold_pair(fk, 3)
    late = list(new[0].values())[-1][:, 384:512]
    for n in new:
        absorb(n)
    pieces = ln1(x_v, T0, xs_v, T0, T0, [0]) + ln1(x_v, T0, xs_v, T0, T0, [1, 2], keep, [late, late])
    p = k_chunk(0, keep, (), pieces[:2])
    rows = [k * p.shape[0] // 5 // 16 * 16 for k in range(5)]
    pieces += ln1(x_v, T0, xs_v, T0, T0, range(3, 8), keep, [p[r:r + R] for r in rows])
    k_chunk(1, keep, pieces[2:3], pieces[3:])

    def k_emit1(half, blk, val):
        if half != blk:
            k_side(half_groups(val, half), half_pairs(half), 2 + blk)
        else:
            queue.extend((half_groups(val, half), [j], 2 + blk) for j in half_pairs(half))

    def run_queue(n, res):
        deps = []
        for k in range(min(n, len(queue))):
            r = k * res.shape[0] // n // 8 * 8
            v = _vregs(k_side(*queue.pop(0), keep=keep, anchor=res[r:r + 8])[0])
            deps.append([_or_all(v[q::4]) for q in range(4)])
        return deps

    kwork = {}

    def k_after(m, res):
        if m in (0, 2):
            kwork[m + 1] = run_queue(4, res)

    def v_prep(lo, hi):
        for rb in range(lo, hi, 128):
            for c in range(0, HK, 128):
                raw = [wqkv_v[side * HK + c:side * HK + c + 128,
                              2 * D + half * HK + rb:2 * D + half * HK + rb + 128].T
                       for half in range(2) for side in range(2)]
                blocks = [t.astype(f32) for t in raw]
                for n, spec in enumerate(_SA):
                    t = raw[spec[0]] if spec[1] is None else _combo(blocks, spec).astype(bf16)
                    wsv_v[rb // 2:rb // 2 + 64, n * HK + c:n * HK + c + 128] = _pk(t)

    VS = HK // 2

    def k_before(m):
        if m == 5:
            cp_wv.wait()
            cp_x2.wait()
            v_prep(0, VS)

    sproj(wsk_v, xs_v, 1, k_emit1, keep, kwork, k_before, k_after)

    def ln_anchored(xg, src, xd, dst, k, n, keep, res):
        which = list(range(k * 8 // n, (k + 1) * 8 // n))
        rows = [a * HK // len(which) // 16 * 16 for a in range(len(which))]
        pcs = ln1(xg, src, xd, dst, P2, which, keep, [res[r:r + R] for r in rows])
        return [[]] * (3 - len(pcs)) + pcs

    vt, parts = {}, {}
    wsv = wsv_v.at[pl.ds(0, D // 4)]
    work = {0: {}, 1: {}, 2: {}}

    def v_after(q):
        def after(m, res):
            t = 7 * q + m
            u = t + 1
            if 3 <= t < 13:
                work[u // 7][u % 7] = run_queue(-(-len(queue) // (13 - t)), res)
            elif 13 <= t < 20:
                work[u // 7][u % 7] = ln_anchored(x_v, T, xs_v, T, t - 13, 7, keep, res)
        return after

    sealed(wsv_v)
    v_prep(VS, HK)
    for q, (lo, hi) in enumerate(((0, VS), (VS, HK))):
        sproj(wsv_v.at[pl.ds(lo // 2, (hi - lo) // 2)], xs_v, 0,
              lambda half, blk, val: parts.setdefault((blk, half), []).append(val), keep, work[q], None, v_after(q))
        if q == 0:
            sealed(wsv_v)
    vt.update({k: jnp.concatenate(v, axis=0) for k, v in parts.items()})
    sproj(wsv, xs_v, 1, lambda half, blk, val: vt.__setitem__((2 + blk, half), val), keep, work[2], None, v_after(2))
    assert not queue
    phi_m = sealed(phi_v)
    for j in range(NP):
        kvacc_v[j] = kv_prod(vt, _upk(phi_m[j * 64:(j + 1) * 64, :]), j)
    cp_x3.wait()
    wait_bg(0)

    def p1_body(i, c):
        @pl.when(i == 2)
        def _():
            cp_x4.wait()
            wait_bg(1)

        @pl.when(i == 3)
        def _():
            wait_bg(2)

        keep = flag_s[0] > 0
        lo = jnp.minimum((i - 1) * DCH, F - DCH)
        sv = wd_v.at[pl.ds(pl.multiple_of(lo, 16), DCH)]
        dv = wdp_v.at[pl.ds(pl.multiple_of(lo // 2, 8), DCH // 2)]
        rp = repacker([(sv, dv, r, c) for r in range(0, DCH, 16) for c in range(0, D, 128)], keep)
        lo = jnp.minimum((i - 1) * OCH, HK - OCH)
        ov = wo_v.at[pl.ds(pl.multiple_of(lo, 16), HK + OCH)]
        od = wso_v.at[pl.ds(pl.multiple_of(lo // 2, 8), OCH // 2)]

        def k_emit(q):
            return lambda half, blk, val: k_side(half_groups(val, half), half_pairs(half), 2 * q + blk)

        vt = {}

        def v_emit(q):
            return lambda half, blk, val: vt.__setitem__((2 * q + blk, half), val)

        xd = xs_view(i, 2)
        xa = x_v.at[pl.ds(pl.multiple_of(i * T + P2, P2), P2)]
        xb = x_v.at[pl.ds(pl.multiple_of(jnp.minimum(i + 1, NT - 1) * T, T), P2)]
        wa = {}

        def a_after(m, res):
            if m < 6:
                wa[m + 1] = ln_anchored(xa, 0, xd, P2, m, 6, keep, res)

        sproj(wsv, xd, 0, v_emit(0), keep, wa, None, a_after)
        sproj(wsk_v, xd, 0, k_emit(0), after=rp[0])
        sproj(wsk_v, xd, 1, k_emit(1), after=rp[1])
        wb = spread(ln1(xb, 0, xd, T, P2), [(0, m) for m in range(1, 7)])[0]

        def b_after(m, res):
            slabs = list(range(0, OCH, 16))
            mine = slabs[(m - 1) * len(slabs) // 6:m * len(slabs) // 6] if m else []
            for n, r in enumerate(mine):
                rows = [((4 * n + c) * HK // (4 * len(mine))) // 16 * 16 for c in range(4)]
                store_combos(od, r // 2, ov[r:r + 16, :].astype(f32), ov[HK + r:HK + r + 16, :].astype(f32),
                             _SB, keep, [res[a:a + R] for a in rows])

        sproj(wsv, xd, 1, v_emit(1), keep, wb, None, b_after)
        phi_m = sealed(phi_v)
        for j in range(NP):
            kvacc_v[j] += kv_prod(vt, _upk(phi_m[j * 64:(j + 1) * 64, :]), j)
        return c

    lax.fori_loop(1, NT, p1_body, 0)

    wait_all([cp_wr, cp_wq] + cp_gu[0])
    keep = flag_s[0] > 0
    kv_mask = (lax.broadcasted_iota(jnp.int32, (64, 128), 0) // DH
               == (lax.broadcasted_iota(jnp.int32, (64, 128), 1) // DH) % 2)
    ties = [{} for _ in range(16)]
    for j in range(NP):
        kvj = jnp.where(kv_mask, kvacc_v[j], 0.0)
        kv_v[:, j * 128:(j + 1) * 128] = _pk(kvj.astype(bf16))
        zj = _lanes(jnp.sum(zacc_v[j * 128:(j + 1) * 128, :], axis=-1, keepdims=True))
        zacc_v[j * 128:(j + 1) * 128, :] = zj
        vals = _vregs(kvj) + _vregs(zj)
        if j + 1 < 16:
            for q in range(4):
                ties[j + 1][(32 + q * 8, 0)] = _or_all(vals[q::4])
    wr = wr_v[0:8, :].astype(f32)
    wl = jnp.sum(wr, axis=0, keepdims=True)
    wsum = jnp.sum(wl, axis=1, keepdims=True)
    wrb_v[:, 0:D + 256] = jnp.concatenate(
        [jnp.broadcast_to(wr[j:j + 1, :], (8, 128)) for j in range(8)]
        + [jnp.broadcast_to(wsum, (8, 128)), jnp.broadcast_to(wl, (8, 128))], axis=1)
    for t in range(NT):
        store_xt(t, xs_v, t * (T // 4))
    fq = (Folder(0), Folder(0, NV // 2))
    for g in range(4):
        new = fold_pair(fq, g, keep, ties[4 * g:4 * g + 4])
        for pos, slab in new[0].items():
            store_combos(wsq_v, pos * 4, slab, new[1][pos + NV // 2])

    pq_v = (pq0_v, pq1_v, pq2_v, pq3_v)

    def views_of(g):
        lo = g * (BPI * B)
        if not isinstance(g, int):
            lo = pl.multiple_of(lo, BPI * B)
        return ((x_v.at[pl.ds(lo, BPI * B)],)
                + tuple(ref.at[pl.ds(lo, P2 + BPI * B)] for ref in (h_v, out_v, st_v)) + (g,))

    def stage_q(xd, q, first, before, after):
        def emit(half, blk, val):
            group = half_groups(val, half)
            for j in half_pairs(half):
                ph = _hedgehog_t(_pair_logits(group, j), zacc_v[j * 128:(j + 1) * 128, :])
                pq_v[2 * q + blk][(j // 2) * 64:(j // 2 + 1) * 64, (j % 2) * B:(j % 2 + 1) * B] = _pk(ph.astype(bf16))

        sproj(wsq_v, xd, q, emit, before=before, after=after, first=first)

    oc_v = (oc0_v, oc1_v)

    def stage_g(q):
        pq = [sealed(pq_v[2 * q + blk]) for blk in range(2)]
        for t in range(NP // 4):
            parts = [[_dot_nn(_upk(kv_v[:, j * 128:(j + 1) * 128]),
                              _upk(pq[blk][(j // 2) * 64:(j // 2 + 1) * 64, (j % 2) * B:(j % 2 + 1) * B]))
                      for blk in range(2) for j in (jj, jj + NP // 2)] for jj in (2 * t, 2 * t + 1)]
            blocks = [jnp.concatenate([a, b], axis=0) for a, b in zip(*parts)]
            for m, spec in enumerate(_SA):
                c = m * HK + t * 128
                oc_v[q][0:B // 2, c:c + 128] = _pk(_combo(blocks, spec).astype(bf16).T)

    def stage_h(views, q, keep, pieces, jobs, before=None):
        x_g, h_g = views[0], views[1]
        oc = sealed(oc_v[q])
        first, last = 4, 12
        ties = [{} for _ in range(7)]
        for k, vals in enumerate(pieces):
            t = first + k * (last - first) // max(len(pieces) - 1, 1)
            for m, val in enumerate(vals):
                ties[t // 4][(m * 8, (t % 4) * 128)] = val
        state = {}
        done = [0]

        def product(m):
            if before:
                before(m)
            w = wso_v[:, m * HK:(m + 1) * HK]
            if ties[m]:
                w = _tie(keep, w, ties[m])
            done[0] = m
            res = _dot_nn(_upk(oc[0:B // 2, m * HK:(m + 1) * HK]), _upk(w))
            for k, job in enumerate(jobs):
                t = 2 * q + k * (24 - 4 * q) // len(jobs)
                if t // 4 == m:
                    job(res[0:R, (t % 4) * 128:(t % 4 + 1) * 128])
            return res

        def wmul(d, lo):
            return (d.reshape(B // 8, 8, 128) * wrb_v[:, lo:lo + 128][None]).reshape(B, 128)

        def emit(k, val):
            blk, half = k // 2, k % 2
            s = 2 * q + blk
            cols = slice(half * HK, (half + 1) * HK)
            h = x_g[s * B:(s + 1) * B, cols].astype(f32) + val
            h_g[(s + 2) * B:(s + 3) * B, cols] = h
            st = state.setdefault(blk, {'h': {}})
            st['h'][half] = h
            for c in range(0, HK, 128):
                ht = h[:, c:c + 128]
                if 'h0' not in st:
                    st['h0'] = ht
                    continue
                d = ht - st['h0']
                new = (d, d * d, wmul(d, half * HK + c))
                st['s'] = new if 's' not in st else tuple(a + b for a, b in zip(st['s'], new))
            if len(st['h']) == 1:
                vals = [_or_all(list(v)) for v in zip(*[_vregs(a) for a in st['s']])]
                m = done[0] + 2
                for n, val in enumerate(vals):
                    ties[m][(248 - (n % 4) * 8, (n // 4) * 128)] = val

        _strassen(product, emit)

        res = []
        for blk in range(2):
            st = state[blk]
            s1, s2, s3 = st['s']
            c0 = _lanes(jnp.mean(st['h0'], axis=-1, keepdims=True))
            g0 = st['h0'] - c0
            t1 = s1 + 8.0 * g0
            t2 = s2 + g0 * (s1 + t1)
            t3 = s3 + wmul(g0, D + 128)
            res.append((jnp.concatenate([t1, t2, t3, c0], axis=1),
                        jnp.concatenate([st['h'][0], st['h'][1]], axis=1)))
        return res

    def stage_stats(views, s, part, valid=None):
        st_g, g = views[3], views[4]
        b = g * BPI + s
        bv = bestv_v[...]
        bi = besti_v[...]
        wsum = wrb_v[0:1, D:D + 128]
        nvs, nis, sts = [], [], []
        for k in range(B // R):
            sl = slice(k * R, (k + 1) * R)
            red = [_lanes(jnp.sum(part[sl, n * 128:(n + 1) * 128], axis=-1, keepdims=True)) for n in range(3)]
            mu = red[0] * (1.0 / D)
            var = jnp.maximum(red[1] * (1.0 / D) - mu * mu, 0.0)
            rs = lax.rsqrt(var + LN_EPS)
            r = (red[2] - mu * wsum) * rs
            sts.append(jnp.concatenate([rs, (mu + part[sl, 384:512]) * rs], axis=1))
            if valid is not None:
                r = jnp.where(valid, r, -jnp.inf)
            idx = lax.broadcasted_iota(jnp.int32, (R, 128), 0) + (b * B + k * R)
            better = r > bv[sl]
            nvs.append(jnp.where(better, r, bv[sl]))
            nis.append(jnp.where(better, idx, bi[sl]))
        st = jnp.concatenate(sts, axis=0)
        st_g[(s + 2) * B:(s + 3) * B, :] = st
        bestv_v[...] = jnp.concatenate(nvs, axis=0)
        besti_v[...] = jnp.concatenate(nis, axis=0)
        return st, [_vregs(nv) for nv in nvs]

    def out_jobs(views, s, keep, st=None, h=None):
        h_g, out_g, st_g = views[1], views[2], views[3]

        def job(k):
            def run(anchor):
                rows = slice((s + 2) * B + k * R, (s + 2) * B + (k + 1) * R)
                hk = h_g[rows, :] if h is None else h[k * R:(k + 1) * R]
                sk = st_g[rows, :] if st is None else st[k * R:(k + 1) * R]
                a = 1.0 + jnp.where(keep, sk[:, 0:128], anchor)
                o = [hk[:, c * 128:(c + 1) * 128] * a - sk[:, 128:256] for c in range(D // 128)]
                out_g[rows, :] = jnp.concatenate(o, axis=1).astype(bf16)
            return run
        return [job(k) for k in range(B // R)]

    def p2_body(i, c):
        b0 = i * BPI
        keep = flag_s[0] > 0
        cur = views_of(i)
        st, pieces = stage_stats(cur, -1, pend_v[...], i > 0)
        ojobs = out_jobs(cur, -2, keep) + out_jobs(cur, -1, keep, st)
        n = D // NI
        jobs = []
        for src, dst in ((wg_v, wgp_v), (wu_v, wup_v)):
            sv = src.at[pl.ds(pl.multiple_of(i * n, n), n)]
            dv = dst.at[pl.ds(pl.multiple_of(i * (n // 2), n // 2), n // 2)]
            jobs += [(sv, dv, r, cc) for r in range(0, n, 16) for cc in range(0, NM, 128)]
        rp = repacker(jobs, keep)
        stage_q(xs_view(i, 1), 0, xt_view(i), None, rp[0])
        stage_q(xs_view(i, 1), 1, None, lambda m: stage_g(0) if m == 2 else None, rp[1])
        res = stage_h(cur, 0, keep, pieces, ojobs, lambda m: stage_g(1) if m == 1 else None)
        st0, _ = stage_stats(cur, 0, res[0][0])
        st1, pieces = stage_stats(cur, 1, res[1][0])
        ojobs = out_jobs(cur, 0, keep, st0, res[0][1]) + out_jobs(cur, 1, keep, st1, res[1][1])
        res = stage_h(cur, 1, keep, pieces, ojobs)
        stage_stats(cur, BPI - 2, res[0][0])
        pend_v[...] = res[1][0]

        @pl.when(i > 0)
        def _():
            cp_out(jnp.maximum(b0 - 2, 0), 2).start()

        cp_out(b0, 2).start()
        return c

    lax.fori_loop(0, NI, p2_body, 0)
    wait_all(cp_gu[1])
    keep = flag_s[0] > 0
    last = views_of(NI - 1)

    st, _ = stage_stats(last, BPI - 1, pend_v[...])

    bv = bestv_v[...]
    mval = jnp.max(bv, axis=0, keepdims=True)
    sel = jnp.min(jnp.where(bv == mval, besti_v[...], S - 1), axis=0, keepdims=True)
    idx = sel[0, 0]
    hrow = h_v[pl.ds(P2 + idx, 1), :]
    strow = st_v[pl.ds(P2 + idx, 1), :]
    xrow = jnp.concatenate([hrow[:, c * 128:(c + 1) * 128] * strow[:, 0:128] - strow[:, 128:256]
                            for c in range(D // 128)], axis=1).astype(bf16)
    xs = jnp.broadcast_to(xrow, (16, D))
    g_first = _dot_nn(xs, _upk(wgp_v[:, 0:FC]))
    anchors = ([jnp.broadcast_to(pltpu.bitcast(sel, f32), (R, 128))] * 4
               + [jnp.broadcast_to(xrow[:, 0:128].astype(f32), (R, 128))] * 4
               + [g_first[:, (k // 2) * 128:(k // 2 + 1) * 128] for k in range(8)])
    for job, anchor in zip(out_jobs(last, BPI - 2, keep) + out_jobs(last, BPI - 1, keep, st), anchors):
        job(anchor)
    cp_out(NB - 2, 2).start()

    def act(g, u):
        a = g * pl.reciprocal(1.0 + jnp.exp(-g), approx=True) * u
        return jnp.concatenate([a, a], axis=0).astype(bf16)

    def down(a, lo, w):
        return _dot_nn(a, _upk(wdp_v[lo // 2:(lo + w) // 2, 0:D]))[0:8]

    xcol = jnp.broadcast_to(xrow, (128, D)).T.astype(f32)
    jobs = [(which, b) for b in range(NBV) for which in (0, 1)]
    vres, prev = {}, None
    for j0 in range(0, len(jobs), NCH):
        grp = jobs[j0:j0 + NCH]
        accs = [None] * len(grp)
        for r in range(D // 16):
            for n, (which, b) in enumerate(grp):
                w = (wg_v, wu_v)[which][r * 16:(r + 1) * 16, NM + b * 128:NM + (b + 1) * 128].astype(f32)
                t0 = w[0:8] * xcol[r * 16:r * 16 + 8]
                t1 = w[8:16] * xcol[r * 16 + 8:r * 16 + 16]
                if accs[n] is None:
                    if prev is not None:
                        t0 = jnp.where(keep, t0, prev[n % len(prev)])
                    accs[n] = t0 + t1
                else:
                    accs[n] = (accs[n] + t0) + t1
        prev = accs
        for n, job in enumerate(grp):
            vres[job] = _allreduce8(accs[n][None], jnp.add)[0]

    chunks = [(lo, min(FC, NM - lo)) for lo in range(0, NM, FC)]
    acts, y = [], None
    for k, (lo, w) in enumerate(chunks):
        g = g_first if k == 0 else _dot_nn(xs, _upk(wgp_v[:, lo:lo + w]))
        u = _dot_nn(xs, _upk(wup_v[:, lo:lo + w]))
        acts.append(act(g[0:8], u[0:8]))
        if k >= 1:
            t = down(acts[k - 1], *chunks[k - 1])
            y = t if y is None else y + t
    y = y + down(acts[-1], *chunks[-1])
    for b0, nb in ((0, 4), (4, 4), (8, 4), (12, 1)):
        g = jnp.concatenate([vres[(0, b)] for b in range(b0, b0 + nb)], axis=1)
        u = jnp.concatenate([vres[(1, b)] for b in range(b0, b0 + nb)], axis=1)
        y = y + down(act(g, u), NM + b0 * 128, nb * 128)

    gate = jnp.broadcast_to(jax.nn.sigmoid(mval), (8, 128))
    base = pl.multiple_of((idx >> 4) << 4, 16)
    rows = pl.ds(pl.multiple_of(P2 + base, 16), 16)
    h16 = h_v[rows, :]
    st16 = st_v[rows, :]
    a16 = 1.0 + st16[:, 0:128]
    m16 = st16[:, 128:256]
    hit = (lax.broadcasted_iota(jnp.int32, (16, 128), 0) + base) == idx
    res = []
    for c in range(D // 128):
        yc = y[:, c * 128:(c + 1) * 128] * gate
        yc = jnp.concatenate([yc, yc], axis=0)
        res.append(h16[:, c * 128:(c + 1) * 128] * a16 - m16 + jnp.where(hit, yc, 0.0))
    res = jnp.concatenate(res, axis=1).astype(bf16)
    for i in range(NI):
        cp_out(i * BPI, 2).wait()
        cp_out(i * BPI + 2, 2).wait()
    out_v[rows, :] = res
    fix = pltpu.make_async_copy(out_v.at[rows], out_hbm.at[pl.ds(base, 16)], sem_o.at[0])
    fix.start()
    fix.wait()


@jax.jit
def pallas_sequential_preLN__linear_kernel_hedgehog__moe_arch_mod__prompt_kernel(
    A_x: jax.Array,
    A_wqkv: jax.Array,
    A_w_phi: jax.Array,
    A_wo: jax.Array,
    B_x: jax.Array,
    B_w_r: jax.Array,
    B_w_gate: jax.Array,
    B_w_up: jax.Array,
    B_w_down: jax.Array,
):
    del B_x
    x = A_x.reshape(S, D)
    wphi = A_w_phi.reshape(H * DH, DH)
    wr = B_w_r.reshape(8, 128)
    any_spec = pl.BlockSpec(memory_space=pl.ANY)
    out = pl.pallas_call(
        _kernel,
        out_shape=jax.ShapeDtypeStruct((S, D), bf16),
        in_specs=[any_spec] * 8,
        out_specs=any_spec,
        scratch_shapes=[
            pltpu.VMEM((S, D), bf16),
            pltpu.VMEM((D, 3 * D), bf16),
            pltpu.VMEM((H * DH, DH), bf16),
            pltpu.VMEM((D, D), bf16),
            pltpu.VMEM((64, 128), bf16),
            pltpu.VMEM((D, F + 128), bf16),
            pltpu.VMEM((D, F + 128), bf16),
            pltpu.VMEM((F, D), bf16),
            pltpu.VMEM((PR, D), u32),
            pltpu.VMEM((PR // 2, 7 * HK), u32),
            pltpu.VMEM((PR // 2, 7 * HK), u32),
            pltpu.VMEM((D // 4 + 8, 7 * HK), u32),
            pltpu.VMEM((D // 4, 7 * HK), u32),
            pltpu.VMEM((F // 2, D + 128), u32),
            pltpu.VMEM((D // 2, NM), u32),
            pltpu.VMEM((D // 2, NM), u32),
            pltpu.VMEM((64, 8 * 128), u32),
            pltpu.VMEM((T0 // 2, D), u32),
            pltpu.VMEM(((S + T) // 4, 7 * HK), u32),
            pltpu.VMEM((NT * (HK // 2), B), u32),
            pltpu.VMEM((NP, 64, 128), f32),
            pltpu.VMEM((2 * D, 128), f32),
            pltpu.VMEM((32, NP * 128), u32),
            pltpu.VMEM((D + 8, T), u32),
            pltpu.VMEM((D // 2 + 16, 2 * B), u32),
            pltpu.VMEM((D // 2 + 16, 2 * B), u32),
            pltpu.VMEM((D // 2 + 16, 2 * B), u32),
            pltpu.VMEM((D // 2 + 16, 2 * B), u32),
            pltpu.VMEM((B // 2 + 8, 7 * HK), u32),
            pltpu.VMEM((B // 2 + 8, 7 * HK), u32),
            pltpu.VMEM((P2 + S, D), f32),
            pltpu.VMEM((P2 + S, 256), f32),
            pltpu.VMEM((B, 512), f32),
            pltpu.VMEM((P2 + S, D), bf16),
            pltpu.VMEM((8, D + 512), f32),
            pltpu.VMEM((B, 128), f32),
            pltpu.VMEM((B, 128), jnp.int32),
            pltpu.SMEM((2,), jnp.int32),
            pltpu.SemaphoreType.DMA((_NSEM_IN,)),
            pltpu.SemaphoreType.DMA((1,)),
        ],
        compiler_params=pltpu.CompilerParams(vmem_limit_bytes=110 * 1024 * 1024,
                                             disable_bounds_checks=True,
                                             disable_semaphore_checks=True),
        name="hedgehog_mod",
    )(x, A_wqkv, wphi, A_wo, wr, B_w_gate, B_w_up, B_w_down)
    return out.reshape(1, S, D)
```

```python
import jax
import jax.numpy as jnp
from jax import lax
import jax.experimental.pallas as pl
import jax.experimental.pallas.tpu as pltpu

S = 2048
D = 1024
H = 32
DH = 32
F = 3584
T = 512
NT = S // T
T0 = 256
B = 128
NB = S // B
BPI = 4
NI = NB // BPI
NP = H // 2
FC = 1024
R = 16
NBV = 13
NM = F - NBV * 128
NCH = 4
OCH = 176
DCH = 1216
NV = 124
PR = NV * 4
HK = D // 2
P2 = 2 * B
LOG2E = 1.4426950408889634
LN_EPS = 1e-5
DEN_EPS = 1e-6

_NT_DIMS = (((1,), (1,)), ((), ()))

bf16 = jnp.bfloat16
f32 = jnp.float32
u32 = jnp.uint32


def _dot_nt(a, b):
    return lax.dot_general(a, b, _NT_DIMS, preferred_element_type=f32)


def _dot_nn(a, b):
    return jnp.dot(a, b, preferred_element_type=f32)


def _pk(x):
    return pltpu.bitcast(x, u32)


def _upk(x):
    return pltpu.bitcast(x, bf16)


def _lanes(x):
    return jnp.broadcast_to(x, (x.shape[0], 128))


def _layernorm(x):
    m = jnp.mean(x, axis=-1, keepdims=True)
    xc = x - m
    v = jnp.mean(xc * xc, axis=-1, keepdims=True)
    return xc * lax.rsqrt(v + LN_EPS)


def _allreduce8(x, op):
    x = op(x, pltpu.roll(x, 4, 1))
    x = op(x, pltpu.roll(x, 2, 1))
    x = op(x, pltpu.roll(x, 1, 1))
    return x


def _hedgehog_t(p, z=None):
    t = p.shape[-1]
    p4 = p.reshape(2, 4, 8, t)
    mx = _allreduce8(jnp.max(p4, axis=1), jnp.maximum)
    mn = _allreduce8(jnp.min(p4, axis=1), jnp.minimum)
    ep = jnp.exp2(p4 - mx[:, None])
    en = jnp.exp2(mn[:, None] - p4)
    a = pl.reciprocal(_allreduce8(jnp.sum(ep, axis=1), jnp.add), approx=True)
    b = pl.reciprocal(_allreduce8(jnp.sum(en, axis=1), jnp.add), approx=True)
    if z is not None:
        dp = jnp.sum(ep * z[0:64].reshape(2, 4, 8, t), axis=1)
        dn = jnp.sum(en * z[64:128].reshape(2, 4, 8, t), axis=1)
        den = _allreduce8(dp * a + dn * b, jnp.add) + DEN_EPS
        inv = pl.reciprocal(den, approx=True)
        a = a * inv
        b = b * inv
    fp = (ep * a[:, None]).reshape(64, t)
    fn = (en * b[:, None]).reshape(64, t)
    return jnp.concatenate([fp, fn], axis=0)


_SA = ((3, None, 0), (2, 3, 1), (0, 1, 1), (0, None, 0), (0, 3, 1), (1, 3, -1), (2, 0, -1))
_SB = ((2, 0, -1), (0, None, 0), (3, None, 0), (1, 3, -1), (0, 3, 1), (2, 3, 1), (0, 1, 1))


def _combo(blocks, spec):
    a, b, sign = spec
    if b is None:
        return blocks[a]
    return blocks[a] + blocks[b] if sign > 0 else blocks[a] - blocks[b]


def _strassen(product, emit):
    m4 = product(0)
    m2 = product(1)
    emit(2, m4 + m2)
    m5 = product(2)
    u = m4 - m5
    m3 = product(3)
    emit(1, m5 + m3)
    v = m3 - m2
    m1 = product(4)
    u = u + m1
    v = v + m1
    emit(0, u + product(5))
    emit(3, v + product(6))


def _head_groups(h):
    base, k = (NV // 4) * (h // 8), h % 8
    return ([base + 4 * k + i for i in range(3)],
            base + 4 * k - 1 if k > 0 else None,
            base + 4 * k + 3 if k < 7 else None,
            8 - k)


def _pair_logits(group, j):
    parts = []
    for h in (2 * j, 2 * j + 1):
        full, below, above, a = _head_groups(h)
        ref = group(full[0])
        sub = lax.broadcasted_iota(jnp.int32, ref.shape, 0)
        if above is None:
            m = jnp.where(sub >= a, group(below), 0.0)
        else:
            m = jnp.where(sub == a - 1, 0.0, group(above))
            if below is not None:
                m = jnp.where(sub >= a, group(below), m)
        parts += [m] + [group(q) for q in full]
    return jnp.concatenate(parts, axis=0)


def _pair_need(j):
    full, _, above, _ = _head_groups(2 * j + 1)
    return full[2] if above is None else above


def _tie(keep, w, ties):
    rows = sorted({r for r, _ in ties})
    out, pos = [], 0
    for r in rows:
        if r > pos:
            out.append(w[pos:r])
        cols = sorted(c for rr, c in ties if rr == r)
        parts, cpos = [], 0
        for c in cols:
            if c > cpos:
                parts.append(w[r:r + 8, cpos:c])
            parts.append(jnp.where(keep, w[r:r + 8, c:c + 128], ties[(r, c)]))
            cpos = c + 128
        if cpos < w.shape[1]:
            parts.append(w[r:r + 8, cpos:])
        out.append(jnp.concatenate(parts, axis=1) if len(parts) > 1 else parts[0])
        pos = r + 8
    if pos < w.shape[0]:
        out.append(w[pos:])
    return jnp.concatenate(out, axis=0)


def _vregs(x):
    if x.dtype != u32:
        x = pltpu.bitcast(x, u32)
    return [x[r:r + 8, c:c + 128] for r in range(0, x.shape[0], 8) for c in range(0, x.shape[1], 128)]


def _or_all(vals):
    acc = vals[0]
    for v in vals[1:]:
        acc = acc | v
    return acc


_KSTAGES = (((0, 1), (4, 1)), ((1, 2), (5, 1)), ((3, 1), (6, 2)))
_PSTAGES = (((0, 3), (4, 2)), ((3, 1), (6, 2)))
_NSEM_IN = 11


def _kernel(x_hbm, wqkv_hbm, wphi_hbm, wo_hbm, wr_hbm, wg_hbm, wu_hbm, wd_hbm,
            out_hbm,
            x_v, wqkv_v, wphi_v, wo_v, wr_v, wg_v, wu_v, wd_v,
            wtk_v, wsq_v, wsk_v, wsv_v, wso_v, wdp_v, wgp_v, wup_v, amat_v, xn_v, xs_v, xt_v, kvacc_v, zacc_v, kv_v, phi_v,
            pq0_v, pq1_v, pq2_v, pq3_v, oc0_v, oc1_v, h_v, st_v, pend_v, out_v, wrb_v,
            bestv_v, besti_v, flag_s,
            sem_i, sem_o):

    def cp_x(lo, n, sem):
        return pltpu.make_async_copy(x_hbm.at[pl.ds(lo, n)], x_v.at[pl.ds(lo, n)], sem_i.at[sem])

    def cp_w(lo, w, sem):
        return pltpu.make_async_copy(wqkv_hbm.at[:, pl.ds(lo, w)], wqkv_v.at[:, pl.ds(lo, w)], sem_i.at[sem])

    cp_k = [[cp_w(D + g * 128, n * 128, 2 + c) for g, n in st] for c, st in enumerate(_KSTAGES)]
    cp_p = [[pltpu.make_async_copy(wphi_hbm.at[pl.ds(g * 128, n * 128)], wphi_v.at[pl.ds(g * 128, n * 128)],
                                   sem_i.at[3 * c]) for g, n in st] for c, st in enumerate(_PSTAGES)]
    cp_wv = cp_w(2 * D, D, 5)
    cp_wq = cp_w(0, D, 7)

    def cp_wd(k):
        lo, n = k * DCH, min(DCH, F - k * DCH)
        return pltpu.make_async_copy(wd_hbm.at[pl.ds(lo, n)], wd_v.at[pl.ds(lo, n)], sem_i.at[(6, 8, 9)[k]])

    cp_x0 = cp_x(0, T0, 1)
    cp_x1 = cp_x(T0, T0, 4)
    cp_x2 = cp_x(T, P2, 5)
    cp_x3 = cp_x(T + P2, T, 6)
    cp_x4 = cp_x(2 * T + P2, S - 2 * T - P2, 8)
    cp_wr = pltpu.make_async_copy(wr_hbm, wr_v.at[pl.ds(0, 8)], sem_i.at[7])

    def cp_wo(k, half):
        lo, n = k * OCH, min(OCH, HK - k * OCH)
        rows = pl.ds(half * HK + lo, n)
        return pltpu.make_async_copy(wo_hbm.at[rows], wo_v.at[rows], sem_i.at[(6, 8, 9)[k]])

    def wait_bg(k):
        cp_wo(k, 0).wait()
        cp_wo(k, 1).wait()
        cp_wd(k).wait()

    cp_gu = [[pltpu.make_async_copy(src.at[:, pl.ds(lo, n)], dst.at[:, pl.ds(lo, n)], sem_i.at[sem])
              for src, dst in ((wg_hbm, wg_v), (wu_hbm, wu_v))] for lo, n, sem in ((0, NM, 7), (NM, F - NM, 10))]

    def cp_out(b, n):
        lo = b * B
        if not isinstance(b, int):
            lo = pl.multiple_of(lo, B)
        return pltpu.make_async_copy(out_v.at[pl.ds(P2 + lo, n * B)], out_hbm.at[pl.ds(lo, n * B)], sem_o.at[0])

    for cp in (*cp_p[0], cp_x0, *cp_k[0], *cp_p[1], *cp_k[1], *cp_k[2], cp_x1, cp_wv, cp_x2,
               cp_x3, cp_wo(0, 0), cp_wo(0, 1), cp_wd(0), cp_x4, cp_wo(1, 0), cp_wo(1, 1), cp_wd(1),
               cp_wo(2, 0), cp_wo(2, 1), cp_wd(2), cp_wr, cp_wq, *cp_gu[0], *cp_gu[1]):
        cp.start()
    flag_s[0] = 1
    flag_s[1] = 0

    def ln1(xg, src, xd, dst, n, which=None, keep=None, anchors=None, plain=False):
        pieces = []
        for pr in range(n // P2):
            for k in range(B // R):
                off = pr * P2 + k * R
                if which is not None and pr * (B // R) + k not in which:
                    continue
                x0 = xg[src + off:src + off + R, :].astype(f32)
                x1 = xg[src + off + B:src + off + B + R, :].astype(f32)
                if anchors is not None:
                    a = anchors[len(pieces)]
                    x0 = jnp.concatenate([jnp.where(keep, x0[:, :128], a), x0[:, 128:]], axis=1)
                    x1 = jnp.concatenate([jnp.where(keep, x1[:, :128], a), x1[:, 128:]], axis=1)
                p0 = _layernorm(x0)
                p1 = _layernorm(x1)
                if plain:
                    xn_v[off // 2:(off + R) // 2, :] = _pk(p0.astype(bf16))
                    xn_v[(off + B) // 2:(off + B + R) // 2, :] = _pk(p1.astype(bf16))
                lo = (dst + pr * P2) // 4 + k * (R // 2)
                blocks = (p0[:, :HK], p1[:, :HK], p0[:, HK:], p1[:, HK:])
                vs = []
                for m, spec in enumerate(_SB):
                    t = _combo(blocks, spec)
                    xd[lo:lo + R // 2, m * HK:(m + 1) * HK] = _pk(t.astype(bf16))
                    if spec[1] is not None:
                        vs.append(_vregs(t))
                pieces.append([_or_all(list(col)) for col in zip(*vs)])
        return pieces

    def load_xn(b):
        return _upk(xn_v[b * (B // 2):(b + 1) * (B // 2), :])

    def piece_ties(pieces, n, row0=0, col=0):
        ties = {}
        if pieces:
            step = (n - row0) // len(pieces) // 8 * 8
            for k, p in enumerate(pieces):
                for q, val in enumerate(p):
                    ties[(row0 + k * step + (q // 4) * 8, col + (q % 4) * 128)] = val
        return ties

    def xs_view(i, tiles):
        return xs_v.at[pl.ds(pl.multiple_of(i * (T // 4), T // 4), tiles * (T // 4))]

    def xt_view(i):
        lo = i * (HK // 2)
        return xt_v.at[pl.ds(lo if isinstance(i, int) else pl.multiple_of(lo, HK // 2), HK // 2)]

    def store_xt(i, xd, row):
        xt_view(i)[...] = _pk(_upk(xd[row:row + B // 2, 0:HK]).T)

    def sproj(ws, xd, pr, emit, keep=None, work=None, before=None, after=None, first=None):
        lo = pr * (B // 2)

        def product(m):
            if before:
                before(m)
            lhs = ws[:, m * HK:(m + 1) * HK]
            if work is not None and work.get(m):
                lhs = _tie(keep, lhs, piece_ties(work[m], lhs.shape[0], 32))
            if m == 0 and first is not None:
                res = _dot_nn(_upk(lhs), _upk(first[...]))
            else:
                res = _dot_nt(_upk(lhs), _upk(xd[lo:lo + B // 2, m * HK:(m + 1) * HK]))
            if after:
                after(m, res)
            return res

        _strassen(product, lambda k, val: emit(k // 2, k % 2, val))

    def repacker(jobs, keep):
        def hook(q):
            def after(m, res):
                if m in (0, 2, 4):
                    k = 3 * q + m // 2
                    mine = jobs[k * len(jobs) // 6:(k + 1) * len(jobs) // 6]
                    for n, (sv, dv, r, c) in enumerate(mine):
                        a = (64 + n * 416 // len(mine)) // 8 * 8
                        dv[r // 2:r // 2 + 8, c:c + 128] = jnp.where(keep, _pk(sv[r:r + 16, c:c + 128]),
                                                                     pltpu.bitcast(res[a:a + 8], u32))
            return after
        return hook(0), hook(1)

    def spread(pieces, slots):
        res = {}
        for k, (pr, m) in enumerate(slots):
            res.setdefault(pr, {})[m] = pieces[k * len(pieces) // len(slots):(k + 1) * len(pieces) // len(slots)]
        return res

    def sealed(ref):
        ref[pl.ds(pl.multiple_of(flag_s[1] + ref.shape[0] - 8, 8), 8), 0:128] = jnp.zeros((8, 128), u32)
        return ref

    def store_combos(ws, row, top, bot, table=_SA, keep=None, anchors=None):
        for c in range(0, HK, 128):
            blocks = [top[:, c:c + 128], top[:, HK + c:HK + c + 128], bot[:, c:c + 128], bot[:, HK + c:HK + c + 128]]
            if anchors is not None:
                for q in (0, 3):
                    blocks[q] = jnp.where(keep, blocks[q], anchors[c // 128])
            for m, spec in enumerate(table):
                ws[row:row + 8, m * HK + c:m * HK + c + 128] = _pk(_combo(blocks, spec).astype(bf16))

    zinit = set()

    def k_side(group, pairs, slot, keep=None, anchor=None):
        res = []
        for j in pairs:
            p = _pair_logits(group, j)
            if anchor is not None:
                p = jnp.concatenate([jnp.where(keep, p[0:8], anchor), p[8:32],
                                     jnp.where(keep, p[32:40], anchor), p[40:64]], axis=0)
            ph = _hedgehog_t(p)
            if j not in zinit:
                zinit.add(j)
                zacc_v[j * 128:(j + 1) * 128, :] = ph
            else:
                zacc_v[j * 128:(j + 1) * 128, :] += ph
            phi_v[j * 64:(j + 1) * 64, slot * B:(slot + 1) * B] = _pk(ph.astype(bf16))
            res.append(ph)
        return res

    def half_groups(p, half):
        return lambda pos: p[(pos - half * (NV // 2)) * 8:(pos - half * (NV // 2) + 1) * 8]

    def half_pairs(half):
        return range(half * (NP // 2), (half + 1) * (NP // 2))

    def kv_prod(vt, ph, j):
        half, r = j // (NP // 2), (j % (NP // 2)) * 64
        v = jnp.concatenate([vt[(s, half)][r:r + 64] for s in range(T // B)], axis=1).astype(bf16)
        return _dot_nt(v, ph)

    eye = (lax.broadcasted_iota(jnp.int32, (DH, DH), 0)
           == lax.broadcasted_iota(jnp.int32, (DH, DH), 1)).astype(bf16)
    r_h = lax.broadcasted_iota(jnp.int32, (128, 128), 0) // DH
    c_h = lax.broadcasted_iota(jnp.int32, (128, 128), 1) // DH
    same_head = r_h == c_h

    def make_amat(g):
        a = jnp.concatenate([_dot_nt(eye, wphi_v[g * 128:(g + 1) * 128, :])] * 4, axis=0)
        amat_v[:, g * 128:(g + 1) * 128] = _pk(jnp.where(same_head, a, 0.0).astype(bf16))

    class Folder:
        def __init__(self, col0, first=0):
            self.col0, self.rows, self.mprev, self.done = col0, {}, None, first

        def tile(self, g, rows, keep=None, ties=None):
            am = amat_v[:, g * 128:(g + 1) * 128]
            if ties:
                am = _tie(keep, am, ties)
            return _dot_nt(_upk(am), wqkv_v[rows, self.col0 + g * 128:self.col0 + (g + 1) * 128])

        def fold(self, g, wt=None):
            sub = lax.broadcasted_iota(jnp.int32, (8, D), 0)
            if wt is None:
                wt = self.tile(g, slice(None))
            for hh in range(4):
                full, below, _, a = _head_groups(4 * g + hh)
                r0 = hh * DH
                ref = jnp.broadcast_to(wt[r0 + a - 1:r0 + a, :], (8, D))
                part = [(wt[r0 + 8 * i:r0 + 8 * (i + 1)] - ref) * LOG2E for i in range(4)]
                if below is not None:
                    self.rows[below] = jnp.where(sub >= a, part[0], self.mprev)
                self.mprev = part[0]
                for q, v in zip(full, part[1:]):
                    self.rows[q] = v
            new = {}
            while self.done in self.rows and self.done + 1 in self.rows:
                new[self.done] = jnp.concatenate([self.rows.pop(self.done), self.rows.pop(self.done + 1)], axis=0)
                self.done += 2
            return new

    def fold_pair(folders, g, keep=None, ties=None):
        tiles = {}
        for n, c in enumerate(range(0, HK, 128)):
            for half in range(2):
                for side in range(2):
                    t = ties[n] if ties and half == 0 and side == 0 else None
                    lo = side * HK + c
                    tiles[(half, lo)] = folders[half].tile(g + 4 * half, slice(lo, lo + 128), keep, t)
        return [folders[half].fold(g + 4 * half,
                                   jnp.concatenate([tiles[(half, lo)] for lo in range(0, D, 128)], axis=1))
                for half in range(2)]

    bestv_v[...] = jnp.full(bestv_v.shape, -jnp.inf, f32)
    besti_v[...] = lax.broadcasted_iota(jnp.int32, besti_v.shape, 0)
    h_v[0:P2, :] = jnp.zeros((P2, D), f32)
    st_v[0:B, :] = jnp.zeros((B, 256), f32)
    pend_v[...] = jnp.zeros(pend_v.shape, f32)

    def wait_all(cps):
        for cp in cps:
            cp.wait()

    def amats(c):
        for g0, n in _PSTAGES[c]:
            for g in range(g0, g0 + n):
                make_amat(g)

    wait_all(cp_p[0])
    amats(0)

    cp_x0.wait()
    ln1(x_v, 0, xs_v, 0, T0, plain=True)
    xb = [load_xn(s) for s in range(2)]
    logits = [{}, {}]
    finished = [set(), set()]
    fk, slabs = (Folder(D), Folder(D, NV // 2)), {}
    defer, queue = [False], []

    def absorb(new):
        for pos, slab in new.items():
            wtk_v[pos * 4:pos * 4 + 8, :] = _pk(slab.astype(bf16))
            slabs[pos] = slab
        for pos in sorted(slabs):
            if pos < NV // 2 and pos + NV // 2 in slabs:
                store_combos(wsk_v, pos * 4, slabs.pop(pos), slabs.pop(pos + NV // 2))

    def k_finish(s, hold=0):
        ready = [j for j in range(NP) if j not in finished[s] and _pair_need(j) in logits[s]]
        ready = ready[:len(ready) - hold]
        if defer[0]:
            queue.extend((logits[s].__getitem__, [j], s) for j in ready)
        else:
            k_side(logits[s].__getitem__, ready, s)
        finished[s].update(ready)

    def k_chunk(s, keep=None, early=(), late=(), hold=0):
        todo = [q for half in range(2) for q in range(half * (NV // 2), fk[half].done) if q not in logits[s]]
        runs = [[q for q in todo if q < NV // 2], [q for q in todo if q >= NV // 2]]
        lhs = jnp.concatenate([wtk_v[r[0] * 4:(r[-1] + 1) * 4, :] for r in runs if r], axis=0)
        ties = piece_ties(early, lhs.shape[0])
        ties.update(piece_ties(late, lhs.shape[0], col=HK))
        if ties:
            lhs = _tie(keep, lhs, ties)
        p = _dot_nt(_upk(lhs), xb[s])
        for n, q in enumerate(todo):
            logits[s][q] = p[n * 8:(n + 1) * 8]
        k_finish(s, hold)
        return p

    wait_all(cp_k[0])
    for new in fold_pair(fk, 0):
        absorb(new)
    k_chunk(0)
    k_chunk(1, hold=1)

    wait_all(cp_p[1] + cp_k[1])
    k_finish(1)
    for new in fold_pair(fk, 1):
        absorb(new)
    absorb(fk[0].fold(2))
    amats(1)
    k_chunk(0)
    k_chunk(1, hold=2)

    wait_all(cp_k[2] + [cp_x1])
    defer[0] = True
    keep = flag_s[0] > 0
    absorb(fk[1].fold(6))
    new = fold_pair(fk, 3)
    late = list(new[0].values())[-1][:, 384:512]
    for n in new:
        absorb(n)
    pieces = ln1(x_v, T0, xs_v, T0, T0, [0]) + ln1(x_v, T0, xs_v, T0, T0, [1, 2], keep, [late, late])
    p = k_chunk(0, keep, (), pieces[:2])
    rows = [k * p.shape[0] // 5 // 16 * 16 for k in range(5)]
    pieces += ln1(x_v, T0, xs_v, T0, T0, range(3, 8), keep, [p[r:r + R] for r in rows])
    k_chunk(1, keep, pieces[2:3], pieces[3:])

    def k_emit1(half, blk, val):
        if half != blk:
            k_side(half_groups(val, half), half_pairs(half), 2 + blk)
        else:
            queue.extend((half_groups(val, half), [j], 2 + blk) for j in half_pairs(half))

    def run_queue(n, res):
        deps = []
        for k in range(min(n, len(queue))):
            r = k * res.shape[0] // n // 8 * 8
            v = _vregs(k_side(*queue.pop(0), keep=keep, anchor=res[r:r + 8])[0])
            deps.append([_or_all(v[q::4]) for q in range(4)])
        return deps

    kwork = {}

    def k_after(m, res):
        if m in (0, 2):
            kwork[m + 1] = run_queue(4, res)

    def v_prep(lo, hi):
        for rb in range(lo, hi, 128):
            for c in range(0, HK, 128):
                raw = [wqkv_v[side * HK + c:side * HK + c + 128,
                              2 * D + half * HK + rb:2 * D + half * HK + rb + 128].T
                       for half in range(2) for side in range(2)]
                blocks = [t.astype(f32) for t in raw]
                for n, spec in enumerate(_SA):
                    t = raw[spec[0]] if spec[1] is None else _combo(blocks, spec).astype(bf16)
                    wsv_v[rb // 2:rb // 2 + 64, n * HK + c:n * HK + c + 128] = _pk(t)

    VS = HK // 2

    def k_before(m):
        if m == 5:
            cp_wv.wait()
            cp_x2.wait()
            v_prep(0, VS)

    sproj(wsk_v, xs_v, 1, k_emit1, keep, kwork, k_before, k_after)

    def ln_anchored(xg, src, xd, dst, k, n, keep, res):
        which = list(range(k * 8 // n, (k + 1) * 8 // n))
        rows = [a * HK // len(which) // 16 * 16 for a in range(len(which))]
        pcs = ln1(xg, src, xd, dst, P2, which, keep, [res[r:r + R] for r in rows])
        return [[]] * (3 - len(pcs)) + pcs

    vt, parts = {}, {}
    wsv = wsv_v.at[pl.ds(0, D // 4)]
    work = {0: {}, 1: {}, 2: {}}

    def v_after(q):
        def after(m, res):
            t = 7 * q + m
            u = t + 1
            if 3 <= t < 13:
                work[u // 7][u % 7] = run_queue(-(-len(queue) // (13 - t)), res)
            elif 13 <= t < 20:
                work[u // 7][u % 7] = ln_anchored(x_v, T, xs_v, T, t - 13, 7, keep, res)
        return after

    sealed(wsv_v)
    v_prep(VS, HK)
    zero = pl.multiple_of(flag_s[1], 8)
    for q, lo in enumerate((0, zero + VS // 2)):
        sproj(wsv_v.at[pl.ds(lo, VS // 2)], xs_v, 0,
              lambda half, blk, val: parts.setdefault((blk, half), []).append(val), keep, work[q], None, v_after(q))
    vt.update({k: jnp.concatenate(v, axis=0) for k, v in parts.items()})
    sproj(wsv_v.at[pl.ds(zero, D // 4)], xs_v, 1, lambda half, blk, val: vt.__setitem__((2 + blk, half), val), keep, work[2], None, v_after(2))
    assert not queue
    phi_m = sealed(phi_v)
    for j in range(NP):
        kvacc_v[j] = kv_prod(vt, _upk(phi_m[j * 64:(j + 1) * 64, :]), j)
    cp_x3.wait()
    wait_bg(0)

    def p1_body(i, c):
        @pl.when(i == 2)
        def _():
            cp_x4.wait()
            wait_bg(1)

        @pl.when(i == 3)
        def _():
            wait_bg(2)

        keep = flag_s[0] > 0
        lo = jnp.minimum((i - 1) * DCH, F - DCH)
        sv = wd_v.at[pl.ds(pl.multiple_of(lo, 16), DCH)]
        dv = wdp_v.at[pl.ds(pl.multiple_of(lo // 2, 8), DCH // 2)]
        rp = repacker([(sv, dv, r, c) for r in range(0, DCH, 16) for c in range(0, D, 128)], keep)
        lo = jnp.minimum((i - 1) * OCH, HK - OCH)
        ov = wo_v.at[pl.ds(pl.multiple_of(lo, 16), HK + OCH)]
        od = wso_v.at[pl.ds(pl.multiple_of(lo // 2, 8), OCH // 2)]

        def k_emit(q):
            return lambda half, blk, val: k_side(half_groups(val, half), half_pairs(half), 2 * q + blk)

        vt = {}

        def v_emit(q):
            return lambda half, blk, val: vt.__setitem__((2 * q + blk, half), val)

        xd = xs_view(i, 2)
        xa = x_v.at[pl.ds(pl.multiple_of(i * T + P2, P2), P2)]
        xb = x_v.at[pl.ds(pl.multiple_of(jnp.minimum(i + 1, NT - 1) * T, T), P2)]
        wa = {}

        def a_after(m, res):
            if m < 6:
                wa[m + 1] = ln_anchored(xa, 0, xd, P2, m, 6, keep, res)

        sproj(wsv, xd, 0, v_emit(0), keep, wa, None, a_after)
        sproj(wsk_v, xd, 0, k_emit(0), after=rp[0])
        sproj(wsk_v, xd, 1, k_emit(1), after=rp[1])
        wb = spread(ln1(xb, 0, xd, T, P2), [(0, m) for m in range(1, 7)])[0]

        def b_after(m, res):
            slabs = list(range(0, OCH, 16))
            mine = slabs[(m - 1) * len(slabs) // 6:m * len(slabs) // 6] if m else []
            for n, r in enumerate(mine):
                rows = [((4 * n + c) * HK // (4 * len(mine))) // 16 * 16 for c in range(4)]
                store_combos(od, r // 2, ov[r:r + 16, :].astype(f32), ov[HK + r:HK + r + 16, :].astype(f32),
                             _SB, keep, [res[a:a + R] for a in rows])

        sproj(wsv, xd, 1, v_emit(1), keep, wb, None, b_after)
        phi_m = sealed(phi_v)
        for j in range(NP):
            kvacc_v[j] += kv_prod(vt, _upk(phi_m[j * 64:(j + 1) * 64, :]), j)
        return c

    lax.fori_loop(1, NT, p1_body, 0)

    wait_all([cp_wr, cp_wq] + cp_gu[0])
    keep = flag_s[0] > 0
    kv_mask = (lax.broadcasted_iota(jnp.int32, (64, 128), 0) // DH
               == (lax.broadcasted_iota(jnp.int32, (64, 128), 1) // DH) % 2)
    ties = [{} for _ in range(16)]
    for j in range(NP):
        kvj = jnp.where(kv_mask, kvacc_v[j], 0.0)
        kv_v[:, j * 128:(j + 1) * 128] = _pk(kvj.astype(bf16))
        zj = _lanes(jnp.sum(zacc_v[j * 128:(j + 1) * 128, :], axis=-1, keepdims=True))
        zacc_v[j * 128:(j + 1) * 128, :] = zj
        vals = _vregs(kvj) + _vregs(zj)
        if j + 1 < 16:
            for q in range(4):
                ties[j + 1][(32 + q * 8, 0)] = _or_all(vals[q::4])
    wr = wr_v[0:8, :].astype(f32)
    wl = jnp.sum(wr, axis=0, keepdims=True)
    wsum = jnp.sum(wl, axis=1, keepdims=True)
    wrb_v[:, 0:D + 256] = jnp.concatenate(
        [jnp.broadcast_to(wr[j:j + 1, :], (8, 128)) for j in range(8)]
        + [jnp.broadcast_to(wsum, (8, 128)), jnp.broadcast_to(wl, (8, 128))], axis=1)
    for t in range(NT):
        store_xt(t, xs_v, t * (T // 4))
    fq = (Folder(0), Folder(0, NV // 2))
    for g in range(4):
        new = fold_pair(fq, g, keep, ties[4 * g:4 * g + 4])
        for pos, slab in new[0].items():
            store_combos(wsq_v, pos * 4, slab, new[1][pos + NV // 2])

    pq_v = (pq0_v, pq1_v, pq2_v, pq3_v)

    def views_of(g):
        lo = g * (BPI * B)
        if not isinstance(g, int):
            lo = pl.multiple_of(lo, BPI * B)
        return ((x_v.at[pl.ds(lo, BPI * B)],)
                + tuple(ref.at[pl.ds(lo, P2 + BPI * B)] for ref in (h_v, out_v, st_v)) + (g,))

    def stage_q(xd, q, first, before, after):
        def emit(half, blk, val):
            group = half_groups(val, half)
            for j in half_pairs(half):
                ph = _hedgehog_t(_pair_logits(group, j), zacc_v[j * 128:(j + 1) * 128, :])
                pq_v[2 * q + blk][(j // 2) * 64:(j // 2 + 1) * 64, (j % 2) * B:(j % 2 + 1) * B] = _pk(ph.astype(bf16))

        sproj(wsq_v, xd, q, emit, before=before, after=after, first=first)

    oc_v = (oc0_v, oc1_v)

    def stage_g(q):
        pq = [sealed(pq_v[2 * q + blk]) for blk in range(2)]
        for t in range(NP // 4):
            parts = [[_dot_nn(_upk(kv_v[:, j * 128:(j + 1) * 128]),
                              _upk(pq[blk][(j // 2) * 64:(j // 2 + 1) * 64, (j % 2) * B:(j % 2 + 1) * B]))
                      for blk in range(2) for j in (jj, jj + NP // 2)] for jj in (2 * t, 2 * t + 1)]
            blocks = [jnp.concatenate([a, b], axis=0) for a, b in zip(*parts)]
            for m, spec in enumerate(_SA):
                c = m * HK + t * 128
                oc_v[q][0:B // 2, c:c + 128] = _pk(_combo(blocks, spec).astype(bf16).T)

    def stage_h(views, q, keep, pieces, jobs, before=None):
        x_g, h_g = views[0], views[1]
        oc = sealed(oc_v[q])
        first, last = 4, 12
        ties = [{} for _ in range(7)]
        for k, vals in enumerate(pieces):
            t = first + k * (last - first) // max(len(pieces) - 1, 1)
            for m, val in enumerate(vals):
                ties[t // 4][(m * 8, (t % 4) * 128)] = val
        state = {}
        done = [0]

        def product(m):
            if before:
                before(m)
            w = wso_v[:, m * HK:(m + 1) * HK]
            if ties[m]:
                w = _tie(keep, w, ties[m])
            done[0] = m
            res = _dot_nn(_upk(oc[0:B // 2, m * HK:(m + 1) * HK]), _upk(w))
            for k, job in enumerate(jobs):
                t = 2 * q + k * (24 - 4 * q) // len(jobs)
                if t // 4 == m:
                    job(res[0:R, (t % 4) * 128:(t % 4 + 1) * 128])
            return res

        def wmul(d, lo):
            return (d.reshape(B // 8, 8, 128) * wrb_v[:, lo:lo + 128][None]).reshape(B, 128)

        def emit(k, val):
            blk, half = k // 2, k % 2
            s = 2 * q + blk
            cols = slice(half * HK, (half + 1) * HK)
            h = x_g[s * B:(s + 1) * B, cols].astype(f32) + val
            h_g[(s + 2) * B:(s + 3) * B, cols] = h
            st = state.setdefault(blk, {'h': {}})
            st['h'][half] = h
            for c in range(0, HK, 128):
                ht = h[:, c:c + 128]
                if 'h0' not in st:
                    st['h0'] = ht
                    continue
                d = ht - st['h0']
                new = (d, d * d, wmul(d, half * HK + c))
                st['s'] = new if 's' not in st else tuple(a + b for a, b in zip(st['s'], new))
            if len(st['h']) == 1:
                vals = [_or_all(list(v)) for v in zip(*[_vregs(a) for a in st['s']])]
                m = done[0] + 2
                for n, val in enumerate(vals):
                    ties[m][(248 - (n % 4) * 8, (n // 4) * 128)] = val

        _strassen(product, emit)

        res = []
        for blk in range(2):
            st = state[blk]
            s1, s2, s3 = st['s']
            c0 = _lanes(jnp.mean(st['h0'], axis=-1, keepdims=True))
            g0 = st['h0'] - c0
            t1 = s1 + 8.0 * g0
            t2 = s2 + g0 * (s1 + t1)
            t3 = s3 + wmul(g0, D + 128)
            res.append((jnp.concatenate([t1, t2, t3, c0], axis=1),
                        jnp.concatenate([st['h'][0], st['h'][1]], axis=1)))
        return res

    def stage_stats(views, s, part, valid=None):
        st_g, g = views[3], views[4]
        b = g * BPI + s
        bv = bestv_v[...]
        bi = besti_v[...]
        wsum = wrb_v[0:1, D:D + 128]
        nvs, nis, sts = [], [], []
        for k in range(B // R):
            sl = slice(k * R, (k + 1) * R)
            red = [_lanes(jnp.sum(part[sl, n * 128:(n + 1) * 128], axis=-1, keepdims=True)) for n in range(3)]
            mu = red[0] * (1.0 / D)
            var = jnp.maximum(red[1] * (1.0 / D) - mu * mu, 0.0)
            rs = lax.rsqrt(var + LN_EPS)
            r = (red[2] - mu * wsum) * rs
            sts.append(jnp.concatenate([rs, (mu + part[sl, 384:512]) * rs], axis=1))
            if valid is not None:
                r = jnp.where(valid, r, -jnp.inf)
            idx = lax.broadcasted_iota(jnp.int32, (R, 128), 0) + (b * B + k * R)
            better = r > bv[sl]
            nvs.append(jnp.where(better, r, bv[sl]))
            nis.append(jnp.where(better, idx, bi[sl]))
        st = jnp.concatenate(sts, axis=0)
        st_g[(s + 2) * B:(s + 3) * B, :] = st
        bestv_v[...] = jnp.concatenate(nvs, axis=0)
        besti_v[...] = jnp.concatenate(nis, axis=0)
        return st, [_vregs(nv) for nv in nvs]

    def out_jobs(views, s, keep, st=None, h=None):
        h_g, out_g, st_g = views[1], views[2], views[3]

        def job(k):
            def run(anchor):
                rows = slice((s + 2) * B + k * R, (s + 2) * B + (k + 1) * R)
                hk = h_g[rows, :] if h is None else h[k * R:(k + 1) * R]
                sk = st_g[rows, :] if st is None else st[k * R:(k + 1) * R]
                a = 1.0 + jnp.where(keep, sk[:, 0:128], anchor)
                o = [hk[:, c * 128:(c + 1) * 128] * a - sk[:, 128:256] for c in range(D // 128)]
                out_g[rows, :] = jnp.concatenate(o, axis=1).astype(bf16)
            return run
        return [job(k) for k in range(B // R)]

    def p2_body(i, c):
        b0 = i * BPI
        keep = flag_s[0] > 0
        cur = views_of(i)
        st, pieces = stage_stats(cur, -1, pend_v[...], i > 0)
        ojobs = out_jobs(cur, -2, keep) + out_jobs(cur, -1, keep, st)
        n = D // NI
        jobs = []
        for src, dst in ((wg_v, wgp_v), (wu_v, wup_v)):
            sv = src.at[pl.ds(pl.multiple_of(i * n, n), n)]
            dv = dst.at[pl.ds(pl.multiple_of(i * (n // 2), n // 2), n // 2)]
            jobs += [(sv, dv, r, cc) for r in range(0, n, 16) for cc in range(0, NM, 128)]
        rp = repacker(jobs, keep)
        stage_q(xs_view(i, 1), 0, xt_view(i), None, rp[0])
        stage_q(xs_view(i, 1), 1, None, lambda m: stage_g(0) if m == 2 else None, rp[1])
        res = stage_h(cur, 0, keep, pieces, ojobs, lambda m: stage_g(1) if m == 1 else None)
        st0, _ = stage_stats(cur, 0, res[0][0])
        st1, pieces = stage_stats(cur, 1, res[1][0])
        ojobs = out_jobs(cur, 0, keep, st0, res[0][1]) + out_jobs(cur, 1, keep, st1, res[1][1])
        res = stage_h(cur, 1, keep, pieces, ojobs)
        stage_stats(cur, BPI - 2, res[0][0])
        pend_v[...] = res[1][0]

        @pl.when(i > 0)
        def _():
            cp_out(jnp.maximum(b0 - 2, 0), 2).start()

        cp_out(b0, 2).start()
        return c

    lax.fori_loop(0, NI, p2_body, 0)
    wait_all(cp_gu[1])
    keep = flag_s[0] > 0
    last = views_of(NI - 1)

    st, _ = stage_stats(last, BPI - 1, pend_v[...])

    bv = bestv_v[...]
    mval = jnp.max(bv, axis=0, keepdims=True)
    sel = jnp.min(jnp.where(bv == mval, besti_v[...], S - 1), axis=0, keepdims=True)
    idx = sel[0, 0]
    hrow = h_v[pl.ds(P2 + idx, 1), :]
    strow = st_v[pl.ds(P2 + idx, 1), :]
    xrow = jnp.concatenate([hrow[:, c * 128:(c + 1) * 128] * strow[:, 0:128] - strow[:, 128:256]
                            for c in range(D // 128)], axis=1).astype(bf16)
    xs = jnp.broadcast_to(xrow, (16, D))
    g_first = _dot_nn(xs, _upk(wgp_v[:, 0:FC]))
    anchors = ([jnp.broadcast_to(pltpu.bitcast(sel, f32), (R, 128))] * 4
               + [jnp.broadcast_to(xrow[:, 0:128].astype(f32), (R, 128))] * 4
               + [g_first[:, (k // 2) * 128:(k // 2 + 1) * 128] for k in range(8)])
    for job, anchor in zip(out_jobs(last, BPI - 2, keep) + out_jobs(last, BPI - 1, keep, st), anchors):
        job(anchor)
    cp_out(NB - 2, 2).start()

    def act(g, u):
        a = g * pl.reciprocal(1.0 + jnp.exp(-g), approx=True) * u
        return jnp.concatenate([a, a], axis=0).astype(bf16)

    def down(a, lo, w):
        return _dot_nn(a, _upk(wdp_v[lo // 2:(lo + w) // 2, 0:D]))[0:8]

    xcol = jnp.broadcast_to(xrow, (128, D)).T.astype(f32)
    jobs = [(which, b) for b in range(NBV) for which in (0, 1)]
    vres, prev = {}, None
    for j0 in range(0, len(jobs), NCH):
        grp = jobs[j0:j0 + NCH]
        accs = [None] * len(grp)
        for r in range(D // 16):
            for n, (which, b) in enumerate(grp):
                w = (wg_v, wu_v)[which][r * 16:(r + 1) * 16, NM + b * 128:NM + (b + 1) * 128].astype(f32)
                t0 = w[0:8] * xcol[r * 16:r * 16 + 8]
                t1 = w[8:16] * xcol[r * 16 + 8:r * 16 + 16]
                if accs[n] is None:
                    if prev is not None:
                        t0 = jnp.where(keep, t0, prev[n % len(prev)])
                    accs[n] = t0 + t1
                else:
                    accs[n] = (accs[n] + t0) + t1
        prev = accs
        for n, job in enumerate(grp):
            vres[job] = _allreduce8(accs[n][None], jnp.add)[0]

    chunks = [(lo, min(FC, NM - lo)) for lo in range(0, NM, FC)]
    acts, y = [], None
    for k, (lo, w) in enumerate(chunks):
        g = g_first if k == 0 else _dot_nn(xs, _upk(wgp_v[:, lo:lo + w]))
        u = _dot_nn(xs, _upk(wup_v[:, lo:lo + w]))
        acts.append(act(g[0:8], u[0:8]))
        if k >= 1:
            t = down(acts[k - 1], *chunks[k - 1])
            y = t if y is None else y + t
    y = y + down(acts[-1], *chunks[-1])
    for b0, nb in ((0, 4), (4, 4), (8, 4), (12, 1)):
        g = jnp.concatenate([vres[(0, b)] for b in range(b0, b0 + nb)], axis=1)
        u = jnp.concatenate([vres[(1, b)] for b in range(b0, b0 + nb)], axis=1)
        y = y + down(act(g, u), NM + b0 * 128, nb * 128)

    gate = jnp.broadcast_to(jax.nn.sigmoid(mval), (8, 128))
    base = pl.multiple_of((idx >> 4) << 4, 16)
    rows = pl.ds(pl.multiple_of(P2 + base, 16), 16)
    h16 = h_v[rows, :]
    st16 = st_v[rows, :]
    a16 = 1.0 + st16[:, 0:128]
    m16 = st16[:, 128:256]
    hit = (lax.broadcasted_iota(jnp.int32, (16, 128), 0) + base) == idx
    res = []
    for c in range(D // 128):
        yc = y[:, c * 128:(c + 1) * 128] * gate
        yc = jnp.concatenate([yc, yc], axis=0)
        res.append(h16[:, c * 128:(c + 1) * 128] * a16 - m16 + jnp.where(hit, yc, 0.0))
    res = jnp.concatenate(res, axis=1).astype(bf16)
    for i in range(NI):
        cp_out(i * BPI, 2).wait()
        cp_out(i * BPI + 2, 2).wait()
    out_v[rows, :] = res
    fix = pltpu.make_async_copy(out_v.at[rows], out_hbm.at[pl.ds(base, 16)], sem_o.at[0])
    fix.start()
    fix.wait()


@jax.jit
def pallas_sequential_preLN__linear_kernel_hedgehog__moe_arch_mod__prompt_kernel(
    A_x: jax.Array,
    A_wqkv: jax.Array,
    A_w_phi: jax.Array,
    A_wo: jax.Array,
    B_x: jax.Array,
    B_w_r: jax.Array,
    B_w_gate: jax.Array,
    B_w_up: jax.Array,
    B_w_down: jax.Array,
):
    del B_x
    x = A_x.reshape(S, D)
    wphi = A_w_phi.reshape(H * DH, DH)
    wr = B_w_r.reshape(8, 128)
    any_spec = pl.BlockSpec(memory_space=pl.ANY)
    out = pl.pallas_call(
        _kernel,
        out_shape=jax.ShapeDtypeStruct((S, D), bf16),
        in_specs=[any_spec] * 8,
        out_specs=any_spec,
        scratch_shapes=[
            pltpu.VMEM((S, D), bf16),
            pltpu.VMEM((D, 3 * D), bf16),
            pltpu.VMEM((H * DH, DH), bf16),
            pltpu.VMEM((D, D), bf16),
            pltpu.VMEM((64, 128), bf16),
            pltpu.VMEM((D, F + 128), bf16),
            pltpu.VMEM((D, F + 128), bf16),
            pltpu.VMEM((F, D), bf16),
            pltpu.VMEM((PR, D), u32),
            pltpu.VMEM((PR // 2, 7 * HK), u32),
            pltpu.VMEM((PR // 2, 7 * HK), u32),
            pltpu.VMEM((D // 4 + 8, 7 * HK), u32),
            pltpu.VMEM((D // 4, 7 * HK), u32),
            pltpu.VMEM((F // 2, D + 128), u32),
            pltpu.VMEM((D // 2, NM), u32),
            pltpu.VMEM((D // 2, NM), u32),
            pltpu.VMEM((64, 8 * 128), u32),
            pltpu.VMEM((T0 // 2, D), u32),
            pltpu.VMEM(((S + T) // 4, 7 * HK), u32),
            pltpu.VMEM((NT * (HK // 2), B), u32),
            pltpu.VMEM((NP, 64, 128), f32),
            pltpu.VMEM((2 * D, 128), f32),
            pltpu.VMEM((32, NP * 128), u32),
            pltpu.VMEM((D + 8, T), u32),
            pltpu.VMEM((D // 2 + 16, 2 * B), u32),
            pltpu.VMEM((D // 2 + 16, 2 * B), u32),
            pltpu.VMEM((D // 2 + 16, 2 * B), u32),
            pltpu.VMEM((D // 2 + 16, 2 * B), u32),
            pltpu.VMEM((B // 2 + 8, 7 * HK), u32),
            pltpu.VMEM((B // 2 + 8, 7 * HK), u32),
            pltpu.VMEM((P2 + S, D), f32),
            pltpu.VMEM((P2 + S, 256), f32),
            pltpu.VMEM((B, 512), f32),
            pltpu.VMEM((P2 + S, D), bf16),
            pltpu.VMEM((8, D + 512), f32),
            pltpu.VMEM((B, 128), f32),
            pltpu.VMEM((B, 128), jnp.int32),
            pltpu.SMEM((2,), jnp.int32),
            pltpu.SemaphoreType.DMA((_NSEM_IN,)),
            pltpu.SemaphoreType.DMA((1,)),
        ],
        compiler_params=pltpu.CompilerParams(vmem_limit_bytes=110 * 1024 * 1024,
                                             disable_bounds_checks=True,
                                             disable_semaphore_checks=True),
        name="hedgehog_mod",
    )(x, A_wqkv, wphi, A_wo, wr, B_w_gate, B_w_up, B_w_down)
    return out.reshape(1, S, D)
```

```python
import jax
import jax.numpy as jnp
from jax import lax
import jax.experimental.pallas as pl
import jax.experimental.pallas.tpu as pltpu

S = 2048
D = 1024
H = 32
DH = 32
F = 3584
T = 512
NT = S // T
T0 = 256
B = 128
NB = S // B
BPI = 4
NI = NB // BPI
NP = H // 2
FC = 1024
R = 16
NBV = 13
NM = F - NBV * 128
NCH = 4
OCH = 176
DCH = 1216
NV = 124
PR = NV * 4
HK = D // 2
P2 = 2 * B
LOG2E = 1.4426950408889634
LN_EPS = 1e-5
DEN_EPS = 1e-6

_NT_DIMS = (((1,), (1,)), ((), ()))

bf16 = jnp.bfloat16
f32 = jnp.float32
u32 = jnp.uint32


def _dot_nt(a, b):
    return lax.dot_general(a, b, _NT_DIMS, preferred_element_type=f32)


def _dot_nn(a, b):
    return jnp.dot(a, b, preferred_element_type=f32)


def _pk(x):
    return pltpu.bitcast(x, u32)


def _upk(x):
    return pltpu.bitcast(x, bf16)


def _lanes(x):
    return jnp.broadcast_to(x, (x.shape[0], 128))


def _layernorm(x):
    m = jnp.mean(x, axis=-1, keepdims=True)
    xc = x - m
    v = jnp.mean(xc * xc, axis=-1, keepdims=True)
    return xc * lax.rsqrt(v + LN_EPS)


def _allreduce8(x, op):
    x = op(x, pltpu.roll(x, 4, 1))
    x = op(x, pltpu.roll(x, 2, 1))
    x = op(x, pltpu.roll(x, 1, 1))
    return x


def _hedgehog_t(p, z=None):
    t = p.shape[-1]
    p4 = p.reshape(2, 4, 8, t)
    mx = _allreduce8(jnp.max(p4, axis=1), jnp.maximum)
    mn = _allreduce8(jnp.min(p4, axis=1), jnp.minimum)
    ep = jnp.exp2(p4 - mx[:, None])
    en = jnp.exp2(mn[:, None] - p4)
    a = pl.reciprocal(_allreduce8(jnp.sum(ep, axis=1), jnp.add), approx=True)
    b = pl.reciprocal(_allreduce8(jnp.sum(en, axis=1), jnp.add), approx=True)
    if z is not None:
        dp = jnp.sum(ep * z[0:64].reshape(2, 4, 8, t), axis=1)
        dn = jnp.sum(en * z[64:128].reshape(2, 4, 8, t), axis=1)
        den = _allreduce8(dp * a + dn * b, jnp.add) + DEN_EPS
        inv = pl.reciprocal(den, approx=True)
        a = a * inv
        b = b * inv
    fp = (ep * a[:, None]).reshape(64, t)
    fn = (en * b[:, None]).reshape(64, t)
    return jnp.concatenate([fp, fn], axis=0)


_SA = ((3, None, 0), (2, 3, 1), (0, 1, 1), (0, None, 0), (0, 3, 1), (1, 3, -1), (2, 0, -1))
_SB = ((2, 0, -1), (0, None, 0), (3, None, 0), (1, 3, -1), (0, 3, 1), (2, 3, 1), (0, 1, 1))


def _combo(blocks, spec):
    a, b, sign = spec
    if b is None:
        return blocks[a]
    return blocks[a] + blocks[b] if sign > 0 else blocks[a] - blocks[b]


def _strassen(product, emit):
    m4 = product(0)
    m2 = product(1)
    emit(2, m4 + m2)
    m5 = product(2)
    u = m4 - m5
    m3 = product(3)
    emit(1, m5 + m3)
    v = m3 - m2
    m1 = product(4)
    u = u + m1
    v = v + m1
    emit(0, u + product(5))
    emit(3, v + product(6))


def _head_groups(h):
    base, k = (NV // 4) * (h // 8), h % 8
    return ([base + 4 * k + i for i in range(3)],
            base + 4 * k - 1 if k > 0 else None,
            base + 4 * k + 3 if k < 7 else None,
            8 - k)


def _pair_logits(group, j):
    parts = []
    for h in (2 * j, 2 * j + 1):
        full, below, above, a = _head_groups(h)
        ref = group(full[0])
        sub = lax.broadcasted_iota(jnp.int32, ref.shape, 0)
        if above is None:
            m = jnp.where(sub >= a, group(below), 0.0)
        else:
            m = jnp.where(sub == a - 1, 0.0, group(above))
            if below is not None:
                m = jnp.where(sub >= a, group(below), m)
        parts += [m] + [group(q) for q in full]
    return jnp.concatenate(parts, axis=0)


def _pair_need(j):
    full, _, above, _ = _head_groups(2 * j + 1)
    return full[2] if above is None else above


def _tie(keep, w, ties):
    rows = sorted({r for r, _ in ties})
    out, pos = [], 0
    for r in rows:
        if r > pos:
            out.append(w[pos:r])
        cols = sorted(c for rr, c in ties if rr == r)
        parts, cpos = [], 0
        for c in cols:
            if c > cpos:
                parts.append(w[r:r + 8, cpos:c])
            parts.append(jnp.where(keep, w[r:r + 8, c:c + 128], ties[(r, c)]))
            cpos = c + 128
        if cpos < w.shape[1]:
            parts.append(w[r:r + 8, cpos:])
        out.append(jnp.concatenate(parts, axis=1) if len(parts) > 1 else parts[0])
        pos = r + 8
    if pos < w.shape[0]:
        out.append(w[pos:])
    return jnp.concatenate(out, axis=0)


def _vregs(x):
    if x.dtype != u32:
        x = pltpu.bitcast(x, u32)
    return [x[r:r + 8, c:c + 128] for r in range(0, x.shape[0], 8) for c in range(0, x.shape[1], 128)]


def _or_all(vals):
    acc = vals[0]
    for v in vals[1:]:
        acc = acc | v
    return acc


def _phys_group(g):
    return 2 * (g % 4) + g // 4


def _phys_pair(j):
    return 2 * _phys_group(j // 2) + j % 2


_KSTAGES = (((0, 2),), ((2, 3),), ((5, 3),))
_PSTAGES = (((0, 5),), ((5, 3),))
_NSEM_IN = 11


def _kernel(x_hbm, wqkv_hbm, wphi_hbm, wo_hbm, wr_hbm, wg_hbm, wu_hbm, wd_hbm,
            out_hbm,
            x_v, wqkv_v, wphi_v, wo_v, wr_v, wg_v, wu_v, wd_v,
            wtk_v, wsq_v, wsk_v, wsv_v, wso_v, wdp_v, wgp_v, wup_v, amat_v, xn_v, xs_v, xt_v, kvacc_v, zacc_v, kv_v, phi_v,
            pq0_v, pq1_v, pq2_v, pq3_v, oc0_v, oc1_v, h_v, st_v, pend_v, out_v, wrb_v,
            bestv_v, besti_v, flag_s,
            sem_i, sem_o):

    def cp_x(lo, n, sem):
        return pltpu.make_async_copy(x_hbm.at[pl.ds(lo, n)], x_v.at[pl.ds(lo, n)], sem_i.at[sem])

    def cp_w(lo, w, sem):
        return pltpu.make_async_copy(wqkv_hbm.at[:, pl.ds(lo, w)], wqkv_v.at[:, pl.ds(lo, w)], sem_i.at[sem])

    cp_k = [[cp_w(D + g * 128, n * 128, 2 + c) for g, n in st] for c, st in enumerate(_KSTAGES)]
    cp_p = [[pltpu.make_async_copy(wphi_hbm.at[pl.ds(g * 128, n * 128)], wphi_v.at[pl.ds(g * 128, n * 128)],
                                   sem_i.at[3 * c]) for g, n in st] for c, st in enumerate(_PSTAGES)]
    cp_wv = cp_w(2 * D, D, 5)
    cp_wq = cp_w(0, D, 7)

    def cp_wd(k):
        lo, n = k * DCH, min(DCH, F - k * DCH)
        return pltpu.make_async_copy(wd_hbm.at[pl.ds(lo, n)], wd_v.at[pl.ds(lo, n)], sem_i.at[(6, 8, 9)[k]])

    cp_x0 = cp_x(0, T0, 1)
    cp_x1 = cp_x(T0, T0, 4)
    cp_x2 = cp_x(T, P2, 5)
    cp_x3 = cp_x(T + P2, T, 6)
    cp_x4 = cp_x(2 * T + P2, S - 2 * T - P2, 8)
    cp_wr = pltpu.make_async_copy(wr_hbm, wr_v.at[pl.ds(0, 8)], sem_i.at[7])

    def cp_wo(k, half):
        lo, n = k * OCH, min(OCH, HK - k * OCH)
        rows = pl.ds(half * HK + lo, n)
        return pltpu.make_async_copy(wo_hbm.at[rows], wo_v.at[rows], sem_i.at[(6, 8, 9)[k]])

    def wait_bg(k):
        cp_wo(k, 0).wait()
        cp_wo(k, 1).wait()
        cp_wd(k).wait()

    cp_gu = [[pltpu.make_async_copy(src.at[:, pl.ds(lo, n)], dst.at[:, pl.ds(lo, n)], sem_i.at[sem])
              for src, dst in ((wg_hbm, wg_v), (wu_hbm, wu_v))] for lo, n, sem in ((0, NM, 7), (NM, F - NM, 10))]

    def cp_out(b, n):
        lo = b * B
        if not isinstance(b, int):
            lo = pl.multiple_of(lo, B)
        return pltpu.make_async_copy(out_v.at[pl.ds(P2 + lo, n * B)], out_hbm.at[pl.ds(lo, n * B)], sem_o.at[0])

    for cp in (*cp_p[0], cp_x0, *cp_k[0], *cp_p[1], *cp_k[1], *cp_k[2], cp_x1, cp_wv, cp_x2,
               cp_x3, cp_wo(0, 0), cp_wo(0, 1), cp_wd(0), cp_x4, cp_wo(1, 0), cp_wo(1, 1), cp_wd(1),
               cp_wo(2, 0), cp_wo(2, 1), cp_wd(2), cp_wr, cp_wq, *cp_gu[0], *cp_gu[1]):
        cp.start()
    flag_s[0] = 1
    flag_s[1] = 0

    def ln1(xg, src, xd, dst, n, which=None, keep=None, anchors=None, plain=False):
        pieces = []
        for pr in range(n // P2):
            for k in range(B // R):
                off = pr * P2 + k * R
                if which is not None and pr * (B // R) + k not in which:
                    continue
                x0 = xg[src + off:src + off + R, :].astype(f32)
                x1 = xg[src + off + B:src + off + B + R, :].astype(f32)
                if anchors is not None:
                    a = anchors[len(pieces)]
                    x0 = jnp.concatenate([jnp.where(keep, x0[:, :128], a), x0[:, 128:]], axis=1)
                    x1 = jnp.concatenate([jnp.where(keep, x1[:, :128], a), x1[:, 128:]], axis=1)
                p0 = _layernorm(x0)
                p1 = _layernorm(x1)
                if plain:
                    xn_v[off // 2:(off + R) // 2, :] = _pk(p0.astype(bf16))
                    xn_v[(off + B) // 2:(off + B + R) // 2, :] = _pk(p1.astype(bf16))
                lo = (dst + pr * P2) // 4 + k * (R // 2)
                blocks = (p0[:, :HK], p1[:, :HK], p0[:, HK:], p1[:, HK:])
                vs = []
                for m, spec in enumerate(_SB):
                    t = _combo(blocks, spec)
                    xd[lo:lo + R // 2, m * HK:(m + 1) * HK] = _pk(t.astype(bf16))
                    if spec[1] is not None:
                        vs.append(_vregs(t))
                pieces.append([_or_all(list(col)) for col in zip(*vs)])
        return pieces

    def load_xn(b):
        return _upk(xn_v[b * (B // 2):(b + 1) * (B // 2), :])

    def piece_ties(pieces, n, row0=0, col=0):
        ties = {}
        if pieces:
            step = (n - row0) // len(pieces) // 8 * 8
            for k, p in enumerate(pieces):
                for q, val in enumerate(p):
                    ties[(row0 + k * step + (q // 4) * 8, col + (q % 4) * 128)] = val
        return ties

    def xs_view(i, tiles):
        return xs_v.at[pl.ds(pl.multiple_of(i * (T // 4), T // 4), tiles * (T // 4))]

    def xt_view(i):
        lo = i * (HK // 2)
        return xt_v.at[pl.ds(lo if isinstance(i, int) else pl.multiple_of(lo, HK // 2), HK // 2)]

    def store_xt(i, xd, row):
        xt_view(i)[...] = _pk(_upk(xd[row:row + B // 2, 0:HK]).T)

    def sproj(ws, xd, pr, emit, keep=None, work=None, before=None, after=None, first=None):
        lo = pr * (B // 2)

        def product(m):
            if before:
                before(m)
            lhs = ws[:, m * HK:(m + 1) * HK]
            if work is not None and work.get(m):
                lhs = _tie(keep, lhs, piece_ties(work[m], lhs.shape[0], 32))
            if m == 0 and first is not None:
                res = _dot_nn(_upk(lhs), _upk(first[...]))
            else:
                res = _dot_nt(_upk(lhs), _upk(xd[lo:lo + B // 2, m * HK:(m + 1) * HK]))
            if after:
                after(m, res)
            return res

        _strassen(product, lambda k, val: emit(k // 2, k % 2, val))

    def repacker(jobs, keep):
        def hook(q):
            def after(m, res):
                if m in (0, 2, 4):
                    k = 3 * q + m // 2
                    mine = jobs[k * len(jobs) // 6:(k + 1) * len(jobs) // 6]
                    for n, (sv, dv, r, c) in enumerate(mine):
                        a = (64 + n * 416 // len(mine)) // 8 * 8
                        dv[r // 2:r // 2 + 8, c:c + 128] = jnp.where(keep, _pk(sv[r:r + 16, c:c + 128]),
                                                                     pltpu.bitcast(res[a:a + 8], u32))
            return after
        return hook(0), hook(1)

    def spread(pieces, slots):
        res = {}
        for k, (pr, m) in enumerate(slots):
            res.setdefault(pr, {})[m] = pieces[k * len(pieces) // len(slots):(k + 1) * len(pieces) // len(slots)]
        return res

    def sealed(ref):
        ref[pl.ds(pl.multiple_of(flag_s[1] + ref.shape[0] - 8, 8), 8), 0:128] = jnp.zeros((8, 128), u32)
        return ref

    def store_combos(ws, row, top, bot, table=_SA, keep=None, anchors=None):
        for c in range(0, HK, 128):
            blocks = [top[:, c:c + 128], top[:, HK + c:HK + c + 128], bot[:, c:c + 128], bot[:, HK + c:HK + c + 128]]
            if anchors is not None:
                for q in (0, 3):
                    blocks[q] = jnp.where(keep, blocks[q], anchors[c // 128])
            for m, spec in enumerate(table):
                ws[row:row + 8, m * HK + c:m * HK + c + 128] = _pk(_combo(blocks, spec).astype(bf16))

    zinit = set()

    def k_side(group, pairs, slot, keep=None, anchor=None):
        res = []
        for j in pairs:
            p = _pair_logits(group, j)
            if anchor is not None:
                p = jnp.concatenate([jnp.where(keep, p[0:8], anchor), p[8:32],
                                     jnp.where(keep, p[32:40], anchor), p[40:64]], axis=0)
            ph = _hedgehog_t(p)
            j = _phys_pair(j)
            if j not in zinit:
                zinit.add(j)
                zacc_v[j * 128:(j + 1) * 128, :] = ph
            else:
                zacc_v[j * 128:(j + 1) * 128, :] += ph
            phi_v[j * 64:(j + 1) * 64, slot * B:(slot + 1) * B] = _pk(ph.astype(bf16))
            res.append(ph)
        return res

    def half_groups(p, half):
        return lambda pos: p[(pos - half * (NV // 2)) * 8:(pos - half * (NV // 2) + 1) * 8]

    def half_pairs(half):
        return range(half * (NP // 2), (half + 1) * (NP // 2))

    def kv_prod(vt, ph, j):
        half, r = j // (NP // 2), (j % (NP // 2)) * 64
        v = jnp.concatenate([vt[(s, half)][r:r + 64] for s in range(T // B)], axis=1).astype(bf16)
        return _dot_nt(v, ph)

    eye = (lax.broadcasted_iota(jnp.int32, (DH, DH), 0)
           == lax.broadcasted_iota(jnp.int32, (DH, DH), 1)).astype(bf16)
    r_h = lax.broadcasted_iota(jnp.int32, (128, 128), 0) // DH
    c_h = lax.broadcasted_iota(jnp.int32, (128, 128), 1) // DH
    same_head = r_h == c_h

    def make_amat(g):
        a = jnp.concatenate([_dot_nt(eye, wphi_v[g * 128:(g + 1) * 128, :])] * 4, axis=0)
        amat_v[:, g * 128:(g + 1) * 128] = _pk(jnp.where(same_head, a, 0.0).astype(bf16))

    class Folder:
        def __init__(self, col0, first=0):
            self.col0, self.rows, self.mprev, self.done = col0, {}, None, first

        def tile(self, g, rows, keep=None, ties=None):
            g = _phys_group(g)
            am = amat_v[:, g * 128:(g + 1) * 128]
            if ties:
                am = _tie(keep, am, ties)
            return _dot_nt(_upk(am), wqkv_v[rows, self.col0 + g * 128:self.col0 + (g + 1) * 128])

        def fold(self, g, wt=None):
            sub = lax.broadcasted_iota(jnp.int32, (8, D), 0)
            if wt is None:
                wt = self.tile(g, slice(None))
            for hh in range(4):
                full, below, _, a = _head_groups(4 * g + hh)
                r0 = hh * DH
                ref = jnp.broadcast_to(wt[r0 + a - 1:r0 + a, :], (8, D))
                part = [(wt[r0 + 8 * i:r0 + 8 * (i + 1)] - ref) * LOG2E for i in range(4)]
                if below is not None:
                    self.rows[below] = jnp.where(sub >= a, part[0], self.mprev)
                self.mprev = part[0]
                for q, v in zip(full, part[1:]):
                    self.rows[q] = v
            new = {}
            while self.done in self.rows and self.done + 1 in self.rows:
                new[self.done] = jnp.concatenate([self.rows.pop(self.done), self.rows.pop(self.done + 1)], axis=0)
                self.done += 2
            return new

    def fold_pair(folders, g, keep=None, ties=None):
        tiles = {}
        for n, c in enumerate(range(0, HK, 128)):
            for half in range(2):
                for side in range(2):
                    t = ties[n] if ties and half == 0 and side == 0 else None
                    lo = side * HK + c
                    tiles[(half, lo)] = folders[half].tile(g + 4 * half, slice(lo, lo + 128), keep, t)
        return [folders[half].fold(g + 4 * half,
                                   jnp.concatenate([tiles[(half, lo)] for lo in range(0, D, 128)], axis=1))
                for half in range(2)]

    bestv_v[...] = jnp.full(bestv_v.shape, -jnp.inf, f32)
    besti_v[...] = lax.broadcasted_iota(jnp.int32, besti_v.shape, 0)
    h_v[0:P2, :] = jnp.zeros((P2, D), f32)
    st_v[0:B, :] = jnp.zeros((B, 256), f32)
    pend_v[...] = jnp.zeros(pend_v.shape, f32)

    def wait_all(cps):
        for cp in cps:
            cp.wait()

    def amats(c):
        for g0, n in _PSTAGES[c]:
            for g in range(g0, g0 + n):
                make_amat(g)

    wait_all(cp_p[0])
    amats(0)

    cp_x0.wait()
    ln1(x_v, 0, xs_v, 0, T0, plain=True)
    xb = [load_xn(s) for s in range(2)]
    logits = [{}, {}]
    finished = [set(), set()]
    fk, slabs = (Folder(D), Folder(D, NV // 2)), {}
    defer, queue = [False], []

    def absorb(new):
        for pos, slab in new.items():
            wtk_v[pos * 4:pos * 4 + 8, :] = _pk(slab.astype(bf16))
            slabs[pos] = slab
        for pos in sorted(slabs):
            if pos < NV // 2 and pos + NV // 2 in slabs:
                store_combos(wsk_v, pos * 4, slabs.pop(pos), slabs.pop(pos + NV // 2))

    def k_finish(s, hold=0):
        ready = [j for j in range(NP) if j not in finished[s] and _pair_need(j) in logits[s]]
        ready = ready[:len(ready) - hold]
        if defer[0]:
            queue.extend((logits[s].__getitem__, [j], s) for j in ready)
        else:
            k_side(logits[s].__getitem__, ready, s)
        finished[s].update(ready)

    def k_chunk(s, keep=None, early=(), late=(), hold=0):
        todo = [q for half in range(2) for q in range(half * (NV // 2), fk[half].done) if q not in logits[s]]
        runs = [[q for q in todo if q < NV // 2], [q for q in todo if q >= NV // 2]]
        lhs = jnp.concatenate([wtk_v[r[0] * 4:(r[-1] + 1) * 4, :] for r in runs if r], axis=0)
        ties = piece_ties(early, lhs.shape[0])
        ties.update(piece_ties(late, lhs.shape[0], col=HK))
        if ties:
            lhs = _tie(keep, lhs, ties)
        p = _dot_nt(_upk(lhs), xb[s])
        for n, q in enumerate(todo):
            logits[s][q] = p[n * 8:(n + 1) * 8]
        k_finish(s, hold)
        return p

    wait_all(cp_k[0])
    for new in fold_pair(fk, 0):
        absorb(new)
    k_chunk(0)
    k_chunk(1, hold=1)

    wait_all(cp_p[1] + cp_k[1])
    k_finish(1)
    for new in fold_pair(fk, 1):
        absorb(new)
    absorb(fk[0].fold(2))
    amats(1)
    k_chunk(0)
    k_chunk(1, hold=2)

    wait_all(cp_k[2] + [cp_x1])
    defer[0] = True
    keep = flag_s[0] > 0
    absorb(fk[1].fold(6))
    new = fold_pair(fk, 3)
    late = list(new[0].values())[-1][:, 384:512]
    for n in new:
        absorb(n)
    pieces = ln1(x_v, T0, xs_v, T0, T0, [0]) + ln1(x_v, T0, xs_v, T0, T0, [1, 2], keep, [late, late])
    p = k_chunk(0, keep, (), pieces[:2])
    rows = [k * p.shape[0] // 5 // 16 * 16 for k in range(5)]
    pieces += ln1(x_v, T0, xs_v, T0, T0, range(3, 8), keep, [p[r:r + R] for r in rows])
    k_chunk(1, keep, pieces[2:3], pieces[3:])

    def k_emit1(half, blk, val):
        if half != blk:
            k_side(half_groups(val, half), half_pairs(half), 2 + blk)
        else:
            queue.extend((half_groups(val, half), [j], 2 + blk) for j in half_pairs(half))

    def run_queue(n, res):
        deps = []
        for k in range(min(n, len(queue))):
            r = k * res.shape[0] // n // 8 * 8
            v = _vregs(k_side(*queue.pop(0), keep=keep, anchor=res[r:r + 8])[0])
            deps.append([_or_all(v[q::4]) for q in range(4)])
        return deps

    kwork = {}

    def k_after(m, res):
        if m in (0, 2):
            kwork[m + 1] = run_queue(4, res)

    def v_prep(lo, hi):
        for rb in range(lo, hi, 128):
            for c in range(0, HK, 128):
                raw = [wqkv_v[side * HK + c:side * HK + c + 128,
                              2 * D + half * HK + rb:2 * D + half * HK + rb + 128].T
                       for half in range(2) for side in range(2)]
                blocks = [t.astype(f32) for t in raw]
                for n, spec in enumerate(_SA):
                    t = raw[spec[0]] if spec[1] is None else _combo(blocks, spec).astype(bf16)
                    wsv_v[rb // 2:rb // 2 + 64, n * HK + c:n * HK + c + 128] = _pk(t)

    VS = HK // 2

    def k_before(m):
        if m == 5:
            cp_wv.wait()
            cp_x2.wait()
            v_prep(0, VS)

    sproj(wsk_v, xs_v, 1, k_emit1, keep, kwork, k_before, k_after)

    def ln_anchored(xg, src, xd, dst, k, n, keep, res):
        which = list(range(k * 8 // n, (k + 1) * 8 // n))
        rows = [a * HK // len(which) // 16 * 16 for a in range(len(which))]
        pcs = ln1(xg, src, xd, dst, P2, which, keep, [res[r:r + R] for r in rows])
        return [[]] * (3 - len(pcs)) + pcs

    vt, parts = {}, {}
    wsv = wsv_v.at[pl.ds(0, D // 4)]
    work = {0: {}, 1: {}, 2: {}}

    def v_after(q):
        def after(m, res):
            t = 7 * q + m
            u = t + 1
            if 3 <= t < 13:
                work[u // 7][u % 7] = run_queue(-(-len(queue) // (13 - t)), res)
            elif 13 <= t < 20:
                work[u // 7][u % 7] = ln_anchored(x_v, T, xs_v, T, t - 13, 7, keep, res)
        return after

    sealed(wsv_v)
    v_prep(VS, HK)
    zero = pl.multiple_of(flag_s[1], 8)
    for q, lo in enumerate((0, zero + VS // 2)):
        sproj(wsv_v.at[pl.ds(lo, VS // 2)], xs_v, 0,
              lambda half, blk, val: parts.setdefault((blk, half), []).append(val), keep, work[q], None, v_after(q))
    vt.update({k: jnp.concatenate(v, axis=0) for k, v in parts.items()})
    sproj(wsv_v.at[pl.ds(zero, D // 4)], xs_v, 1, lambda half, blk, val: vt.__setitem__((2 + blk, half), val), keep, work[2], None, v_after(2))
    assert not queue
    phi_m = sealed(phi_v)
    for j in range(NP):
        kvacc_v[j] = kv_prod(vt, _upk(phi_m[j * 64:(j + 1) * 64, :]), j)
    cp_x3.wait()
    wait_bg(0)

    def p1_body(i, c):
        @pl.when(i == 2)
        def _():
            cp_x4.wait()
            wait_bg(1)

        @pl.when(i == 3)
        def _():
            wait_bg(2)

        keep = flag_s[0] > 0
        lo = jnp.minimum((i - 1) * DCH, F - DCH)
        sv = wd_v.at[pl.ds(pl.multiple_of(lo, 16), DCH)]
        dv = wdp_v.at[pl.ds(pl.multiple_of(lo // 2, 8), DCH // 2)]
        rp = repacker([(sv, dv, r, c) for r in range(0, DCH, 16) for c in range(0, D, 128)], keep)
        lo = jnp.minimum((i - 1) * OCH, HK - OCH)
        ov = wo_v.at[pl.ds(pl.multiple_of(lo, 16), HK + OCH)]
        od = wso_v.at[pl.ds(pl.multiple_of(lo // 2, 8), OCH // 2)]

        def k_emit(q):
            return lambda half, blk, val: k_side(half_groups(val, half), half_pairs(half), 2 * q + blk)

        vt = {}

        def v_emit(q):
            return lambda half, blk, val: vt.__setitem__((2 * q + blk, half), val)

        xd = xs_view(i, 2)
        xa = x_v.at[pl.ds(pl.multiple_of(i * T + P2, P2), P2)]
        xb = x_v.at[pl.ds(pl.multiple_of(jnp.minimum(i + 1, NT - 1) * T, T), P2)]
        wa = {}

        def a_after(m, res):
            if m < 6:
                wa[m + 1] = ln_anchored(xa, 0, xd, P2, m, 6, keep, res)

        sproj(wsv, xd, 0, v_emit(0), keep, wa, None, a_after)
        sproj(wsk_v, xd, 0, k_emit(0), after=rp[0])
        sproj(wsk_v, xd, 1, k_emit(1), after=rp[1])
        wb = spread(ln1(xb, 0, xd, T, P2), [(0, m) for m in range(1, 7)])[0]

        def b_after(m, res):
            slabs = list(range(0, OCH, 16))
            mine = slabs[(m - 1) * len(slabs) // 6:m * len(slabs) // 6] if m else []
            for n, r in enumerate(mine):
                rows = [((4 * n + c) * HK // (4 * len(mine))) // 16 * 16 for c in range(4)]
                store_combos(od, r // 2, ov[r:r + 16, :].astype(f32), ov[HK + r:HK + r + 16, :].astype(f32),
                             _SB, keep, [res[a:a + R] for a in rows])

        sproj(wsv, xd, 1, v_emit(1), keep, wb, None, b_after)
        phi_m = sealed(phi_v)
        for j in range(NP):
            kvacc_v[j] += kv_prod(vt, _upk(phi_m[j * 64:(j + 1) * 64, :]), j)
        return c

    lax.fori_loop(1, NT, p1_body, 0)

    wait_all([cp_wr, cp_wq] + cp_gu[0])
    keep = flag_s[0] > 0
    kv_mask = (lax.broadcasted_iota(jnp.int32, (64, 128), 0) // DH
               == (lax.broadcasted_iota(jnp.int32, (64, 128), 1) // DH) % 2)
    ties = [{} for _ in range(16)]
    for j in range(NP):
        kvj = jnp.where(kv_mask, kvacc_v[j], 0.0)
        kv_v[:, j * 128:(j + 1) * 128] = _pk(kvj.astype(bf16))
        zj = _lanes(jnp.sum(zacc_v[j * 128:(j + 1) * 128, :], axis=-1, keepdims=True))
        zacc_v[j * 128:(j + 1) * 128, :] = zj
        vals = _vregs(kvj) + _vregs(zj)
        if j + 1 < 16:
            for q in range(4):
                ties[j + 1][(32 + q * 8, 0)] = _or_all(vals[q::4])
    wr = wr_v[0:8, :].astype(f32)
    wl = jnp.sum(wr, axis=0, keepdims=True)
    wsum = jnp.sum(wl, axis=1, keepdims=True)
    wrb_v[:, 0:D + 256] = jnp.concatenate(
        [jnp.broadcast_to(wr[j:j + 1, :], (8, 128)) for j in range(8)]
        + [jnp.broadcast_to(wsum, (8, 128)), jnp.broadcast_to(wl, (8, 128))], axis=1)
    for t in range(NT):
        store_xt(t, xs_v, t * (T // 4))
    fq = (Folder(0), Folder(0, NV // 2))
    for g in range(4):
        new = fold_pair(fq, g, keep, ties[4 * g:4 * g + 4])
        for pos, slab in new[0].items():
            store_combos(wsq_v, pos * 4, slab, new[1][pos + NV // 2])

    pq_v = (pq0_v, pq1_v, pq2_v, pq3_v)

    def views_of(g):
        lo = g * (BPI * B)
        if not isinstance(g, int):
            lo = pl.multiple_of(lo, BPI * B)
        return ((x_v.at[pl.ds(lo, BPI * B)],)
                + tuple(ref.at[pl.ds(lo, P2 + BPI * B)] for ref in (h_v, out_v, st_v)) + (g,))

    def stage_q(xd, q, first, before, after):
        def emit(half, blk, val):
            group = half_groups(val, half)
            for j in half_pairs(half):
                p, j = _pair_logits(group, j), _phys_pair(j)
                ph = _hedgehog_t(p, zacc_v[j * 128:(j + 1) * 128, :])
                pq_v[2 * q + blk][(j // 2) * 64:(j // 2 + 1) * 64, (j % 2) * B:(j % 2 + 1) * B] = _pk(ph.astype(bf16))

        sproj(wsq_v, xd, q, emit, before=before, after=after, first=first)

    oc_v = (oc0_v, oc1_v)

    def stage_g(q):
        pq = [sealed(pq_v[2 * q + blk]) for blk in range(2)]
        for t in range(NP // 4):
            parts = [[_dot_nn(_upk(kv_v[:, j * 128:(j + 1) * 128]),
                              _upk(pq[blk][(j // 2) * 64:(j // 2 + 1) * 64, (j % 2) * B:(j % 2 + 1) * B]))
                      for blk in range(2) for j in (jj, jj + NP // 2)] for jj in (2 * t, 2 * t + 1)]
            blocks = [jnp.concatenate([a, b], axis=0) for a, b in zip(*parts)]
            for m, spec in enumerate(_SA):
                c = m * HK + t * 128
                oc_v[q][0:B // 2, c:c + 128] = _pk(_combo(blocks, spec).astype(bf16).T)

    def stage_h(views, q, keep, pieces, jobs, before=None):
        x_g, h_g = views[0], views[1]
        oc = sealed(oc_v[q])
        first, last = 4, 12
        ties = [{} for _ in range(7)]
        for k, vals in enumerate(pieces):
            t = first + k * (last - first) // max(len(pieces) - 1, 1)
            for m, val in enumerate(vals):
                ties[t // 4][(m * 8, (t % 4) * 128)] = val
        state = {}
        done = [0]

        def product(m):
            if before:
                before(m)
            w = wso_v[:, m * HK:(m + 1) * HK]
            if ties[m]:
                w = _tie(keep, w, ties[m])
            done[0] = m
            res = _dot_nn(_upk(oc[0:B // 2, m * HK:(m + 1) * HK]), _upk(w))
            for k, job in enumerate(jobs):
                t = 2 * q + k * (24 - 4 * q) // len(jobs)
                if t // 4 == m:
                    job(res[0:R, (t % 4) * 128:(t % 4 + 1) * 128])
            return res

        def wmul(d, lo):
            return (d.reshape(B // 8, 8, 128) * wrb_v[:, lo:lo + 128][None]).reshape(B, 128)

        def emit(k, val):
            blk, half = k // 2, k % 2
            s = 2 * q + blk
            cols = slice(half * HK, (half + 1) * HK)
            h = x_g[s * B:(s + 1) * B, cols].astype(f32) + val
            h_g[(s + 2) * B:(s + 3) * B, cols] = h
            st = state.setdefault(blk, {'h': {}})
            st['h'][half] = h
            for c in range(0, HK, 128):
                ht = h[:, c:c + 128]
                if 'h0' not in st:
                    st['h0'] = ht
                    continue
                d = ht - st['h0']
                new = (d, d * d, wmul(d, half * HK + c))
                st['s'] = new if 's' not in st else tuple(a + b for a, b in zip(st['s'], new))
            if len(st['h']) == 1:
                vals = [_or_all(list(v)) for v in zip(*[_vregs(a) for a in st['s']])]
                m = done[0] + 2
                for n, val in enumerate(vals):
                    ties[m][(248 - (n % 4) * 8, (n // 4) * 128)] = val

        _strassen(product, emit)

        res = []
        for blk in range(2):
            st = state[blk]
            s1, s2, s3 = st['s']
            c0 = _lanes(jnp.mean(st['h0'], axis=-1, keepdims=True))
            g0 = st['h0'] - c0
            t1 = s1 + 8.0 * g0
            t2 = s2 + g0 * (s1 + t1)
            t3 = s3 + wmul(g0, D + 128)
            res.append((jnp.concatenate([t1, t2, t3, c0], axis=1),
                        jnp.concatenate([st['h'][0], st['h'][1]], axis=1)))
        return res

    def stage_stats(views, s, part, valid=None):
        st_g, g = views[3], views[4]
        b = g * BPI + s
        bv = bestv_v[...]
        bi = besti_v[...]
        wsum = wrb_v[0:1, D:D + 128]
        nvs, nis, sts = [], [], []
        for k in range(B // R):
            sl = slice(k * R, (k + 1) * R)
            red = [_lanes(jnp.sum(part[sl, n * 128:(n + 1) * 128], axis=-1, keepdims=True)) for n in range(3)]
            mu = red[0] * (1.0 / D)
            var = jnp.maximum(red[1] * (1.0 / D) - mu * mu, 0.0)
            rs = lax.rsqrt(var + LN_EPS)
            r = (red[2] - mu * wsum) * rs
            sts.append(jnp.concatenate([rs, (mu + part[sl, 384:512]) * rs], axis=1))
            if valid is not None:
                r = jnp.where(valid, r, -jnp.inf)
            idx = lax.broadcasted_iota(jnp.int32, (R, 128), 0) + (b * B + k * R)
            better = r > bv[sl]
            nvs.append(jnp.where(better, r, bv[sl]))
            nis.append(jnp.where(better, idx, bi[sl]))
        st = jnp.concatenate(sts, axis=0)
        st_g[(s + 2) * B:(s + 3) * B, :] = st
        bestv_v[...] = jnp.concatenate(nvs, axis=0)
        besti_v[...] = jnp.concatenate(nis, axis=0)
        return st, [_vregs(nv) for nv in nvs]

    def out_jobs(views, s, keep, st=None, h=None):
        h_g, out_g, st_g = views[1], views[2], views[3]

        def job(k):
            def run(anchor):
                rows = slice((s + 2) * B + k * R, (s + 2) * B + (k + 1) * R)
                hk = h_g[rows, :] if h is None else h[k * R:(k + 1) * R]
                sk = st_g[rows, :] if st is None else st[k * R:(k + 1) * R]
                a = 1.0 + jnp.where(keep, sk[:, 0:128], anchor)
                o = [hk[:, c * 128:(c + 1) * 128] * a - sk[:, 128:256] for c in range(D // 128)]
                out_g[rows, :] = jnp.concatenate(o, axis=1).astype(bf16)
            return run
        return [job(k) for k in range(B // R)]

    def p2_body(i, c):
        b0 = i * BPI
        keep = flag_s[0] > 0
        cur = views_of(i)
        st, pieces = stage_stats(cur, -1, pend_v[...], i > 0)
        ojobs = out_jobs(cur, -2, keep) + out_jobs(cur, -1, keep, st)
        n = D // NI
        jobs = []
        for src, dst in ((wg_v, wgp_v), (wu_v, wup_v)):
            sv = src.at[pl.ds(pl.multiple_of(i * n, n), n)]
            dv = dst.at[pl.ds(pl.multiple_of(i * (n // 2), n // 2), n // 2)]
            jobs += [(sv, dv, r, cc) for r in range(0, n, 16) for cc in range(0, NM, 128)]
        rp = repacker(jobs, keep)
        stage_q(xs_view(i, 1), 0, xt_view(i), None, rp[0])
        stage_q(xs_view(i, 1), 1, None, lambda m: stage_g(0) if m == 2 else None, rp[1])
        res = stage_h(cur, 0, keep, pieces, ojobs, lambda m: stage_g(1) if m == 1 else None)
        st0, _ = stage_stats(cur, 0, res[0][0])
        st1, pieces = stage_stats(cur, 1, res[1][0])
        ojobs = out_jobs(cur, 0, keep, st0, res[0][1]) + out_jobs(cur, 1, keep, st1, res[1][1])
        res = stage_h(cur, 1, keep, pieces, ojobs)
        stage_stats(cur, BPI - 2, res[0][0])
        pend_v[...] = res[1][0]

        @pl.when(i > 0)
        def _():
            cp_out(jnp.maximum(b0 - 2, 0), 2).start()

        cp_out(b0, 2).start()
        return c

    lax.fori_loop(0, NI, p2_body, 0)
    wait_all(cp_gu[1])
    keep = flag_s[0] > 0
    last = views_of(NI - 1)

    st, _ = stage_stats(last, BPI - 1, pend_v[...])

    bv = bestv_v[...]
    mval = jnp.max(bv, axis=0, keepdims=True)
    sel = jnp.min(jnp.where(bv == mval, besti_v[...], S - 1), axis=0, keepdims=True)
    idx = sel[0, 0]
    hrow = h_v[pl.ds(P2 + idx, 1), :]
    strow = st_v[pl.ds(P2 + idx, 1), :]
    xrow = jnp.concatenate([hrow[:, c * 128:(c + 1) * 128] * strow[:, 0:128] - strow[:, 128:256]
                            for c in range(D // 128)], axis=1).astype(bf16)
    xs = jnp.broadcast_to(xrow, (16, D))
    g_first = _dot_nn(xs, _upk(wgp_v[:, 0:FC]))
    anchors = ([jnp.broadcast_to(pltpu.bitcast(sel, f32), (R, 128))] * 4
               + [jnp.broadcast_to(xrow[:, 0:128].astype(f32), (R, 128))] * 4
               + [g_first[:, (k // 2) * 128:(k // 2 + 1) * 128] for k in range(8)])
    for job, anchor in zip(out_jobs(last, BPI - 2, keep) + out_jobs(last, BPI - 1, keep, st), anchors):
        job(anchor)
    cp_out(NB - 2, 2).start()

    def act(g, u):
        a = g * pl.reciprocal(1.0 + jnp.exp(-g), approx=True) * u
        return jnp.concatenate([a, a], axis=0).astype(bf16)

    def down(a, lo, w):
        return _dot_nn(a, _upk(wdp_v[lo // 2:(lo + w) // 2, 0:D]))[0:8]

    xcol = jnp.broadcast_to(xrow, (128, D)).T.astype(f32)
    jobs = [(which, b) for b in range(NBV) for which in (0, 1)]
    vres, prev = {}, None
    for j0 in range(0, len(jobs), NCH):
        grp = jobs[j0:j0 + NCH]
        accs = [None] * len(grp)
        for r in range(D // 16):
            for n, (which, b) in enumerate(grp):
                w = (wg_v, wu_v)[which][r * 16:(r + 1) * 16, NM + b * 128:NM + (b + 1) * 128].astype(f32)
                t0 = w[0:8] * xcol[r * 16:r * 16 + 8]
                t1 = w[8:16] * xcol[r * 16 + 8:r * 16 + 16]
                if accs[n] is None:
                    if prev is not None:
                        t0 = jnp.where(keep, t0, prev[n % len(prev)])
                    accs[n] = t0 + t1
                else:
                    accs[n] = (accs[n] + t0) + t1
        prev = accs
        for n, job in enumerate(grp):
            vres[job] = _allreduce8(accs[n][None], jnp.add)[0]

    chunks = [(lo, min(FC, NM - lo)) for lo in range(0, NM, FC)]
    acts, y = [], None
    for k, (lo, w) in enumerate(chunks):
        g = g_first if k == 0 else _dot_nn(xs, _upk(wgp_v[:, lo:lo + w]))
        u = _dot_nn(xs, _upk(wup_v[:, lo:lo + w]))
        acts.append(act(g[0:8], u[0:8]))
        if k >= 1:
            t = down(acts[k - 1], *chunks[k - 1])
            y = t if y is None else y + t
    y = y + down(acts[-1], *chunks[-1])
    for b0, nb in ((0, 4), (4, 4), (8, 4), (12, 1)):
        g = jnp.concatenate([vres[(0, b)] for b in range(b0, b0 + nb)], axis=1)
        u = jnp.concatenate([vres[(1, b)] for b in range(b0, b0 + nb)], axis=1)
        y = y + down(act(g, u), NM + b0 * 128, nb * 128)

    gate = jnp.broadcast_to(jax.nn.sigmoid(mval), (8, 128))
    base = pl.multiple_of((idx >> 4) << 4, 16)
    rows = pl.ds(pl.multiple_of(P2 + base, 16), 16)
    h16 = h_v[rows, :]
    st16 = st_v[rows, :]
    a16 = 1.0 + st16[:, 0:128]
    m16 = st16[:, 128:256]
    hit = (lax.broadcasted_iota(jnp.int32, (16, 128), 0) + base) == idx
    res = []
    for c in range(D // 128):
        yc = y[:, c * 128:(c + 1) * 128] * gate
        yc = jnp.concatenate([yc, yc], axis=0)
        res.append(h16[:, c * 128:(c + 1) * 128] * a16 - m16 + jnp.where(hit, yc, 0.0))
    res = jnp.concatenate(res, axis=1).astype(bf16)
    for i in range(NI):
        cp_out(i * BPI, 2).wait()
        cp_out(i * BPI + 2, 2).wait()
    out_v[rows, :] = res
    fix = pltpu.make_async_copy(out_v.at[rows], out_hbm.at[pl.ds(base, 16)], sem_o.at[0])
    fix.start()
    fix.wait()


@jax.jit
def pallas_sequential_preLN__linear_kernel_hedgehog__moe_arch_mod__prompt_kernel(
    A_x: jax.Array,
    A_wqkv: jax.Array,
    A_w_phi: jax.Array,
    A_wo: jax.Array,
    B_x: jax.Array,
    B_w_r: jax.Array,
    B_w_gate: jax.Array,
    B_w_up: jax.Array,
    B_w_down: jax.Array,
):
    del B_x
    x = A_x.reshape(S, D)
    wphi = A_w_phi.reshape(H * DH, DH)
    wr = B_w_r.reshape(8, 128)
    any_spec = pl.BlockSpec(memory_space=pl.ANY)
    out = pl.pallas_call(
        _kernel,
        out_shape=jax.ShapeDtypeStruct((S, D), bf16),
        in_specs=[any_spec] * 8,
        out_specs=any_spec,
        scratch_shapes=[
            pltpu.VMEM((S, D), bf16),
            pltpu.VMEM((D, 3 * D), bf16),
            pltpu.VMEM((H * DH, DH), bf16),
            pltpu.VMEM((D, D), bf16),
            pltpu.VMEM((64, 128), bf16),
            pltpu.VMEM((D, F + 128), bf16),
            pltpu.VMEM((D, F + 128), bf16),
            pltpu.VMEM((F, D), bf16),
            pltpu.VMEM((PR, D), u32),
            pltpu.VMEM((PR // 2, 7 * HK), u32),
            pltpu.VMEM((PR // 2, 7 * HK), u32),
            pltpu.VMEM((D // 4 + 8, 7 * HK), u32),
            pltpu.VMEM((D // 4, 7 * HK), u32),
            pltpu.VMEM((F // 2, D + 128), u32),
            pltpu.VMEM((D // 2, NM), u32),
            pltpu.VMEM((D // 2, NM), u32),
            pltpu.VMEM((64, 8 * 128), u32),
            pltpu.VMEM((T0 // 2, D), u32),
            pltpu.VMEM(((S + T) // 4, 7 * HK), u32),
            pltpu.VMEM((NT * (HK // 2), B), u32),
            pltpu.VMEM((NP, 64, 128), f32),
            pltpu.VMEM((2 * D, 128), f32),
            pltpu.VMEM((32, NP * 128), u32),
            pltpu.VMEM((D + 8, T), u32),
            pltpu.VMEM((D // 2 + 16, 2 * B), u32),
            pltpu.VMEM((D // 2 + 16, 2 * B), u32),
            pltpu.VMEM((D // 2 + 16, 2 * B), u32),
            pltpu.VMEM((D // 2 + 16, 2 * B), u32),
            pltpu.VMEM((B // 2 + 8, 7 * HK), u32),
            pltpu.VMEM((B // 2 + 8, 7 * HK), u32),
            pltpu.VMEM((P2 + S, D), f32),
            pltpu.VMEM((P2 + S, 256), f32),
            pltpu.VMEM((B, 512), f32),
            pltpu.VMEM((P2 + S, D), bf16),
            pltpu.VMEM((8, D + 512), f32),
            pltpu.VMEM((B, 128), f32),
            pltpu.VMEM((B, 128), jnp.int32),
            pltpu.SMEM((2,), jnp.int32),
            pltpu.SemaphoreType.DMA((_NSEM_IN,)),
            pltpu.SemaphoreType.DMA((1,)),
        ],
        compiler_params=pltpu.CompilerParams(vmem_limit_bytes=110 * 1024 * 1024,
                                             disable_bounds_checks=True,
                                             disable_semaphore_checks=True),
        name="hedgehog_mod",
    )(x, A_wqkv, wphi, A_wo, wr, B_w_gate, B_w_up, B_w_down)
    return out.reshape(1, S, D)
```

```python
import jax
import jax.numpy as jnp
from jax import lax
import jax.experimental.pallas as pl
import jax.experimental.pallas.tpu as pltpu

S = 2048
D = 1024
H = 32
DH = 32
F = 3584
T = 512
NT = S // T
T0 = 256
B = 128
NB = S // B
BPI = 4
NI = NB // BPI
NP = H // 2
FC = 1024
R = 16
NBV = 13
NM = F - NBV * 128
NCH = 4
OCH = 176
DCH = 1216
NV = 124
PR = NV * 4
HK = D // 2
P2 = 2 * B
LOG2E = 1.4426950408889634
LN_EPS = 1e-5
DEN_EPS = 1e-6

_NT_DIMS = (((1,), (1,)), ((), ()))

bf16 = jnp.bfloat16
f32 = jnp.float32
u32 = jnp.uint32


def _dot_nt(a, b):
    return lax.dot_general(a, b, _NT_DIMS, preferred_element_type=f32)


def _dot_nn(a, b):
    return jnp.dot(a, b, preferred_element_type=f32)


def _pk(x):
    return pltpu.bitcast(x, u32)


def _upk(x):
    return pltpu.bitcast(x, bf16)


def _lanes(x):
    return jnp.broadcast_to(x, (x.shape[0], 128))


def _layernorm(x):
    m = jnp.mean(x, axis=-1, keepdims=True)
    xc = x - m
    v = jnp.mean(xc * xc, axis=-1, keepdims=True)
    return xc * lax.rsqrt(v + LN_EPS)


def _allreduce8(x, op):
    x = op(x, pltpu.roll(x, 4, 1))
    x = op(x, pltpu.roll(x, 2, 1))
    x = op(x, pltpu.roll(x, 1, 1))
    return x


def _hedgehog_t(p, z=None):
    t = p.shape[-1]
    p4 = p.reshape(2, 4, 8, t)
    mx = _allreduce8(jnp.max(p4, axis=1), jnp.maximum)
    mn = _allreduce8(jnp.min(p4, axis=1), jnp.minimum)
    ep = jnp.exp2(p4 - mx[:, None])
    en = jnp.exp2(mn[:, None] - p4)
    a = pl.reciprocal(_allreduce8(jnp.sum(ep, axis=1), jnp.add), approx=True)
    b = pl.reciprocal(_allreduce8(jnp.sum(en, axis=1), jnp.add), approx=True)
    if z is not None:
        dp = jnp.sum(ep * z[0:64].reshape(2, 4, 8, t), axis=1)
        dn = jnp.sum(en * z[64:128].reshape(2, 4, 8, t), axis=1)
        den = _allreduce8(dp * a + dn * b, jnp.add) + DEN_EPS
        inv = pl.reciprocal(den, approx=True)
        a = a * inv
        b = b * inv
    fp = (ep * a[:, None]).reshape(64, t)
    fn = (en * b[:, None]).reshape(64, t)
    return jnp.concatenate([fp, fn], axis=0)


_SA = ((3, None, 0), (2, 3, 1), (0, 1, 1), (0, None, 0), (0, 3, 1), (1, 3, -1), (2, 0, -1))
_SB = ((2, 0, -1), (0, None, 0), (3, None, 0), (1, 3, -1), (0, 3, 1), (2, 3, 1), (0, 1, 1))


def _combo(blocks, spec):
    a, b, sign = spec
    if b is None:
        return blocks[a]
    return blocks[a] + blocks[b] if sign > 0 else blocks[a] - blocks[b]


def _strassen(product, emit):
    m4 = product(0)
    m2 = product(1)
    emit(2, m4 + m2)
    m5 = product(2)
    u = m4 - m5
    m3 = product(3)
    emit(1, m5 + m3)
    v = m3 - m2
    m1 = product(4)
    u = u + m1
    v = v + m1
    emit(0, u + product(5))
    emit(3, v + product(6))


def _head_groups(h):
    base, k = (NV // 4) * (h // 8), h % 8
    return ([base + 4 * k + i for i in range(3)],
            base + 4 * k - 1 if k > 0 else None,
            base + 4 * k + 3 if k < 7 else None,
            8 - k)


def _pair_logits(group, j):
    parts = []
    for h in (2 * j, 2 * j + 1):
        full, below, above, a = _head_groups(h)
        ref = group(full[0])
        sub = lax.broadcasted_iota(jnp.int32, ref.shape, 0)
        if above is None:
            m = jnp.where(sub >= a, group(below), 0.0)
        else:
            m = jnp.where(sub == a - 1, 0.0, group(above))
            if below is not None:
                m = jnp.where(sub >= a, group(below), m)
        parts += [m] + [group(q) for q in full]
    return jnp.concatenate(parts, axis=0)


def _pair_need(j):
    full, _, above, _ = _head_groups(2 * j + 1)
    return full[2] if above is None else above


def _tie(keep, w, ties):
    rows = sorted({r for r, _ in ties})
    out, pos = [], 0
    for r in rows:
        if r > pos:
            out.append(w[pos:r])
        cols = sorted(c for rr, c in ties if rr == r)
        parts, cpos = [], 0
        for c in cols:
            if c > cpos:
                parts.append(w[r:r + 8, cpos:c])
            parts.append(jnp.where(keep, w[r:r + 8, c:c + 128], ties[(r, c)]))
            cpos = c + 128
        if cpos < w.shape[1]:
            parts.append(w[r:r + 8, cpos:])
        out.append(jnp.concatenate(parts, axis=1) if len(parts) > 1 else parts[0])
        pos = r + 8
    if pos < w.shape[0]:
        out.append(w[pos:])
    return jnp.concatenate(out, axis=0)


def _vregs(x):
    if x.dtype != u32:
        x = pltpu.bitcast(x, u32)
    return [x[r:r + 8, c:c + 128] for r in range(0, x.shape[0], 8) for c in range(0, x.shape[1], 128)]


def _or_all(vals):
    acc = vals[0]
    for v in vals[1:]:
        acc = acc | v
    return acc


def _phys_group(g):
    return 2 * (g % 4) + g // 4


def _phys_pair(j):
    return 2 * _phys_group(j // 2) + j % 2


_KSTAGES = (((0, 2),), ((2, 3),), ((5, 3),))
_PSTAGES = (((0, 5),), ((5, 3),))
_NSEM_IN = 11


def _kernel(x_hbm, wqkv_hbm, wphi_hbm, wo_hbm, wr_hbm, wg_hbm, wu_hbm, wd_hbm,
            out_hbm,
            x_v, wqkv_v, wphi_v, wo_v, wr_v, wg_v, wu_v, wd_v,
            wtk_v, wsq_v, wsk_v, wsv_v, wso_v, wdp_v, wgp_v, wup_v, amat_v, xn_v, xs_v, xt_v,
            kvacc_v, zacc_v, kv_v, phi_v,
            pq0_v, pq1_v, pq2_v, pq3_v, oc0_v, oc1_v, h_v, st_v, pend_v, out_v, wrb_v,
            bestv_v, besti_v, flag_s,
            sem_i, sem_o):

    def cp_x(lo, n, sem):
        return pltpu.make_async_copy(x_hbm.at[pl.ds(lo, n)], x_v.at[pl.ds(lo, n)], sem_i.at[sem])

    def cp_w(lo, w, sem):
        return pltpu.make_async_copy(wqkv_hbm.at[:, pl.ds(lo, w)], wqkv_v.at[:, pl.ds(lo, w)], sem_i.at[sem])

    cp_k = [[cp_w(D + g * 128, n * 128, 2 + c) for g, n in st] for c, st in enumerate(_KSTAGES)]
    cp_p = [[pltpu.make_async_copy(wphi_hbm.at[pl.ds(g * 128, n * 128)], wphi_v.at[pl.ds(g * 128, n * 128)],
                                   sem_i.at[3 * c]) for g, n in st] for c, st in enumerate(_PSTAGES)]
    cp_wv = cp_w(2 * D, D, 5)
    cp_wq = cp_w(0, D, 7)

    def cp_wd(k):
        lo, n = k * DCH, min(DCH, F - k * DCH)
        return pltpu.make_async_copy(wd_hbm.at[pl.ds(lo, n)], wd_v.at[pl.ds(lo, n)], sem_i.at[(6, 8, 9)[k]])

    cp_x0 = cp_x(0, T0, 1)
    cp_x1 = cp_x(T0, T0, 4)
    cp_x2 = cp_x(T, P2, 5)
    cp_x3 = cp_x(T + P2, T, 6)
    cp_x4 = cp_x(2 * T + P2, S - 2 * T - P2, 8)
    cp_wr = pltpu.make_async_copy(wr_hbm, wr_v.at[pl.ds(0, 8)], sem_i.at[7])

    def cp_wo(k, half):
        lo, n = k * OCH, min(OCH, HK - k * OCH)
        rows = pl.ds(half * HK + lo, n)
        return pltpu.make_async_copy(wo_hbm.at[rows], wo_v.at[rows], sem_i.at[(6, 8, 9)[k]])

    def wait_bg(k):
        cp_wo(k, 0).wait()
        cp_wo(k, 1).wait()
        cp_wd(k).wait()

    cp_gu = [[pltpu.make_async_copy(src.at[:, pl.ds(lo, n)], dst.at[:, pl.ds(lo, n)], sem_i.at[sem])
              for src, dst in ((wg_hbm, wg_v), (wu_hbm, wu_v))] for lo, n, sem in ((0, NM, 7), (NM, F - NM, 10))]

    def cp_out(b, n):
        lo = b * B
        if not isinstance(b, int):
            lo = pl.multiple_of(lo, B)
        return pltpu.make_async_copy(out_v.at[pl.ds(P2 + lo, n * B)], out_hbm.at[pl.ds(lo, n * B)], sem_o.at[0])

    for cp in (*cp_p[0], cp_x0, *cp_k[0], *cp_p[1], *cp_k[1], *cp_k[2], cp_x1, cp_wv, cp_x2,
               cp_x3, cp_wo(0, 0), cp_wo(0, 1), cp_wd(0), cp_x4, cp_wo(1, 0), cp_wo(1, 1), cp_wd(1),
               cp_wo(2, 0), cp_wo(2, 1), cp_wd(2), cp_wr, cp_wq, *cp_gu[0], *cp_gu[1]):
        cp.start()
    flag_s[0] = 1
    flag_s[1] = 0

    def ln1(xg, src, xd, dst, n, which=None, keep=None, anchors=None, plain=False):
        pieces = []
        for pr in range(n // P2):
            for k in range(B // R):
                off = pr * P2 + k * R
                if which is not None and pr * (B // R) + k not in which:
                    continue
                x0 = xg[src + off:src + off + R, :].astype(f32)
                x1 = xg[src + off + B:src + off + B + R, :].astype(f32)
                if anchors is not None:
                    a = anchors[len(pieces)]
                    x0 = jnp.concatenate([jnp.where(keep, x0[:, :128], a), x0[:, 128:]], axis=1)
                    x1 = jnp.concatenate([jnp.where(keep, x1[:, :128], a), x1[:, 128:]], axis=1)
                p0 = _layernorm(x0)
                p1 = _layernorm(x1)
                if plain:
                    xn_v[off // 2:(off + R) // 2, :] = _pk(p0.astype(bf16))
                    xn_v[(off + B) // 2:(off + B + R) // 2, :] = _pk(p1.astype(bf16))
                lo = (dst + pr * P2) // 4 + k * (R // 2)
                blocks = (p0[:, :HK], p1[:, :HK], p0[:, HK:], p1[:, HK:])
                vs = []
                for m, spec in enumerate(_SB):
                    t = _combo(blocks, spec)
                    xd[lo:lo + R // 2, m * HK:(m + 1) * HK] = _pk(t.astype(bf16))
                    if spec[1] is not None:
                        vs.append(_vregs(t))
                pieces.append([_or_all(list(col)) for col in zip(*vs)])
        return pieces

    def load_xn(b):
        return _upk(xn_v[b * (B // 2):(b + 1) * (B // 2), :])

    def piece_ties(pieces, n, row0=0, col=0):
        ties = {}
        if pieces:
            step = (n - row0) // len(pieces) // 8 * 8
            for k, p in enumerate(pieces):
                for q, val in enumerate(p):
                    ties[(row0 + k * step + (q // 4) * 8, col + (q % 4) * 128)] = val
        return ties

    def xs_view(i, tiles):
        return xs_v.at[pl.ds(pl.multiple_of(i * (T // 4), T // 4), tiles * (T // 4))]

    def xt_view(i):
        lo = i * (HK // 2)
        return xt_v.at[pl.ds(lo if isinstance(i, int) else pl.multiple_of(lo, HK // 2), HK // 2)]

    def store_xt(i, xd, row, keep=None, anchor=None):
        v = xd[row:row + B // 2, 0:HK]
        if anchor is not None:
            v = _tie(keep, v, {(0, c): anchor for c in range(0, HK, 128)})
        xt_view(i)[...] = _pk(_upk(v).T)

    def sproj(ws, xd, pr, emit, keep=None, work=None, before=None, after=None, first=None):
        lo = pr * (B // 2)

        def product(m):
            if before:
                before(m)
            lhs = ws[:, m * HK:(m + 1) * HK]
            if work is not None and work.get(m):
                lhs = _tie(keep, lhs, piece_ties(work[m], lhs.shape[0], 32))
            if m == 0 and first is not None:
                res = _dot_nn(_upk(lhs), _upk(first[...]))
            else:
                res = _dot_nt(_upk(lhs), _upk(xd[lo:lo + B // 2, m * HK:(m + 1) * HK]))
            if after:
                after(m, res)
            return res

        _strassen(product, lambda k, val: emit(k // 2, k % 2, val))

    def repacker(jobs, keep):
        def hook(q):
            def after(m, res):
                if m in (0, 2, 4):
                    k = 3 * q + m // 2
                    mine = jobs[k * len(jobs) // 6:(k + 1) * len(jobs) // 6]
                    for n, (sv, dv, r, c) in enumerate(mine):
                        a = (64 + n * 416 // len(mine)) // 8 * 8
                        dv[r // 2:r // 2 + 8, c:c + 128] = jnp.where(keep, _pk(sv[r:r + 16, c:c + 128]),
                                                                     pltpu.bitcast(res[a:a + 8], u32))
            return after
        return hook(0), hook(1)

    def spread(pieces, slots):
        res = {}
        for k, (pr, m) in enumerate(slots):
            res.setdefault(pr, {})[m] = pieces[k * len(pieces) // len(slots):(k + 1) * len(pieces) // len(slots)]
        return res

    def sealed(ref):
        ref[pl.ds(pl.multiple_of(flag_s[1] + ref.shape[0] - 8, 8), 8), 0:128] = jnp.zeros((8, 128), u32)
        return ref

    def store_combos(ws, row, top, bot, table=_SA, keep=None, anchors=None):
        for c in range(0, HK, 128):
            blocks = [top[:, c:c + 128], top[:, HK + c:HK + c + 128], bot[:, c:c + 128], bot[:, HK + c:HK + c + 128]]
            if anchors is not None:
                for q in (0, 3):
                    blocks[q] = jnp.where(keep, blocks[q], anchors[c // 128])
            for m, spec in enumerate(table):
                ws[row:row + 8, m * HK + c:m * HK + c + 128] = _pk(_combo(blocks, spec).astype(bf16))

    zinit = set()

    def k_side(group, pairs, slot, keep=None, anchor=None):
        res = []
        for j in pairs:
            p = _pair_logits(group, j)
            if anchor is not None:
                p = jnp.concatenate([jnp.where(keep, p[0:8], anchor), p[8:32],
                                     jnp.where(keep, p[32:40], anchor), p[40:64]], axis=0)
            ph = _hedgehog_t(p)
            j = _phys_pair(j)
            if j not in zinit:
                zinit.add(j)
                zacc_v[j * 128:(j + 1) * 128, :] = ph
            else:
                zacc_v[j * 128:(j + 1) * 128, :] += ph
            phi_v[j * 64:(j + 1) * 64, slot * B:(slot + 1) * B] = _pk(ph.astype(bf16))
            res.append(ph)
        return res

    def half_groups(p, half):
        return lambda pos: p[(pos - half * (NV // 2)) * 8:(pos - half * (NV // 2) + 1) * 8]

    def half_pairs(half):
        return range(half * (NP // 2), (half + 1) * (NP // 2))

    def kv_prod(vt, ph, j):
        half, r = j // (NP // 2), (j % (NP // 2)) * 64
        v = jnp.concatenate([vt[(s, half)][r:r + 64] for s in range(T // B)], axis=1).astype(bf16)
        return _dot_nt(v, ph)

    eye = (lax.broadcasted_iota(jnp.int32, (DH, DH), 0)
           == lax.broadcasted_iota(jnp.int32, (DH, DH), 1)).astype(bf16)
    r_h = lax.broadcasted_iota(jnp.int32, (128, 128), 0) // DH
    c_h = lax.broadcasted_iota(jnp.int32, (128, 128), 1) // DH
    same_head = r_h == c_h

    def make_amat(g):
        a = jnp.concatenate([_dot_nt(eye, wphi_v[g * 128:(g + 1) * 128, :])] * 4, axis=0)
        amat_v[:, g * 128:(g + 1) * 128] = _pk(jnp.where(same_head, a, 0.0).astype(bf16))

    class Folder:
        def __init__(self, col0, first=0):
            self.col0, self.rows, self.mprev, self.done = col0, {}, None, first

        def tile(self, g, rows, keep=None, ties=None):
            g = _phys_group(g)
            am = amat_v[:, g * 128:(g + 1) * 128]
            if ties:
                am = _tie(keep, am, ties)
            return _dot_nt(_upk(am), wqkv_v[rows, self.col0 + g * 128:self.col0 + (g + 1) * 128])

        def fold(self, g, wt=None):
            sub = lax.broadcasted_iota(jnp.int32, (8, D), 0)
            if wt is None:
                wt = self.tile(g, slice(None))
            for hh in range(4):
                full, below, _, a = _head_groups(4 * g + hh)
                r0 = hh * DH
                ref = jnp.broadcast_to(wt[r0 + a - 1:r0 + a, :], (8, D))
                part = [(wt[r0 + 8 * i:r0 + 8 * (i + 1)] - ref) * LOG2E for i in range(4)]
                if below is not None:
                    self.rows[below] = jnp.where(sub >= a, part[0], self.mprev)
                self.mprev = part[0]
                for q, v in zip(full, part[1:]):
                    self.rows[q] = v
            new = {}
            while self.done in self.rows and self.done + 1 in self.rows:
                new[self.done] = jnp.concatenate([self.rows.pop(self.done), self.rows.pop(self.done + 1)], axis=0)
                self.done += 2
            return new

    def fold_pair(folders, g, keep=None, ties=None):
        tiles = {}
        for n, c in enumerate(range(0, HK, 128)):
            for half in range(2):
                for side in range(2):
                    t = ties[n] if ties and half == 0 and side == 0 else None
                    lo = side * HK + c
                    tiles[(half, lo)] = folders[half].tile(g + 4 * half, slice(lo, lo + 128), keep, t)
        return [folders[half].fold(g + 4 * half,
                                   jnp.concatenate([tiles[(half, lo)] for lo in range(0, D, 128)], axis=1))
                for half in range(2)]

    bestv_v[...] = jnp.full(bestv_v.shape, -jnp.inf, f32)
    besti_v[...] = lax.broadcasted_iota(jnp.int32, besti_v.shape, 0)
    h_v[0:P2, :] = jnp.zeros((P2, D), f32)
    st_v[0:B, :] = jnp.zeros((B, 256), f32)
    pend_v[...] = jnp.zeros(pend_v.shape, f32)

    def wait_all(cps):
        for cp in cps:
            cp.wait()

    def amats(c):
        for g0, n in _PSTAGES[c]:
            for g in range(g0, g0 + n):
                make_amat(g)

    wait_all(cp_p[0])
    amats(0)

    cp_x0.wait()
    ln1(x_v, 0, xs_v, 0, T0, plain=True)
    xb = [load_xn(s) for s in range(2)]
    logits = [{}, {}]
    finished = [set(), set()]
    fk, slabs = (Folder(D), Folder(D, NV // 2)), {}
    defer, queue = [False], []

    def absorb(new):
        for pos, slab in new.items():
            wtk_v[pos * 4:pos * 4 + 8, :] = _pk(slab.astype(bf16))
            slabs[pos] = slab
        for pos in sorted(slabs):
            if pos < NV // 2 and pos + NV // 2 in slabs:
                store_combos(wsk_v, pos * 4, slabs.pop(pos), slabs.pop(pos + NV // 2))

    def k_finish(s, hold=0):
        ready = [j for j in range(NP) if j not in finished[s] and _pair_need(j) in logits[s]]
        ready = ready[:len(ready) - hold]
        if defer[0]:
            queue.extend((logits[s].__getitem__, [j], s) for j in ready)
        else:
            k_side(logits[s].__getitem__, ready, s)
        finished[s].update(ready)

    def k_chunk(s, keep=None, early=(), late=(), hold=0):
        todo = [q for half in range(2) for q in range(half * (NV // 2), fk[half].done) if q not in logits[s]]
        runs = [[q for q in todo if q < NV // 2], [q for q in todo if q >= NV // 2]]
        lhs = jnp.concatenate([wtk_v[r[0] * 4:(r[-1] + 1) * 4, :] for r in runs if r], axis=0)
        ties = piece_ties(early, lhs.shape[0])
        ties.update(piece_ties(late, lhs.shape[0], col=HK))
        if ties:
            lhs = _tie(keep, lhs, ties)
        p = _dot_nt(_upk(lhs), xb[s])
        for n, q in enumerate(todo):
            logits[s][q] = p[n * 8:(n + 1) * 8]
        k_finish(s, hold)
        return p

    wait_all(cp_k[0])
    for new in fold_pair(fk, 0):
        absorb(new)
    k_chunk(0)
    k_chunk(1, hold=1)

    wait_all(cp_p[1] + cp_k[1])
    k_finish(1)
    for new in fold_pair(fk, 1):
        absorb(new)
    absorb(fk[0].fold(2))
    amats(1)
    k_chunk(0)
    k_chunk(1, hold=2)

    wait_all(cp_k[2] + [cp_x1])
    defer[0] = True
    keep = flag_s[0] > 0
    absorb(fk[1].fold(6))
    new = fold_pair(fk, 3)
    late = list(new[0].values())[-1][:, 384:512]
    for n in new:
        absorb(n)
    pieces = ln1(x_v, T0, xs_v, T0, T0, [0]) + ln1(x_v, T0, xs_v, T0, T0, [1, 2], keep, [late, late])
    p = k_chunk(0, keep, (), pieces[:2])
    rows = [k * p.shape[0] // 5 // 16 * 16 for k in range(5)]
    pieces += ln1(x_v, T0, xs_v, T0, T0, range(3, 8), keep, [p[r:r + R] for r in rows])
    k_chunk(1, keep, pieces[2:3], pieces[3:])

    def k_emit1(half, blk, val):
        if half != blk:
            k_side(half_groups(val, half), half_pairs(half), 2 + blk)
        else:
            queue.extend((half_groups(val, half), [j], 2 + blk) for j in half_pairs(half))

    def run_queue(n, res):
        deps = []
        for k in range(min(n, len(queue))):
            r = k * res.shape[0] // n // 8 * 8
            v = _vregs(k_side(*queue.pop(0), keep=keep, anchor=res[r:r + 8])[0])
            deps.append([_or_all(v[q::4]) for q in range(4)])
        return deps

    kwork = {}

    def k_after(m, res):
        if m in (0, 2):
            kwork[m + 1] = run_queue(4, res)

    def v_prep(lo, hi):
        for rb in range(lo, hi, 128):
            for c in range(0, HK, 128):
                raw = [wqkv_v[side * HK + c:side * HK + c + 128,
                              2 * D + half * HK + rb:2 * D + half * HK + rb + 128].T
                       for half in range(2) for side in range(2)]
                blocks = [t.astype(f32) for t in raw]
                for n, spec in enumerate(_SA):
                    t = raw[spec[0]] if spec[1] is None else _combo(blocks, spec).astype(bf16)
                    wsv_v[rb // 2:rb // 2 + 64, n * HK + c:n * HK + c + 128] = _pk(t)

    VS = HK // 2

    def k_before(m):
        if m == 5:
            cp_wv.wait()
            cp_x2.wait()
            v_prep(0, VS)

    sproj(wsk_v, xs_v, 1, k_emit1, keep, kwork, k_before, k_after)

    def ln_anchored(xg, src, xd, dst, k, n, keep, res):
        which = list(range(k * 8 // n, (k + 1) * 8 // n))
        rows = [a * HK // len(which) // 16 * 16 for a in range(len(which))]
        pcs = ln1(xg, src, xd, dst, P2, which, keep, [res[r:r + R] for r in rows])
        return [[]] * (3 - len(pcs)) + pcs

    vt, parts = {}, {}
    wsv = wsv_v.at[pl.ds(0, D // 4)]
    work = {0: {}, 1: {}, 2: {}}

    def v_after(q):
        def after(m, res):
            t = 7 * q + m
            u = t + 1
            if 3 <= t < 13:
                work[u // 7][u % 7] = run_queue(-(-len(queue) // (13 - t)), res)
            elif 13 <= t < 20:
                work[u // 7][u % 7] = ln_anchored(x_v, T, xs_v, T, t - 13, 7, keep, res)
        return after

    sealed(wsv_v)
    v_prep(VS, HK)
    zero = pl.multiple_of(flag_s[1], 8)
    for q, lo in enumerate((0, zero + VS // 2)):
        sproj(wsv_v.at[pl.ds(lo, VS // 2)], xs_v, 0,
              lambda half, blk, val: parts.setdefault((blk, half), []).append(val), keep, work[q], None, v_after(q))
    vt.update({k: jnp.concatenate(v, axis=0) for k, v in parts.items()})
    sproj(wsv_v.at[pl.ds(zero, D // 4)], xs_v, 1, lambda half, blk, val: vt.__setitem__((2 + blk, half), val), keep, work[2], None, v_after(2))
    assert not queue
    phi_m = sealed(phi_v)
    for j in range(NP):
        prod = kv_prod(vt, _upk(phi_m[j * 64:(j + 1) * 64, :]), j)
        kvacc_v[j] = prod
        if j == 2:
            store_xt(1, xs_view(flag_s[1], 2), T // 4, keep, pltpu.bitcast(prod[0:8], u32))
    cp_x3.wait()
    wait_bg(0)

    def p1_body(i, c):
        @pl.when(i == 2)
        def _():
            cp_x4.wait()
            wait_bg(1)

        @pl.when(i == 3)
        def _():
            wait_bg(2)

        keep = flag_s[0] > 0
        lo = jnp.minimum((i - 1) * DCH, F - DCH)
        sv = wd_v.at[pl.ds(pl.multiple_of(lo, 16), DCH)]
        dv = wdp_v.at[pl.ds(pl.multiple_of(lo // 2, 8), DCH // 2)]
        rp = repacker([(sv, dv, r, c) for r in range(0, DCH, 16) for c in range(0, D, 128)], keep)
        lo = jnp.minimum((i - 1) * OCH, HK - OCH)
        ov = wo_v.at[pl.ds(pl.multiple_of(lo, 16), HK + OCH)]
        od = wso_v.at[pl.ds(pl.multiple_of(lo // 2, 8), OCH // 2)]

        def k_emit(q):
            return lambda half, blk, val: k_side(half_groups(val, half), half_pairs(half), 2 * q + blk)

        vt = {}

        def v_emit(q):
            return lambda half, blk, val: vt.__setitem__((2 * q + blk, half), val)

        xd = xs_view(i, 2)
        xa = x_v.at[pl.ds(pl.multiple_of(i * T + P2, P2), P2)]
        xb = x_v.at[pl.ds(pl.multiple_of(jnp.minimum(i + 1, NT - 1) * T, T), P2)]
        wa = {}

        def a_after(m, res):
            if m < 6:
                wa[m + 1] = ln_anchored(xa, 0, xd, P2, m, 6, keep, res)

        sproj(wsv, xd, 0, v_emit(0), keep, wa, None, a_after, xt_view(i))
        sproj(wsk_v, xd, 0, k_emit(0), after=rp[0])
        sproj(wsk_v, xd, 1, k_emit(1), after=rp[1])
        wb = spread(ln1(xb, 0, xd, T, P2), [(0, m) for m in range(1, 7)])[0]

        def b_after(m, res):
            slabs = list(range(0, OCH, 16))
            mine = slabs[(m - 1) * len(slabs) // 6:m * len(slabs) // 6] if m else []
            for n, r in enumerate(mine):
                rows = [((4 * n + c) * HK // (4 * len(mine))) // 16 * 16 for c in range(4)]
                store_combos(od, r // 2, ov[r:r + 16, :].astype(f32), ov[HK + r:HK + r + 16, :].astype(f32),
                             _SB, keep, [res[a:a + R] for a in rows])

        sproj(wsv, xd, 1, v_emit(1), keep, wb, None, b_after)
        phi_m = sealed(phi_v)
        for j in range(NP):
            prod = kv_prod(vt, _upk(phi_m[j * 64:(j + 1) * 64, :]), j)
            kvacc_v[j] += prod
            if j == 2:
                store_xt(i + 1, xd, T // 4, keep, pltpu.bitcast(prod[0:8], u32))
        return c

    lax.fori_loop(1, NT, p1_body, 0)

    wait_all([cp_wr, cp_wq] + cp_gu[0])
    keep = flag_s[0] > 0
    kv_mask = (lax.broadcasted_iota(jnp.int32, (64, 128), 0) // DH
               == (lax.broadcasted_iota(jnp.int32, (64, 128), 1) // DH) % 2)
    ties = [{} for _ in range(16)]
    for j in range(NP):
        kvj = jnp.where(kv_mask, kvacc_v[j], 0.0)
        kv_v[:, j * 128:(j + 1) * 128] = _pk(kvj.astype(bf16))
        zj = _lanes(jnp.sum(zacc_v[j * 128:(j + 1) * 128, :], axis=-1, keepdims=True))
        zacc_v[j * 128:(j + 1) * 128, :] = zj
        vals = _vregs(kvj) + _vregs(zj)
        if j + 1 < 16:
            for q in range(4):
                ties[j + 1][(32 + q * 8, 0)] = _or_all(vals[q::4])
    wr = wr_v[0:8, :].astype(f32)
    wl = jnp.sum(wr, axis=0, keepdims=True)
    wsum = jnp.sum(wl, axis=1, keepdims=True)
    wrb_v[:, 0:D + 256] = jnp.concatenate(
        [jnp.broadcast_to(wr[j:j + 1, :], (8, 128)) for j in range(8)]
        + [jnp.broadcast_to(wsum, (8, 128)), jnp.broadcast_to(wl, (8, 128))], axis=1)
    store_xt(0, xs_v, 0)
    fq = (Folder(0), Folder(0, NV // 2))
    for g in range(4):
        new = fold_pair(fq, g, keep, ties[4 * g:4 * g + 4])
        for pos, slab in new[0].items():
            store_combos(wsq_v, pos * 4, slab, new[1][pos + NV // 2])

    pq_v = (pq0_v, pq1_v, pq2_v, pq3_v)

    def views_of(g):
        lo = g * (BPI * B)
        if not isinstance(g, int):
            lo = pl.multiple_of(lo, BPI * B)
        return ((x_v.at[pl.ds(lo, BPI * B)],)
                + tuple(ref.at[pl.ds(lo, P2 + BPI * B)] for ref in (h_v, out_v, st_v)) + (g,))

    def stage_q(xd, q, first, before, after):
        def emit(half, blk, val):
            group = half_groups(val, half)
            for j in half_pairs(half):
                p, j = _pair_logits(group, j), _phys_pair(j)
                ph = _hedgehog_t(p, zacc_v[j * 128:(j + 1) * 128, :])
                pq_v[2 * q + blk][(j // 2) * 64:(j // 2 + 1) * 64, (j % 2) * B:(j % 2 + 1) * B] = _pk(ph.astype(bf16))

        sproj(wsq_v, xd, q, emit, before=before, after=after, first=first)

    oc_v = (oc0_v, oc1_v)

    def stage_g(q):
        pq = [sealed(pq_v[2 * q + blk]) for blk in range(2)]
        for t in range(NP // 4):
            parts = [[_dot_nn(_upk(kv_v[:, j * 128:(j + 1) * 128]),
                              _upk(pq[blk][(j // 2) * 64:(j // 2 + 1) * 64, (j % 2) * B:(j % 2 + 1) * B]))
                      for blk in range(2) for j in (jj, jj + NP // 2)] for jj in (2 * t, 2 * t + 1)]
            blocks = [jnp.concatenate([a, b], axis=0) for a, b in zip(*parts)]
            for m, spec in enumerate(_SA):
                c = m * HK + t * 128
                oc_v[q][0:B // 2, c:c + 128] = _pk(_combo(blocks, spec).astype(bf16).T)

    def stage_h(views, q, keep, pieces, jobs, before=None):
        x_g, h_g = views[0], views[1]
        oc = sealed(oc_v[q])
        first, last = 4, 12
        ties = [{} for _ in range(7)]
        for k, vals in enumerate(pieces):
            t = first + k * (last - first) // max(len(pieces) - 1, 1)
            for m, val in enumerate(vals):
                ties[t // 4][(m * 8, (t % 4) * 128)] = val
        state = {}
        done = [0]

        def product(m):
            if before:
                before(m)
            w = wso_v[:, m * HK:(m + 1) * HK]
            if ties[m]:
                w = _tie(keep, w, ties[m])
            done[0] = m
            res = _dot_nn(_upk(oc[0:B // 2, m * HK:(m + 1) * HK]), _upk(w))
            for k, job in enumerate(jobs):
                t = 2 * q + k * (24 - 4 * q) // len(jobs)
                if t // 4 == m:
                    job(res[0:R, (t % 4) * 128:(t % 4 + 1) * 128])
            return res

        def wmul(d, lo):
            return (d.reshape(B // 8, 8, 128) * wrb_v[:, lo:lo + 128][None]).reshape(B, 128)

        def emit(k, val):
            blk, half = k // 2, k % 2
            s = 2 * q + blk
            cols = slice(half * HK, (half + 1) * HK)
            h = x_g[s * B:(s + 1) * B, cols].astype(f32) + val
            h_g[(s + 2) * B:(s + 3) * B, cols] = h
            st = state.setdefault(blk, {'h': {}})
            st['h'][half] = h
            for c in range(0, HK, 128):
                ht = h[:, c:c + 128]
                if 'h0' not in st:
                    st['h0'] = ht
                    continue
                d = ht - st['h0']
                new = (d, d * d, wmul(d, half * HK + c))
                st['s'] = new if 's' not in st else tuple(a + b for a, b in zip(st['s'], new))
            if len(st['h']) == 1:
                vals = [_or_all(list(v)) for v in zip(*[_vregs(a) for a in st['s']])]
                m = done[0] + 2
                for n, val in enumerate(vals):
                    ties[m][(248 - (n % 4) * 8, (n // 4) * 128)] = val

        _strassen(product, emit)

        res = []
        for blk in range(2):
            st = state[blk]
            s1, s2, s3 = st['s']
            c0 = _lanes(jnp.mean(st['h0'], axis=-1, keepdims=True))
            g0 = st['h0'] - c0
            t1 = s1 + 8.0 * g0
            t2 = s2 + g0 * (s1 + t1)
            t3 = s3 + wmul(g0, D + 128)
            res.append((jnp.concatenate([t1, t2, t3, c0], axis=1),
                        jnp.concatenate([st['h'][0], st['h'][1]], axis=1)))
        return res

    def stage_stats(views, s, part, valid=None):
        st_g, g = views[3], views[4]
        b = g * BPI + s
        bv = bestv_v[...]
        bi = besti_v[...]
        wsum = wrb_v[0:1, D:D + 128]
        nvs, nis, sts = [], [], []
        for k in range(B // R):
            sl = slice(k * R, (k + 1) * R)
            red = [_lanes(jnp.sum(part[sl, n * 128:(n + 1) * 128], axis=-1, keepdims=True)) for n in range(3)]
            mu = red[0] * (1.0 / D)
            var = jnp.maximum(red[1] * (1.0 / D) - mu * mu, 0.0)
            rs = lax.rsqrt(var + LN_EPS)
            r = (red[2] - mu * wsum) * rs
            sts.append(jnp.concatenate([rs, (mu + part[sl, 384:512]) * rs], axis=1))
            if valid is not None:
                r = jnp.where(valid, r, -jnp.inf)
            idx = lax.broadcasted_iota(jnp.int32, (R, 128), 0) + (b * B + k * R)
            better = r > bv[sl]
            nvs.append(jnp.where(better, r, bv[sl]))
            nis.append(jnp.where(better, idx, bi[sl]))
        st = jnp.concatenate(sts, axis=0)
        st_g[(s + 2) * B:(s + 3) * B, :] = st
        bestv_v[...] = jnp.concatenate(nvs, axis=0)
        besti_v[...] = jnp.concatenate(nis, axis=0)
        return st, [_vregs(nv) for nv in nvs]

    def out_jobs(views, s, keep, st=None, h=None):
        h_g, out_g, st_g = views[1], views[2], views[3]

        def job(k):
            def run(anchor):
                rows = slice((s + 2) * B + k * R, (s + 2) * B + (k + 1) * R)
                hk = h_g[rows, :] if h is None else h[k * R:(k + 1) * R]
                sk = st_g[rows, :] if st is None else st[k * R:(k + 1) * R]
                a = 1.0 + jnp.where(keep, sk[:, 0:128], anchor)
                o = [hk[:, c * 128:(c + 1) * 128] * a - sk[:, 128:256] for c in range(D // 128)]
                out_g[rows, :] = jnp.concatenate(o, axis=1).astype(bf16)
            return run
        return [job(k) for k in range(B // R)]

    def p2_body(i, c):
        b0 = i * BPI
        keep = flag_s[0] > 0
        cur = views_of(i)
        st, pieces = stage_stats(cur, -1, pend_v[...], i > 0)
        ojobs = out_jobs(cur, -2, keep) + out_jobs(cur, -1, keep, st)
        n = D // NI
        jobs = []
        for src, dst in ((wg_v, wgp_v), (wu_v, wup_v)):
            sv = src.at[pl.ds(pl.multiple_of(i * n, n), n)]
            dv = dst.at[pl.ds(pl.multiple_of(i * (n // 2), n // 2), n // 2)]
            jobs += [(sv, dv, r, cc) for r in range(0, n, 16) for cc in range(0, NM, 128)]
        rp = repacker(jobs, keep)
        stage_q(xs_view(i, 1), 0, xt_view(i), None, rp[0])
        stage_q(xs_view(i, 1), 1, None, lambda m: stage_g(0) if m == 2 else None, rp[1])
        res = stage_h(cur, 0, keep, pieces, ojobs, lambda m: stage_g(1) if m == 1 else None)
        st0, _ = stage_stats(cur, 0, res[0][0])
        st1, pieces = stage_stats(cur, 1, res[1][0])
        ojobs = out_jobs(cur, 0, keep, st0, res[0][1]) + out_jobs(cur, 1, keep, st1, res[1][1])
        res = stage_h(cur, 1, keep, pieces, ojobs)
        stage_stats(cur, BPI - 2, res[0][0])
        pend_v[...] = res[1][0]

        @pl.when(i > 0)
        def _():
            cp_out(jnp.maximum(b0 - 2, 0), 2).start()

        cp_out(b0, 2).start()
        return c

    lax.fori_loop(0, NI, p2_body, 0)
    wait_all(cp_gu[1])
    keep = flag_s[0] > 0
    last = views_of(NI - 1)

    st, _ = stage_stats(last, BPI - 1, pend_v[...])

    bv = bestv_v[...]
    mval = jnp.max(bv, axis=0, keepdims=True)
    sel = jnp.min(jnp.where(bv == mval, besti_v[...], S - 1), axis=0, keepdims=True)
    idx = jnp.clip(sel[0, 0], 0, S - 1)
    hrow = h_v[pl.ds(P2 + idx, 1), :]
    strow = st_v[pl.ds(P2 + idx, 1), :]
    xrow = jnp.concatenate([hrow[:, c * 128:(c + 1) * 128] * strow[:, 0:128] - strow[:, 128:256]
                            for c in range(D // 128)], axis=1).astype(bf16)
    xs = jnp.broadcast_to(xrow, (16, D))
    g_first = _dot_nn(xs, _upk(wgp_v[:, 0:FC]))
    anchors = ([jnp.broadcast_to(pltpu.bitcast(sel, f32), (R, 128))] * 4
               + [jnp.broadcast_to(xrow[:, 0:128].astype(f32), (R, 128))] * 4
               + [g_first[:, (k // 2) * 128:(k // 2 + 1) * 128] for k in range(8)])
    for job, anchor in zip(out_jobs(last, BPI - 2, keep) + out_jobs(last, BPI - 1, keep, st), anchors):
        job(anchor)
    cp_out(NB - 2, 2).start()

    def act(g, u):
        a = g * pl.reciprocal(1.0 + jnp.exp(-g), approx=True) * u
        return jnp.concatenate([a, a], axis=0).astype(bf16)

    def down(a, lo, w):
        return _dot_nn(a, _upk(wdp_v[lo // 2:(lo + w) // 2, 0:D]))[0:8]

    xcol = jnp.broadcast_to(xrow, (128, D)).T.astype(f32)
    jobs = [(which, b) for b in range(NBV) for which in (0, 1)]
    vres, prev = {}, None
    for j0 in range(0, len(jobs), NCH):
        grp = jobs[j0:j0 + NCH]
        accs = [None] * len(grp)
        for r in range(D // 16):
            for n, (which, b) in enumerate(grp):
                w = (wg_v, wu_v)[which][r * 16:(r + 1) * 16, NM + b * 128:NM + (b + 1) * 128].astype(f32)
                t0 = w[0:8] * xcol[r * 16:r * 16 + 8]
                t1 = w[8:16] * xcol[r * 16 + 8:r * 16 + 16]
                if accs[n] is None:
                    if prev is not None:
                        t0 = jnp.where(keep, t0, prev[n % len(prev)])
                    accs[n] = t0 + t1
                else:
                    accs[n] = (accs[n] + t0) + t1
        prev = accs
        for n, job in enumerate(grp):
            vres[job] = _allreduce8(accs[n][None], jnp.add)[0]

    chunks = [(lo, min(FC, NM - lo)) for lo in range(0, NM, FC)]
    acts, y = [], None
    for k, (lo, w) in enumerate(chunks):
        g = g_first if k == 0 else _dot_nn(xs, _upk(wgp_v[:, lo:lo + w]))
        u = _dot_nn(xs, _upk(wup_v[:, lo:lo + w]))
        acts.append(act(g[0:8], u[0:8]))
        if k >= 1:
            t = down(acts[k - 1], *chunks[k - 1])
            y = t if y is None else y + t
    y = y + down(acts[-1], *chunks[-1])
    for b0, nb in ((0, 4), (4, 4), (8, 4), (12, 1)):
        g = jnp.concatenate([vres[(0, b)] for b in range(b0, b0 + nb)], axis=1)
        u = jnp.concatenate([vres[(1, b)] for b in range(b0, b0 + nb)], axis=1)
        y = y + down(act(g, u), NM + b0 * 128, nb * 128)

    gate = jnp.broadcast_to(jax.nn.sigmoid(mval), (8, 128))
    base = pl.multiple_of((idx >> 4) << 4, 16)
    rows = pl.ds(pl.multiple_of(P2 + base, 16), 16)
    h16 = h_v[rows, :]
    st16 = st_v[rows, :]
    a16 = 1.0 + st16[:, 0:128]
    m16 = st16[:, 128:256]
    hit = (lax.broadcasted_iota(jnp.int32, (16, 128), 0) + base) == idx
    res = []
    for c in range(D // 128):
        yc = y[:, c * 128:(c + 1) * 128] * gate
        yc = jnp.concatenate([yc, yc], axis=0)
        res.append(h16[:, c * 128:(c + 1) * 128] * a16 - m16 + jnp.where(hit, yc, 0.0))
    res = jnp.concatenate(res, axis=1).astype(bf16)
    for i in range(NI):
        cp_out(i * BPI, 2).wait()
        cp_out(i * BPI + 2, 2).wait()
    out_v[rows, :] = res
    fix = pltpu.make_async_copy(out_v.at[rows], out_hbm.at[pl.ds(base, 16)], sem_o.at[0])
    fix.start()
    fix.wait()


@jax.jit
def pallas_sequential_preLN__linear_kernel_hedgehog__moe_arch_mod__prompt_kernel(
    A_x: jax.Array,
    A_wqkv: jax.Array,
    A_w_phi: jax.Array,
    A_wo: jax.Array,
    B_x: jax.Array,
    B_w_r: jax.Array,
    B_w_gate: jax.Array,
    B_w_up: jax.Array,
    B_w_down: jax.Array,
):
    del B_x
    x = A_x.reshape(S, D)
    wphi = A_w_phi.reshape(H * DH, DH)
    wr = B_w_r.reshape(8, 128)
    any_spec = pl.BlockSpec(memory_space=pl.ANY)
    out = pl.pallas_call(
        _kernel,
        out_shape=jax.ShapeDtypeStruct((S, D), bf16),
        in_specs=[any_spec] * 8,
        out_specs=any_spec,
        scratch_shapes=[
            pltpu.VMEM((S, D), bf16),
            pltpu.VMEM((D, 3 * D), bf16),
            pltpu.VMEM((H * DH, DH), bf16),
            pltpu.VMEM((D, D), bf16),
            pltpu.VMEM((64, 128), bf16),
            pltpu.VMEM((D, F + 128), bf16),
            pltpu.VMEM((D, F + 128), bf16),
            pltpu.VMEM((F, D), bf16),
            pltpu.VMEM((PR, D), u32),
            pltpu.VMEM((PR // 2, 7 * HK), u32),
            pltpu.VMEM((PR // 2, 7 * HK), u32),
            pltpu.VMEM((D // 4 + 8, 7 * HK), u32),
            pltpu.VMEM((D // 4, 7 * HK), u32),
            pltpu.VMEM((F // 2, D + 128), u32),
            pltpu.VMEM((D // 2, NM), u32),
            pltpu.VMEM((D // 2, NM), u32),
            pltpu.VMEM((64, 8 * 128), u32),
            pltpu.VMEM((T0 // 2, D), u32),
            pltpu.VMEM(((S + T) // 4, 7 * HK), u32),
            pltpu.VMEM(((NT + 1) * (HK // 2), B), u32),
            pltpu.VMEM((NP, 64, 128), f32),
            pltpu.VMEM((2 * D, 128), f32),
            pltpu.VMEM((32, NP * 128), u32),
            pltpu.VMEM((D + 8, T), u32),
            pltpu.VMEM((D // 2 + 16, 2 * B), u32),
            pltpu.VMEM((D // 2 + 16, 2 * B), u32),
            pltpu.VMEM((D // 2 + 16, 2 * B), u32),
            pltpu.VMEM((D // 2 + 16, 2 * B), u32),
            pltpu.VMEM((B // 2 + 8, 7 * HK), u32),
            pltpu.VMEM((B // 2 + 8, 7 * HK), u32),
            pltpu.VMEM((P2 + S, D), f32),
            pltpu.VMEM((P2 + S, 256), f32),
            pltpu.VMEM((B, 512), f32),
            pltpu.VMEM((P2 + S, D), bf16),
            pltpu.VMEM((8, D + 512), f32),
            pltpu.VMEM((B, 128), f32),
            pltpu.VMEM((B, 128), jnp.int32),
            pltpu.SMEM((2,), jnp.int32),
            pltpu.SemaphoreType.DMA((_NSEM_IN,)),
            pltpu.SemaphoreType.DMA((1,)),
        ],
        compiler_params=pltpu.CompilerParams(vmem_limit_bytes=110 * 1024 * 1024,
                                             disable_bounds_checks=True,
                                             disable_semaphore_checks=True),
        name="hedgehog_mod",
    )(x, A_wqkv, wphi, A_wo, wr, B_w_gate, B_w_up, B_w_down)
    return out.reshape(1, S, D)
```

```python
import jax
import jax.numpy as jnp
from jax import lax
import jax.experimental.pallas as pl
import jax.experimental.pallas.tpu as pltpu

S = 2048
D = 1024
H = 32
DH = 32
F = 3584
T = 512
NT = S // T
T0 = 256
B = 128
NB = S // B
BPI = 4
NI = NB // BPI
NP = H // 2
FC = 1024
R = 16
NBV = 13
NM = F - NBV * 128
NCH = 4
QK = D // 4
OCH = 96
DCH = 1216
NV = 124
PR = NV * 4
HK = D // 2
P2 = 2 * B
LOG2E = 1.4426950408889634
LN_EPS = 1e-5
DEN_EPS = 1e-6

_NT_DIMS = (((1,), (1,)), ((), ()))

bf16 = jnp.bfloat16
f32 = jnp.float32
u32 = jnp.uint32


def _dot_nt(a, b):
    return lax.dot_general(a, b, _NT_DIMS, preferred_element_type=f32)


def _dot_nn(a, b):
    return jnp.dot(a, b, preferred_element_type=f32)


def _pk(x):
    return pltpu.bitcast(x, u32)


def _upk(x):
    return pltpu.bitcast(x, bf16)


def _lanes(x):
    return jnp.broadcast_to(x, (x.shape[0], 128))


def _layernorm(x):
    m = jnp.mean(x, axis=-1, keepdims=True)
    xc = x - m
    v = jnp.mean(xc * xc, axis=-1, keepdims=True)
    return xc * lax.rsqrt(v + LN_EPS)


def _allreduce8(x, op):
    x = op(x, pltpu.roll(x, 4, 1))
    x = op(x, pltpu.roll(x, 2, 1))
    x = op(x, pltpu.roll(x, 1, 1))
    return x


def _hedgehog_t(p, z=None):
    t = p.shape[-1]
    p4 = p.reshape(2, 4, 8, t)
    mx = _allreduce8(jnp.max(p4, axis=1), jnp.maximum)
    mn = _allreduce8(jnp.min(p4, axis=1), jnp.minimum)
    ep = jnp.exp2(p4 - mx[:, None])
    en = jnp.exp2(mn[:, None] - p4)
    a = pl.reciprocal(_allreduce8(jnp.sum(ep, axis=1), jnp.add), approx=True)
    b = pl.reciprocal(_allreduce8(jnp.sum(en, axis=1), jnp.add), approx=True)
    if z is not None:
        dp = jnp.sum(ep * z[0:64].reshape(2, 4, 8, t), axis=1)
        dn = jnp.sum(en * z[64:128].reshape(2, 4, 8, t), axis=1)
        den = _allreduce8(dp * a + dn * b, jnp.add) + DEN_EPS
        inv = pl.reciprocal(den, approx=True)
        a = a * inv
        b = b * inv
    fp = (ep * a[:, None]).reshape(64, t)
    fn = (en * b[:, None]).reshape(64, t)
    return jnp.concatenate([fp, fn], axis=0)


_SA = ((3, None, 0), (2, 3, 1), (0, 1, 1), (0, None, 0), (0, 3, 1), (1, 3, -1), (2, 0, -1))
_SB = ((2, 0, -1), (0, None, 0), (3, None, 0), (1, 3, -1), (0, 3, 1), (2, 3, 1), (0, 1, 1))


def _combo(blocks, spec):
    a, b, sign = spec
    if b is None:
        return blocks[a]
    return blocks[a] + blocks[b] if sign > 0 else blocks[a] - blocks[b]


def _strassen(product, emit):
    m4 = product(0)
    m2 = product(1)
    emit(2, m4 + m2)
    m5 = product(2)
    u = m4 - m5
    m3 = product(3)
    emit(1, m5 + m3)
    v = m3 - m2
    m1 = product(4)
    u = u + m1
    v = v + m1
    emit(0, u + product(5))
    emit(3, v + product(6))


def _head_groups(h):
    base, k = (NV // 4) * (h // 8), h % 8
    return ([base + 4 * k + i for i in range(3)],
            base + 4 * k - 1 if k > 0 else None,
            base + 4 * k + 3 if k < 7 else None,
            8 - k)


def _pair_logits(group, j):
    parts = []
    for h in (2 * j, 2 * j + 1):
        full, below, above, a = _head_groups(h)
        ref = group(full[0])
        sub = lax.broadcasted_iota(jnp.int32, ref.shape, 0)
        if above is None:
            m = jnp.where(sub >= a, group(below), 0.0)
        else:
            m = jnp.where(sub == a - 1, 0.0, group(above))
            if below is not None:
                m = jnp.where(sub >= a, group(below), m)
        parts += [m] + [group(q) for q in full]
    return jnp.concatenate(parts, axis=0)


def _pair_need(j):
    full, _, above, _ = _head_groups(2 * j + 1)
    return full[2] if above is None else above


def _tie(keep, w, ties):
    rows = sorted({r for r, _ in ties})
    out, pos = [], 0
    for r in rows:
        if r > pos:
            out.append(w[pos:r])
        cols = sorted(c for rr, c in ties if rr == r)
        parts, cpos = [], 0
        for c in cols:
            if c > cpos:
                parts.append(w[r:r + 8, cpos:c])
            parts.append(jnp.where(keep, w[r:r + 8, c:c + 128], ties[(r, c)]))
            cpos = c + 128
        if cpos < w.shape[1]:
            parts.append(w[r:r + 8, cpos:])
        out.append(jnp.concatenate(parts, axis=1) if len(parts) > 1 else parts[0])
        pos = r + 8
    if pos < w.shape[0]:
        out.append(w[pos:])
    return jnp.concatenate(out, axis=0)


def _vregs(x):
    if x.dtype != u32:
        x = pltpu.bitcast(x, u32)
    return [x[r:r + 8, c:c + 128] for r in range(0, x.shape[0], 8) for c in range(0, x.shape[1], 128)]


def _or_all(vals):
    acc = vals[0]
    for v in vals[1:]:
        acc = acc | v
    return acc


def _phys_group(g):
    return 2 * (g % 4) + g // 4


def _phys_pair(j):
    return 2 * _phys_group(j // 2) + j % 2


_KSTAGES = (((0, 2),), ((2, 3),), ((5, 3),))
_PSTAGES = (((0, 5),), ((5, 3),))
_NSEM_IN = 11


def _kernel(x_hbm, wqkv_hbm, wphi_hbm, wo_hbm, wr_hbm, wg_hbm, wu_hbm, wd_hbm,
            out_hbm,
            x_v, wqkv_v, wphi_v, wo_v, wr_v, wg_v, wu_v, wd_v,
            wtk_v, wsq_v, wsk_v, wsv_v, wso_v, wdp_v, wgp_v, wup_v, amat_v, xn_v, xs_v, xt_v,
            kvacc_v, zacc_v, kv_v, phi_v,
            pq0_v, pq1_v, pq2_v, pq3_v, oc0_v, oc1_v, on0_v, on1_v, h_v, st_v, mom0_v, mom1_v, out_v, wrb_v,
            bestv_v, besti_v, flag_s,
            sem_i, sem_o):

    def cp_x(lo, n, sem):
        return pltpu.make_async_copy(x_hbm.at[pl.ds(lo, n)], x_v.at[pl.ds(lo, n)], sem_i.at[sem])

    def cp_w(lo, w, sem):
        return pltpu.make_async_copy(wqkv_hbm.at[:, pl.ds(lo, w)], wqkv_v.at[:, pl.ds(lo, w)], sem_i.at[sem])

    cp_k = [[cp_w(D + g * 128, n * 128, 2 + c) for g, n in st] for c, st in enumerate(_KSTAGES)]
    cp_p = [[pltpu.make_async_copy(wphi_hbm.at[pl.ds(g * 128, n * 128)], wphi_v.at[pl.ds(g * 128, n * 128)],
                                   sem_i.at[3 * c]) for g, n in st] for c, st in enumerate(_PSTAGES)]
    cp_wv = cp_w(2 * D, D, 5)
    cp_wq = cp_w(0, D, 7)

    def cp_wd(k):
        lo, n = k * DCH, min(DCH, F - k * DCH)
        return pltpu.make_async_copy(wd_hbm.at[pl.ds(lo, n)], wd_v.at[pl.ds(lo, n)], sem_i.at[(6, 8, 9)[k]])

    cp_x0 = cp_x(0, T0, 1)
    cp_x1 = cp_x(T0, T0, 4)
    cp_x2 = cp_x(T, P2, 5)
    cp_x3 = cp_x(T + P2, T, 6)
    cp_x4 = cp_x(2 * T + P2, S - 2 * T - P2, 8)
    cp_wr = pltpu.make_async_copy(wr_hbm, wr_v.at[pl.ds(0, 8)], sem_i.at[7])

    def cp_wo(k):
        lo, n = k * OCH, min(OCH, QK - k * OCH)
        return [pltpu.make_async_copy(wo_hbm.at[pl.ds(a * QK + lo, n)], wo_v.at[pl.ds(a * QK + lo, n)],
                                      sem_i.at[(6, 8, 9)[k]]) for a in range(4)]

    def wait_bg(k):
        for cp in cp_wo(k):
            cp.wait()
        cp_wd(k).wait()

    cp_gu = [[pltpu.make_async_copy(src.at[:, pl.ds(lo, n)], dst.at[:, pl.ds(lo, n)], sem_i.at[sem])
              for src, dst in ((wg_hbm, wg_v), (wu_hbm, wu_v))] for lo, n, sem in ((0, NM, 7), (NM, F - NM, 10))]

    def cp_out(b, n):
        lo = b * B
        if not isinstance(b, int):
            lo = pl.multiple_of(lo, B)
        return pltpu.make_async_copy(out_v.at[pl.ds(P2 + lo, n * B)], out_hbm.at[pl.ds(lo, n * B)], sem_o.at[0])

    for cp in (*cp_p[0], cp_x0, *cp_k[0], *cp_p[1], *cp_k[1], *cp_k[2], cp_x1, cp_wv, cp_x2,
               cp_x3, *cp_wo(0), cp_wd(0), cp_x4, *cp_wo(1), cp_wd(1), *cp_wo(2), cp_wd(2), cp_wr, cp_wq, *cp_gu[0], *cp_gu[1]):
        cp.start()
    flag_s[0] = 1
    flag_s[1] = 0

    def ln1(xg, src, xd, dst, n, which=None, keep=None, anchors=None, plain=False):
        pieces = []
        for pr in range(n // P2):
            for k in range(B // R):
                off = pr * P2 + k * R
                if which is not None and pr * (B // R) + k not in which:
                    continue
                x0 = xg[src + off:src + off + R, :].astype(f32)
                x1 = xg[src + off + B:src + off + B + R, :].astype(f32)
                if anchors is not None:
                    a = anchors[len(pieces)]
                    x0 = jnp.concatenate([jnp.where(keep, x0[:, :128], a), x0[:, 128:]], axis=1)
                    x1 = jnp.concatenate([jnp.where(keep, x1[:, :128], a), x1[:, 128:]], axis=1)
                p0 = _layernorm(x0)
                p1 = _layernorm(x1)
                if plain:
                    xn_v[off // 2:(off + R) // 2, :] = _pk(p0.astype(bf16))
                    xn_v[(off + B) // 2:(off + B + R) // 2, :] = _pk(p1.astype(bf16))
                lo = (dst + pr * P2) // 4 + k * (R // 2)
                blocks = (p0[:, :HK], p1[:, :HK], p0[:, HK:], p1[:, HK:])
                vs = []
                for m, spec in enumerate(_SB):
                    t = _combo(blocks, spec)
                    xd[lo:lo + R // 2, m * HK:(m + 1) * HK] = _pk(t.astype(bf16))
                    if spec[1] is not None:
                        vs.append(_vregs(t))
                pieces.append([_or_all(list(col)) for col in zip(*vs)])
        return pieces

    def load_xn(b):
        return _upk(xn_v[b * (B // 2):(b + 1) * (B // 2), :])

    def piece_ties(pieces, n, row0=0, col=0):
        ties = {}
        if pieces:
            step = (n - row0) // len(pieces) // 8 * 8
            for k, p in enumerate(pieces):
                for q, val in enumerate(p):
                    ties[(row0 + k * step + (q // 4) * 8, col + (q % 4) * 128)] = val
        return ties

    def xs_view(i, tiles):
        return xs_v.at[pl.ds(pl.multiple_of(i * (T // 4), T // 4), tiles * (T // 4))]

    def xt_view(i):
        lo = i * (HK // 2)
        return xt_v.at[pl.ds(lo if isinstance(i, int) else pl.multiple_of(lo, HK // 2), HK // 2)]

    def store_xt(i, xd, row, keep=None, anchor=None):
        v = xd[row:row + B // 2, 0:HK]
        if anchor is not None:
            v = _tie(keep, v, {(0, c): anchor for c in range(0, HK, 128)})
        xt_view(i)[...] = _pk(_upk(v).T)

    def sproj(ws, xd, pr, emit, keep=None, work=None, before=None, after=None, first=None):
        lo = pr * (B // 2)

        def product(m):
            if before:
                before(m)
            lhs = ws[:, m * HK:(m + 1) * HK]
            if work is not None and work.get(m):
                lhs = _tie(keep, lhs, piece_ties(work[m], lhs.shape[0], 32))
            if m == 0 and first is not None:
                res = _dot_nn(_upk(lhs), _upk(first[...]))
            else:
                res = _dot_nt(_upk(lhs), _upk(xd[lo:lo + B // 2, m * HK:(m + 1) * HK]))
            if after:
                after(m, res)
            return res

        _strassen(product, lambda k, val: emit(k // 2, k % 2, val))

    def repacker(jobs, keep, slots):
        def hook(q):
            def after(m, res):
                if (q, m) in slots:
                    k = slots.index((q, m))
                    mine = jobs[k * len(jobs) // len(slots):(k + 1) * len(jobs) // len(slots)]
                    for n, (sv, dv, r, c) in enumerate(mine):
                        a = (64 + n * 416 // len(mine)) // 8 * 8
                        dv[r // 2:r // 2 + 8, c:c + 128] = jnp.where(keep, _pk(sv[r:r + 16, c:c + 128]),
                                                                     pltpu.bitcast(res[a:a + 8], u32))
            return after
        return hook(0), hook(1)

    def spread(pieces, slots):
        res = {}
        for k, (pr, m) in enumerate(slots):
            res.setdefault(pr, {})[m] = pieces[k * len(pieces) // len(slots):(k + 1) * len(pieces) // len(slots)]
        return res

    def sealed(ref):
        ref[pl.ds(pl.multiple_of(flag_s[1] + ref.shape[0] - 8, 8), 8), 0:128] = jnp.zeros((8, 128), ref.dtype)
        return ref

    def store_combos(ws, row, top, bot):
        for c in range(0, HK, 128):
            blocks = [top[:, c:c + 128], top[:, HK + c:HK + c + 128], bot[:, c:c + 128], bot[:, HK + c:HK + c + 128]]
            for m, spec in enumerate(_SA):
                ws[row:row + 8, m * HK + c:m * HK + c + 128] = _pk(_combo(blocks, spec).astype(bf16))

    def combo2_jobs(dst, row, c, get, table, keep):
        def job(m):
            def run(anchor):
                a, b, sign = table[m]
                o = []
                for i1 in range(2):
                    for j1 in range(2):
                        v = get(a // 2, i1, a % 2, j1)
                        if i1 == j1:
                            v = jnp.where(keep, v, anchor)
                        if b is not None:
                            w = get(b // 2, i1, b % 2, j1)
                            v = v + w if sign > 0 else v - w
                        o.append(v)
                for n, si in enumerate(table):
                    col = (7 * m + n) * QK + c
                    dst[row:row + 8, col:col + 128] = _pk(_combo(o, si).astype(bf16))
            return run
        return [job(m) for m in range(7)]

    def run_on(jobs, res, lo=0, hi=None):
        hi = res.shape[0] - R if hi is None else hi
        for n, job in enumerate(jobs):
            a = (lo + n * (hi - lo) // len(jobs)) // 8 * 8
            job(res[a:a + R, 0:128])

    zinit = set()

    def k_side(group, pairs, slot, keep=None, anchor=None):
        res = []
        for j in pairs:
            p = _pair_logits(group, j)
            if anchor is not None:
                p = jnp.concatenate([jnp.where(keep, p[0:8], anchor), p[8:32],
                                     jnp.where(keep, p[32:40], anchor), p[40:64]], axis=0)
            ph = _hedgehog_t(p)
            j = _phys_pair(j)
            if j not in zinit:
                zinit.add(j)
                zacc_v[j * 128:(j + 1) * 128, :] = ph
            else:
                zacc_v[j * 128:(j + 1) * 128, :] += ph
            phi_v[j * 64:(j + 1) * 64, slot * B:(slot + 1) * B] = _pk(ph.astype(bf16))
            res.append(ph)
        return res

    def half_groups(p, half):
        return lambda pos: p[(pos - half * (NV // 2)) * 8:(pos - half * (NV // 2) + 1) * 8]

    def half_pairs(half):
        return range(half * (NP // 2), (half + 1) * (NP // 2))

    def kv_prod(vt, ph, j):
        half, r = j // (NP // 2), (j % (NP // 2)) * 64
        v = jnp.concatenate([vt[(s, half)][r:r + 64] for s in range(T // B)], axis=1).astype(bf16)
        return _dot_nt(v, ph)

    eye = (lax.broadcasted_iota(jnp.int32, (DH, DH), 0)
           == lax.broadcasted_iota(jnp.int32, (DH, DH), 1)).astype(bf16)
    r_h = lax.broadcasted_iota(jnp.int32, (128, 128), 0) // DH
    c_h = lax.broadcasted_iota(jnp.int32, (128, 128), 1) // DH
    same_head = r_h == c_h

    def make_amat(g):
        a = jnp.concatenate([_dot_nt(eye, wphi_v[g * 128:(g + 1) * 128, :])] * 4, axis=0)
        amat_v[:, g * 128:(g + 1) * 128] = _pk(jnp.where(same_head, a, 0.0).astype(bf16))

    class Folder:
        def __init__(self, col0, first=0):
            self.col0, self.rows, self.mprev, self.done = col0, {}, None, first

        def tile(self, g, rows, keep=None, ties=None):
            g = _phys_group(g)
            am = amat_v[:, g * 128:(g + 1) * 128]
            if ties:
                am = _tie(keep, am, ties)
            return _dot_nt(_upk(am), wqkv_v[rows, self.col0 + g * 128:self.col0 + (g + 1) * 128])

        def fold(self, g, wt=None):
            sub = lax.broadcasted_iota(jnp.int32, (8, D), 0)
            if wt is None:
                wt = self.tile(g, slice(None))
            for hh in range(4):
                full, below, _, a = _head_groups(4 * g + hh)
                r0 = hh * DH
                ref = jnp.broadcast_to(wt[r0 + a - 1:r0 + a, :], (8, D))
                part = [(wt[r0 + 8 * i:r0 + 8 * (i + 1)] - ref) * LOG2E for i in range(4)]
                if below is not None:
                    self.rows[below] = jnp.where(sub >= a, part[0], self.mprev)
                self.mprev = part[0]
                for q, v in zip(full, part[1:]):
                    self.rows[q] = v
            new = {}
            while self.done in self.rows and self.done + 1 in self.rows:
                new[self.done] = jnp.concatenate([self.rows.pop(self.done), self.rows.pop(self.done + 1)], axis=0)
                self.done += 2
            return new

    def fold_pair(folders, g, keep=None, ties=None):
        tiles = {}
        for n, c in enumerate(range(0, HK, 128)):
            for half in range(2):
                for side in range(2):
                    t = ties[n] if ties and half == 0 and side == 0 else None
                    lo = side * HK + c
                    tiles[(half, lo)] = folders[half].tile(g + 4 * half, slice(lo, lo + 128), keep, t)
        return [folders[half].fold(g + 4 * half,
                                   jnp.concatenate([tiles[(half, lo)] for lo in range(0, D, 128)], axis=1))
                for half in range(2)]

    bestv_v[...] = jnp.full(bestv_v.shape, -jnp.inf, f32)
    besti_v[...] = lax.broadcasted_iota(jnp.int32, besti_v.shape, 0)
    h_v[0:P2, :] = jnp.zeros((P2, D), f32)
    st_v[0:B, :] = jnp.zeros((B, 256), f32)
    mom1_v[...] = jnp.zeros(mom1_v.shape, f32)

    def wait_all(cps):
        for cp in cps:
            cp.wait()

    def amats(c):
        for g0, n in _PSTAGES[c]:
            for g in range(g0, g0 + n):
                make_amat(g)

    wait_all(cp_p[0])
    amats(0)

    cp_x0.wait()
    ln1(x_v, 0, xs_v, 0, T0, plain=True)
    xb = [load_xn(s) for s in range(2)]
    logits = [{}, {}]
    finished = [set(), set()]
    fk, slabs = (Folder(D), Folder(D, NV // 2)), {}
    defer, queue = [False], []

    def absorb(new):
        for pos, slab in new.items():
            wtk_v[pos * 4:pos * 4 + 8, :] = _pk(slab.astype(bf16))
            slabs[pos] = slab
        for pos in sorted(slabs):
            if pos < NV // 2 and pos + NV // 2 in slabs:
                store_combos(wsk_v, pos * 4, slabs.pop(pos), slabs.pop(pos + NV // 2))

    def k_finish(s, hold=0):
        ready = [j for j in range(NP) if j not in finished[s] and _pair_need(j) in logits[s]]
        ready = ready[:len(ready) - hold]
        if defer[0]:
            queue.extend((logits[s].__getitem__, [j], s) for j in ready)
        else:
            k_side(logits[s].__getitem__, ready, s)
        finished[s].update(ready)

    def k_chunk(s, keep=None, early=(), late=(), hold=0):
        todo = [q for half in range(2) for q in range(half * (NV // 2), fk[half].done) if q not in logits[s]]
        runs = [[q for q in todo if q < NV // 2], [q for q in todo if q >= NV // 2]]
        lhs = jnp.concatenate([wtk_v[r[0] * 4:(r[-1] + 1) * 4, :] for r in runs if r], axis=0)
        ties = piece_ties(early, lhs.shape[0])
        ties.update(piece_ties(late, lhs.shape[0], col=HK))
        if ties:
            lhs = _tie(keep, lhs, ties)
        p = _dot_nt(_upk(lhs), xb[s])
        for n, q in enumerate(todo):
            logits[s][q] = p[n * 8:(n + 1) * 8]
        k_finish(s, hold)
        return p

    wait_all(cp_k[0])
    for new in fold_pair(fk, 0):
        absorb(new)
    k_chunk(0)
    k_chunk(1, hold=1)

    wait_all(cp_p[1] + cp_k[1])
    k_finish(1)
    for new in fold_pair(fk, 1):
        absorb(new)
    absorb(fk[0].fold(2))
    amats(1)
    k_chunk(0)
    k_chunk(1, hold=2)

    wait_all(cp_k[2] + [cp_x1])
    defer[0] = True
    keep = flag_s[0] > 0
    absorb(fk[1].fold(6))
    new = fold_pair(fk, 3)
    late = list(new[0].values())[-1][:, 384:512]
    for n in new:
        absorb(n)
    pieces = ln1(x_v, T0, xs_v, T0, T0, [0]) + ln1(x_v, T0, xs_v, T0, T0, [1, 2], keep, [late, late])
    p = k_chunk(0, keep, (), pieces[:2])
    rows = [k * p.shape[0] // 5 // 16 * 16 for k in range(5)]
    pieces += ln1(x_v, T0, xs_v, T0, T0, range(3, 8), keep, [p[r:r + R] for r in rows])
    k_chunk(1, keep, pieces[2:3], pieces[3:])

    def k_emit1(half, blk, val):
        if half != blk:
            k_side(half_groups(val, half), half_pairs(half), 2 + blk)
        else:
            queue.extend((half_groups(val, half), [j], 2 + blk) for j in half_pairs(half))

    def run_queue(n, res):
        deps = []
        for k in range(min(n, len(queue))):
            r = k * res.shape[0] // n // 8 * 8
            v = _vregs(k_side(*queue.pop(0), keep=keep, anchor=res[r:r + 8])[0])
            deps.append([_or_all(v[q::4]) for q in range(4)])
        return deps

    kwork = {}

    def k_after(m, res):
        if m in (0, 2):
            kwork[m + 1] = run_queue(4, res)

    def v_prep(lo, hi):
        for rb in range(lo, hi, 128):
            for c in range(0, HK, 128):
                raw = [wqkv_v[side * HK + c:side * HK + c + 128,
                              2 * D + half * HK + rb:2 * D + half * HK + rb + 128].T
                       for half in range(2) for side in range(2)]
                blocks = [t.astype(f32) for t in raw]
                for n, spec in enumerate(_SA):
                    t = raw[spec[0]] if spec[1] is None else _combo(blocks, spec).astype(bf16)
                    wsv_v[rb // 2:rb // 2 + 64, n * HK + c:n * HK + c + 128] = _pk(t)

    VS = HK // 2

    def k_before(m):
        if m == 5:
            cp_wv.wait()
            cp_x2.wait()
            v_prep(0, VS)

    sproj(wsk_v, xs_v, 1, k_emit1, keep, kwork, k_before, k_after)

    def ln_anchored(xg, src, xd, dst, k, n, keep, res):
        which = list(range(k * 8 // n, (k + 1) * 8 // n))
        rows = [a * HK // len(which) // 16 * 16 for a in range(len(which))]
        pcs = ln1(xg, src, xd, dst, P2, which, keep, [res[r:r + R] for r in rows])
        return [[]] * (3 - len(pcs)) + pcs

    vt, parts = {}, {}
    wsv = wsv_v.at[pl.ds(0, D // 4)]
    work = {0: {}, 1: {}, 2: {}}

    def v_after(q):
        def after(m, res):
            t = 7 * q + m
            u = t + 1
            if 3 <= t < 13:
                work[u // 7][u % 7] = run_queue(-(-len(queue) // (13 - t)), res)
            elif 13 <= t < 20:
                work[u // 7][u % 7] = ln_anchored(x_v, T, xs_v, T, t - 13, 7, keep, res)
        return after

    sealed(wsv_v)
    v_prep(VS, HK)
    zero = pl.multiple_of(flag_s[1], 8)
    for q, lo in enumerate((0, zero + VS // 2)):
        sproj(wsv_v.at[pl.ds(lo, VS // 2)], xs_v, 0,
              lambda half, blk, val: parts.setdefault((blk, half), []).append(val), keep, work[q], None, v_after(q))
    vt.update({k: jnp.concatenate(v, axis=0) for k, v in parts.items()})
    sproj(wsv_v.at[pl.ds(zero, D // 4)], xs_v, 1, lambda half, blk, val: vt.__setitem__((2 + blk, half), val), keep, work[2], None, v_after(2))
    assert not queue
    phi_m = sealed(phi_v)
    for j in range(NP):
        prod = kv_prod(vt, _upk(phi_m[j * 64:(j + 1) * 64, :]), j)
        kvacc_v[j] = prod
        if j == 2:
            store_xt(1, xs_view(flag_s[1], 2), T // 4, keep, pltpu.bitcast(prod[0:8], u32))
    cp_x3.wait()
    wait_bg(0)

    def p1_body(i, c):
        @pl.when(i == 2)
        def _():
            cp_x4.wait()
            wait_bg(1)

        @pl.when(i == 3)
        def _():
            wait_bg(2)

        keep = flag_s[0] > 0
        lo = jnp.minimum((i - 1) * DCH, F - DCH)
        sv = wd_v.at[pl.ds(pl.multiple_of(lo, 16), DCH)]
        dv = wdp_v.at[pl.ds(pl.multiple_of(lo // 2, 8), DCH // 2)]
        rp = repacker([(sv, dv, r, c) for r in range(0, DCH, 16) for c in range(0, D, 128)], keep,
                      [(q, m) for q in range(2) for m in (0, 2, 4)])
        lo = jnp.minimum((i - 1) * OCH, QK - OCH)
        ov = wo_v.at[pl.ds(pl.multiple_of(lo, 16), 3 * QK + OCH)]
        od = wso_v.at[pl.ds(pl.multiple_of(lo // 2, 8), OCH // 2)]

        def k_emit(q):
            return lambda half, blk, val: k_side(half_groups(val, half), half_pairs(half), 2 * q + blk)

        vt = {}

        def v_emit(q):
            return lambda half, blk, val: vt.__setitem__((2 * q + blk, half), val)

        xd = xs_view(i, 2)
        xa = x_v.at[pl.ds(pl.multiple_of(i * T + P2, P2), P2)]
        xb = x_v.at[pl.ds(pl.multiple_of(jnp.minimum(i + 1, NT - 1) * T, T), P2)]
        wa = {}

        def wo_get(r, c):
            return lambda i0, i1, j0, j1: ov[i0 * HK + i1 * QK + r:i0 * HK + i1 * QK + r + 16,
                                             j0 * HK + j1 * QK + c:j0 * HK + j1 * QK + c + 128].astype(f32)

        wjobs = [job for r in range(0, OCH, 16) for c in (0, 128)
                 for job in combo2_jobs(od, r // 2, c, wo_get(r, c), _SB, keep)]
        wslots = [1, 2, 3, 4, 5, 8, 9, 10, 11, 12, 13]

        def wo_step(t, res):
            if t in wslots:
                k = wslots.index(t)
                run_on(wjobs[k * len(wjobs) // len(wslots):(k + 1) * len(wjobs) // len(wslots)], res)

        def a_after(m, res):
            if m < 6:
                wa[m + 1] = ln_anchored(xa, 0, xd, P2, m, 6, keep, res)
            wo_step(m, res)

        sproj(wsv, xd, 0, v_emit(0), keep, wa, None, a_after, xt_view(i))
        sproj(wsk_v, xd, 0, k_emit(0), after=rp[0])
        sproj(wsk_v, xd, 1, k_emit(1), after=rp[1])
        wb = spread(ln1(xb, 0, xd, T, P2), [(0, m) for m in range(1, 7)])[0]

        def b_after(m, res):
            wo_step(7 + m, res)

        sproj(wsv, xd, 1, v_emit(1), keep, wb, None, b_after)
        phi_m = sealed(phi_v)
        for j in range(NP):
            prod = kv_prod(vt, _upk(phi_m[j * 64:(j + 1) * 64, :]), j)
            kvacc_v[j] += prod
            if j == 2:
                store_xt(i + 1, xd, T // 4, keep, pltpu.bitcast(prod[0:8], u32))
        return c

    lax.fori_loop(1, NT, p1_body, 0)

    wait_all([cp_wr, cp_wq] + cp_gu[0])
    keep = flag_s[0] > 0
    kv_mask = (lax.broadcasted_iota(jnp.int32, (64, 128), 0) // DH
               == (lax.broadcasted_iota(jnp.int32, (64, 128), 1) // DH) % 2)
    ties = [{} for _ in range(16)]
    for j in range(NP):
        kvj = jnp.where(kv_mask, kvacc_v[j], 0.0)
        kv_v[:, j * 128:(j + 1) * 128] = _pk(kvj.astype(bf16))
        zj = _lanes(jnp.sum(zacc_v[j * 128:(j + 1) * 128, :], axis=-1, keepdims=True))
        zacc_v[j * 128:(j + 1) * 128, :] = zj
        vals = _vregs(kvj) + _vregs(zj)
        if j + 1 < 16:
            for q in range(4):
                ties[j + 1][(32 + q * 8, 0)] = _or_all(vals[q::4])
    wr = wr_v[0:8, :].astype(f32)
    wl = jnp.sum(wr, axis=0, keepdims=True)
    wsum = jnp.sum(wl, axis=1, keepdims=True)
    wrb_v[:, 0:D + 256] = jnp.concatenate(
        [jnp.broadcast_to(wr[j:j + 1, :], (8, 128)) for j in range(8)]
        + [jnp.broadcast_to(wsum, (8, 128)), jnp.broadcast_to(wl, (8, 128))], axis=1)
    store_xt(0, xs_v, 0)
    fq = (Folder(0), Folder(0, NV // 2))
    for g in range(4):
        new = fold_pair(fq, g, keep, ties[4 * g:4 * g + 4])
        for pos, slab in new[0].items():
            store_combos(wsq_v, pos * 4, slab, new[1][pos + NV // 2])

    pq_v = (pq0_v, pq1_v, pq2_v, pq3_v)

    def views_of(g):
        lo = g * (BPI * B)
        if not isinstance(g, int):
            lo = pl.multiple_of(lo, BPI * B)
        return ((x_v.at[pl.ds(lo, BPI * B)],)
                + tuple(ref.at[pl.ds(lo, P2 + BPI * B)] for ref in (h_v, out_v, st_v)) + (g,))

    def stage_q(xd, q, first, before, after):
        def emit(half, blk, val):
            group = half_groups(val, half)
            for j in half_pairs(half):
                p, j = _pair_logits(group, j), _phys_pair(j)
                ph = _hedgehog_t(p, zacc_v[j * 128:(j + 1) * 128, :])
                pq_v[2 * q + blk][(j // 2) * 64:(j // 2 + 1) * 64, (j % 2) * B:(j % 2 + 1) * B] = _pk(ph.astype(bf16))

        sproj(wsq_v, xd, q, emit, before=before, after=after, first=first)

    oc_v = (oc0_v, oc1_v)
    on_v = (on0_v, on1_v)

    def stage_g(q):
        pq = [sealed(pq_v[2 * q + blk]) for blk in range(2)]
        for t in range(NP // 4):
            parts = [[_dot_nn(_upk(kv_v[:, j * 128:(j + 1) * 128]),
                              _upk(pq[blk][(j // 2) * 64:(j // 2 + 1) * 64, (j % 2) * B:(j % 2 + 1) * B]))
                      for blk in range(2) for j in (jj, jj + NP // 2)] for jj in (2 * t, 2 * t + 1)]
            blocks = [jnp.concatenate([a, b], axis=0) for a, b in zip(*parts)]
            for k, blk in enumerate(blocks):
                c = (k % 2) * HK + t * 128
                on_v[q][(k // 2) * B:(k // 2 + 1) * B, c:c + 128] = blk.T

    def combo_jobs(q, keep):
        def get(r, c):
            def f(i0, i1, j0, j1):
                on = on_v[q].at[pl.ds(pl.multiple_of(flag_s[1], 8), P2)]
                return on[i0 * B + i1 * 64 + r:i0 * B + i1 * 64 + r + 16,
                          j0 * HK + j1 * QK + c:j0 * HK + j1 * QK + c + 128]
            return f
        return [job for c in (0, 128) for r in range(0, 64, 16)
                for job in combo2_jobs(oc_v[q], r // 2, c, get(r, c), _SA, keep)]

    def stage_h(views, q, sched, before, emitted):
        x_g, h_g = views[0], views[1]
        oc = sealed(oc_v[q])

        def product(m):
            if before:
                before(m)
            quad = {}

            def inner(n):
                col = (7 * m + n) * QK
                res = _dot_nn(_upk(oc[0:B // 4, col:col + QK]), _upk(wso_v[:, col:col + QK]))
                mine = sched.pop(49 * q + 7 * m + n, [])
                if mine:
                    run_on(mine, res)
                return res

            _strassen(inner, quad.__setitem__)
            return jnp.concatenate([jnp.concatenate([quad[0], quad[1]], axis=1),
                                    jnp.concatenate([quad[2], quad[3]], axis=1)], axis=0)

        def emit(k, val):
            blk, half = k // 2, k % 2
            s = 2 * q + blk
            cols = slice(half * HK, (half + 1) * HK)
            h = x_g[s * B:(s + 1) * B, cols].astype(f32) + val
            h_g[(s + 2) * B:(s + 3) * B, cols] = h
            emitted(blk, half, h)

        _strassen(product, emit)

    def wmul(d, lo):
        return (d.reshape(d.shape[0] // 8, 8, 128) * wrb_v[:, lo:lo + 128][None]).reshape(d.shape)

    def moments(st, mom, k, half, h, keep=None, anchor=None):
        first = 'h0' not in st
        if first:
            st['h0'] = h[:, 0:128]
            acc = None
        else:
            prev = mom[pl.ds(pl.multiple_of(flag_s[1] + k * R, R), R), :]
            acc = [prev[:, n * 128:(n + 1) * 128] for n in range(3)]
        h0 = st['h0'] if anchor is None else jnp.where(keep, st['h0'], anchor)
        for c in range(128 if first else 0, HK, 128):
            d = h[:, c:c + 128] - h0
            new = (d, d * d, wmul(d, half * HK + c))
            acc = new if acc is None else [a + b for a, b in zip(acc, new)]
        if first:
            mom[k * R:(k + 1) * R, :] = jnp.concatenate(list(acc) + [_lanes(jnp.mean(h0, axis=-1, keepdims=True))], axis=1)
            return None
        s1, s2, s3 = acc
        c0 = prev[:, 384:512]
        g0 = st['h0'] - c0
        t1 = s1 + 8.0 * g0
        return jnp.concatenate([t1, s2 + g0 * (s1 + t1), s3 + wmul(g0, D + 128), c0], axis=1)

    def stats(views, s, k, part, valid=None):
        st_g, g = views[3], views[4]
        sl = slice(k * R, (k + 1) * R)
        red = [_lanes(jnp.sum(part[:, n * 128:(n + 1) * 128], axis=-1, keepdims=True)) for n in range(3)]
        mu = red[0] * (1.0 / D)
        var = jnp.maximum(red[1] * (1.0 / D) - mu * mu, 0.0)
        rs = lax.rsqrt(var + LN_EPS)
        r = (red[2] - mu * wrb_v[0:1, D:D + 128]) * rs
        st = jnp.concatenate([rs, (mu + part[:, 384:512]) * rs], axis=1)
        st_g[(s + 2) * B + k * R:(s + 2) * B + (k + 1) * R, :] = st
        if valid is not None:
            r = jnp.where(valid, r, -jnp.inf)
        idx = lax.broadcasted_iota(jnp.int32, (R, 128), 0) + ((g * BPI + s) * B + k * R)
        bv = bestv_v[sl, :]
        better = r > bv
        bestv_v[sl, :] = jnp.where(better, r, bv)
        besti_v[sl, :] = jnp.where(better, idx, besti_v[sl, :])

    def out_jobs(views, s, keep):
        h_g, out_g, st_g = views[1], views[2], views[3]

        def job(k):
            def run(anchor):
                rows = slice((s + 2) * B + k * R, (s + 2) * B + (k + 1) * R)
                hk = h_g[rows, :]
                sk = st_g[rows, :]
                a = 1.0 + jnp.where(keep, sk[:, 0:128], anchor)
                o = [hk[:, c * 128:(c + 1) * 128] * a - sk[:, 128:256] for c in range(D // 128)]
                out_g[rows, :] = jnp.concatenate(o, axis=1).astype(bf16)
            return run
        return [job(k) for k in range(B // R)]

    def late_stats(views, s, k, keep=None, anchor=None, valid=None):
        r0 = (s + 2) * B + k * R
        blk = s % 2
        c0, c1 = (0, HK) if blk else (HK, 0)
        st = {'h0': views[1][r0:r0 + R, c0:c0 + 128]}
        part = moments(st, (mom0_v, mom1_v)[blk], k, c1 // HK, views[1][r0:r0 + R, c1:c1 + HK], keep, anchor)
        stats(views, s, k, part, valid)

    def p2_body(i, c):
        b0 = i * BPI
        keep = flag_s[0] > 0
        cur = views_of(i)
        n = D // NI
        jobs = []
        for src, dst in ((wg_v, wgp_v), (wu_v, wup_v)):
            sv = src.at[pl.ds(pl.multiple_of(i * n, n), n)]
            dv = dst.at[pl.ds(pl.multiple_of(i * (n // 2), n // 2), n // 2)]
            jobs += [(sv, dv, r, cc) for r in range(0, n, 16) for cc in range(0, NM, 128)]
        rp, _ = repacker(jobs, keep, [(0, 0), (0, 2), (0, 4)])

        def q0_after(m, res):
            rp(m, res)
            if m == 0:
                run_on([lambda a, k=k: late_stats(cur, -1, k, keep, a, i > 0) for k in range(B // R)], res, 0, 400)

        cj = combo_jobs(0, keep)

        def q1_after(m, res):
            if m in (2, 4):
                run_on(cj[(m // 4) * 28:(m // 4 + 1) * 28], res, 32)

        stage_q(xs_view(i, 1), 0, xt_view(i), None, q0_after)
        stage_q(xs_view(i, 1), 1, None, lambda m: stage_g(0) if m == 1 else None, q1_after)

        sched = {}

        def at(jobs, lo, hi):
            for k, job in enumerate(jobs):
                sched.setdefault(lo + k * (hi - lo) // len(jobs), []).append(job)

        at(out_jobs(cur, -2, keep), 3, 7)
        at(out_jobs(cur, -1, keep), 36, 44)
        at(combo_jobs(1, keep), 15, 44)
        state = {}
        when = {(1, False): (18, 28), (0, False): (30, 40), (0, True): (44, 54), (1, True): (54, 63),
                (3, False): (67, 77), (2, False): (79, 89), (2, True): (91, 94)}

        def emitted(q):
            def f(blk, half, h):
                s = 2 * q + blk
                second = s in state
                sts = state.setdefault(s, [{} for _ in range(B // R)])

                def job(k):
                    def run(anchor):
                        part = moments(sts[k], (mom0_v, mom1_v)[blk], k, half, h[k * R:(k + 1) * R], keep, anchor)
                        if second:
                            stats(cur, s, k, part)
                    return run

                if (s, second) in when:
                    at([job(k) for k in range(B // R)], *when[(s, second)])
                if second and q == 0:
                    at(out_jobs(cur, s, keep), 70 + 14 * blk, 77 + 14 * blk)
            return f

        stage_h(cur, 0, sched, lambda m: stage_g(1) if m == 1 else None, emitted(0))
        stage_h(cur, 1, sched, None, emitted(1))
        assert not sched

        @pl.when(i > 0)
        def _():
            cp_out(jnp.maximum(b0 - 2, 0), 2).start()

        cp_out(b0, 2).start()
        return c

    lax.fori_loop(0, NI, p2_body, 0)
    wait_all(cp_gu[1])
    keep = flag_s[0] > 0
    last = views_of(NI - 1)

    for k in range(B // R):
        late_stats(last, BPI - 1, k)

    bv = bestv_v[...]
    mval = jnp.max(bv, axis=0, keepdims=True)
    sel = jnp.min(jnp.where(bv == mval, besti_v[...], S - 1), axis=0, keepdims=True)
    idx = jnp.clip(sel[0, 0], 0, S - 1)
    hrow = h_v[pl.ds(P2 + idx, 1), :]
    strow = st_v[pl.ds(P2 + idx, 1), :]
    xrow = jnp.concatenate([hrow[:, c * 128:(c + 1) * 128] * strow[:, 0:128] - strow[:, 128:256]
                            for c in range(D // 128)], axis=1).astype(bf16)
    xs = jnp.broadcast_to(xrow, (16, D))
    g_first = _dot_nn(xs, _upk(wgp_v[:, 0:FC]))
    anchors = ([jnp.broadcast_to(pltpu.bitcast(sel, f32), (R, 128))] * 4
               + [jnp.broadcast_to(xrow[:, 0:128].astype(f32), (R, 128))] * 4
               + [g_first[:, (k // 2) * 128:(k // 2 + 1) * 128] for k in range(8)])
    for job, anchor in zip(out_jobs(last, BPI - 2, keep) + out_jobs(last, BPI - 1, keep), anchors):
        job(anchor)
    cp_out(NB - 2, 2).start()

    def act(g, u):
        a = g * pl.reciprocal(1.0 + jnp.exp(-g), approx=True) * u
        return jnp.concatenate([a, a], axis=0).astype(bf16)

    def down(a, lo, w):
        return _dot_nn(a, _upk(wdp_v[lo // 2:(lo + w) // 2, 0:D]))[0:8]

    xcol = jnp.broadcast_to(xrow, (128, D)).T.astype(f32)
    jobs = [(which, b) for b in range(NBV) for which in (0, 1)]
    vres, prev = {}, None
    for j0 in range(0, len(jobs), NCH):
        grp = jobs[j0:j0 + NCH]
        accs = [None] * len(grp)
        for r in range(D // 16):
            for n, (which, b) in enumerate(grp):
                w = (wg_v, wu_v)[which][r * 16:(r + 1) * 16, NM + b * 128:NM + (b + 1) * 128].astype(f32)
                t0 = w[0:8] * xcol[r * 16:r * 16 + 8]
                t1 = w[8:16] * xcol[r * 16 + 8:r * 16 + 16]
                if accs[n] is None:
                    if prev is not None:
                        t0 = jnp.where(keep, t0, prev[n % len(prev)])
                    accs[n] = t0 + t1
                else:
                    accs[n] = (accs[n] + t0) + t1
        prev = accs
        for n, job in enumerate(grp):
            vres[job] = _allreduce8(accs[n][None], jnp.add)[0]

    chunks = [(lo, min(FC, NM - lo)) for lo in range(0, NM, FC)]
    acts, y = [], None
    for k, (lo, w) in enumerate(chunks):
        g = g_first if k == 0 else _dot_nn(xs, _upk(wgp_v[:, lo:lo + w]))
        u = _dot_nn(xs, _upk(wup_v[:, lo:lo + w]))
        acts.append(act(g[0:8], u[0:8]))
        if k >= 1:
            t = down(acts[k - 1], *chunks[k - 1])
            y = t if y is None else y + t
    y = y + down(acts[-1], *chunks[-1])
    for b0, nb in ((0, 4), (4, 4), (8, 4), (12, 1)):
        g = jnp.concatenate([vres[(0, b)] for b in range(b0, b0 + nb)], axis=1)
        u = jnp.concatenate([vres[(1, b)] for b in range(b0, b0 + nb)], axis=1)
        y = y + down(act(g, u), NM + b0 * 128, nb * 128)

    gate = jnp.broadcast_to(jax.nn.sigmoid(mval), (8, 128))
    base = pl.multiple_of((idx >> 4) << 4, 16)
    rows = pl.ds(pl.multiple_of(P2 + base, 16), 16)
    h16 = h_v[rows, :]
    st16 = st_v[rows, :]
    a16 = 1.0 + st16[:, 0:128]
    m16 = st16[:, 128:256]
    hit = (lax.broadcasted_iota(jnp.int32, (16, 128), 0) + base) == idx
    res = []
    for c in range(D // 128):
        yc = y[:, c * 128:(c + 1) * 128] * gate
        yc = jnp.concatenate([yc, yc], axis=0)
        res.append(h16[:, c * 128:(c + 1) * 128] * a16 - m16 + jnp.where(hit, yc, 0.0))
    res = jnp.concatenate(res, axis=1).astype(bf16)
    for i in range(NI):
        cp_out(i * BPI, 2).wait()
        cp_out(i * BPI + 2, 2).wait()
    out_v[rows, :] = res
    fix = pltpu.make_async_copy(out_v.at[rows], out_hbm.at[pl.ds(base, 16)], sem_o.at[0])
    fix.start()
    fix.wait()


@jax.jit
def pallas_sequential_preLN__linear_kernel_hedgehog__moe_arch_mod__prompt_kernel(
    A_x: jax.Array,
    A_wqkv: jax.Array,
    A_w_phi: jax.Array,
    A_wo: jax.Array,
    B_x: jax.Array,
    B_w_r: jax.Array,
    B_w_gate: jax.Array,
    B_w_up: jax.Array,
    B_w_down: jax.Array,
):
    del B_x
    x = A_x.reshape(S, D)
    wphi = A_w_phi.reshape(H * DH, DH)
    wr = B_w_r.reshape(8, 128)
    any_spec = pl.BlockSpec(memory_space=pl.ANY)
    out = pl.pallas_call(
        _kernel,
        out_shape=jax.ShapeDtypeStruct((S, D), bf16),
        in_specs=[any_spec] * 8,
        out_specs=any_spec,
        scratch_shapes=[
            pltpu.VMEM((S, D), bf16),
            pltpu.VMEM((D, 3 * D), bf16),
            pltpu.VMEM((H * DH, DH), bf16),
            pltpu.VMEM((D, D), bf16),
            pltpu.VMEM((64, 128), bf16),
            pltpu.VMEM((D, F + 128), bf16),
            pltpu.VMEM((D, F + 128), bf16),
            pltpu.VMEM((F, D), bf16),
            pltpu.VMEM((PR, D), u32),
            pltpu.VMEM((PR // 2, 7 * HK), u32),
            pltpu.VMEM((PR // 2, 7 * HK), u32),
            pltpu.VMEM((D // 4 + 8, 7 * HK), u32),
            pltpu.VMEM((QK // 2, 49 * QK), u32),
            pltpu.VMEM((F // 2, D + 128), u32),
            pltpu.VMEM((D // 2, NM), u32),
            pltpu.VMEM((D // 2, NM), u32),
            pltpu.VMEM((64, 8 * 128), u32),
            pltpu.VMEM((T0 // 2, D), u32),
            pltpu.VMEM(((S + T) // 4, 7 * HK), u32),
            pltpu.VMEM(((NT + 1) * (HK // 2), B), u32),
            pltpu.VMEM((NP, 64, 128), f32),
            pltpu.VMEM((2 * D, 128), f32),
            pltpu.VMEM((32, NP * 128), u32),
            pltpu.VMEM((D + 8, T), u32),
            pltpu.VMEM((D // 2 + 16, 2 * B), u32),
            pltpu.VMEM((D // 2 + 16, 2 * B), u32),
            pltpu.VMEM((D // 2 + 16, 2 * B), u32),
            pltpu.VMEM((D // 2 + 16, 2 * B), u32),
            pltpu.VMEM((B // 4 + 16, 49 * QK), u32),
            pltpu.VMEM((B // 4 + 16, 49 * QK), u32),
            pltpu.VMEM((P2, D), f32),
            pltpu.VMEM((P2, D), f32),
            pltpu.VMEM((P2 + S, D), f32),
            pltpu.VMEM((P2 + S, 256), f32),
            pltpu.VMEM((B, 512), f32),
            pltpu.VMEM((B, 512), f32),
            pltpu.VMEM((P2 + S, D), bf16),
            pltpu.VMEM((8, D + 512), f32),
            pltpu.VMEM((B, 128), f32),
            pltpu.VMEM((B, 128), jnp.int32),
            pltpu.SMEM((2,), jnp.int32),
            pltpu.SemaphoreType.DMA((_NSEM_IN,)),
            pltpu.SemaphoreType.DMA((1,)),
        ],
        compiler_params=pltpu.CompilerParams(vmem_limit_bytes=120 * 1024 * 1024,
                                             disable_bounds_checks=True,
                                             disable_semaphore_checks=True),
        name="hedgehog_mod",
    )(x, A_wqkv, wphi, A_wo, wr, B_w_gate, B_w_up, B_w_down)
    return out.reshape(1, S, D)
```

```python
import jax
import jax.numpy as jnp
from jax import lax
import jax.experimental.pallas as pl
import jax.experimental.pallas.tpu as pltpu

S = 2048
D = 1024
H = 32
DH = 32
F = 3584
T = 512
NT = S // T
T0 = 256
B = 128
NB = S // B
BPI = 4
NI = NB // BPI
NP = H // 2
FC = 1024
R = 16
NBV = 13
NM = F - NBV * 128
NCH = 4
QK = D // 4
OCH = 96
DCH = 1216
NV = 124
PR = NV * 4
HK = D // 2
P2 = 2 * B
LOG2E = 1.4426950408889634
LN_EPS = 1e-5
DEN_EPS = 1e-6

_NT_DIMS = (((1,), (1,)), ((), ()))

bf16 = jnp.bfloat16
f32 = jnp.float32
u32 = jnp.uint32


def _dot_nt(a, b):
    return lax.dot_general(a, b, _NT_DIMS, preferred_element_type=f32)


def _dot_nn(a, b):
    return jnp.dot(a, b, preferred_element_type=f32)


def _pk(x):
    return pltpu.bitcast(x, u32)


def _upk(x):
    return pltpu.bitcast(x, bf16)


def _lanes(x):
    return jnp.broadcast_to(x, (x.shape[0], 128))


def _layernorm(x):
    m = jnp.mean(x, axis=-1, keepdims=True)
    xc = x - m
    v = jnp.mean(xc * xc, axis=-1, keepdims=True)
    return xc * lax.rsqrt(v + LN_EPS)


def _lane_dot(x, w):
    acc = None
    for c in range(0, x.shape[1], 128):
        t = x[:, c:c + 128].reshape(x.shape[0] // 8, 8, 128) * w[:, c:c + 128][None]
        acc = t if acc is None else acc + t
    return acc.reshape(x.shape[0], 128)


def _allreduce8(x, op):
    x = op(x, pltpu.roll(x, 4, 1))
    x = op(x, pltpu.roll(x, 2, 1))
    x = op(x, pltpu.roll(x, 1, 1))
    return x


def _hedgehog_t(p, z=None):
    t = p.shape[-1]
    p4 = p.reshape(2, 4, 8, t)
    mx = _allreduce8(jnp.max(p4, axis=1), jnp.maximum)
    mn = _allreduce8(jnp.min(p4, axis=1), jnp.minimum)
    ep = jnp.exp2(p4 - mx[:, None])
    en = jnp.exp2(mn[:, None] - p4)
    a = pl.reciprocal(_allreduce8(jnp.sum(ep, axis=1), jnp.add), approx=True)
    b = pl.reciprocal(_allreduce8(jnp.sum(en, axis=1), jnp.add), approx=True)
    if z is not None:
        dp = jnp.sum(ep * z[0:64].reshape(2, 4, 8, t), axis=1)
        dn = jnp.sum(en * z[64:128].reshape(2, 4, 8, t), axis=1)
        den = _allreduce8(dp * a + dn * b, jnp.add) + DEN_EPS
        inv = pl.reciprocal(den, approx=True)
        a = a * inv
        b = b * inv
    fp = (ep * a[:, None]).reshape(64, t)
    fn = (en * b[:, None]).reshape(64, t)
    return jnp.concatenate([fp, fn], axis=0)


_SA = ((3, None, 0), (2, 3, 1), (0, 1, 1), (0, None, 0), (0, 3, 1), (1, 3, -1), (2, 0, -1))
_SB = ((2, 0, -1), (0, None, 0), (3, None, 0), (1, 3, -1), (0, 3, 1), (2, 3, 1), (0, 1, 1))


def _combo(blocks, spec):
    a, b, sign = spec
    if b is None:
        return blocks[a]
    return blocks[a] + blocks[b] if sign > 0 else blocks[a] - blocks[b]


def _strassen(product, emit):
    m4 = product(0)
    m2 = product(1)
    emit(2, m4 + m2)
    m5 = product(2)
    u = m4 - m5
    m3 = product(3)
    emit(1, m5 + m3)
    v = m3 - m2
    m1 = product(4)
    u = u + m1
    v = v + m1
    emit(0, u + product(5))
    emit(3, v + product(6))


def _head_groups(h):
    base, k = (NV // 4) * (h // 8), h % 8
    return ([base + 4 * k + i for i in range(3)],
            base + 4 * k - 1 if k > 0 else None,
            base + 4 * k + 3 if k < 7 else None,
            8 - k)


def _pair_logits(group, j):
    parts = []
    for h in (2 * j, 2 * j + 1):
        full, below, above, a = _head_groups(h)
        ref = group(full[0])
        sub = lax.broadcasted_iota(jnp.int32, ref.shape, 0)
        if above is None:
            m = jnp.where(sub >= a, group(below), 0.0)
        else:
            m = jnp.where(sub == a - 1, 0.0, group(above))
            if below is not None:
                m = jnp.where(sub >= a, group(below), m)
        parts += [m] + [group(q) for q in full]
    return jnp.concatenate(parts, axis=0)


def _pair_need(j):
    full, _, above, _ = _head_groups(2 * j + 1)
    return full[2] if above is None else above


def _tie(keep, w, ties):
    rows = sorted({r for r, _ in ties})
    out, pos = [], 0
    for r in rows:
        if r > pos:
            out.append(w[pos:r])
        cols = sorted(c for rr, c in ties if rr == r)
        parts, cpos = [], 0
        for c in cols:
            if c > cpos:
                parts.append(w[r:r + 8, cpos:c])
            parts.append(jnp.where(keep, w[r:r + 8, c:c + 128], ties[(r, c)]))
            cpos = c + 128
        if cpos < w.shape[1]:
            parts.append(w[r:r + 8, cpos:])
        out.append(jnp.concatenate(parts, axis=1) if len(parts) > 1 else parts[0])
        pos = r + 8
    if pos < w.shape[0]:
        out.append(w[pos:])
    return jnp.concatenate(out, axis=0)


def _vregs(x):
    if x.dtype != u32:
        x = pltpu.bitcast(x, u32)
    return [x[r:r + 8, c:c + 128] for r in range(0, x.shape[0], 8) for c in range(0, x.shape[1], 128)]


def _or_all(vals):
    acc = vals[0]
    for v in vals[1:]:
        acc = acc | v
    return acc


def _phys_group(g):
    return 2 * (g % 4) + g // 4


def _phys_pair(j):
    return 2 * _phys_group(j // 2) + j % 2


_KSTAGES = (((0, 2),), ((2, 3),), ((5, 3),))
_PSTAGES = (((0, 5),), ((5, 3),))
_NSEM_IN = 11


def _kernel(x_hbm, wqkv_hbm, wphi_hbm, wo_hbm, wr_hbm, wg_hbm, wu_hbm, wd_hbm,
            out_hbm,
            x_v, wqkv_v, wphi_v, wo_v, wr_v, wg_v, wu_v, wd_v,
            wtk_v, wsq_v, wsk_v, wsv_v, wso_v, wdp_v, wgp_v, wup_v, amat_v, xn_v, xs_v, xt_v,
            kvacc_v, zacc_v, kv_v, phi_v,
            pq0_v, pq1_v, pq2_v, pq3_v, oc0_v, oc1_v, on0_v, on1_v, h_v, st_v, mom0_v, mom1_v, out_v, wrb_v, cb_v, wow_v, num_v,
            bestv_v, besti_v, flag_s,
            sem_i, sem_o):

    def cp_x(lo, n, sem):
        return pltpu.make_async_copy(x_hbm.at[pl.ds(lo, n)], x_v.at[pl.ds(lo, n)], sem_i.at[sem])

    def cp_w(lo, w, sem):
        return pltpu.make_async_copy(wqkv_hbm.at[:, pl.ds(lo, w)], wqkv_v.at[:, pl.ds(lo, w)], sem_i.at[sem])

    cp_k = [[cp_w(D + g * 128, n * 128, 2 + c) for g, n in st] for c, st in enumerate(_KSTAGES)]
    cp_p = [[pltpu.make_async_copy(wphi_hbm.at[pl.ds(g * 128, n * 128)], wphi_v.at[pl.ds(g * 128, n * 128)],
                                   sem_i.at[3 * c]) for g, n in st] for c, st in enumerate(_PSTAGES)]
    cp_wv = cp_w(2 * D, D, 5)
    cp_wq = cp_w(0, D, 7)

    def cp_wd(k):
        lo, n = k * DCH, min(DCH, F - k * DCH)
        return pltpu.make_async_copy(wd_hbm.at[pl.ds(lo, n)], wd_v.at[pl.ds(lo, n)], sem_i.at[(6, 8, 9)[k]])

    cp_x0 = cp_x(0, T0, 1)
    cp_x1 = cp_x(T0, T0, 4)
    cp_x2 = cp_x(T, P2, 5)
    cp_x3 = cp_x(T + P2, T, 6)
    cp_x4 = cp_x(2 * T + P2, S - 2 * T - P2, 8)
    cp_wr = pltpu.make_async_copy(wr_hbm, wr_v.at[pl.ds(0, 8)], sem_i.at[0])

    def cp_wo(k):
        lo, n = k * OCH, min(OCH, QK - k * OCH)
        return [pltpu.make_async_copy(wo_hbm.at[pl.ds(a * QK + lo, n)], wo_v.at[pl.ds(a * QK + lo, n)],
                                      sem_i.at[(6, 8, 9)[k]]) for a in range(4)]

    def wait_bg(k):
        for cp in cp_wo(k):
            cp.wait()
        cp_wd(k).wait()

    cp_gu = [[pltpu.make_async_copy(src.at[:, pl.ds(lo, n)], dst.at[:, pl.ds(lo, n)], sem_i.at[sem])
              for src, dst in ((wg_hbm, wg_v), (wu_hbm, wu_v))] for lo, n, sem in ((0, NM, 7), (NM, F - NM, 10))]

    def cp_out(b, n):
        lo = b * B
        if not isinstance(b, int):
            lo = pl.multiple_of(lo, B)
        return pltpu.make_async_copy(out_v.at[pl.ds(P2 + lo, n * B)], out_hbm.at[pl.ds(lo, n * B)], sem_o.at[0])

    for cp in (cp_wr, *cp_p[0], cp_x0, *cp_k[0], *cp_p[1], *cp_k[1], *cp_k[2], cp_x1, cp_wv, cp_x2,
               cp_x3, *cp_wo(0), cp_wd(0), cp_x4, *cp_wo(1), cp_wd(1), *cp_wo(2), cp_wd(2), cp_wq, *cp_gu[0], *cp_gu[1]):
        cp.start()
    flag_s[0] = 1
    flag_s[1] = 0

    def ln1(xg, src, xd, dst, n, which=None, keep=None, anchors=None, plain=False):
        pieces = []
        for pr in range(n // P2):
            for k in range(B // R):
                off = pr * P2 + k * R
                if which is not None and pr * (B // R) + k not in which:
                    continue
                x0 = xg[src + off:src + off + R, :].astype(f32)
                x1 = xg[src + off + B:src + off + B + R, :].astype(f32)
                if anchors is not None:
                    a = anchors[len(pieces)]
                    x0 = jnp.concatenate([jnp.where(keep, x0[:, :128], a), x0[:, 128:]], axis=1)
                    x1 = jnp.concatenate([jnp.where(keep, x1[:, :128], a), x1[:, 128:]], axis=1)
                p0 = _layernorm(x0)
                p1 = _layernorm(x1)
                if plain:
                    xn_v[off // 2:(off + R) // 2, :] = _pk(p0.astype(bf16))
                    xn_v[(off + B) // 2:(off + B + R) // 2, :] = _pk(p1.astype(bf16))
                lo = (dst + pr * P2) // 4 + k * (R // 2)
                blocks = (p0[:, :HK], p1[:, :HK], p0[:, HK:], p1[:, HK:])
                vs = []
                for m, spec in enumerate(_SB):
                    t = _combo(blocks, spec)
                    xd[lo:lo + R // 2, m * HK:(m + 1) * HK] = _pk(t.astype(bf16))
                    if spec[1] is not None:
                        vs.append(_vregs(t))
                pieces.append([_or_all(list(col)) for col in zip(*vs)])
        return pieces

    def load_xn(b):
        return _upk(xn_v[b * (B // 2):(b + 1) * (B // 2), :])

    def piece_ties(pieces, n, row0=0, col=0):
        ties = {}
        if pieces:
            step = (n - row0) // len(pieces) // 8 * 8
            for k, p in enumerate(pieces):
                for q, val in enumerate(p):
                    ties[(row0 + k * step + (q // 4) * 8, col + (q % 4) * 128)] = val
        return ties

    def xs_view(i, tiles):
        return xs_v.at[pl.ds(pl.multiple_of(i * (T // 4), T // 4), tiles * (T // 4))]

    def xt_view(i):
        lo = i * (HK // 2)
        return xt_v.at[pl.ds(lo if isinstance(i, int) else pl.multiple_of(lo, HK // 2), HK // 2)]

    def store_xt(i, xd, row, keep=None, anchor=None):
        v = xd[row:row + B // 2, 0:HK]
        if anchor is not None:
            v = _tie(keep, v, {(0, c): anchor for c in range(0, HK, 128)})
        xt_view(i)[...] = _pk(_upk(v).T)

    def sproj(ws, xd, pr, emit, keep=None, work=None, before=None, after=None, first=None):
        lo = pr * (B // 2)

        def product(m):
            if before:
                before(m)
            lhs = ws[:, m * HK:(m + 1) * HK]
            if work is not None and work.get(m):
                lhs = _tie(keep, lhs, piece_ties(work[m], lhs.shape[0], 32))
            if m == 0 and first is not None:
                res = _dot_nn(_upk(lhs), _upk(first[...]))
            else:
                res = _dot_nt(_upk(lhs), _upk(xd[lo:lo + B // 2, m * HK:(m + 1) * HK]))
            if after:
                after(m, res)
            return res

        _strassen(product, lambda k, val: emit(k // 2, k % 2, val))

    def repacker(jobs, keep, slots):
        def hook(q):
            def after(m, res):
                if (q, m) in slots:
                    k = slots.index((q, m))
                    mine = jobs[k * len(jobs) // len(slots):(k + 1) * len(jobs) // len(slots)]
                    for n, (sv, dv, r, c) in enumerate(mine):
                        a = (64 + n * 416 // len(mine)) // 8 * 8
                        dv[r // 2:r // 2 + 8, c:c + 128] = jnp.where(keep, _pk(sv[r:r + 16, c:c + 128]),
                                                                     pltpu.bitcast(res[a:a + 8], u32))
            return after
        return hook(0), hook(1)

    def spread(pieces, slots):
        res = {}
        for k, (pr, m) in enumerate(slots):
            res.setdefault(pr, {})[m] = pieces[k * len(pieces) // len(slots):(k + 1) * len(pieces) // len(slots)]
        return res

    def sealed(ref):
        ref[pl.ds(pl.multiple_of(flag_s[1] + ref.shape[0] - 8, 8), 8), 0:128] = jnp.zeros((8, 128), ref.dtype)
        return ref

    def store_combos(ws, row, top, bot):
        for c in range(0, HK, 128):
            blocks = [top[:, c:c + 128], top[:, HK + c:HK + c + 128], bot[:, c:c + 128], bot[:, HK + c:HK + c + 128]]
            for m, spec in enumerate(_SA):
                ws[row:row + 8, m * HK + c:m * HK + c + 128] = _pk(_combo(blocks, spec).astype(bf16))

    def combo2_jobs(dst, row, c, get, table, keep):
        def job(m):
            def run(anchor):
                a, b, sign = table[m]
                o = []
                for i1 in range(2):
                    for j1 in range(2):
                        v = get(a // 2, i1, a % 2, j1)
                        if i1 == j1:
                            v = jnp.where(keep, v, anchor)
                        if b is not None:
                            w = get(b // 2, i1, b % 2, j1)
                            v = v + w if sign > 0 else v - w
                        o.append(v)
                for n, si in enumerate(table):
                    col = (7 * m + n) * QK + c
                    dst[row:row + 8, col:col + 128] = _pk(_combo(o, si).astype(bf16))
            return run
        return [job(m) for m in range(7)]

    def run_on(jobs, res, lo=0, hi=None):
        hi = res.shape[0] - R if hi is None else hi
        for n, job in enumerate(jobs):
            a = (lo + n * (hi - lo) // len(jobs)) // 8 * 8
            job(res[a:a + R, 0:128])

    def dot_jobs(src, dst, rows, keep):
        def job(r):
            def run(anchor):
                w = src[r:r + R, :].astype(f32)
                w = jnp.concatenate([jnp.where(keep, w[:, :128], anchor), w[:, 128:]], axis=1)
                dst[r:r + R, :] = _lane_dot(w, wrb_v)
            return run
        return [job(r) for r in rows]

    zinit = set()

    def k_side(group, pairs, slot, keep=None, anchor=None):
        res = []
        for j in pairs:
            p = _pair_logits(group, j)
            if anchor is not None:
                p = jnp.concatenate([jnp.where(keep, p[0:8], anchor), p[8:32],
                                     jnp.where(keep, p[32:40], anchor), p[40:64]], axis=0)
            ph = _hedgehog_t(p)
            j = _phys_pair(j)
            if j not in zinit:
                zinit.add(j)
                zacc_v[j * 128:(j + 1) * 128, :] = ph
            else:
                zacc_v[j * 128:(j + 1) * 128, :] += ph
            phi_v[j * 64:(j + 1) * 64, slot * B:(slot + 1) * B] = _pk(ph.astype(bf16))
            res.append(ph)
        return res

    def half_groups(p, half):
        return lambda pos: p[(pos - half * (NV // 2)) * 8:(pos - half * (NV // 2) + 1) * 8]

    def half_pairs(half):
        return range(half * (NP // 2), (half + 1) * (NP // 2))

    def kv_prod(vt, ph, j):
        half, r = j // (NP // 2), (j % (NP // 2)) * 64
        v = jnp.concatenate([vt[(s, half)][r:r + 64] for s in range(T // B)], axis=1).astype(bf16)
        return _dot_nt(v, ph)

    eye = (lax.broadcasted_iota(jnp.int32, (DH, DH), 0)
           == lax.broadcasted_iota(jnp.int32, (DH, DH), 1)).astype(bf16)
    r_h = lax.broadcasted_iota(jnp.int32, (128, 128), 0) // DH
    c_h = lax.broadcasted_iota(jnp.int32, (128, 128), 1) // DH
    same_head = r_h == c_h

    def make_amat(g):
        a = jnp.concatenate([_dot_nt(eye, wphi_v[g * 128:(g + 1) * 128, :])] * 4, axis=0)
        amat_v[:, g * 128:(g + 1) * 128] = _pk(jnp.where(same_head, a, 0.0).astype(bf16))

    class Folder:
        def __init__(self, col0, first=0):
            self.col0, self.rows, self.mprev, self.done = col0, {}, None, first

        def tile(self, g, rows, keep=None, ties=None):
            g = _phys_group(g)
            am = amat_v[:, g * 128:(g + 1) * 128]
            if ties:
                am = _tie(keep, am, ties)
            return _dot_nt(_upk(am), wqkv_v[rows, self.col0 + g * 128:self.col0 + (g + 1) * 128])

        def fold(self, g, wt=None):
            sub = lax.broadcasted_iota(jnp.int32, (8, D), 0)
            if wt is None:
                wt = self.tile(g, slice(None))
            for hh in range(4):
                full, below, _, a = _head_groups(4 * g + hh)
                r0 = hh * DH
                ref = jnp.broadcast_to(wt[r0 + a - 1:r0 + a, :], (8, D))
                part = [(wt[r0 + 8 * i:r0 + 8 * (i + 1)] - ref) * LOG2E for i in range(4)]
                if below is not None:
                    self.rows[below] = jnp.where(sub >= a, part[0], self.mprev)
                self.mprev = part[0]
                for q, v in zip(full, part[1:]):
                    self.rows[q] = v
            new = {}
            while self.done in self.rows and self.done + 1 in self.rows:
                new[self.done] = jnp.concatenate([self.rows.pop(self.done), self.rows.pop(self.done + 1)], axis=0)
                self.done += 2
            return new

    def fold_pair(folders, g, keep=None, ties=None):
        tiles = {}
        for n, c in enumerate(range(0, HK, 128)):
            for half in range(2):
                for side in range(2):
                    t = ties[n] if ties and half == 0 and side == 0 else None
                    lo = side * HK + c
                    tiles[(half, lo)] = folders[half].tile(g + 4 * half, slice(lo, lo + 128), keep, t)
        return [folders[half].fold(g + 4 * half,
                                   jnp.concatenate([tiles[(half, lo)] for lo in range(0, D, 128)], axis=1))
                for half in range(2)]

    bestv_v[...] = jnp.full(bestv_v.shape, -jnp.inf, f32)
    besti_v[...] = lax.broadcasted_iota(jnp.int32, besti_v.shape, 0)
    h_v[0:P2, :] = jnp.zeros((P2, D), f32)
    st_v[0:B, :] = jnp.zeros((B, 256), f32)
    mom1_v[...] = jnp.zeros(mom1_v.shape, f32)

    def wait_all(cps):
        for cp in cps:
            cp.wait()

    def amats(c):
        for g0, n in _PSTAGES[c]:
            for g in range(g0, g0 + n):
                make_amat(g)

    wait_all([cp_wr] + cp_p[0])
    amats(0)
    wr = wr_v[0:8, :].astype(f32)
    wc = wr - jnp.sum(jnp.sum(wr, axis=0, keepdims=True), axis=1, keepdims=True) * (1.0 / D)
    wrb_v[...] = jnp.concatenate([jnp.broadcast_to(wc[j:j + 1, :], (8, 128)) for j in range(8)], axis=1)
    num_v[0:P2, :] = jnp.zeros((P2, 128), f32)

    cp_x0.wait()
    ln1(x_v, 0, xs_v, 0, T0, plain=True)
    xb = [load_xn(s) for s in range(2)]
    logits = [{}, {}]
    finished = [set(), set()]
    fk, slabs = (Folder(D), Folder(D, NV // 2)), {}
    defer, queue = [False], []

    def absorb(new):
        for pos, slab in new.items():
            wtk_v[pos * 4:pos * 4 + 8, :] = _pk(slab.astype(bf16))
            slabs[pos] = slab
        for pos in sorted(slabs):
            if pos < NV // 2 and pos + NV // 2 in slabs:
                store_combos(wsk_v, pos * 4, slabs.pop(pos), slabs.pop(pos + NV // 2))

    def k_finish(s, hold=0):
        ready = [j for j in range(NP) if j not in finished[s] and _pair_need(j) in logits[s]]
        ready = ready[:len(ready) - hold]
        if defer[0]:
            queue.extend((logits[s].__getitem__, [j], s) for j in ready)
        else:
            k_side(logits[s].__getitem__, ready, s)
        finished[s].update(ready)

    def k_chunk(s, keep=None, early=(), late=(), hold=0):
        todo = [q for half in range(2) for q in range(half * (NV // 2), fk[half].done) if q not in logits[s]]
        runs = [[q for q in todo if q < NV // 2], [q for q in todo if q >= NV // 2]]
        lhs = jnp.concatenate([wtk_v[r[0] * 4:(r[-1] + 1) * 4, :] for r in runs if r], axis=0)
        ties = piece_ties(early, lhs.shape[0])
        ties.update(piece_ties(late, lhs.shape[0], col=HK))
        if ties:
            lhs = _tie(keep, lhs, ties)
        p = _dot_nt(_upk(lhs), xb[s])
        for n, q in enumerate(todo):
            logits[s][q] = p[n * 8:(n + 1) * 8]
        k_finish(s, hold)
        return p

    wait_all(cp_k[0])
    for new in fold_pair(fk, 0):
        absorb(new)
    k_chunk(0)
    k_chunk(1, hold=1)

    wait_all(cp_p[1] + cp_k[1])
    k_finish(1)
    for new in fold_pair(fk, 1):
        absorb(new)
    absorb(fk[0].fold(2))
    amats(1)
    k_chunk(0)
    k_chunk(1, hold=2)

    wait_all(cp_k[2] + [cp_x1])
    defer[0] = True
    keep = flag_s[0] > 0
    absorb(fk[1].fold(6))
    new = fold_pair(fk, 3)
    late = list(new[0].values())[-1][:, 384:512]
    for n in new:
        absorb(n)
    pieces = ln1(x_v, T0, xs_v, T0, T0, [0]) + ln1(x_v, T0, xs_v, T0, T0, [1, 2], keep, [late, late])
    p = k_chunk(0, keep, (), pieces[:2])
    rows = [k * p.shape[0] // 5 // 16 * 16 for k in range(5)]
    pieces += ln1(x_v, T0, xs_v, T0, T0, range(3, 8), keep, [p[r:r + R] for r in rows])
    k_chunk(1, keep, pieces[2:3], pieces[3:])

    def k_emit1(half, blk, val):
        if half != blk:
            k_side(half_groups(val, half), half_pairs(half), 2 + blk)
        else:
            queue.extend((half_groups(val, half), [j], 2 + blk) for j in half_pairs(half))

    def run_queue(n, res):
        deps = []
        for k in range(min(n, len(queue))):
            r = k * res.shape[0] // n // 8 * 8
            v = _vregs(k_side(*queue.pop(0), keep=keep, anchor=res[r:r + 8])[0])
            deps.append([_or_all(v[q::4]) for q in range(4)])
        return deps

    kwork = {}

    def k_after(m, res):
        if m in (0, 2):
            kwork[m + 1] = run_queue(4, res)

    def v_prep(lo, hi):
        for rb in range(lo, hi, 128):
            for c in range(0, HK, 128):
                raw = [wqkv_v[side * HK + c:side * HK + c + 128,
                              2 * D + half * HK + rb:2 * D + half * HK + rb + 128].T
                       for half in range(2) for side in range(2)]
                blocks = [t.astype(f32) for t in raw]
                for n, spec in enumerate(_SA):
                    t = raw[spec[0]] if spec[1] is None else _combo(blocks, spec).astype(bf16)
                    wsv_v[rb // 2:rb // 2 + 64, n * HK + c:n * HK + c + 128] = _pk(t)

    VS = HK // 2

    def k_before(m):
        if m == 5:
            cp_wv.wait()
            cp_x2.wait()
            v_prep(0, VS)

    sproj(wsk_v, xs_v, 1, k_emit1, keep, kwork, k_before, k_after)

    def ln_anchored(xg, src, xd, dst, k, n, keep, res):
        which = list(range(k * 8 // n, (k + 1) * 8 // n))
        rows = [a * HK // len(which) // 16 * 16 for a in range(len(which))]
        pcs = ln1(xg, src, xd, dst, P2, which, keep, [res[r:r + R] for r in rows])
        return [[]] * (3 - len(pcs)) + pcs

    vt, parts = {}, {}
    wsv = wsv_v.at[pl.ds(0, D // 4)]
    work = {0: {}, 1: {}, 2: {}}

    def v_after(q):
        def after(m, res):
            t = 7 * q + m
            u = t + 1
            if 3 <= t < 13:
                work[u // 7][u % 7] = run_queue(-(-len(queue) // (13 - t)), res)
            elif 13 <= t < 20:
                work[u // 7][u % 7] = ln_anchored(x_v, T, xs_v, T, t - 13, 7, keep, res)
        return after

    sealed(wsv_v)
    v_prep(VS, HK)
    zero = pl.multiple_of(flag_s[1], 8)
    for q, lo in enumerate((0, zero + VS // 2)):
        sproj(wsv_v.at[pl.ds(lo, VS // 2)], xs_v, 0,
              lambda half, blk, val: parts.setdefault((blk, half), []).append(val), keep, work[q], None, v_after(q))
    vt.update({k: jnp.concatenate(v, axis=0) for k, v in parts.items()})
    sproj(wsv_v.at[pl.ds(zero, D // 4)], xs_v, 1, lambda half, blk, val: vt.__setitem__((2 + blk, half), val), keep, work[2], None, v_after(2))
    assert not queue
    xjobs = dot_jobs(x_v, num_v.at[pl.ds(P2, T)], range(0, T, R), keep)
    phi_m = sealed(phi_v)
    for j in range(NP):
        prod = kv_prod(vt, _upk(phi_m[j * 64:(j + 1) * 64, :]), j)
        kvacc_v[j] = prod
        if j < 11:
            run_on(xjobs[3 * j:3 * j + 3], prod)
        if j == 2:
            store_xt(1, xs_view(flag_s[1], 2), T // 4, keep, pltpu.bitcast(prod[0:8], u32))
    cp_x3.wait()
    wait_bg(0)

    def p1_body(i, c):
        @pl.when(i == 2)
        def _():
            cp_x4.wait()
            wait_bg(1)

        @pl.when(i == 3)
        def _():
            wait_bg(2)

        keep = flag_s[0] > 0
        lo = jnp.minimum((i - 1) * DCH, F - DCH)
        sv = wd_v.at[pl.ds(pl.multiple_of(lo, 16), DCH)]
        dv = wdp_v.at[pl.ds(pl.multiple_of(lo // 2, 8), DCH // 2)]
        rp = repacker([(sv, dv, r, c) for r in range(0, DCH, 16) for c in range(0, D, 128)], keep,
                      [(q, m) for q in range(2) for m in (0, 2, 4)])
        lo = jnp.minimum((i - 1) * OCH, QK - OCH)
        ov = wo_v.at[pl.ds(pl.multiple_of(lo, 16), 3 * QK + OCH)]
        od = wso_v.at[pl.ds(pl.multiple_of(lo // 2, 8), OCH // 2)]

        def k_emit(q):
            return lambda half, blk, val: k_side(half_groups(val, half), half_pairs(half), 2 * q + blk)

        vt = {}

        def v_emit(q):
            return lambda half, blk, val: vt.__setitem__((2 * q + blk, half), val)

        xd = xs_view(i, 2)
        xa = x_v.at[pl.ds(pl.multiple_of(i * T + P2, P2), P2)]
        xb = x_v.at[pl.ds(pl.multiple_of(jnp.minimum(i + 1, NT - 1) * T, T), P2)]
        wa = {}

        def wo_get(r, c):
            return lambda i0, i1, j0, j1: ov[i0 * HK + i1 * QK + r:i0 * HK + i1 * QK + r + 16,
                                             j0 * HK + j1 * QK + c:j0 * HK + j1 * QK + c + 128].astype(f32)

        wjobs = [job for r in range(0, OCH, 16) for c in (0, 128)
                 for job in combo2_jobs(od, r // 2, c, wo_get(r, c), _SB, keep)]
        assert len(wjobs) == 36 + 6 * 8
        wv = wow_v.at[pl.ds(pl.multiple_of(lo, 16), 3 * QK + OCH)]

        pjobs = dot_jobs(ov, wv, [a * QK + r for a in range(4) for r in range(0, OCH, 16)], keep)
        pjobs += dot_jobs(x_v.at[pl.ds(pl.multiple_of(i * T, T), T)],
                          num_v.at[pl.ds(pl.multiple_of(P2 + i * T, P2), T)], range(0, T, R), keep)

        def k_after(q):
            def after(m, res):
                rp[q](m, res)
                if m in (0, 2, 4):
                    k = 3 * q + m // 2
                    run_on(pjobs[k * len(pjobs) // 6:(k + 1) * len(pjobs) // 6], res, 64)
            return after

        def a_after(m, res):
            if m < 6:
                wa[m + 1] = ln_anchored(xa, 0, xd, P2, m, 6, keep, res)

        sproj(wsv, xd, 0, v_emit(0), keep, wa, None, a_after, xt_view(i))
        sproj(wsk_v, xd, 0, k_emit(0), after=k_after(0))
        sproj(wsk_v, xd, 1, k_emit(1), after=k_after(1))
        wb = spread(ln1(xb, 0, xd, T, P2), [(0, m) for m in range(1, 7)])[0]

        def b_after(m, res):
            if m:
                run_on(wjobs[36 + 8 * (m - 1):36 + 8 * m], res)

        sproj(wsv, xd, 1, v_emit(1), keep, wb, None, b_after)
        phi_m = sealed(phi_v)
        for j in range(NP):
            prod = kv_prod(vt, _upk(phi_m[j * 64:(j + 1) * 64, :]), j)
            kvacc_v[j] += prod
            if j < 12:
                run_on(wjobs[3 * j:3 * j + 3], prod)
            if j == 2:
                store_xt(i + 1, xd, T // 4, keep, pltpu.bitcast(prod[0:8], u32))
        return c

    lax.fori_loop(1, NT, p1_body, 0)

    wait_all([cp_wq] + cp_gu[0])
    keep = flag_s[0] > 0
    kv_mask = (lax.broadcasted_iota(jnp.int32, (64, 128), 0) // DH
               == (lax.broadcasted_iota(jnp.int32, (64, 128), 1) // DH) % 2)
    ties = [{} for _ in range(16)]
    for j in range(NP):
        kvj = jnp.where(kv_mask, kvacc_v[j], 0.0)
        kv_v[:, j * 128:(j + 1) * 128] = _pk(kvj.astype(bf16))
        zj = _lanes(jnp.sum(zacc_v[j * 128:(j + 1) * 128, :], axis=-1, keepdims=True))
        zacc_v[j * 128:(j + 1) * 128, :] = zj
        vals = _vregs(kvj) + _vregs(zj)
        if j + 1 < 16:
            for q in range(4):
                ties[j + 1][(32 + q * 8, 0)] = _or_all(vals[q::4])
    for c in range(0, D, 128):
        t = jnp.sum(wow_v[c:c + 128, :].T.reshape(16, 8, 128), axis=0)
        cb_v[:, c:c + 128] = _allreduce8(t[None], jnp.add)[0]
    store_xt(0, xs_v, 0)
    fq = (Folder(0), Folder(0, NV // 2))
    for g in range(4):
        new = fold_pair(fq, g, keep, ties[4 * g:4 * g + 4])
        for pos, slab in new[0].items():
            store_combos(wsq_v, pos * 4, slab, new[1][pos + NV // 2])

    pq_v = (pq0_v, pq1_v, pq2_v, pq3_v)

    def views_of(g):
        lo = g * (BPI * B)
        if not isinstance(g, int):
            lo = pl.multiple_of(lo, BPI * B)
        return ((x_v.at[pl.ds(lo, BPI * B)],)
                + tuple(ref.at[pl.ds(lo, P2 + BPI * B)] for ref in (h_v, out_v, st_v)) + (g, num_v.at[pl.ds(lo, P2 + BPI * B)]))

    def stage_q(xd, q, first, before, after):
        def emit(half, blk, val):
            group = half_groups(val, half)
            for j in half_pairs(half):
                p, j = _pair_logits(group, j), _phys_pair(j)
                ph = _hedgehog_t(p, zacc_v[j * 128:(j + 1) * 128, :])
                pq_v[2 * q + blk][(j // 2) * 64:(j // 2 + 1) * 64, (j % 2) * B:(j % 2 + 1) * B] = _pk(ph.astype(bf16))

        sproj(wsq_v, xd, q, emit, before=before, after=after, first=first)

    oc_v = (oc0_v, oc1_v)
    on_v = (on0_v, on1_v)

    def stage_g(q):
        pq = [sealed(pq_v[2 * q + blk]) for blk in range(2)]
        for t in range(NP // 4):
            parts = [[_dot_nn(_upk(kv_v[:, j * 128:(j + 1) * 128]),
                              _upk(pq[blk][(j // 2) * 64:(j // 2 + 1) * 64, (j % 2) * B:(j % 2 + 1) * B]))
                      for blk in range(2) for j in (jj, jj + NP // 2)] for jj in (2 * t, 2 * t + 1)]
            blocks = [jnp.concatenate([a, b], axis=0) for a, b in zip(*parts)]
            for k, blk in enumerate(blocks):
                c = (k % 2) * HK + t * 128
                on_v[q][(k // 2) * B:(k // 2 + 1) * B, c:c + 128] = blk.T

    def combo_jobs(q, keep):
        def get(r, c):
            def f(i0, i1, j0, j1):
                on = on_v[q].at[pl.ds(pl.multiple_of(flag_s[1], 8), P2)]
                return on[i0 * B + i1 * 64 + r:i0 * B + i1 * 64 + r + 16,
                          j0 * HK + j1 * QK + c:j0 * HK + j1 * QK + c + 128]
            return f
        return [job for c in (0, 128) for r in range(0, 64, 16)
                for job in combo2_jobs(oc_v[q], r // 2, c, get(r, c), _SA, keep)]

    def stage_h(views, q, sched, before, emitted):
        x_g, h_g = views[0], views[1]
        oc = sealed(oc_v[q])

        def product(m):
            if before:
                before(m)
            quad = {}

            def inner(n):
                col = (7 * m + n) * QK
                res = _dot_nn(_upk(oc[0:B // 4, col:col + QK]), _upk(wso_v[:, col:col + QK]))
                mine = sched.pop(49 * q + 7 * m + n, [])
                if mine:
                    run_on(mine, res)
                return res

            _strassen(inner, quad.__setitem__)
            return jnp.concatenate([jnp.concatenate([quad[0], quad[1]], axis=1),
                                    jnp.concatenate([quad[2], quad[3]], axis=1)], axis=0)

        def emit(k, val):
            blk, half = k // 2, k % 2
            s = 2 * q + blk
            cols = slice(half * HK, (half + 1) * HK)
            h = x_g[s * B:(s + 1) * B, cols].astype(f32) + val
            h_g[(s + 2) * B:(s + 3) * B, cols] = h
            emitted(blk, half, h)

        _strassen(product, emit)

    def num_jobs(views, q, keep):
        def job(r):
            def run(anchor):
                on = on_v[q].at[pl.ds(pl.multiple_of(flag_s[1], 8), P2)]
                rows = slice((2 * q + 2) * B + r, (2 * q + 2) * B + r + R)
                o = on[r:r + R, :]
                o = jnp.concatenate([jnp.where(keep, o[:, :128], anchor), o[:, 128:]], axis=1)
                t = _lane_dot(o, cb_v) + views[5][rows, :]
                views[5][rows, :] = _lanes(jnp.sum(t, axis=-1, keepdims=True))
            return run
        return [job(r) for r in range(0, P2, R)]

    def moments(st, mom, k, h, keep=None, anchor=None):
        first = 'h0' not in st
        if first:
            st['h0'] = h[:, 0:128]
            acc = None
        else:
            prev = mom[pl.ds(pl.multiple_of(flag_s[1] + k * R, R), R), :]
            acc = [prev[:, n * 128:(n + 1) * 128] for n in range(2)]
        h0 = st['h0'] if anchor is None else jnp.where(keep, st['h0'], anchor)
        for c in range(128 if first else 0, HK, 128):
            d = h[:, c:c + 128] - h0
            new = (d, d * d)
            acc = new if acc is None else [a + b for a, b in zip(acc, new)]
        if first:
            mom[k * R:(k + 1) * R, :] = jnp.concatenate(
                list(acc) + [_lanes(jnp.mean(h0, axis=-1, keepdims=True))], axis=1)
            return None
        s1, s2 = acc
        c0 = prev[:, 256:384]
        g0 = st['h0'] - c0
        t1 = s1 + 8.0 * g0
        return t1, s2 + g0 * (s1 + t1), c0

    def stats(views, s, k, part, valid=None):
        st_g, g = views[3], views[4]
        sl = slice(k * R, (k + 1) * R)
        rows = slice((s + 2) * B + k * R, (s + 2) * B + (k + 1) * R)
        mu = _lanes(jnp.sum(part[0], axis=-1, keepdims=True)) * (1.0 / D)
        m2 = _lanes(jnp.sum(part[1], axis=-1, keepdims=True)) * (1.0 / D)
        rs = lax.rsqrt(jnp.maximum(m2 - mu * mu, 0.0) + LN_EPS)
        st_g[rows, :] = jnp.concatenate([rs, (mu + part[2]) * rs], axis=1)
        r = views[5][rows, :] * rs
        if valid is not None:
            r = jnp.where(valid, r, -jnp.inf)
        idx = lax.broadcasted_iota(jnp.int32, (R, 128), 0) + ((g * BPI + s) * B + k * R)
        bv = bestv_v[sl, :]
        better = r > bv
        bestv_v[sl, :] = jnp.where(better, r, bv)
        besti_v[sl, :] = jnp.where(better, idx, besti_v[sl, :])

    def out_jobs(views, s, keep):
        h_g, out_g, st_g = views[1], views[2], views[3]

        def job(k):
            def run(anchor):
                rows = slice((s + 2) * B + k * R, (s + 2) * B + (k + 1) * R)
                hk = h_g[rows, :]
                sk = st_g[rows, :]
                a = 1.0 + jnp.where(keep, sk[:, 0:128], anchor)
                o = [hk[:, c * 128:(c + 1) * 128] * a - sk[:, 128:256] for c in range(D // 128)]
                out_g[rows, :] = jnp.concatenate(o, axis=1).astype(bf16)
            return run
        return [job(k) for k in range(B // R)]

    def late_stats(views, s, k, keep=None, anchor=None, valid=None):
        r0 = (s + 2) * B + k * R
        blk = s % 2
        c0, c1 = (0, HK) if blk else (HK, 0)
        st = {'h0': views[1][r0:r0 + R, c0:c0 + 128]}
        part = moments(st, (mom0_v, mom1_v)[blk], k, views[1][r0:r0 + R, c1:c1 + HK], keep, anchor)
        stats(views, s, k, part, valid)

    def p2_body(i, c):
        b0 = i * BPI
        keep = flag_s[0] > 0
        cur = views_of(i)
        n = D // NI
        jobs = []
        for src, dst in ((wg_v, wgp_v), (wu_v, wup_v)):
            sv = src.at[pl.ds(pl.multiple_of(i * n, n), n)]
            dv = dst.at[pl.ds(pl.multiple_of(i * (n // 2), n // 2), n // 2)]
            jobs += [(sv, dv, r, cc) for r in range(0, n, 16) for cc in range(0, NM, 128)]
        rp, _ = repacker(jobs, keep, [(0, 0), (0, 2), (0, 4)])

        def q0_after(m, res):
            rp(m, res)
            if m == 0:
                run_on([lambda a, k=k: late_stats(cur, -1, k, keep, a, i > 0) for k in range(B // R)], res, 0, 400)

        cj = combo_jobs(0, keep)

        def q1_after(m, res):
            if m in (2, 4):
                run_on(cj[(m // 4) * 28:(m // 4 + 1) * 28], res, 32)

        stage_q(xs_view(i, 1), 0, xt_view(i), None, q0_after)
        stage_q(xs_view(i, 1), 1, None, lambda m: stage_g(0) if m == 1 else None, q1_after)

        sched = {}

        def at(jobs, lo, hi):
            for k, job in enumerate(jobs):
                sched.setdefault(lo + k * (hi - lo) // len(jobs), []).append(job)

        at(out_jobs(cur, -2, keep), 3, 7)
        at(out_jobs(cur, -1, keep), 36, 44)
        at(combo_jobs(1, keep), 15, 44)
        at(num_jobs(cur, 0, keep), 20, 40)
        at(num_jobs(cur, 1, keep), 63, 79)
        state = {}
        when = {(1, False): (18, 28), (0, False): (30, 40), (0, True): (44, 54), (1, True): (54, 63),
                (3, False): (67, 77), (2, False): (79, 89), (2, True): (91, 94)}

        def emitted(q):
            def f(blk, half, h):
                s = 2 * q + blk
                second = s in state
                sts = state.setdefault(s, [{} for _ in range(B // R)])

                def job(k):
                    def run(anchor):
                        part = moments(sts[k], (mom0_v, mom1_v)[blk], k, h[k * R:(k + 1) * R], keep, anchor)
                        if second:
                            stats(cur, s, k, part)
                    return run

                if (s, second) in when:
                    at([job(k) for k in range(B // R)], *when[(s, second)])
                if second and q == 0:
                    at(out_jobs(cur, s, keep), 70 + 14 * blk, 77 + 14 * blk)
            return f

        stage_h(cur, 0, sched, lambda m: stage_g(1) if m == 1 else None, emitted(0))
        stage_h(cur, 1, sched, None, emitted(1))
        assert not sched

        @pl.when(i > 0)
        def _():
            cp_out(jnp.maximum(b0 - 2, 0), 2).start()

        cp_out(b0, 2).start()
        return c

    lax.fori_loop(0, NI, p2_body, 0)
    wait_all(cp_gu[1])
    keep = flag_s[0] > 0
    last = views_of(NI - 1)

    for k in range(B // R):
        late_stats(last, BPI - 1, k)

    bv = bestv_v[...]
    mval = jnp.max(bv, axis=0, keepdims=True)
    sel = jnp.min(jnp.where(bv == mval, besti_v[...], S - 1), axis=0, keepdims=True)
    idx = jnp.clip(sel[0, 0], 0, S - 1)
    hrow = h_v[pl.ds(P2 + idx, 1), :]
    strow = st_v[pl.ds(P2 + idx, 1), :]
    xrow = jnp.concatenate([hrow[:, c * 128:(c + 1) * 128] * strow[:, 0:128] - strow[:, 128:256]
                            for c in range(D // 128)], axis=1).astype(bf16)
    xs = jnp.broadcast_to(xrow, (16, D))
    g_first = _dot_nn(xs, _upk(wgp_v[:, 0:FC]))
    anchors = ([jnp.broadcast_to(pltpu.bitcast(sel, f32), (R, 128))] * 4
               + [jnp.broadcast_to(xrow[:, 0:128].astype(f32), (R, 128))] * 4
               + [g_first[:, (k // 2) * 128:(k // 2 + 1) * 128] for k in range(8)])
    for job, anchor in zip(out_jobs(last, BPI - 2, keep) + out_jobs(last, BPI - 1, keep), anchors):
        job(anchor)
    cp_out(NB - 2, 2).start()

    def act(g, u):
        a = g * pl.reciprocal(1.0 + jnp.exp(-g), approx=True) * u
        return jnp.concatenate([a, a], axis=0).astype(bf16)

    def down(a, lo, w):
        return _dot_nn(a, _upk(wdp_v[lo // 2:(lo + w) // 2, 0:D]))[0:8]

    xcol = jnp.broadcast_to(xrow, (128, D)).T.astype(f32)
    jobs = [(which, b) for b in range(NBV) for which in (0, 1)]
    vres, prev = {}, None
    for j0 in range(0, len(jobs), NCH):
        grp = jobs[j0:j0 + NCH]
        accs = [None] * len(grp)
        for r in range(D // 16):
            for n, (which, b) in enumerate(grp):
                w = (wg_v, wu_v)[which][r * 16:(r + 1) * 16, NM + b * 128:NM + (b + 1) * 128].astype(f32)
                t0 = w[0:8] * xcol[r * 16:r * 16 + 8]
                t1 = w[8:16] * xcol[r * 16 + 8:r * 16 + 16]
                if accs[n] is None:
                    if prev is not None:
                        t0 = jnp.where(keep, t0, prev[n % len(prev)])
                    accs[n] = t0 + t1
                else:
                    accs[n] = (accs[n] + t0) + t1
        prev = accs
        for n, job in enumerate(grp):
            vres[job] = _allreduce8(accs[n][None], jnp.add)[0]

    chunks = [(lo, min(FC, NM - lo)) for lo in range(0, NM, FC)]
    acts, y = [], None
    for k, (lo, w) in enumerate(chunks):
        g = g_first if k == 0 else _dot_nn(xs, _upk(wgp_v[:, lo:lo + w]))
        u = _dot_nn(xs, _upk(wup_v[:, lo:lo + w]))
        acts.append(act(g[0:8], u[0:8]))
        if k >= 1:
            t = down(acts[k - 1], *chunks[k - 1])
            y = t if y is None else y + t
    y = y + down(acts[-1], *chunks[-1])
    for b0, nb in ((0, 4), (4, 4), (8, 4), (12, 1)):
        g = jnp.concatenate([vres[(0, b)] for b in range(b0, b0 + nb)], axis=1)
        u = jnp.concatenate([vres[(1, b)] for b in range(b0, b0 + nb)], axis=1)
        y = y + down(act(g, u), NM + b0 * 128, nb * 128)

    gate = jnp.broadcast_to(jax.nn.sigmoid(mval), (8, 128))
    base = pl.multiple_of((idx >> 4) << 4, 16)
    rows = pl.ds(pl.multiple_of(P2 + base, 16), 16)
    h16 = h_v[rows, :]
    st16 = st_v[rows, :]
    a16 = 1.0 + st16[:, 0:128]
    m16 = st16[:, 128:256]
    hit = (lax.broadcasted_iota(jnp.int32, (16, 128), 0) + base) == idx
    res = []
    for c in range(D // 128):
        yc = y[:, c * 128:(c + 1) * 128] * gate
        yc = jnp.concatenate([yc, yc], axis=0)
        res.append(h16[:, c * 128:(c + 1) * 128] * a16 - m16 + jnp.where(hit, yc, 0.0))
    res = jnp.concatenate(res, axis=1).astype(bf16)
    for i in range(NI):
        cp_out(i * BPI, 2).wait()
        cp_out(i * BPI + 2, 2).wait()
    out_v[rows, :] = res
    fix = pltpu.make_async_copy(out_v.at[rows], out_hbm.at[pl.ds(base, 16)], sem_o.at[0])
    fix.start()
    fix.wait()


@jax.jit
def pallas_sequential_preLN__linear_kernel_hedgehog__moe_arch_mod__prompt_kernel(
    A_x: jax.Array,
    A_wqkv: jax.Array,
    A_w_phi: jax.Array,
    A_wo: jax.Array,
    B_x: jax.Array,
    B_w_r: jax.Array,
    B_w_gate: jax.Array,
    B_w_up: jax.Array,
    B_w_down: jax.Array,
):
    del B_x
    x = A_x.reshape(S, D)
    wphi = A_w_phi.reshape(H * DH, DH)
    wr = B_w_r.reshape(8, 128)
    any_spec = pl.BlockSpec(memory_space=pl.ANY)
    out = pl.pallas_call(
        _kernel,
        out_shape=jax.ShapeDtypeStruct((S, D), bf16),
        in_specs=[any_spec] * 8,
        out_specs=any_spec,
        scratch_shapes=[
            pltpu.VMEM((S, D), bf16),
            pltpu.VMEM((D, 3 * D), bf16),
            pltpu.VMEM((H * DH, DH), bf16),
            pltpu.VMEM((D, D), bf16),
            pltpu.VMEM((64, 128), bf16),
            pltpu.VMEM((D, F + 128), bf16),
            pltpu.VMEM((D, F + 128), bf16),
            pltpu.VMEM((F, D), bf16),
            pltpu.VMEM((PR, D), u32),
            pltpu.VMEM((PR // 2, 7 * HK), u32),
            pltpu.VMEM((PR // 2, 7 * HK), u32),
            pltpu.VMEM((D // 4 + 8, 7 * HK), u32),
            pltpu.VMEM((QK // 2, 49 * QK), u32),
            pltpu.VMEM((F // 2, D + 128), u32),
            pltpu.VMEM((D // 2, NM), u32),
            pltpu.VMEM((D // 2, NM), u32),
            pltpu.VMEM((64, 8 * 128), u32),
            pltpu.VMEM((T0 // 2, D), u32),
            pltpu.VMEM(((S + T) // 4, 7 * HK), u32),
            pltpu.VMEM(((NT + 1) * (HK // 2), B), u32),
            pltpu.VMEM((NP, 64, 128), f32),
            pltpu.VMEM((2 * D, 128), f32),
            pltpu.VMEM((32, NP * 128), u32),
            pltpu.VMEM((D + 8, T), u32),
            pltpu.VMEM((D // 2 + 16, 2 * B), u32),
            pltpu.VMEM((D // 2 + 16, 2 * B), u32),
            pltpu.VMEM((D // 2 + 16, 2 * B), u32),
            pltpu.VMEM((D // 2 + 16, 2 * B), u32),
            pltpu.VMEM((B // 4 + 16, 49 * QK), u32),
            pltpu.VMEM((B // 4 + 16, 49 * QK), u32),
            pltpu.VMEM((P2, D), f32),
            pltpu.VMEM((P2, D), f32),
            pltpu.VMEM((P2 + S, D), f32),
            pltpu.VMEM((P2 + S, 256), f32),
            pltpu.VMEM((B, 384), f32),
            pltpu.VMEM((B, 384), f32),
            pltpu.VMEM((P2 + S, D), bf16),
            pltpu.VMEM((8, D), f32),
            pltpu.VMEM((8, D), f32),
            pltpu.VMEM((D, 128), f32),
            pltpu.VMEM((P2 + S, 128), f32),
            pltpu.VMEM((B, 128), f32),
            pltpu.VMEM((B, 128), jnp.int32),
            pltpu.SMEM((2,), jnp.int32),
            pltpu.SemaphoreType.DMA((_NSEM_IN,)),
            pltpu.SemaphoreType.DMA((1,)),
        ],
        compiler_params=pltpu.CompilerParams(vmem_limit_bytes=120 * 1024 * 1024,
                                             disable_bounds_checks=True,
                                             disable_semaphore_checks=True),
        name="hedgehog_mod",
    )(x, A_wqkv, wphi, A_wo, wr, B_w_gate, B_w_up, B_w_down)
    return out.reshape(1, S, D)
```

```python
import jax
import jax.numpy as jnp
from jax import lax
import jax.experimental.pallas as pl
import jax.experimental.pallas.tpu as pltpu

S = 2048
D = 1024
H = 32
DH = 32
F = 3584
T = 512
NT = S // T
T0 = 256
B = 128
NB = S // B
BPI = 4
NI = NB // BPI
NP = H // 2
FC = 1024
R = 16
NBV = 13
NM = F - NBV * 128
NCH = 4
QK = D // 4
OCH = 96
DCH = 1216
NV = 124
PR = NV * 4
HK = D // 2
P2 = 2 * B
LOG2E = 1.4426950408889634
LN_EPS = 1e-5
DEN_EPS = 1e-6

_NT_DIMS = (((1,), (1,)), ((), ()))

bf16 = jnp.bfloat16
f32 = jnp.float32
u32 = jnp.uint32


def _dot_nt(a, b):
    return lax.dot_general(a, b, _NT_DIMS, preferred_element_type=f32)


def _dot_nn(a, b):
    return jnp.dot(a, b, preferred_element_type=f32)


def _pk(x):
    return pltpu.bitcast(x, u32)


def _upk(x):
    return pltpu.bitcast(x, bf16)


def _lanes(x):
    return jnp.broadcast_to(x, (x.shape[0], 128))


def _layernorm(x):
    m = jnp.mean(x, axis=-1, keepdims=True)
    xc = x - m
    v = jnp.mean(xc * xc, axis=-1, keepdims=True)
    return xc * lax.rsqrt(v + LN_EPS)


def _lane_dot(x, w):
    acc = None
    for c in range(0, x.shape[1], 128):
        t = x[:, c:c + 128].reshape(x.shape[0] // 8, 8, 128) * w[:, c:c + 128][None]
        acc = t if acc is None else acc + t
    return acc.reshape(x.shape[0], 128)


def _allreduce8(x, op):
    x = op(x, pltpu.roll(x, 4, 1))
    x = op(x, pltpu.roll(x, 2, 1))
    x = op(x, pltpu.roll(x, 1, 1))
    return x


def _hedgehog_t(p, z=None):
    t = p.shape[-1]
    p4 = p.reshape(2, 4, 8, t)
    mx = _allreduce8(jnp.max(p4, axis=1), jnp.maximum)
    mn = _allreduce8(jnp.min(p4, axis=1), jnp.minimum)
    ep = jnp.exp2(p4 - mx[:, None])
    en = jnp.exp2(mn[:, None] - p4)
    a = pl.reciprocal(_allreduce8(jnp.sum(ep, axis=1), jnp.add), approx=True)
    b = pl.reciprocal(_allreduce8(jnp.sum(en, axis=1), jnp.add), approx=True)
    if z is not None:
        dp = jnp.sum(ep * z[0:64].reshape(2, 4, 8, t), axis=1)
        dn = jnp.sum(en * z[64:128].reshape(2, 4, 8, t), axis=1)
        den = _allreduce8(dp * a + dn * b, jnp.add) + DEN_EPS
        inv = pl.reciprocal(den, approx=True)
        a = a * inv
        b = b * inv
    fp = (ep * a[:, None]).reshape(64, t)
    fn = (en * b[:, None]).reshape(64, t)
    return jnp.concatenate([fp, fn], axis=0)


_SA = ((3, None, 0), (2, 3, 1), (0, 1, 1), (0, None, 0), (0, 3, 1), (1, 3, -1), (2, 0, -1))
_SB = ((2, 0, -1), (0, None, 0), (3, None, 0), (1, 3, -1), (0, 3, 1), (2, 3, 1), (0, 1, 1))


def _combo(blocks, spec):
    a, b, sign = spec
    if b is None:
        return blocks[a]
    return blocks[a] + blocks[b] if sign > 0 else blocks[a] - blocks[b]


def _strassen(product, emit):
    m4 = product(0)
    m2 = product(1)
    emit(2, m4 + m2)
    m5 = product(2)
    u = m4 - m5
    m3 = product(3)
    emit(1, m5 + m3)
    v = m3 - m2
    m1 = product(4)
    u = u + m1
    v = v + m1
    emit(0, u + product(5))
    emit(3, v + product(6))


def _head_groups(h):
    base, k = (NV // 4) * (h // 8), h % 8
    return ([base + 4 * k + i for i in range(3)],
            base + 4 * k - 1 if k > 0 else None,
            base + 4 * k + 3 if k < 7 else None,
            8 - k)


def _pair_logits(group, j):
    parts = []
    for h in (2 * j, 2 * j + 1):
        full, below, above, a = _head_groups(h)
        ref = group(full[0])
        sub = lax.broadcasted_iota(jnp.int32, ref.shape, 0)
        if above is None:
            m = jnp.where(sub >= a, group(below), 0.0)
        else:
            m = jnp.where(sub == a - 1, 0.0, group(above))
            if below is not None:
                m = jnp.where(sub >= a, group(below), m)
        parts += [m] + [group(q) for q in full]
    return jnp.concatenate(parts, axis=0)


def _pair_need(j):
    full, _, above, _ = _head_groups(2 * j + 1)
    return full[2] if above is None else above


def _tie(keep, w, ties):
    rows = sorted({r for r, _ in ties})
    out, pos = [], 0
    for r in rows:
        if r > pos:
            out.append(w[pos:r])
        cols = sorted(c for rr, c in ties if rr == r)
        parts, cpos = [], 0
        for c in cols:
            if c > cpos:
                parts.append(w[r:r + 8, cpos:c])
            parts.append(jnp.where(keep, w[r:r + 8, c:c + 128], ties[(r, c)]))
            cpos = c + 128
        if cpos < w.shape[1]:
            parts.append(w[r:r + 8, cpos:])
        out.append(jnp.concatenate(parts, axis=1) if len(parts) > 1 else parts[0])
        pos = r + 8
    if pos < w.shape[0]:
        out.append(w[pos:])
    return jnp.concatenate(out, axis=0)


def _vregs(x):
    if x.dtype != u32:
        x = pltpu.bitcast(x, u32)
    return [x[r:r + 8, c:c + 128] for r in range(0, x.shape[0], 8) for c in range(0, x.shape[1], 128)]


def _or_all(vals):
    acc = vals[0]
    for v in vals[1:]:
        acc = acc | v
    return acc


def _phys_group(g):
    return 2 * (g % 4) + g // 4


def _phys_pair(j):
    return 2 * _phys_group(j // 2) + j % 2


_KSTAGES = (((0, 2),), ((2, 3),), ((5, 3),))
_PSTAGES = (((0, 5),), ((5, 3),))
_NSEM_IN = 11


def _kernel(x_hbm, wqkv_hbm, wphi_hbm, wo_hbm, wr_hbm, wg_hbm, wu_hbm, wd_hbm,
            out_hbm,
            x_v, wqkv_v, wphi_v, wo_v, wr_v, wg_v, wu_v, wd_v,
            wtk_v, wsq_v, wsk_v, wsv_v, wso_v, wdp_v, wgp_v, wup_v, amat_v, xn_v, xs_v, xt_v,
            kvacc_v, zacc_v, kv_v, phi_v,
            pq0_v, pq1_v, pq2_v, pq3_v, oc0_v, oc1_v, on0_v, on1_v, h_v, st_v, mom0_v, mom1_v, out_v, wrb_v, cb_v, wow_v, num_v,
            bestv_v, besti_v, flag_s,
            sem_i, sem_o):

    def cp_x(lo, n, sem):
        return pltpu.make_async_copy(x_hbm.at[pl.ds(lo, n)], x_v.at[pl.ds(lo, n)], sem_i.at[sem])

    def cp_w(lo, w, sem):
        return pltpu.make_async_copy(wqkv_hbm.at[:, pl.ds(lo, w)], wqkv_v.at[:, pl.ds(lo, w)], sem_i.at[sem])

    cp_k = [[cp_w(D + g * 128, n * 128, 2 + c) for g, n in st] for c, st in enumerate(_KSTAGES)]
    cp_p = [[pltpu.make_async_copy(wphi_hbm.at[pl.ds(g * 128, n * 128)], wphi_v.at[pl.ds(g * 128, n * 128)],
                                   sem_i.at[3 * c]) for g, n in st] for c, st in enumerate(_PSTAGES)]
    cp_wv = cp_w(2 * D, D, 5)
    cp_wq = cp_w(0, D, 7)

    def cp_wd(k):
        lo, n = k * DCH, min(DCH, F - k * DCH)
        return pltpu.make_async_copy(wd_hbm.at[pl.ds(lo, n)], wd_v.at[pl.ds(lo, n)], sem_i.at[(6, 8, 9)[k]])

    cp_x0 = cp_x(0, T0, 1)
    cp_x1 = cp_x(T0, T0, 4)
    cp_x2 = cp_x(T, P2, 5)
    cp_x3 = cp_x(T + P2, T, 6)
    cp_x4 = cp_x(2 * T + P2, S - 2 * T - P2, 8)
    cp_wr = pltpu.make_async_copy(wr_hbm, wr_v.at[pl.ds(0, 8)], sem_i.at[0])

    def cp_wo(k):
        lo, n = k * OCH, min(OCH, QK - k * OCH)
        return [pltpu.make_async_copy(wo_hbm.at[pl.ds(a * QK + lo, n)], wo_v.at[pl.ds(a * QK + lo, n)],
                                      sem_i.at[(6, 8, 9)[k]]) for a in range(4)]

    def wait_bg(k):
        for cp in cp_wo(k):
            cp.wait()
        cp_wd(k).wait()

    cp_gu = [[pltpu.make_async_copy(src.at[:, pl.ds(lo, n)], dst.at[:, pl.ds(lo, n)], sem_i.at[sem])
              for src, dst in ((wg_hbm, wg_v), (wu_hbm, wu_v))] for lo, n, sem in ((0, NM, 7), (NM, F - NM, 10))]

    def cp_out(b, n):
        lo = b * B
        if not isinstance(b, int):
            lo = pl.multiple_of(lo, B)
        return pltpu.make_async_copy(out_v.at[pl.ds(P2 + lo, n * B)], out_hbm.at[pl.ds(lo, n * B)], sem_o.at[0])

    for cp in (cp_wr, *cp_p[0], cp_x0, *cp_k[0], *cp_p[1], *cp_k[1], *cp_k[2], cp_x1, cp_wv, cp_x2,
               cp_x3, *cp_wo(0), cp_wd(0), cp_x4, *cp_wo(1), cp_wd(1), *cp_wo(2), cp_wd(2), cp_wq, *cp_gu[0], *cp_gu[1]):
        cp.start()
    flag_s[0] = 1
    flag_s[1] = 0

    def ln1(xg, src, xd, dst, n, which=None, keep=None, anchors=None, plain=False):
        pieces = []
        for pr in range(n // P2):
            for k in range(B // R):
                off = pr * P2 + k * R
                if which is not None and pr * (B // R) + k not in which:
                    continue
                x0 = xg[src + off:src + off + R, :].astype(f32)
                x1 = xg[src + off + B:src + off + B + R, :].astype(f32)
                if anchors is not None:
                    a = anchors[len(pieces)]
                    x0 = jnp.concatenate([jnp.where(keep, x0[:, :128], a), x0[:, 128:]], axis=1)
                    x1 = jnp.concatenate([jnp.where(keep, x1[:, :128], a), x1[:, 128:]], axis=1)
                p0 = _layernorm(x0)
                p1 = _layernorm(x1)
                if plain:
                    xn_v[off // 2:(off + R) // 2, :] = _pk(p0.astype(bf16))
                    xn_v[(off + B) // 2:(off + B + R) // 2, :] = _pk(p1.astype(bf16))
                lo = (dst + pr * P2) // 4 + k * (R // 2)
                blocks = (p0[:, :HK], p1[:, :HK], p0[:, HK:], p1[:, HK:])
                vs = []
                for m, spec in enumerate(_SB):
                    t = _combo(blocks, spec)
                    xd[lo:lo + R // 2, m * HK:(m + 1) * HK] = _pk(t.astype(bf16))
                    if spec[1] is not None:
                        vs.append(_vregs(t))
                pieces.append([_or_all(list(col)) for col in zip(*vs)])
        return pieces

    def load_xn(b):
        return _upk(xn_v[b * (B // 2):(b + 1) * (B // 2), :])

    def piece_ties(pieces, n, row0=0, col=0):
        ties = {}
        if pieces:
            step = (n - row0) // len(pieces) // 8 * 8
            for k, p in enumerate(pieces):
                for q, val in enumerate(p):
                    ties[(row0 + k * step + (q // 4) * 8, col + (q % 4) * 128)] = val
        return ties

    def xs_view(i, tiles):
        return xs_v.at[pl.ds(pl.multiple_of(i * (T // 4), T // 4), tiles * (T // 4))]

    def xt_view(i):
        lo = i * (HK // 2)
        return xt_v.at[pl.ds(lo if isinstance(i, int) else pl.multiple_of(lo, HK // 2), HK // 2)]

    def store_xt(i, xd, row, keep=None, anchor=None):
        v = xd[row:row + B // 2, 0:HK]
        if anchor is not None:
            v = _tie(keep, v, {(0, c): anchor for c in range(0, HK, 128)})
        xt_view(i)[...] = _pk(_upk(v).T)

    def sproj(ws, xd, pr, emit, keep=None, work=None, before=None, after=None, first=None):
        lo = pr * (B // 2)

        def product(m):
            if before:
                before(m)
            lhs = ws[:, m * HK:(m + 1) * HK]
            if work is not None and work.get(m):
                lhs = _tie(keep, lhs, piece_ties(work[m], lhs.shape[0], 32))
            if m == 0 and first is not None:
                res = _dot_nn(_upk(lhs), _upk(first[...]))
            else:
                res = _dot_nt(_upk(lhs), _upk(xd[lo:lo + B // 2, m * HK:(m + 1) * HK]))
            if after:
                after(m, res)
            return res

        _strassen(product, lambda k, val: emit(k // 2, k % 2, val))

    def repacker(jobs, keep, slots):
        def hook(q):
            def after(m, res):
                if (q, m) in slots:
                    k = slots.index((q, m))
                    mine = jobs[k * len(jobs) // len(slots):(k + 1) * len(jobs) // len(slots)]
                    for n, (sv, dv, r, c) in enumerate(mine):
                        a = (64 + n * 416 // len(mine)) // 8 * 8
                        dv[r // 2:r // 2 + 8, c:c + 128] = jnp.where(keep, _pk(sv[r:r + 16, c:c + 128]),
                                                                     pltpu.bitcast(res[a:a + 8], u32))
            return after
        return hook(0), hook(1)

    def spread(pieces, slots):
        res = {}
        for k, (pr, m) in enumerate(slots):
            res.setdefault(pr, {})[m] = pieces[k * len(pieces) // len(slots):(k + 1) * len(pieces) // len(slots)]
        return res

    def sealed(ref):
        ref[pl.ds(pl.multiple_of(flag_s[1] + ref.shape[0] - 8, 8), 8), 0:128] = jnp.zeros((8, 128), ref.dtype)
        return ref

    def store_combos(ws, row, top, bot):
        for c in range(0, HK, 128):
            blocks = [top[:, c:c + 128], top[:, HK + c:HK + c + 128], bot[:, c:c + 128], bot[:, HK + c:HK + c + 128]]
            for m, spec in enumerate(_SA):
                ws[row:row + 8, m * HK + c:m * HK + c + 128] = _pk(_combo(blocks, spec).astype(bf16))

    def combo2_jobs(dst, row, c, get, table, keep):
        def job(m):
            def run(anchor):
                a, b, sign = table[m]
                o = []
                for i1 in range(2):
                    for j1 in range(2):
                        v = get(a // 2, i1, a % 2, j1)
                        if i1 == j1:
                            v = jnp.where(keep, v, anchor)
                        if b is not None:
                            w = get(b // 2, i1, b % 2, j1)
                            v = v + w if sign > 0 else v - w
                        o.append(v)
                for n, si in enumerate(table):
                    col = (7 * m + n) * QK + c
                    dst[row:row + 8, col:col + 128] = _pk(_combo(o, si).astype(bf16))
            return run
        return [job(m) for m in range(7)]

    def run_on(jobs, res, lo=0, hi=None):
        hi = res.shape[0] - R if hi is None else hi
        for n, job in enumerate(jobs):
            a = (lo + n * (hi - lo) // len(jobs)) // 8 * 8
            job(res[a:a + R, 0:128])

    def dot_jobs(src, dst, rows, keep):
        def job(r):
            def run(anchor):
                w = src[r:r + R, :].astype(f32)
                w = jnp.concatenate([jnp.where(keep, w[:, :128], anchor), w[:, 128:]], axis=1)
                dst[r:r + R, :] = _lane_dot(w, wrb_v)
            return run
        return [job(r) for r in rows]

    zinit = set()

    def k_side(group, pairs, slot, keep=None, anchor=None):
        res = []
        for j in pairs:
            p = _pair_logits(group, j)
            if anchor is not None:
                p = jnp.concatenate([jnp.where(keep, p[0:8], anchor), p[8:32],
                                     jnp.where(keep, p[32:40], anchor), p[40:64]], axis=0)
            ph = _hedgehog_t(p)
            j = _phys_pair(j)
            if j not in zinit:
                zinit.add(j)
                zacc_v[j * 128:(j + 1) * 128, :] = ph
            else:
                zacc_v[j * 128:(j + 1) * 128, :] += ph
            phi_v[j * 64:(j + 1) * 64, slot * B:(slot + 1) * B] = _pk(ph.astype(bf16))
            res.append(ph)
        return res

    def half_groups(p, half):
        return lambda pos: p[(pos - half * (NV // 2)) * 8:(pos - half * (NV // 2) + 1) * 8]

    def half_pairs(half):
        return range(half * (NP // 2), (half + 1) * (NP // 2))

    def kv_prod(vt, ph, j):
        half, r = j // (NP // 2), (j % (NP // 2)) * 64
        v = jnp.concatenate([vt[(s, half)][r:r + 64] for s in range(T // B)], axis=1).astype(bf16)
        return _dot_nt(v, ph)

    eye = (lax.broadcasted_iota(jnp.int32, (DH, DH), 0)
           == lax.broadcasted_iota(jnp.int32, (DH, DH), 1)).astype(bf16)
    r_h = lax.broadcasted_iota(jnp.int32, (128, 128), 0) // DH
    c_h = lax.broadcasted_iota(jnp.int32, (128, 128), 1) // DH
    same_head = r_h == c_h

    def make_amat(g):
        a = jnp.concatenate([_dot_nt(eye, wphi_v[g * 128:(g + 1) * 128, :])] * 4, axis=0)
        amat_v[:, g * 128:(g + 1) * 128] = _pk(jnp.where(same_head, a, 0.0).astype(bf16))

    class Folder:
        def __init__(self, col0, first=0):
            self.col0, self.rows, self.mprev, self.done = col0, {}, None, first

        def tile(self, g, rows, keep=None, ties=None):
            g = _phys_group(g)
            am = amat_v[:, g * 128:(g + 1) * 128]
            if ties:
                am = _tie(keep, am, ties)
            return _dot_nt(_upk(am), wqkv_v[rows, self.col0 + g * 128:self.col0 + (g + 1) * 128])

        def fold(self, g, wt=None):
            sub = lax.broadcasted_iota(jnp.int32, (8, D), 0)
            if wt is None:
                wt = self.tile(g, slice(None))
            for hh in range(4):
                full, below, _, a = _head_groups(4 * g + hh)
                r0 = hh * DH
                ref = jnp.broadcast_to(wt[r0 + a - 1:r0 + a, :], (8, D))
                part = [(wt[r0 + 8 * i:r0 + 8 * (i + 1)] - ref) * LOG2E for i in range(4)]
                if below is not None:
                    self.rows[below] = jnp.where(sub >= a, part[0], self.mprev)
                self.mprev = part[0]
                for q, v in zip(full, part[1:]):
                    self.rows[q] = v
            new = {}
            while self.done in self.rows and self.done + 1 in self.rows:
                new[self.done] = jnp.concatenate([self.rows.pop(self.done), self.rows.pop(self.done + 1)], axis=0)
                self.done += 2
            return new

    def fold_pair(folders, g, keep=None, ties=None):
        tiles = {}
        for n, c in enumerate(range(0, HK, 128)):
            for half in range(2):
                for side in range(2):
                    t = ties[n] if ties and half == 0 and side == 0 else None
                    lo = side * HK + c
                    tiles[(half, lo)] = folders[half].tile(g + 4 * half, slice(lo, lo + 128), keep, t)
        return [folders[half].fold(g + 4 * half,
                                   jnp.concatenate([tiles[(half, lo)] for lo in range(0, D, 128)], axis=1))
                for half in range(2)]

    bestv_v[...] = jnp.full(bestv_v.shape, -jnp.inf, f32)
    besti_v[...] = lax.broadcasted_iota(jnp.int32, besti_v.shape, 0)
    h_v[0:P2, :] = jnp.zeros((P2, D), f32)
    st_v[0:B, :] = jnp.zeros((B, 256), f32)
    mom1_v[...] = jnp.zeros(mom1_v.shape, f32)

    def wait_all(cps):
        for cp in cps:
            cp.wait()

    def amats(c):
        for g0, n in _PSTAGES[c]:
            for g in range(g0, g0 + n):
                make_amat(g)

    wait_all([cp_wr] + cp_p[0])
    amats(0)
    wr = wr_v[0:8, :].astype(f32)
    wc = wr - jnp.sum(jnp.sum(wr, axis=0, keepdims=True), axis=1, keepdims=True) * (1.0 / D)
    wrb_v[...] = jnp.concatenate([jnp.broadcast_to(wc[j:j + 1, :], (8, 128)) for j in range(8)], axis=1)
    num_v[0:P2, :] = jnp.zeros((P2, 128), f32)

    cp_x0.wait()
    ln1(x_v, 0, xs_v, 0, T0, plain=True)
    xb = [load_xn(s) for s in range(2)]
    logits = [{}, {}]
    finished = [set(), set()]
    fk, slabs = (Folder(D), Folder(D, NV // 2)), {}
    defer, queue = [False], []

    def absorb(new):
        for pos, slab in new.items():
            wtk_v[pos * 4:pos * 4 + 8, :] = _pk(slab.astype(bf16))
            slabs[pos] = slab
        for pos in sorted(slabs):
            if pos < NV // 2 and pos + NV // 2 in slabs:
                store_combos(wsk_v, pos * 4, slabs.pop(pos), slabs.pop(pos + NV // 2))

    def k_finish(s, hold=0):
        ready = [j for j in range(NP) if j not in finished[s] and _pair_need(j) in logits[s]]
        ready = ready[:len(ready) - hold]
        if defer[0]:
            queue.extend((logits[s].__getitem__, [j], s) for j in ready)
        else:
            k_side(logits[s].__getitem__, ready, s)
        finished[s].update(ready)

    def k_chunk(s, keep=None, early=(), late=(), hold=0):
        todo = [q for half in range(2) for q in range(half * (NV // 2), fk[half].done) if q not in logits[s]]
        runs = [[q for q in todo if q < NV // 2], [q for q in todo if q >= NV // 2]]
        lhs = jnp.concatenate([wtk_v[r[0] * 4:(r[-1] + 1) * 4, :] for r in runs if r], axis=0)
        ties = piece_ties(early, lhs.shape[0])
        ties.update(piece_ties(late, lhs.shape[0], col=HK))
        if ties:
            lhs = _tie(keep, lhs, ties)
        p = _dot_nt(_upk(lhs), xb[s])
        for n, q in enumerate(todo):
            logits[s][q] = p[n * 8:(n + 1) * 8]
        k_finish(s, hold)
        return p

    wait_all(cp_k[0])
    for new in fold_pair(fk, 0):
        absorb(new)
    k_chunk(0)
    k_chunk(1, hold=1)

    wait_all(cp_p[1] + cp_k[1])
    k_finish(1)
    for new in fold_pair(fk, 1):
        absorb(new)
    absorb(fk[0].fold(2))
    amats(1)
    k_chunk(0)
    k_chunk(1, hold=2)

    wait_all(cp_k[2] + [cp_x1])
    defer[0] = True
    keep = flag_s[0] > 0
    absorb(fk[1].fold(6))
    new = fold_pair(fk, 3)
    late = list(new[0].values())[-1][:, 384:512]
    for n in new:
        absorb(n)
    pieces = ln1(x_v, T0, xs_v, T0, T0, [0]) + ln1(x_v, T0, xs_v, T0, T0, [1, 2], keep, [late, late])
    p = k_chunk(0, keep, (), pieces[:2])
    rows = [k * p.shape[0] // 5 // 16 * 16 for k in range(5)]
    pieces += ln1(x_v, T0, xs_v, T0, T0, range(3, 8), keep, [p[r:r + R] for r in rows])
    k_chunk(1, keep, pieces[2:3], pieces[3:])

    def k_emit1(half, blk, val):
        if half != blk:
            k_side(half_groups(val, half), half_pairs(half), 2 + blk)
        else:
            queue.extend((half_groups(val, half), [j], 2 + blk) for j in half_pairs(half))

    def run_queue(n, res):
        deps = []
        for k in range(min(n, len(queue))):
            r = k * res.shape[0] // n // 8 * 8
            v = _vregs(k_side(*queue.pop(0), keep=keep, anchor=res[r:r + 8])[0])
            deps.append([_or_all(v[q::4]) for q in range(4)])
        return deps

    kwork = {}

    def k_after(m, res):
        if m in (0, 2):
            kwork[m + 1] = run_queue(4, res)

    def v_prep(lo, hi):
        for rb in range(lo, hi, 128):
            for c in range(0, HK, 128):
                raw = [wqkv_v[side * HK + c:side * HK + c + 128,
                              2 * D + half * HK + rb:2 * D + half * HK + rb + 128].T
                       for half in range(2) for side in range(2)]
                blocks = [t.astype(f32) for t in raw]
                for n, spec in enumerate(_SA):
                    t = raw[spec[0]] if spec[1] is None else _combo(blocks, spec).astype(bf16)
                    wsv_v[rb // 2:rb // 2 + 64, n * HK + c:n * HK + c + 128] = _pk(t)

    VS = HK // 2

    def k_before(m):
        if m == 5:
            cp_wv.wait()
            cp_x2.wait()
            v_prep(0, VS)

    sproj(wsk_v, xs_v, 1, k_emit1, keep, kwork, k_before, k_after)

    def ln_anchored(xg, src, xd, dst, k, n, keep, res):
        which = list(range(k * 8 // n, (k + 1) * 8 // n))
        rows = [a * HK // len(which) // 16 * 16 for a in range(len(which))]
        pcs = ln1(xg, src, xd, dst, P2, which, keep, [res[r:r + R] for r in rows])
        return [[]] * (3 - len(pcs)) + pcs

    vt, parts = {}, {}
    wsv = wsv_v.at[pl.ds(0, D // 4)]
    work = {0: {}, 1: {}, 2: {}}

    def v_after(q):
        def after(m, res):
            t = 7 * q + m
            u = t + 1
            if 3 <= t < 13:
                work[u // 7][u % 7] = run_queue(-(-len(queue) // (13 - t)), res)
            elif 13 <= t < 20:
                work[u // 7][u % 7] = ln_anchored(x_v, T, xs_v, T, t - 13, 7, keep, res)
        return after

    sealed(wsv_v)
    v_prep(VS, HK)
    zero = pl.multiple_of(flag_s[1], 8)
    for q, lo in enumerate((0, zero + VS // 2)):
        sproj(wsv_v.at[pl.ds(lo, VS // 2)], xs_v, 0,
              lambda half, blk, val: parts.setdefault((blk, half), []).append(val), keep, work[q], None, v_after(q))
    vt.update({k: jnp.concatenate(v, axis=0) for k, v in parts.items()})
    sproj(wsv_v.at[pl.ds(zero, D // 4)], xs_v, 1, lambda half, blk, val: vt.__setitem__((2 + blk, half), val),
          keep, work[2], None, v_after(2))
    assert not queue
    xjobs = dot_jobs(x_v, num_v.at[pl.ds(P2, T)], range(0, T, R), keep)
    phi_m = sealed(phi_v)
    for j in range(NP):
        prod = kv_prod(vt, _upk(phi_m[j * 64:(j + 1) * 64, :]), j)
        kvacc_v[j] = prod
        if j < 11:
            run_on(xjobs[3 * j:3 * j + 3], prod)
        if j == 2:
            store_xt(1, xs_view(flag_s[1], 2), T // 4, keep, pltpu.bitcast(prod[0:8], u32))
    cp_x3.wait()
    wait_bg(0)

    def p1_body(i, c):
        @pl.when(i == 2)
        def _():
            cp_x4.wait()
            wait_bg(1)

        @pl.when(i == 3)
        def _():
            wait_bg(2)

        keep = flag_s[0] > 0
        lo = jnp.minimum((i - 1) * DCH, F - DCH)
        sv = wd_v.at[pl.ds(pl.multiple_of(lo, 16), DCH)]
        dv = wdp_v.at[pl.ds(pl.multiple_of(lo // 2, 8), DCH // 2)]
        rp = repacker([(sv, dv, r, c) for r in range(0, DCH, 16) for c in range(0, D, 128)], keep,
                      [(q, m) for q in range(2) for m in (0, 2, 4)])
        lo = jnp.minimum((i - 1) * OCH, QK - OCH)
        ov = wo_v.at[pl.ds(pl.multiple_of(lo, 16), 3 * QK + OCH)]
        od = wso_v.at[pl.ds(pl.multiple_of(lo // 2, 8), OCH // 2)]

        def k_emit(q):
            return lambda half, blk, val: k_side(half_groups(val, half), half_pairs(half), 2 * q + blk)

        vt = {}

        def v_emit(q):
            return lambda half, blk, val: vt.__setitem__((2 * q + blk, half), val)

        xd = xs_view(i, 2)
        xa = x_v.at[pl.ds(pl.multiple_of(i * T + P2, P2), P2)]
        xb = x_v.at[pl.ds(pl.multiple_of(jnp.minimum(i + 1, NT - 1) * T, T), P2)]
        wa = {}

        def wo_get(r, c):
            return lambda i0, i1, j0, j1: ov[i0 * HK + i1 * QK + r:i0 * HK + i1 * QK + r + 16,
                                             j0 * HK + j1 * QK + c:j0 * HK + j1 * QK + c + 128].astype(f32)

        wjobs = [job for r in range(0, OCH, 16) for c in (0, 128)
                 for job in combo2_jobs(od, r // 2, c, wo_get(r, c), _SB, keep)]
        assert len(wjobs) == 36 + 6 * 8
        wv = wow_v.at[pl.ds(pl.multiple_of(lo, 16), 3 * QK + OCH)]

        pjobs = dot_jobs(ov, wv, [a * QK + r for a in range(4) for r in range(0, OCH, 16)], keep)
        pjobs += dot_jobs(x_v.at[pl.ds(pl.multiple_of(i * T, T), T)],
                          num_v.at[pl.ds(pl.multiple_of(P2 + i * T, P2), T)], range(0, T, R), keep)

        def k_after(q):
            def after(m, res):
                rp[q](m, res)
                if m in (0, 2, 4):
                    k = 3 * q + m // 2
                    run_on(pjobs[k * len(pjobs) // 6:(k + 1) * len(pjobs) // 6], res, 64)
            return after

        def a_after(m, res):
            if m < 6:
                wa[m + 1] = ln_anchored(xa, 0, xd, P2, m, 6, keep, res)

        sproj(wsv, xd, 0, v_emit(0), keep, wa, None, a_after, xt_view(i))
        sproj(wsk_v, xd, 0, k_emit(0), after=k_after(0))
        sproj(wsk_v, xd, 1, k_emit(1), after=k_after(1))
        wb = spread(ln1(xb, 0, xd, T, P2), [(0, m) for m in range(1, 7)])[0]

        def b_after(m, res):
            if m:
                run_on(wjobs[36 + 8 * (m - 1):36 + 8 * m], res)

        sproj(wsv, xd, 1, v_emit(1), keep, wb, None, b_after)
        phi_m = sealed(phi_v)
        for j in range(NP):
            prod = kv_prod(vt, _upk(phi_m[j * 64:(j + 1) * 64, :]), j)
            kvacc_v[j] += prod
            if j < 12:
                run_on(wjobs[3 * j:3 * j + 3], prod)
            if j == 2:
                store_xt(i + 1, xd, T // 4, keep, pltpu.bitcast(prod[0:8], u32))
        return c

    lax.fori_loop(1, NT, p1_body, 0)

    wait_all([cp_wq] + cp_gu[0])
    keep = flag_s[0] > 0
    kv_mask = (lax.broadcasted_iota(jnp.int32, (64, 128), 0) // DH
               == (lax.broadcasted_iota(jnp.int32, (64, 128), 1) // DH) % 2)
    ties = [{} for _ in range(16)]
    for j in range(NP):
        kvj = jnp.where(kv_mask, kvacc_v[j], 0.0)
        kv_v[:, j * 128:(j + 1) * 128] = _pk(kvj.astype(bf16))
        zj = _lanes(jnp.sum(zacc_v[j * 128:(j + 1) * 128, :], axis=-1, keepdims=True))
        zacc_v[j * 128:(j + 1) * 128, :] = zj
        vals = _vregs(kvj) + _vregs(zj)
        if j + 1 < 16:
            for q in range(4):
                ties[j + 1][(32 + q * 8, 0)] = _or_all(vals[q::4])
    for c in range(0, D, 128):
        t = jnp.sum(wow_v[c:c + 128, :].T.reshape(16, 8, 128), axis=0)
        cb_v[:, c:c + 128] = _allreduce8(t[None], jnp.add)[0]
    store_xt(0, xs_v, 0)
    fq = (Folder(0), Folder(0, NV // 2))
    for g in range(4):
        new = fold_pair(fq, g, keep, ties[4 * g:4 * g + 4])
        for pos, slab in new[0].items():
            store_combos(wsq_v, pos * 4, slab, new[1][pos + NV // 2])

    pq_v = (pq0_v, pq1_v, pq2_v, pq3_v)

    def views_of(g):
        lo = g * (BPI * B)
        if not isinstance(g, int):
            lo = pl.multiple_of(lo, BPI * B)
        return ((x_v.at[pl.ds(lo, BPI * B)],)
                + tuple(ref.at[pl.ds(lo, P2 + BPI * B)] for ref in (h_v, out_v, st_v))
                + (g, num_v.at[pl.ds(lo, P2 + BPI * B)]))

    def stage_q(xd, q, first, before, after):
        def emit(half, blk, val):
            group = half_groups(val, half)
            for j in half_pairs(half):
                p, j = _pair_logits(group, j), _phys_pair(j)
                ph = _hedgehog_t(p, zacc_v[j * 128:(j + 1) * 128, :])
                pq_v[2 * q + blk][(j // 2) * 64:(j // 2 + 1) * 64, (j % 2) * B:(j % 2 + 1) * B] = _pk(ph.astype(bf16))

        sproj(wsq_v, xd, q, emit, before=before, after=after, first=first)

    oc_v = (oc0_v, oc1_v)
    on_v = (on0_v, on1_v)

    def stage_g(q):
        pq = [sealed(pq_v[2 * q + blk]) for blk in range(2)]
        for t in range(NP // 4):
            parts = [[_dot_nn(_upk(kv_v[:, j * 128:(j + 1) * 128]),
                              _upk(pq[blk][(j // 2) * 64:(j // 2 + 1) * 64, (j % 2) * B:(j % 2 + 1) * B]))
                      for blk in range(2) for j in (jj, jj + NP // 2)] for jj in (2 * t, 2 * t + 1)]
            blocks = [jnp.concatenate([a, b], axis=0) for a, b in zip(*parts)]
            for k, blk in enumerate(blocks):
                c = (k % 2) * HK + t * 128
                on_v[q][(k // 2) * B:(k // 2 + 1) * B, c:c + 128] = blk.T

    def combo_jobs(q, keep):
        def get(r, c):
            def f(i0, i1, j0, j1):
                on = on_v[q].at[pl.ds(pl.multiple_of(flag_s[1], 8), P2)]
                return on[i0 * B + i1 * 64 + r:i0 * B + i1 * 64 + r + 16,
                          j0 * HK + j1 * QK + c:j0 * HK + j1 * QK + c + 128]
            return f
        return [job for c in (0, 128) for r in range(0, 64, 16)
                for job in combo2_jobs(oc_v[q], r // 2, c, get(r, c), _SA, keep)]

    def stage_h(views, q, sched, before, emitted):
        x_g, h_g = views[0], views[1]
        oc = sealed(oc_v[q])

        def product(m):
            if before:
                before(m)
            quad = {}

            def inner(n):
                col = (7 * m + n) * QK
                res = _dot_nn(_upk(oc[0:B // 4, col:col + QK]), _upk(wso_v[:, col:col + QK]))
                mine = sched.pop(49 * q + 7 * m + n, [])
                if mine:
                    run_on(mine, res)
                return res

            _strassen(inner, quad.__setitem__)
            return jnp.concatenate([jnp.concatenate([quad[0], quad[1]], axis=1),
                                    jnp.concatenate([quad[2], quad[3]], axis=1)], axis=0)

        def emit(k, val):
            blk, half = k // 2, k % 2
            s = 2 * q + blk
            cols = slice(half * HK, (half + 1) * HK)
            h = x_g[s * B:(s + 1) * B, cols].astype(f32) + val
            h_g[(s + 2) * B:(s + 3) * B, cols] = h
            emitted(blk, half, h)

        _strassen(product, emit)

    def num_jobs(views, q, keep):
        def job(r):
            def run(anchor):
                on = on_v[q].at[pl.ds(pl.multiple_of(flag_s[1], 8), P2)]
                rows = slice((2 * q + 2) * B + r, (2 * q + 2) * B + r + R)
                o = on[r:r + R, :]
                o = jnp.concatenate([jnp.where(keep, o[:, :128], anchor), o[:, 128:]], axis=1)
                t = _lane_dot(o, cb_v) + views[5][rows, :]
                views[5][rows, :] = _lanes(jnp.sum(t, axis=-1, keepdims=True))
            return run
        return [job(r) for r in range(0, P2, R)]

    def moments(st, mom, k, h, keep=None, anchor=None):
        first = 'h0' not in st
        if first:
            st['h0'] = h[:, 0:128]
            acc = None
        else:
            prev = mom.at[pl.ds(pl.multiple_of(flag_s[1], B), B)][k * R:(k + 1) * R, :]
            acc = [prev[:, n * 128:(n + 1) * 128] for n in range(2)]
        h0 = st['h0'] if anchor is None else jnp.where(keep, st['h0'], anchor)
        for c in range(128 if first else 0, HK, 128):
            d = h[:, c:c + 128] - h0
            new = (d, d * d)
            acc = new if acc is None else [a + b for a, b in zip(acc, new)]
        if first:
            mom[k * R:(k + 1) * R, :] = jnp.concatenate(
                list(acc) + [_lanes(jnp.mean(h0, axis=-1, keepdims=True))], axis=1)
            return None
        s1, s2 = acc
        c0 = prev[:, 256:384]
        g0 = st['h0'] - c0
        t1 = s1 + 8.0 * g0
        return t1, s2 + g0 * (s1 + t1), c0

    def stats(views, s, k, part, valid=None):
        st_g, g = views[3], views[4]
        sl = slice(k * R, (k + 1) * R)
        rows = slice((s + 2) * B + k * R, (s + 2) * B + (k + 1) * R)
        mu = _lanes(jnp.sum(part[0], axis=-1, keepdims=True)) * (1.0 / D)
        m2 = _lanes(jnp.sum(part[1], axis=-1, keepdims=True)) * (1.0 / D)
        rs = lax.rsqrt(jnp.maximum(m2 - mu * mu, 0.0) + LN_EPS)
        st_g[rows, :] = jnp.concatenate([rs, (mu + part[2]) * rs], axis=1)
        r = views[5][rows, :] * rs
        if valid is not None:
            r = jnp.where(valid, r, -jnp.inf)
        idx = lax.broadcasted_iota(jnp.int32, (R, 128), 0) + ((g * BPI + s) * B + k * R)
        bv = bestv_v[sl, :]
        better = r > bv
        bestv_v[sl, :] = jnp.where(better, r, bv)
        besti_v[sl, :] = jnp.where(better, idx, besti_v[sl, :])

    def out_jobs(views, s, keep):
        h_g, out_g, st_g = views[1], views[2], views[3]

        def job(k):
            def run(anchor):
                rows = slice((s + 2) * B + k * R, (s + 2) * B + (k + 1) * R)
                hk = h_g[rows, :]
                sk = st_g[rows, :]
                a = 1.0 + jnp.where(keep, sk[:, 0:128], anchor)
                o = [hk[:, c * 128:(c + 1) * 128] * a - sk[:, 128:256] for c in range(D // 128)]
                out_g[rows, :] = jnp.concatenate(o, axis=1).astype(bf16)
            return run
        return [job(k) for k in range(B // R)]

    def late_stats(views, s, k, keep=None, anchor=None, valid=None):
        r0 = (s + 2) * B + k * R
        blk = s % 2
        c0, c1 = (0, HK) if blk else (HK, 0)
        st = {'h0': views[1][r0:r0 + R, c0:c0 + 128]}
        part = moments(st, (mom0_v, mom1_v)[blk], k, views[1][r0:r0 + R, c1:c1 + HK], keep, anchor)
        stats(views, s, k, part, valid)

    def p2_body(i, c):
        b0 = i * BPI
        keep = flag_s[0] > 0
        cur = views_of(i)
        n = D // NI
        jobs = []
        for src, dst in ((wg_v, wgp_v), (wu_v, wup_v)):
            sv = src.at[pl.ds(pl.multiple_of(i * n, n), n)]
            dv = dst.at[pl.ds(pl.multiple_of(i * (n // 2), n // 2), n // 2)]
            jobs += [(sv, dv, r, cc) for r in range(0, n, 16) for cc in range(0, NM, 128)]
        rp, _ = repacker(jobs, keep, [(0, 0), (0, 2), (0, 4)])

        def q0_after(m, res):
            rp(m, res)
            if m == 0:
                run_on([lambda a, k=k: late_stats(cur, -1, k, keep, a, i > 0) for k in range(B // R)], res, 0, 400)

        cj = combo_jobs(0, keep)

        def q1_after(m, res):
            if m in (2, 4):
                run_on(cj[(m // 4) * 28:(m // 4 + 1) * 28], res, 32)

        stage_q(xs_view(i, 1), 0, xt_view(i), None, q0_after)
        stage_q(xs_view(i, 1), 1, None, lambda m: stage_g(0) if m == 1 else None, q1_after)

        sched = {}

        def at(jobs, lo, hi):
            for k, job in enumerate(jobs):
                sched.setdefault(lo + k * (hi - lo) // len(jobs), []).append(job)

        at(out_jobs(cur, -2, keep), 3, 7)
        at(out_jobs(cur, -1, keep), 36, 44)
        at(combo_jobs(1, keep), 15, 44)
        at(num_jobs(cur, 0, keep), 20, 40)
        at(num_jobs(cur, 1, keep), 63, 79)
        state = {}
        when = {(1, False): (18, 28), (0, False): (30, 40), (0, True): (44, 54), (1, True): (54, 63),
                (3, False): (67, 77), (2, False): (79, 89), (2, True): (91, 94)}

        def emitted(q):
            def f(blk, half, h):
                s = 2 * q + blk
                second = s in state
                sts = state.setdefault(s, [{} for _ in range(B // R)])

                def job(k):
                    def run(anchor):
                        part = moments(sts[k], (mom0_v, mom1_v)[blk], k, h[k * R:(k + 1) * R], keep, anchor)
                        if second:
                            stats(cur, s, k, part)
                    return run

                if (s, second) in when:
                    at([job(k) for k in range(B // R)], *when[(s, second)])
                if second and q == 0:
                    at(out_jobs(cur, s, keep), 70 + 14 * blk, 77 + 14 * blk)
            return f

        stage_h(cur, 0, sched, lambda m: stage_g(1) if m == 1 else None, emitted(0))
        stage_h(cur, 1, sched, None, emitted(1))
        assert not sched

        @pl.when(i > 0)
        def _():
            cp_out(jnp.maximum(b0 - 2, 0), 2).start()

        cp_out(b0, 2).start()
        return c

    lax.fori_loop(0, NI, p2_body, 0)
    wait_all(cp_gu[1])
    keep = flag_s[0] > 0
    last = views_of(NI - 1)

    for k in range(B // R):
        late_stats(last, BPI - 1, k)

    bv = bestv_v[...]
    mval = jnp.max(bv, axis=0, keepdims=True)
    sel = jnp.min(jnp.where(bv == mval, besti_v[...], S - 1), axis=0, keepdims=True)
    idx = jnp.clip(sel[0, 0], 0, S - 1)
    hrow = h_v[pl.ds(P2 + idx, 1), :]
    strow = st_v[pl.ds(P2 + idx, 1), :]
    xrow = jnp.concatenate([hrow[:, c * 128:(c + 1) * 128] * strow[:, 0:128] - strow[:, 128:256]
                            for c in range(D // 128)], axis=1).astype(bf16)
    xs = jnp.broadcast_to(xrow, (16, D))
    g_first = _dot_nn(xs, _upk(wgp_v[:, 0:FC]))
    anchors = ([jnp.broadcast_to(pltpu.bitcast(sel, f32), (R, 128))] * 4
               + [jnp.broadcast_to(xrow[:, 0:128].astype(f32), (R, 128))] * 4
               + [g_first[:, (k // 2) * 128:(k // 2 + 1) * 128] for k in range(8)])
    for job, anchor in zip(out_jobs(last, BPI - 2, keep) + out_jobs(last, BPI - 1, keep), anchors):
        job(anchor)
    cp_out(NB - 2, 2).start()

    def act(g, u):
        a = g * pl.reciprocal(1.0 + jnp.exp(-g), approx=True) * u
        return jnp.concatenate([a, a], axis=0).astype(bf16)

    def down(a, lo, w):
        return _dot_nn(a, _upk(wdp_v[lo // 2:(lo + w) // 2, 0:D]))[0:8]

    xcol = jnp.broadcast_to(xrow, (128, D)).T.astype(f32)
    jobs = [(which, b) for b in range(NBV) for which in (0, 1)]
    vres, prev = {}, None
    for j0 in range(0, len(jobs), NCH):
        grp = jobs[j0:j0 + NCH]
        accs = [None] * len(grp)
        for r in range(D // 16):
            for n, (which, b) in enumerate(grp):
                w = (wg_v, wu_v)[which][r * 16:(r + 1) * 16, NM + b * 128:NM + (b + 1) * 128].astype(f32)
                t0 = w[0:8] * xcol[r * 16:r * 16 + 8]
                t1 = w[8:16] * xcol[r * 16 + 8:r * 16 + 16]
                if accs[n] is None:
                    if prev is not None:
                        t0 = jnp.where(keep, t0, prev[n % len(prev)])
                    accs[n] = t0 + t1
                else:
                    accs[n] = (accs[n] + t0) + t1
        prev = accs
        for n, job in enumerate(grp):
            vres[job] = _allreduce8(accs[n][None], jnp.add)[0]

    chunks = [(lo, min(FC, NM - lo)) for lo in range(0, NM, FC)]
    acts, y = [], None
    for k, (lo, w) in enumerate(chunks):
        g = g_first if k == 0 else _dot_nn(xs, _upk(wgp_v[:, lo:lo + w]))
        u = _dot_nn(xs, _upk(wup_v[:, lo:lo + w]))
        acts.append(act(g[0:8], u[0:8]))
        if k >= 1:
            t = down(acts[k - 1], *chunks[k - 1])
            y = t if y is None else y + t
    y = y + down(acts[-1], *chunks[-1])
    for b0, nb in ((0, 4), (4, 4), (8, 4), (12, 1)):
        g = jnp.concatenate([vres[(0, b)] for b in range(b0, b0 + nb)], axis=1)
        u = jnp.concatenate([vres[(1, b)] for b in range(b0, b0 + nb)], axis=1)
        y = y + down(act(g, u), NM + b0 * 128, nb * 128)

    gate = jnp.broadcast_to(jax.nn.sigmoid(mval), (8, 128))
    base = pl.multiple_of((idx >> 4) << 4, 16)
    rows = pl.ds(pl.multiple_of(P2 + base, 16), 16)
    h16 = h_v[rows, :]
    st16 = st_v[rows, :]
    a16 = 1.0 + st16[:, 0:128]
    m16 = st16[:, 128:256]
    hit = (lax.broadcasted_iota(jnp.int32, (16, 128), 0) + base) == idx
    res = []
    for c in range(D // 128):
        yc = y[:, c * 128:(c + 1) * 128] * gate
        yc = jnp.concatenate([yc, yc], axis=0)
        res.append(h16[:, c * 128:(c + 1) * 128] * a16 - m16 + jnp.where(hit, yc, 0.0))
    res = jnp.concatenate(res, axis=1).astype(bf16)
    for i in range(NI):
        cp_out(i * BPI, 2).wait()
        cp_out(i * BPI + 2, 2).wait()
    out_v[rows, :] = res
    fix = pltpu.make_async_copy(out_v.at[rows], out_hbm.at[pl.ds(base, 16)], sem_o.at[0])
    fix.start()
    fix.wait()


@jax.jit
def pallas_sequential_preLN__linear_kernel_hedgehog__moe_arch_mod__prompt_kernel(
    A_x: jax.Array,
    A_wqkv: jax.Array,
    A_w_phi: jax.Array,
    A_wo: jax.Array,
    B_x: jax.Array,
    B_w_r: jax.Array,
    B_w_gate: jax.Array,
    B_w_up: jax.Array,
    B_w_down: jax.Array,
):
    del B_x
    x = A_x.reshape(S, D)
    wphi = A_w_phi.reshape(H * DH, DH)
    wr = B_w_r.reshape(8, 128)
    any_spec = pl.BlockSpec(memory_space=pl.ANY)
    out = pl.pallas_call(
        _kernel,
        out_shape=jax.ShapeDtypeStruct((S, D), bf16),
        in_specs=[any_spec] * 8,
        out_specs=any_spec,
        scratch_shapes=[
            pltpu.VMEM((S, D), bf16),
            pltpu.VMEM((D, 3 * D), bf16),
            pltpu.VMEM((H * DH, DH), bf16),
            pltpu.VMEM((D, D), bf16),
            pltpu.VMEM((64, 128), bf16),
            pltpu.VMEM((D, F + 128), bf16),
            pltpu.VMEM((D, F + 128), bf16),
            pltpu.VMEM((F, D), bf16),
            pltpu.VMEM((PR, D), u32),
            pltpu.VMEM((PR // 2, 7 * HK), u32),
            pltpu.VMEM((PR // 2, 7 * HK), u32),
            pltpu.VMEM((D // 4 + 8, 7 * HK), u32),
            pltpu.VMEM((QK // 2, 49 * QK), u32),
            pltpu.VMEM((F // 2, D + 128), u32),
            pltpu.VMEM((D // 2, NM), u32),
            pltpu.VMEM((D // 2, NM), u32),
            pltpu.VMEM((64, 8 * 128), u32),
            pltpu.VMEM((T0 // 2, D), u32),
            pltpu.VMEM(((S + T) // 4, 7 * HK), u32),
            pltpu.VMEM(((NT + 1) * (HK // 2), B), u32),
            pltpu.VMEM((NP, 64, 128), f32),
            pltpu.VMEM((2 * D, 128), f32),
            pltpu.VMEM((32, NP * 128), u32),
            pltpu.VMEM((D + 8, T), u32),
            pltpu.VMEM((D // 2 + 16, 2 * B), u32),
            pltpu.VMEM((D // 2 + 16, 2 * B), u32),
            pltpu.VMEM((D // 2 + 16, 2 * B), u32),
            pltpu.VMEM((D // 2 + 16, 2 * B), u32),
            pltpu.VMEM((B // 4 + 16, 49 * QK), u32),
            pltpu.VMEM((B // 4 + 16, 49 * QK), u32),
            pltpu.VMEM((P2, D), f32),
            pltpu.VMEM((P2, D), f32),
            pltpu.VMEM((P2 + S, D), f32),
            pltpu.VMEM((P2 + S, 256), f32),
            pltpu.VMEM((B, 384), f32),
            pltpu.VMEM((B, 384), f32),
            pltpu.VMEM((P2 + S, D), bf16),
            pltpu.VMEM((8, D), f32),
            pltpu.VMEM((8, D), f32),
            pltpu.VMEM((D, 128), f32),
            pltpu.VMEM((P2 + S, 128), f32),
            pltpu.VMEM((B, 128), f32),
            pltpu.VMEM((B, 128), jnp.int32),
            pltpu.SMEM((2,), jnp.int32),
            pltpu.SemaphoreType.DMA((_NSEM_IN,)),
            pltpu.SemaphoreType.DMA((1,)),
        ],
        compiler_params=pltpu.CompilerParams(vmem_limit_bytes=120 * 1024 * 1024,
                                             disable_bounds_checks=True,
                                             disable_semaphore_checks=True),
        name="hedgehog_mod",
    )(x, A_wqkv, wphi, A_wo, wr, B_w_gate, B_w_up, B_w_down)
    return out.reshape(1, S, D)
```
